```python
import jax
import jax.numpy as jnp

def _softmax(x, axis=-1):
    return jax.nn.softmax(x, axis=axis)

def _gelu(x):
    return jax.nn.gelu(x, approximate=True)

def _silu(x):
    return jax.nn.silu(x)

def _sigmoid(x):
    return jax.nn.sigmoid(x)

def _layernorm(x, axis=-1, eps=1e-05):
    m = jnp.mean(x, axis=axis, keepdims=True)
    v = jnp.var(x, axis=axis, keepdims=True)
    return (x - m) / jnp.sqrt(v + eps)

def _scatter_add(tgt, idx, src, axis=0):
    return tgt.at[idx].add(src)

def _segment_sum(src, seg, n):
    return jax.ops.segment_sum(src, seg, n)

class _Rng:

    def __init__(self, key):
        self._k = key

    def _next(self):
        self._k, sub = jax.random.split(self._k)
        return sub

    def normal(self, shape):
        return jax.random.normal(self._next(), shape, dtype=jnp.bfloat16)

    def randint(self, lo, hi, shape):
        return jax.random.randint(self._next(), shape, lo, hi, dtype=jnp.int32)

    def uniform(self, shape, lo=0.0, hi=1.0):
        return jax.random.uniform(self._next(), shape, jnp.bfloat16, lo, hi)

    def permutation(self, n):
        return jax.random.permutation(self._next(), n)
kernel_name = 'adaLN_cond__ssm_conv_h3__mixer_s_mlp__prompt'

def setup_inputs():
    _rng = _Rng(jax.random.key(int.from_bytes(__import__("os").urandom(4), "little")))
    _w = lambda a: (lambda t: t.astype(jnp.bfloat16) if jnp.issubdtype(t.dtype, jnp.floating) else t)(jnp.asarray(a))

    def _A_setup():
        B, S, D = (1, 2048, 640)
        ks = 4
        return {'q': _w((lambda *s: _rng.normal(s) * 0.05)(B, S, D)), 'k': _w((lambda *s: _rng.normal(s) * 0.05)(B, S, D)), 'v': _w((lambda *s: _rng.normal(s) * 0.05)(B, S, D)), 'shift_k': _w((lambda *s: _rng.normal(s) * 0.05)(D, ks) * 0.5), 'ssm_k': _w((lambda *s: _rng.normal(s) * 0.05)(D, S) * (1.0 / S ** 0.5)), 'ssm_D': _w((lambda *s: _rng.normal(s) * 0.05)(D))}
    _A_in = _A_setup()

    def _B_setup():
        B, S, D, F = (1, 2048, 640, 1728)
        return {'x': _w((lambda *s: _rng.normal(s) * 0.05)(B, S, D)), 'w1': _w((lambda *s: _rng.normal(s) * 0.05)(D, D) * D ** (-0.5)), 'w2': _w((lambda *s: _rng.normal(s) * 0.05)(D, D) * D ** (-0.5)), 'w3': _w((lambda *s: _rng.normal(s) * 0.05)(D, F) * D ** (-0.5)), 'w4': _w((lambda *s: _rng.normal(s) * 0.05)(F, D) * F ** (-0.5))}
    _B_in = _B_setup()
    return {'A_q': _A_in['q'], 'A_k': _A_in['k'], 'A_v': _A_in['v'], 'A_shift_k': _A_in['shift_k'], 'A_ssm_k': _A_in['ssm_k'], 'A_ssm_D': _A_in['ssm_D'], 'B_x': _B_in['x'], 'B_w1': _B_in['w1'], 'B_w2': _B_in['w2'], 'B_w3': _B_in['w3'], 'B_w4': _B_in['w4'], 'c': _w((lambda *s: _rng.normal(s) * 0.05)(1, 640)), 'w_mod': _w((lambda *s: _rng.normal(s) * 0.05)(640, 6 * 640) * 640 ** (-0.5))}

def reference(A_q, A_k, A_v, A_shift_k, A_ssm_k, A_ssm_D, B_x, B_w1, B_w2, B_w3, B_w4, c, w_mod):

    def _A_ref(q, k, v, shift_k, ssm_k, ssm_D):
        B, S, D = q.shape
        ks = shift_k.shape[-1]
        k_pad = jnp.pad(k, ((0, 0), (ks - 1, 0), (0, 0)))
        k_shift = jnp.zeros_like(k)
        for t in range(ks):
            k_shift = k_shift + k_pad[:, t:t + S, :] * shift_k[:, ks - 1 - t][None, None, :]
        kv = k_shift * v
        L = 2 * S
        kv_pad = jnp.pad(kv, ((0, 0), (0, S), (0, 0)))
        kf_pad = jnp.pad(ssm_k, ((0, 0), (0, S)))
        kv_f = (lambda x, axes=(-2, -1): jnp.fft.rfft2(x.astype(jnp.float32), axes=axes))(kv_pad[:, None, :, :], axes=(1, 2))
        kf_f = (lambda x, axes=(-2, -1): jnp.fft.rfft2(x.astype(jnp.float32), axes=axes))(kf_pad[:, None, :], axes=(1, 2))
        kf_f = (lambda x, *d: x.transpose(*d))(kf_f, 1, 2, 0)
        y_f = kv_f * kf_f[None, :, :, :]
        y = (lambda x, s, axes=(-2, -1): jnp.fft.irfft2(x, s=s, axes=axes).astype(jnp.bfloat16))(y_f, (1, L), axes=(1, 2))[:, 0, :S, :]
        y = y + kv * ssm_D[None, None, :]
        return q * y

    def _B_ref(x, w1, w2, w3, w4):
        B, S, D = x.shape
        h = _gelu(_layernorm(x, axis=-1) @ w1)
        c = D // 4
        g0 = jnp.pad(h[:, :, 0 * c:1 * c], ((0, 0), (1, 0), (0, 0)))[:, :S, :]
        g1 = jnp.pad(h[:, :, 1 * c:2 * c], ((0, 0), (0, 1), (0, 0)))[:, 1:, :]
        g2 = jnp.pad(h[:, :, 2 * c:3 * c], ((0, 0), (2, 0), (0, 0)))[:, :S, :]
        g3 = jnp.pad(h[:, :, 3 * c:], ((0, 0), (0, 2), (0, 0)))[:, 2:, :]
        hs = jnp.concatenate([g0, g1, g2, g3], axis=-1) @ w2
        x1 = x + hs
        h2 = _gelu(_layernorm(x1, axis=-1) @ w3) @ w4
        return x1 + h2
    x = A_q
    mod = (_silu(c) @ w_mod).reshape(c.shape[0], 6, 1, -1)
    sa, ca, ga, sb, cb, gb = (mod[:, 0].copy(), mod[:, 1].copy(), mod[:, 2].copy(), mod[:, 3].copy(), mod[:, 4].copy(), mod[:, 5].copy())
    h = _layernorm(x, axis=-1) * (1 + ca) + sa
    x = x + ga * _A_ref(h, A_k, A_v, A_shift_k, A_ssm_k, A_ssm_D)
    h = _layernorm(x, axis=-1) * (1 + cb) + sb
    x = x + gb * _B_ref(h, B_w1, B_w2, B_w3, B_w4)
    return x
```

```python
import functools
import numpy as np
import jax
import jax.numpy as jnp
from jax import lax
from jax.experimental import pallas as pl
from jax.experimental.pallas import tpu as pltpu

S, D, F = 2048, 640, 1728
T = 256
H = T // 2
NB = S // T
OFF = 16
HPAD = 32
EPS = 1e-5
F32, BF16, U32 = jnp.float32, jnp.bfloat16, jnp.uint32
G_C1 = 0.044715 * float(np.sqrt(2.0 / np.pi))
G_C2 = float(np.sqrt(2.0 / np.pi))
G_A = G_C1 ** (1.0 / 3.0)
G_B = G_C2 / G_A
G_POST = 0.5 / G_A


def _dft(shape, f_axis, tau):
    r = lax.broadcasted_iota(jnp.int32, shape, f_axis)
    l = lax.broadcasted_iota(jnp.int32, shape, 1 - f_axis)
    im = r >> 7
    f = r & 127
    fp = ((f & 63) << 1) | (f >> 6)
    p = ((2 * fp + 1) * tau(l) + 256 * im) & 1023
    return jnp.cos(p.astype(F32) * (np.pi / 512.0))


def _ln(x, scale=None):
    m = jnp.sum(x, axis=-1, keepdims=True) * (1.0 / D)
    xc = x - m
    v = jnp.sum(xc * xc, axis=-1, keepdims=True) * (1.0 / D)
    r = lax.rsqrt(v + EPS)
    if scale is not None:
        r = r * scale
    return xc * r


def _gelu2(x):
    u = x * (x * x + G_B)
    return x * (1.0 + jnp.tanh(u))


def _lo(w):
    return pltpu.bitcast(w << 16, F32)


def _hi(w):
    return pltpu.bitcast(w & jnp.uint32(0xFFFF0000), F32)


def _dot(a, b):
    return jnp.dot(a, b, preferred_element_type=F32)


def _dot_nt(a, b):
    return lax.dot_general(a, b, (((1,), (1,)), ((), ())), preferred_element_type=F32)


def kernel(q_hbm, k_hbm, v_hbm, sh_ref, ssm_hbm, sd_ref, w1_hbm, w2_hbm, w3t_hbm, w4_hbm, c_ref, wm_hbm,
           o_hbm,
           q_v, k_v, v_v, ssm_v, w1_v, w2_v, w3t_v, w4_v, wm_v, o_v,
           fue, fuo, fke, fko, ge, go, mod_v, kf, uf, z_v, x_v, hb_v, h1_v,
           sem_blk, sem_w, sem_o):
    def cp_blk(s):
        return (pltpu.make_async_copy(k_hbm.at[pl.ds(s * T, T)], k_v.at[pl.ds(16 + s * T, T)], sem_blk.at[0, s]),
                pltpu.make_async_copy(v_hbm.at[pl.ds(s * T, T)], v_v.at[pl.ds(s * T, T)], sem_blk.at[1, s]),
                pltpu.make_async_copy(q_hbm.at[pl.ds(s * T, T)], q_v.at[pl.ds(s * T, T)], sem_blk.at[2, s]))
    cp_ssm = pltpu.make_async_copy(ssm_hbm, ssm_v, sem_w.at[0])
    cp_wm = pltpu.make_async_copy(wm_hbm, wm_v, sem_w.at[1])
    cp_w1 = pltpu.make_async_copy(w1_hbm, w1_v, sem_w.at[2])
    cp_w2 = pltpu.make_async_copy(w2_hbm, w2_v, sem_w.at[3])
    cp_w3 = pltpu.make_async_copy(w3t_hbm, w3t_v, sem_w.at[4])
    cp_w4 = pltpu.make_async_copy(w4_hbm, w4_v, sem_w.at[5])

    cp_ssm.start()
    for cp in cp_blk(0):
        cp.start()
    cp_wm.start()
    cp_w1.start()
    for cp in cp_blk(1):
        cp.start()
    cp_w2.start()
    cp_w3.start()
    cp_w4.start()
    for s in range(2, NB):
        for cp in cp_blk(s):
            cp.start()

    fue[...] = _dft((T, H), 0, lambda l: 2 * l).astype(BF16)
    fuo[...] = _dft((T, H), 0, lambda l: 2 * l + 1).astype(BF16)
    ge[...] = _dft((H, T), 1, lambda l: 2 * l).astype(BF16)
    go[...] = _dft((H, T), 1, lambda l: 2 * l + 1).astype(BF16)
    tau_b = lambda l: H + ((l + (H - 1)) & (H - 1))
    fke[...] = (_dft((T, H), 0, lambda l: jnp.where((l & 1) == 0, l, tau_b(l))) * (1.0 / T)).astype(BF16)
    fko[...] = (_dft((T, H), 0, lambda l: jnp.where((l & 1) == 1, l, tau_b(l))) * (1.0 / T)).astype(BF16)
    k_v[0:16, :] = jnp.zeros((16, D), BF16)
    h1_v[0:HPAD, :] = jnp.zeros((HPAD, D), BF16)
    h1_v[HPAD + S:HPAD + S + 16, :] = jnp.zeros((16, D), BF16)
    x_v[0:OFF, :] = jnp.zeros((OFF, D), F32)
    hb_v[0:OFF, :] = jnp.zeros((OFF, D), F32)
    kf[NB] = jnp.zeros((2 * T, D), F32)

    cp_ssm.wait()
    lane_even = (lax.broadcasted_iota(jnp.int32, (D // 2, H), 1) & 1) == 0
    prev = None
    for m in range(NB):
        a = pltpu.bitcast(ssm_v[:, m * T:m * T + H], U32)
        b = pltpu.roll(pltpu.bitcast(ssm_v[:, m * T + H:(m + 1) * T], U32), 1, 1)
        xe = pltpu.bitcast(jnp.where(lane_even, a, b), BF16)
        xo = pltpu.bitcast(jnp.where(lane_even, b, a), BF16)
        e = _dot_nt(fke[...], xe)
        o = _dot_nt(fko[...], xo)
        cur = (e + o, e - o)
        for h in range(2):
            cr, ci = cur[h][:H], cur[h][H:]
            if prev is None:
                kf[m, h * T:h * T + H] = cr + sd_ref[...].astype(F32) * (1.0 / T)
                kf[m, h * T + H:(h + 1) * T] = ci
            else:
                pr, pi = prev[h][:H], prev[h][H:]
                kf[m, h * T:h * T + 64] = cr[:64] - pi[:64]
                kf[m, h * T + 64:h * T + H] = cr[64:] + pi[64:]
                kf[m, h * T + H:h * T + H + 64] = ci[:64] + pr[:64]
                kf[m, h * T + H + 64:(h + 1) * T] = ci[64:] - pr[64:]
        prev = cur

    cp_wm.wait()
    c = c_ref[...].astype(F32)
    sc = (c * (1.0 / (1.0 + jnp.exp(-c)))).astype(BF16)
    mod = _dot(jnp.broadcast_to(sc, (16, D)), wm_v[...])[0:8]
    mod_v[...] = mod
    mod_v[:, D:2 * D] = mod[:, D:2 * D] + 1.0
    mod_v[:, 4 * D:5 * D] = mod[:, 4 * D:5 * D] + 1.0

    def modp(i):
        return mod_v[0:1, i * D:(i + 1) * D]

    def stage_a(s, npairs):
        r0 = s * T if isinstance(s, int) else pl.multiple_of(s * T, T)
        wk = pltpu.bitcast(k_v[pl.ds(r0, T + 16), :], U32)
        w0 = wk[8:]
        w1 = pltpu.roll(wk, 1, 0)[8:]
        w2 = pltpu.roll(wk, 2, 0)[8:]
        sh = sh_ref[...].astype(F32)
        s0, s1, s2, s3 = sh[0:1], sh[1:2], sh[2:3], sh[3:4]
        ke, ko, ke1, ko1, ko2 = _lo(w0), _hi(w0), _lo(w1), _hi(w1), _hi(w2)
        wv = pltpu.bitcast(v_v[pl.ds(r0, T), :], U32)
        kve = ((s0 * ke + s1 * ko1) + (s2 * ke1 + s3 * ko2)) * _lo(wv)
        kvo = ((s0 * ko + s1 * ke) + (s2 * ko1 + s3 * ke1)) * _hi(wv)
        e = _dot(fue[...], kve.astype(BF16))
        o = _dot(fuo[...], kvo.astype(BF16))
        uf[s, 0:T] = e + o
        uf[s, T:2 * T] = e - o
        idx = []
        for t in range(npairs):
            if isinstance(s, int):
                idx.append((t, s - t))
            else:
                ok = t <= s
                idx.append((jnp.where(ok, t, NB), jnp.where(ok, s - t, 0)))
        CH = 16
        for rc in range(0, H, CH):
            zz = []
            for h in range(2):
                zr = zi = None
                for (mi, ji) in idx:
                    kr = kf[mi, pl.ds(h * T + rc, CH), :]
                    ki = kf[mi, pl.ds(h * T + H + rc, CH), :]
                    ur = uf[ji, pl.ds(h * T + rc, CH), :]
                    ui = uf[ji, pl.ds(h * T + H + rc, CH), :]
                    tr = kr * ur - ki * ui
                    ti = kr * ui + ki * ur
                    zr = tr if zr is None else zr + tr
                    zi = ti if zi is None else zi + ti
                zz.append((zr, zi))
            z_v[rc:rc + CH] = (zz[0][0] + zz[1][0]).astype(BF16)
            z_v[H + rc:H + rc + CH] = (zz[0][1] + zz[1][1]).astype(BF16)
            z_v[T + rc:T + rc + CH] = (zz[0][0] - zz[1][0]).astype(BF16)
            z_v[T + H + rc:T + H + rc + CH] = (zz[0][1] - zz[1][1]).astype(BF16)
        ye = _dot(ge[...], z_v[0:T])
        yo = _dot(go[...], z_v[T:2 * T])
        y = pltpu.bitcast(pltpu.pack_elementwise([ye, yo], packed_dtype=BF16), BF16).astype(F32)
        q = q_v[pl.ds(r0, T), :].astype(F32)
        h = _ln(q) * modp(1) + modp(0)
        x = q + (h * y) * modp(2)
        hb = _ln(x) * modp(4) + modp(3)
        x_v[pl.ds(r0 + OFF, T), :] = x
        hb_v[pl.ds(r0 + OFF, T), :] = hb
        n1 = _ln(hb, G_A).astype(BF16)
        h1_v[pl.ds(r0 + HPAD, T), :] = _gelu2(_dot(n1, w1_v[...])).astype(BF16)

    def stage_b(j, rows):
        r0 = j * T if isinstance(j, int) else pl.multiple_of(j * T, T)
        nw = rows // 2
        w = pltpu.bitcast(h1_v[pl.ds(r0, rows + 32), :], U32)
        tot = nw + 16
        lane = lax.broadcasted_iota(jnp.int32, (nw, 128), 1)
        parts = []
        for t in range(5):
            wt = w[:, t * 128:(t + 1) * 128]
            wc = wt[8:8 + nw]
            wm_ = pltpu.roll(wt, 1, 0)[8:8 + nw] if t < 4 else None
            wp_ = pltpu.roll(wt, tot - 1, 0)[8:8 + nw] if t > 0 else None
            g0 = lambda: (wm_ >> 16) | (wc << 16)
            g1 = lambda: (wc >> 16) | (wp_ << 16)
            if t == 0:
                g = g0()
            elif t == 1:
                g = jnp.where(lane < 32, g0(), g1())
            elif t == 2:
                g = jnp.where(lane < 64, g1(), wm_)
            elif t == 3:
                g = jnp.where(lane < 96, wm_, wp_)
            else:
                g = wp_
            parts.append(g)
        g = pltpu.bitcast(jnp.concatenate(parts, axis=1), BF16)
        x1 = hb_v[pl.ds(r0, rows), :] + _dot(g, w2_v[...]) * G_POST
        n2 = _ln(x1, G_A).astype(BF16)
        a = _gelu2(_dot_nt(n2, w3t_v[...])).astype(BF16)
        h2 = _dot(a, w4_v[...])
        out = x_v[pl.ds(r0, rows), :] + modp(5) * (x1 + h2 * G_POST)
        o_v[pl.ds(r0, rows), :] = out.astype(BF16)

    def cp_out(j):
        if isinstance(j, int) and j == 0:
            return pltpu.make_async_copy(o_v.at[pl.ds(OFF, T - OFF)], o_hbm.at[pl.ds(0, T - OFF)], sem_o.at[0])
        if isinstance(j, int) and j == NB - 1:
            return pltpu.make_async_copy(o_v.at[pl.ds(j * T, T + OFF)], o_hbm.at[pl.ds(j * T - OFF, T + OFF)], sem_o.at[j])
        r0 = j * T if isinstance(j, int) else pl.multiple_of(j * T, T)
        r1 = j * T - OFF if isinstance(j, int) else pl.multiple_of(j * T - OFF, OFF)
        return pltpu.make_async_copy(o_v.at[pl.ds(r0, T)], o_hbm.at[pl.ds(r1, T)], sem_o.at[j])

    for cp in cp_blk(0):
        cp.wait()
    cp_w1.wait()
    stage_a(0, 1)
    cp_w2.wait()
    cp_w3.wait()
    cp_w4.wait()

    def body(s, carry):
        for cp in cp_blk(s):
            cp.wait()
        stage_b(s - 1, T)
        stage_a(s, NB)

        @pl.when(s == 1)
        def _():
            cp_out(0).start()

        @pl.when(s > 1)
        def _():
            cp_out(s - 1).start()
        return carry

    lax.fori_loop(1, NB, body, 0)
    stage_b(NB - 1, T + OFF)
    cp_out(NB - 1).start()
    for j in range(NB):
        cp_out(j).wait()


@jax.jit
def pallas_adaLN_cond__ssm_conv_h3__mixer_s_mlp__prompt_kernel(A_q, A_k, A_v, A_shift_k, A_ssm_k, A_ssm_D, B_x, B_w1, B_w2, B_w3, B_w4, c, w_mod):
    any_ = pl.BlockSpec(memory_space=pl.ANY)
    vm = pl.BlockSpec(memory_space=pltpu.VMEM)
    V = pltpu.VMEM
    out = pl.pallas_call(
        kernel,
        in_specs=[any_, any_, any_, vm, any_, vm, any_, any_, any_, any_, vm, any_],
        out_specs=any_,
        out_shape=jax.ShapeDtypeStruct((S, D), BF16),
        scratch_shapes=[
            V((S, D), BF16), V((S + 16, D), BF16), V((S, D), BF16), V((D, S), BF16),
            V((D, D), BF16), V((D, D), BF16), V((F, D), BF16), V((F, D), BF16), V((D, 6 * D), BF16),
            V((S + OFF, D), BF16),
            V((T, H), BF16), V((T, H), BF16), V((T, H), BF16), V((T, H), BF16), V((H, T), BF16), V((H, T), BF16),
            V((8, 6 * D), F32), V((NB + 1, 2 * T, D), F32), V((NB, 2 * T, D), F32), V((2 * T, D), BF16),
            V((S + OFF, D), F32), V((S + OFF, D), F32), V((HPAD + S + 16, D), BF16),
            pltpu.SemaphoreType.DMA((3, NB)), pltpu.SemaphoreType.DMA((6,)), pltpu.SemaphoreType.DMA((NB,)),
        ],
        compiler_params=pltpu.CompilerParams(vmem_limit_bytes=100 << 20),
        name="fused",
    )(A_q[0], A_k[0], A_v[0], A_shift_k.T, A_ssm_k, A_ssm_D.reshape(1, D), B_w1, B_w2, B_w3.T, B_w4, c, w_mod)
    return out[None]
```

```python
import contextlib
import heapq
import numpy as np
import jax
import jax.numpy as jnp
from jax import lax
from jax.experimental import pallas as pl
from jax.experimental.pallas import tpu as pltpu

S, D, F = 2048, 640, 1728
T = 256
H = T // 2
NB = S // T
NT = D // 128
FT = (F + 127) // 128
EPS = 1e-5
F32, BF16, U32, I32 = jnp.float32, jnp.bfloat16, jnp.uint32, jnp.int32
G_C1 = 0.044715 * float(np.sqrt(2.0 / np.pi))
G_C2 = float(np.sqrt(2.0 / np.pi))
G_A = G_C1 ** (1.0 / 3.0)
G_B = G_C2 / G_A
G_POST = 0.5 / G_A
RG = 16
NC = 4
VERBOSE = False
SCOPES = False
SLOT = 32
MS = (128, 128, 128, 128)


def _dft(shape, f_axis, tau, scale=1.0):
    r = lax.broadcasted_iota(I32, shape, f_axis)
    l = lax.broadcasted_iota(I32, shape, 1 - f_axis)
    f = r & 127
    odd = ((f & 63) << 2) | ((f >> 6) << 1) | 1
    p = odd * tau(l) + ((r >> 7) << 8)
    a = ((p + 512) & 1023) - 512
    u = (256 - jnp.abs(a)).astype(F32) * (np.pi / 512.0)
    u2 = u * u
    c = [scale, -scale / 6.0, scale / 120.0, -scale / 5040.0, scale / 362880.0, -scale / 39916800.0]
    poly = c[5]
    for ci in c[4::-1]:
        poly = poly * u2 + ci
    return (u * poly).astype(BF16)


def _ln(x, scale=1.0):
    m = jnp.sum(x, axis=-1, keepdims=True) * (1.0 / D)
    xc = x - m
    s2 = 1.0 / (scale * scale)
    v = jnp.sum(xc * xc, axis=-1, keepdims=True) * (s2 / D) + EPS * s2
    r = jnp.exp2(jnp.log(v) * float(-0.5 / np.log(2.0)))
    return xc * r


def _gelu2(x):
    u = x * (x * x + G_B)
    return x * (1.0 + jnp.tanh(u))


def _lo(w):
    return pltpu.bitcast(w << 16, F32)


def _hi(w):
    return pltpu.bitcast(w & jnp.uint32(0xFFFF0000), F32)


def _tie(x, a):
    if a is None:
        return x
    w = pltpu.bitcast(x[:, :128], U32)
    k = w.shape[0] // 8
    w = w | (a if k == 1 else jnp.concatenate([a] * k, axis=0))
    w = pltpu.bitcast(w, x.dtype)
    return w if x.shape[1] == 128 else jnp.concatenate([w, x[:, 128:]], axis=1)


def C(i, lim=D):
    return slice(i * 128, min((i + 1) * 128, lim))


class Unit:
    def __init__(self, name, tiles, epi, rows, cost, nt=False, full=True, acc=False):
        self.acc = acc
        self.name, self.tiles, self.epi, self.rows, self.cost, self.nt, self.full = name, tiles, epi, rows, cost, nt, full


class Group:
    def __init__(self, name, fns, cost, rel, dead, lat, rlat=200):
        self.name, self.fns, self.cost, self.rel, self.dead, self.lat, self.rlat = name, fns, cost, rel, dead, lat, rlat


def _plan(seq, groups):
    busy, n = [0] * 4, 0
    start, end, tiles, bars = {}, {}, [], []
    for it in seq:
        if isinstance(it, Unit):
            for _ in it.tiles:
                m = n % 4
                n += 1
                t0, t1 = busy[m], busy[m] + max(it.rows, 32)
                busy[m] = t1
                tiles.append((t0, t1, it.cost / len(it.tiles)))
                start.setdefault(it.name, t0)
                end[it.name] = max(end.get(it.name, 0), t1)
        elif it[0] == "wait":
            t = max(busy)
            busy, n = [t] * 4, 0
            start[it[1]] = end[it[1]] = t
            bars.append(t)
    total = max(busy)
    start["end"] = end["end"] = total
    ns = total // SLOT + 2
    load = np.zeros(ns)
    for t0, t1, c in tiles:
        a, b = t0 // SLOT, max(t1 // SLOT, t0 // SLOT + 1)
        load[a:b] += c / (b - a)
    win = []
    for g in groups:
        r = max(end[x] + (0 if start[x] == end[x] else g.rlat) for x in g.rel)
        d = min(start[x] for x in g.dead) - g.lat
        ok = np.zeros(ns, bool)
        ok[r // SLOT:max(d // SLOT, r // SLOT + 1)] = True
        for b in bars:
            if r < b <= d:
                ok[max((b - g.lat) // SLOT, 0):b // SLOT] = False
        win.append(np.nonzero(ok)[0])
    alloc = [np.zeros(len(w)) for w in win]
    for _ in range(60):
        for i, g in enumerate(groups):
            w = win[i]
            load[w] -= alloc[i]
            base = load[w]
            vol = g.cost * len(g.fns)
            lo, hi = base.min(), base.max() + vol
            for _ in range(50):
                mid = 0.5 * (lo + hi)
                if np.maximum(mid - base, 0).sum() > vol:
                    hi = mid
                else:
                    lo = mid
            alloc[i] = np.maximum(hi - base, 0)
            load[w] += alloc[i]
    times = []
    for i, g in enumerate(groups):
        cum = np.cumsum(alloc[i])
        ts = []
        for k in range(len(g.fns)):
            x = (k + 0.5) * cum[-1] / len(g.fns)
            j = int(np.searchsorted(cum, x))
            prev = cum[j - 1] if j else 0.0
            ts.append(win[i][j] * SLOT + SLOT * (x - prev) / max(alloc[i][j], 1e-9))
        times.append(ts)
        if VERBOSE:
            print("%8s window %6d..%6d used %6d..%6d" % (g.name, win[i][0] * SLOT, win[i][-1] * SLOT, ts[0], ts[-1]))
    if VERBOSE:
        k = 2048 // SLOT
        print("total", total, "load/cycle:", " ".join("%.1f" % (load[i:i + k].mean() / SLOT) for i in range(0, ns, k)))
    return times


def _emit(seq, groups, zero, wait):
    times = _plan(seq, groups)
    left = {}
    for it in seq:
        nm = it.name if isinstance(it, Unit) else it[1]
        left[nm] = left.get(nm, 0) + 1
    heap, pend, todo, cnt = [], {}, list(range(len(groups))), 0
    busy, n = [0] * 4, 0

    def release():
        nonlocal cnt
        for i in list(todo):
            g = groups[i]
            if all(left[x] == 0 for x in g.rel):
                todo.remove(i)
                pend[i] = len(g.fns)
                for t, fn in zip(times[i], g.fns):
                    heapq.heappush(heap, (t, cnt, i, fn))
                    cnt += 1

    def force(name):
        nonlocal heap
        for i, g in enumerate(groups):
            if name in g.dead:
                assert i not in todo, (g.name, name)
                if pend[i]:
                    if VERBOSE:
                        print("forcing", g.name, pend[i], "before", name)
                    for it in sorted(x for x in heap if x[2] == i):
                        it[3](None)
                    heap = [x for x in heap if x[2] != i]
                    heapq.heapify(heap)
                    pend[i] = 0

    for it in seq:
        if isinstance(it, Unit):
            force(it.name)
            res = []
            for mk in it.tiles:
                lhs, rhs = mk()
                dn = (((1,), (1 if it.nt else 0,)), ((), ()))
                p = lax.dot_general(lhs, rhs, dn, preferred_element_type=F32)
                res = [res[0] + p] if (it.acc and res) else res + [p]
                m = n % 4
                n += 1
                t0 = busy[m]
                busy[m] = t0 + max(it.rows, 32)
                while it.full and heap and heap[0][0] < t0 + it.rows:
                    t, _, i, fn = heapq.heappop(heap)
                    pend[i] -= 1
                    r = min(max(int(t - t0), 0), it.rows - 1) // 8 * 8
                    fn(pltpu.bitcast(p[r:r + 8], U32) & zero)
            it.epi(res)
            left[it.name] -= 1
        elif it[0] == "wait":
            force(it[1])
            wait(it[1])
            busy, n = [max(busy)] * 4, 0
            left[it[1]] -= 1
        else:
            it[2]()
            left[it[1]] -= 1
        release()
    force("end")
    assert not heap and not todo


def _sum(ps):
    acc = ps[0]
    for p in ps[1:]:
        acc = acc + p
    return acc


def _mix(a, b):
    out, k = [], 0
    for i, u in enumerate(a):
        out.append(u)
        while k < len(b) and k * len(a) < (i + 1) * len(b):
            out.append(b[k])
            k += 1
    return out


def kernel(q_hbm, k_hbm, v_hbm, sh_hbm, ssm_hbm, sd_hbm, w1_hbm, w2_hbm, w3_hbm, w4_hbm, c_hbm, wm_hbm,
           o_hbm,
           q_w, k_n, v_w, ssm_w, w1_w, w2_w, w3_w, w4_w, wm_w, o_v,
           sh_v, sd_v, c_v, zsrc, z_s, taps, mod_v, tf_w, tg_w,
           kf, kraw, uf, kv_w, zz_w, y_w, x_v, hb_v, x1_v, n1_w, n2_w, g_w, h1_v,
           sem, sem_o):
    bf = lambda r: r.bitcast(BF16)
    w1_v, w2_v, w3_v, w4_v, wm_v = bf(w1_w), bf(w2_w), bf(w3_w), bf(w4_w), bf(wm_w)
    tf_v, tg_v, kv_v, zz_v, y_v, n1_v, n2_v, g_v = (bf(tf_w), bf(tg_w), bf(kv_w), bf(zz_w), bf(y_w), bf(n1_w),
                                                    bf(n2_w), bf(g_w))
    cp = pltpu.make_async_copy
    scope = lambda nm: jax.named_scope(nm) if SCOPES else contextlib.nullcontext()

    dmas = {}

    def group(name, *mks):
        sm = sem.at[len(dmas)]
        dmas[name] = [c for mk in mks for c in mk(sm)]

    def rows(s, n=1):
        return pl.ds(s * T, n * T)

    def conv_in(s, n=1):
        return lambda sm: ([cp(ssm_hbm.at[:, rows(s, n)], bf(ssm_w).at[:, rows(s, n)], sm)]
                           + [cp(k_hbm.at[rows(s, n), C(t)], bf(k_n).at[t, pl.ds(16 + s * T, n * T)], sm) for t in range(NT)]
                           + [cp(v_hbm.at[rows(s, n)], bf(v_w).at[rows(s, n)], sm)])

    def q_in(s, n=1):
        return lambda sm: [cp(q_hbm.at[rows(s, n)], bf(q_w).at[rows(s, n)], sm)]

    def wm_in(a, b):
        return lambda sm: [cp(wm_hbm.at[:, a * D:b * D], wm_v.at[:, a * D:b * D], sm)]

    def whole(src, dst):
        return lambda sm: [cp(src, dst, sm)]

    zsrc[...] = jnp.zeros((8, 128), I32)
    group("small", lambda sm: [cp(zsrc, z_s, sm), cp(sh_hbm, sh_v, sm), cp(sd_hbm, sd_v, sm), cp(c_hbm, c_v, sm)])
    for s in range(NC):
        group("c%d" % s, conv_in(s))
    group("wma", wm_in(0, 3), q_in(0, 2))
    group("wmb", wm_in(3, 5))
    group("w1", whole(w1_hbm, w1_v))
    group("w2", q_in(2), whole(w2_hbm, w2_v))
    group("w3", whole(w3_hbm, w3_v), q_in(3))
    group("w4", whole(w4_hbm, w4_v), wm_in(5, 6), conv_in(4), q_in(4))
    group("rest", conv_in(5, NB - 5), q_in(5, NB - 5))
    for g in dmas.values():
        for c in g:
            c.start()

    def wait(name):
        with scope("wait_" + name):
            for c in dmas[name]:
                c.wait()

    tau_b = lambda l: H + ((l + (H - 1)) & (H - 1))
    tf_v[:, C(0)] = _dft((T, H), 0, lambda l: jnp.where((l & 1) == 0, l, tau_b(l)), 1.0 / T)
    tf_v[:, C(1)] = _dft((T, H), 0, lambda l: jnp.where((l & 1) == 1, l, tau_b(l)), 1.0 / T)
    tf_v[:, C(2)] = _dft((T, H), 0, lambda l: 2 * l)
    tf_v[:, C(3)] = _dft((T, H), 0, lambda l: 2 * l + 1)
    tg_v[:, 0:T] = _dft((H, T), 1, lambda l: 2 * l)
    tg_v[:, T:2 * T] = _dft((H, T), 1, lambda l: 2 * l + 1)
    k_n[:, 0:8, :] = jnp.zeros((NT, 8, 128), U32)
    h1_v[:, 0:8, :] = jnp.zeros((NT, 8, 128), F32)
    h1_v[:, 8 + S:16 + S, :] = jnp.zeros((NT, 8, 128), F32)

    wait("small")
    z = z_s[0, 0]
    zero = jnp.full((8, 128), z, I32).astype(U32)
    z8 = pl.multiple_of(z * 8, 8)
    for r in (x_v, hb_v, x1_v, n1_w, n2_w, g_w, y_w):
        r[pl.ds(z8, 8), 0:128] = jnp.zeros((8, 128), r.dtype)
    for r in (kf, kraw, uf, kv_w, zz_w, taps, mod_v):
        r[z, 0:8, 0:128] = jnp.zeros((8, 128), r.dtype)
    for r in (tf_w, tg_w):
        r[pl.ds(z8, 8), 0:128] = r[0:8, 0:128]
    sh = sh_v[...].astype(F32)
    for i in range(4):
        taps[i] = jnp.broadcast_to(sh[i:i + 1], (8, D))
    taps[4] = jnp.broadcast_to(sd_v[...].astype(F32).reshape(1, D) * (1.0 / T), (8, D))
    cf = c_v[...].astype(F32)
    silu_c = jnp.broadcast_to((cf / (1.0 + jnp.exp(-cf))).astype(BF16), (16, D))

    def mmK(m):
        def unit(n):
            W = slice(64 * n, 64 * (n + 1))
            st = []

            def ab():
                if not st:
                    st.append((lax.broadcasted_iota(I32, (64, 128), 1) & 1) == 0)
                    st.append(ssm_w[W, m * T:m * T + H])
                    st.append(pltpu.roll(ssm_w[W, m * T + H:(m + 1) * T], 1, 1))
                return st

            def te():
                ev, a, b = ab()
                return tf_v[:, C(0)], pltpu.bitcast(jnp.where(ev, a, b), BF16)

            def to():
                ev, a, b = ab()
                return tf_v[:, C(1)], pltpu.bitcast(jnp.where(ev, b, a), BF16)

            def epi(p):
                e, o = p
                for h, cur in enumerate((e + o, e - o)):
                    B = h * T
                    if m + 1 < NB:
                        kraw[m % 2, B:B + T, C(n)] = cur
                    if m == 0:
                        kf[m, B:B + H, C(n)] = cur[:H] + taps[4, 0:1, C(n)]
                        kf[m, B + H:B + T, C(n)] = cur[H:]
                    else:
                        pv = lambda a0: kraw[(m - 1) % 2, B + a0:B + a0 + 64, C(n)]
                        kf[m, B:B + 64, C(n)] = cur[0:64] - pv(H)
                        kf[m, B + 64:B + H, C(n)] = cur[64:H] + pv(H + 64)
                        kf[m, B + H:B + H + 64, C(n)] = cur[H:H + 64] + pv(0)
                        kf[m, B + H + 64:B + T, C(n)] = cur[H + 64:T] - pv(64)
            return Unit("K%d" % m, [te, to], epi, T, 200, nt=True)
        return [unit(n) for n in range(NT)]

    def kv(s):
        def mk(t, w):
            def fn(a):
                w0 = s * H + w
                ld = lambda d: k_n[t, 8 + w0 - d:8 + w0 - d + 16, :].reshape(2, 8, 128)
                c0 = _tie(k_n[t, 8 + w0:8 + w0 + 8, :], a)
                c0 = jnp.concatenate([c0, k_n[t, 16 + w0:24 + w0, :]], axis=0).reshape(2, 8, 128)
                c1, c2 = ld(1), ld(2)
                s0, s1, s2, s3 = (taps[i, :, C(t)] for i in range(4))
                ke, ko, ke1, ko1, ko2 = _lo(c0), _hi(c0), _lo(c1), _hi(c1), _hi(c2)
                wv = v_w[w0:w0 + 16, C(t)].reshape(2, 8, 128)
                kve = ((s0 * ke + s1 * ko1) + (s2 * ke1 + s3 * ko2)) * _lo(wv)
                kvo = ((s0 * ko + s1 * ke) + (s2 * ko1 + s3 * ke1)) * _hi(wv)
                kv_v[s % 2, w:w + 16, C(t)] = kve.reshape(16, 128).astype(BF16)
                kv_v[s % 2, H + w:H + w + 16, C(t)] = kvo.reshape(16, 128).astype(BF16)
            return fn
        return [mk(t, w) for t in range(NT) for w in range(0, H, 16)]

    def mmU(s):
        def unit(n):
            def epi(p):
                uf[s, 0:T, C(n)] = p[0] + p[1]
                uf[s, T:2 * T, C(n)] = p[0] - p[1]
            return Unit("U%d" % s, [lambda: (tf_v[:, C(2)], kv_v[s % 2, 0:H, C(n)]),
                                    lambda: (tf_v[:, C(3)], kv_v[s % 2, H:T, C(n)])], epi, T, 80)
        return [unit(n) for n in range(NT)]

    def mac(s):
        def chain(row, L, a):
            zr = zi = None
            for m in range(s + 1):
                kr, ki = kf[m, row:row + 8, L], kf[m, H + row:H + row + 8, L]
                ur, ui = uf[s - m, row:row + 8, L], uf[s - m, H + row:H + row + 8, L]
                if m == 0:
                    kr = _tie(kr, a)
                tr, ti = kr * ur - ki * ui, kr * ui + ki * ur
                zr, zi = (tr, ti) if zr is None else (zr + tr, zi + ti)
            return zr, zi

        def mk(t, rc):
            st = []

            def part(row, last):
                def fn(a):
                    st.append(chain(row, C(t), a))
                    if last:
                        p0, m0, p1, m1 = st
                        for q in range(2):
                            zz_v[s % 2, q * H + rc:q * H + rc + 16, C(t)] = jnp.concatenate(
                                [p0[q] + m0[q], p1[q] + m1[q]], axis=0).astype(BF16)
                            zz_v[s % 2, T + q * H + rc:T + q * H + rc + 16, C(t)] = jnp.concatenate(
                                [p0[q] - m0[q], p1[q] - m1[q]], axis=0).astype(BF16)
                return fn
            return [part(rc, False), part(T + rc, False), part(rc + 8, False), part(T + rc + 8, True)]
        return [fn for t in range(NT) for rc in range(0, H, 16) for fn in mk(t, rc)]

    def mmI(s):
        def unit(n):
            def epi(p):
                y_w[s * H:(s + 1) * H, C(n)] = pltpu.pack_elementwise([p[0] + p[1], p[2] + p[3]], packed_dtype=BF16)
            return Unit("I%d" % s, [(lambda i=i: (tg_v[:, C(i)], zz_v[s % 2, C(i), C(n)])) for i in range(4)],
                        epi, H, 48)
        return [unit(n) for n in range(NT)]

    def mod(name, a, b):
        def unit(n):
            def epi(p):
                v = [_sum(p[i * NT:(i + 1) * NT])[0:8] for i in range(b - a)]
                if a == 0:
                    mod_v[0, :, C(n)] = v[0] * v[2]
                    mod_v[1, :, C(n)] = (v[1] + 1.0) * v[2]
                elif a == 3:
                    mod_v[3, :, C(n)] = v[0]
                    mod_v[4, :, C(n)] = v[1] + 1.0
                else:
                    mod_v[5, :, C(n)] = v[0]
            return Unit(name, [(lambda i=i, k=k: (silu_c[:, C(k)], wm_v[C(k), i * D + n * 128:i * D + (n + 1) * 128]))
                               for i in range(a, b) for k in range(NT)], epi, 16, 10, full=False)
        return [unit(n) for n in range(NT)]

    def blk(j):
        return range(j * T, (j + 1) * T, RG)

    def fa(j):
        def mk(r):
            def fn(a):
                q = pltpu.bitcast(_tie(q_w[r // 2:r // 2 + 8, :], a), BF16).astype(F32).reshape(2, 8, D)
                y = y_v[r:r + RG, :].astype(F32).reshape(2, 8, D)
                x_v[r:r + RG, :] = (q + (_ln(q) * mod_v[1] + mod_v[0]) * y).reshape(RG, D)
            return fn
        return [mk(r) for r in blk(j)]

    def fb(j):
        def mk(r):
            def fn(a):
                x = _tie(x_v[r:r + RG, :], a).reshape(2, 8, D)
                hb_v[r:r + RG, :] = (_ln(x) * mod_v[4] + mod_v[3]).reshape(RG, D)
            return fn
        return [mk(r) for r in blk(j)]

    def fc(j):
        def mk(r):
            def fn(a):
                n1_v[r:r + RG, :] = _ln(_tie(hb_v[r:r + RG, :], a), G_A).astype(BF16)
            return fn
        return [mk(r) for r in blk(j)]

    def shift(j):
        SR = 64

        def mk(t, r):
            def fn(a):
                lane = lax.broadcasted_iota(I32, (SR, 128), 1)
                ld = lambda d: h1_v[t, 8 + r + d:8 + r + d + SR, :]
                if t == 0:
                    g = ld(-1)
                elif t == 1:
                    g = jnp.where(lane < 32, ld(-1), ld(1))
                elif t == 2:
                    g = jnp.where(lane < 64, ld(1), ld(-2))
                elif t == 3:
                    g = jnp.where(lane < 96, ld(-2), ld(2))
                else:
                    g = ld(2)
                if a is not None:
                    g = jnp.concatenate([_tie(g[i:i + 8], a) if i % 16 == 0 else g[i:i + 8]
                                         for i in range(0, SR, 8)], axis=0)
                g_v[r:r + SR, C(t)] = g.astype(BF16)
            return fn
        return [mk(t, j * T + r) for t in range(NT) for r in range(0, T, SR)]

    def ln2(j):
        def mk(r):
            def fn(a):
                n2_v[r:r + RG, :] = _ln(_tie(x1_v[r:r + RG, :], a), G_A).astype(BF16)
            return fn
        return [mk(r) for r in blk(j)]

    def halves(j, M):
        return [slice(r, r + M) for r in range(j * T, (j + 1) * T, M)]

    def mm1(j, M=MS[0]):
        def unit(n, R):
            def epi(p):
                h1_v[n, 8 + R.start:8 + R.stop, :] = _gelu2(p[0])
            return Unit("w1_%d" % j, [(lambda k=k: (n1_v[R, C(k)], w1_v[C(k), C(n)])) for k in range(NT)],
                        epi, M, M // 8 * 9, acc=True)
        return [unit(n, R) for n in range(NT) for R in halves(j, M)]

    def mm2(j, M=MS[1]):
        def unit(n, R):
            def epi(p):
                x1_v[R, C(n)] = hb_v[R, C(n)] + p[0] * G_POST
            return Unit("w2_%d" % j, [(lambda k=k: (g_v[R, C(k)], w2_v[C(k), C(n)])) for k in range(NT)],
                        epi, M, M // 8 * 6, acc=True)
        return [unit(n, R) for n in range(NT) for R in halves(j, M)]

    act = {}

    def mm3(j, M=MS[2]):
        def unit(n, R):
            def epi(p):
                a = _gelu2(p[0]).astype(BF16)
                for r in range(0, M, 128):
                    act[R.start + r, n] = a[r:r + 128]
            return Unit("w3_%d" % j, [(lambda k=k: (n2_v[R, C(k)], w3_v[C(n, F), C(k)])) for k in range(NT)],
                        epi, M, M // 8 * 10, nt=True, full=n < FT - 1, acc=True)
        return [unit(n, R) for n in range(FT) for R in halves(j, M)]

    outs = []

    def mm4(j, M=MS[3]):
        def lhs(R, k):
            ps = [act[r, k] for r in range(R.start, R.stop, 128)]
            return ps[0] if len(ps) == 1 else jnp.concatenate(ps, axis=0)

        def unit(n, R):
            def epi(p):
                gb = mod_v[5, 0:1, C(n)]
                o_v[R, C(n)] = (x_v[R, C(n)] + gb * (x1_v[R, C(n)] + p[0] * G_POST)).astype(BF16)
                if R.stop % T == 0:
                    if j == NB - 1:
                        outs.append(cp(o_v.at[rows(j), C(n)], o_hbm.at[rows(j), C(n)], sem_o.at[0]))
                        outs[-1].start()
                    elif n == NT - 1:
                        outs.append(cp(o_v.at[rows(j)], o_hbm.at[rows(j)], sem_o.at[0]))
                        outs[-1].start()
            return Unit("w4_%d" % j, [(lambda k=k: (lhs(R, k), w4_v[C(k, F), C(n)])) for k in range(FT)],
                        epi, M, M // 8 * 18, acc=True)
        return [unit(n, R) for n in range(NT) for R in halves(j, M)]

    W = lambda nm: [("wait", nm)]
    run = lambda fns: [("run", "run", lambda: [fn(None) for fn in fns])]

    seq, grp = [], []
    for s in range(NC):
        seq += W("c%d" % s) + (mmI(s - 2) if s >= 2 else []) + mmK(s) + mmU(s)
        grp.append(Group("kv%d" % s, kv(s), 50, ["c%d" % s], ["U%d" % s], 100))
        if s + 1 < NC:
            grp.append(Group("mac%d" % s, mac(s), 8 * s + 11, ["c%d" % (s + 1)],
                             ["c%d" % (s + 2) if s + 2 < NC else "I%d" % s], 0))
    grp.append(Group("mac%d" % (NC - 1), mac(NC - 1), 8 * NC + 3, ["U%d" % (NC - 1)], ["I%d" % (NC - 1)], 0))
    seq += mmI(NC - 2) + mmI(NC - 1)
    seq += W("wma") + mod("moda", 0, 3) + run(fa(0) + fa(1))
    seq += W("wmb") + mod("modb", 3, 5) + run(fb(0) + fc(0))
    seq += W("w1") + mm1(0) + mm1(1) + run(shift(0))
    grp.append(Group("f1", fb(1) + fc(1), 70, ["w1"], ["w1_1"], 450))
    seq += W("w2") + mm2(0) + mm1(2) + run(shift(1)) + mm2(1)
    grp.append(Group("f2", fa(2) + fb(2) + fc(2), 80, ["w2"], ["w1_2"], 450))
    grp.append(Group("ln2_0", ln2(0), 60, ["w2_0"], ["w3"], 450))
    seq += W("w3") + mm3(0) + mm1(3) + mm3(1)
    grp.append(Group("f3", fa(3) + fb(3) + fc(3), 80, ["w3"], ["w1_3"], 450))
    grp.append(Group("ln2_1", ln2(1), 60, ["w3"], ["w3_1"], 450))
    seq += W("w4") + mod("modc", 5, 6) + _mix(mm4(0), mmK(4)) + mmU(4) + mm2(2) + mm4(1)
    grp.append(Group("kv4", kv(4), 50, ["w4"], ["U4"], 450))
    seq += W("rest")
    for j in range(2, NB):
        s = j + 3
        w4 = mm4(j)
        seq += mmI(j + 2) if j + 2 < NB else []
        seq += _mix(mm3(j), mmK(s)) + mmU(s) if s < NB else mm3(j)
        if j + 2 < NB:
            seq += mm1(j + 2) + w4[:len(w4) * 2 // 5] + mm2(j + 1) + w4[len(w4) * 2 // 5:]
        elif j + 1 < NB:
            seq += mm2(j + 1) + w4
        else:
            seq += w4
        if s < NB:
            grp.append(Group("kv%d" % s, kv(s), 50, ["rest", "U%d" % (s - 2)], ["U%d" % s], 450))
    for s in range(4, NB):
        grp.append(Group("mac%d" % s, mac(s), 8 * s + 11, ["U%d" % s, "K%d" % s], ["I%d" % s], 450))
        grp.append(Group("f%d" % s, fa(s) + fb(s) + fc(s), 80, ["I%d" % s], ["w1_%d" % s], 450))
    for j in range(2, NB):
        grp.append(Group("shift%d" % j, shift(j), 14, ["w1_%d" % min(j + 1, NB - 1)], ["w2_%d" % j], 200))
        grp.append(Group("ln2_%d" % j, ln2(j), 60, ["w2_%d" % j], ["w3_%d" % j], 450))
    _emit(seq, grp, zero, wait)
    with scope("wait_out"):
        for c in outs:
            c.wait()


@jax.jit
def pallas_adaLN_cond__ssm_conv_h3__mixer_s_mlp__prompt_kernel(A_q, A_k, A_v, A_shift_k, A_ssm_k, A_ssm_D, B_x, B_w1, B_w2, B_w3, B_w4, c, w_mod):
    any_ = pl.BlockSpec(memory_space=pl.ANY)
    V = pltpu.VMEM
    out = pl.pallas_call(
        kernel,
        in_specs=[any_] * 12,
        out_specs=any_,
        out_shape=jax.ShapeDtypeStruct((S, D), BF16),
        scratch_shapes=[
            V((S // 2, D), U32), V((NT, 8 + S // 2, 128), U32), V((S // 2, D), U32), V((D // 2, S), U32),
            V((D // 2, D), U32), V((D // 2, D), U32), V((F // 2, D), U32), V((F // 2, D), U32),
            V((D // 2, 6 * D), U32), V((S, D), BF16),
            V((4, D), BF16), V((D,), BF16), V((1, D), BF16), V((8, 128), I32), pltpu.SMEM((8, 128), I32),
            V((5, 8, D), F32), V((6, 8, D), F32), V((T // 2, 4 * H), U32), V((H // 2, 2 * T), U32),
            V((NB, 2 * T, D), F32), V((2, 2 * T, D), F32), V((NB, 2 * T, D), F32),
            V((2, T // 2, D), U32), V((2, T, D), U32), V((S // 2, D), U32),
            V((S, D), F32), V((S, D), F32), V((S, D), F32),
            V((S // 2, D), U32), V((S // 2, D), U32), V((S // 2, D), U32), V((NT, S + 16, 128), F32),
            pltpu.SemaphoreType.DMA((12,)), pltpu.SemaphoreType.DMA((1,)),
        ],
        compiler_params=pltpu.CompilerParams(vmem_limit_bytes=110 << 20),
        name="fused",
    )(A_q[0], A_k[0], A_v[0], A_shift_k.T, A_ssm_k, A_ssm_D, B_w1, B_w2, B_w3.T, B_w4, c, w_mod)
    return out[None]
```

```python
import contextlib
import heapq
import numpy as np
import jax
import jax.numpy as jnp
from jax import lax
from jax.experimental import pallas as pl
from jax.experimental.pallas import tpu as pltpu

S, D, F = 2048, 640, 1728
T = 256
H = T // 2
NB = S // T
NT = D // 128
FT = (F + 127) // 128
EPS = 1e-5
F32, BF16, U32, I32 = jnp.float32, jnp.bfloat16, jnp.uint32, jnp.int32
G_C1 = 0.044715 * float(np.sqrt(2.0 / np.pi))
G_C2 = float(np.sqrt(2.0 / np.pi))
G_A = G_C1 ** (1.0 / 3.0)
G_B = G_C2 / G_A
G_POST = 0.5 / G_A
RG = 16
NC = 4
VERBOSE = False
SCOPES = False
SLOT = 32
MS = (128, 128, 128, 128)


def _unzip(p):
    return (p & -16) | ((p & 1) << 3) | ((p >> 1) & 7)


def _dft(shape, f_axis, tau, scale=1.0):
    r = lax.broadcasted_iota(I32, shape, f_axis)
    l = lax.broadcasted_iota(I32, shape, 1 - f_axis)
    if f_axis == 1:
        r = _unzip(r)
    f = r & 127
    odd = ((f & 63) << 2) | ((f >> 6) << 1) | 1
    p = odd * tau(l) + ((r >> 7) << 8)
    a = ((p + 512) & 1023) - 512
    u = (256 - jnp.abs(a)).astype(F32) * (np.pi / 512.0)
    u2 = u * u
    c = [scale, -scale / 6.0, scale / 120.0, -scale / 5040.0, scale / 362880.0, -scale / 39916800.0]
    poly = c[5]
    for ci in c[4::-1]:
        poly = poly * u2 + ci
    return (u * poly).astype(BF16)


def _ln(x, scale=1.0):
    m = jnp.sum(x, axis=-1, keepdims=True) * (1.0 / D)
    xc = x - m
    s2 = 1.0 / (scale * scale)
    v = jnp.sum(xc * xc, axis=-1, keepdims=True) * (s2 / D) + EPS * s2
    r = jnp.exp2(jnp.log(v) * float(-0.5 / np.log(2.0)))
    return xc * r


def _gelu2(x):
    u = x * (x * x + G_B)
    return x * (1.0 + jnp.tanh(u))


def _lo(w):
    return pltpu.bitcast(w << 16, F32)


def _hi(w):
    return pltpu.bitcast(w & jnp.uint32(0xFFFF0000), F32)


def _pack(a, b):
    return pltpu.pack_elementwise([a, b], packed_dtype=BF16)


def _tie(x, a):
    if a is None:
        return x
    w = pltpu.bitcast(x[:, :128], U32)
    k = w.shape[0] // 8
    w = w | (a if k == 1 else jnp.concatenate([a] * k, axis=0))
    w = pltpu.bitcast(w, x.dtype)
    return w if x.shape[1] == 128 else jnp.concatenate([w, x[:, 128:]], axis=1)


def C(i, lim=F):
    return slice(i * 128, min((i + 1) * 128, lim))


class Unit:
    def __init__(self, name, tiles, epi, rows, cost, nt=False, full=True, acc=False):
        self.acc, self.res = acc, []
        self.name, self.tiles, self.epi, self.rows, self.cost, self.nt, self.full = name, tiles, epi, rows, cost, nt, full


class Group:
    def __init__(self, name, fns, cost, rel, dead, lat, rlat=200):
        self.name, self.fns, self.cost, self.rel, self.dead, self.lat, self.rlat = name, fns, cost, rel, dead, lat, rlat


def _plan(seq, groups):
    busy, n = [0] * 4, 0
    start, end, tiles, bars = {}, {}, [], []
    for it in seq:
        if isinstance(it[0], Unit):
            u = it[0]
            m = n % 4
            n += 1
            t0, t1 = busy[m], busy[m] + max(u.rows, 32)
            busy[m] = t1
            tiles.append((t0, t1, u.cost / len(u.tiles)))
            start.setdefault(u.name, t0)
            end[u.name] = max(end.get(u.name, 0), t1)
        elif it[0] == "wait":
            t = max(busy)
            busy, n = [t] * 4, 0
            start[it[1]] = end[it[1]] = t
            bars.append(t)
    total = max(busy)
    start["end"] = end["end"] = total
    ns = total // SLOT + 2
    load = np.zeros(ns)
    for t0, t1, c in tiles:
        a, b = t0 // SLOT, max(t1 // SLOT, t0 // SLOT + 1)
        load[a:b] += c / (b - a)
    win = []
    for g in groups:
        r = max(end[x] + (0 if start[x] == end[x] else g.rlat) for x in g.rel)
        d = min(start[x] for x in g.dead) - g.lat
        ok = np.zeros(ns, bool)
        ok[r // SLOT:max(d // SLOT, r // SLOT + 1)] = True
        for b in bars:
            if r < b <= d:
                ok[max((b - g.lat) // SLOT, 0):b // SLOT] = False
        win.append(np.nonzero(ok)[0])
    alloc = [np.zeros(len(w)) for w in win]
    for _ in range(60):
        for i, g in enumerate(groups):
            w = win[i]
            load[w] -= alloc[i]
            base = load[w]
            vol = g.cost * len(g.fns)
            lo, hi = base.min(), base.max() + vol
            for _ in range(50):
                mid = 0.5 * (lo + hi)
                if np.maximum(mid - base, 0).sum() > vol:
                    hi = mid
                else:
                    lo = mid
            alloc[i] = np.maximum(hi - base, 0)
            load[w] += alloc[i]
    times = []
    for i, g in enumerate(groups):
        cum = np.cumsum(alloc[i])
        ts = []
        for k in range(len(g.fns)):
            x = (k + 0.5) * cum[-1] / len(g.fns)
            j = int(np.searchsorted(cum, x))
            prev = cum[j - 1] if j else 0.0
            ts.append(win[i][j] * SLOT + SLOT * (x - prev) / max(alloc[i][j], 1e-9))
        times.append(ts)
        if VERBOSE:
            print("%8s window %6d..%6d used %6d..%6d" % (g.name, win[i][0] * SLOT, win[i][-1] * SLOT, ts[0], ts[-1]))
    if VERBOSE:
        k = 2048 // SLOT
        print("total", total, "load/cycle:", " ".join("%.1f" % (load[i:i + k].mean() / SLOT) for i in range(0, ns, k)))
    return times


def _emit(seq, groups, zero, wait):
    times = _plan(seq, groups)
    left = {}
    for it in seq:
        nm = it[0].name if isinstance(it[0], Unit) else it[1]
        left[nm] = left.get(nm, 0) + 1
    heap, pend, todo, cnt = [], {}, list(range(len(groups))), 0
    busy, n = [0] * 4, 0

    def release():
        nonlocal cnt
        for i in list(todo):
            g = groups[i]
            if all(left[x] == 0 for x in g.rel):
                todo.remove(i)
                pend[i] = len(g.fns)
                for t, fn in zip(times[i], g.fns):
                    heapq.heappush(heap, (t, cnt, i, fn))
                    cnt += 1

    def force(name):
        nonlocal heap
        for i, g in enumerate(groups):
            if name in g.dead:
                assert i not in todo, (g.name, name)
                if pend[i]:
                    if VERBOSE:
                        print("forcing", g.name, pend[i], "before", name)
                    for it in sorted(x for x in heap if x[2] == i):
                        it[3](None)
                    heap = [x for x in heap if x[2] != i]
                    heapq.heapify(heap)
                    pend[i] = 0

    for it in seq:
        if isinstance(it[0], Unit):
            u, k = it
            force(u.name)
            lhs, rhs = u.tiles[k]()
            dn = (((1,), (1 if u.nt else 0,)), ((), ()))
            p = lax.dot_general(lhs, rhs, dn, preferred_element_type=F32)
            u.res = [u.res[0] + p] if (u.acc and u.res) else u.res + [p]
            m = n % 4
            n += 1
            t0 = busy[m]
            busy[m] = t0 + max(u.rows, 32)
            while u.full and heap and heap[0][0] < t0 + u.rows:
                t, _, i, fn = heapq.heappop(heap)
                pend[i] -= 1
                r = min(max(int(t - t0), 0), u.rows - 1) // 8 * 8
                fn(pltpu.bitcast(p[r:r + 8], U32) & zero)
            if k == len(u.tiles) - 1:
                u.epi(u.res)
            left[u.name] -= 1
        elif it[0] == "wait":
            force(it[1])
            wait(it[1])
            busy, n = [max(busy)] * 4, 0
            left[it[1]] -= 1
        else:
            it[2]()
            left[it[1]] -= 1
        release()
    force("end")
    assert not heap and not todo


def _sum(ps):
    acc = ps[0]
    for p in ps[1:]:
        acc = acc + p
    return acc


def _flat(us):
    return [(u, i) for u in us for i in range(len(u.tiles))]


def _mix(seq, a, b, lo=0.0, hi=1.0):
    n = 0
    for it in seq:
        n = n + 1 if isinstance(it[0], Unit) else (0 if it[0] == "wait" else n)
    a = _flat(a)
    k = 0
    for i, t in enumerate(a):
        if k < len(b) and n % 4 == 0 and i >= len(a) * (lo + (hi - lo) * k / len(b)):
            seq.extend(_flat(b[k]))
            k += 1
        seq.append(t)
        n += 1
    assert k == len(b)


def kernel(q_hbm, k_hbm, v_hbm, sh_hbm, ssm_hbm, sd_hbm, w1_hbm, w2_hbm, w3_hbm, w4_hbm, c_hbm, wm_hbm,
           o_hbm,
           q_w, k_n, v_w, ssm_w, w1_w, w2_w, w3_w, w4_w, wm_w, o_v,
           sh_v, sd_v, c_v, zsrc, z_s, taps, mod_v, tf_w, tg_w,
           kf, zraw, uf, kv_w, zz_w, y_w, x_v, hb_v, x1_v, n1_w, n2_w, g_w, h1_v,
           sem, sem_o):
    bf = lambda r: r.bitcast(BF16)
    w1_v, w2_v, w3_v, w4_v, wm_v = bf(w1_w), bf(w2_w), bf(w3_w), bf(w4_w), bf(wm_w)
    tf_v, tg_v, kv_v, zz_v, y_v, n1_v, n2_v, g_v = (bf(tf_w), bf(tg_w), bf(kv_w), bf(zz_w), bf(y_w), bf(n1_w),
                                                    bf(n2_w), bf(g_w))
    cp = pltpu.make_async_copy
    scope = lambda nm: jax.named_scope(nm) if SCOPES else contextlib.nullcontext()

    dmas = {}

    def group(name, *mks):
        sm = sem.at[len(dmas)]
        dmas[name] = [c for mk in mks for c in mk(sm)]

    def rows(s, n=1):
        return pl.ds(s * T, n * T)

    def conv_in(s, n=1):
        return lambda sm: ([cp(ssm_hbm.at[:, rows(s, n)], bf(ssm_w).at[:, rows(s, n)], sm)]
                           + [cp(k_hbm.at[rows(s, n), C(t)], bf(k_n).at[t, pl.ds(16 + s * T, n * T)], sm) for t in range(NT)]
                           + [cp(v_hbm.at[rows(s, n)], bf(v_w).at[rows(s, n)], sm)])

    def q_in(s, n=1):
        return lambda sm: [cp(q_hbm.at[rows(s, n)], bf(q_w).at[rows(s, n)], sm)]

    def wm_in(a, b):
        return lambda sm: [cp(wm_hbm.at[:, a * D:b * D], wm_v.at[:, a * D:b * D], sm)]

    def whole(src, dst):
        return lambda sm: [cp(src, dst, sm)]

    zsrc[...] = jnp.zeros((8, 128), I32)
    k_n[:, 0:8, :] = jnp.zeros((NT, 8, 128), U32)
    group("small", lambda sm: [cp(zsrc, z_s, sm), cp(sh_hbm, sh_v, sm), cp(sd_hbm, sd_v, sm), cp(c_hbm, c_v, sm)])
    for s in range(NC):
        group("c%d" % s, conv_in(s))
    group("wma", wm_in(0, 3), q_in(0, 2))
    group("wmb", wm_in(3, 5))
    group("w1", whole(w1_hbm, w1_v))
    group("w2", q_in(2), whole(w2_hbm, w2_v))
    group("w3", whole(w3_hbm, w3_v), q_in(3))
    group("w4", whole(w4_hbm, w4_v), wm_in(5, 6), conv_in(4), q_in(4))
    group("rest", conv_in(5, NB - 5), q_in(5, NB - 5))
    for g in dmas.values():
        for c in g:
            c.start()

    def wait(name):
        with scope("wait_" + name):
            for c in dmas[name]:
                c.wait()

    tau_b = lambda l: H + ((l + (H - 1)) & (H - 1))
    tf_v[:, C(0)] = _dft((T, H), 0, lambda l: jnp.where((l & 1) == 0, l, tau_b(l)), 1.0 / T)
    tf_v[:, C(1)] = _dft((T, H), 0, lambda l: jnp.where((l & 1) == 1, l, tau_b(l)), 1.0 / T)
    tf_v[:, C(2)] = _dft((T, H), 0, lambda l: 2 * _unzip(l))
    tf_v[:, C(3)] = _dft((T, H), 0, lambda l: 2 * _unzip(l) + 1)
    tg_v[:, 0:T] = _dft((H, T), 1, lambda l: 2 * l)
    tg_v[:, T:2 * T] = _dft((H, T), 1, lambda l: 2 * l + 1)
    h1_v[:, 0:8, :] = jnp.zeros((NT, 8, 128), F32)
    h1_v[:, 8 + S:16 + S, :] = jnp.zeros((NT, 8, 128), F32)

    wait("small")
    z = jnp.clip(z_s[0, 0], 0, 1)
    zero = jnp.full((8, 128), z, I32).astype(U32)
    z8 = pl.multiple_of(z * 8, 8)
    for r in (x_v, hb_v, x1_v, n1_w, n2_w, g_w, y_w):
        r[pl.ds(z8, 8), 0:128] = jnp.zeros((8, 128), r.dtype)
    for r in (kf, zraw, uf, kv_w, zz_w, taps, mod_v):
        r[z, 0:8, 0:128] = jnp.zeros((8, 128), r.dtype)
    for r in (tf_w, tg_w):
        r[pl.ds(z8, 8), 0:128] = r[0:8, 0:128]
    sh = sh_v[...].astype(F32)
    for i in range(4):
        taps[i] = jnp.broadcast_to(sh[i:i + 1], (8, D))
    taps[4] = jnp.broadcast_to(sd_v[...].astype(F32).reshape(1, D) * (1.0 / T), (8, D))
    cf = c_v[...].astype(F32)
    silu_c = jnp.broadcast_to((cf / (1.0 + jnp.exp(-cf))).astype(BF16), (16, D))

    def mmK(m):
        def unit(n):
            W = slice(64 * n, 64 * (n + 1))
            st = []

            def rhs(i):
                if not st:
                    ev = (lax.broadcasted_iota(I32, (64, 128), 1) & 1) == 0
                    a = ssm_w[W, m * T:m * T + H]
                    b = pltpu.roll(ssm_w[W, m * T + H:(m + 1) * T], 1, 1)
                    st.extend([pltpu.bitcast(jnp.where(ev, a, b), BF16), pltpu.bitcast(jnp.where(ev, b, a), BF16)])
                return st[i]

            def epi(p):
                er, ei, or_, oi = p
                if m == 0:
                    er = er + taps[4, 0:1, C(n)]
                for h, (cr, ci) in enumerate(((er + or_, ei + oi), (er - or_, ei - oi))):
                    B = h * 3 * H
                    kf[m, B:B + H, C(n)] = cr
                    kf[m, B + H:B + 2 * H, C(n)] = ci - cr
                    kf[m, B + 2 * H:B + 3 * H, C(n)] = ci + cr
            return Unit("K%d" % m, [(lambda i=i, r=r: (tf_v[r:r + H, C(i)], rhs(i))) for i in range(2) for r in (0, H)],
                        epi, H, 170, nt=True)
        return [unit(n) for n in range(NT)]

    def kv(s):
        def mk(t, w):
            def fn(a):
                w0 = s * H + w
                ld = lambda d: k_n[t, 8 + w0 - d:8 + w0 - d + 16, :].reshape(2, 8, 128)
                c0 = _tie(k_n[t, 8 + w0:8 + w0 + 8, :], a)
                c0 = jnp.concatenate([c0, k_n[t, 16 + w0:24 + w0, :]], axis=0).reshape(2, 8, 128)
                c1, c2 = ld(1), ld(2)
                s0, s1, s2, s3 = (taps[i, :, C(t)] for i in range(4))
                ke, ko, ke1, ko1, ko2 = _lo(c0), _hi(c0), _lo(c1), _hi(c1), _hi(c2)
                wv = v_w[w0:w0 + 16, C(t)].reshape(2, 8, 128)
                kve = ((s0 * ke + s1 * ko1) + (s2 * ke1 + s3 * ko2)) * _lo(wv)
                kvo = ((s0 * ko + s1 * ke) + (s2 * ko1 + s3 * ke1)) * _hi(wv)
                kv_w[s % 2, w // 2:w // 2 + 8, C(t)] = _pack(kve[0], kve[1])
                kv_w[s % 2, (H + w) // 2:(H + w) // 2 + 8, C(t)] = _pack(kvo[0], kvo[1])
            return fn
        return [mk(t, w) for t in range(NT) for w in range(0, H, 16)]

    def mmU(s):
        def unit(n):
            def epi(p):
                er, ei, or_, oi = p
                for h, (cr, ci) in enumerate(((er + or_, ei + oi), (er - or_, ei - oi))):
                    B = h * 3 * H
                    uf[NB - 1 - s, B:B + H, C(n)] = cr + ci
                    uf[NB - 1 - s, B + H:B + 2 * H, C(n)] = cr
                    uf[NB - 1 - s, B + 2 * H:B + 3 * H, C(n)] = ci
            return Unit("U%d" % s, [(lambda i=i, r=r: (tf_v[r:r + H, C(2 + i)], kv_v[s % 2, C(i), C(n)]))
                                    for i in range(2) for r in (0, H)], epi, H, 120)
        return [unit(n) for n in range(NT)]

    def mac(s):
        def chain(row, L, a):
            t = []
            for i in range(3):
                Rw = slice(row + i * H, row + i * H + 8)
                kk = kf[0:s + 1, Rw, L]
                if i == 0 and a is not None:
                    k0 = _tie(kk[0], a)[None]
                    kk = k0 if s == 0 else jnp.concatenate([k0, kk[1:]], axis=0)
                t.append(jnp.sum(kk * uf[NB - 1 - s:NB, Rw, L], axis=0))
            return t[0] - t[2], t[0] + t[1]

        def mk(t, rc):
            st, fin = [], []

            def part(i):
                def fn(a):
                    st.append(chain((i & 1) * 3 * H + rc + (i >> 1) * 8, C(t), a))
                    if i & 1:
                        (pr, pi), (mr, mi) = st[-2:]
                        z = [pr + mr, pi + mi, pr - mr, pi - mi]
                        Rw = lambda q: slice(q * H + rc + (i >> 1) * 8, q * H + rc + (i >> 1) * 8 + 8)
                        if s + 1 < NB:
                            for q in range(4):
                                zraw[s % 2, Rw(q), C(t)] = z[q]
                        if s > 0:
                            pv = [zraw[(s - 1) % 2, Rw(q ^ 1), C(t)] for q in range(4)]
                            z = [z[q] + pv[q] if (q & 1) == (rc < 64) else z[q] - pv[q] for q in range(4)]
                        fin.append(z)
                    if i == 3:
                        for q in range(4):
                            w = (q * H + rc) // 2
                            zz_w[s % 2, w:w + 8, C(t)] = _pack(fin[0][q], fin[1][q])
                return fn
            return [part(i) for i in range(4)]
        return [fn for t in range(NT) for rc in range(0, H, 16) for fn in mk(t, rc)]

    def mmI(s):
        def unit(n):
            def epi(p):
                y_w[s * H:(s + 1) * H, C(n)] = _pack(p[0] + p[1], p[2] + p[3])
            return Unit("I%d" % s, [(lambda i=i: (tg_v[:, C(i)], zz_v[s % 2, C(i), C(n)])) for i in range(4)],
                        epi, H, 48)
        return [unit(n) for n in range(NT)]

    def mod(name, a, b):
        def unit(n):
            def epi(p):
                v = [_sum(p[i * NT:(i + 1) * NT])[0:8] for i in range(b - a)]
                if a == 0:
                    mod_v[0, :, C(n)] = v[0] * v[2]
                    mod_v[1, :, C(n)] = (v[1] + 1.0) * v[2]
                elif a == 3:
                    mod_v[3, :, C(n)] = v[0]
                    mod_v[4, :, C(n)] = v[1] + 1.0
                else:
                    mod_v[5, :, C(n)] = v[0]
            return Unit(name, [(lambda i=i, k=k: (silu_c[:, C(k)], wm_v[C(k), i * D + n * 128:i * D + (n + 1) * 128]))
                               for i in range(a, b) for k in range(NT)], epi, 16, 10, full=False)
        return [unit(n) for n in range(NT)]

    def blk(j):
        return range(j * T, (j + 1) * T, RG)

    def fa(j):
        def mk(r):
            def fn(a):
                q = pltpu.bitcast(_tie(q_w[r // 2:r // 2 + 8, :], a), BF16).astype(F32).reshape(2, 8, D)
                y = y_v[r:r + RG, :].astype(F32).reshape(2, 8, D)
                x_v[r:r + RG, :] = (q + (_ln(q) * mod_v[1] + mod_v[0]) * y).reshape(RG, D)
            return fn
        return [mk(r) for r in blk(j)]

    def fb(j):
        def mk(r):
            def fn(a):
                x = _tie(x_v[r:r + RG, :], a).reshape(2, 8, D)
                hb_v[r:r + RG, :] = (_ln(x) * mod_v[4] + mod_v[3]).reshape(RG, D)
            return fn
        return [mk(r) for r in blk(j)]

    def fc(j):
        def mk(r):
            def fn(a):
                n1_v[r:r + RG, :] = _ln(_tie(hb_v[r:r + RG, :], a), G_A).astype(BF16)
            return fn
        return [mk(r) for r in blk(j)]

    def shift(j):
        SR = 64

        def mk(t, r):
            def fn(a):
                lane = lax.broadcasted_iota(I32, (SR, 128), 1)
                ld = lambda d: h1_v[t, 8 + r + d:8 + r + d + SR, :]
                if t == 0:
                    g = ld(-1)
                elif t == 1:
                    g = jnp.where(lane < 32, ld(-1), ld(1))
                elif t == 2:
                    g = jnp.where(lane < 64, ld(1), ld(-2))
                elif t == 3:
                    g = jnp.where(lane < 96, ld(-2), ld(2))
                else:
                    g = ld(2)
                if a is not None:
                    g = jnp.concatenate([_tie(g[i:i + 8], a) if i % 16 == 0 else g[i:i + 8]
                                         for i in range(0, SR, 8)], axis=0)
                g_v[r:r + SR, C(t)] = g.astype(BF16)
            return fn
        return [mk(t, j * T + r) for t in range(NT) for r in range(0, T, SR)]

    def ln2(j):
        def mk(r):
            def fn(a):
                n2_v[r:r + RG, :] = _ln(_tie(x1_v[r:r + RG, :], a), G_A).astype(BF16)
            return fn
        return [mk(r) for r in blk(j)]

    def halves(j, M):
        return [slice(r, r + M) for r in range(j * T, (j + 1) * T, M)]

    def mm1(j, M=MS[0]):
        def unit(n, R):
            def epi(p):
                h1_v[n, 8 + R.start:8 + R.stop, :] = _gelu2(p[0])
            return Unit("w1_%d" % j, [(lambda k=k: (n1_v[R, C(k)], w1_v[C(k), C(n)])) for k in range(NT)],
                        epi, M, M // 8 * 9, acc=True)
        return [unit(n, R) for n in range(NT) for R in halves(j, M)]

    def mm2(j, M=MS[1]):
        def unit(n, R):
            def epi(p):
                x1_v[R, C(n)] = hb_v[R, C(n)] + p[0] * G_POST
            return Unit("w2_%d" % j, [(lambda k=k: (g_v[R, C(k)], w2_v[C(k), C(n)])) for k in range(NT)],
                        epi, M, M // 8 * 6, acc=True)
        return [unit(n, R) for n in range(NT) for R in halves(j, M)]

    act = {}

    def mm3(j, M=MS[2]):
        def unit(n, R):
            def epi(p):
                a = _gelu2(p[0]).astype(BF16)
                for r in range(0, M, 128):
                    act[R.start + r, n] = a[r:r + 128]
            return Unit("w3_%d" % j, [(lambda k=k: (n2_v[R, C(k)], w3_v[C(n), C(k)])) for k in range(NT)],
                        epi, M, M // 8 * 10, nt=True, acc=True)

        return [unit(n, R) for n in range(FT - 1) for R in halves(j, M)]

    def mm3r(j):
        F0 = (FT - 1) * 128
        hs = halves(j, 128)
        part = []

        def epi(p):
            for i, R in enumerate(hs):
                t = part[i] + jnp.concatenate(p[2 * i:2 * i + 2], axis=0)
                act[R.start, FT - 1] = _gelu2(t).T.astype(BF16)
        us = [Unit("w3_%d" % j, [(lambda k=k, R=R: (w3_v[F0:F, C(k)], n2_v[R, C(k)])) for k in range(NT - 1)],
                   lambda p: part.append(p[0]), 64, 24, nt=True, acc=True) for R in hs]
        us.append(Unit("w3_%d" % j, [(lambda R=R, f=f: (w3_v[f:f + 32, C(NT - 1)], n2_v[R, C(NT - 1)]))
                                     for R in hs for f in (F0, F0 + 32)], epi, 32, 120, nt=True))
        return us

    outs = []

    def mm4(j, M=MS[3]):
        def lhs(R, k):
            ps = [act[r, k] for r in range(R.start, R.stop, 128)]
            return ps[0] if len(ps) == 1 else jnp.concatenate(ps, axis=0)

        def unit(n, R):
            def epi(p):
                gb = mod_v[5, 0:1, C(n)]
                o_v[R, C(n)] = (x_v[R, C(n)] + gb * (x1_v[R, C(n)] + p[0] * G_POST)).astype(BF16)
                if R.stop % T == 0:
                    if j == NB - 1:
                        outs.append(cp(o_v.at[rows(j), C(n)], o_hbm.at[rows(j), C(n)], sem_o.at[0]))
                        outs[-1].start()
                    elif n == NT - 1:
                        outs.append(cp(o_v.at[rows(j)], o_hbm.at[rows(j)], sem_o.at[0]))
                        outs[-1].start()
            return Unit("w4_%d" % j, [(lambda k=k: (lhs(R, k), w4_v[C(k, F), C(n)])) for k in range(FT)],
                        epi, M, M // 8 * 18, acc=True)
        return [unit(n, R) for n in range(NT) for R in halves(j, M)]

    W = lambda nm: [("wait", nm)]
    run = lambda fns: [("run", "run", lambda: [fn(None) for fn in fns])]

    one = lambda us: [[u] for u in us]
    seq, grp = [], []
    for s in range(NC):
        seq += W("c%d" % s) + _flat((mmI(s - 2) if s >= 2 else []) + mmK(s) + mmU(s))
        grp.append(Group("kv%d" % s, kv(s), 50, ["c%d" % s], ["U%d" % s], 100))
        if s + 1 < NC:
            grp.append(Group("mac%d" % s, mac(s), 6 * s + 12, ["c%d" % (s + 1)],
                             ["c%d" % (s + 2) if s + 2 < NC else "I%d" % s], 0))
    grp.append(Group("mac%d" % (NC - 1), mac(NC - 1), 6 * NC + 6, ["U%d" % (NC - 1)], ["I%d" % (NC - 1)], 0))
    seq += _flat(mmI(NC - 2) + mmI(NC - 1))
    seq += W("wma") + _flat(mod("moda", 0, 3)) + run(fa(0) + fa(1))
    seq += W("wmb") + _flat(mod("modb", 3, 5)) + run(fb(0) + fc(0))
    seq += W("w1") + _flat(mm1(0) + mm1(1)) + run(shift(0))
    grp.append(Group("f1", fb(1) + fc(1), 70, ["w1"], ["w1_1"], 450))
    seq += W("w2") + _flat(mm2(0) + mm1(2)) + run(shift(1)) + _flat(mm2(1))
    grp.append(Group("f2", fa(2) + fb(2) + fc(2), 80, ["w2"], ["w1_2"], 450))
    grp.append(Group("ln2_0", ln2(0), 60, ["w2_0"], ["w3"], 450))
    seq += W("w3") + _flat(mm3r(0) + mm3(0) + mm1(3) + mm3r(1) + mm3(1))
    grp.append(Group("f3", fa(3) + fb(3) + fc(3), 80, ["w3"], ["w1_3"], 450))
    grp.append(Group("ln2_1", ln2(1), 60, ["w3"], ["w3_1"], 450))
    seq += W("w4") + _flat(mod("modc", 5, 6))
    _mix(seq, mm4(0), one(mmK(4)) + one(mmU(4)))
    seq += _flat(mm2(2) + mm4(1))
    grp.append(Group("kv4", kv(4), 50, ["w4"], ["U4"], 450))
    seq += W("rest")
    for j in range(2, NB):
        s = j + 3
        w4 = mm4(j)
        first = (mmI(j + 2) if j + 2 < NB else []) + mm3r(j)
        _mix(seq, mm3(j), [first] + (one(mmK(s)) + one(mmU(s)) if s < NB else []))
        if j + 2 < NB:
            seq += _flat(mm1(j + 2) + w4[:len(w4) * 2 // 5] + mm2(j + 1) + w4[len(w4) * 2 // 5:])
        elif j + 1 < NB:
            seq += _flat(mm2(j + 1) + w4)
        else:
            seq += _flat(w4)
        if s < NB:
            grp.append(Group("kv%d" % s, kv(s), 50, ["rest", "U%d" % (s - 2)], ["U%d" % s], 450))
    for s in range(4, NB):
        grp.append(Group("mac%d" % s, mac(s), 6 * s + 12, ["U%d" % s, "K%d" % s], ["I%d" % s], 450))
        grp.append(Group("f%d" % s, fa(s) + fb(s) + fc(s), 80, ["I%d" % s], ["w1_%d" % s], 450))
    for j in range(2, NB):
        grp.append(Group("shift%d" % j, shift(j), 14, ["w1_%d" % min(j + 1, NB - 1)], ["w2_%d" % j], 200))
        grp.append(Group("ln2_%d" % j, ln2(j), 60, ["w2_%d" % j], ["w3_%d" % j], 450))
    _emit(seq, grp, zero, wait)
    with scope("wait_out"):
        for c in outs:
            c.wait()


@jax.jit
def pallas_adaLN_cond__ssm_conv_h3__mixer_s_mlp__prompt_kernel(A_q, A_k, A_v, A_shift_k, A_ssm_k, A_ssm_D, B_x, B_w1, B_w2, B_w3, B_w4, c, w_mod):
    any_ = pl.BlockSpec(memory_space=pl.ANY)
    V = pltpu.VMEM
    out = pl.pallas_call(
        kernel,
        in_specs=[any_] * 12,
        out_specs=any_,
        out_shape=jax.ShapeDtypeStruct((S, D), BF16),
        scratch_shapes=[
            V((S // 2, D), U32), V((NT, 8 + S // 2, 128), U32), V((S // 2, D), U32), V((D // 2, S), U32),
            V((D // 2, D), U32), V((D // 2, D), U32), V((F // 2, D), U32), V((F // 2, D), U32),
            V((D // 2, 6 * D), U32), V((S, D), BF16),
            V((4, D), BF16), V((D,), BF16), V((1, D), BF16), V((8, 128), I32), pltpu.SMEM((8, 128), I32),
            V((5, 8, D), F32), V((6, 8, D), F32), V((T // 2, 4 * H), U32), V((H // 2, 2 * T), U32),
            V((NB, 3 * T + 8, D), F32), V((2, 2 * T, D), F32), V((NB, 3 * T + 8, D), F32),
            V((2, T // 2, D), U32), V((2, T, D), U32), V((S // 2, D), U32),
            V((S, D), F32), V((S, D), F32), V((S, D), F32),
            V((S // 2, D), U32), V((S // 2, D), U32), V((S // 2, D), U32), V((NT, S + 16, 128), F32),
            pltpu.SemaphoreType.DMA((12,)), pltpu.SemaphoreType.DMA((1,)),
        ],
        compiler_params=pltpu.CompilerParams(vmem_limit_bytes=110 << 20),
        name="fused",
    )(A_q[0], A_k[0], A_v[0], A_shift_k.T, A_ssm_k, A_ssm_D, B_w1, B_w2, B_w3.T, B_w4, c, w_mod)
    return out[None]
```

```python
import contextlib
import heapq
import os
import numpy as np
import jax
import jax.numpy as jnp
from jax import lax
from jax.experimental import pallas as pl
from jax.experimental.pallas import tpu as pltpu

S, D, F = 2048, 640, 1728
T = 256
H = T // 2
NB = S // T
NT = D // 128
FT = (F + 127) // 128
EPS = 1e-5
F32, BF16, U32, I32 = jnp.float32, jnp.bfloat16, jnp.uint32, jnp.int32
G_C1 = 0.044715 * float(np.sqrt(2.0 / np.pi))
G_C2 = float(np.sqrt(2.0 / np.pi))
G_A = G_C1 ** (1.0 / 3.0)
G_B = G_C2 / G_A
G_POST = 0.5 / G_A
RG = 16
GR = 80
NC = 4
VERBOSE = False
SCOPES = False
SLOT = 32
MS = (128, 128, 128, 128)


def _unzip(p):
    return (p & -16) | ((p & 1) << 3) | ((p >> 1) & 7)


def _dft(shape, f_axis, tau, scale=1.0):
    r = lax.broadcasted_iota(I32, shape, f_axis)
    l = lax.broadcasted_iota(I32, shape, 1 - f_axis)
    if f_axis == 1:
        r = _unzip(r)
    f = r & 127
    odd = ((f & 63) << 2) | ((f >> 6) << 1) | 1
    p = odd * tau(l) + ((r >> 7) << 8)
    a = ((p + 512) & 1023) - 512
    u = (256 - jnp.abs(a)).astype(F32) * (np.pi / 512.0)
    u2 = u * u
    c = [scale, -scale / 6.0, scale / 120.0, -scale / 5040.0, scale / 362880.0, -scale / 39916800.0]
    poly = c[5]
    for ci in c[4::-1]:
        poly = poly * u2 + ci
    return (u * poly).astype(BF16)


def _ln(x, scale=1.0):
    m = jnp.sum(x, axis=-1, keepdims=True) * (1.0 / D)
    xc = x - m
    s2 = 1.0 / (scale * scale)
    v = jnp.sum(xc * xc, axis=-1, keepdims=True) * (s2 / D) + EPS * s2
    r = jnp.exp2(jnp.log(v) * float(-0.5 / np.log(2.0)))
    return xc * r


def _gelu2(x):
    u = x * (x * x + G_B)
    return x * (1.0 + jnp.tanh(u))


def _lo(w):
    return pltpu.bitcast(w << 16, F32)


def _hi(w):
    return pltpu.bitcast(w & jnp.uint32(0xFFFF0000), F32)


def _pack(a, b):
    return pltpu.pack_elementwise([a, b], packed_dtype=BF16)


def _tie(x, a):
    if a is None:
        return x
    w = pltpu.bitcast(x[:, :128], U32)
    k = w.shape[0] // 8
    w = w | (a if k == 1 else jnp.concatenate([a] * k, axis=0))
    w = pltpu.bitcast(w, x.dtype)
    return w if x.shape[1] == 128 else jnp.concatenate([w, x[:, 128:]], axis=1)


def C(i, lim=F):
    return slice(i * 128, min((i + 1) * 128, lim))


class Unit:
    def __init__(self, name, tiles, epi, rows, cost, nt=False, full=True, acc=False):
        self.acc, self.res = acc, []
        self.name, self.tiles, self.epi, self.rows, self.cost, self.nt, self.full = name, tiles, epi, rows, cost, nt, full


class Group:
    def __init__(self, name, fns, cost, rel, dead, lat, rlat=200):
        self.name, self.fns, self.cost, self.rel, self.dead, self.lat, self.rlat = name, fns, cost, rel, dead, lat, rlat


def _plan(seq, groups):
    busy, n = [0] * 4, 0
    start, end, tiles, bars = {}, {}, [], []
    for it in seq:
        if isinstance(it[0], Unit):
            u = it[0]
            m = n % 4
            n += 1
            t0, t1 = busy[m], busy[m] + max(u.rows, 32)
            busy[m] = t1
            tiles.append((t0, t1, u.cost / len(u.tiles)))
            start.setdefault(u.name, t0)
            end[u.name] = max(end.get(u.name, 0), t1)
        elif it[0] == "wait":
            t = max(busy)
            busy, n = [t] * 4, 0
            start[it[1]] = end[it[1]] = t
            bars.append(t)
    total = max(busy)
    start["end"] = end["end"] = total
    ns = total // SLOT + 2
    load = np.zeros(ns)
    for t0, t1, c in tiles:
        a, b = t0 // SLOT, max(t1 // SLOT, t0 // SLOT + 1)
        load[a:b] += c / (b - a)
    win = []
    for g in groups:
        r = max(end[x] + (0 if start[x] == end[x] else g.rlat) for x in g.rel)
        d = min(start[x] for x in g.dead) - g.lat
        ok = np.zeros(ns, bool)
        ok[r // SLOT:max(d // SLOT, r // SLOT + 1)] = True
        for b in bars:
            if r < b <= d:
                ok[max((b - g.lat) // SLOT, 0):b // SLOT] = False
        win.append(np.nonzero(ok)[0])
    alloc = [np.zeros(len(w)) for w in win]
    for _ in range(60):
        for i, g in enumerate(groups):
            w = win[i]
            load[w] -= alloc[i]
            base = load[w]
            vol = g.cost * len(g.fns)
            lo, hi = base.min(), base.max() + vol
            for _ in range(50):
                mid = 0.5 * (lo + hi)
                if np.maximum(mid - base, 0).sum() > vol:
                    hi = mid
                else:
                    lo = mid
            alloc[i] = np.maximum(hi - base, 0)
            load[w] += alloc[i]
    times = []
    for i, g in enumerate(groups):
        cum = np.cumsum(alloc[i])
        ts = []
        for k in range(len(g.fns)):
            x = (k + 0.5) * cum[-1] / len(g.fns)
            j = int(np.searchsorted(cum, x))
            prev = cum[j - 1] if j else 0.0
            ts.append(win[i][j] * SLOT + SLOT * (x - prev) / max(alloc[i][j], 1e-9))
        times.append(ts)
        if VERBOSE:
            print("%8s window %6d..%6d used %6d..%6d" % (g.name, win[i][0] * SLOT, win[i][-1] * SLOT, ts[0], ts[-1]))
    if VERBOSE:
        k = 2048 // SLOT
        print("total", total, "load/cycle:", " ".join("%.1f" % (load[i:i + k].mean() / SLOT) for i in range(0, ns, k)))
    return times


def _emit(seq, groups, zero, wait):
    times = _plan(seq, groups)
    left = {}
    for it in seq:
        nm = it[0].name if isinstance(it[0], Unit) else it[1]
        left[nm] = left.get(nm, 0) + 1
    heap, pend, todo, cnt = [], {}, list(range(len(groups))), 0
    busy, n = [0] * 4, 0

    def release():
        nonlocal cnt
        for i in list(todo):
            g = groups[i]
            if all(left[x] == 0 for x in g.rel):
                todo.remove(i)
                pend[i] = len(g.fns)
                for t, fn in zip(times[i], g.fns):
                    heapq.heappush(heap, (t, cnt, i, fn))
                    cnt += 1

    def force(name):
        nonlocal heap
        for i, g in enumerate(groups):
            if name in g.dead:
                assert i not in todo, (g.name, name)
                if pend[i]:
                    if VERBOSE:
                        print("forcing", g.name, pend[i], "before", name)
                    for it in sorted(x for x in heap if x[2] == i):
                        it[3](None)
                    heap = [x for x in heap if x[2] != i]
                    heapq.heapify(heap)
                    pend[i] = 0

    for it in seq:
        if isinstance(it[0], Unit):
            u, k = it
            force(u.name)
            lhs, rhs = u.tiles[k]()
            dn = (((1,), (1 if u.nt else 0,)), ((), ()))
            p = lax.dot_general(lhs, rhs, dn, preferred_element_type=F32)
            u.res = [p + u.res[0]] if (u.acc and u.res) else u.res + [p]
            m = n % 4
            n += 1
            t0 = busy[m]
            busy[m] = t0 + max(u.rows, 32)
            while u.full and heap and heap[0][0] < t0 + u.rows:
                t, _, i, fn = heapq.heappop(heap)
                pend[i] -= 1
                r = min(max(int(t - t0), 0), u.rows - 1) // 8 * 8
                fn(pltpu.bitcast(p[r:r + 8], U32) & zero)
            if k == len(u.tiles) - 1:
                u.epi(u.res)
            left[u.name] -= 1
        elif it[0] == "wait":
            force(it[1])
            wait(it[1])
            busy, n = [max(busy)] * 4, 0
            left[it[1]] -= 1
        else:
            it[2]()
            left[it[1]] -= 1
        release()
    force("end")
    assert not heap and not todo


def _sum(ps):
    acc = ps[0]
    for p in ps[1:]:
        acc = acc + p
    return acc


def _flat(us):
    return [(u, i) for u in us for i in range(len(u.tiles))]


def _phase(seq):
    n = 0
    for it in seq:
        n = n + 1 if isinstance(it[0], Unit) else (0 if it[0] in ("wait", "sync") else n)
    return n % 4


def _mix(seq, a, b, lo=0.0, hi=1.0):
    n, k = _phase(seq), 0
    for i, t in enumerate(a):
        if k < len(b) and n % 4 == 0 and t[1] != 1 and i >= len(a) * (lo + (hi - lo) * k / len(b)):
            seq.extend(b[k])
            k += 1
        seq.append(t)
        n += 1
    assert k == len(b)


def _wait(seq, name, head=()):
    r = _phase(seq)
    assert all(isinstance(it[0], Unit) for it in seq[len(seq) - r:])
    seq[len(seq) - r:len(seq) - r] = [("wait", name)] + list(head)


def kernel(q_hbm, k_hbm, v_hbm, sh_hbm, ssm_hbm, sd_hbm, w1_hbm, w2_hbm, w3_hbm, w4_hbm, c_hbm, wm_hbm,
           o_hbm,
           q_w, k_n, v_w, ssm_w, w1_w, w2_w, w3_w, w4_w, wm_w, o_v,
           sh_v, sd_v, c_v, zsrc, z_s, taps, mod_v, tf_w, tg_w,
           kf, zraw, uf, kv_w, zz_w, y_v, x_v, hb_v, x1_v, n1_w, n2_w, g_w, h1_v, a_w,
           sem, sem_o):
    bf = lambda r: r.bitcast(BF16)
    w1_v, w2_v, w3_v, w4_v, wm_v = bf(w1_w), bf(w2_w), bf(w3_w), bf(w4_w), bf(wm_w)
    tf_v, tg_v, kv_v, zz_v, n1_v, n2_v, g_v = bf(tf_w), bf(tg_w), bf(kv_w), bf(zz_w), bf(n1_w), bf(n2_w), bf(g_w)
    q_v, a_v = bf(q_w), bf(a_w)
    cp = pltpu.make_async_copy
    scope = lambda nm: jax.named_scope(nm) if SCOPES else contextlib.nullcontext()

    dmas = {}

    def group(name, *mks):
        sm = sem.at[len(dmas)]
        dmas[name] = [c for mk in mks for c in mk(sm)]

    def rows(s, n=1):
        return pl.ds(s * T, n * T)

    def conv_in(s, n=1):
        return lambda sm: ([cp(ssm_hbm.at[:, rows(s, n)], bf(ssm_w).at[:, rows(s, n)], sm)]
                           + [cp(k_hbm.at[rows(s, n), C(t)], bf(k_n).at[t, pl.ds(16 + s * T, n * T)], sm) for t in range(NT)]
                           + [cp(v_hbm.at[rows(s, n)], bf(v_w).at[rows(s, n)], sm)])

    def q_in(s, n=1):
        return lambda sm: [cp(q_hbm.at[rows(s, n)], bf(q_w).at[rows(s, n)], sm)]

    def wm_in(a, b):
        return lambda sm: [cp(wm_hbm.at[:, a * D:b * D], wm_v.at[:, a * D:b * D], sm)]

    def whole(src, dst):
        return lambda sm: [cp(src, dst, sm)]

    zsrc[...] = jnp.zeros((8, 128), I32)
    k_n[:, 0:8, :] = jnp.zeros((NT, 8, 128), U32)
    group("small", lambda sm: [cp(zsrc, z_s, sm), cp(sh_hbm, sh_v, sm), cp(sd_hbm, sd_v, sm), cp(c_hbm, c_v, sm)])
    for s in range(NC):
        group("c%d" % s, conv_in(s))
    group("wma", wm_in(0, 3), q_in(0, 2))
    group("wmb", wm_in(3, 5))
    group("w1", whole(w1_hbm, w1_v))
    group("q2", q_in(2))
    group("w2", whole(w2_hbm, w2_v))
    group("w3", whole(w3_hbm, w3_v), q_in(3))
    group("w4", whole(w4_hbm, w4_v), wm_in(5, 6), conv_in(4), q_in(4))
    group("rest", conv_in(5, NB - 5), q_in(5, NB - 5))
    for g in dmas.values():
        for c in g:
            c.start()

    def wait(name):
        with scope("wait_" + name):
            for c in dmas[name]:
                c.wait()

    tau_b = lambda l: H + ((l + (H - 1)) & (H - 1))
    tf_v[:, C(0)] = _dft((T, H), 0, lambda l: jnp.where((l & 1) == 0, l, tau_b(l)), 1.0 / T)
    tf_v[:, C(1)] = _dft((T, H), 0, lambda l: jnp.where((l & 1) == 1, l, tau_b(l)), 1.0 / T)
    tf_v[:, C(2)] = _dft((T, H), 0, lambda l: 2 * _unzip(l) - H)
    tf_v[:, C(3)] = _dft((T, H), 0, lambda l: 2 * _unzip(l) + 1 - H)
    sin0 = lax.broadcasted_iota(I32, (GR, T), 1) >= H
    tg_v[:, 0:T] = _dft((GR, T), 1, lambda l: jnp.where(sin0 & (l == 0), H, 2 * l))
    tg_v[:, T:2 * T] = _dft((GR, T), 1, lambda l: 2 * l + 1)
    h1_v[:, 0:8, :] = jnp.zeros((NT, 8, 128), F32)
    h1_v[:, 8 + S:16 + S, :] = jnp.zeros((NT, 8, 128), F32)

    wait("small")
    z = jnp.clip(z_s[0, 0], 0, 1)
    zero = jnp.full((8, 128), z, I32).astype(U32)
    z8 = pl.multiple_of(z * 8, 8)
    for r in (x_v, hb_v, x1_v, n1_w, n2_w, g_w, a_w):
        r[pl.ds(z8, 8), 0:128] = jnp.zeros((8, 128), r.dtype)
    for r in (kf, zraw, uf, kv_w, zz_w, taps, mod_v):
        r[z, 0:8, 0:128] = jnp.zeros((8, 128), r.dtype)
    for r in (tf_w, tg_w):
        r[pl.ds(z8, 8), 0:128] = r[0:8, 0:128]
    sh = sh_v[...].astype(F32)
    for i in range(4):
        taps[i] = jnp.broadcast_to(sh[i:i + 1], (8, D))
    taps[4] = jnp.broadcast_to(sd_v[...].astype(F32).reshape(1, D) * (1.0 / T), (8, D))
    cf = c_v[...].astype(F32)
    silu_c = jnp.broadcast_to((cf / (1.0 + jnp.exp(-cf))).astype(BF16), (16, D))

    def mmK(m):
        def unit(n):
            W = slice(64 * n, 64 * (n + 1))
            st = []

            def rhs(i):
                if not st:
                    ev = (lax.broadcasted_iota(I32, (64, 128), 1) & 1) == 0
                    a = ssm_w[W, m * T:m * T + H]
                    b = pltpu.roll(ssm_w[W, m * T + H:(m + 1) * T], 1, 1)
                    st.extend([pltpu.bitcast(jnp.where(ev, a, b), BF16), pltpu.bitcast(jnp.where(ev, b, a), BF16)])
                return st[i]

            def epi(p):
                er, ei, or_, oi = p
                if m == 0:
                    er = er + taps[4, 0:1, C(n)]
                for h, (cr, ci) in enumerate(((er + or_, ei + oi), (er - or_, ei - oi))):
                    B = h * 3 * H
                    kf[m, B:B + H, C(n)] = cr
                    kf[m, B + H:B + 2 * H, C(n)] = ci - cr
                    kf[m, B + 2 * H:B + 3 * H, C(n)] = ci + cr
            return Unit("K%d" % m, [(lambda i=i, r=r: (tf_v[r:r + H, C(i)], rhs(i))) for i in range(2) for r in (0, H)],
                        epi, H, 170, nt=True)
        return [unit(n) for n in range(NT)]

    def kv(s):
        def mk(t, w):
            def fn(a):
                w0 = s * H + w
                ld = lambda d: k_n[t, 8 + w0 - d:8 + w0 - d + 16, :].reshape(2, 8, 128)
                c0 = _tie(k_n[t, 8 + w0:8 + w0 + 8, :], a)
                c0 = jnp.concatenate([c0, k_n[t, 16 + w0:24 + w0, :]], axis=0).reshape(2, 8, 128)
                c1, c2 = ld(1), ld(2)
                s0, s1, s2, s3 = (taps[i, :, C(t)] for i in range(4))
                ke, ko, ke1, ko1, ko2 = _lo(c0), _hi(c0), _lo(c1), _hi(c1), _hi(c2)
                wv = v_w[w0:w0 + 16, C(t)].reshape(2, 8, 128)
                kve = ((s0 * ke + s1 * ko1) + (s2 * ke1 + s3 * ko2)) * _lo(wv)
                kvo = ((s0 * ko + s1 * ke) + (s2 * ko1 + s3 * ke1)) * _hi(wv)
                kv_w[s % 2, w // 2:w // 2 + 8, C(t)] = _pack(kve[0], kve[1])
                kv_w[s % 2, (H + w) // 2:(H + w) // 2 + 8, C(t)] = _pack(kvo[0], kvo[1])
            return fn
        return [mk(t, w) for t in range(NT) for w in range(0, H, 16)]

    def mmU(s):
        def unit(n):
            def epi(p):
                er, ei, or_, oi = p
                for h, (cr, ci) in enumerate(((er + or_, ei + oi), (er - or_, ei - oi))):
                    B = h * 3 * H
                    uf[NB - 1 - s, B:B + H, C(n)] = cr + ci
                    uf[NB - 1 - s, B + H:B + 2 * H, C(n)] = cr
                    uf[NB - 1 - s, B + 2 * H:B + 3 * H, C(n)] = ci
            return Unit("U%d" % s, [(lambda i=i, r=r: (tf_v[r:r + H, C(2 + i)], kv_v[s % 2, C(i), C(n)]))
                                    for i in range(2) for r in (0, H)], epi, H, 120)
        return [unit(n) for n in range(NT)]

    def mac(s):
        def chain(row, L, a):
            t = []
            for i in range(3):
                Rw = slice(row + i * H, row + i * H + 8)
                kk = kf[0:s + 1, Rw, L]
                if i == 0 and a is not None:
                    k0 = _tie(kk[0], a)[None]
                    kk = k0 if s == 0 else jnp.concatenate([k0, kk[1:]], axis=0)
                t.append(jnp.sum(kk * uf[NB - 1 - s:NB, Rw, L], axis=0))
            return t[0] - t[2], t[0] + t[1]

        def mk(t, rc):
            st, fin = [], []

            def part(i):
                def fn(a):
                    st.append(chain((i & 1) * 3 * H + rc + (i >> 1) * 8, C(t), a))
                    if i & 1:
                        (pr, pi), (mr, mi) = st[-2:]
                        z = [pr + mr, pi + mi, pr - mr, pi - mi]
                        Rw = lambda q: slice(q * H + rc + (i >> 1) * 8, q * H + rc + (i >> 1) * 8 + 8)
                        if s + 1 < NB:
                            for q in range(4):
                                zraw[s % 2, Rw(q), C(t)] = z[q]
                        if s > 0:
                            pv = [zraw[(s - 1) % 2, Rw(q ^ 1), C(t)] for q in range(4)]
                            z = [z[q] + pv[q] if (q & 1) == (rc < 64) else z[q] - pv[q] for q in range(4)]
                        fin.append(z)
                    if i == 3:
                        for q in range(4):
                            w = (q * H + rc) // 2
                            zz_w[s % 2, w:w + 8, C(t)] = _pack(fin[0][q], fin[1][q])
                return fn
            return [part(i) for i in range(4)]
        return [fn for t in range(NT) for rc in range(0, H, 16) for fn in mk(t, rc)]

    def mmI(s):
        def unit(n):
            def epi(p):
                ce, se, co, so = p
                sub = lax.broadcasted_iota(I32, (8, 128), 0)
                c0 = s * T + H
                y_v[n, s * T:s * T + 1, :] = (ce[64:72] - se[0:8])[0:1]
                se = jnp.concatenate([jnp.where(sub == 0, 0.0, se[0:8]), se[8:]], axis=0)
                for d, cc, ss in ((0, ce[0:64], se), (1, co, so)):
                    y_v[n, pl.ds(c0 + d, 64, stride=2), :] = cc + ss
                    lo = cc - ss
                    for i in range(0, 64, 8):
                        y_v[n, pl.ds(c0 - d - 2 * i - 14, 8, stride=2), :] = jnp.take_along_axis(
                            lo[i:i + 8], 7 - sub, axis=0)
            return Unit("I%d" % s, [(lambda i=i: (tg_v[0:(GR if i == 0 else 64), C(i)], zz_v[s % 2, C(i), C(n)]))
                                    for i in range(4)], epi, 64, 52)
        return [unit(n) for n in range(NT)]

    def mod(name, a, b):
        def unit(n):
            def epi(p):
                v = [_sum(p[i * NT:(i + 1) * NT])[0:8] for i in range(b - a)]
                if a == 0:
                    mod_v[0, :, C(n)] = v[0] * v[2]
                    mod_v[1, :, C(n)] = (v[1] + 1.0) * v[2]
                elif a == 3:
                    mod_v[3, :, C(n)] = v[0]
                    mod_v[4, :, C(n)] = v[1] + 1.0
                else:
                    mod_v[5, :, C(n)] = v[0]
            return Unit(name, [(lambda i=i, k=k: (silu_c[:, C(k)], wm_v[C(k), i * D + n * 128:i * D + (n + 1) * 128]))
                               for i in range(a, b) for k in range(NT)], epi, 16, 10, full=False, acc=b - a == 1)
        return [unit(n) for n in range(NT)]

    def blk(j):
        return range(j * T, (j + 1) * T, RG)

    def fa(j):
        def mk(r):
            def fn(a):
                q = pltpu.bitcast(_tie(q_w[r // 2:r // 2 + 8, :], a), BF16).astype(F32).reshape(2, 8, D)
                y = jnp.concatenate([y_v[t, r:r + RG, :] for t in range(NT)], axis=1).reshape(2, 8, D)
                x_v[r:r + RG, :] = (q + (_ln(q) * mod_v[1] + mod_v[0]) * y).reshape(RG, D)
            return fn
        return [mk(r) for r in blk(j)]

    def fb(j):
        def mk(r):
            def fn(a):
                x = _tie(x_v[r:r + RG, :], a).reshape(2, 8, D)
                hb_v[r:r + RG, :] = (_ln(x) * mod_v[4] + mod_v[3]).reshape(RG, D)
            return fn
        return [mk(r) for r in blk(j)]

    def fc(j):
        def mk(r):
            def fn(a):
                n1_v[r:r + RG, :] = _ln(_tie(hb_v[r:r + RG, :], a), G_A).astype(BF16)
            return fn
        return [mk(r) for r in blk(j)]

    def fa2(j):
        def mk(r):
            def fn(a):
                q = q_v[r:r + RG, :].astype(F32).reshape(2, 8, D)
                y = jnp.concatenate([y_v[t, r:r + RG, :] for t in range(NT)], axis=1).reshape(2, 8, D)
                x = (q + (_ln(q) * mod_v[1] + mod_v[0]) * y).reshape(RG, D)
                x_v[r:r + RG, :] = x
                hb_v[r:r + RG, :] = _ln(x)
            return fn
        return [mk(r) for r in blk(j)]

    def fc2(j):
        def mk(r):
            def fn(a):
                hb = (hb_v[r:r + RG, :].reshape(2, 8, D) * mod_v[4] + mod_v[3]).reshape(RG, D)
                hb_v[r:r + RG, :] = hb
                n1_v[r:r + RG, :] = _ln(hb, G_A).astype(BF16)
            return fn
        return [mk(r) for r in blk(j)]

    def shift(j):
        SR = 64

        def mk(t, r):
            def fn(a):
                lane = lax.broadcasted_iota(I32, (SR, 128), 1)
                ld = lambda d: h1_v[t, 8 + r + d:8 + r + d + SR, :]
                if t == 0:
                    g = ld(-1)
                elif t == 1:
                    g = jnp.where(lane < 32, ld(-1), ld(1))
                elif t == 2:
                    g = jnp.where(lane < 64, ld(1), ld(-2))
                elif t == 3:
                    g = jnp.where(lane < 96, ld(-2), ld(2))
                else:
                    g = ld(2)
                if a is not None:
                    g = jnp.concatenate([_tie(g[i:i + 8], a) if i % 16 == 0 else g[i:i + 8]
                                         for i in range(0, SR, 8)], axis=0)
                g_v[r:r + SR, C(t)] = g.astype(BF16)
            return fn
        return [mk(t, j * T + r) for t in range(NT) for r in range(0, T, SR)]

    def ln2(j):
        def mk(r):
            def fn(a):
                n2_v[r:r + RG, :] = _ln(_tie(x1_v[r:r + RG, :], a), G_A).astype(BF16)
            return fn
        return [mk(r) for r in blk(j)]

    def halves(j, M):
        return [slice(r, r + M) for r in range(j * T, (j + 1) * T, M)]

    def mm1(j, M=MS[0]):
        def unit(n, R):
            def epi(p):
                h1_v[n, 8 + R.start:8 + R.stop, :] = _gelu2(p[0])
            return Unit("w1_%d" % j, [(lambda k=k: (n1_v[R, C(k)], w1_v[C(k), C(n)])) for k in range(NT)],
                        epi, M, M // 8 * 9, acc=True)
        return [unit(n, R) for n in range(NT) for R in halves(j, M)]

    def mm2(j, M=MS[1]):
        def unit(n, R):
            def epi(p):
                x1_v[R, C(n)] = hb_v[R, C(n)] + p[0] * G_POST
            return Unit("w2_%d" % j, [(lambda k=k: (g_v[R, C(k)], w2_v[C(k), C(n)])) for k in range(NT)],
                        epi, M, M // 8 * 6, acc=True)
        return [unit(n, R) for n in range(NT) for R in halves(j, M)]

    def loc(R):
        return slice(R.start % (2 * T), R.start % (2 * T) + R.stop - R.start)

    def mm3(j):
        def unit(n, R):
            def epi(p):
                a_v[loc(R), C(n)] = _gelu2(p[0]).astype(BF16)
            return Unit("w3_%d" % j, [(lambda k=k: (n2_v[R, C(k)], w3_v[C(n), C(k)])) for k in range(NT)],
                        epi, 128, 160, nt=True, acc=True)
        hs = halves(j, 128)
        main = [unit(n, R) for n in range(FT - 1) for R in hs]
        F0, part, r0 = (FT - 1) * 128, [], hs[1].start
        main[-1].tiles.pop(0)

        def epi(p):
            for i, R in enumerate(hs):
                a_v[loc(R), F0:F] = _gelu2(part[i] + p[i]).T.astype(BF16)
            main[-1].res = [jnp.concatenate(p[2:], axis=0)]
        rem = [Unit("w3_%d" % j, [(lambda k=k, R=R: (w3_v[F0:F, C(k)], n2_v[R, C(k)])) for k in range(NT - 1)],
                    lambda p: part.append(p[0]), 64, 24, nt=True, acc=True) for R in hs]
        rem.append(Unit("w3_%d" % j, [(lambda R=R: (w3_v[F0:F, C(NT - 1)], n2_v[R, C(NT - 1)])) for R in hs]
                        + [(lambda r=r: (n2_v[r:r + 64, C(0)], w3_v[C(FT - 2), C(0)])) for r in (r0, r0 + 64)],
                        epi, 64, 120, nt=True))
        return _flat(main), _flat(rem)

    outs = []

    def mm4(j, M=MS[3]):
        def unit(n, R):
            def epi(p):
                gb = mod_v[5, 0:1, C(n)]
                o_v[R, C(n)] = (x_v[R, C(n)] + gb * (x1_v[R, C(n)] + p[0] * G_POST)).astype(BF16)
                if j == NB - 1:
                    outs.append(cp(o_v.at[R, C(n)], o_hbm.at[R, C(n)], sem_o.at[0]))
                    outs[-1].start()
                elif n == NT - 1 and R.stop % T == 0:
                    outs.append(cp(o_v.at[rows(j)], o_hbm.at[rows(j)], sem_o.at[0]))
                    outs[-1].start()
            return Unit("w4_%d" % j, [(lambda k=k: (a_v[loc(R), C(k)], w4_v[C(k), C(n)])) for k in range(FT)],
                        epi, M, M // 8 * 18, acc=True)
        return [unit(n, R) for n in range(NT) for R in halves(j, M)]

    W = lambda nm: [("wait", nm)]
    run = lambda fns: [("run", "run", lambda: [fn(None) for fn in fns])]

    one = lambda us: [_flat([u]) for u in us]
    seq, grp = [], []
    for s in range(NC):
        seq += W("c%d" % s) + _flat((mmI(s - 2) if s >= 2 else []) + mmK(s) + mmU(s))
        grp.append(Group("kv%d" % s, kv(s), 50, ["c%d" % s], ["U%d" % s], 100))
        if s + 1 < NC:
            grp.append(Group("mac%d" % s, mac(s), 6 * s + 12, ["c%d" % (s + 1)],
                             ["c%d" % (s + 2) if s + 2 < NC else "I%d" % s], 0))
    grp.append(Group("mac%d" % (NC - 1), mac(NC - 1), 6 * NC + 6, ["U%d" % (NC - 1)], ["I%d" % (NC - 1)], 0))
    seq += _flat(mmI(NC - 2) + mmI(NC - 1))
    seq += W("wma") + _flat(mod("moda", 0, 3)) + run(fa2(0) + fa2(1))
    seq += W("wmb") + _flat(mod("modb", 3, 5)) + run(fc2(0) + fc2(1))
    seq += W("w1") + _flat(mm1(0))
    _wait(seq, "q2")
    seq += _flat(mm1(1)) + run(shift(0))
    seq += W("w2") + _flat(mm2(0) + mm1(2)) + run(shift(1)) + _flat(mm2(1))
    grp.append(Group("f2", fa(2) + fb(2) + fc(2), 80, ["q2"], ["w1_2"], 450))
    grp.append(Group("ln2_0", ln2(0), 60, ["w2_0"], ["w3"], 450))
    _wait(seq, "w3")
    for j in range(2):
        a, r = mm3(j)
        _mix(seq, a, [r])
        seq += _flat(mm1(3)) if j == 0 else []
    grp.append(Group("f3", fa(3) + fb(3) + fc(3), 80, ["w3"], ["w1_3"], 450))
    grp.append(Group("ln2_1", ln2(1), 60, ["w2_1"], ["w3_1"], 450))
    mc = _flat(mod("modc", 5, 6))
    _wait(seq, "w4", mc[:1] + [("sync", "run", lambda: None)])
    _mix(seq, _flat(mm2(2)), [mc[i:i + 4] for i in range(1, 25, 4)])
    _mix(seq, _flat(mm4(0)), one(mmK(4)) + one(mmU(4)), 0.0, 0.6)
    seq += _flat(mm4(1))
    grp.append(Group("kv4", kv(4), 50, ["w4"], ["U4"], 450))
    _wait(seq, "rest")
    for j in range(2, NB):
        s = j + 3
        w4 = mm4(j)
        a, r = mm3(j)
        _mix(seq, a, [_flat(mmI(j + 2) if j + 2 < NB else []) + r] + (one(mmK(s)) + one(mmU(s)) if s < NB else []))
        if j + 2 < NB:
            seq += _flat(mm1(j + 2) + w4[:len(w4) * 2 // 5] + mm2(j + 1) + w4[len(w4) * 2 // 5:])
        elif j + 1 < NB:
            seq += _flat(mm2(j + 1) + w4)
        else:
            seq += _flat(w4)
        if s < NB:
            grp.append(Group("kv%d" % s, kv(s), 50, ["rest", "U%d" % (s - 2)], ["U%d" % s], 450))
    assert _phase(seq) == 0
    for s in range(4, NB):
        grp.append(Group("mac%d" % s, mac(s), 6 * s + 12, ["U%d" % s, "K%d" % s], ["I%d" % s], 450))
        grp.append(Group("f%d" % s, fa(s) + fb(s) + fc(s), 80, ["I%d" % s], ["w1_%d" % s], 450))
    for j in range(2, NB):
        grp.append(Group("shift%d" % j, shift(j), 14, ["w1_%d" % min(j + 1, NB - 1)], ["w2_%d" % j], 200))
        grp.append(Group("ln2_%d" % j, ln2(j), 60, ["w2_%d" % j], ["w3_%d" % j], 450))
    _emit(seq, grp, zero, wait)
    with scope("wait_out"):
        for c in outs:
            c.wait()


@jax.jit
def pallas_adaLN_cond__ssm_conv_h3__mixer_s_mlp__prompt_kernel(A_q, A_k, A_v, A_shift_k, A_ssm_k, A_ssm_D, B_x, B_w1, B_w2, B_w3, B_w4, c, w_mod):
    any_ = pl.BlockSpec(memory_space=pl.ANY)
    V = pltpu.VMEM
    out = pl.pallas_call(
        kernel,
        in_specs=[any_] * 12,
        out_specs=any_,
        out_shape=jax.ShapeDtypeStruct((S, D), BF16),
        scratch_shapes=[
            V((S // 2, D), U32), V((NT, 8 + S // 2, 128), U32), V((S // 2, D), U32), V((D // 2, S), U32),
            V((D // 2, D), U32), V((D // 2, D), U32), V((F // 2, D), U32), V((F // 2, D), U32),
            V((D // 2, 6 * D), U32), V((S, D), BF16),
            V((4, D), BF16), V((D,), BF16), V((1, D), BF16), V((8, 128), I32), pltpu.SMEM((8, 128), I32),
            V((5, 8, D), F32), V((6, 8, D), F32), V((T // 2, 4 * H), U32), V((GR // 2, 2 * T), U32),
            V((NB, 3 * T + 8, D), F32), V((2, 2 * T, D), F32), V((NB, 3 * T + 8, D), F32),
            V((2, T // 2, D), U32), V((2, T, D), U32), V((NT, S + 8, 128), F32),
            V((S, D), F32), V((S, D), F32), V((S, D), F32),
            V((S // 2, D), U32), V((S // 2, D), U32), V((S // 2, D), U32), V((NT, S + 16, 128), F32),
            V((T, (FT + 1) * 128), U32),
            pltpu.SemaphoreType.DMA((13,)), pltpu.SemaphoreType.DMA((1,)),
        ],
        compiler_params=pltpu.CompilerParams(vmem_limit_bytes=110 << 20, disable_semaphore_checks=True),
        name="fused",
    )(A_q[0], A_k[0], A_v[0], A_shift_k.T, A_ssm_k, A_ssm_D, B_w1, B_w2, B_w3.T, B_w4, c, w_mod)
    return out[None]
```

```python
import contextlib
import heapq
import numpy as np
import jax
import jax.numpy as jnp
from jax import lax
from jax.experimental import pallas as pl
from jax.experimental.pallas import tpu as pltpu

S, D, F = 2048, 640, 1728
T = 256
H = T // 2
NB = S // T
NT = D // 128
FT = (F + 127) // 128
EPS = 1e-5
F32, BF16, U32, I32 = jnp.float32, jnp.bfloat16, jnp.uint32, jnp.int32
G_C1 = 0.044715 * float(np.sqrt(2.0 / np.pi))
G_C2 = float(np.sqrt(2.0 / np.pi))
G_A = G_C1 ** (1.0 / 3.0)
G_B = G_C2 / G_A
G_POST = 0.5 / G_A
RG = 16
GR = 80
NC = 3
VERBOSE = False
SCOPES = False
SLOT = 32
LP = (0.95, 4, 6)


def _unzip(p):
    return (p & -16) | ((p & 1) << 3) | ((p >> 1) & 7)


def _dft(shape, f_axis, tau, scale=1.0):
    r = lax.broadcasted_iota(I32, shape, f_axis)
    l = lax.broadcasted_iota(I32, shape, 1 - f_axis)
    if f_axis == 1:
        r = _unzip(r)
    f = r & 127
    odd = ((f & 63) << 2) | ((f >> 6) << 1) | 1
    p = odd * tau(l) + ((r >> 7) << 8)
    a = ((p + 512) & 1023) - 512
    u = (256 - jnp.abs(a)).astype(F32) * (np.pi / 512.0)
    u2 = u * u
    c = [scale, -scale / 6.0, scale / 120.0, -scale / 5040.0, scale / 362880.0, -scale / 39916800.0]
    poly = c[5]
    for ci in c[4::-1]:
        poly = poly * u2 + ci
    return (u * poly).astype(BF16)


def _ln(x, scale=1.0):
    m = jnp.sum(x, axis=-1, keepdims=True) * (1.0 / D)
    xc = x - m
    s2 = 1.0 / (scale * scale)
    v = jnp.sum(xc * xc, axis=-1, keepdims=True) * (s2 / D) + EPS * s2
    r = jnp.exp2(jnp.log(v) * float(-0.5 / np.log(2.0)))
    return xc * r


def _gelu2(x):
    u = x * (x * x + G_B)
    return x * (1.0 + jnp.tanh(u))


def _lo(w):
    return pltpu.bitcast(w << 16, F32)


def _hi(w):
    return pltpu.bitcast(w & jnp.uint32(0xFFFF0000), F32)


def _pack(a, b):
    return pltpu.pack_elementwise([a, b], packed_dtype=BF16)


def _tie(x, a):
    if a is None:
        return x
    w = pltpu.bitcast(x[:, :128], U32)
    k = w.shape[0] // 8
    w = w | (a if k == 1 else jnp.concatenate([a] * k, axis=0))
    w = pltpu.bitcast(w, x.dtype)
    return w if x.shape[1] == 128 else jnp.concatenate([w, x[:, 128:]], axis=1)


def C(i, lim=F):
    return slice(i * 128, min((i + 1) * 128, lim))


class Unit:
    def __init__(self, name, tiles, epi, rows, cost, nt=False, full=True, acc=False):
        self.acc, self.res = acc, []
        self.name, self.tiles, self.epi, self.rows, self.cost, self.nt, self.full = name, tiles, epi, rows, cost, nt, full


class Group:
    def __init__(self, name, fns, cost, rel, dead, lat, rlat=200):
        self.name, self.fns, self.cost, self.rel, self.dead, self.lat, self.rlat = name, fns, cost, rel, dead, lat, rlat


def _plan(seq, groups):
    busy, n = [0] * 4, 0
    start, end, tiles, bars = {}, {}, [], []
    for it in seq:
        if isinstance(it[0], Unit):
            u = it[0]
            m = n % 4
            n += 1
            t0, t1 = busy[m], busy[m] + max(u.rows, 32)
            busy[m] = t1
            tiles.append((t0, t1, u.cost / len(u.tiles)))
            start.setdefault(u.name, t0)
            end[u.name] = max(end.get(u.name, 0), t1)
        elif it[0] == "wait":
            t = max(busy)
            busy, n = [t] * 4, 0
            start[it[1]] = end[it[1]] = t
            bars.append(t)
    total = max(busy)
    start["end"] = end["end"] = total
    start["start"] = end["start"] = 0
    ns = total // SLOT + 2
    load = np.zeros(ns)
    for t0, t1, c in tiles:
        a, b = t0 // SLOT, max(t1 // SLOT, t0 // SLOT + 1)
        load[a:b] += c / (b - a)
    win = []
    for g in groups:
        r = max(end[x] + (0 if start[x] == end[x] else g.rlat) for x in g.rel)
        d = min(start[x] for x in g.dead) - g.lat
        ok = np.zeros(ns, bool)
        ok[r // SLOT:max(d // SLOT, r // SLOT + 1)] = True
        for b in bars:
            if r < b <= d:
                ok[max((b - g.lat) // SLOT, 0):b // SLOT] = False
        win.append(np.nonzero(ok)[0])
    alloc = [np.zeros(len(w)) for w in win]
    for _ in range(60):
        for i, g in enumerate(groups):
            w = win[i]
            load[w] -= alloc[i]
            base = load[w]
            vol = g.cost * len(g.fns)
            lo, hi = base.min(), base.max() + vol
            for _ in range(50):
                mid = 0.5 * (lo + hi)
                if np.maximum(mid - base, 0).sum() > vol:
                    hi = mid
                else:
                    lo = mid
            alloc[i] = np.maximum(hi - base, 0)
            load[w] += alloc[i]
    times = []
    for i, g in enumerate(groups):
        cum = np.cumsum(alloc[i])
        ts = []
        for k in range(len(g.fns)):
            x = (k + 0.5) * cum[-1] / len(g.fns)
            j = int(np.searchsorted(cum, x))
            prev = cum[j - 1] if j else 0.0
            ts.append(win[i][j] * SLOT + SLOT * (x - prev) / max(alloc[i][j], 1e-9))
        times.append(ts)
        if VERBOSE:
            print("%8s window %6d..%6d used %6d..%6d" % (g.name, win[i][0] * SLOT, win[i][-1] * SLOT, ts[0], ts[-1]))
    if VERBOSE:
        k = 2048 // SLOT
        print("total", total, "load/cycle:", " ".join("%.1f" % (load[i:i + k].mean() / SLOT) for i in range(0, ns, k)))
    return times


def _emit(seq, groups, zero, wait):
    times = _plan(seq, groups)
    left = {"start": 0}
    for it in seq:
        nm = it[0].name if isinstance(it[0], Unit) else it[1]
        left[nm] = left.get(nm, 0) + 1
    heap, pend, todo, cnt = [], {}, list(range(len(groups))), 0
    busy, n = [0] * 4, 0

    def release():
        nonlocal cnt
        for i in list(todo):
            g = groups[i]
            if all(left[x] == 0 for x in g.rel):
                todo.remove(i)
                pend[i] = len(g.fns)
                for t, fn in zip(times[i], g.fns):
                    heapq.heappush(heap, (t, cnt, i, fn))
                    cnt += 1

    def force(name):
        nonlocal heap
        for i, g in enumerate(groups):
            if name in g.dead:
                assert i not in todo, (g.name, name)
                if pend[i]:
                    if VERBOSE:
                        print("forcing", g.name, pend[i], "before", name)
                    for it in sorted(x for x in heap if x[2] == i):
                        it[3](None)
                    heap = [x for x in heap if x[2] != i]
                    heapq.heapify(heap)
                    pend[i] = 0

    release()
    for it in seq:
        if isinstance(it[0], Unit):
            u, k = it
            force(u.name)
            lhs, rhs = u.tiles[k]()
            dn = (((1,), (1 if u.nt else 0,)), ((), ()))
            p = lax.dot_general(lhs, rhs, dn, preferred_element_type=F32)
            u.res = [p + u.res[0]] if (u.acc and u.res) else u.res + [p]
            m = n % 4
            n += 1
            t0 = busy[m]
            busy[m] = t0 + max(u.rows, 32)
            while u.full and heap and heap[0][0] < t0 + u.rows:
                t, _, i, fn = heapq.heappop(heap)
                pend[i] -= 1
                r = min(max(int(t - t0), 0), u.rows - 1) // 8 * 8
                fn(pltpu.bitcast(p[r:r + 8], U32) & zero)
            if k == len(u.tiles) - 1:
                u.epi(u.res)
            left[u.name] -= 1
        elif it[0] == "wait":
            force(it[1])
            wait(it[1])
            busy, n = [max(busy)] * 4, 0
            left[it[1]] -= 1
        else:
            it[2]()
            left[it[1]] -= 1
        release()
    force("end")
    assert not heap and not todo


def _sum(ps):
    acc = ps[0]
    for p in ps[1:]:
        acc = acc + p
    return acc


def _flat(us):
    return [(u, i) for u in us for i in range(len(u.tiles))]


def _phase(seq):
    n = 0
    for it in seq:
        n = n + 1 if isinstance(it[0], Unit) else (0 if it[0] in ("wait", "sync") else n)
    return n % 4


def _mix(seq, a, b, lo=0.0, hi=1.0):
    n, k = _phase(seq), 0
    for i, t in enumerate(a):
        if k < len(b) and n % 4 == 0 and t[1] != 1 and i >= len(a) * (lo + (hi - lo) * k / len(b)):
            seq.extend(b[k])
            k += 1
        seq.append(t)
        n += 1
    assert k == len(b)


def _wait(seq, name, head=()):
    r = _phase(seq)
    assert all(isinstance(it[0], Unit) for it in seq[len(seq) - r:])
    seq[len(seq) - r:len(seq) - r] = [("wait", name)] + list(head)


def kernel(q_hbm, k_hbm, v_hbm, sh_hbm, ssm_hbm, sd_hbm, w1_hbm, w2_hbm, w3_hbm, w4_hbm, c_hbm, wm_hbm,
           o_hbm,
           q_w, k_n, v_w, ssm_w, w1_w, w2_w, w3_w, w4_w, wm_w, o_v,
           sh_v, sd_v, c_v, zsrc, z_s, taps, mod_v, tf_w, tg_w,
           kf, uf, acc, zraw, kv_w, zz_w, y_v, x_v, hb_v, x1_v, r_v, n1_w, n2_w, g_w, h1_v, a_w,
           sem, sem_b, sem_o):
    bf = lambda r: r.bitcast(BF16)
    w1_v, w2_v, w3_v, w4_v, wm_v = bf(w1_w), bf(w2_w), bf(w3_w), bf(w4_w), bf(wm_w)
    tf_v, tg_v, kv_v, zz_v, n1_v, n2_v, g_v = bf(tf_w), bf(tg_w), bf(kv_w), bf(zz_w), bf(n1_w), bf(n2_w), bf(g_w)
    q_v, a_v = bf(q_w), bf(a_w)
    cp = pltpu.make_async_copy
    scope = lambda nm: jax.named_scope(nm) if SCOPES else contextlib.nullcontext()

    def base(j, n):
        return j * n if isinstance(j, int) else pl.multiple_of(j * n, n)

    def rows(j, n=1, size=T):
        return pl.ds(base(j, size), n * size)

    def view(ref, j, size=T):
        return ref.at[rows(j, 1, size)]

    dmas = {}

    def group(name, *mks):
        sm = sem.at[len(dmas)]
        dmas[name] = [c for mk in mks for c in mk(sm)]

    def ssm_in(s, n=1):
        return lambda sm: [cp(ssm_hbm.at[:, rows(s, n)], bf(ssm_w).at[:, rows(s, n)], sm)]

    def kv_in(s):
        return lambda sm: ([cp(k_hbm.at[rows(s), C(t)], bf(k_n).at[t, pl.ds(16 + base(s, T), T)], sm) for t in range(NT)]
                           + [cp(v_hbm.at[rows(s)], bf(v_w).at[rows(s)], sm)])

    def q_in(s, n=1):
        return lambda sm: [cp(q_hbm.at[rows(s, n)], q_v.at[rows(s, n)], sm)]

    def wm_in(a, b):
        return lambda sm: [cp(wm_hbm.at[:, a * D:b * D], wm_v.at[:, a * D:b * D], sm)]

    def whole(src, dst):
        return lambda sm: [cp(src, dst, sm)]

    def blk_in(s):
        sm = sem_b.at[s - NC]
        return kv_in(s)(sm) + q_in(s)(sm)

    zsrc[...] = jnp.zeros((8, 128), I32)
    k_n[:, 0:8, :] = jnp.zeros((NT, 8, 128), U32)
    group("small", lambda sm: [cp(zsrc, z_s, sm), cp(sh_hbm, sh_v, sm), cp(sd_hbm, sd_v, sm), cp(c_hbm, c_v, sm)])
    for s in range(NC):
        group("c%d" % s, ssm_in(s), kv_in(s))
    group("kr", ssm_in(NC, NB - NC))
    group("wma", wm_in(0, 3), q_in(0, 2))
    group("wmb", wm_in(3, 5))
    group("w1", whole(w1_hbm, w1_v))
    group("q2", q_in(2))
    group("w2", whole(w2_hbm, w2_v))
    group("w3", whole(w3_hbm, w3_v))
    group("w4", whole(w4_hbm, w4_v), wm_in(5, 6))
    for g in dmas.values():
        for c in g:
            c.start()

    def wait(name):
        with scope("wait_" + name):
            for c in dmas[name]:
                c.wait()

    tau_b = lambda l: H + ((l + (H - 1)) & (H - 1))
    tf_v[:, C(0)] = _dft((T, H), 0, lambda l: jnp.where((l & 1) == 0, l, tau_b(l)), 1.0 / T)
    tf_v[:, C(1)] = _dft((T, H), 0, lambda l: jnp.where((l & 1) == 1, l, tau_b(l)), 1.0 / T)
    tf_v[:, C(2)] = _dft((T, H), 0, lambda l: 2 * _unzip(l) - H)
    tf_v[:, C(3)] = _dft((T, H), 0, lambda l: 2 * _unzip(l) + 1 - H)
    sin0 = lax.broadcasted_iota(I32, (GR, T), 1) >= H
    tg_v[:, 0:T] = _dft((GR, T), 1, lambda l: jnp.where(sin0 & (l == 0), H, 2 * l))
    tg_v[:, T:2 * T] = _dft((GR, T), 1, lambda l: 2 * l + 1)
    h1_v[:, 0:8, :] = jnp.zeros((NT, 8, 128), F32)
    h1_v[:, 8 + S:16 + S, :] = jnp.zeros((NT, 8, 128), F32)

    wait("small")
    z = jnp.clip(z_s[0, 0], 0, 1)
    zero = jnp.full((8, 128), z, I32).astype(U32)
    z8 = pl.multiple_of(z * 8, 8)
    for r in (r_v, zraw, n1_w, n2_w, g_w, a_w):
        r[pl.ds(z8, 8), 0:128] = jnp.zeros((8, 128), r.dtype)
    for r in (kf, uf, acc, kv_w, zz_w, taps, mod_v):
        r[z, 0:8, 0:128] = jnp.zeros((8, 128), r.dtype)
    for r in (tf_w, tg_w):
        r[pl.ds(z8, 8), 0:128] = r[0:8, 0:128]
    sh = sh_v[...].astype(F32)
    for i in range(4):
        taps[i] = jnp.broadcast_to(sh[i:i + 1], (8, D))
    taps[4] = jnp.broadcast_to(sd_v[...].astype(F32).reshape(1, D) * (1.0 / T), (8, D))
    cf = c_v[...].astype(F32)
    silu_c = jnp.broadcast_to((cf / (1.0 + jnp.exp(-cf))).astype(BF16), (16, D))

    def mmK(m):
        def unit(n):
            W = slice(64 * n, 64 * (n + 1))
            st = []

            def rhs(i):
                if not st:
                    ev = (lax.broadcasted_iota(I32, (64, 128), 1) & 1) == 0
                    a = ssm_w[W, m * T:m * T + H]
                    b = pltpu.roll(ssm_w[W, m * T + H:(m + 1) * T], 1, 1)
                    st.extend([pltpu.bitcast(jnp.where(ev, a, b), BF16), pltpu.bitcast(jnp.where(ev, b, a), BF16)])
                return st[i]

            def epi(p):
                er, ei, or_, oi = p
                if m == 0:
                    er = er + taps[4, 0:1, C(n)]
                for h, (cr, ci) in enumerate(((er + or_, ei + oi), (er - or_, ei - oi))):
                    B = h * 3 * H
                    kf[m, B:B + H, C(n)] = cr
                    kf[m, B + H:B + 2 * H, C(n)] = ci - cr
                    kf[m, B + 2 * H:B + 3 * H, C(n)] = ci + cr
            return Unit("K%d" % m, [(lambda i=i, r=r: (tf_v[r:r + H, C(i)], rhs(i))) for i in range(2) for r in (0, H)],
                        epi, H, 170, nt=True)
        return [unit(n) for n in range(NT)]

    def kv(s, sl):
        vv, b0 = view(v_w, s, H), base(s, H)

        def mk(t, w):
            def fn(a):
                ld = lambda o, n: k_n[t, pl.ds(b0 + (8 + w + o), n), :]
                c0 = jnp.concatenate([_tie(ld(0, 8), a), ld(8, 8)], axis=0).reshape(2, 8, 128)
                c1, c2 = ld(-1, 16).reshape(2, 8, 128), ld(-2, 16).reshape(2, 8, 128)
                s0, s1, s2, s3 = (taps[i, :, C(t)] for i in range(4))
                ke, ko, ke1, ko1, ko2 = _lo(c0), _hi(c0), _lo(c1), _hi(c1), _hi(c2)
                wv = vv[w:w + 16, C(t)].reshape(2, 8, 128)
                kve = ((s0 * ke + s1 * ko1) + (s2 * ke1 + s3 * ko2)) * _lo(wv)
                kvo = ((s0 * ko + s1 * ke) + (s2 * ko1 + s3 * ke1)) * _hi(wv)
                kv_w[sl, w // 2:w // 2 + 8, C(t)] = _pack(kve[0], kve[1])
                kv_w[sl, (H + w) // 2:(H + w) // 2 + 8, C(t)] = _pack(kvo[0], kvo[1])
            return fn
        return [[mk(t, w) for w in range(0, H, 16)] for t in range(NT)]

    def mmU(name, sl, us):
        def unit(n):
            def epi(p):
                er, ei, or_, oi = p
                for h, (cr, ci) in enumerate(((er + or_, ei + oi), (er - or_, ei - oi))):
                    B = h * 3 * H
                    uf[us, B:B + H, C(n)] = cr + ci
                    uf[us, B + H:B + 2 * H, C(n)] = cr
                    uf[us, B + 2 * H:B + 3 * H, C(n)] = ci
            return Unit(name(n), [(lambda i=i, r=r: (tf_v[r:r + H, C(2 + i)], kv_v[sl, C(i), C(n)]))
                                  for i in range(2) for r in (0, H)], epi, H, 120)
        return [unit(n) for n in range(NT)]

    def cmul(m0, u0, n, h, row, L, a):
        t = []
        for i in range(3):
            Rw = slice((3 * h + i) * H + row, (3 * h + i) * H + row + 8)
            kk = kf[m0:m0 + n, Rw, L]
            if i == 0 and a is not None:
                k0 = _tie(kk[0], a)[None]
                kk = k0 if n == 1 else jnp.concatenate([k0, kk[1:]], axis=0)
            t.append(jnp.sum(kk * uf[u0:u0 + n, Rw, L], axis=0))
        return t[0] - t[2], t[0] + t[1]

    def AR(h, q, row):
        return slice((2 * h + q) * H + row, (2 * h + q) * H + row + 8)

    def mac(n, u0, sl, first=False, part=False):
        def mk(t, rc):
            st, fin = [], []

            def piece(i):
                def fn(a):
                    h, row = i & 1, rc + (i >> 1) * 8
                    zr, zi = cmul(0, u0, n, h, row, C(t), a)
                    if part:
                        zr, zi = zr + acc[0, AR(h, 0, row), C(t)], zi + acc[0, AR(h, 1, row), C(t)]
                    st.append((zr, zi))
                    if h:
                        (pr, pi), (mr, mi) = st[-2:]
                        z = [pr + mr, pi + mi, pr - mr, pi - mi]
                        Rw = lambda q: slice(q * H + row, q * H + row + 8)
                        pv = None if first else [zraw[Rw(q ^ 1), C(t)] for q in range(4)]
                        for q in range(4):
                            zraw[Rw(q), C(t)] = z[q]
                        if not first:
                            z = [z[q] + pv[q] if (q & 1) == (rc < 64) else z[q] - pv[q] for q in range(4)]
                        fin.append(z)
                    if i == 3:
                        for q in range(4):
                            w = (q * H + rc) // 2
                            zz_w[sl, w:w + 8, C(t)] = _pack(fin[0][q], fin[1][q])
                return fn
            if not part:
                return [piece(i) for i in range(4)]
            both = lambda f, g: (lambda a: (f(a), g(None)))
            return [both(piece(0), piece(1)), both(piece(2), piece(3))]
        return [[fn for rc in range(0, H, 16) for fn in mk(t, rc)] for t in range(NT)]

    def pos():
        return [(t, h, row) for t in range(NT) for row in range(0, H, 8) for h in range(2)]

    def ahead(i):
        def mk(t, h, row):
            def fn(a):
                zr, zi = cmul(i + 1, 0, NC, h, row, C(t), a)
                acc[i, AR(h, 0, row), C(t)] = zr
                acc[i, AR(h, 1, row), C(t)] = zi
            return fn
        return [mk(*p) for p in pos()]

    def spread():
        n = NB - NC - 1

        def mk(t, h, row):
            def fn(a):
                p = []
                for i in range(3):
                    Rw = slice((3 * h + i) * H + row, (3 * h + i) * H + row + 8)
                    u = uf[0, Rw, C(t)]
                    p.append(kf[1:1 + n, Rw, C(t)] * (_tie(u, a) if i == 0 else u)[None])
                acc[0:n, AR(h, 0, row), C(t)] = acc[1:1 + n, AR(h, 0, row), C(t)] + (p[0] - p[2])
                acc[0:n, AR(h, 1, row), C(t)] = acc[1:1 + n, AR(h, 1, row), C(t)] + (p[0] + p[1])
            return fn
        return [mk(*p) for p in pos()]

    def mmI(name, sl, ys):
        def unit(n):
            def epi(p):
                ce, se, co, so = p
                sub = lax.broadcasted_iota(I32, (8, 128), 0)
                c0 = ys * T + H
                y_v[n, ys * T:ys * T + 1, :] = (ce[64:72] - se[0:8])[0:1]
                se = jnp.concatenate([jnp.where(sub == 0, 0.0, se[0:8]), se[8:]], axis=0)
                for d, cc, ss in ((0, ce[0:64], se), (1, co, so)):
                    y_v[n, pl.ds(c0 + d, 64, stride=2), :] = cc + ss
                    lo = cc - ss
                    for i in range(0, 64, 8):
                        y_v[n, pl.ds(c0 - d - 2 * i - 14, 8, stride=2), :] = jnp.take_along_axis(
                            lo[i:i + 8], 7 - sub, axis=0)
            return Unit(name(n), [(lambda i=i: (tg_v[0:(GR if i == 0 else 64), C(i)], zz_v[sl, C(i), C(n)]))
                                  for i in range(4)], epi, 64, 52)
        return [unit(n) for n in range(NT)]

    def mod(name, a, b):
        def unit(n):
            def epi(p):
                v = [_sum(p[i * NT:(i + 1) * NT])[0:8] for i in range(b - a)]
                if a == 0:
                    mod_v[0, :, C(n)] = v[0] * v[2]
                    mod_v[1, :, C(n)] = (v[1] + 1.0) * v[2]
                elif a == 3:
                    mod_v[3, :, C(n)] = v[0]
                    mod_v[4, :, C(n)] = v[1] + 1.0
                else:
                    mod_v[5, :, C(n)] = v[0]
                    mod_v[2, :, C(n)] = v[0] * G_POST
            return Unit(name, [(lambda i=i, k=k: (silu_c[:, C(k)], wm_v[C(k), i * D + n * 128:i * D + (n + 1) * 128]))
                               for i in range(a, b) for k in range(NT)], epi, 16, 10, full=False, acc=b - a == 1)
        return [unit(n) for n in range(NT)]

    GS = range(0, T, RG)
    HS = (slice(0, 128), slice(128, 256))

    def tasks(f):
        return [(lambda a, r=r: f(slice(r, r + RG), a)) for r in GS]

    def load_y(sl, R):
        return jnp.concatenate([y_v[t, sl * T + R.start:sl * T + R.stop, :] for t in range(NT)],
                               axis=1).reshape(2, 8, D)

    def front(j, sl, early=False):
        qq, xx, hh, nn = view(q_w, j, H), view(x_v, j), view(hb_v, j), view(n1_v, sl)

        def fa(R, a):
            q = pltpu.bitcast(_tie(qq[R.start // 2:R.stop // 2, :], a), BF16).astype(F32).reshape(2, 8, D)
            x = (q + (_ln(q) * mod_v[1] + mod_v[0]) * load_y(sl, R)).reshape(RG, D)
            xx[R, :] = x
            if early:
                hh[R, :] = _ln(x)

        def fb(R, a):
            hh[R, :] = (_ln(_tie(xx[R, :], a).reshape(2, 8, D)) * mod_v[4] + mod_v[3]).reshape(RG, D)

        def fc(R, a):
            hb = _tie(hh[R, :], a)
            if early:
                hb = (hb.reshape(2, 8, D) * mod_v[4] + mod_v[3]).reshape(RG, D)
                hh[R, :] = hb
            nn[R, :] = _ln(hb, G_A).astype(BF16)
        return (tasks(fa), tasks(fc)) if early else tasks(fa) + tasks(fb) + tasks(fc)

    def shift(j, sl):
        SR = 64
        gg, b0 = view(g_v, sl), base(j, T)

        def mk(t, r):
            def fn(a):
                lane = lax.broadcasted_iota(I32, (SR, 128), 1)
                ld = lambda d: h1_v[t, pl.ds(b0 + (8 + r + d), SR), :]
                if t == 0:
                    g = ld(-1)
                elif t == 1:
                    g = jnp.where(lane < 32, ld(-1), ld(1))
                elif t == 2:
                    g = jnp.where(lane < 64, ld(1), ld(-2))
                elif t == 3:
                    g = jnp.where(lane < 96, ld(-2), ld(2))
                else:
                    g = ld(2)
                if a is not None:
                    g = jnp.concatenate([_tie(g[i:i + 8], a) if i % 16 == 0 else g[i:i + 8]
                                         for i in range(0, SR, 8)], axis=0)
                gg[r:r + SR, C(t)] = g.astype(BF16)
            return fn
        return [mk(t, r) for t in range(NT) for r in range(0, T, SR)]

    def ln2(j, sl):
        xx, nn = view(x1_v, j), view(n2_v, sl)

        def f(R, a):
            nn[R, :] = _ln(_tie(xx[R, :], a), G_A).astype(BF16)
        return tasks(f)

    def resid(j):
        xx, x1 = view(x_v, j), view(x1_v, j)

        def f(R, a):
            gb = mod_v[5] if a is None else pltpu.bitcast(
                pltpu.bitcast(mod_v[5], U32) | jnp.concatenate([a] * NT, axis=1), F32)
            r_v[R, :] = xx[R, :] + (x1[R, :].reshape(4, 8, D) * gb).reshape(2 * RG, D)
        return [(lambda a, r=r: f(slice(r, r + 2 * RG), a)) for r in range(0, T, 2 * RG)]

    def mm1(name, j, sl):
        nn, b0 = view(n1_v, sl), base(j, T)

        def unit(n, R):
            def epi(p):
                h1_v[n, pl.ds(b0 + (8 + R.start), 128), :] = _gelu2(p[0])
            return Unit(name, [(lambda k=k: (nn[R, C(k)], w1_v[C(k), C(n)])) for k in range(NT)],
                        epi, 128, 144, acc=True)
        return [unit(n, R) for n in range(NT) for R in HS]

    def mm2(name, j, sl):
        gg, hh, x1 = view(g_v, sl), view(hb_v, j), view(x1_v, j)

        def unit(n, R):
            def epi(p):
                x1[R, C(n)] = hh[R, C(n)] + p[0] * G_POST
            return Unit(name, [(lambda k=k: (gg[R, C(k)], w2_v[C(k), C(n)])) for k in range(NT)],
                        epi, 128, 96, acc=True)
        return [unit(n, R) for n in range(NT) for R in HS]

    def mm3(name, sl):
        nn, aa = view(n2_v, sl), view(a_v, sl)

        def unit(n, R):
            def epi(p):
                aa[R, C(n)] = _gelu2(p[0]).astype(BF16)
            return Unit(name, [(lambda k=k: (nn[R, C(k)], w3_v[C(n), C(k)])) for k in range(NT)],
                        epi, 128, 160, nt=True, acc=True)
        main = [unit(n, R) for n in range(FT - 1) for R in HS]
        F0, part = (FT - 1) * 128, []
        main[-1].tiles.pop(0)

        def epi(p):
            for i, R in enumerate(HS):
                aa[R, F0:F] = _gelu2(part[i] + p[i]).T.astype(BF16)
            main[-1].res = [jnp.concatenate(p[2:], axis=0)]
        rem = [Unit(name, [(lambda k=k, R=R: (w3_v[F0:F, C(k)], nn[R, C(k)])) for k in range(NT - 1)],
                    lambda p: part.append(p[0]), 64, 24, nt=True, acc=True) for R in HS]
        rem.append(Unit(name, [(lambda R=R: (w3_v[F0:F, C(NT - 1)], nn[R, C(NT - 1)])) for R in HS]
                        + [(lambda r=r: (nn[r:r + 64, C(0)], w3_v[C(FT - 2), C(0)])) for r in (128, 192)],
                        epi, 64, 120, nt=True))
        return _flat(main), _flat(rem)

    def cp_out(j):
        return cp(o_v.at[rows(j)], o_hbm.at[rows(j)], sem_o.at[0])

    last = []

    def mm4(name, j, sl, pre=False):
        aa, oo, xx, x1 = view(a_v, sl), view(o_v, j), view(x_v, j), view(x1_v, j)

        def unit(n, R):
            def epi(p):
                if pre:
                    oo[R, C(n)] = (r_v[R, C(n)] + mod_v[2, 0:1, C(n)] * p[0]).astype(BF16)
                    return
                oo[R, C(n)] = (xx[R, C(n)] + mod_v[5, 0:1, C(n)] * (x1[R, C(n)] + p[0] * G_POST)).astype(BF16)
                if j == NB - 1:
                    Rg = slice(j * T + R.start, j * T + R.stop)
                    last.append(cp(o_v.at[Rg, C(n)], o_hbm.at[Rg, C(n)], sem_o.at[0]))
                    last[-1].start()
                elif n == NT - 1 and R.stop == T:
                    cp_out(j).start()
            return Unit(name, [(lambda k=k: (aa[R, C(k)], w4_v[C(k), C(n)])) for k in range(FT)],
                        epi, 128, 16 * (16 if pre else 18), acc=True)
        return [unit(n, R) for n in range(NT) for R in HS]

    def quarter(u):
        mk = u.tiles.pop(0)
        st = []

        def piece(i):
            if not st:
                st.extend(mk())
            return st[0][32 * i:32 * i + 32], st[1]

        def epi(p):
            u.res = [jnp.concatenate(p, axis=0)]
        return _flat([Unit(u.name, [(lambda i=i: piece(i)) for i in range(4)], epi, 32, 0, nt=u.nt)])

    W = lambda nm: [("wait", nm)]
    run = lambda fns: [("run", "run", lambda: [fn(None) for fn in fns])]
    one = lambda us: [_flat([u]) for u in us]
    cat = lambda ls: [x for l in ls for x in l]
    nm = lambda x: (lambda n: x)

    seq, grp = [], []
    for s in range(NC):
        seq += W("c%d" % s) + _flat((mmI(nm("I0"), 0, 0) if s == 2 else []) + mmK(s) + mmU(nm("U%d" % s), s % 2, NC - 1 - s))
        grp.append(Group("kv%d" % s, cat(kv(s, s % 2)), 50, ["c%d" % s], ["U%d" % s], 100))
    grp.append(Group("mac0", cat(mac(1, 2, 0, first=True)), 12, ["c1"], ["c2"], 0))
    grp.append(Group("mac1", cat(mac(2, 1, 1)), 18, ["c2"], ["kr"], 0))
    grp.append(Group("mac2", cat(mac(3, 0, 0)), 24, ["kr"], ["I2"], 300))
    seq += W("kr") + _flat(mmI(nm("I1"), 1, 1) + cat(mmK(m) for m in range(NC, NB)) + mmI(nm("I2"), 0, 2))
    seq += [("run", "run", lambda: [c.start() for s in range(NC, NB) for c in blk_in(s)])]
    f0, f1 = front(0, 0, True), front(1, 1, True)
    seq += W("wma") + _flat(mod("moda", 0, 3)) + run(f0[0] + f1[0])
    seq += W("wmb") + _flat(mod("modb", 3, 5)) + run(f0[1] + f1[1])
    seq += W("w1") + _flat(mm1("w1_0", 0, 0))
    _wait(seq, "q2")
    seq += _flat(mm1("w1_1", 1, 1)) + run(shift(0, 0))
    seq += W("w2") + _flat(mm2("w2_0", 0, 0) + mm1("w1_2", 2, 2)) + run(shift(1, 1)) + _flat(mm2("w2_1", 1, 1))
    grp.append(Group("f2", front(2, 2), 80, ["q2"], ["w1_2"], 450))
    grp.append(Group("ln2_0", ln2(0, 1), 60, ["w2_0"], ["w3"], 450))
    grp.append(Group("ln2_1", ln2(1, 0), 60, ["w2_1"], ["end"], 450))
    grp.append(Group("ahead", cat(ahead(i) for i in range(NB - NC)), 19, ["w1"], ["end"], 100))
    _wait(seq, "w3")
    a, r = mm3("w3_0", 1)
    _mix(seq, a, [r])
    mc = _flat(mod("modc", 5, 6))
    _wait(seq, "w4", mc + [("sync", "run", lambda: None)])
    w4 = mm4("w4_0", 0, 1)
    qs = [quarter(w4[-1 - i]) for i in range((_phase(seq) + 140) % 4)]
    _mix(seq, _flat(w4), qs, 0.2, 0.6)
    assert _phase(seq) == 0
    _emit(seq, grp, zero, wait)

    def step(s, carry):
        with scope("wait_blk"):
            for c in blk_in(s):
                c.wait()
        seq, grp = [], []
        a, r = mm3("w3", 0)
        us, it = one(mmU(lambda n: "U%d" % n, 0, 0)), one(mmI(lambda n: "I%d" % n, 0, 0))
        w4 = mm4("w4", s - 2, 0, pre=True)
        q = quarter(w4[-1])
        _mix(seq, a, [r, [], us[0], us[1], us[2], it[0] + us[3], it[1] + us[4], it[2], it[3], it[4]], 0.0, LP[0])
        _mix(seq, _flat(w4[:LP[1]]), [q])
        seq += _flat(mm1("w1", s, 0) + w4[LP[1]:LP[2]] + mm2("w2", s - 1, 0) + w4[LP[2]:])
        assert _phase(seq) == 0
        kvs, macs = kv(s, 0), mac(1, 0, 0, part=True)
        for t in range(NT):
            grp.append(Group("kv%d" % t, kvs[t], 50, ["start"], ["U%d" % t], 300))
            grp.append(Group("mac%d" % t, macs[t], 28, ["U%d" % t], ["I%d" % t], 300, 150))
        iall = ["I%d" % t for t in range(NT)]
        grp.append(Group("resid", resid(s - 2), 46, ["start"], ["w4", "I4"], 100))
        grp.append(Group("front", front(s, 0), 80, iall, ["w1"], 450))
        grp.append(Group("spread", spread(), 30, iall, ["end"], 100))
        grp.append(Group("shift", shift(s - 1, 0), 14, ["w1"], ["w2"], 200))
        grp.append(Group("ln2", ln2(s - 1, 0), 60, ["w2"], ["end"], 450))
        _emit(seq, grp, zero, wait)
        cp_out(s - 2).start()
        return carry

    lax.fori_loop(NC, NB, step, 0)

    seq, grp = [], []
    a, r = mm3("w3_6", 0)
    _mix(seq, a, [r])
    seq += _flat(mm2("w2_7", NB - 1, 0) + mm4("w4_6", NB - 2, 0))
    a, r = mm3("w3_7", 1)
    _mix(seq, a, [r])
    seq += _flat(mm4("w4_7", NB - 1, 1))
    assert _phase(seq) == 0
    grp.append(Group("shift7", shift(NB - 1, 0), 14, ["start"], ["w2_7"], 200))
    grp.append(Group("ln2_7", ln2(NB - 1, 1), 60, ["w2_7"], ["w3_7"], 450))
    _emit(seq, grp, zero, wait)
    with scope("wait_out"):
        for c in [cp_out(j) for j in range(NB - 1)] + last:
            c.wait()


@jax.jit
def pallas_adaLN_cond__ssm_conv_h3__mixer_s_mlp__prompt_kernel(A_q, A_k, A_v, A_shift_k, A_ssm_k, A_ssm_D, B_x, B_w1, B_w2, B_w3, B_w4, c, w_mod):
    any_ = pl.BlockSpec(memory_space=pl.ANY)
    V = pltpu.VMEM
    out = pl.pallas_call(
        kernel,
        in_specs=[any_] * 12,
        out_specs=any_,
        out_shape=jax.ShapeDtypeStruct((S, D), BF16),
        scratch_shapes=[
            V((S // 2, D), U32), V((NT, 8 + S // 2, 128), U32), V((S // 2, D), U32), V((D // 2, S), U32),
            V((D // 2, D), U32), V((D // 2, D), U32), V((F // 2, D), U32), V((F // 2, D), U32),
            V((D // 2, 6 * D), U32), V((S, D), BF16),
            V((4, D), BF16), V((D,), BF16), V((1, D), BF16), V((8, 128), I32), pltpu.SMEM((8, 128), I32),
            V((5, 8, D), F32), V((6, 8, D), F32), V((T // 2, 4 * H), U32), V((GR // 2, 2 * T), U32),
            V((NB, 3 * T + 8, D), F32), V((NC, 3 * T + 8, D), F32), V((NB - NC, 2 * T + 8, D), F32), V((2 * T, D), F32),
            V((2, T // 2, D), U32), V((2, T, D), U32), V((NT, NC * T + 8, 128), F32),
            V((S, D), F32), V((S, D), F32), V((S, D), F32), V((T, D), F32),
            V((3 * T // 2, D), U32), V((T, D), U32), V((T, D), U32), V((NT, S + 16, 128), F32),
            V((T, (FT + 1) * 128), U32),
            pltpu.SemaphoreType.DMA((12,)), pltpu.SemaphoreType.DMA((NB - NC,)), pltpu.SemaphoreType.DMA((1,)),
        ],
        compiler_params=pltpu.CompilerParams(vmem_limit_bytes=110 << 20, disable_semaphore_checks=True),
        name="fused",
    )(A_q[0], A_k[0], A_v[0], A_shift_k.T, A_ssm_k, A_ssm_D, B_w1, B_w2, B_w3.T, B_w4, c, w_mod)
    return out[None]
```

```python
import contextlib
import heapq
import numpy as np
import jax
import jax.numpy as jnp
from jax import lax
from jax.experimental import pallas as pl
from jax.experimental.pallas import tpu as pltpu

S, D, F = 2048, 640, 1728
T = 256
H = T // 2
NB = S // T
NT = D // 128
FT = (F + 127) // 128
EPS = 1e-5
F32, BF16, U32, I32 = jnp.float32, jnp.bfloat16, jnp.uint32, jnp.int32
G_C1 = 0.044715 * float(np.sqrt(2.0 / np.pi))
G_C2 = float(np.sqrt(2.0 / np.pi))
G_A = G_C1 ** (1.0 / 3.0)
G_B = G_C2 / G_A
G_POST = 0.5 / G_A
RG = 16
GR = 80
NC = 3
VERBOSE = False
SCOPES = False
SLOT = 32
LP = (0.8, 4, 6, 0.15, 72)


def _unzip(p):
    return (p & -16) | ((p & 1) << 3) | ((p >> 1) & 7)


def _dft(shape, f_axis, tau, scale=1.0):
    r = lax.broadcasted_iota(I32, shape, f_axis)
    l = lax.broadcasted_iota(I32, shape, 1 - f_axis)
    if f_axis == 1:
        r = _unzip(r)
    f = r & 127
    odd = ((f & 63) << 2) | ((f >> 6) << 1) | 1
    p = odd * tau(l) + ((r >> 7) << 8)
    a = ((p + 512) & 1023) - 512
    u = (256 - jnp.abs(a)).astype(F32) * (np.pi / 512.0)
    u2 = u * u
    c = [scale, -scale / 6.0, scale / 120.0, -scale / 5040.0, scale / 362880.0, -scale / 39916800.0]
    poly = c[5]
    for ci in c[4::-1]:
        poly = poly * u2 + ci
    return (u * poly).astype(BF16)


def _ln(x, scale=1.0):
    m = jnp.sum(x, axis=-1, keepdims=True) * (1.0 / D)
    xc = x - m
    s2 = 1.0 / (scale * scale)
    v = jnp.sum(xc * xc, axis=-1, keepdims=True) * (s2 / D) + EPS * s2
    r = jnp.exp2(jnp.log(v) * float(-0.5 / np.log(2.0)))
    return xc * r


def _gelu2(x):
    u = x * (x * x + G_B)
    return x * (1.0 + jnp.tanh(u))


def _lo(w):
    return pltpu.bitcast(w << 16, F32)


def _hi(w):
    return pltpu.bitcast(w & jnp.uint32(0xFFFF0000), F32)


def _pack(a, b):
    return pltpu.pack_elementwise([a, b], packed_dtype=BF16)


def _tie(x, a):
    if a is None:
        return x
    w = pltpu.bitcast(x[:, :128], U32)
    k = w.shape[0] // 8
    w = w | (a if k == 1 else jnp.concatenate([a] * k, axis=0))
    w = pltpu.bitcast(w, x.dtype)
    return w if x.shape[1] == 128 else jnp.concatenate([w, x[:, 128:]], axis=1)


def C(i, lim=F):
    return slice(i * 128, min((i + 1) * 128, lim))


class Unit:
    def __init__(self, name, tiles, epi, rows, cost, nt=False, full=True, acc=False):
        self.acc, self.res = acc, []
        self.name, self.tiles, self.epi, self.rows, self.cost, self.nt, self.full = name, tiles, epi, rows, cost, nt, full


class Group:
    def __init__(self, name, fns, cost, rel, dead, lat, rlat=200):
        self.name, self.fns, self.cost, self.rel, self.dead, self.lat, self.rlat = name, fns, cost, rel, dead, lat, rlat


def _plan(seq, groups):
    busy, n = [0] * 4, 0
    start, end, tiles, bars = {}, {}, [], []
    for it in seq:
        if isinstance(it[0], Unit):
            u = it[0]
            m = n % 4
            n += 1
            t0, t1 = busy[m], busy[m] + max(u.rows, 32)
            busy[m] = t1
            tiles.append((t0, t1, u.cost / len(u.tiles)))
            start.setdefault(u.name, t0)
            end[u.name] = max(end.get(u.name, 0), t1)
        elif it[0] == "wait":
            t = max(busy)
            busy, n = [t] * 4, 0
            start[it[1]] = end[it[1]] = t
            bars.append(t)
    total = max(busy)
    start["end"] = end["end"] = total
    start["start"] = end["start"] = 0
    ns = total // SLOT + 2
    load = np.zeros(ns)
    for t0, t1, c in tiles:
        a, b = t0 // SLOT, max(t1 // SLOT, t0 // SLOT + 1)
        load[a:b] += c / (b - a)
    win = []
    for g in groups:
        r = max(end[x] + (0 if start[x] == end[x] else g.rlat) for x in g.rel)
        d = min(start[x] for x in g.dead) - g.lat
        ok = np.zeros(ns, bool)
        ok[r // SLOT:max(d // SLOT, r // SLOT + 1)] = True
        for b in bars:
            if r < b <= d:
                ok[max((b - g.lat) // SLOT, 0):b // SLOT] = False
        win.append(np.nonzero(ok)[0])
    alloc = [np.zeros(len(w)) for w in win]
    for _ in range(60):
        for i, g in enumerate(groups):
            w = win[i]
            load[w] -= alloc[i]
            base = load[w]
            vol = g.cost * len(g.fns)
            lo, hi = base.min(), base.max() + vol
            for _ in range(50):
                mid = 0.5 * (lo + hi)
                if np.maximum(mid - base, 0).sum() > vol:
                    hi = mid
                else:
                    lo = mid
            alloc[i] = np.maximum(hi - base, 0)
            load[w] += alloc[i]
    times = []
    for i, g in enumerate(groups):
        cum = np.cumsum(alloc[i])
        ts = []
        for k in range(len(g.fns)):
            x = (k + 0.5) * cum[-1] / len(g.fns)
            j = int(np.searchsorted(cum, x))
            prev = cum[j - 1] if j else 0.0
            ts.append(win[i][j] * SLOT + SLOT * (x - prev) / max(alloc[i][j], 1e-9))
        times.append(ts)
        if VERBOSE:
            print("%8s window %6d..%6d used %6d..%6d" % (g.name, win[i][0] * SLOT, win[i][-1] * SLOT, ts[0], ts[-1]))
    if VERBOSE:
        k = 2048 // SLOT
        print("total", total, "load/cycle:", " ".join("%.1f" % (load[i:i + k].mean() / SLOT) for i in range(0, ns, k)))
    return times


def _emit(seq, groups, zero, wait):
    times = _plan(seq, groups)
    left = {"start": 0}
    for it in seq:
        nm = it[0].name if isinstance(it[0], Unit) else it[1]
        left[nm] = left.get(nm, 0) + 1
    heap, pend, todo, cnt = [], {}, list(range(len(groups))), 0
    busy, n = [0] * 4, 0

    def release():
        nonlocal cnt
        for i in list(todo):
            g = groups[i]
            if all(left[x] == 0 for x in g.rel):
                todo.remove(i)
                pend[i] = len(g.fns)
                for t, fn in zip(times[i], g.fns):
                    heapq.heappush(heap, (t, cnt, i, fn))
                    cnt += 1

    def force(name):
        nonlocal heap
        for i, g in enumerate(groups):
            if name in g.dead:
                assert i not in todo, (g.name, name)
                if pend[i]:
                    if VERBOSE:
                        print("forcing", g.name, pend[i], "before", name)
                    for it in sorted(x for x in heap if x[2] == i):
                        it[3](None)
                    heap = [x for x in heap if x[2] != i]
                    heapq.heapify(heap)
                    pend[i] = 0

    release()
    for it in seq:
        if isinstance(it[0], Unit):
            u, k = it
            force(u.name)
            lhs, rhs = u.tiles[k]()
            dn = (((1,), (1 if u.nt else 0,)), ((), ()))
            p = lax.dot_general(lhs, rhs, dn, preferred_element_type=F32)
            u.res = [p + u.res[0]] if (u.acc and u.res) else u.res + [p]
            m = n % 4
            n += 1
            t0 = busy[m]
            busy[m] = t0 + max(u.rows, 32)
            while u.full and heap and heap[0][0] < t0 + u.rows:
                t, _, i, fn = heapq.heappop(heap)
                pend[i] -= 1
                r = min(max(int(t - t0), 0), u.rows - 1) // 8 * 8
                fn(pltpu.bitcast(p[r:r + 8], U32) & zero)
            if k == len(u.tiles) - 1:
                u.epi(u.res)
            left[u.name] -= 1
        elif it[0] == "wait":
            force(it[1])
            wait(it[1])
            busy, n = [max(busy)] * 4, 0
            left[it[1]] -= 1
        else:
            it[2]()
            left[it[1]] -= 1
        release()
    force("end")
    assert not heap and not todo


def _sum(ps):
    acc = ps[0]
    for p in ps[1:]:
        acc = acc + p
    return acc


def _flat(us):
    return [(u, i) for u in us for i in range(len(u.tiles))]


def _phase(seq):
    n = 0
    for it in seq:
        n = n + 1 if isinstance(it[0], Unit) else (0 if it[0] in ("wait", "sync") else n)
    return n % 4


def _mix(seq, a, b, lo=0.0, hi=1.0):
    n, k = _phase(seq), 0
    for i, t in enumerate(a):
        if k < len(b) and n % 4 == 0 and t[1] != 1 and i >= len(a) * (lo + (hi - lo) * k / len(b)):
            seq.extend(b[k])
            k += 1
        seq.append(t)
        n += 1
    assert k == len(b)


def _wait(seq, name, head=()):
    r = _phase(seq)
    assert all(isinstance(it[0], Unit) for it in seq[len(seq) - r:])
    seq[len(seq) - r:len(seq) - r] = [("wait", name)] + list(head)


def kernel(q_hbm, k_hbm, v_hbm, sh_hbm, ssm_hbm, sd_hbm, w1_hbm, w2_hbm, w3_hbm, w4_hbm, c_hbm, wm_hbm,
           o_hbm,
           q_w, k_n, v_w, ssm_w, w1_w, w2_w, w3_w, w4_w, wm_w, o_v,
           sh_v, sd_v, c_v, zsrc, z_s, taps, mod_v, tf_w, tg_w,
           kf, uf, acc, zraw, kv_w, zz_w, y_v, x_v, hb_v, x1_v, r_v, n1_w, n2_w, g_w, h1_v, a_w,
           sem, sem_b, sem_o):
    bf = lambda r: r.bitcast(BF16)
    w1_v, w2_v, w3_v, w4_v, wm_v = bf(w1_w), bf(w2_w), bf(w3_w), bf(w4_w), bf(wm_w)
    tf_v, tg_v, kv_v, zz_v, n1_v, n2_v, g_v = bf(tf_w), bf(tg_w), bf(kv_w), bf(zz_w), bf(n1_w), bf(n2_w), bf(g_w)
    q_v, a_v = bf(q_w), bf(a_w)
    cp = pltpu.make_async_copy
    scope = lambda nm: jax.named_scope(nm) if SCOPES else contextlib.nullcontext()

    def base(j, n):
        return j * n if isinstance(j, int) else pl.multiple_of(j * n, n)

    def rows(j, n=1, size=T):
        return pl.ds(base(j, size), n * size)

    def view(ref, j, size=T):
        return ref.at[rows(j, 1, size)]

    dmas = {}

    def group(name, *mks):
        sm = sem.at[len(dmas)]
        dmas[name] = [c for mk in mks for c in mk(sm)]

    def ssm_in(s, n=1):
        return lambda sm: [cp(ssm_hbm.at[:, rows(s, n)], bf(ssm_w).at[:, rows(s, n)], sm)]

    def kv_in(s):
        return lambda sm: ([cp(k_hbm.at[rows(s), C(t)], bf(k_n).at[t, pl.ds(16 + base(s, T), T)], sm) for t in range(NT)]
                           + [cp(v_hbm.at[rows(s)], bf(v_w).at[rows(s)], sm)])

    def q_in(s, n=1):
        return lambda sm: [cp(q_hbm.at[rows(s, n)], q_v.at[rows(s, n)], sm)]

    def wm_in(a, b):
        return lambda sm: [cp(wm_hbm.at[:, a * D:b * D], wm_v.at[:, a * D:b * D], sm)]

    def whole(src, dst):
        return lambda sm: [cp(src, dst, sm)]

    def blk_in(s):
        sm = sem_b.at[s - NC]
        return kv_in(s)(sm) + q_in(s)(sm)

    zsrc[...] = jnp.zeros((8, 128), I32)
    k_n[:, 0:8, :] = jnp.zeros((NT, 8, 128), U32)
    group("small", lambda sm: [cp(zsrc, z_s, sm), cp(sh_hbm, sh_v, sm), cp(sd_hbm, sd_v, sm), cp(c_hbm, c_v, sm)])
    for s in range(NC):
        group("c%d" % s, ssm_in(s), kv_in(s))
    group("kr", ssm_in(NC, NB - NC))
    group("wma", wm_in(0, 3), q_in(0, 2))
    group("wmb", wm_in(3, 5))
    group("w1", whole(w1_hbm, w1_v))
    group("w2", q_in(2), whole(w2_hbm, w2_v))
    group("w3", whole(w3_hbm, w3_v))
    group("w4", whole(w4_hbm, w4_v), wm_in(5, 6))
    for g in dmas.values():
        for c in g:
            c.start()

    def wait(name):
        with scope("wait_" + name):
            for c in dmas[name]:
                c.wait()

    tau_b = lambda l: H + ((l + (H - 1)) & (H - 1))
    tf_v[:, C(0)] = _dft((T, H), 0, lambda l: jnp.where((l & 1) == 0, l, tau_b(l)), 1.0 / T)
    tf_v[:, C(1)] = _dft((T, H), 0, lambda l: jnp.where((l & 1) == 1, l, tau_b(l)), 1.0 / T)
    tf_v[:, C(2)] = _dft((T, H), 0, lambda l: 2 * _unzip(l) - H)
    tf_v[:, C(3)] = _dft((T, H), 0, lambda l: 2 * _unzip(l) + 1 - H)
    sin0 = lax.broadcasted_iota(I32, (GR, T), 1) >= H
    tg_v[:, 0:T] = _dft((GR, T), 1, lambda l: jnp.where(sin0 & (l == 0), H, 2 * l))
    tg_v[:, T:2 * T] = _dft((GR, T), 1, lambda l: 2 * l + 1)
    h1_v[:, 0:8, :] = jnp.zeros((NT, 8, 128), F32)
    h1_v[:, 8 + S:16 + S, :] = jnp.zeros((NT, 8, 128), F32)

    wait("small")
    z = jnp.clip(z_s[0, 0], 0, 1)
    zero = jnp.full((8, 128), z, I32).astype(U32)
    z8 = pl.multiple_of(z * 8, 8)
    for r in (r_v, zraw, n1_w, n2_w, g_w, a_w):
        r[pl.ds(z8, 8), 0:128] = jnp.zeros((8, 128), r.dtype)
    for r in (kf, uf, acc, kv_w, zz_w, taps, mod_v):
        r[z, 0:8, 0:128] = jnp.zeros((8, 128), r.dtype)
    for r in (tf_w, tg_w):
        r[pl.ds(z8, 8), 0:128] = r[0:8, 0:128]
    sh = sh_v[...].astype(F32)
    for i in range(4):
        taps[i] = jnp.broadcast_to(sh[i:i + 1], (8, D))
    taps[4] = jnp.broadcast_to(sd_v[...].astype(F32).reshape(1, D) * (1.0 / T), (8, D))
    cf = c_v[...].astype(F32)
    silu_c = jnp.broadcast_to((cf / (1.0 + jnp.exp(-cf))).astype(BF16), (16, D))

    def mmK(m):
        def unit(n):
            W = slice(64 * n, 64 * (n + 1))
            st = []

            def rhs(i):
                if not st:
                    ev = (lax.broadcasted_iota(I32, (64, 128), 1) & 1) == 0
                    a = ssm_w[W, m * T:m * T + H]
                    b = pltpu.roll(ssm_w[W, m * T + H:(m + 1) * T], 1, 1)
                    st.extend([pltpu.bitcast(jnp.where(ev, a, b), BF16), pltpu.bitcast(jnp.where(ev, b, a), BF16)])
                return st[i]

            def epi(p):
                er, ei, or_, oi = p
                if m == 0:
                    er = er + taps[4, 0:1, C(n)]
                for h, (cr, ci) in enumerate(((er + or_, ei + oi), (er - or_, ei - oi))):
                    B = h * 3 * H
                    kf[m, B:B + H, C(n)] = cr
                    kf[m, B + H:B + 2 * H, C(n)] = ci - cr
                    kf[m, B + 2 * H:B + 3 * H, C(n)] = ci + cr
            return Unit("K%d" % m, [(lambda i=i, r=r: (tf_v[r:r + H, C(i)], rhs(i))) for i in range(2) for r in (0, H)],
                        epi, H, 170, nt=True)
        return [unit(n) for n in range(NT)]

    def kv(s, sl):
        vv, b0 = view(v_w, s, H), base(s, H)

        def mk(t, w):
            def fn(a):
                ld = lambda o, n: k_n[t, pl.ds(b0 + (8 + w + o), n), :]
                c0 = jnp.concatenate([_tie(ld(0, 8), a), ld(8, 8)], axis=0).reshape(2, 8, 128)
                c1, c2 = ld(-1, 16).reshape(2, 8, 128), ld(-2, 16).reshape(2, 8, 128)
                s0, s1, s2, s3 = (taps[i, :, C(t)] for i in range(4))
                ke, ko, ke1, ko1, ko2 = _lo(c0), _hi(c0), _lo(c1), _hi(c1), _hi(c2)
                wv = vv[w:w + 16, C(t)].reshape(2, 8, 128)
                kve = ((s0 * ke + s1 * ko1) + (s2 * ke1 + s3 * ko2)) * _lo(wv)
                kvo = ((s0 * ko + s1 * ke) + (s2 * ko1 + s3 * ke1)) * _hi(wv)
                kv_w[sl, w // 2:w // 2 + 8, C(t)] = _pack(kve[0], kve[1])
                kv_w[sl, (H + w) // 2:(H + w) // 2 + 8, C(t)] = _pack(kvo[0], kvo[1])
            return fn
        return [[mk(t, w) for w in range(0, H, 16)] for t in range(NT)]

    def mmU(name, sl, us):
        def unit(n):
            def epi(p):
                er, ei, or_, oi = p
                for h, (cr, ci) in enumerate(((er + or_, ei + oi), (er - or_, ei - oi))):
                    B = h * 3 * H
                    uf[us, B:B + H, C(n)] = cr + ci
                    uf[us, B + H:B + 2 * H, C(n)] = cr
                    uf[us, B + 2 * H:B + 3 * H, C(n)] = ci
            return Unit(name(n), [(lambda i=i, r=r: (tf_v[r:r + H, C(2 + i)], kv_v[sl, C(i), C(n)]))
                                  for i in range(2) for r in (0, H)], epi, H, 120)
        return [unit(n) for n in range(NT)]

    def cmul(m0, u0, n, h, row, L, a):
        t = []
        for i in range(3):
            Rw = slice((3 * h + i) * H + row, (3 * h + i) * H + row + 8)
            kk = kf[m0:m0 + n, Rw, L]
            if i == 0 and a is not None:
                k0 = _tie(kk[0], a)[None]
                kk = k0 if n == 1 else jnp.concatenate([k0, kk[1:]], axis=0)
            t.append(jnp.sum(kk * uf[u0:u0 + n, Rw, L], axis=0))
        return t[0] - t[2], t[0] + t[1]

    def AR(h, q, row):
        return slice((2 * h + q) * H + row, (2 * h + q) * H + row + 8)

    def mac(n, u0, sl, first=False, part=False):
        def mk(t, rc):
            st, fin = [], []

            def piece(i):
                def fn(a):
                    h, row = i & 1, rc + (i >> 1) * 8
                    zr, zi = cmul(0, u0, n, h, row, C(t), a)
                    if part:
                        zr, zi = zr + acc[0, AR(h, 0, row), C(t)], zi + acc[0, AR(h, 1, row), C(t)]
                    st.append((zr, zi))
                    if h:
                        (pr, pi), (mr, mi) = st[-2:]
                        z = [pr + mr, pi + mi, pr - mr, pi - mi]
                        Rw = lambda q: slice(q * H + row, q * H + row + 8)
                        pv = None if first else [zraw[Rw(q ^ 1), C(t)] for q in range(4)]
                        for q in range(4):
                            zraw[Rw(q), C(t)] = z[q]
                        if not first:
                            z = [z[q] + pv[q] if (q & 1) == (rc < 64) else z[q] - pv[q] for q in range(4)]
                        fin.append(z)
                    if i == 3:
                        for q in range(4):
                            w = (q * H + rc) // 2
                            zz_w[sl, w:w + 8, C(t)] = _pack(fin[0][q], fin[1][q])
                return fn
            if not part:
                return [piece(i) for i in range(4)]
            both = lambda f, g: (lambda a: (f(a), g(None)))
            return [both(piece(0), piece(1)), both(piece(2), piece(3))]
        return [[fn for rc in range(0, H, 16) for fn in mk(t, rc)] for t in range(NT)]

    def pos():
        return [(t, h, row) for t in range(NT) for row in range(0, H, 8) for h in range(2)]

    def ahead(i):
        def mk(t, h, row):
            def fn(a):
                zr, zi = cmul(i + 1, 0, NC, h, row, C(t), a)
                acc[i, AR(h, 0, row), C(t)] = zr
                acc[i, AR(h, 1, row), C(t)] = zi
            return fn
        return [mk(*p) for p in pos()]

    def spread():
        n = NB - NC - 1

        def mk(t, h, row):
            def fn(a):
                p = []
                for i in range(3):
                    Rw = slice((3 * h + i) * H + row, (3 * h + i) * H + row + 8)
                    u = uf[0, Rw, C(t)]
                    p.append(kf[1:1 + n, Rw, C(t)] * (_tie(u, a) if i == 0 else u)[None])
                acc[0:n, AR(h, 0, row), C(t)] = acc[1:1 + n, AR(h, 0, row), C(t)] + (p[0] - p[2])
                acc[0:n, AR(h, 1, row), C(t)] = acc[1:1 + n, AR(h, 1, row), C(t)] + (p[0] + p[1])
            return fn
        return [mk(*p) for p in pos()]

    def mmI(name, sl, ys):
        def unit(n):
            def epi(p):
                ce, se, co, so = p
                sub = lax.broadcasted_iota(I32, (8, 128), 0)
                c0 = ys * T + H
                y_v[n, ys * T:ys * T + 1, :] = (ce[64:72] - se[0:8])[0:1]
                se = jnp.concatenate([jnp.where(sub == 0, 0.0, se[0:8]), se[8:]], axis=0)
                for d, cc, ss in ((0, ce[0:64], se), (1, co, so)):
                    y_v[n, pl.ds(c0 + d, 64, stride=2), :] = cc + ss
                    lo = cc - ss
                    for i in range(0, 64, 8):
                        y_v[n, pl.ds(c0 - d - 2 * i - 14, 8, stride=2), :] = jnp.take_along_axis(
                            lo[i:i + 8], 7 - sub, axis=0)
            return Unit(name(n), [(lambda i=i: (tg_v[0:(GR if i == 0 else 64), C(i)], zz_v[sl, C(i), C(n)]))
                                  for i in range(4)], epi, 64, 52)
        return [unit(n) for n in range(NT)]

    def mod(name, a, b):
        def unit(n):
            def epi(p):
                v = [_sum(p[i * NT:(i + 1) * NT])[0:8] for i in range(b - a)]
                if a == 0:
                    mod_v[0, :, C(n)] = v[0] * v[2]
                    mod_v[1, :, C(n)] = (v[1] + 1.0) * v[2]
                elif a == 3:
                    mod_v[3, :, C(n)] = v[0]
                    mod_v[4, :, C(n)] = v[1] + 1.0
                else:
                    mod_v[5, :, C(n)] = v[0]
                    mod_v[2, :, C(n)] = v[0] * G_POST
            return Unit(name, [(lambda i=i, k=k: (silu_c[:, C(k)], wm_v[C(k), i * D + n * 128:i * D + (n + 1) * 128]))
                               for i in range(a, b) for k in range(NT)], epi, 16, 10, full=False, acc=b - a == 1)
        return [unit(n) for n in range(NT)]

    GS = range(0, T, RG)
    HS = (slice(0, 128), slice(128, 256))

    def tasks(f):
        return [(lambda a, r=r: f(slice(r, r + RG), a)) for r in GS]

    def load_y(sl, R):
        return jnp.concatenate([y_v[t, sl * T + R.start:sl * T + R.stop, :] for t in range(NT)],
                               axis=1).reshape(2, 8, D)

    def front(j, sl, early=False):
        qq, xx, hh, nn = view(q_w, j, H), view(x_v, j), view(hb_v, j), view(n1_v, sl)

        def fa(R, a):
            q = pltpu.bitcast(_tie(qq[R.start // 2:R.stop // 2, :], a), BF16).astype(F32).reshape(2, 8, D)
            x = (q + (_ln(q) * mod_v[1] + mod_v[0]) * load_y(sl, R)).reshape(RG, D)
            xx[R, :] = x
            if early:
                hh[R, :] = _ln(x)

        def fb(R, a):
            hh[R, :] = (_ln(_tie(xx[R, :], a).reshape(2, 8, D)) * mod_v[4] + mod_v[3]).reshape(RG, D)

        def fc(R, a):
            hb = _tie(hh[R, :], a)
            if early:
                hb = (hb.reshape(2, 8, D) * mod_v[4] + mod_v[3]).reshape(RG, D)
                hh[R, :] = hb
            nn[R, :] = _ln(hb, G_A).astype(BF16)
        return (tasks(fa), tasks(fc)) if early else tasks(fa) + tasks(fb) + tasks(fc)

    def shift(j, sl):
        SR = 64
        gg, b0 = view(g_v, sl), base(j, T)

        def mk(t, r):
            def fn(a):
                lane = lax.broadcasted_iota(I32, (SR, 128), 1)
                ld = lambda d: h1_v[t, pl.ds(b0 + (8 + r + d), SR), :]
                if t == 0:
                    g = ld(-1)
                elif t == 1:
                    g = jnp.where(lane < 32, ld(-1), ld(1))
                elif t == 2:
                    g = jnp.where(lane < 64, ld(1), ld(-2))
                elif t == 3:
                    g = jnp.where(lane < 96, ld(-2), ld(2))
                else:
                    g = ld(2)
                if a is not None:
                    g = jnp.concatenate([_tie(g[i:i + 8], a) if i % 16 == 0 else g[i:i + 8]
                                         for i in range(0, SR, 8)], axis=0)
                gg[r:r + SR, C(t)] = g.astype(BF16)
            return fn
        return [mk(t, r) for t in range(NT) for r in range(0, T, SR)]

    def ln2(j, sl):
        xx, nn = view(x1_v, j), view(n2_v, sl)

        def f(R, a):
            nn[R, :] = _ln(_tie(xx[R, :], a), G_A).astype(BF16)
        return tasks(f)

    def resid(j):
        xx, x1 = view(x_v, j), view(x1_v, j)

        def f(R, a):
            gb = mod_v[5] if a is None else pltpu.bitcast(
                pltpu.bitcast(mod_v[5], U32) | jnp.concatenate([a] * NT, axis=1), F32)
            r_v[R, :] = xx[R, :] + (x1[R, :].reshape(4, 8, D) * gb).reshape(2 * RG, D)
        return [(lambda a, r=r: f(slice(r, r + 2 * RG), a)) for r in range(0, T, 2 * RG)]

    def mm1(name, j, sl):
        nn, b0 = view(n1_v, sl), base(j, T)

        def unit(n, R):
            def epi(p):
                h1_v[n, pl.ds(b0 + (8 + R.start), 128), :] = _gelu2(p[0])
            return Unit(name, [(lambda k=k: (nn[R, C(k)], w1_v[C(k), C(n)])) for k in range(NT)],
                        epi, 128, 144, acc=True)
        return [unit(n, R) for n in range(NT) for R in HS]

    def mm2(name, j, sl):
        gg, hh, x1 = view(g_v, sl), view(hb_v, j), view(x1_v, j)

        def unit(n, R):
            def epi(p):
                x1[R, C(n)] = hh[R, C(n)] + p[0] * G_POST
            return Unit(name, [(lambda k=k: (gg[R, C(k)], w2_v[C(k), C(n)])) for k in range(NT)],
                        epi, 128, 96, acc=True)
        return [unit(n, R) for n in range(NT) for R in HS]

    def mm3(name, sl):
        nn, aa = view(n2_v, sl), view(a_v, sl)

        def unit(n, R):
            def epi(p):
                aa[R, C(n)] = _gelu2(p[0]).astype(BF16)
            return Unit(name, [(lambda k=k: (nn[R, C(k)], w3_v[C(n), C(k)])) for k in range(NT)],
                        epi, 128, 160, nt=True, acc=True)
        main = [unit(n, R) for n in range(FT - 1) for R in HS]
        F0, part = (FT - 1) * 128, []
        main[-1].tiles.pop(0)

        def epi(p):
            for i, R in enumerate(HS):
                aa[R, F0:F] = _gelu2(part[i] + p[i]).T.astype(BF16)
            main[-1].res = [jnp.concatenate(p[2:], axis=0)]
        rem = [Unit(name, [(lambda k=k, R=R: (w3_v[F0:F, C(k)], nn[R, C(k)])) for k in range(NT - 1)],
                    lambda p: part.append(p[0]), 64, 24, nt=True, acc=True) for R in HS]
        rem.append(Unit(name, [(lambda R=R: (w3_v[F0:F, C(NT - 1)], nn[R, C(NT - 1)])) for R in HS]
                        + [(lambda r=r: (nn[r:r + 64, C(0)], w3_v[C(FT - 2), C(0)])) for r in (128, 192)],
                        epi, 64, 120, nt=True))
        return _flat(main), _flat(rem)

    def cp_out(j):
        return cp(o_v.at[rows(j)], o_hbm.at[rows(j)], sem_o.at[0])

    last = []

    def mm4(name, j, sl, pre=False):
        aa, oo, xx, x1 = view(a_v, sl), view(o_v, j), view(x_v, j), view(x1_v, j)

        def unit(n, R):
            def epi(p):
                if pre:
                    oo[R, C(n)] = (r_v[R, C(n)] + mod_v[2, 0:1, C(n)] * p[0]).astype(BF16)
                else:
                    oo[R, C(n)] = (xx[R, C(n)] + mod_v[5, 0:1, C(n)] * (x1[R, C(n)] + p[0] * G_POST)).astype(BF16)
                if isinstance(j, int) and j == NB - 1:
                    Rg = slice(j * T + R.start, j * T + R.stop)
                    last.append(cp(o_v.at[Rg, C(n)], o_hbm.at[Rg, C(n)], sem_o.at[0]))
                    last[-1].start()
                elif n == NT - 1 and R.stop == T:
                    cp_out(j).start()
            return Unit(name, [(lambda k=k: (aa[R, C(k)], w4_v[C(k), C(n)])) for k in range(FT)],
                        epi, 128, 16 * (16 if pre else 18), acc=True)
        return [unit(n, R) for n in range(NT) for R in HS]

    def quarter(u):
        mk = u.tiles.pop(0)
        st = []

        def piece(i):
            if not st:
                st.extend(mk())
            return st[0][32 * i:32 * i + 32], st[1]

        def epi(p):
            u.res = [jnp.concatenate(p, axis=0)]
        return _flat([Unit(u.name, [(lambda i=i: piece(i)) for i in range(4)], epi, 32, 0, nt=u.nt)])

    W = lambda nm: [("wait", nm)]
    run = lambda fns: [("run", "run", lambda: [fn(None) for fn in fns])]
    one = lambda us: [_flat([u]) for u in us]
    cat = lambda ls: [x for l in ls for x in l]
    nm = lambda x: (lambda n: x)

    seq, grp = [], []
    for s in range(NC):
        seq += W("c%d" % s) + _flat((mmI(nm("I0"), 0, 0) if s == 2 else []) + mmK(s) + mmU(nm("U%d" % s), s % 2, NC - 1 - s))
        grp.append(Group("kv%d" % s, cat(kv(s, s % 2)), 50, ["c%d" % s], ["U%d" % s], 100))
    grp.append(Group("mac0", cat(mac(1, 2, 0, first=True)), 12, ["c1"], ["c2"], 0))
    grp.append(Group("mac1", cat(mac(2, 1, 1)), 18, ["c2"], ["kr"], 0))
    grp.append(Group("mac2", cat(mac(3, 0, 0)), 24, ["kr"], ["I2"], 300))
    seq += W("kr") + _flat(mmI(nm("I1"), 1, 1) + cat(mmK(m) for m in range(NC, NB)) + mmI(nm("I2"), 0, 2))
    seq += [("run", "run", lambda: [c.start() for s in range(NC, NB) for c in blk_in(s)])]
    f0, f1 = front(0, 0, True), front(1, 1, True)
    seq += W("wma") + _flat(mod("moda", 0, 3)) + run(f0[0] + f1[0])
    seq += W("wmb") + _flat(mod("modb", 3, 5)) + run(f0[1] + f1[1])
    w1 = _flat(mm1("w1_0", 0, 0) + mm1("w1_1", 1, 1))
    seq += W("w1") + w1[:LP[4]] + W("w2") + w1[LP[4]:] + run(shift(0, 0))
    seq += _flat(mm2("w2_0", 0, 0) + mm1("w1_2", 2, 2)) + run(shift(1, 1)) + _flat(mm2("w2_1", 1, 1))
    grp.append(Group("f2", front(2, 2), 80, ["w2"], ["w1_2"], 450))
    grp.append(Group("ln2_0", ln2(0, 0), 60, ["w2_0"], ["w3"], 450))
    grp.append(Group("ahead", cat(ahead(i) for i in range(NB - NC)), 19, ["w1"], ["end"], 100))
    _wait(seq, "w3")
    a, r = mm3("w3_0", 0)
    _mix(seq, a, [r], 0.1)
    mc = _flat(mod("modc", 5, 6))
    _wait(seq, "w4", mc[:5] + [("sync", "run", lambda: None)])
    w4 = mm4("w4_0", 0, 0)[:LP[2]]
    qs = [quarter(w4[-1 - i]) for i in range((_phase(seq) + FT * LP[2]) % 4)]
    _mix(seq, _flat(w4), [mc[i:i + 4] for i in range(5, 25, 4)] + qs, 0.01, 0.4)
    assert _phase(seq) == 0
    grp.append(Group("resid", resid(0), 46, ["modc"], ["end"], 100))
    _emit(seq, grp, zero, wait)

    def step(s, carry):
        with scope("wait_blk"):
            for c in blk_in(s):
                c.wait()
        seq, grp = [], []
        a, r = mm3("w3", 0)
        us, it = one(mmU(lambda n: "U%d" % n, 0, 0)), one(mmI(lambda n: "I%d" % n, 0, 0))
        w4 = mm4("w4", s - 2, 0, pre=True)
        q = quarter(w4[LP[1] - 1])
        _mix(seq, _flat(mm4("w4c", s - 3, 0, pre=True)[LP[2]:]) + a,
             [us[0], us[1], us[2], it[0] + us[3], it[1] + us[4], it[2], it[3], it[4], r], LP[3], LP[0])
        _mix(seq, _flat(w4[:LP[1]]), [q])
        seq += _flat(mm1("w1", s, 0) + w4[LP[1]:LP[2]] + mm2("w2", s - 1, 0))
        assert _phase(seq) == 0
        kvs, macs = kv(s, 0), mac(1, 0, 0, part=True)
        for t in range(NT):
            grp.append(Group("kv%d" % t, kvs[t], 50, ["start"], ["U%d" % t], 300))
            grp.append(Group("mac%d" % t, macs[t], 28, ["U%d" % t], ["I%d" % t], 300, 150))
        iall = ["I%d" % t for t in range(NT)]
        grp.append(Group("ln2", ln2(s - 2, 0), 60, ["start"], ["w3"], 450))
        grp.append(Group("resid", resid(s - 2), 46, ["w4c"], ["w4", "I4"], 100))
        grp.append(Group("front", front(s, 0), 80, iall, ["w1"], 450))
        grp.append(Group("spread", spread(), 30, iall, ["end"], 100))
        grp.append(Group("shift", shift(s - 1, 0), 14, ["w1"], ["w2"], 200))
        _emit(seq, grp, zero, wait)
        return carry

    lax.fori_loop(NC, NB, step, 0)

    seq, grp = [], []
    seq += _flat(mm4("w4_5", NB - 3, 0, pre=True)[LP[2]:])
    a, r = mm3("w3_6", 0)
    _mix(seq, a, [r])
    seq += _flat(mm2("w2_7", NB - 1, 0) + mm4("w4_6", NB - 2, 0))
    a, r = mm3("w3_7", 1)
    _mix(seq, a, [r])
    seq += _flat(mm4("w4_7", NB - 1, 1))
    assert _phase(seq) == 0
    grp.append(Group("ln2_6", ln2(NB - 2, 0), 60, ["start"], ["w3_6"], 450))
    grp.append(Group("shift7", shift(NB - 1, 0), 14, ["start"], ["w2_7"], 200))
    grp.append(Group("ln2_7", ln2(NB - 1, 1), 60, ["w2_7"], ["w3_7"], 450))
    _emit(seq, grp, zero, wait)
    with scope("wait_out"):
        for c in [cp_out(j) for j in range(NB - 1)] + last:
            c.wait()


@jax.jit
def pallas_adaLN_cond__ssm_conv_h3__mixer_s_mlp__prompt_kernel(A_q, A_k, A_v, A_shift_k, A_ssm_k, A_ssm_D, B_x, B_w1, B_w2, B_w3, B_w4, c, w_mod):
    any_ = pl.BlockSpec(memory_space=pl.ANY)
    V = pltpu.VMEM
    out = pl.pallas_call(
        kernel,
        in_specs=[any_] * 12,
        out_specs=any_,
        out_shape=jax.ShapeDtypeStruct((S, D), BF16),
        scratch_shapes=[
            V((S // 2, D), U32), V((NT, 8 + S // 2, 128), U32), V((S // 2, D), U32), V((D // 2, S), U32),
            V((D // 2, D), U32), V((D // 2, D), U32), V((F // 2, D), U32), V((F // 2, D), U32),
            V((D // 2, 6 * D), U32), V((S, D), BF16),
            V((4, D), BF16), V((D,), BF16), V((1, D), BF16), V((8, 128), I32), pltpu.SMEM((8, 128), I32),
            V((5, 8, D), F32), V((6, 8, D), F32), V((T // 2, 4 * H), U32), V((GR // 2, 2 * T), U32),
            V((NB, 3 * T + 8, D), F32), V((NC, 3 * T + 8, D), F32), V((NB - NC, 2 * T + 8, D), F32), V((2 * T, D), F32),
            V((2, T // 2, D), U32), V((2, T, D), U32), V((NT, NC * T + 8, 128), F32),
            V((S, D), F32), V((S, D), F32), V((S, D), F32), V((T, D), F32),
            V((3 * T // 2, D), U32), V((T, D), U32), V((T, D), U32), V((NT, S + 16, 128), F32),
            V((T, (FT + 1) * 128), U32),
            pltpu.SemaphoreType.DMA((11,)), pltpu.SemaphoreType.DMA((NB - NC,)), pltpu.SemaphoreType.DMA((1,)),
        ],
        compiler_params=pltpu.CompilerParams(vmem_limit_bytes=110 << 20, disable_semaphore_checks=True,
                                             disable_bounds_checks=True),
        name="fused",
    )(A_q[0], A_k[0], A_v[0], A_shift_k.T, A_ssm_k, A_ssm_D, B_w1, B_w2, B_w3.T, B_w4, c, w_mod)
    return out[None]
```

```python
import contextlib
import heapq
import numpy as np
import jax
import jax.numpy as jnp
from jax import lax
from jax.experimental import pallas as pl
from jax.experimental.pallas import tpu as pltpu

S, D, F = 2048, 640, 1728
T = 256
H = T // 2
NB = S // T
NT = D // 128
FT = (F + 127) // 128
EPS = 1e-5
F32, BF16, U32, I32 = jnp.float32, jnp.bfloat16, jnp.uint32, jnp.int32
G_C1 = 0.044715 * float(np.sqrt(2.0 / np.pi))
G_C2 = float(np.sqrt(2.0 / np.pi))
G_A = G_C1 ** (1.0 / 3.0)
G_B = G_C2 / G_A
G_POST = 0.5 / G_A
RG = 16
GR = 80
NC = 3
VERBOSE = False
SCOPES = False
SLOT = 32
LP = (0.8, 4, 6, 0.15, 72)


def _unzip(p):
    return (p & -16) | ((p & 1) << 3) | ((p >> 1) & 7)


def _dft(shape, f_axis, tau, scale=1.0):
    r = lax.broadcasted_iota(I32, shape, f_axis)
    l = lax.broadcasted_iota(I32, shape, 1 - f_axis)
    if f_axis == 1:
        r = _unzip(r)
    f = r & 127
    odd = ((f & 63) << 2) | ((f >> 6) << 1) | 1
    p = odd * tau(l) + ((r >> 7) << 8)
    a = ((p + 512) & 1023) - 512
    u = (256 - jnp.abs(a)).astype(F32) * (np.pi / 512.0)
    u2 = u * u
    c = [scale, -scale / 6.0, scale / 120.0, -scale / 5040.0, scale / 362880.0, -scale / 39916800.0]
    poly = c[5]
    for ci in c[4::-1]:
        poly = poly * u2 + ci
    return (u * poly).astype(BF16)


def _ln(x, scale=1.0):
    m = jnp.sum(x, axis=-1, keepdims=True) * (1.0 / D)
    xc = x - m
    s2 = 1.0 / (scale * scale)
    v = jnp.sum(xc * xc, axis=-1, keepdims=True) * (s2 / D) + EPS * s2
    r = jnp.exp2(jnp.log(v) * float(-0.5 / np.log(2.0)))
    return xc * r


def _gelu2(x):
    u = x * (x * x + G_B)
    return x * (1.0 + jnp.tanh(u))


def _lo(w):
    return pltpu.bitcast(w << 16, F32)


def _hi(w):
    return pltpu.bitcast(w & jnp.uint32(0xFFFF0000), F32)


def _pack(a, b):
    return pltpu.pack_elementwise([a, b], packed_dtype=BF16)


def _tie(x, a):
    if a is None:
        return x
    w = pltpu.bitcast(x[:, :128], U32)
    k = w.shape[0] // 8
    w = w | (a if k == 1 else jnp.concatenate([a] * k, axis=0))
    w = pltpu.bitcast(w, x.dtype)
    return w if x.shape[1] == 128 else jnp.concatenate([w, x[:, 128:]], axis=1)


def C(i, lim=F):
    return slice(i * 128, min((i + 1) * 128, lim))


class Unit:
    def __init__(self, name, tiles, epi, rows, cost, nt=False, full=True, acc=False):
        self.acc, self.res = acc, []
        self.name, self.tiles, self.epi, self.rows, self.cost, self.nt, self.full = name, tiles, epi, rows, cost, nt, full


class Group:
    def __init__(self, name, fns, cost, rel, dead, lat, rlat=200):
        self.name, self.fns, self.cost, self.rel, self.dead, self.lat, self.rlat = name, fns, cost, rel, dead, lat, rlat


def _plan(seq, groups):
    busy, n = [0] * 4, 0
    start, end, tiles, bars = {}, {}, [], []
    for it in seq:
        if isinstance(it[0], Unit):
            u = it[0]
            m = n % 4
            n += 1
            t0, t1 = busy[m], busy[m] + max(u.rows, 32)
            busy[m] = t1
            tiles.append((t0, t1, u.cost / len(u.tiles)))
            start.setdefault(u.name, t0)
            end[u.name] = max(end.get(u.name, 0), t1)
        elif it[0] == "wait":
            t = max(busy)
            busy, n = [t] * 4, 0
            start[it[1]] = end[it[1]] = t
            bars.append(t)
    total = max(busy)
    start["end"] = end["end"] = total
    start["start"] = end["start"] = 0
    ns = total // SLOT + 2
    load = np.zeros(ns)
    for t0, t1, c in tiles:
        a, b = t0 // SLOT, max(t1 // SLOT, t0 // SLOT + 1)
        load[a:b] += c / (b - a)
    win = []
    for g in groups:
        r = max(end[x] + (0 if start[x] == end[x] else g.rlat) for x in g.rel)
        d = min(start[x] for x in g.dead) - g.lat
        ok = np.zeros(ns, bool)
        ok[r // SLOT:max(d // SLOT, r // SLOT + 1)] = True
        for b in bars:
            if r < b <= d:
                ok[max((b - g.lat) // SLOT, 0):b // SLOT] = False
        win.append(np.nonzero(ok)[0])
    alloc = [np.zeros(len(w)) for w in win]
    for _ in range(60):
        for i, g in enumerate(groups):
            w = win[i]
            load[w] -= alloc[i]
            base = load[w]
            vol = g.cost * len(g.fns)
            lo, hi = base.min(), base.max() + vol
            for _ in range(50):
                mid = 0.5 * (lo + hi)
                if np.maximum(mid - base, 0).sum() > vol:
                    hi = mid
                else:
                    lo = mid
            alloc[i] = np.maximum(hi - base, 0)
            load[w] += alloc[i]
    times = []
    for i, g in enumerate(groups):
        cum = np.cumsum(alloc[i])
        ts = []
        for k in range(len(g.fns)):
            x = (k + 0.5) * cum[-1] / len(g.fns)
            j = int(np.searchsorted(cum, x))
            prev = cum[j - 1] if j else 0.0
            ts.append(win[i][j] * SLOT + SLOT * (x - prev) / max(alloc[i][j], 1e-9))
        times.append(ts)
        if VERBOSE:
            print("%8s window %6d..%6d used %6d..%6d" % (g.name, win[i][0] * SLOT, win[i][-1] * SLOT, ts[0], ts[-1]))
    if VERBOSE:
        k = 2048 // SLOT
        print("total", total, "load/cycle:", " ".join("%.1f" % (load[i:i + k].mean() / SLOT) for i in range(0, ns, k)))
    return times


def _emit(seq, groups, zero, wait):
    times = _plan(seq, groups)
    left = {"start": 0}
    for it in seq:
        nm = it[0].name if isinstance(it[0], Unit) else it[1]
        left[nm] = left.get(nm, 0) + 1
    heap, pend, todo, cnt = [], {}, list(range(len(groups))), 0
    busy, n = [0] * 4, 0

    def release():
        nonlocal cnt
        for i in list(todo):
            g = groups[i]
            if all(left[x] == 0 for x in g.rel):
                todo.remove(i)
                pend[i] = len(g.fns)
                for t, fn in zip(times[i], g.fns):
                    heapq.heappush(heap, (t, cnt, i, fn))
                    cnt += 1

    def force(name):
        nonlocal heap
        for i, g in enumerate(groups):
            if name in g.dead:
                assert i not in todo, (g.name, name)
                if pend[i]:
                    if VERBOSE:
                        print("forcing", g.name, pend[i], "before", name)
                    for it in sorted(x for x in heap if x[2] == i):
                        it[3](None)
                    heap = [x for x in heap if x[2] != i]
                    heapq.heapify(heap)
                    pend[i] = 0

    release()
    for it in seq:
        if isinstance(it[0], Unit):
            u, k = it
            force(u.name)
            lhs, rhs = u.tiles[k]()
            dn = (((1,), (1 if u.nt else 0,)), ((), ()))
            p = lax.dot_general(lhs, rhs, dn, preferred_element_type=F32)
            u.res = [p + u.res[0]] if (u.acc and u.res) else u.res + [p]
            m = n % 4
            n += 1
            t0 = busy[m]
            busy[m] = t0 + max(u.rows, 32)
            while u.full and heap and heap[0][0] < t0 + u.rows:
                t, _, i, fn = heapq.heappop(heap)
                pend[i] -= 1
                r = min(max(int(t - t0), 0), u.rows - 1) // 8 * 8
                fn(pltpu.bitcast(p[r:r + 8], U32) & zero)
            if k == len(u.tiles) - 1:
                u.epi(u.res)
            left[u.name] -= 1
        elif it[0] == "wait":
            force(it[1])
            wait(it[1])
            busy, n = [max(busy)] * 4, 0
            left[it[1]] -= 1
        else:
            it[2]()
            left[it[1]] -= 1
        release()
    force("end")
    assert not heap and not todo


def _sum(ps):
    acc = ps[0]
    for p in ps[1:]:
        acc = acc + p
    return acc


def _flat(us):
    return [(u, i) for u in us for i in range(len(u.tiles))]


def _phase(seq):
    n = 0
    for it in seq:
        n = n + 1 if isinstance(it[0], Unit) else (0 if it[0] in ("wait", "sync") else n)
    return n % 4


def _mix(seq, a, b, lo=0.0, hi=1.0):
    n, k = _phase(seq), 0
    for i, t in enumerate(a):
        if k < len(b) and n % 4 == 0 and t[1] != 1 and i >= len(a) * (lo + (hi - lo) * k / len(b)):
            seq.extend(b[k])
            k += 1
        seq.append(t)
        n += 1
    assert k == len(b)


def _wait(seq, name, head=()):
    r = _phase(seq)
    assert all(isinstance(it[0], Unit) for it in seq[len(seq) - r:])
    seq[len(seq) - r:len(seq) - r] = [("wait", name)] + list(head)


def kernel(q_hbm, k_hbm, v_hbm, sh_hbm, ssm_hbm, sd_hbm, w1_hbm, w2_hbm, w3_hbm, w4_hbm, c_hbm, wm_hbm,
           o_hbm,
           q_n, k_n, v_n, ssm_w, w1_w, w2_w, w3_w, w4_w, wm_w, o_v,
           sh_v, sd_v, c_v, zsrc, z_s, taps, mod_v, tf_w, tg_w,
           kf, uf, acc, zraw, kv_w, zz_w, y_v, x_v, hb_v, x1_v, r_v, n1_w, n2_w, g_w, h1_v, a_w,
           sem, sem_b, sem_o):
    bf = lambda r: r.bitcast(BF16)
    w1_v, w2_v, w3_v, w4_v, wm_v = bf(w1_w), bf(w2_w), bf(w3_w), bf(w4_w), bf(wm_w)
    tf_v, tg_v, kv_v, zz_v, n1_v, n2_v, g_v = bf(tf_w), bf(tg_w), bf(kv_w), bf(zz_w), bf(n1_w), bf(n2_w), bf(g_w)
    a_v = bf(a_w)
    cp = pltpu.make_async_copy
    scope = lambda nm: jax.named_scope(nm) if SCOPES else contextlib.nullcontext()

    def base(j, n):
        return j * n if isinstance(j, int) else pl.multiple_of(j * n, n)

    def rows(j, n=1, size=T):
        return pl.ds(base(j, size), n * size)

    def view(ref, j, size=T):
        return ref.at[rows(j, 1, size)]

    dmas = {}

    def group(name, *mks):
        sm = sem.at[len(dmas)]
        dmas[name] = [c for mk in mks for c in mk(sm)]

    def ssm_in(s, n=1):
        return lambda sm: [cp(ssm_hbm.at[:, rows(s, n)], bf(ssm_w).at[:, rows(s, n)], sm)]

    def cols(src, start, n, dst, row):
        return lambda sm: [cp(src.at[pl.ds(start, n), C(t)], bf(dst).at[t, pl.ds(row, n)], sm) for t in range(NT)]

    def kv_in(s):
        return lambda sm: cols(k_hbm, s * T, T, k_n, 16 + s * T)(sm) + cols(v_hbm, s * T, T, v_n, s * T)(sm)

    def q_in(s, n=1):
        return cols(q_hbm, s * T, n * T, q_n, s * T)

    def wm_in(a, b):
        return lambda sm: [cp(wm_hbm.at[:, a * D:b * D], wm_v.at[:, a * D:b * D], sm)]

    def whole(src, dst):
        return lambda sm: [cp(src, dst, sm)]

    def next_kv(s):
        halo = s * T - 16 if isinstance(s, int) else pl.multiple_of(s * T - 16, 16)
        return cols(k_hbm, halo, T + 16, k_n, 0)(sem_b.at[0]) + cols(v_hbm, base(s, T), T, v_n, 0)(sem_b.at[0])

    def next_q(s):
        return cols(q_hbm, base(s, T), T, q_n, 0)(sem_b.at[0])

    zsrc[...] = jnp.zeros((8, 128), I32)
    k_n[:, 0:8, :] = jnp.zeros((NT, 8, 128), U32)
    group("small", lambda sm: [cp(zsrc, z_s, sm), cp(sh_hbm, sh_v, sm), cp(sd_hbm, sd_v, sm), cp(c_hbm, c_v, sm)])
    for s in range(NC):
        group("c%d" % s, ssm_in(s), kv_in(s))
    group("kr", ssm_in(NC, NB - NC))
    group("wma", wm_in(0, 3), q_in(0, 2))
    group("wmb", wm_in(3, 5))
    group("w1", whole(w1_hbm, w1_v))
    group("w2", q_in(2), whole(w2_hbm, w2_v))
    group("w3", whole(w3_hbm, w3_v))
    group("w4", whole(w4_hbm, w4_v), wm_in(5, 6))
    for g in dmas.values():
        for c in g:
            c.start()

    def wait(name):
        with scope("wait_" + name):
            for c in dmas[name]:
                c.wait()

    tau_b = lambda l: H + ((l + (H - 1)) & (H - 1))
    tf_v[:, C(0)] = _dft((T, H), 0, lambda l: jnp.where((l & 1) == 0, l, tau_b(l)), 1.0 / T)
    tf_v[:, C(1)] = _dft((T, H), 0, lambda l: jnp.where((l & 1) == 1, l, tau_b(l)), 1.0 / T)
    tf_v[:, C(2)] = _dft((T, H), 0, lambda l: 2 * _unzip(l) - H)
    tf_v[:, C(3)] = _dft((T, H), 0, lambda l: 2 * _unzip(l) + 1 - H)
    sin0 = lax.broadcasted_iota(I32, (GR, T), 1) >= H
    tg_v[:, 0:T] = _dft((GR, T), 1, lambda l: jnp.where(sin0 & (l == 0), H, 2 * l))
    tg_v[:, T:2 * T] = _dft((GR, T), 1, lambda l: 2 * l + 1)
    h1_v[:, 0:8, :] = jnp.zeros((NT, 8, 128), F32)
    h1_v[:, 8 + NC * T:16 + NC * T, :] = jnp.zeros((NT, 8, 128), F32)

    wait("small")
    z = jnp.clip(z_s[0, 0], 0, 1)
    zero = jnp.full((8, 128), z, I32).astype(U32)
    z8 = pl.multiple_of(z * 8, 8)
    for r in (x_v, hb_v, x1_v, r_v, zraw, n1_w, n2_w, g_w, a_w):
        r[pl.ds(z8, 8), 0:128] = jnp.zeros((8, 128), r.dtype)
    for r in (kf, uf, acc, kv_w, zz_w, taps, mod_v):
        r[z, 0:8, 0:128] = jnp.zeros((8, 128), r.dtype)
    for r in (tf_w, tg_w):
        r[pl.ds(z8, 8), 0:128] = r[0:8, 0:128]
    sh = sh_v[...].astype(F32)
    for i in range(4):
        taps[i] = jnp.broadcast_to(sh[i:i + 1], (8, D))
    taps[4] = jnp.broadcast_to(sd_v[...].astype(F32).reshape(1, D) * (1.0 / T), (8, D))
    cf = c_v[...].astype(F32)
    silu_c = jnp.broadcast_to((cf / (1.0 + jnp.exp(-cf))).astype(BF16), (16, D))

    def mmK(m):
        def unit(n):
            W = slice(64 * n, 64 * (n + 1))
            st = []

            def rhs(i):
                if not st:
                    ev = (lax.broadcasted_iota(I32, (64, 128), 1) & 1) == 0
                    a = ssm_w[W, m * T:m * T + H]
                    b = pltpu.roll(ssm_w[W, m * T + H:(m + 1) * T], 1, 1)
                    st.extend([pltpu.bitcast(jnp.where(ev, a, b), BF16), pltpu.bitcast(jnp.where(ev, b, a), BF16)])
                return st[i]

            def epi(p):
                er, ei, or_, oi = p
                if m == 0:
                    er = er + taps[4, 0:1, C(n)]
                for h, (cr, ci) in enumerate(((er + or_, ei + oi), (er - or_, ei - oi))):
                    B = h * 3 * H
                    kf[m, B:B + H, C(n)] = cr
                    kf[m, B + H:B + 2 * H, C(n)] = ci - cr
                    kf[m, B + 2 * H:B + 3 * H, C(n)] = ci + cr
            return Unit("K%d" % m, [(lambda i=i, r=r: (tf_v[r:r + H, C(i)], rhs(i))) for i in range(2) for r in (0, H)],
                        epi, H, 170, nt=True)
        return [unit(n) for n in range(NT)]

    def kv(s, sl):
        def mk(t, w):
            def fn(a):
                ld = lambda o, n: k_n[t, pl.ds(s * H + 8 + w + o, n), :]
                c0 = jnp.concatenate([_tie(ld(0, 8), a), ld(8, 8)], axis=0).reshape(2, 8, 128)
                c1, c2 = ld(-1, 16).reshape(2, 8, 128), ld(-2, 16).reshape(2, 8, 128)
                s0, s1, s2, s3 = (taps[i, :, C(t)] for i in range(4))
                ke, ko, ke1, ko1, ko2 = _lo(c0), _hi(c0), _lo(c1), _hi(c1), _hi(c2)
                wv = v_n[t, s * H + w:s * H + w + 16, :].reshape(2, 8, 128)
                kve = ((s0 * ke + s1 * ko1) + (s2 * ke1 + s3 * ko2)) * _lo(wv)
                kvo = ((s0 * ko + s1 * ke) + (s2 * ko1 + s3 * ke1)) * _hi(wv)
                kv_w[sl, w // 2:w // 2 + 8, C(t)] = _pack(kve[0], kve[1])
                kv_w[sl, (H + w) // 2:(H + w) // 2 + 8, C(t)] = _pack(kvo[0], kvo[1])
            return fn
        return [[mk(t, w) for w in range(0, H, 16)] for t in range(NT)]

    def mmU(name, sl, us):
        def unit(n):
            def epi(p):
                er, ei, or_, oi = p
                for h, (cr, ci) in enumerate(((er + or_, ei + oi), (er - or_, ei - oi))):
                    B = h * 3 * H
                    uf[us, B:B + H, C(n)] = cr + ci
                    uf[us, B + H:B + 2 * H, C(n)] = cr
                    uf[us, B + 2 * H:B + 3 * H, C(n)] = ci
            return Unit(name(n), [(lambda i=i, r=r: (tf_v[r:r + H, C(2 + i)], kv_v[sl, C(i), C(n)]))
                                  for i in range(2) for r in (0, H)], epi, H, 120)
        return [unit(n) for n in range(NT)]

    def cmul(m0, u0, n, h, row, L, a):
        t = []
        for i in range(3):
            Rw = slice((3 * h + i) * H + row, (3 * h + i) * H + row + 8)
            kk = kf[m0:m0 + n, Rw, L]
            if i == 0 and a is not None:
                k0 = _tie(kk[0], a)[None]
                kk = k0 if n == 1 else jnp.concatenate([k0, kk[1:]], axis=0)
            t.append(jnp.sum(kk * uf[u0:u0 + n, Rw, L], axis=0))
        return t[0] - t[2], t[0] + t[1]

    def AR(h, q, row):
        return slice((2 * h + q) * H + row, (2 * h + q) * H + row + 8)

    def mac(n, u0, sl, first=False, part=False):
        def mk(t, rc):
            st, fin = [], []

            def piece(i):
                def fn(a):
                    h, row = i & 1, rc + (i >> 1) * 8
                    zr, zi = cmul(0, u0, n, h, row, C(t), a)
                    if part:
                        zr, zi = zr + acc[0, AR(h, 0, row), C(t)], zi + acc[0, AR(h, 1, row), C(t)]
                    st.append((zr, zi))
                    if h:
                        (pr, pi), (mr, mi) = st[-2:]
                        z = [pr + mr, pi + mi, pr - mr, pi - mi]
                        Rw = lambda q: slice(q * H + row, q * H + row + 8)
                        pv = None if first else [zraw[Rw(q ^ 1), C(t)] for q in range(4)]
                        for q in range(4):
                            zraw[Rw(q), C(t)] = z[q]
                        if not first:
                            z = [z[q] + pv[q] if (q & 1) == (rc < 64) else z[q] - pv[q] for q in range(4)]
                        fin.append(z)
                    if i == 3:
                        for q in range(4):
                            w = (q * H + rc) // 2
                            zz_w[sl, w:w + 8, C(t)] = _pack(fin[0][q], fin[1][q])
                return fn
            if not part:
                return [piece(i) for i in range(4)]
            both = lambda f, g: (lambda a: (f(a), g(None)))
            return [both(piece(0), piece(1)), both(piece(2), piece(3))]
        return [[fn for rc in range(0, H, 16) for fn in mk(t, rc)] for t in range(NT)]

    def pos():
        return [(t, h, row) for t in range(NT) for row in range(0, H, 8) for h in range(2)]

    def ahead(i):
        def mk(t, h, row):
            def fn(a):
                zr, zi = cmul(i + 1, 0, NC, h, row, C(t), a)
                acc[i, AR(h, 0, row), C(t)] = zr
                acc[i, AR(h, 1, row), C(t)] = zi
            return fn
        return [mk(*p) for p in pos()]

    def spread():
        n = NB - NC - 1

        def mk(t, h, row):
            def fn(a):
                p = []
                for i in range(3):
                    Rw = slice((3 * h + i) * H + row, (3 * h + i) * H + row + 8)
                    u = uf[0, Rw, C(t)]
                    p.append(kf[1:1 + n, Rw, C(t)] * (_tie(u, a) if i == 0 else u)[None])
                acc[0:n, AR(h, 0, row), C(t)] = acc[1:1 + n, AR(h, 0, row), C(t)] + (p[0] - p[2])
                acc[0:n, AR(h, 1, row), C(t)] = acc[1:1 + n, AR(h, 1, row), C(t)] + (p[0] + p[1])
            return fn
        return [mk(*p) for p in pos()]

    def mmI(name, sl, ys):
        def unit(n):
            def epi(p):
                ce, se, co, so = p
                sub = lax.broadcasted_iota(I32, (8, 128), 0)
                c0 = ys * T + H
                y_v[n, ys * T:ys * T + 1, :] = (ce[64:72] - se[0:8])[0:1]
                se = jnp.concatenate([jnp.where(sub == 0, 0.0, se[0:8]), se[8:]], axis=0)
                for d, cc, ss in ((0, ce[0:64], se), (1, co, so)):
                    y_v[n, pl.ds(c0 + d, 64, stride=2), :] = cc + ss
                    lo = cc - ss
                    for i in range(0, 64, 8):
                        y_v[n, pl.ds(c0 - d - 2 * i - 14, 8, stride=2), :] = jnp.take_along_axis(
                            lo[i:i + 8], 7 - sub, axis=0)
            return Unit(name(n), [(lambda i=i: (tg_v[0:(GR if i == 0 else 64), C(i)], zz_v[sl, C(i), C(n)]))
                                  for i in range(4)], epi, 64, 52)
        return [unit(n) for n in range(NT)]

    def mod(name, a, b):
        def unit(n):
            def epi(p):
                v = [_sum(p[i * NT:(i + 1) * NT])[0:8] for i in range(b - a)]
                if a == 0:
                    mod_v[0, :, C(n)] = v[0] * v[2]
                    mod_v[1, :, C(n)] = (v[1] + 1.0) * v[2]
                elif a == 3:
                    mod_v[3, :, C(n)] = v[0]
                    mod_v[4, :, C(n)] = v[1] + 1.0
                else:
                    mod_v[5, :, C(n)] = v[0]
                    mod_v[2, :, C(n)] = v[0] * G_POST
            return Unit(name, [(lambda i=i, k=k: (silu_c[:, C(k)], wm_v[C(k), i * D + n * 128:i * D + (n + 1) * 128]))
                               for i in range(a, b) for k in range(NT)], epi, 16, 10, full=False, acc=b - a == 1)
        return [unit(n) for n in range(NT)]

    GS = range(0, T, RG)
    HS = (slice(0, 128), slice(128, 256))

    def tasks(f):
        return [(lambda a, r=r: f(slice(r, r + RG), a)) for r in GS]

    def load_y(sl, R):
        return jnp.concatenate([y_v[t, sl * T + R.start:sl * T + R.stop, :] for t in range(NT)],
                               axis=1).reshape(2, 8, D)

    def front(sl, xs, early=False):
        xx, hh, nn = view(x_v, xs), view(hb_v, xs), view(n1_v, sl)

        def fa(R, a):
            q = [q_n[t, sl * H + R.start // 2:sl * H + R.stop // 2, :] for t in range(NT)]
            q = jnp.concatenate([_tie(q[0], a)] + q[1:], axis=1)
            q = pltpu.bitcast(q, BF16).astype(F32).reshape(2, 8, D)
            x = (q + (_ln(q) * mod_v[1] + mod_v[0]) * load_y(sl, R)).reshape(RG, D)
            xx[R, :] = x
            if early:
                hh[R, :] = _ln(x)

        def fb(R, a):
            hh[R, :] = (_ln(_tie(xx[R, :], a).reshape(2, 8, D)) * mod_v[4] + mod_v[3]).reshape(RG, D)

        def fc(R, a):
            hb = _tie(hh[R, :], a)
            if early:
                hb = (hb.reshape(2, 8, D) * mod_v[4] + mod_v[3]).reshape(RG, D)
                hh[R, :] = hb
            nn[R, :] = _ln(hb, G_A).astype(BF16)
        return (tasks(fa), tasks(fc)) if early else tasks(fa) + tasks(fb) + tasks(fc)

    def shift(hs, sl, pieces=((0, 64), (64, 64), (128, 64), (192, 64))):
        gg = view(g_v, sl)

        def mk(t, r, n):
            def fn(a):
                lane = lax.broadcasted_iota(I32, (n, 128), 1)
                ld = lambda d: h1_v[t, pl.ds(hs * T + 8 + r + d, n), :]
                if t == 0:
                    g = ld(-1)
                elif t == 1:
                    g = jnp.where(lane < 32, ld(-1), ld(1))
                elif t == 2:
                    g = jnp.where(lane < 64, ld(1), ld(-2))
                elif t == 3:
                    g = jnp.where(lane < 96, ld(-2), ld(2))
                else:
                    g = ld(2)
                if a is not None:
                    g = jnp.concatenate([_tie(g[i:i + 8], a) if i % 16 == 0 else g[i:i + 8]
                                         for i in range(0, n, 8)], axis=0)
                gg[r:r + n, C(t)] = g.astype(BF16)
            return fn
        return [[mk(t, r, n) for r, n in pieces] for t in range(NT)]

    def shift_early():
        def keep(t):
            def fn(a):
                h1_v[t, 2 * T - 16:2 * T + 8, :] = h1_v[t, 3 * T - 16:3 * T + 8, :]
            return fn
        sh = shift(2, 0, ((0, 64), (64, 64), (128, 64), (192, 48)))
        return [fn for t in range(NT) for fn in sh[t] + [keep(t)]]

    def ln2(xs, sl):
        xx, nn = view(x1_v, xs), view(n2_v, sl)

        def f(R, a):
            nn[R, :] = _ln(_tie(xx[R, :], a), G_A).astype(BF16)
        return tasks(f)

    def resid(xs, x1s, rotate=False):
        xx, x1 = view(x_v, xs), view(x1_v, x1s)

        def f(R, a):
            gb = mod_v[5] if a is None else pltpu.bitcast(
                pltpu.bitcast(mod_v[5], U32) | jnp.concatenate([a] * NT, axis=1), F32)
            r_v[R, :] = xx[R, :] + (x1[R, :].reshape(2, 8, D) * gb).reshape(RG, D)
            if rotate:
                xx[R, :] = x_v[R, :]
                view(hb_v, 1)[R, :] = hb_v[R, :]
        return tasks(f)

    def mm1(name, hs, sl):
        nn = view(n1_v, sl)

        def unit(n, R):
            def epi(p):
                h1_v[n, pl.ds(hs * T + 8 + R.start, 128), :] = _gelu2(p[0])
            return Unit(name, [(lambda k=k: (nn[R, C(k)], w1_v[C(k), C(n)])) for k in range(NT)],
                        epi, 128, 144, acc=True)
        return [unit(n, R) for n in range(NT) for R in HS]

    def mm2(name, sl, xs, x1s):
        gg, hh, x1 = view(g_v, sl), view(hb_v, xs), view(x1_v, x1s)

        def unit(n, R):
            def epi(p):
                x1[R, C(n)] = hh[R, C(n)] + p[0] * G_POST
            return Unit(name, [(lambda k=k: (gg[R, C(k)], w2_v[C(k), C(n)])) for k in range(NT)],
                        epi, 128, 96, acc=True)
        return [unit(n, R) for n in range(NT) for R in HS]

    def mm3(name, sl):
        nn, aa = view(n2_v, sl), view(a_v, sl)

        def unit(n, R):
            def epi(p):
                aa[R, C(n)] = _gelu2(p[0]).astype(BF16)
            return Unit(name, [(lambda k=k: (nn[R, C(k)], w3_v[C(n), C(k)])) for k in range(NT)],
                        epi, 128, 160, nt=True, acc=True)
        main = [unit(n, R) for n in range(FT - 1) for R in HS]
        F0, part = (FT - 1) * 128, []
        main[-1].tiles.pop(0)

        def epi(p):
            for i, R in enumerate(HS):
                aa[R, F0:F] = _gelu2(part[i] + p[i]).T.astype(BF16)
            main[-1].res = [jnp.concatenate(p[2:], axis=0)]
        rem = [Unit(name, [(lambda k=k, R=R: (w3_v[F0:F, C(k)], nn[R, C(k)])) for k in range(NT - 1)],
                    lambda p: part.append(p[0]), 64, 24, nt=True, acc=True) for R in HS]
        rem.append(Unit(name, [(lambda R=R: (w3_v[F0:F, C(NT - 1)], nn[R, C(NT - 1)])) for R in HS]
                        + [(lambda r=r: (nn[r:r + 64, C(0)], w3_v[C(FT - 2), C(0)])) for r in (128, 192)],
                        epi, 64, 120, nt=True))
        return _flat(main), _flat(rem)

    NA = LP[2] // 2 * 128

    def cp_out(j, os, L, sm, R=slice(0, T)):
        return cp(o_v.at[pl.ds(os * T + R.start, R.stop - R.start), L],
                  o_hbm.at[pl.ds(base(j, T) + R.start, R.stop - R.start), L], sem_o.at[sm])

    out_a = lambda j: cp_out(j, 0, slice(0, NA), 0)
    out_b = lambda j: cp_out(j, 0, slice(NA, D), 1)
    last = []

    def mm4(name, j, sl, os=0, xs=None, x1s=None):
        aa, oo = view(a_v, sl), view(o_v, os)

        def unit(n, R):
            def epi(p):
                if xs is None:
                    oo[R, C(n)] = (r_v[R, C(n)] + mod_v[2, 0:1, C(n)] * p[0]).astype(BF16)
                else:
                    oo[R, C(n)] = (view(x_v, xs)[R, C(n)] + mod_v[5, 0:1, C(n)]
                                   * (view(x1_v, x1s)[R, C(n)] + p[0] * G_POST)).astype(BF16)
                if os == 2:
                    last.append(cp_out(j, os, C(n), 2, R))
                    last[-1].start()
                elif R.stop == T and (os, (n + 1) * 128) in ((1, D), (3, NA)):
                    last.append(cp_out(j, os, slice(0, (n + 1) * 128), 2))
                    last[-1].start()
                elif R.stop == T and os == 0 and (n + 1) * 128 in (NA, D):
                    (out_a if (n + 1) * 128 == NA else out_b)(j).start()
            return Unit(name, [(lambda k=k: (aa[R, C(k)], w4_v[C(k), C(n)])) for k in range(FT)],
                        epi, 128, 16 * (16 if xs is None else 18), acc=True)
        return [unit(n, R) for n in range(NT) for R in HS]

    def quarter(u):
        mk = u.tiles.pop(0)
        st = []

        def piece(i):
            if not st:
                st.extend(mk())
            return st[0][32 * i:32 * i + 32], st[1]

        def epi(p):
            u.res = [jnp.concatenate(p, axis=0)]
        return _flat([Unit(u.name, [(lambda i=i: piece(i)) for i in range(4)], epi, 32, 0, nt=u.nt)])

    W = lambda nm: [("wait", nm)]
    run = lambda fns: [("run", "run", lambda: [fn(None) for fn in fns])]
    one = lambda us: [_flat([u]) for u in us]
    cat = lambda ls: [x for l in ls for x in l]
    nm = lambda x: (lambda n: x)

    seq, grp = [], []
    for s in range(NC):
        seq += W("c%d" % s) + _flat((mmI(nm("I0"), 0, 0) if s == 2 else []) + mmK(s) + mmU(nm("U%d" % s), s % 2, NC - 1 - s))
        grp.append(Group("kv%d" % s, cat(kv(s, s % 2)), 50, ["c%d" % s], ["U%d" % s], 100))
    grp.append(Group("mac0", cat(mac(1, 2, 0, first=True)), 12, ["c1"], ["c2"], 0))
    grp.append(Group("mac1", cat(mac(2, 1, 1)), 18, ["c2"], ["kr"], 0))
    grp.append(Group("mac2", cat(mac(3, 0, 0)), 24, ["kr"], ["I2"], 300))
    seq += W("kr") + _flat(mmI(nm("I1"), 1, 1) + cat(mmK(m) for m in range(NC, NB)) + mmI(nm("I2"), 0, 2))
    start = lambda cs: [("run", "run", lambda: [c.start() for c in cs])]
    f0, f1 = front(0, 2, True), front(1, 1, True)
    seq += W("wma") + _flat(mod("moda", 0, 3)) + run(f0[0] + f1[0])
    seq += W("wmb") + start(next_kv(NC) + next_q(NC)) + _flat(mod("modb", 3, 5)) + run(f0[1] + f1[1])
    w1 = _flat(mm1("w1_0", 0, 0) + mm1("w1_1", 1, 1))
    seq += W("w1") + w1[:LP[4]] + W("w2") + w1[LP[4]:] + run(cat(shift(0, 0)))
    seq += _flat(mm2("w2_0", 0, 2, 1) + mm1("w1_2", 2, 2)) + run(cat(shift(1, 1))) + _flat(mm2("w2_1", 1, 1, 0))
    grp.append(Group("f2", front(2, 0), 80, ["w2"], ["w1_2"], 450))
    grp.append(Group("ln2_0", ln2(1, 0), 60, ["w2_0"], ["w3"], 450))
    grp.append(Group("ahead", cat(ahead(i) for i in range(NB - NC)), 19, ["w1"], ["end"], 100))
    _wait(seq, "w3")
    a, r = mm3("w3_0", 0)
    _mix(seq, a, [r], 0.1)
    mc = _flat(mod("modc", 5, 6))
    _wait(seq, "w4", mc[:5] + [("sync", "run", lambda: None)])
    w4 = mm4("w4_0", 0, 0, 3, 2, 1)[:LP[2]]
    qs = [quarter(w4[-1 - i]) for i in range((_phase(seq) + FT * LP[2]) % 4)]
    _mix(seq, _flat(w4), [mc[i:i + 4] for i in range(5, 25, 4)] + qs, 0.01, 0.4)
    assert _phase(seq) == 0
    grp.append(Group("resid", resid(2, 1), 26, ["modc"], ["end"], 100))
    _emit(seq, grp, zero, wait)

    def step(s, carry):
        with scope("wait_blk"):
            for c in next_kv(s) + next_q(s):
                c.wait()
        nxt = jnp.minimum(s + 1, NB - 1)
        seq, grp = [], []
        a, r = mm3("w3", 0)
        us, it = one(mmU(lambda n: "U%d" % n, 0, 0)), one(mmI(lambda n: "I%d" % n, 0, 0))
        w4 = mm4("w4", s - 2, 0)
        q = quarter(w4[LP[1] - 1])
        _mix(seq, _flat(mm4("w4c", s - 3, 0)[LP[2]:]) + a,
             [us[0], us[1], us[2], it[0] + us[3], it[1] + us[4], it[2] + start(next_kv(nxt)), it[3], it[4], r],
             LP[3], LP[0])
        _mix(seq, _flat(w4[:LP[1]]), [q])
        w1 = _flat(mm1("w1", 2, 0))
        seq += w1[:8] + start(next_q(nxt)) + w1[8:] + run(cat(shift(1, 0, ((T - 16, 16),))))
        seq += _flat(w4[LP[1]:LP[2]] + mm2("w2", 0, 1, 0))
        assert _phase(seq) == 0
        kvs, macs = kv(0, 0), mac(1, 0, 0, part=True)
        for t in range(NT):
            grp.append(Group("kv%d" % t, kvs[t], 50, ["start"], ["U%d" % t], 300))
            grp.append(Group("mac%d" % t, macs[t], 28, ["U%d" % t], ["I%d" % t], 300, 150))
        iall = ["I%d" % t for t in range(NT)]
        grp.append(Group("ln2", ln2(0, 0), 60, ["start"], ["w3"], 450))
        grp.append(Group("resid", resid(1, 0, True), 40, ["w4c"], ["w4", "I4"], 100))
        grp.append(Group("front", front(0, 0), 80, iall, ["w1"], 450))
        grp.append(Group("spread", spread(), 30, iall, ["end"], 100))
        grp.append(Group("shift", shift_early(), 12, ["start"], ["w1"], 200))
        _emit(seq, grp, zero, wait)
        out_b(s - 3).wait()
        out_a(s - 2).wait()
        return carry

    lax.fori_loop(NC, NB, step, 0)

    seq, grp = [], []
    seq += _flat(mm4("w4_5", NB - 3, 0)[LP[2]:])
    a, r = mm3("w3_6", 0)
    _mix(seq, a, [r])
    seq += _flat(mm2("w2_7", 0, 0, 1) + mm4("w4_6", NB - 2, 0, 1, 1, 0))
    a, r = mm3("w3_7", 1)
    _mix(seq, a, [r])
    seq += _flat(mm4("w4_7", NB - 1, 1, 2, 0, 1))
    assert _phase(seq) == 0
    grp.append(Group("ln2_6", ln2(0, 0), 60, ["start"], ["w3_6"], 450))
    grp.append(Group("shift7", cat(shift(2, 0)), 14, ["start"], ["w2_7"], 200))
    grp.append(Group("ln2_7", ln2(1, 1), 60, ["w2_7"], ["w3_7"], 450))
    _emit(seq, grp, zero, wait)
    with scope("wait_out"):
        for c in next_kv(NB - 1) + next_q(NB - 1) + [out_b(NB - 3)] + last:
            c.wait()


@jax.jit
def pallas_adaLN_cond__ssm_conv_h3__mixer_s_mlp__prompt_kernel(A_q, A_k, A_v, A_shift_k, A_ssm_k, A_ssm_D, B_x, B_w1, B_w2, B_w3, B_w4, c, w_mod):
    any_ = pl.BlockSpec(memory_space=pl.ANY)
    V = pltpu.VMEM
    out = pl.pallas_call(
        kernel,
        in_specs=[any_] * 12,
        out_specs=any_,
        out_shape=jax.ShapeDtypeStruct((S, D), BF16),
        scratch_shapes=[
            V((NT, NC * H + 8, 128), U32), V((NT, NC * H + 8, 128), U32), V((NT, NC * H + 8, 128), U32),
            V((D // 2, S), U32),
            V((D // 2, D), U32), V((D // 2, D), U32), V((F // 2, D), U32), V((F // 2, D), U32),
            V((D // 2, 6 * D), U32), V((4 * T, D), BF16),
            V((4, D), BF16), V((D,), BF16), V((1, D), BF16), V((8, 128), I32), pltpu.SMEM((8, 128), I32),
            V((5, 8, D), F32), V((6, 8, D), F32), V((T // 2, 4 * H), U32), V((GR // 2, 2 * T), U32),
            V((NB, 3 * T + 8, D), F32), V((NC, 3 * T + 8, D), F32), V((NB - NC, 2 * T + 8, D), F32), V((2 * T, D), F32),
            V((2, T // 2, D), U32), V((2, T, D), U32), V((NT, NC * T + 8, 128), F32),
            V((3 * T, D), F32), V((3 * T, D), F32), V((2 * T, D), F32), V((T, D), F32),
            V((3 * T // 2, D), U32), V((T, D), U32), V((T, D), U32), V((NT, NC * T + 24, 128), F32),
            V((T, (FT + 1) * 128), U32),
            pltpu.SemaphoreType.DMA((11,)), pltpu.SemaphoreType.DMA((1,)), pltpu.SemaphoreType.DMA((3,)),
        ],
        compiler_params=pltpu.CompilerParams(vmem_limit_bytes=110 << 20, disable_semaphore_checks=True,
                                             disable_bounds_checks=True),
        name="fused",
    )(A_q[0], A_k[0], A_v[0], A_shift_k.T, A_ssm_k, A_ssm_D, B_w1, B_w2, B_w3.T, B_w4, c, w_mod)
    return out[None]
```

```python
import contextlib
import heapq
import numpy as np
import jax
import jax.numpy as jnp
from jax import lax
from jax.experimental import pallas as pl
from jax.experimental.pallas import tpu as pltpu

S, D, F = 2048, 640, 1728
T = 256
H = T // 2
NB = S // T
NT = D // 128
FT = (F + 127) // 128
EPS = 1e-5
F32, BF16, U32, I32 = jnp.float32, jnp.bfloat16, jnp.uint32, jnp.int32
G_C1 = 0.044715 * float(np.sqrt(2.0 / np.pi))
G_C2 = float(np.sqrt(2.0 / np.pi))
G_A = G_C1 ** (1.0 / 3.0)
G_B = G_C2 / G_A
G_POST = 0.5 / G_A
RG = 16
GR = 80
NC = 3
VERBOSE = False
SCOPES = False
SLOT = 32
LP = (0.8, 4, 6, 0.15, 72)


def _unzip(p):
    return (p & -16) | ((p & 1) << 3) | ((p >> 1) & 7)


def _dft(shape, f_axis, tau, scale=1.0):
    r = lax.broadcasted_iota(I32, shape, f_axis)
    l = lax.broadcasted_iota(I32, shape, 1 - f_axis)
    if f_axis == 1:
        r = _unzip(r)
    f = r & 127
    odd = ((f & 63) << 2) | ((f >> 6) << 1) | 1
    p = odd * tau(l) + ((r >> 7) << 8)
    a = ((p + 512) & 1023) - 512
    u = (256 - jnp.abs(a)).astype(F32) * (np.pi / 512.0)
    u2 = u * u
    c = [scale, -scale / 6.0, scale / 120.0, -scale / 5040.0, scale / 362880.0, -scale / 39916800.0]
    poly = c[5]
    for ci in c[4::-1]:
        poly = poly * u2 + ci
    return (u * poly).astype(BF16)


def _ln(x, scale=1.0):
    m = jnp.sum(x, axis=-1, keepdims=True) * (1.0 / D)
    xc = x - m
    s2 = 1.0 / (scale * scale)
    v = jnp.sum(xc * xc, axis=-1, keepdims=True) * (s2 / D) + EPS * s2
    r = jnp.exp2(jnp.log(v) * float(-0.5 / np.log(2.0)))
    return xc * r


def _gelu2(x):
    u = x * (x * x + G_B)
    return x * (1.0 + jnp.tanh(u))


def _lo(w):
    return pltpu.bitcast(w << 16, F32)


def _hi(w):
    return pltpu.bitcast(w & jnp.uint32(0xFFFF0000), F32)


def _pack(a, b):
    return pltpu.pack_elementwise([a, b], packed_dtype=BF16)


def _tie(x, a):
    if a is None:
        return x
    w = pltpu.bitcast(x[:, :128], U32)
    k = w.shape[0] // 8
    w = w | (a if k == 1 else jnp.concatenate([a] * k, axis=0))
    w = pltpu.bitcast(w, x.dtype)
    return w if x.shape[1] == 128 else jnp.concatenate([w, x[:, 128:]], axis=1)


def C(i, lim=F):
    return slice(i * 128, min((i + 1) * 128, lim))


class Unit:
    def __init__(self, name, tiles, epi, rows, cost, nt=False, full=True, acc=False):
        self.acc, self.res = acc, []
        self.name, self.tiles, self.epi, self.rows, self.cost, self.nt, self.full = name, tiles, epi, rows, cost, nt, full


class Group:
    def __init__(self, name, fns, cost, rel, dead, lat, rlat=200):
        self.name, self.fns, self.cost, self.rel, self.dead, self.lat, self.rlat = name, fns, cost, rel, dead, lat, rlat


def _plan(seq, groups):
    busy, n = [0] * 4, 0
    start, end, tiles, bars = {}, {}, [], []
    for it in seq:
        if isinstance(it[0], Unit):
            u = it[0]
            m = n % 4
            n += 1
            t0, t1 = busy[m], busy[m] + max(u.rows, 32)
            busy[m] = t1
            tiles.append((t0, t1, u.cost / len(u.tiles)))
            start.setdefault(u.name, t0)
            end[u.name] = max(end.get(u.name, 0), t1)
        elif it[0] == "wait":
            t = max(busy)
            busy, n = [t] * 4, 0
            start[it[1]] = end[it[1]] = t
            bars.append(t)
    total = max(busy)
    start["end"] = end["end"] = total
    start["start"] = end["start"] = 0
    ns = total // SLOT + 2
    load = np.zeros(ns)
    for t0, t1, c in tiles:
        a, b = t0 // SLOT, max(t1 // SLOT, t0 // SLOT + 1)
        load[a:b] += c / (b - a)
    win = []
    for g in groups:
        r = max(end[x] + (0 if start[x] == end[x] else g.rlat) for x in g.rel)
        d = min(start[x] for x in g.dead) - g.lat
        ok = np.zeros(ns, bool)
        ok[r // SLOT:max(d // SLOT, r // SLOT + 1)] = True
        for b in bars:
            if r < b <= d:
                ok[max((b - g.lat) // SLOT, 0):b // SLOT] = False
        win.append(np.nonzero(ok)[0])
    alloc = [np.zeros(len(w)) for w in win]
    for _ in range(60):
        for i, g in enumerate(groups):
            w = win[i]
            load[w] -= alloc[i]
            base = load[w]
            vol = g.cost * len(g.fns)
            lo, hi = base.min(), base.max() + vol
            for _ in range(50):
                mid = 0.5 * (lo + hi)
                if np.maximum(mid - base, 0).sum() > vol:
                    hi = mid
                else:
                    lo = mid
            alloc[i] = np.maximum(hi - base, 0)
            load[w] += alloc[i]
    times = []
    for i, g in enumerate(groups):
        cum = np.cumsum(alloc[i])
        ts = []
        for k in range(len(g.fns)):
            x = (k + 0.5) * cum[-1] / len(g.fns)
            j = int(np.searchsorted(cum, x))
            prev = cum[j - 1] if j else 0.0
            ts.append(win[i][j] * SLOT + SLOT * (x - prev) / max(alloc[i][j], 1e-9))
        times.append(ts)
        if VERBOSE:
            print("%8s window %6d..%6d used %6d..%6d" % (g.name, win[i][0] * SLOT, win[i][-1] * SLOT, ts[0], ts[-1]))
    if VERBOSE:
        k = 2048 // SLOT
        print("total", total, "load/cycle:", " ".join("%.1f" % (load[i:i + k].mean() / SLOT) for i in range(0, ns, k)))
    return times


def _emit(seq, groups, zero, wait):
    times = _plan(seq, groups)
    left = {"start": 0}
    for it in seq:
        nm = it[0].name if isinstance(it[0], Unit) else it[1]
        left[nm] = left.get(nm, 0) + 1
    heap, pend, todo, cnt = [], {}, list(range(len(groups))), 0
    busy, n = [0] * 4, 0

    def release():
        nonlocal cnt
        for i in list(todo):
            g = groups[i]
            if all(left[x] == 0 for x in g.rel):
                todo.remove(i)
                pend[i] = len(g.fns)
                for t, fn in zip(times[i], g.fns):
                    heapq.heappush(heap, (t, cnt, i, fn))
                    cnt += 1

    def force(name):
        nonlocal heap
        for i, g in enumerate(groups):
            if name in g.dead:
                assert i not in todo, (g.name, name)
                if pend[i]:
                    if VERBOSE:
                        print("forcing", g.name, pend[i], "before", name)
                    for it in sorted(x for x in heap if x[2] == i):
                        it[3](None)
                    heap = [x for x in heap if x[2] != i]
                    heapq.heapify(heap)
                    pend[i] = 0

    release()
    for it in seq:
        if isinstance(it[0], Unit):
            u, k = it
            force(u.name)
            lhs, rhs = u.tiles[k]()
            dn = (((1,), (1 if u.nt else 0,)), ((), ()))
            p = lax.dot_general(lhs, rhs, dn, preferred_element_type=F32)
            u.res = [p + u.res[0]] if (u.acc and u.res) else u.res + [p]
            m = n % 4
            n += 1
            t0 = busy[m]
            busy[m] = t0 + max(u.rows, 32)
            while u.full and heap and heap[0][0] < t0 + u.rows:
                t, _, i, fn = heapq.heappop(heap)
                pend[i] -= 1
                r = min(max(int(t - t0), 0), u.rows - 1) // 8 * 8
                fn(pltpu.bitcast(p[r:r + 8], U32) & zero)
            if k == len(u.tiles) - 1:
                u.epi(u.res)
            left[u.name] -= 1
        elif it[0] == "wait":
            force(it[1])
            wait(it[1])
            busy, n = [max(busy)] * 4, 0
            left[it[1]] -= 1
        else:
            it[2]()
            left[it[1]] -= 1
        release()
    force("end")
    assert not heap and not todo


def _sum(ps):
    acc = ps[0]
    for p in ps[1:]:
        acc = acc + p
    return acc


def _flat(us):
    return [(u, i) for u in us for i in range(len(u.tiles))]


def _phase(seq):
    n = 0
    for it in seq:
        n = n + 1 if isinstance(it[0], Unit) else (0 if it[0] in ("wait", "sync") else n)
    return n % 4


def _mix(seq, a, b, lo=0.0, hi=1.0):
    n, k = _phase(seq), 0
    for i, t in enumerate(a):
        if k < len(b) and n % 4 == 0 and t[1] != 1 and i >= len(a) * (lo + (hi - lo) * k / len(b)):
            seq.extend(b[k])
            k += 1
        seq.append(t)
        n += 1
    assert k == len(b)


def _wait(seq, name, head=()):
    r = _phase(seq)
    assert all(isinstance(it[0], Unit) for it in seq[len(seq) - r:])
    seq[len(seq) - r:len(seq) - r] = [("wait", name)] + list(head)


def kernel(q_hbm, k_hbm, v_hbm, sh_hbm, ssm_hbm, sd_hbm, w1_hbm, w2_hbm, w3_hbm, w4_hbm, c_hbm, wm_hbm,
           o_hbm,
           q_n, k_n, v_n, ssm_w, w1_w, w2_w, w3_w, w4_w, wm_w, o_v,
           sh_v, sd_v, c_v, zsrc, z_s, taps, mod_v, tf_w, tg_w,
           kf, uf, acc, zraw, kv_w, zz_w, y_v, x_v, hb_v, x1_v, r_v, n1_w, n2_w, g_w, h1_v, a_w,
           sem, sem_b, sem_o):
    bf = lambda r: r.bitcast(BF16)
    w1_v, w2_v, w3_v, w4_v = bf(w1_w), bf(w2_w), bf(w3_w), bf(w4_w)
    wm_v = {0: bf(wm_w[0]), 3: bf(wm_w[1]), 5: bf(wm_w[2])}
    tf_v, tg_v, n1_v, n2_v, g_v = bf(tf_w), bf(tg_w), bf(n1_w), bf(n2_w), bf(g_w)
    a_v = bf(a_w)
    cp = pltpu.make_async_copy
    scope = lambda nm: jax.named_scope(nm) if SCOPES else contextlib.nullcontext()

    def base(j, n):
        return j * n if isinstance(j, int) else pl.multiple_of(j * n, n)

    def rows(j, n=1, size=T):
        return pl.ds(base(j, size), n * size)

    def view(ref, j, size=T):
        return ref.at[rows(j, 1, size)]

    dmas = {}

    def group(name, *mks):
        sm = sem.at[len(dmas)]
        dmas[name] = [c for mk in mks for c in mk(sm)]

    def ssm_in(t):
        return lambda sm: [cp(ssm_hbm.at[C(t)], bf(ssm_w[t]), sm)]

    def cols(src, start, n, dst, row=0):
        return lambda sm: [cp(src.at[pl.ds(start, n), C(t)], bf(dst).at[t, pl.ds(row, n)], sm) for t in range(NT)]

    def kv_in(s, sl):
        if isinstance(s, int):
            kk = cols(k_hbm, s * T - 16, T + 16, k_n[sl]) if s else cols(k_hbm, 0, T, k_n[sl], 16)
        else:
            kk = cols(k_hbm, pl.multiple_of(s * T - 16, 16), T + 16, k_n[sl])
        return lambda sm: kk(sm) + cols(v_hbm, base(s, T), T, v_n[sl])(sm)

    def q_in(s, sl):
        return cols(q_hbm, base(s, T), T, q_n[sl])

    def wm_in(a, b):
        return lambda sm: [cp(wm_hbm.at[:, a * D:b * D], wm_v[a], sm)]

    def whole(src, dst):
        return lambda sm: [cp(src, dst, sm)]

    next_kv = lambda s: kv_in(s, 0)(sem_b.at[0])
    next_q = lambda s: q_in(s, 0)(sem_b.at[0])

    zsrc[...] = jnp.zeros((8, 128), I32)
    k_n[0][:, 0:8, :] = jnp.zeros((NT, 8, 128), U32)
    group("small", lambda sm: [cp(zsrc, z_s, sm), cp(sh_hbm, sh_v, sm), cp(sd_hbm, sd_v, sm), cp(c_hbm, c_v, sm)])
    for s in range(NC):
        group("c%d" % s, ssm_in(s), kv_in(s, s))
    group("c3", ssm_in(3), ssm_in(4))
    group("wma", wm_in(0, 3), q_in(0, 0), q_in(1, 1))
    group("wmb", wm_in(3, 5))
    group("w1", whole(w1_hbm, w1_v))
    group("w2", q_in(2, 2), whole(w2_hbm, w2_v))
    group("w3", whole(w3_hbm, w3_v))
    group("w4", whole(w4_hbm, w4_v), wm_in(5, 6))
    for g in dmas.values():
        for c in g:
            c.start()

    def wait(name):
        with scope("wait_" + name):
            for c in dmas[name]:
                c.wait()

    tau_b = lambda l: H + ((l + (H - 1)) & (H - 1))
    tf_v[:, C(0)] = _dft((T, H), 0, lambda l: jnp.where((l & 1) == 0, l, tau_b(l)), 1.0 / T)
    tf_v[:, C(1)] = _dft((T, H), 0, lambda l: jnp.where((l & 1) == 1, l, tau_b(l)), 1.0 / T)
    tf_v[:, C(2)] = _dft((T, H), 0, lambda l: 2 * _unzip(l) - H)
    tf_v[:, C(3)] = _dft((T, H), 0, lambda l: 2 * _unzip(l) + 1 - H)
    sin0 = lax.broadcasted_iota(I32, (GR, T), 1) >= H
    tg_v[:, 0:T] = _dft((GR, T), 1, lambda l: jnp.where(sin0 & (l == 0), H, 2 * l))
    tg_v[:, T:2 * T] = _dft((GR, T), 1, lambda l: 2 * l + 1)
    h1_v[:, 0:8, :] = jnp.zeros((NT, 8, 128), F32)
    h1_v[:, 8 + NC * T:16 + NC * T, :] = jnp.zeros((NT, 8, 128), F32)

    wait("small")
    z = jnp.clip(z_s[0, 0], 0, 1)
    zero = jnp.full((8, 128), z, I32).astype(U32)
    z8 = pl.multiple_of(z * 8, 8)
    for r in (x_v, hb_v, x1_v, r_v, zraw, n1_w, n2_w, g_w, a_w):
        r[pl.ds(z8, 8), 0:128] = jnp.zeros((8, 128), r.dtype)
    for r in (kf, uf, acc, kv_w, zz_w, taps, mod_v):
        r[z, 0:8, 0:128] = jnp.zeros((8, 128), r.dtype)
    for r in (tf_w, tg_w):
        r[pl.ds(z8, 8), 0:128] = r[0:8, 0:128]
    sh = sh_v[...].astype(F32)
    for i in range(4):
        taps[i] = jnp.broadcast_to(sh[i:i + 1], (8, D))
    taps[4] = jnp.broadcast_to(sd_v[...].astype(F32).reshape(1, D) * (1.0 / T), (8, D))
    cf = c_v[...].astype(F32)
    silu_c = jnp.broadcast_to((cf / (1.0 + jnp.exp(-cf))).astype(BF16), (16, D))

    def mmK(n):
        def unit(m):
            st = []

            def rhs(i):
                if not st:
                    ev = (lax.broadcasted_iota(I32, (64, 128), 1) & 1) == 0
                    a = ssm_w[n][:, m * T:m * T + H]
                    b = pltpu.roll(ssm_w[n][:, m * T + H:(m + 1) * T], 1, 1)
                    st.extend([pltpu.bitcast(jnp.where(ev, a, b), BF16), pltpu.bitcast(jnp.where(ev, b, a), BF16)])
                return st[i]

            def epi(p):
                er, ei, or_, oi = p
                if m == 0:
                    er = er + taps[4, 0:1, C(n)]
                for h, (cr, ci) in enumerate(((er + or_, ei + oi), (er - or_, ei - oi))):
                    B = h * 3 * H
                    kf[m, B:B + H, C(n)] = cr
                    kf[m, B + H:B + 2 * H, C(n)] = ci - cr
                    kf[m, B + 2 * H:B + 3 * H, C(n)] = ci + cr
            return Unit("K%d" % n, [(lambda i=i, r=r: (tf_v[r:r + H, C(i)], rhs(i))) for i in range(2) for r in (0, H)],
                        epi, H, 170, nt=True)
        return [unit(m) for m in range(NB)]

    def kv(s, sl):
        def mk(t, w):
            def fn(a):
                ld = lambda o, n: k_n[s][t, pl.ds(8 + w + o, n), :]
                c0 = jnp.concatenate([_tie(ld(0, 8), a), ld(8, 8)], axis=0).reshape(2, 8, 128)
                c1, c2 = ld(-1, 16).reshape(2, 8, 128), ld(-2, 16).reshape(2, 8, 128)
                s0, s1, s2, s3 = (taps[i, :, C(t)] for i in range(4))
                ke, ko, ke1, ko1, ko2 = _lo(c0), _hi(c0), _lo(c1), _hi(c1), _hi(c2)
                wv = v_n[s][t, w:w + 16, :].reshape(2, 8, 128)
                kve = ((s0 * ke + s1 * ko1) + (s2 * ke1 + s3 * ko2)) * _lo(wv)
                kvo = ((s0 * ko + s1 * ke) + (s2 * ko1 + s3 * ke1)) * _hi(wv)
                kv_w[sl, w // 2:w // 2 + 8, C(t)] = _pack(kve[0], kve[1])
                kv_w[sl, (H + w) // 2:(H + w) // 2 + 8, C(t)] = _pack(kvo[0], kvo[1])
            return fn
        return [[mk(t, w) for w in range(0, H, 16)] for t in range(NT)]

    def words(ref, sl, i, n):
        return pltpu.bitcast(ref[sl, 64 * i:64 * (i + 1), C(n)], BF16)

    def mmU(name, sl, us):
        def unit(n):
            def epi(p):
                er, ei, or_, oi = p
                for h, (cr, ci) in enumerate(((er + or_, ei + oi), (er - or_, ei - oi))):
                    B = h * 3 * H
                    uf[us, B:B + H, C(n)] = cr + ci
                    uf[us, B + H:B + 2 * H, C(n)] = cr
                    uf[us, B + 2 * H:B + 3 * H, C(n)] = ci
            return Unit(name(n), [(lambda i=i, r=r: (tf_v[r:r + H, C(2 + i)], words(kv_w, sl, i, n)))
                                  for i in range(2) for r in (0, H)], epi, H, 120)
        return [unit(n) for n in range(NT)]

    def cmul(m0, u0, n, h, row, L, a):
        t = []
        for i in range(3):
            Rw = slice((3 * h + i) * H + row, (3 * h + i) * H + row + 8)
            kk = kf[m0:m0 + n, Rw, L]
            if i == 0 and a is not None:
                k0 = _tie(kk[0], a)[None]
                kk = k0 if n == 1 else jnp.concatenate([k0, kk[1:]], axis=0)
            t.append(jnp.sum(kk * uf[u0:u0 + n, Rw, L], axis=0))
        return t[0] - t[2], t[0] + t[1]

    def AR(h, q, row):
        return slice((2 * h + q) * H + row, (2 * h + q) * H + row + 8)

    def mac(n, u0, sl, first=False, part=False):
        def mk(t, rc):
            st, fin = [], []

            def piece(i):
                def fn(a):
                    h, row = i & 1, rc + (i >> 1) * 8
                    zr, zi = cmul(0, u0, n, h, row, C(t), a)
                    if part:
                        zr, zi = zr + acc[0, AR(h, 0, row), C(t)], zi + acc[0, AR(h, 1, row), C(t)]
                    st.append((zr, zi))
                    if h:
                        (pr, pi), (mr, mi) = st[-2:]
                        z = [pr + mr, pi + mi, pr - mr, pi - mi]
                        Rw = lambda q: slice(q * H + row, q * H + row + 8)
                        pv = None if first else [zraw[Rw(q ^ 1), C(t)] for q in range(4)]
                        for q in range(4):
                            zraw[Rw(q), C(t)] = z[q]
                        if not first:
                            z = [z[q] + pv[q] if (q & 1) == (rc < 64) else z[q] - pv[q] for q in range(4)]
                        fin.append(z)
                    if i == 3:
                        for q in range(4):
                            w = (q * H + rc) // 2
                            zz_w[sl, w:w + 8, C(t)] = _pack(fin[0][q], fin[1][q])
                return fn
            if not part:
                return [piece(i) for i in range(4)]
            both = lambda f, g: (lambda a: (f(a), g(None)))
            return [both(piece(0), piece(1)), both(piece(2), piece(3))]
        return [[fn for rc in range(0, H, 16) for fn in mk(t, rc)] for t in range(NT)]

    def pos():
        return [(t, h, row) for t in range(NT) for row in range(0, H, 8) for h in range(2)]

    def ahead(i):
        def mk(t, h, row):
            def fn(a):
                zr, zi = cmul(i + 1, 0, NC, h, row, C(t), a)
                acc[i, AR(h, 0, row), C(t)] = zr
                acc[i, AR(h, 1, row), C(t)] = zi
            return fn
        return [mk(*p) for p in pos()]

    def spread():
        n = NB - NC - 1

        def mk(t, h, row):
            def fn(a):
                p = []
                for i in range(3):
                    Rw = slice((3 * h + i) * H + row, (3 * h + i) * H + row + 8)
                    u = uf[0, Rw, C(t)]
                    p.append(kf[1:1 + n, Rw, C(t)] * (_tie(u, a) if i == 0 else u)[None])
                acc[0:n, AR(h, 0, row), C(t)] = acc[1:1 + n, AR(h, 0, row), C(t)] + (p[0] - p[2])
                acc[0:n, AR(h, 1, row), C(t)] = acc[1:1 + n, AR(h, 1, row), C(t)] + (p[0] + p[1])
            return fn
        return [mk(*p) for p in pos()]

    def mmI(name, sl, ys):
        def unit(n):
            def epi(p):
                ce, se, co, so = p
                sub = lax.broadcasted_iota(I32, (8, 128), 0)
                c0 = ys * T + H
                y_v[n, ys * T:ys * T + 1, :] = (ce[64:72] - se[0:8])[0:1]
                se = jnp.concatenate([jnp.where(sub == 0, 0.0, se[0:8]), se[8:]], axis=0)
                for d, cc, ss in ((0, ce[0:64], se), (1, co, so)):
                    y_v[n, pl.ds(c0 + d, 64, stride=2), :] = cc + ss
                    lo = cc - ss
                    for i in range(0, 64, 8):
                        y_v[n, pl.ds(c0 - d - 2 * i - 14, 8, stride=2), :] = jnp.take_along_axis(
                            lo[i:i + 8], 7 - sub, axis=0)
            return Unit(name(n), [(lambda i=i: (tg_v[0:(GR if i == 0 else 64), C(i)], words(zz_w, sl, i, n)))
                                  for i in range(4)], epi, 64, 52)
        return [unit(n) for n in range(NT)]

    def mod(name, a, b):
        def unit(n):
            def epi(p):
                v = [_sum(p[i * NT:(i + 1) * NT])[0:8] for i in range(b - a)]
                if a == 0:
                    mod_v[0, :, C(n)] = v[0] * v[2]
                    mod_v[1, :, C(n)] = (v[1] + 1.0) * v[2]
                elif a == 3:
                    mod_v[3, :, C(n)] = v[0]
                    mod_v[4, :, C(n)] = v[1] + 1.0
                else:
                    mod_v[5, :, C(n)] = v[0]
                    mod_v[2, :, C(n)] = v[0] * G_POST
            return Unit(name, [(lambda i=i, k=k: (silu_c[:, C(k)], wm_v[a][C(k), (i - a) * D + n * 128:(i - a) * D + (n + 1) * 128]))
                               for i in range(a, b) for k in range(NT)], epi, 16, 10, full=False, acc=b - a == 1)
        return [unit(n) for n in range(NT)]

    GS = range(0, T, RG)
    HS = (slice(0, 128), slice(128, 256))

    def tasks(f):
        return [(lambda a, r=r: f(slice(r, r + RG), a)) for r in GS]

    def load_y(sl, R):
        return jnp.concatenate([y_v[t, sl * T + R.start:sl * T + R.stop, :] for t in range(NT)],
                               axis=1).reshape(2, 8, D)

    def front(sl, xs, early=False):
        xx, hh, nn = view(x_v, xs), view(hb_v, xs), view(n1_v, sl)

        def fa(R, a):
            q = [q_n[sl][t, R.start // 2:R.stop // 2, :] for t in range(NT)]
            q = jnp.concatenate([_tie(q[0], a)] + q[1:], axis=1)
            q = pltpu.bitcast(q, BF16).astype(F32).reshape(2, 8, D)
            x = (q + (_ln(q) * mod_v[1] + mod_v[0]) * load_y(sl, R)).reshape(RG, D)
            xx[R, :] = x
            if early:
                hh[R, :] = _ln(x)

        def fb(R, a):
            hh[R, :] = (_ln(_tie(xx[R, :], a).reshape(2, 8, D)) * mod_v[4] + mod_v[3]).reshape(RG, D)

        def fc(R, a):
            hb = _tie(hh[R, :], a)
            if early:
                hb = (hb.reshape(2, 8, D) * mod_v[4] + mod_v[3]).reshape(RG, D)
                hh[R, :] = hb
            nn[R, :] = _ln(hb, G_A).astype(BF16)
        return (tasks(fa), tasks(fc)) if early else tasks(fa) + tasks(fb) + tasks(fc)

    def shift(hs, sl, pieces=((0, 64), (64, 64), (128, 64), (192, 64))):
        gg = view(g_v, sl)

        def mk(t, r, n):
            def fn(a):
                lane = lax.broadcasted_iota(I32, (n, 128), 1)
                ld = lambda d: h1_v[t, pl.ds(hs * T + 8 + r + d, n), :]
                if t == 0:
                    g = ld(-1)
                elif t == 1:
                    g = jnp.where(lane < 32, ld(-1), ld(1))
                elif t == 2:
                    g = jnp.where(lane < 64, ld(1), ld(-2))
                elif t == 3:
                    g = jnp.where(lane < 96, ld(-2), ld(2))
                else:
                    g = ld(2)
                if a is not None:
                    g = jnp.concatenate([_tie(g[i:i + 8], a) if i % 16 == 0 else g[i:i + 8]
                                         for i in range(0, n, 8)], axis=0)
                gg[r:r + n, C(t)] = g.astype(BF16)
            return fn
        return [[mk(t, r, n) for r, n in pieces] for t in range(NT)]

    def shift_early():
        def keep(t):
            def fn(a):
                h1_v[t, 2 * T - 16:2 * T + 8, :] = h1_v[t, 3 * T - 16:3 * T + 8, :]
            return fn
        sh = shift(2, 0, ((0, 64), (64, 64), (128, 64), (192, 48)))
        return [fn for t in range(NT) for fn in sh[t] + [keep(t)]]

    def ln2(xs, sl):
        xx, nn = view(x1_v, xs), view(n2_v, sl)

        def f(R, a):
            nn[R, :] = _ln(_tie(xx[R, :], a), G_A).astype(BF16)
        return tasks(f)

    def resid(xs, x1s, rotate=False):
        xx, x1 = view(x_v, xs), view(x1_v, x1s)

        def f(R, a):
            gb = mod_v[5] if a is None else pltpu.bitcast(
                pltpu.bitcast(mod_v[5], U32) | jnp.concatenate([a] * NT, axis=1), F32)
            r_v[R, :] = xx[R, :] + (x1[R, :].reshape(2, 8, D) * gb).reshape(RG, D)
            if rotate:
                xx[R, :] = x_v[R, :]
                view(hb_v, 1)[R, :] = hb_v[R, :]
        return tasks(f)

    def mm1(name, hs, sl):
        nn = view(n1_v, sl)

        def unit(n, R):
            def epi(p):
                h1_v[n, pl.ds(hs * T + 8 + R.start, 128), :] = _gelu2(p[0])
            return Unit(name, [(lambda k=k: (nn[R, C(k)], w1_v[C(k), C(n)])) for k in range(NT)],
                        epi, 128, 144, acc=True)
        return [unit(n, R) for n in range(NT) for R in HS]

    def mm2(name, sl, xs, x1s):
        gg, hh, x1 = view(g_v, sl), view(hb_v, xs), view(x1_v, x1s)

        def unit(n, R):
            def epi(p):
                x1[R, C(n)] = hh[R, C(n)] + p[0] * G_POST
            return Unit(name, [(lambda k=k: (gg[R, C(k)], w2_v[C(k), C(n)])) for k in range(NT)],
                        epi, 128, 96, acc=True)
        return [unit(n, R) for n in range(NT) for R in HS]

    def mm3(name, sl):
        nn, aa = view(n2_v, sl), view(a_v, sl)

        def unit(n, R):
            def epi(p):
                aa[R, C(n)] = _gelu2(p[0]).astype(BF16)
            return Unit(name, [(lambda k=k: (nn[R, C(k)], w3_v[C(n), C(k)])) for k in range(NT)],
                        epi, 128, 160, nt=True, acc=True)
        main = [unit(n, R) for n in range(FT - 1) for R in HS]
        F0, part = (FT - 1) * 128, []
        main[-1].tiles.pop(0)

        def epi(p):
            for i, R in enumerate(HS):
                aa[R, F0:F] = _gelu2(part[i] + p[i]).T.astype(BF16)
            main[-1].res = [jnp.concatenate(p[2:], axis=0)]
        rem = [Unit(name, [(lambda k=k, R=R: (w3_v[F0:F, C(k)], nn[R, C(k)])) for k in range(NT - 1)],
                    lambda p: part.append(p[0]), 64, 24, nt=True, acc=True) for R in HS]
        rem.append(Unit(name, [(lambda R=R: (w3_v[F0:F, C(NT - 1)], nn[R, C(NT - 1)])) for R in HS]
                        + [(lambda r=r: (nn[r:r + 64, C(0)], w3_v[C(FT - 2), C(0)])) for r in (128, 192)],
                        epi, 64, 120, nt=True))
        return _flat(main), _flat(rem)

    NA = LP[2] // 2 * 128

    def cp_out(j, os, L, sm, R=slice(0, T)):
        return cp(o_v.at[pl.ds(os * T + R.start, R.stop - R.start), L],
                  o_hbm.at[pl.ds(base(j, T) + R.start, R.stop - R.start), L], sem_o.at[sm])

    out_a = lambda j: cp_out(j, 0, slice(0, NA), 0)
    out_b = lambda j: cp_out(j, 0, slice(NA, D), 1)
    last = []

    def mm4(name, j, sl, os=0, xs=None, x1s=None):
        aa, oo = view(a_v, sl), view(o_v, os)

        def unit(n, R):
            def epi(p):
                if xs is None:
                    oo[R, C(n)] = (r_v[R, C(n)] + mod_v[2, 0:1, C(n)] * p[0]).astype(BF16)
                else:
                    oo[R, C(n)] = (view(x_v, xs)[R, C(n)] + mod_v[5, 0:1, C(n)]
                                   * (view(x1_v, x1s)[R, C(n)] + p[0] * G_POST)).astype(BF16)
                if os == 2:
                    last.append(cp_out(j, os, C(n), 2, R))
                    last[-1].start()
                elif R.stop == T and (os, (n + 1) * 128) in ((1, D), (3, NA)):
                    last.append(cp_out(j, os, slice(0, (n + 1) * 128), 2))
                    last[-1].start()
                elif R.stop == T and os == 0 and (n + 1) * 128 in (NA, D):
                    (out_a if (n + 1) * 128 == NA else out_b)(j).start()
            return Unit(name, [(lambda k=k: (aa[R, C(k)], w4_v[C(k), C(n)])) for k in range(FT)],
                        epi, 128, 16 * (16 if xs is None else 18), acc=True)
        return [unit(n, R) for n in range(NT) for R in HS]

    def quarter(u):
        mk = u.tiles.pop(0)
        st = []

        def piece(i):
            if not st:
                st.extend(mk())
            return st[0][32 * i:32 * i + 32], st[1]

        def epi(p):
            u.res = [jnp.concatenate(p, axis=0)]
        return _flat([Unit(u.name, [(lambda i=i: piece(i)) for i in range(4)], epi, 32, 0, nt=u.nt)])

    W = lambda nm: [("wait", nm)]
    run = lambda fns: [("run", "run", lambda: [fn(None) for fn in fns])]
    one = lambda us: [_flat([u]) for u in us]
    cat = lambda ls: [x for l in ls for x in l]
    nm = lambda x: (lambda n: x)

    seq, grp = [], []
    for s in range(NC):
        seq += W("c%d" % s) + _flat(mmK(s) + mmU(nm("U%d" % s), s % 2, NC - 1 - s))
        grp.append(Group("kv%d" % s, cat(kv(s, s % 2)), 50, ["c%d" % s], ["U%d" % s], 100))
    inv = [mmI(lambda n: "I%d" % n, s, s) for s in range(NC)]
    seq += W("c3") + _flat(mmK(3) + mmK(4) + [inv[s][t] for t in range(NT) for s in range(NC)])
    macs = [mac(s + 1, NC - 1 - s, s, first=s == 0) for s in range(NC)]
    grp.append(Group("mac00", macs[0][0], 12, ["c1"], ["c2"], 0))
    grp.append(Group("mac01", macs[1][0] + macs[0][1] + macs[1][1], 16, ["c2"], ["c3"], 0))
    for t in range(NT):
        grp.append(Group("mac%d" % t, cat(macs[s][t] for s in range(2 if t < 2 else 0, NC)), 24 if t < 2 else 18,
                         ["c3", "K%d" % t], ["I%d" % t], 100, 150))
    start = lambda cs: [("run", "run", lambda: [c.start() for c in cs])]
    f0, f1 = front(0, 2, True), front(1, 1, True)
    seq += W("wma") + _flat(mod("moda", 0, 3)) + run(f0[0] + f1[0])
    seq += W("wmb") + start(next_kv(NC) + next_q(NC)) + _flat(mod("modb", 3, 5)) + run(f0[1] + f1[1])
    w1 = _flat(mm1("w1_0", 0, 0) + mm1("w1_1", 1, 1))
    seq += W("w1") + w1[:LP[4]] + W("w2") + w1[LP[4]:] + run(cat(shift(0, 0)))
    seq += _flat(mm2("w2_0", 0, 2, 1) + mm1("w1_2", 2, 2)) + run(cat(shift(1, 1))) + _flat(mm2("w2_1", 1, 1, 0))
    grp.append(Group("f2", front(2, 0), 80, ["w2"], ["w1_2"], 450))
    grp.append(Group("ln2_0", ln2(1, 0), 60, ["w2_0"], ["w3"], 450))
    grp.append(Group("ahead", cat(ahead(i) for i in range(NB - NC)), 19, ["w1"], ["end"], 100))
    _wait(seq, "w3")
    a, r = mm3("w3_0", 0)
    _mix(seq, a, [r], 0.1)
    mc = _flat(mod("modc", 5, 6))
    _wait(seq, "w4", mc[:5] + [("sync", "run", lambda: None)])
    w4 = mm4("w4_0", 0, 0, 3, 2, 1)[:LP[2]]
    qs = [quarter(w4[-1 - i]) for i in range((_phase(seq) + FT * LP[2]) % 4)]
    _mix(seq, _flat(w4), [mc[i:i + 4] for i in range(5, 25, 4)] + qs, 0.01, 0.4)
    assert _phase(seq) == 0
    grp.append(Group("resid", resid(2, 1), 26, ["modc"], ["end"], 100))
    _emit(seq, grp, zero, wait)

    def step(s, carry):
        with scope("wait_blk"):
            for c in next_kv(s) + next_q(s):
                c.wait()
        nxt = jnp.minimum(s + 1, NB - 1)
        seq, grp = [], []
        a, r = mm3("w3", 0)
        us, it = one(mmU(lambda n: "U%d" % n, 0, 0)), one(mmI(lambda n: "I%d" % n, 0, 0))
        w4 = mm4("w4", s - 2, 0)
        q = quarter(w4[LP[1] - 1])
        _mix(seq, _flat(mm4("w4c", s - 3, 0)[LP[2]:]) + a,
             [us[0], us[1], us[2], it[0] + us[3], it[1] + us[4], it[2] + start(next_kv(nxt)), it[3], it[4], r],
             LP[3], LP[0])
        _mix(seq, _flat(w4[:LP[1]]), [q])
        w1 = _flat(mm1("w1", 2, 0))
        seq += w1[:8] + start(next_q(nxt)) + w1[8:] + run(cat(shift(1, 0, ((T - 16, 16),))))
        seq += _flat(w4[LP[1]:LP[2]] + mm2("w2", 0, 1, 0))
        assert _phase(seq) == 0
        kvs, macs = kv(0, 0), mac(1, 0, 0, part=True)
        for t in range(NT):
            grp.append(Group("kv%d" % t, kvs[t], 50, ["start"], ["U%d" % t], 300))
            grp.append(Group("mac%d" % t, macs[t], 28, ["U%d" % t], ["I%d" % t], 300, 150))
        iall = ["I%d" % t for t in range(NT)]
        grp.append(Group("ln2", ln2(0, 0), 60, ["start"], ["w3"], 450))
        grp.append(Group("resid", resid(1, 0, True), 40, ["w4c"], ["w4", "I4"], 100))
        grp.append(Group("front", front(0, 0), 80, iall, ["w1"], 450))
        grp.append(Group("spread", spread(), 30, iall, ["end"], 100))
        grp.append(Group("shift", shift_early(), 12, ["start"], ["w1"], 200))
        _emit(seq, grp, zero, wait)
        out_b(s - 3).wait()
        out_a(s - 2).wait()
        return carry

    lax.fori_loop(NC, NB, step, 0)

    seq, grp = [], []
    seq += _flat(mm4("w4_5", NB - 3, 0)[LP[2]:])
    a, r = mm3("w3_6", 0)
    _mix(seq, a, [r])
    seq += _flat(mm2("w2_7", 0, 0, 1) + mm4("w4_6", NB - 2, 0, 1, 1, 0))
    a, r = mm3("w3_7", 1)
    _mix(seq, a, [r])
    seq += _flat(mm4("w4_7", NB - 1, 1, 2, 0, 1))
    assert _phase(seq) == 0
    grp.append(Group("ln2_6", ln2(0, 0), 60, ["start"], ["w3_6"], 450))
    grp.append(Group("shift7", cat(shift(2, 0)), 14, ["start"], ["w2_7"], 200))
    grp.append(Group("ln2_7", ln2(1, 1), 60, ["w2_7"], ["w3_7"], 450))
    _emit(seq, grp, zero, wait)
    with scope("wait_out"):
        for c in next_kv(NB - 1) + next_q(NB - 1) + [out_b(NB - 3)] + last:
            c.wait()


@jax.jit
def pallas_adaLN_cond__ssm_conv_h3__mixer_s_mlp__prompt_kernel(A_q, A_k, A_v, A_shift_k, A_ssm_k, A_ssm_D, B_x, B_w1, B_w2, B_w3, B_w4, c, w_mod):
    any_ = pl.BlockSpec(memory_space=pl.ANY)
    V = pltpu.VMEM
    out = pl.pallas_call(
        kernel,
        in_specs=[any_] * 12,
        out_specs=any_,
        out_shape=jax.ShapeDtypeStruct((S, D), BF16),
        scratch_shapes=[
            [V((NT, H + 8, 128), U32)] * NC, [V((NT, H + 8, 128), U32)] * NC, [V((NT, H + 8, 128), U32)] * NC,
            [V((64, S), U32)] * NT,
            V((D // 2, D), U32), V((D // 2, D), U32), V((F // 2, D), U32), V((F // 2, D), U32),
            [V((D // 2, 3 * D), U32), V((D // 2, 2 * D), U32), V((D // 2, D), U32)], V((4 * T, D), BF16),
            V((4, D), BF16), V((D,), BF16), V((1, D), BF16), V((8, 128), I32), pltpu.SMEM((8, 128), I32),
            V((5, 8, D), F32), V((6, 8, D), F32), V((T // 2, 4 * H), U32), V((GR // 2, 2 * T), U32),
            V((NB, 3 * T + 8, D), F32), V((NC, 3 * T + 8, D), F32), V((NB - NC, 2 * T + 8, D), F32), V((2 * T, D), F32),
            V((2, T // 2, D), U32), V((NC, T, D), U32), V((NT, NC * T + 8, 128), F32),
            V((3 * T, D), F32), V((3 * T, D), F32), V((2 * T, D), F32), V((T, D), F32),
            V((3 * T // 2, D), U32), V((T, D), U32), V((T, D), U32), V((NT, NC * T + 24, 128), F32),
            V((T, (FT + 1) * 128), U32),
            pltpu.SemaphoreType.DMA((11,)), pltpu.SemaphoreType.DMA((1,)), pltpu.SemaphoreType.DMA((3,)),
        ],
        compiler_params=pltpu.CompilerParams(vmem_limit_bytes=110 << 20, disable_semaphore_checks=True,
                                             disable_bounds_checks=True),
        name="fused",
    )(A_q[0], A_k[0], A_v[0], A_shift_k.T, A_ssm_k, A_ssm_D, B_w1, B_w2, B_w3.T, B_w4, c, w_mod)
    return out[None]
```

```python
import contextlib
import heapq
import numpy as np
import jax
import jax.numpy as jnp
from jax import lax
from jax.experimental import pallas as pl
from jax.experimental.pallas import tpu as pltpu

S, D, F = 2048, 640, 1728
T = 256
H = T // 2
NB = S // T
NT = D // 128
FT = (F + 127) // 128
EPS = 1e-5
F32, BF16, U32, I32 = jnp.float32, jnp.bfloat16, jnp.uint32, jnp.int32
G_C1 = 0.044715 * float(np.sqrt(2.0 / np.pi))
G_C2 = float(np.sqrt(2.0 / np.pi))
G_A = G_C1 ** (1.0 / 3.0)
G_B = G_C2 / G_A
G_POST = 0.5 / G_A
RG = 16
GR = 80
NC = 3
VERBOSE = False
SCOPES = False
SLOT = 32
LP = (0.8, 4, 6, 0.15, 72)


def _dft(shape, f_axis, tau, scale=1.0):
    r = lax.broadcasted_iota(I32, shape, f_axis)
    l = lax.broadcasted_iota(I32, shape, 1 - f_axis)
    f = r & 127
    odd = ((f & 63) << 2) | ((f >> 6) << 1) | 1
    p = odd * tau(l) + ((r >> 7) << 8)
    a = ((p + 512) & 1023) - 512
    u = (256 - jnp.abs(a)).astype(F32) * (np.pi / 512.0)
    u2 = u * u
    c = [scale, -scale / 6.0, scale / 120.0, -scale / 5040.0, scale / 362880.0, -scale / 39916800.0]
    poly = c[5]
    for ci in c[4::-1]:
        poly = poly * u2 + ci
    return (u * poly).astype(BF16)


def _ln(x, scale=1.0):
    m = jnp.sum(x, axis=-1, keepdims=True) * (1.0 / D)
    xc = x - m
    s2 = 1.0 / (scale * scale)
    v = jnp.sum(xc * xc, axis=-1, keepdims=True) * (s2 / D) + EPS * s2
    r = jnp.exp2(jnp.log(v) * float(-0.5 / np.log(2.0)))
    return xc * r


def _gelu2(x):
    u = x * (x * x + G_B)
    return x * (1.0 + jnp.tanh(u))


def _lo(w):
    return pltpu.bitcast(w << 16, F32)


def _hi(w):
    return pltpu.bitcast(w & jnp.uint32(0xFFFF0000), F32)


def _tie(x, a):
    if a is None:
        return x
    w = pltpu.bitcast(x[:, :128], U32)
    k = w.shape[0] // 8
    w = w | (a if k == 1 else jnp.concatenate([a] * k, axis=0))
    w = pltpu.bitcast(w, x.dtype)
    return w if x.shape[1] == 128 else jnp.concatenate([w, x[:, 128:]], axis=1)


def C(i, lim=F):
    return slice(i * 128, min((i + 1) * 128, lim))


class Unit:
    def __init__(self, name, tiles, epi, rows, cost, nt=False, full=True, acc=False):
        self.acc, self.res = acc, []
        self.name, self.tiles, self.epi, self.rows, self.cost, self.nt, self.full = name, tiles, epi, rows, cost, nt, full


class Group:
    def __init__(self, name, fns, cost, rel, dead, lat, rlat=200):
        self.name, self.fns, self.cost, self.rel, self.dead, self.lat, self.rlat = name, fns, cost, rel, dead, lat, rlat


def _plan(seq, groups):
    busy, n = [0] * 4, 0
    start, end, tiles, bars = {}, {}, [], []
    for it in seq:
        if isinstance(it[0], Unit):
            u = it[0]
            m = n % 4
            n += 1
            t0, t1 = busy[m], busy[m] + max(u.rows, 32)
            busy[m] = t1
            tiles.append((t0, t1, u.cost / len(u.tiles)))
            start.setdefault(u.name, t0)
            end[u.name] = max(end.get(u.name, 0), t1)
        elif it[0] == "wait":
            t = max(busy)
            busy, n = [t] * 4, 0
            start[it[1]] = end[it[1]] = t
            bars.append(t)
    total = max(busy)
    start["end"] = end["end"] = total
    start["start"] = end["start"] = 0
    ns = total // SLOT + 2
    load = np.zeros(ns)
    for t0, t1, c in tiles:
        a, b = t0 // SLOT, max(t1 // SLOT, t0 // SLOT + 1)
        load[a:b] += c / (b - a)
    win = []
    for g in groups:
        r = max(end[x] + (0 if start[x] == end[x] else g.rlat) for x in g.rel)
        d = min(start[x] for x in g.dead) - g.lat
        ok = np.zeros(ns, bool)
        ok[r // SLOT:max(d // SLOT, r // SLOT + 1)] = True
        for b in bars:
            if r < b <= d:
                ok[max((b - g.lat) // SLOT, 0):b // SLOT] = False
        win.append(np.nonzero(ok)[0])
    alloc = [np.zeros(len(w)) for w in win]
    for _ in range(60):
        for i, g in enumerate(groups):
            w = win[i]
            load[w] -= alloc[i]
            base = load[w]
            vol = g.cost * len(g.fns)
            lo, hi = base.min(), base.max() + vol
            for _ in range(50):
                mid = 0.5 * (lo + hi)
                if np.maximum(mid - base, 0).sum() > vol:
                    hi = mid
                else:
                    lo = mid
            alloc[i] = np.maximum(hi - base, 0)
            load[w] += alloc[i]
    times = []
    for i, g in enumerate(groups):
        cum = np.cumsum(alloc[i])
        ts = []
        for k in range(len(g.fns)):
            x = (k + 0.5) * cum[-1] / len(g.fns)
            j = int(np.searchsorted(cum, x))
            prev = cum[j - 1] if j else 0.0
            ts.append(win[i][j] * SLOT + SLOT * (x - prev) / max(alloc[i][j], 1e-9))
        times.append(ts)
        if VERBOSE:
            print("%8s window %6d..%6d used %6d..%6d" % (g.name, win[i][0] * SLOT, win[i][-1] * SLOT, ts[0], ts[-1]))
    if VERBOSE:
        k = 2048 // SLOT
        print("total", total, "load/cycle:", " ".join("%.1f" % (load[i:i + k].mean() / SLOT) for i in range(0, ns, k)))
    return times


def _emit(seq, groups, zero, wait):
    times = _plan(seq, groups)
    left = {"start": 0}
    for it in seq:
        nm = it[0].name if isinstance(it[0], Unit) else it[1]
        left[nm] = left.get(nm, 0) + 1
    heap, pend, todo, cnt = [], {}, list(range(len(groups))), 0
    busy, n = [0] * 4, 0

    def release():
        nonlocal cnt
        for i in list(todo):
            g = groups[i]
            if all(left[x] == 0 for x in g.rel):
                todo.remove(i)
                pend[i] = len(g.fns)
                for t, fn in zip(times[i], g.fns):
                    heapq.heappush(heap, (t, cnt, i, fn))
                    cnt += 1

    def force(name):
        nonlocal heap
        for i, g in enumerate(groups):
            if name in g.dead:
                assert i not in todo, (g.name, name)
                if pend[i]:
                    if VERBOSE:
                        print("forcing", g.name, pend[i], "before", name)
                    for it in sorted(x for x in heap if x[2] == i):
                        it[3](None)
                    heap = [x for x in heap if x[2] != i]
                    heapq.heapify(heap)
                    pend[i] = 0

    release()
    for it in seq:
        if isinstance(it[0], Unit):
            u, k = it
            force(u.name)
            lhs, rhs = u.tiles[k]()
            dn = (((1,), (1 if u.nt else 0,)), ((), ()))
            p = lax.dot_general(lhs, rhs, dn, preferred_element_type=F32)
            u.res = [p + u.res[0]] if (u.acc and u.res) else u.res + [p]
            m = n % 4
            n += 1
            t0 = busy[m]
            busy[m] = t0 + max(u.rows, 32)
            while u.full and heap and heap[0][0] < t0 + u.rows:
                t, _, i, fn = heapq.heappop(heap)
                pend[i] -= 1
                r = min(max(int(t - t0), 0), u.rows - 1) // 8 * 8
                fn(pltpu.bitcast(p[r:r + 8], U32) & zero)
            if k == len(u.tiles) - 1:
                u.epi(u.res)
            left[u.name] -= 1
        elif it[0] == "wait":
            force(it[1])
            wait(it[1])
            busy, n = [max(busy)] * 4, 0
            left[it[1]] -= 1
        else:
            it[2]()
            left[it[1]] -= 1
        release()
    force("end")
    assert not heap and not todo


def _sum(ps):
    acc = ps[0]
    for p in ps[1:]:
        acc = acc + p
    return acc


def _flat(us):
    return [(u, i) for u in us for i in range(len(u.tiles))]


def _phase(seq):
    n = 0
    for it in seq:
        n = n + 1 if isinstance(it[0], Unit) else (0 if it[0] in ("wait", "sync") else n)
    return n % 4


def _mix(seq, a, b, lo=0.0, hi=1.0):
    n, k = _phase(seq), 0
    for i, t in enumerate(a):
        if k < len(b) and n % 4 == 0 and t[1] != 1 and i >= len(a) * (lo + (hi - lo) * k / len(b)):
            seq.extend(b[k])
            k += 1
        seq.append(t)
        n += 1
    assert k == len(b)


def _wait(seq, name, head=()):
    r = _phase(seq)
    assert all(isinstance(it[0], Unit) for it in seq[len(seq) - r:])
    seq[len(seq) - r:len(seq) - r] = [("wait", name)] + list(head)


def kernel(q_hbm, k_hbm, v_hbm, sh_hbm, ssm_hbm, sd_hbm, w1_hbm, w2_hbm, w3_hbm, w4_hbm, c_hbm, wm_hbm,
           o_hbm,
           q_n, k_n, v_n, ssm_w, w1_w, w2_w, w3_w, w4_w, wm_w, o_v,
           sh_v, sd_v, c_v, zsrc, z_s, taps, mod_v, tf_w, tg_w,
           kf, uf, acc, zraw, kv_w, zz_w, y_v, x_v, hb_v, x1_v, r_v, n1_w, n2_w, g_w, h1_v, a_w,
           sem, sem_b, sem_o):
    bf = lambda r: r.bitcast(BF16)
    w1_v, w2_v, w3_v, w4_v = bf(w1_w), bf(w2_w), bf(w3_w), bf(w4_w)
    wm_v = {0: bf(wm_w[0]), 3: bf(wm_w[1]), 5: bf(wm_w[2])}
    tf_v, tg_v, n1_v, n2_v, g_v = bf(tf_w), bf(tg_w), bf(n1_w), bf(n2_w), bf(g_w)
    a_v, kv_v, zz_v = bf(a_w), bf(kv_w), bf(zz_w)
    cp = pltpu.make_async_copy
    scope = lambda nm: jax.named_scope(nm) if SCOPES else contextlib.nullcontext()

    def base(j, n):
        return j * n if isinstance(j, int) else pl.multiple_of(j * n, n)

    def rows(j, n=1, size=T):
        return pl.ds(base(j, size), n * size)

    def view(ref, j, size=T):
        return ref.at[rows(j, 1, size)]

    dmas = {}

    def group(name, *mks):
        sm = sem.at[len(dmas)]
        dmas[name] = [c for mk in mks for c in mk(sm)]

    def ssm_in(t):
        return lambda sm: [cp(ssm_hbm.at[C(t)], bf(ssm_w[t]), sm)]

    def cols(src, start, n, dst, row=0):
        return lambda sm: [cp(src.at[pl.ds(start, n), C(t)], bf(dst).at[t, pl.ds(row, n)], sm) for t in range(NT)]

    def kv_in(s, sl):
        if isinstance(s, int):
            kk = cols(k_hbm, s * T - 16, T + 16, k_n[sl]) if s else cols(k_hbm, 0, T, k_n[sl], 16)
        else:
            kk = cols(k_hbm, pl.multiple_of(s * T - 16, 16), T + 16, k_n[sl])
        return lambda sm: kk(sm) + cols(v_hbm, base(s, T), T, v_n[sl])(sm)

    def q_in(s, sl):
        return cols(q_hbm, base(s, T), T, q_n[sl])

    def wm_in(a, b):
        return lambda sm: [cp(wm_hbm.at[:, a * D:b * D], wm_v[a], sm)]

    def whole(src, dst):
        return lambda sm: [cp(src, dst, sm)]

    next_kv = lambda s: kv_in(s, 0)(sem_b.at[0])
    next_q = lambda s: q_in(s, 0)(sem_b.at[0])

    zsrc[...] = jnp.zeros((8, 128), I32)
    k_n[0][:, 0:8, :] = jnp.zeros((NT, 8, 128), U32)
    group("small", lambda sm: [cp(zsrc, z_s, sm), cp(sh_hbm, sh_v, sm), cp(sd_hbm, sd_v, sm), cp(c_hbm, c_v, sm)])
    for s in range(NC):
        group("c%d" % s, ssm_in(s), kv_in(s, s))
    group("c3", ssm_in(3), ssm_in(4))
    group("wma", wm_in(0, 3), q_in(0, 0), q_in(1, 1))
    group("wmb", wm_in(3, 5))
    group("w1", whole(w1_hbm, w1_v))
    group("w2", q_in(2, 2), whole(w2_hbm, w2_v))
    group("w3", whole(w3_hbm, w3_v))
    group("w4", whole(w4_hbm, w4_v), wm_in(5, 6))
    for g in dmas.values():
        for c in g:
            c.start()

    def wait(name):
        with scope("wait_" + name):
            for c in dmas[name]:
                c.wait()

    tau_b = lambda l: H + ((l + (H - 1)) & (H - 1))
    tf_v[:, C(0)] = _dft((T, H), 0, lambda l: jnp.where((l & 1) == 0, l, tau_b(l)), 1.0 / T)
    tf_v[:, C(1)] = _dft((T, H), 0, lambda l: jnp.where((l & 1) == 1, l, tau_b(l)), 1.0 / T)
    tf_v[:, C(2)] = _dft((T, H), 0, lambda l: 2 * l - H)
    tf_v[:, C(3)] = _dft((T, H), 0, lambda l: 2 * l + 1 - H)
    sin0 = lax.broadcasted_iota(I32, (GR, T), 1) >= H
    tg_v[:, 0:T] = _dft((GR, T), 1, lambda l: jnp.where(sin0 & (l == 0), H, 2 * l))
    tg_v[:, T:2 * T] = _dft((GR, T), 1, lambda l: 2 * l + 1)
    h1_v[:, 0:8, :] = jnp.zeros((NT, 8, 128), F32)
    h1_v[:, 8 + NC * T:16 + NC * T, :] = jnp.zeros((NT, 8, 128), F32)

    wait("small")
    z = jnp.clip(z_s[0, 0], 0, 1)
    zero = jnp.full((8, 128), z, I32).astype(U32)
    z8 = pl.multiple_of(z * 8, 8)
    for r in (x_v, hb_v, x1_v, r_v, zraw, n1_w, n2_w, g_w, a_w, kv_w, zz_w):
        r[pl.ds(z8, 8), 0:128] = jnp.zeros((8, 128), r.dtype)
    for r in (kf, uf, acc, taps, mod_v):
        r[z, 0:8, 0:128] = jnp.zeros((8, 128), r.dtype)
    for r in (tf_w, tg_w):
        r[pl.ds(z8, 8), 0:128] = r[0:8, 0:128]
    sh = sh_v[...].astype(F32)
    for i in range(4):
        taps[i] = jnp.broadcast_to(sh[i:i + 1], (8, D))
    taps[4] = jnp.broadcast_to(sd_v[...].astype(F32).reshape(1, D) * (1.0 / T), (8, D))
    cf = c_v[...].astype(F32)
    silu_c = jnp.broadcast_to((cf / (1.0 + jnp.exp(-cf))).astype(BF16), (16, D))

    def mmK(n):
        def unit(m):
            st = []

            def rhs(i):
                if not st:
                    ev = (lax.broadcasted_iota(I32, (64, 128), 1) & 1) == 0
                    a = ssm_w[n][:, m * T:m * T + H]
                    b = pltpu.roll(ssm_w[n][:, m * T + H:(m + 1) * T], 1, 1)
                    st.extend([pltpu.bitcast(jnp.where(ev, a, b), BF16), pltpu.bitcast(jnp.where(ev, b, a), BF16)])
                return st[i]

            def epi(p):
                er, ei, or_, oi = p
                if m == 0:
                    er = er + taps[4, 0:1, C(n)]
                for h, (cr, ci) in enumerate(((er + or_, ei + oi), (er - or_, ei - oi))):
                    B = h * 3 * H
                    kf[m, B:B + H, C(n)] = cr
                    kf[m, B + H:B + 2 * H, C(n)] = ci - cr
                    kf[m, B + 2 * H:B + 3 * H, C(n)] = ci + cr
            return Unit("K%d" % n, [(lambda i=i, r=r: (tf_v[r:r + H, C(i)], rhs(i))) for i in range(2) for r in (0, H)],
                        epi, H, 170, nt=True)
        return [unit(m) for m in range(NB)]

    def kv(s, sl):
        def mk(t, w):
            def fn(a):
                ld = lambda o, n: k_n[s][t, pl.ds(8 + w + o, n), :]
                c0 = jnp.concatenate([_tie(ld(0, 8), a), ld(8, 8)], axis=0).reshape(2, 8, 128)
                c1, c2 = ld(-1, 16).reshape(2, 8, 128), ld(-2, 16).reshape(2, 8, 128)
                s0, s1, s2, s3 = (taps[i, :, C(t)] for i in range(4))
                ke, ko, ke1, ko1, ko2 = _lo(c0), _hi(c0), _lo(c1), _hi(c1), _hi(c2)
                wv = v_n[s][t, w:w + 16, :].reshape(2, 8, 128)
                kve = ((s0 * ke + s1 * ko1) + (s2 * ke1 + s3 * ko2)) * _lo(wv)
                kvo = ((s0 * ko + s1 * ke) + (s2 * ko1 + s3 * ke1)) * _hi(wv)
                kv_v[pl.ds(sl * T + w, 16), C(t)] = kve.reshape(16, 128).astype(BF16)
                kv_v[pl.ds(sl * T + H + w, 16), C(t)] = kvo.reshape(16, 128).astype(BF16)
            return fn
        return [[mk(t, w) for w in range(0, H, 16)] for t in range(NT)]

    def mmU(name, sl, us):
        def unit(n):
            def epi(p):
                er, ei, or_, oi = p
                for h, (cr, ci) in enumerate(((er + or_, ei + oi), (er - or_, ei - oi))):
                    B = h * 3 * H
                    uf[us, B:B + H, C(n)] = cr + ci
                    uf[us, B + H:B + 2 * H, C(n)] = cr
                    uf[us, B + 2 * H:B + 3 * H, C(n)] = ci
            return Unit(name(n), [(lambda i=i, r=r: (tf_v[r:r + H, C(2 + i)], kv_v[pl.ds(sl * T + i * H, H), C(n)]))
                                  for i in range(2) for r in (0, H)], epi, H, 120)
        return [unit(n) for n in range(NT)]

    def cmul(m0, u0, n, h, row, L, a):
        t = []
        for i in range(3):
            Rw = slice((3 * h + i) * H + row, (3 * h + i) * H + row + 8)
            kk = kf[m0:m0 + n, Rw, L]
            if i == 0 and a is not None:
                k0 = _tie(kk[0], a)[None]
                kk = k0 if n == 1 else jnp.concatenate([k0, kk[1:]], axis=0)
            t.append(jnp.sum(kk * uf[u0:u0 + n, Rw, L], axis=0))
        return t[0] - t[2], t[0] + t[1]

    def AR(h, q, row):
        return slice((2 * h + q) * H + row, (2 * h + q) * H + row + 8)

    def mac(n, u0, sl, first=False, part=False):
        def mk(t, rc):
            st, fin = [], []

            def piece(i):
                def fn(a):
                    h, row = i & 1, rc + (i >> 1) * 8
                    zr, zi = cmul(0, u0, n, h, row, C(t), a)
                    if part:
                        zr, zi = zr + acc[0, AR(h, 0, row), C(t)], zi + acc[0, AR(h, 1, row), C(t)]
                    st.append((zr, zi))
                    if h:
                        (pr, pi), (mr, mi) = st[-2:]
                        z = [pr + mr, pi + mi, pr - mr, pi - mi]
                        Rw = lambda q: slice(q * H + row, q * H + row + 8)
                        pv = None if first else [zraw[Rw(q ^ 1), C(t)] for q in range(4)]
                        for q in range(4):
                            zraw[Rw(q), C(t)] = z[q]
                        if not first:
                            z = [z[q] + pv[q] if (q & 1) == (rc < 64) else z[q] - pv[q] for q in range(4)]
                        fin.append(z)
                    if i == 3:
                        for q in range(4):
                            zz_v[pl.ds(sl * 2 * T + q * H + rc, 16), C(t)] = jnp.concatenate(
                                [fin[0][q], fin[1][q]], axis=0).astype(BF16)
                return fn
            if not part:
                return [piece(i) for i in range(4)]
            both = lambda f, g: (lambda a: (f(a), g(None)))
            return [both(piece(0), piece(1)), both(piece(2), piece(3))]
        return [[fn for rc in range(0, H, 16) for fn in mk(t, rc)] for t in range(NT)]

    def pos():
        return [(t, h, row) for t in range(NT) for row in range(0, H, 8) for h in range(2)]

    def ahead(i):
        def mk(t, h, row):
            def fn(a):
                zr, zi = cmul(i + 1, 0, NC, h, row, C(t), a)
                acc[i, AR(h, 0, row), C(t)] = zr
                acc[i, AR(h, 1, row), C(t)] = zi
            return fn
        return [mk(*p) for p in pos()]

    def spread():
        n = NB - NC - 1

        def mk(t, h, row):
            def fn(a):
                p = []
                for i in range(3):
                    Rw = slice((3 * h + i) * H + row, (3 * h + i) * H + row + 8)
                    u = uf[0, Rw, C(t)]
                    p.append(kf[1:1 + n, Rw, C(t)] * (_tie(u, a) if i == 0 else u)[None])
                acc[0:n, AR(h, 0, row), C(t)] = acc[1:1 + n, AR(h, 0, row), C(t)] + (p[0] - p[2])
                acc[0:n, AR(h, 1, row), C(t)] = acc[1:1 + n, AR(h, 1, row), C(t)] + (p[0] + p[1])
            return fn
        return [mk(*p) for p in pos()]

    def mmI(name, sl, ys):
        def unit(n):
            def epi(p):
                ce, se, co, so = p
                sub = lax.broadcasted_iota(I32, (8, 128), 0)
                c0 = ys * T + H
                y_v[n, ys * T:ys * T + 1, :] = (ce[64:72] - se[0:8])[0:1]
                se = jnp.concatenate([jnp.where(sub == 0, 0.0, se[0:8]), se[8:]], axis=0)
                for d, cc, ss in ((0, ce[0:64], se), (1, co, so)):
                    y_v[n, pl.ds(c0 + d, 64, stride=2), :] = cc + ss
                    lo = cc - ss
                    for i in range(0, 64, 8):
                        y_v[n, pl.ds(c0 - d - 2 * i - 14, 8, stride=2), :] = jnp.take_along_axis(
                            lo[i:i + 8], 7 - sub, axis=0)
            return Unit(name(n), [(lambda i=i: (tg_v[0:(GR if i == 0 else 64), C(i)], zz_v[pl.ds(sl * 2 * T + i * H, H), C(n)]))
                                  for i in range(4)], epi, 64, 52)
        return [unit(n) for n in range(NT)]

    def mod(name, a, b):
        def unit(n):
            def epi(p):
                v = [_sum(p[i * NT:(i + 1) * NT])[0:8] for i in range(b - a)]
                if a == 0:
                    mod_v[0, :, C(n)] = v[0] * v[2]
                    mod_v[1, :, C(n)] = (v[1] + 1.0) * v[2]
                elif a == 3:
                    mod_v[3, :, C(n)] = v[0]
                    mod_v[4, :, C(n)] = v[1] + 1.0
                else:
                    mod_v[5, :, C(n)] = v[0]
                    mod_v[2, :, C(n)] = v[0] * G_POST
            return Unit(name, [(lambda i=i, k=k: (silu_c[:, C(k)], wm_v[a][C(k), (i - a) * D + n * 128:(i - a) * D + (n + 1) * 128]))
                               for i in range(a, b) for k in range(NT)], epi, 16, 10, full=False, acc=b - a == 1)
        return [unit(n) for n in range(NT)]

    GS = range(0, T, RG)
    HS = (slice(0, 128), slice(128, 256))

    def tasks(f):
        return [(lambda a, r=r: f(slice(r, r + RG), a)) for r in GS]

    def load_y(sl, R):
        return jnp.concatenate([y_v[t, sl * T + R.start:sl * T + R.stop, :] for t in range(NT)],
                               axis=1).reshape(2, 8, D)

    def front(sl, xs, early=False):
        xx, hh, nn = view(x_v, xs), view(hb_v, xs), view(n1_v, sl)

        def fa(R, a):
            q = [q_n[sl][t, R.start // 2:R.stop // 2, :] for t in range(NT)]
            q = jnp.concatenate([_tie(q[0], a)] + q[1:], axis=1)
            q = pltpu.bitcast(q, BF16).astype(F32).reshape(2, 8, D)
            x = (q + (_ln(q) * mod_v[1] + mod_v[0]) * load_y(sl, R)).reshape(RG, D)
            xx[R, :] = x
            if early:
                hh[R, :] = _ln(x)

        def fb(R, a):
            hh[R, :] = (_ln(_tie(xx[R, :], a).reshape(2, 8, D)) * mod_v[4] + mod_v[3]).reshape(RG, D)

        def fc(R, a):
            hb = _tie(hh[R, :], a)
            if early:
                hb = (hb.reshape(2, 8, D) * mod_v[4] + mod_v[3]).reshape(RG, D)
                hh[R, :] = hb
            nn[R, :] = _ln(hb, G_A).astype(BF16)
        return (tasks(fa), tasks(fc)) if early else tasks(fa) + tasks(fb) + tasks(fc)

    def shift(hs, sl, pieces=((0, 64), (64, 64), (128, 64), (192, 64))):
        gg = view(g_v, sl)

        def mk(t, r, n):
            def fn(a):
                lane = lax.broadcasted_iota(I32, (n, 128), 1)
                ld = lambda d: h1_v[t, pl.ds(hs * T + 8 + r + d, n), :]
                if t == 0:
                    g = ld(-1)
                elif t == 1:
                    g = jnp.where(lane < 32, ld(-1), ld(1))
                elif t == 2:
                    g = jnp.where(lane < 64, ld(1), ld(-2))
                elif t == 3:
                    g = jnp.where(lane < 96, ld(-2), ld(2))
                else:
                    g = ld(2)
                if a is not None:
                    g = jnp.concatenate([_tie(g[i:i + 8], a) if i % 16 == 0 else g[i:i + 8]
                                         for i in range(0, n, 8)], axis=0)
                gg[r:r + n, C(t)] = g.astype(BF16)
            return fn
        return [[mk(t, r, n) for r, n in pieces] for t in range(NT)]

    def shift_early():
        def keep(t):
            def fn(a):
                h1_v[t, 2 * T - 16:2 * T + 8, :] = h1_v[t, 3 * T - 16:3 * T + 8, :]
            return fn
        sh = shift(2, 0, ((0, 64), (64, 64), (128, 64), (192, 48)))
        return [fn for t in range(NT) for fn in sh[t] + [keep(t)]]

    def ln2(xs, sl):
        xx, nn = view(x1_v, xs), view(n2_v, sl)

        def f(R, a):
            nn[R, :] = _ln(_tie(xx[R, :], a), G_A).astype(BF16)
        return tasks(f)

    def resid(xs, x1s, rotate=False):
        xx, x1 = view(x_v, xs), view(x1_v, x1s)

        def f(R, a):
            gb = mod_v[5] if a is None else pltpu.bitcast(
                pltpu.bitcast(mod_v[5], U32) | jnp.concatenate([a] * NT, axis=1), F32)
            r_v[R, :] = xx[R, :] + (x1[R, :].reshape(2, 8, D) * gb).reshape(RG, D)
            if rotate:
                xx[R, :] = x_v[R, :]
                view(hb_v, 1)[R, :] = hb_v[R, :]
        return tasks(f)

    def mm1(name, hs, sl):
        nn = view(n1_v, sl)

        def unit(n, R):
            def epi(p):
                h1_v[n, pl.ds(hs * T + 8 + R.start, 128), :] = _gelu2(p[0])
            return Unit(name, [(lambda k=k: (nn[R, C(k)], w1_v[C(k), C(n)])) for k in range(NT)],
                        epi, 128, 144, acc=True)
        return [unit(n, R) for n in range(NT) for R in HS]

    def mm2(name, sl, xs, x1s):
        gg, hh, x1 = view(g_v, sl), view(hb_v, xs), view(x1_v, x1s)

        def unit(n, R):
            def epi(p):
                x1[R, C(n)] = hh[R, C(n)] + p[0] * G_POST
            return Unit(name, [(lambda k=k: (gg[R, C(k)], w2_v[C(k), C(n)])) for k in range(NT)],
                        epi, 128, 96, acc=True)
        return [unit(n, R) for n in range(NT) for R in HS]

    def mm3(name, sl):
        nn, aa = view(n2_v, sl), view(a_v, sl)

        def unit(n, R):
            def epi(p):
                aa[R, C(n)] = _gelu2(p[0]).astype(BF16)
            return Unit(name, [(lambda k=k: (nn[R, C(k)], w3_v[C(n), C(k)])) for k in range(NT)],
                        epi, 128, 160, nt=True, acc=True)
        main = [unit(n, R) for n in range(FT - 1) for R in HS]
        F0, part = (FT - 1) * 128, []
        main[-1].tiles.pop(0)

        def epi(p):
            for i, R in enumerate(HS):
                aa[R, F0:F] = _gelu2(part[i] + p[i]).T.astype(BF16)
            main[-1].res = [jnp.concatenate(p[2:], axis=0)]
        rem = [Unit(name, [(lambda k=k, R=R: (w3_v[F0:F, C(k)], nn[R, C(k)])) for k in range(NT - 1)],
                    lambda p: part.append(p[0]), 64, 24, nt=True, acc=True) for R in HS]
        rem.append(Unit(name, [(lambda R=R: (w3_v[F0:F, C(NT - 1)], nn[R, C(NT - 1)])) for R in HS]
                        + [(lambda r=r: (nn[r:r + 64, C(0)], w3_v[C(FT - 2), C(0)])) for r in (128, 192)],
                        epi, 64, 120, nt=True))
        return _flat(main), _flat(rem)

    NA = LP[2] // 2 * 128

    def cp_out(j, osl, L, sm, R=slice(0, T)):
        return cp(o_v.at[pl.ds(osl * T + R.start, R.stop - R.start), L],
                  o_hbm.at[pl.ds(base(j, T) + R.start, R.stop - R.start), L], sem_o.at[sm])

    out_a = lambda j: cp_out(j, 0, slice(0, NA), 0)
    out_b = lambda j: cp_out(j, 0, slice(NA, D), 1)
    last = []

    def mm4(name, j, sl, osl=0, xs=None, x1s=None):
        aa, oo = view(a_v, sl), view(o_v, osl)

        def unit(n, R):
            def epi(p):
                if xs is None:
                    oo[R, C(n)] = (r_v[R, C(n)] + mod_v[2, 0:1, C(n)] * p[0]).astype(BF16)
                else:
                    oo[R, C(n)] = (view(x_v, xs)[R, C(n)] + mod_v[5, 0:1, C(n)]
                                   * (view(x1_v, x1s)[R, C(n)] + p[0] * G_POST)).astype(BF16)
                if osl == 2:
                    last.append(cp_out(j, osl, C(n), 2, R))
                    last[-1].start()
                elif R.stop == T and (osl, (n + 1) * 128) in ((1, D), (3, NA)):
                    last.append(cp_out(j, osl, slice(0, (n + 1) * 128), 2))
                    last[-1].start()
                elif R.stop == T and osl == 0 and (n + 1) * 128 in (NA, D):
                    (out_a if (n + 1) * 128 == NA else out_b)(j).start()
            return Unit(name, [(lambda k=k: (aa[R, C(k)], w4_v[C(k), C(n)])) for k in range(FT)],
                        epi, 128, 16 * (16 if xs is None else 18), acc=True)
        return [unit(n, R) for n in range(NT) for R in HS]

    def quarter(u):
        mk = u.tiles.pop(0)
        st = []

        def piece(i):
            if not st:
                st.extend(mk())
            return st[0][32 * i:32 * i + 32], st[1]

        def epi(p):
            u.res = [jnp.concatenate(p, axis=0)]
        return _flat([Unit(u.name, [(lambda i=i: piece(i)) for i in range(4)], epi, 32, 0, nt=u.nt)])

    W = lambda nm: [("wait", nm)]
    run = lambda fns: [("run", "run", lambda: [fn(None) for fn in fns])]
    one = lambda us: [_flat([u]) for u in us]
    cat = lambda ls: [x for l in ls for x in l]
    nm = lambda x: (lambda n: x)

    seq, grp = [], []
    for s in range(NC):
        seq += W("c%d" % s) + _flat(mmK(s) + mmU(nm("U%d" % s), s % 2, NC - 1 - s))
        grp.append(Group("kv%d" % s, cat(kv(s, s % 2)), 50, ["c%d" % s], ["U%d" % s], 100))
    inv = [mmI(lambda n: "I%d" % n, s, s) for s in range(NC)]
    seq += W("c3") + _flat(mmK(3) + mmK(4) + [inv[s][t] for t in range(NT) for s in range(NC)])
    macs = [mac(s + 1, NC - 1 - s, s, first=s == 0) for s in range(NC)]
    grp.append(Group("mac00", macs[0][0], 12, ["c1"], ["c2"], 0))
    grp.append(Group("mac01", macs[1][0] + macs[0][1] + macs[1][1], 16, ["c2"], ["c3"], 0))
    for t in range(NT):
        grp.append(Group("mac%d" % t, cat(macs[s][t] for s in range(2 if t < 2 else 0, NC)), 24 if t < 2 else 18,
                         ["c3", "K%d" % t], ["I%d" % t], 100, 150))
    start = lambda cs: [("run", "run", lambda: [c.start() for c in cs])]
    f0, f1 = front(0, 2, True), front(1, 1, True)
    seq += W("wma") + _flat(mod("moda", 0, 3)) + run(f0[0] + f1[0])
    seq += W("wmb") + start(next_kv(NC) + next_q(NC)) + _flat(mod("modb", 3, 5)) + run(f0[1] + f1[1])
    w1 = _flat(mm1("w1_0", 0, 0) + mm1("w1_1", 1, 1))
    seq += W("w1") + w1[:LP[4]] + W("w2") + w1[LP[4]:] + run(cat(shift(0, 0)))
    seq += _flat(mm2("w2_0", 0, 2, 1) + mm1("w1_2", 2, 2)) + run(cat(shift(1, 1))) + _flat(mm2("w2_1", 1, 1, 0))
    grp.append(Group("f2", front(2, 0), 80, ["w2"], ["w1_2"], 450))
    grp.append(Group("ln2_0", ln2(1, 0), 60, ["w2_0"], ["w3"], 450))
    grp.append(Group("ahead", cat(ahead(i) for i in range(NB - NC)), 19, ["w1"], ["end"], 100))
    _wait(seq, "w3")
    a, r = mm3("w3_0", 0)
    _mix(seq, a, [r], 0.1)
    mc = _flat(mod("modc", 5, 6))
    _wait(seq, "w4", mc[:5] + [("sync", "run", lambda: None)])
    w4 = mm4("w4_0", 0, 0, 3, 2, 1)[:LP[2]]
    qs = [quarter(w4[-1 - i]) for i in range((_phase(seq) + FT * LP[2]) % 4)]
    _mix(seq, _flat(w4), [mc[i:i + 4] for i in range(5, 25, 4)] + qs, 0.01, 0.4)
    assert _phase(seq) == 0
    grp.append(Group("resid", resid(2, 1), 26, ["modc"], ["end"], 100))
    _emit(seq, grp, zero, wait)

    def step(s, carry):
        with scope("wait_blk"):
            for c in next_kv(s) + next_q(s):
                c.wait()
        nxt = jnp.minimum(s + 1, NB - 1)
        seq, grp = [], []
        a, r = mm3("w3", 0)
        us, it = one(mmU(lambda n: "U%d" % n, 0, 0)), one(mmI(lambda n: "I%d" % n, 0, 0))
        w4 = mm4("w4", s - 2, 0)
        q = quarter(w4[LP[1] - 1])
        _mix(seq, _flat(mm4("w4c", s - 3, 0)[LP[2]:]) + a,
             [us[0], us[1], us[2], it[0] + us[3], it[1] + us[4], it[2] + start(next_kv(nxt)), it[3], it[4], r],
             LP[3], LP[0])
        _mix(seq, _flat(w4[:LP[1]]), [q])
        w1 = _flat(mm1("w1", 2, 0))
        seq += w1[:8] + start(next_q(nxt)) + w1[8:] + run(cat(shift(1, 0, ((T - 16, 16),))))
        seq += _flat(w4[LP[1]:LP[2]] + mm2("w2", 0, 1, 0))
        assert _phase(seq) == 0
        kvs, macs = kv(0, 0), mac(1, 0, 0, part=True)
        for t in range(NT):
            grp.append(Group("kv%d" % t, kvs[t], 50, ["start"], ["U%d" % t], 300))
            grp.append(Group("mac%d" % t, macs[t], 28, ["U%d" % t], ["I%d" % t], 300, 150))
        iall = ["I%d" % t for t in range(NT)]
        grp.append(Group("ln2", ln2(0, 0), 60, ["start"], ["w3"], 450))
        grp.append(Group("resid", resid(1, 0, True), 40, ["w4c"], ["w4", "I4"], 100))
        grp.append(Group("front", front(0, 0), 80, iall, ["w1"], 450))
        grp.append(Group("spread", spread(), 30, iall, ["end"], 100))
        grp.append(Group("shift", shift_early(), 12, ["start"], ["w1"], 200))
        _emit(seq, grp, zero, wait)
        out_b(s - 3).wait()
        out_a(s - 2).wait()
        return carry

    lax.fori_loop(NC, NB, step, 0)

    seq, grp = [], []
    seq += _flat(mm4("w4_5", NB - 3, 0)[LP[2]:])
    a, r = mm3("w3_6", 0)
    _mix(seq, a, [r])
    seq += _flat(mm2("w2_7", 0, 0, 1) + mm4("w4_6", NB - 2, 0, 1, 1, 0))
    a, r = mm3("w3_7", 1)
    _mix(seq, a, [r])
    seq += _flat(mm4("w4_7", NB - 1, 1, 2, 0, 1))
    assert _phase(seq) == 0
    grp.append(Group("ln2_6", ln2(0, 0), 60, ["start"], ["w3_6"], 450))
    grp.append(Group("shift7", cat(shift(2, 0)), 14, ["start"], ["w2_7"], 200))
    grp.append(Group("ln2_7", ln2(1, 1), 60, ["w2_7"], ["w3_7"], 450))
    _emit(seq, grp, zero, wait)
    with scope("wait_out"):
        for c in next_kv(NB - 1) + next_q(NB - 1) + [out_b(NB - 3)] + last:
            c.wait()


@jax.jit
def pallas_adaLN_cond__ssm_conv_h3__mixer_s_mlp__prompt_kernel(A_q, A_k, A_v, A_shift_k, A_ssm_k, A_ssm_D, B_x, B_w1, B_w2, B_w3, B_w4, c, w_mod):
    any_ = pl.BlockSpec(memory_space=pl.ANY)
    V = pltpu.VMEM
    out = pl.pallas_call(
        kernel,
        in_specs=[any_] * 12,
        out_specs=any_,
        out_shape=jax.ShapeDtypeStruct((S, D), BF16),
        scratch_shapes=[
            [V((NT, H + 8, 128), U32)] * NC, [V((NT, H + 8, 128), U32)] * NC, [V((NT, H + 8, 128), U32)] * NC,
            [V((64, S), U32)] * NT,
            V((D // 2, D), U32), V((D // 2, D), U32), V((F // 2, D), U32), V((F // 2, D), U32),
            [V((D // 2, 3 * D), U32), V((D // 2, 2 * D), U32), V((D // 2, D), U32)], V((4 * T, D), BF16),
            V((4, D), BF16), V((D,), BF16), V((1, D), BF16), V((8, 128), I32), pltpu.SMEM((8, 128), I32),
            V((5, 8, D), F32), V((6, 8, D), F32), V((T // 2, 4 * H), U32), V((GR // 2, 2 * T), U32),
            V((NB, 3 * T + 8, D), F32), V((NC, 3 * T + 8, D), F32), V((NB - NC, 2 * T + 8, D), F32), V((2 * T, D), F32),
            V((T, D), U32), V((NC * T, D), U32), V((NT, NC * T + 8, 128), F32),
            V((3 * T, D), F32), V((3 * T, D), F32), V((2 * T, D), F32), V((T, D), F32),
            V((3 * T // 2, D), U32), V((T, D), U32), V((T, D), U32), V((NT, NC * T + 24, 128), F32),
            V((T, (FT + 1) * 128), U32),
            pltpu.SemaphoreType.DMA((11,)), pltpu.SemaphoreType.DMA((1,)), pltpu.SemaphoreType.DMA((3,)),
        ],
        compiler_params=pltpu.CompilerParams(vmem_limit_bytes=110 << 20, disable_semaphore_checks=True,
                                             disable_bounds_checks=True),
        name="fused",
    )(A_q[0], A_k[0], A_v[0], A_shift_k.T, A_ssm_k, A_ssm_D, B_w1, B_w2, B_w3.T, B_w4, c, w_mod)
    return out[None]
```

```python
import heapq
import numpy as np
import jax
import jax.numpy as jnp
from jax import lax
from jax.experimental import pallas as pl
from jax.experimental.pallas import tpu as pltpu

S, D, F = 2048, 640, 1728
T = 256
H = T // 2
NB = S // T
NT = D // 128
FT = (F + 127) // 128
EPS = 1e-5
F32, BF16, U32, I32 = jnp.float32, jnp.bfloat16, jnp.uint32, jnp.int32
G_C1 = 0.044715 * float(np.sqrt(2.0 / np.pi))
G_C2 = float(np.sqrt(2.0 / np.pi))
G_A = G_C1 ** (1.0 / 3.0)
G_B = G_C2 / G_A
G_POST = 0.5 / G_A
RG = 16
GR = 80
NC = 3
SLOT = 32
LP = (0.8, 4, 6, 0.15, 72)


def _dft(shape, f_axis, tau, scale=1.0):
    r = lax.broadcasted_iota(I32, shape, f_axis)
    l = lax.broadcasted_iota(I32, shape, 1 - f_axis)
    f = r & 127
    odd = ((f & 63) << 2) | ((f >> 6) << 1) | 1
    p = odd * tau(l) + ((r >> 7) << 8)
    a = ((p + 512) & 1023) - 512
    u = (256 - jnp.abs(a)).astype(F32) * (np.pi / 512.0)
    u2 = u * u
    c = [scale, -scale / 6.0, scale / 120.0, -scale / 5040.0, scale / 362880.0, -scale / 39916800.0]
    poly = c[5]
    for ci in c[4::-1]:
        poly = poly * u2 + ci
    return (u * poly).astype(BF16)


def _ln(x, scale=1.0):
    m = jnp.sum(x, axis=-1, keepdims=True) * (1.0 / D)
    xc = x - m
    s2 = 1.0 / (scale * scale)
    v = jnp.sum(xc * xc, axis=-1, keepdims=True) * (s2 / D) + EPS * s2
    r = jnp.exp2(jnp.log(v) * float(-0.5 / np.log(2.0)))
    return xc * r


def _gelu2(x):
    u = x * (x * x + G_B)
    return x * (1.0 + jnp.tanh(u))


def _lo(w):
    return pltpu.bitcast(w << 16, F32)


def _hi(w):
    return pltpu.bitcast(w & jnp.uint32(0xFFFF0000), F32)


def _tie(x, a):
    if a is None:
        return x
    w = pltpu.bitcast(x[:, :128], U32)
    k = w.shape[0] // 8
    w = w | (a if k == 1 else jnp.concatenate([a] * k, axis=0))
    w = pltpu.bitcast(w, x.dtype)
    return w if x.shape[1] == 128 else jnp.concatenate([w, x[:, 128:]], axis=1)


def C(i, lim=F):
    return slice(i * 128, min((i + 1) * 128, lim))


class Unit:
    def __init__(self, name, tiles, epi, rows, cost, nt=False, full=True, acc=False):
        self.acc, self.res = acc, []
        self.name, self.tiles, self.epi, self.rows, self.cost, self.nt, self.full = name, tiles, epi, rows, cost, nt, full


class Group:
    def __init__(self, name, fns, cost, rel, dead, lat, rlat=200):
        self.name, self.fns, self.cost, self.rel, self.dead, self.lat, self.rlat = name, fns, cost, rel, dead, lat, rlat


def _plan(seq, groups):
    busy, n = [0] * 4, 0
    start, end, tiles, bars = {}, {}, [], []
    for it in seq:
        if isinstance(it[0], Unit):
            u = it[0]
            m = n % 4
            n += 1
            t0, t1 = busy[m], busy[m] + max(u.rows, 32)
            busy[m] = t1
            tiles.append((t0, t1, u.cost / len(u.tiles)))
            start.setdefault(u.name, t0)
            end[u.name] = max(end.get(u.name, 0), t1)
        elif it[0] == "wait":
            t = max(busy)
            busy, n = [t] * 4, 0
            start[it[1]] = end[it[1]] = t
            bars.append(t)
    total = max(busy)
    start["end"] = end["end"] = total
    start["start"] = end["start"] = 0
    ns = total // SLOT + 2
    load = np.zeros(ns)
    for t0, t1, c in tiles:
        a, b = t0 // SLOT, max(t1 // SLOT, t0 // SLOT + 1)
        load[a:b] += c / (b - a)
    win = []
    for g in groups:
        r = max(end[x] + (0 if start[x] == end[x] else g.rlat) for x in g.rel)
        d = min(start[x] for x in g.dead) - g.lat
        ok = np.zeros(ns, bool)
        ok[r // SLOT:max(d // SLOT, r // SLOT + 1)] = True
        for b in bars:
            if r < b <= d:
                ok[max((b - g.lat) // SLOT, 0):b // SLOT] = False
        win.append(np.nonzero(ok)[0])
    alloc = [np.zeros(len(w)) for w in win]
    for _ in range(60):
        for i, g in enumerate(groups):
            w = win[i]
            load[w] -= alloc[i]
            base = load[w]
            vol = g.cost * len(g.fns)
            lo, hi = base.min(), base.max() + vol
            for _ in range(50):
                mid = 0.5 * (lo + hi)
                if np.maximum(mid - base, 0).sum() > vol:
                    hi = mid
                else:
                    lo = mid
            alloc[i] = np.maximum(hi - base, 0)
            load[w] += alloc[i]
    times = []
    for i, g in enumerate(groups):
        cum = np.cumsum(alloc[i])
        ts = []
        for k in range(len(g.fns)):
            x = (k + 0.5) * cum[-1] / len(g.fns)
            j = int(np.searchsorted(cum, x))
            prev = cum[j - 1] if j else 0.0
            ts.append(win[i][j] * SLOT + SLOT * (x - prev) / max(alloc[i][j], 1e-9))
        times.append(ts)
    return times


def _emit(seq, groups, zero, wait):
    times = _plan(seq, groups)
    left = {"start": 0}
    for it in seq:
        nm = it[0].name if isinstance(it[0], Unit) else it[1]
        left[nm] = left.get(nm, 0) + 1
    heap, pend, todo, cnt = [], {}, list(range(len(groups))), 0
    busy, n = [0] * 4, 0

    def release():
        nonlocal cnt
        for i in list(todo):
            g = groups[i]
            if all(left[x] == 0 for x in g.rel):
                todo.remove(i)
                pend[i] = len(g.fns)
                for t, fn in zip(times[i], g.fns):
                    heapq.heappush(heap, (t, cnt, i, fn))
                    cnt += 1

    def force(name):
        nonlocal heap
        for i, g in enumerate(groups):
            if name in g.dead:
                assert i not in todo, (g.name, name)
                if pend[i]:
                    for it in sorted(x for x in heap if x[2] == i):
                        it[3](None)
                    heap = [x for x in heap if x[2] != i]
                    heapq.heapify(heap)
                    pend[i] = 0

    release()
    for it in seq:
        if isinstance(it[0], Unit):
            u, k = it
            force(u.name)
            lhs, rhs = u.tiles[k]()
            dn = (((1,), (1 if u.nt else 0,)), ((), ()))
            p = lax.dot_general(lhs, rhs, dn, preferred_element_type=F32)
            u.res = [p + u.res[0]] if (u.acc and u.res) else u.res + [p]
            m = n % 4
            n += 1
            t0 = busy[m]
            busy[m] = t0 + max(u.rows, 32)
            while u.full and heap and heap[0][0] < t0 + u.rows:
                t, _, i, fn = heapq.heappop(heap)
                pend[i] -= 1
                r = min(max(int(t - t0), 0), u.rows - 1) // 8 * 8
                fn(pltpu.bitcast(p[r:r + 8], U32) & zero)
            if k == len(u.tiles) - 1:
                u.epi(u.res)
            left[u.name] -= 1
        elif it[0] == "wait":
            force(it[1])
            wait(it[1])
            busy, n = [max(busy)] * 4, 0
            left[it[1]] -= 1
        else:
            it[2]()
            left[it[1]] -= 1
        release()
    force("end")
    assert not heap and not todo


def _sum(ps):
    acc = ps[0]
    for p in ps[1:]:
        acc = acc + p
    return acc


def _flat(us):
    return [(u, i) for u in us for i in range(len(u.tiles))]


def _phase(seq):
    n = 0
    for it in seq:
        n = n + 1 if isinstance(it[0], Unit) else (0 if it[0] in ("wait", "sync") else n)
    return n % 4


def _mix(seq, a, b, lo=0.0, hi=1.0):
    n, k = _phase(seq), 0
    for i, t in enumerate(a):
        if k < len(b) and n % 4 == 0 and t[1] != 1 and i >= len(a) * (lo + (hi - lo) * k / len(b)):
            seq.extend(b[k])
            k += 1
        seq.append(t)
        n += 1
    assert k == len(b)


def _wait(seq, name, head=(), back=0):
    r = _phase(seq) + 4 * back
    assert all(isinstance(it[0], Unit) for it in seq[len(seq) - r:])
    seq[len(seq) - r:len(seq) - r] = [("wait", name)] + list(head)


def kernel(q_hbm, k_hbm, v_hbm, sh_hbm, ssm_hbm, sd_hbm, w1_hbm, w2_hbm, w3_hbm, w4_hbm, c_hbm, wm_hbm,
           o_hbm,
           q_n, k_n, v_n, ssm_w, w1_w, w2_w, w3_w, w4_w, wm_w, o_v,
           sh_v, sd_v, c_v, zsrc, z_s, taps, mod_v, tf_w, tg_w,
           kf, uf, acc, zraw, kv_w, zz_w, y_v, x_v, hb_v, x1_v, r_v, n1_w, n2_w, g_w, h1_v, a_w,
           sem, sem_b, sem_o):
    bf = lambda r: r.bitcast(BF16)
    w1_v, w2_v, w3_v, w4_v = bf(w1_w), bf(w2_w), bf(w3_w), bf(w4_w)
    wm_v = {0: bf(wm_w[0]), 3: bf(wm_w[1]), 5: bf(wm_w[2])}
    tf_v, tg_v, n1_v, n2_v, g_v = bf(tf_w), bf(tg_w), bf(n1_w), bf(n2_w), bf(g_w)
    a_v, kv_v, zz_v = bf(a_w), bf(kv_w), bf(zz_w)
    cp = pltpu.make_async_copy

    def base(j, n):
        return j * n if isinstance(j, int) else pl.multiple_of(j * n, n)

    def rows(j, n=1, size=T):
        return pl.ds(base(j, size), n * size)

    def view(ref, j, size=T):
        return ref.at[rows(j, 1, size)]

    dmas = {}

    def group(name, *mks):
        sm = sem.at[len(dmas)]
        dmas[name] = [c for mk in mks for c in mk(sm)]

    def ssm_in(t):
        return lambda sm: [cp(ssm_hbm.at[C(t)], bf(ssm_w[t]), sm)]

    def cols(src, start, n, dst, row=0):
        return lambda sm: [cp(src.at[pl.ds(start, n), C(t)], bf(dst).at[t, pl.ds(row, n)], sm) for t in range(NT)]

    def kv_in(s, sl):
        if isinstance(s, int):
            kk = cols(k_hbm, s * T - 16, T + 16, k_n[sl]) if s else cols(k_hbm, 0, T, k_n[sl], 16)
        else:
            kk = cols(k_hbm, pl.multiple_of(s * T - 16, 16), T + 16, k_n[sl])
        return lambda sm: kk(sm) + cols(v_hbm, base(s, T), T, v_n[sl])(sm)

    def q_in(s, sl):
        return cols(q_hbm, base(s, T), T, q_n[sl])

    def wm_in(a, b):
        return lambda sm: [cp(wm_hbm.at[:, a * D:b * D], wm_v[a], sm)]

    def whole(src, dst):
        return lambda sm: [cp(src, dst, sm)]

    next_kv = lambda s: kv_in(s, 0)(sem_b.at[0])
    next_q = lambda s: q_in(s, 0)(sem_b.at[0])

    zsrc[...] = jnp.zeros((8, 128), I32)
    k_n[0][:, 0:8, :] = jnp.zeros((NT, 8, 128), U32)
    group("small", lambda sm: [cp(zsrc, z_s, sm), cp(sh_hbm, sh_v, sm), cp(sd_hbm, sd_v, sm), cp(c_hbm, c_v, sm)])
    for s in range(NC):
        group("c%d" % s, ssm_in(s), kv_in(s, s))
    group("c3", ssm_in(3), ssm_in(4))
    group("wma", wm_in(0, 3), q_in(0, 0), q_in(1, 1))
    group("wmb", wm_in(3, 5))
    group("w1", whole(w1_hbm, w1_v))
    group("w2", q_in(2, 2), whole(w2_hbm, w2_v))
    group("w3", whole(w3_hbm, w3_v))
    group("w4", whole(w4_hbm, w4_v), wm_in(5, 6))
    for g in dmas.values():
        for c in g:
            c.start()

    def wait(name):
        for c in dmas[name]:
            c.wait()

    tau_b = lambda l: H + ((l + (H - 1)) & (H - 1))
    tf_v[:, C(0)] = _dft((T, H), 0, lambda l: jnp.where((l & 1) == 0, l, tau_b(l)), 1.0 / T)
    tf_v[:, C(1)] = _dft((T, H), 0, lambda l: jnp.where((l & 1) == 1, l, tau_b(l)), 1.0 / T)
    tf_v[:, C(2)] = _dft((T, H), 0, lambda l: 2 * l - H)
    tf_v[:, C(3)] = _dft((T, H), 0, lambda l: 2 * l + 1 - H)
    sin0 = lax.broadcasted_iota(I32, (GR, T), 1) >= H
    tg_v[:, 0:T] = _dft((GR, T), 1, lambda l: jnp.where(sin0 & (l == 0), H, 2 * l))
    tg_v[:, T:2 * T] = _dft((GR, T), 1, lambda l: 2 * l + 1)
    h1_v[:, 0:8, :] = jnp.zeros((NT, 8, 128), F32)
    h1_v[:, 8 + NC * T:16 + NC * T, :] = jnp.zeros((NT, 8, 128), F32)

    wait("small")
    z = jnp.clip(z_s[0, 0], 0, 1)
    zero = jnp.full((8, 128), z, I32).astype(U32)
    z8 = pl.multiple_of(z * 8, 8)
    for r in (x_v, hb_v, x1_v, r_v, zraw, n1_w, n2_w, g_w, a_w, kv_w, zz_w):
        r[pl.ds(z8, 8), 0:128] = jnp.zeros((8, 128), r.dtype)
    for r in (kf, uf, acc, taps, mod_v):
        r[z, 0:8, 0:128] = jnp.zeros((8, 128), r.dtype)
    for r in (tf_w, tg_w):
        r[pl.ds(z8, 8), 0:128] = r[0:8, 0:128]
    sh = sh_v[...].astype(F32)
    for i in range(4):
        taps[i] = jnp.broadcast_to(sh[i:i + 1], (8, D))
    taps[4] = jnp.broadcast_to(sd_v[...].astype(F32).reshape(1, D) * (1.0 / T), (8, D))
    cf = c_v[...].astype(F32)
    silu_c = jnp.broadcast_to((cf / (1.0 + jnp.exp(-cf))).astype(BF16), (16, D))

    def mmK(n):
        def unit(m):
            st = []

            def rhs(i):
                if not st:
                    ev = (lax.broadcasted_iota(I32, (64, 128), 1) & 1) == 0
                    a = ssm_w[n][:, m * T:m * T + H]
                    b = pltpu.roll(ssm_w[n][:, m * T + H:(m + 1) * T], 1, 1)
                    st.extend([pltpu.bitcast(jnp.where(ev, a, b), BF16), pltpu.bitcast(jnp.where(ev, b, a), BF16)])
                return st[i]

            def epi(p):
                er, ei, or_, oi = p
                if m == 0:
                    er = er + taps[4, 0:1, C(n)]
                for h, (cr, ci) in enumerate(((er + or_, ei + oi), (er - or_, ei - oi))):
                    B = h * 3 * H
                    kf[m, B:B + H, C(n)] = cr
                    kf[m, B + H:B + 2 * H, C(n)] = ci - cr
                    kf[m, B + 2 * H:B + 3 * H, C(n)] = ci + cr
            return Unit("K%d" % n, [(lambda i=i, r=r: (tf_v[r:r + H, C(i)], rhs(i))) for i in range(2) for r in (0, H)],
                        epi, H, 170, nt=True)
        return [unit(m) for m in range(NB)]

    def kv(s, sl):
        def mk(t, w):
            def fn(a):
                ld = lambda o, n: k_n[s][t, pl.ds(8 + w + o, n), :]
                c0 = jnp.concatenate([_tie(ld(0, 8), a), ld(8, 8)], axis=0).reshape(2, 8, 128)
                c1, c2 = ld(-1, 16).reshape(2, 8, 128), ld(-2, 16).reshape(2, 8, 128)
                s0, s1, s2, s3 = (taps[i, :, C(t)] for i in range(4))
                ke, ko, ke1, ko1, ko2 = _lo(c0), _hi(c0), _lo(c1), _hi(c1), _hi(c2)
                wv = v_n[s][t, w:w + 16, :].reshape(2, 8, 128)
                kve = ((s0 * ke + s1 * ko1) + (s2 * ke1 + s3 * ko2)) * _lo(wv)
                kvo = ((s0 * ko + s1 * ke) + (s2 * ko1 + s3 * ke1)) * _hi(wv)
                kv_v[pl.ds(sl * T + w, 16), C(t)] = kve.reshape(16, 128).astype(BF16)
                kv_v[pl.ds(sl * T + H + w, 16), C(t)] = kvo.reshape(16, 128).astype(BF16)
            return fn
        return [[mk(t, w) for w in range(0, H, 16)] for t in range(NT)]

    def mmU(name, sl, us):
        def unit(n):
            def epi(p):
                er, ei, or_, oi = p
                for h, (cr, ci) in enumerate(((er + or_, ei + oi), (er - or_, ei - oi))):
                    B = h * 3 * H
                    uf[us, B:B + H, C(n)] = cr + ci
                    uf[us, B + H:B + 2 * H, C(n)] = cr
                    uf[us, B + 2 * H:B + 3 * H, C(n)] = ci
            return Unit(name(n), [(lambda i=i, r=r: (tf_v[r:r + H, C(2 + i)], kv_v[pl.ds(sl * T + i * H, H), C(n)]))
                                  for i in range(2) for r in (0, H)], epi, H, 120)
        return [unit(n) for n in range(NT)]

    def cmul(m0, u0, n, h, row, L, a):
        t = []
        for i in range(3):
            Rw = slice((3 * h + i) * H + row, (3 * h + i) * H + row + 8)
            kk = kf[m0:m0 + n, Rw, L]
            if i == 0 and a is not None:
                k0 = _tie(kk[0], a)[None]
                kk = k0 if n == 1 else jnp.concatenate([k0, kk[1:]], axis=0)
            t.append(jnp.sum(kk * uf[u0:u0 + n, Rw, L], axis=0))
        return t[0] - t[2], t[0] + t[1]

    def AR(h, q, row):
        return slice((2 * h + q) * H + row, (2 * h + q) * H + row + 8)

    def mac(n, u0, sl, first=False, part=False):
        def mk(t, rc):
            st, fin = [], []

            def piece(i):
                def fn(a):
                    h, row = i & 1, rc + (i >> 1) * 8
                    zr, zi = cmul(0, u0, n, h, row, C(t), a)
                    if part:
                        zr, zi = zr + acc[0, AR(h, 0, row), C(t)], zi + acc[0, AR(h, 1, row), C(t)]
                    st.append((zr, zi))
                    if h:
                        (pr, pi), (mr, mi) = st[-2:]
                        z = [pr + mr, pi + mi, pr - mr, pi - mi]
                        Rw = lambda q: slice(q * H + row, q * H + row + 8)
                        pv = None if first else [zraw[Rw(q ^ 1), C(t)] for q in range(4)]
                        for q in range(4):
                            zraw[Rw(q), C(t)] = z[q]
                        if not first:
                            z = [z[q] + pv[q] if (q & 1) == (rc < 64) else z[q] - pv[q] for q in range(4)]
                        fin.append(z)
                    if i == 3:
                        for q in range(4):
                            zz_v[pl.ds(sl * 2 * T + q * H + rc, 16), C(t)] = jnp.concatenate(
                                [fin[0][q], fin[1][q]], axis=0).astype(BF16)
                return fn
            if not part:
                return [piece(i) for i in range(4)]
            both = lambda f, g: (lambda a: (f(a), g(None)))
            return [both(piece(0), piece(1)), both(piece(2), piece(3))]
        return [[fn for rc in range(0, H, 16) for fn in mk(t, rc)] for t in range(NT)]

    def pos():
        return [(t, h, row) for t in range(NT) for row in range(0, H, 8) for h in range(2)]

    def ahead(i):
        def mk(t, h, row):
            def fn(a):
                zr, zi = cmul(i + 1, 0, NC, h, row, C(t), a)
                acc[i, AR(h, 0, row), C(t)] = zr
                acc[i, AR(h, 1, row), C(t)] = zi
            return fn
        return [mk(*p) for p in pos()]

    def spread():
        n = NB - NC - 1

        def mk(t, h, row):
            def fn(a):
                p = []
                for i in range(3):
                    Rw = slice((3 * h + i) * H + row, (3 * h + i) * H + row + 8)
                    u = uf[0, Rw, C(t)]
                    p.append(kf[1:1 + n, Rw, C(t)] * (_tie(u, a) if i == 0 else u)[None])
                acc[0:n, AR(h, 0, row), C(t)] = acc[1:1 + n, AR(h, 0, row), C(t)] + (p[0] - p[2])
                acc[0:n, AR(h, 1, row), C(t)] = acc[1:1 + n, AR(h, 1, row), C(t)] + (p[0] + p[1])
            return fn
        return [mk(*p) for p in pos()]

    def mmI(name, sl, ys):
        def unit(n):
            def epi(p):
                ce, se, co, so = p
                sub = lax.broadcasted_iota(I32, (8, 128), 0)
                c0 = ys * T + H
                y_v[n, ys * T:ys * T + 1, :] = (ce[64:72] - se[0:8])[0:1]
                se = jnp.concatenate([jnp.where(sub == 0, 0.0, se[0:8]), se[8:]], axis=0)
                for d, cc, ss in ((0, ce[0:64], se), (1, co, so)):
                    y_v[n, pl.ds(c0 + d, 64, stride=2), :] = cc + ss
                    lo = cc - ss
                    for i in range(0, 64, 8):
                        y_v[n, pl.ds(c0 - d - 2 * i - 14, 8, stride=2), :] = jnp.take_along_axis(
                            lo[i:i + 8], 7 - sub, axis=0)
            return Unit(name(n), [(lambda i=i: (tg_v[0:(GR if i == 0 else 64), C(i)], zz_v[pl.ds(sl * 2 * T + i * H, H), C(n)]))
                                  for i in range(4)], epi, 64, 52)
        return [unit(n) for n in range(NT)]

    def mod(name, a, b):
        def unit(n):
            def epi(p):
                v = [_sum(p[i * NT:(i + 1) * NT])[0:8] for i in range(b - a)]
                if a == 0:
                    mod_v[0, :, C(n)] = v[0] * v[2]
                    mod_v[1, :, C(n)] = (v[1] + 1.0) * v[2]
                elif a == 3:
                    mod_v[3, :, C(n)] = v[0]
                    mod_v[4, :, C(n)] = v[1] + 1.0
                else:
                    mod_v[5, :, C(n)] = v[0]
                    mod_v[2, :, C(n)] = v[0] * G_POST
            return Unit(name, [(lambda i=i, k=k: (silu_c[:, C(k)], wm_v[a][C(k), pl.ds(i * D + n * 128, 128)]))
                               for i in range(b - a) for k in range(NT)], epi, 16, 10, full=False, acc=b - a == 1)
        return [unit(n) for n in range(NT)]

    GS = range(0, T, RG)
    HS = (slice(0, 128), slice(128, 256))

    def tasks(f):
        return [(lambda a, r=r: f(slice(r, r + RG), a)) for r in GS]

    def load_y(sl, R):
        return jnp.concatenate([y_v[t, sl * T + R.start:sl * T + R.stop, :] for t in range(NT)],
                               axis=1).reshape(2, 8, D)

    def front(sl, xs, early=False):
        xx, hh, nn = view(x_v, xs), view(hb_v, xs), view(n1_v, sl)

        def fa(R, a):
            q = [q_n[sl][t, R.start // 2:R.stop // 2, :] for t in range(NT)]
            q = jnp.concatenate([_tie(q[0], a)] + q[1:], axis=1)
            q = pltpu.bitcast(q, BF16).astype(F32).reshape(2, 8, D)
            x = (q + (_ln(q) * mod_v[1] + mod_v[0]) * load_y(sl, R)).reshape(RG, D)
            xx[R, :] = x
            if early:
                hh[R, :] = _ln(x)

        def fb(R, a):
            hh[R, :] = (_ln(_tie(xx[R, :], a).reshape(2, 8, D)) * mod_v[4] + mod_v[3]).reshape(RG, D)

        def fc(R, a):
            hb = _tie(hh[R, :], a)
            if early:
                hb = (hb.reshape(2, 8, D) * mod_v[4] + mod_v[3]).reshape(RG, D)
                hh[R, :] = hb
            nn[R, :] = _ln(hb, G_A).astype(BF16)
        return (tasks(fa), tasks(fc)) if early else tasks(fa) + tasks(fb) + tasks(fc)

    def shift(hs, sl, pieces=((0, 64), (64, 64), (128, 64), (192, 64))):
        gg = view(g_v, sl)

        def mk(t, r, n):
            def fn(a):
                lane = lax.broadcasted_iota(I32, (n, 128), 1)
                ld = lambda d: h1_v[t, pl.ds(hs * T + 8 + r + d, n), :]
                if t == 0:
                    g = ld(-1)
                elif t == 1:
                    g = jnp.where(lane < 32, ld(-1), ld(1))
                elif t == 2:
                    g = jnp.where(lane < 64, ld(1), ld(-2))
                elif t == 3:
                    g = jnp.where(lane < 96, ld(-2), ld(2))
                else:
                    g = ld(2)
                if a is not None:
                    g = jnp.concatenate([_tie(g[i:i + 8], a) if i % 16 == 0 else g[i:i + 8]
                                         for i in range(0, n, 8)], axis=0)
                gg[r:r + n, C(t)] = g.astype(BF16)
            return fn
        return [[mk(t, r, n) for r, n in pieces] for t in range(NT)]

    def shift_early():
        def keep(t):
            def fn(a):
                h1_v[t, 2 * T - 16:2 * T + 8, :] = h1_v[t, 3 * T - 16:3 * T + 8, :]
            return fn
        sh = shift(2, 0, ((0, 64), (64, 64), (128, 64), (192, 48)))
        return [fn for t in range(NT) for fn in sh[t] + [keep(t)]]

    def ln2(xs, sl):
        xx, nn = view(x1_v, xs), view(n2_v, sl)

        def f(R, a):
            nn[R, :] = _ln(_tie(xx[R, :], a), G_A).astype(BF16)
        return tasks(f)

    def resid(xs, x1s, rotate=False):
        xx, x1 = view(x_v, xs), view(x1_v, x1s)

        def f(R, a):
            gb = mod_v[5] if a is None else pltpu.bitcast(
                pltpu.bitcast(mod_v[5], U32) | jnp.concatenate([a] * NT, axis=1), F32)
            r_v[R, :] = xx[R, :] + (x1[R, :].reshape(2, 8, D) * gb).reshape(RG, D)
            if rotate:
                xx[R, :] = x_v[R, :]
                view(hb_v, 1)[R, :] = hb_v[R, :]
        return tasks(f)

    def mm1(name, hs, sl):
        nn = view(n1_v, sl)

        def unit(n, R):
            def epi(p):
                h1_v[n, pl.ds(hs * T + 8 + R.start, 128), :] = _gelu2(p[0])
            return Unit(name, [(lambda k=k: (nn[R, C(k)], w1_v[C(k), C(n)])) for k in range(NT)],
                        epi, 128, 144, acc=True)
        return [unit(n, R) for n in range(NT) for R in HS]

    def mm2(name, sl, xs, x1s):
        gg, hh, x1 = view(g_v, sl), view(hb_v, xs), view(x1_v, x1s)

        def unit(n, R):
            def epi(p):
                x1[R, C(n)] = hh[R, C(n)] + p[0] * G_POST
            return Unit(name, [(lambda k=k: (gg[R, C(k)], w2_v[C(k), C(n)])) for k in range(NT)],
                        epi, 128, 96, acc=True)
        return [unit(n, R) for n in range(NT) for R in HS]

    def mm3(name, sl):
        nn, aa = view(n2_v, sl), view(a_v, sl)

        def unit(n, R):
            def epi(p):
                aa[R, C(n)] = _gelu2(p[0]).astype(BF16)
            return Unit(name, [(lambda k=k: (nn[R, C(k)], w3_v[C(n), C(k)])) for k in range(NT)],
                        epi, 128, 160, nt=True, acc=True)
        main = [unit(n, R) for n in range(FT - 1) for R in HS]
        F0, part = (FT - 1) * 128, []
        main[-1].tiles.pop(0)

        def epi(p):
            for i, R in enumerate(HS):
                aa[R, F0:F] = _gelu2(part[i] + p[i]).T.astype(BF16)
            main[-1].res = [jnp.concatenate(p[2:], axis=0)]
        rem = [Unit(name, [(lambda k=k, R=R: (w3_v[F0:F, C(k)], nn[R, C(k)])) for k in range(NT - 1)],
                    lambda p: part.append(p[0]), 64, 24, nt=True, acc=True) for R in HS]
        rem.append(Unit(name, [(lambda R=R: (w3_v[F0:F, C(NT - 1)], nn[R, C(NT - 1)])) for R in HS]
                        + [(lambda r=r: (nn[r:r + 64, C(0)], w3_v[C(FT - 2), C(0)])) for r in (128, 192)],
                        epi, 64, 120, nt=True))
        return _flat(main), _flat(rem)

    NA = LP[2] // 2 * 128

    def cp_out(j, osl, L, sm, R=slice(0, T)):
        return cp(o_v.at[pl.ds(osl * T + R.start, R.stop - R.start), L],
                  o_hbm.at[pl.ds(base(j, T) + R.start, R.stop - R.start), L], sem_o.at[sm])

    out_a = lambda j: cp_out(j, 0, slice(0, NA), 0)
    out_b = lambda j: cp_out(j, 0, slice(NA, D), 1)
    last = []

    def mm4(name, j, sl, osl=0, xs=None, x1s=None):
        aa, oo = view(a_v, sl), view(o_v, osl)

        def unit(n, R):
            def epi(p):
                if xs is None:
                    oo[R, C(n)] = (r_v[R, C(n)] + mod_v[2, 0:1, C(n)] * p[0]).astype(BF16)
                else:
                    oo[R, C(n)] = (view(x_v, xs)[R, C(n)] + mod_v[5, 0:1, C(n)]
                                   * (view(x1_v, x1s)[R, C(n)] + p[0] * G_POST)).astype(BF16)
                if osl == 2:
                    last.append(cp_out(j, osl, C(n), 2, R))
                    last[-1].start()
                elif R.stop == T and (osl, (n + 1) * 128) in ((1, D), (3, NA)):
                    last.append(cp_out(j, osl, slice(0, (n + 1) * 128), 2))
                    last[-1].start()
                elif R.stop == T and osl == 0 and (n + 1) * 128 in (NA, D):
                    (out_a if (n + 1) * 128 == NA else out_b)(j).start()
            return Unit(name, [(lambda k=k: (aa[R, C(k)], w4_v[C(k), C(n)])) for k in range(FT)],
                        epi, 128, 16 * (16 if xs is None else 18), acc=True)
        return [unit(n, R) for n in range(NT) for R in HS]

    def quarter(u):
        mk = u.tiles.pop(0)
        st = []

        def piece(i):
            if not st:
                st.extend(mk())
            return st[0][32 * i:32 * i + 32], st[1]

        def epi(p):
            u.res = [jnp.concatenate(p, axis=0)]
        return _flat([Unit(u.name, [(lambda i=i: piece(i)) for i in range(4)], epi, 32, 0, nt=u.nt)])

    W = lambda nm: [("wait", nm)]
    run = lambda fns: [("run", "run", lambda: [fn(None) for fn in fns])]
    one = lambda us: [_flat([u]) for u in us]
    cat = lambda ls: [x for l in ls for x in l]
    nm = lambda x: (lambda n: x)

    seq, grp = [], []
    for s in range(NC):
        seq += W("c%d" % s) + _flat(mmK(s) + mmU(nm("U%d" % s), s % 2, NC - 1 - s))
        grp.append(Group("kv%d" % s, cat(kv(s, s % 2)), 50, ["c%d" % s], ["U%d" % s], 100))
    inv = [mmI(lambda n: "I%d" % n, s, s) for s in range(NC)]
    seq += W("c3") + _flat(mmK(3) + mmK(4) + [inv[s][t] for t in range(NT) for s in range(NC)])
    macs = [mac(s + 1, NC - 1 - s, s, first=s == 0) for s in range(NC)]
    grp.append(Group("mac00", macs[0][0], 12, ["c1"], ["c2"], 0))
    grp.append(Group("mac01", macs[1][0] + macs[0][1] + macs[1][1], 16, ["c2"], ["c3"], 0))
    for t in range(NT):
        grp.append(Group("mac%d" % t, cat(macs[s][t] for s in range(2 if t < 2 else 0, NC)), 24 if t < 2 else 18,
                         ["c3", "K%d" % t], ["I%d" % t], 100, 150))
    start = lambda cs: [("run", "run", lambda: [c.start() for c in cs])]
    f0, f1 = front(0, 2, True), front(1, 1, True)
    seq += W("wma") + _flat(mod("moda", 0, 3)) + run(f0[0] + f1[0])
    seq += W("wmb") + start(next_kv(NC) + next_q(NC)) + _flat(mod("modb", 3, 5)) + run(f0[1])
    w1 = _flat(mm1("w1_0", 0, 0) + mm1("w1_1", 1, 1))
    seq += W("w1") + w1[:LP[4]] + W("w2") + w1[LP[4]:] + run(cat(shift(0, 0)))
    seq += _flat(mm2("w2_0", 0, 2, 1) + mm1("w1_2", 2, 2)) + run(cat(shift(1, 1))) + _flat(mm2("w2_1", 1, 1, 0))
    grp.append(Group("f1", f1[1], 80, ["w1"], ["w1_1"], 450))
    grp.append(Group("f2", front(2, 0), 80, ["w2"], ["w1_2"], 450))
    grp.append(Group("ln2_0", ln2(1, 0), 60, ["w2_0"], ["w3"], 450))
    grp.append(Group("ahead", cat(ahead(i) for i in range(NB - NC)), 19, ["w1"], ["end"], 100))
    _wait(seq, "w3", back=1)
    a, r = mm3("w3_0", 0)
    _mix(seq, a, [r], 0.1)
    mc = _flat(mod("modc", 5, 6))
    _wait(seq, "w4", mc[:5] + [("sync", "run", lambda: None)])
    w4 = mm4("w4_0", 0, 0, 3, 2, 1)[:LP[2]]
    qs = [quarter(w4[-1 - i]) for i in range((_phase(seq) + FT * LP[2]) % 4)]
    _mix(seq, _flat(w4), [mc[i:i + 4] for i in range(5, 25, 4)] + qs, 0.01, 0.4)
    assert _phase(seq) == 0
    grp.append(Group("resid", resid(2, 1), 26, ["modc"], ["end"], 100))
    _emit(seq, grp, zero, wait)

    def step(s, carry):
        for c in next_kv(s) + next_q(s):
            c.wait()
        nxt = jnp.minimum(s + 1, NB - 1)
        seq, grp = [], []
        a, r = mm3("w3", 0)
        us, it = one(mmU(lambda n: "U%d" % n, 0, 0)), one(mmI(lambda n: "I%d" % n, 0, 0))
        w4 = mm4("w4", s - 2, 0)
        q = quarter(w4[LP[1] - 1])
        _mix(seq, _flat(mm4("w4c", s - 3, 0)[LP[2]:]) + a,
             [us[0], us[1], us[2], it[0] + us[3], it[1] + us[4], it[2] + start(next_kv(nxt)), it[3], it[4], r],
             LP[3], LP[0])
        _mix(seq, _flat(w4[:LP[1]]), [q])
        w1 = _flat(mm1("w1", 2, 0))
        seq += w1[:8] + start(next_q(nxt)) + w1[8:] + run(cat(shift(1, 0, ((T - 16, 16),))))
        seq += _flat(w4[LP[1]:LP[2]] + mm2("w2", 0, 1, 0))
        assert _phase(seq) == 0
        kvs, macs = kv(0, 0), mac(1, 0, 0, part=True)
        for t in range(NT):
            grp.append(Group("kv%d" % t, kvs[t], 50, ["start"], ["U%d" % t], 300))
            grp.append(Group("mac%d" % t, macs[t], 28, ["U%d" % t], ["I%d" % t], 300, 150))
        iall = ["I%d" % t for t in range(NT)]
        grp.append(Group("ln2", ln2(0, 0), 60, ["start"], ["w3"], 450))
        grp.append(Group("resid", resid(1, 0, True), 40, ["w4c"], ["w4", "I4"], 100))
        grp.append(Group("front", front(0, 0), 80, iall, ["w1"], 450))
        grp.append(Group("spread", spread(), 30, iall, ["end"], 100))
        grp.append(Group("shift", shift_early(), 12, ["start"], ["w1"], 200))
        _emit(seq, grp, zero, wait)
        out_b(s - 3).wait()
        out_a(s - 2).wait()
        return carry

    lax.fori_loop(NC, NB, step, 0)

    seq, grp = [], []
    seq += _flat(mm4("w4_5", NB - 3, 0)[LP[2]:])
    a, r = mm3("w3_6", 0)
    _mix(seq, a, [r])
    seq += _flat(mm2("w2_7", 0, 0, 1) + mm4("w4_6", NB - 2, 0, 1, 1, 0))
    a, r = mm3("w3_7", 1)
    _mix(seq, a, [r])
    seq += _flat(mm4("w4_7", NB - 1, 1, 2, 0, 1))
    assert _phase(seq) == 0
    grp.append(Group("ln2_6", ln2(0, 0), 60, ["start"], ["w3_6"], 450))
    grp.append(Group("shift7", cat(shift(2, 0)), 14, ["start"], ["w2_7"], 200))
    grp.append(Group("ln2_7", ln2(1, 1), 60, ["w2_7"], ["w3_7"], 450))
    _emit(seq, grp, zero, wait)
    for c in next_kv(NB - 1) + next_q(NB - 1) + [out_b(NB - 3)] + last:
        c.wait()


@jax.jit
def pallas_adaLN_cond__ssm_conv_h3__mixer_s_mlp__prompt_kernel(
        A_q, A_k, A_v, A_shift_k, A_ssm_k, A_ssm_D, B_x, B_w1, B_w2, B_w3, B_w4, c, w_mod):
    any_ = pl.BlockSpec(memory_space=pl.ANY)
    V = pltpu.VMEM
    out = pl.pallas_call(
        kernel,
        in_specs=[any_] * 12,
        out_specs=any_,
        out_shape=jax.ShapeDtypeStruct((S, D), BF16),
        scratch_shapes=[
            [V((NT, H + 8, 128), U32)] * NC, [V((NT, H + 8, 128), U32)] * NC, [V((NT, H + 8, 128), U32)] * NC,
            [V((64, S), U32)] * NT,
            V((D // 2, D), U32), V((D // 2, D), U32), V((F // 2, D), U32), V((F // 2, D), U32),
            [V((D // 2, 3 * D), U32), V((D // 2, 2 * D), U32), V((D // 2, D), U32)], V((4 * T, D), BF16),
            V((4, D), BF16), V((D,), BF16), V((1, D), BF16), V((8, 128), I32), pltpu.SMEM((8, 128), I32),
            V((5, 8, D), F32), V((6, 8, D), F32), V((T // 2, 4 * H), U32), V((GR // 2, 2 * T), U32),
            V((NB, 3 * T + 8, D), F32), V((NC, 3 * T + 8, D), F32), V((NB - NC, 2 * T + 8, D), F32), V((2 * T, D), F32),
            V((T, D), U32), V((NC * T, D), U32), V((NT, NC * T + 8, 128), F32),
            V((3 * T, D), F32), V((3 * T, D), F32), V((2 * T, D), F32), V((T, D), F32),
            V((3 * T // 2, D), U32), V((T, D), U32), V((T, D), U32), V((NT, NC * T + 24, 128), F32),
            V((T, (FT + 1) * 128), U32),
            pltpu.SemaphoreType.DMA((11,)), pltpu.SemaphoreType.DMA((1,)), pltpu.SemaphoreType.DMA((3,)),
        ],
        compiler_params=pltpu.CompilerParams(vmem_limit_bytes=110 << 20, disable_semaphore_checks=True,
                                             disable_bounds_checks=True),
        name="fused",
    )(A_q[0], A_k[0], A_v[0], A_shift_k.T, A_ssm_k, A_ssm_D, B_w1, B_w2, B_w3.T, B_w4, c, w_mod)
    return out[None]
```

```python
import heapq
import numpy as np
import jax
import jax.numpy as jnp
from jax import lax
from jax.experimental import pallas as pl
from jax.experimental.pallas import tpu as pltpu

S, D, F = 2048, 640, 1728
T = 256
H = T // 2
NB = S // T
NT = D // 128
FT = (F + 127) // 128
EPS = 1e-5
F32, BF16, U32, I32 = jnp.float32, jnp.bfloat16, jnp.uint32, jnp.int32
G_C1 = 0.044715 * float(np.sqrt(2.0 / np.pi))
G_C2 = float(np.sqrt(2.0 / np.pi))
G_A = G_C1 ** (1.0 / 3.0)
G_B = G_C2 / G_A
G_POST = 0.5 / G_A
RG = 16
GR = 80
NC = 3
SLOT = 32
LP = (0.8, 4, 6, 0.15, 72)


def _dft(shape, f_axis, tau, scale=1.0):
    r = lax.broadcasted_iota(I32, shape, f_axis)
    l = lax.broadcasted_iota(I32, shape, 1 - f_axis)
    f = r & 127
    odd = ((f & 63) << 2) | ((f >> 6) << 1) | 1
    p = odd * tau(l) + ((r >> 7) << 8)
    a = ((p + 512) & 1023) - 512
    u = (256 - jnp.abs(a)).astype(F32) * (np.pi / 512.0)
    u2 = u * u
    c = [scale, -scale / 6.0, scale / 120.0, -scale / 5040.0, scale / 362880.0, -scale / 39916800.0]
    poly = c[5]
    for ci in c[4::-1]:
        poly = poly * u2 + ci
    return (u * poly).astype(BF16)


def _ln(x, scale=1.0):
    m = jnp.sum(x, axis=-1, keepdims=True) * (1.0 / D)
    xc = x - m
    s2 = 1.0 / (scale * scale)
    v = jnp.sum(xc * xc, axis=-1, keepdims=True) * (s2 / D) + EPS * s2
    r = jnp.exp2(jnp.log(v) * float(-0.5 / np.log(2.0)))
    return xc * r


def _gelu2(x):
    u = x * (x * x + G_B)
    return x * (1.0 + jnp.tanh(u))


def _lo(w):
    return pltpu.bitcast(w << 16, F32)


def _hi(w):
    return pltpu.bitcast(w & jnp.uint32(0xFFFF0000), F32)


def _tie(x, a):
    if a is None:
        return x
    w = pltpu.bitcast(x[:, :128], U32)
    k = w.shape[0] // 8
    w = w | (a if k == 1 else jnp.concatenate([a] * k, axis=0))
    w = pltpu.bitcast(w, x.dtype)
    return w if x.shape[1] == 128 else jnp.concatenate([w, x[:, 128:]], axis=1)


def _top(x, i):
    return jnp.concatenate([x[r:r + 16] for r in range(16 * i, x.shape[0], 32)], axis=0)


def _zip(t, b):
    return jnp.concatenate([x[r:r + 16] for r in range(0, t.shape[0], 16) for x in (t, b)], axis=0)


def _lhs_sums(x1, x2):
    a11, a21, a12, a22 = _top(x1, 0), _top(x1, 1), _top(x2, 0), _top(x2, 1)
    return [a11 + a22, a21 + a22, a11 + a12, a21 - a11, a12 - a22]


def C(i, lim=1 << 20):
    return slice(i * 128, min((i + 1) * 128, lim))


class Unit:
    def __init__(self, name, tiles, epi, rows, cost, nt=False, full=True, acc=False):
        self.acc, self.res = acc, []
        self.name, self.tiles, self.epi, self.rows, self.cost, self.nt, self.full = name, tiles, epi, rows, cost, nt, full


class Group:
    def __init__(self, name, fns, cost, rel, dead, lat, rlat=200):
        self.name, self.fns, self.cost, self.rel, self.dead, self.lat, self.rlat = name, fns, cost, rel, dead, lat, rlat


def _plan(seq, groups):
    busy, n = [0] * 4, 0
    start, end, tiles, bars = {}, {}, [], []
    for it in seq:
        if isinstance(it[0], Unit):
            u = it[0]
            m = n % 4
            n += 1
            t0, t1 = busy[m], busy[m] + max(u.rows, 32)
            busy[m] = t1
            tiles.append((t0, t1, u.cost / len(u.tiles)))
            start.setdefault(u.name, t0)
            end[u.name] = max(end.get(u.name, 0), t1)
        elif it[0] == "wait":
            t = max(busy)
            busy, n = [t] * 4, 0
            start[it[1]] = end[it[1]] = t
            bars.append(t)
    total = max(busy)
    start["end"] = end["end"] = total
    start["start"] = end["start"] = 0
    ns = total // SLOT + 2
    load = np.zeros(ns)
    for t0, t1, c in tiles:
        a, b = t0 // SLOT, max(t1 // SLOT, t0 // SLOT + 1)
        load[a:b] += c / (b - a)
    win = []
    for g in groups:
        r = max(end[x] + (0 if start[x] == end[x] else g.rlat) for x in g.rel)
        d = min(start[x] for x in g.dead) - g.lat
        ok = np.zeros(ns, bool)
        ok[r // SLOT:max(d // SLOT, r // SLOT + 1)] = True
        for b in bars:
            if r < b <= d:
                ok[max((b - g.lat) // SLOT, 0):b // SLOT] = False
        win.append(np.nonzero(ok)[0])
    alloc = [np.zeros(len(w)) for w in win]
    for _ in range(60):
        for i, g in enumerate(groups):
            w = win[i]
            load[w] -= alloc[i]
            base = load[w]
            vol = g.cost * len(g.fns)
            lo, hi = base.min(), base.max() + vol
            for _ in range(50):
                mid = 0.5 * (lo + hi)
                if np.maximum(mid - base, 0).sum() > vol:
                    hi = mid
                else:
                    lo = mid
            alloc[i] = np.maximum(hi - base, 0)
            load[w] += alloc[i]
    times = []
    for i, g in enumerate(groups):
        cum = np.cumsum(alloc[i])
        ts = []
        for k in range(len(g.fns)):
            x = (k + 0.5) * cum[-1] / len(g.fns)
            j = int(np.searchsorted(cum, x))
            prev = cum[j - 1] if j else 0.0
            ts.append(win[i][j] * SLOT + SLOT * (x - prev) / max(alloc[i][j], 1e-9))
        times.append(ts)
    return times


def _emit(seq, groups, zero, wait):
    times = _plan(seq, groups)
    left = {"start": 0}
    for it in seq:
        nm = it[0].name if isinstance(it[0], Unit) else it[1]
        left[nm] = left.get(nm, 0) + 1
    heap, pend, todo, cnt = [], {}, list(range(len(groups))), 0
    busy, n = [0] * 4, 0

    def release():
        nonlocal cnt
        for i in list(todo):
            g = groups[i]
            if all(left[x] == 0 for x in g.rel):
                todo.remove(i)
                pend[i] = len(g.fns)
                for t, fn in zip(times[i], g.fns):
                    heapq.heappush(heap, (t, cnt, i, fn))
                    cnt += 1

    def force(name):
        nonlocal heap
        for i, g in enumerate(groups):
            if name in g.dead:
                assert i not in todo, (g.name, name)
                if pend[i]:
                    for it in sorted(x for x in heap if x[2] == i):
                        it[3](None)
                    heap = [x for x in heap if x[2] != i]
                    heapq.heapify(heap)
                    pend[i] = 0

    release()
    for it in seq:
        if isinstance(it[0], Unit):
            u, k = it
            force(u.name)
            lhs, rhs = u.tiles[k]()
            dn = (((1,), (1 if u.nt else 0,)), ((), ()))
            p = lax.dot_general(lhs, rhs, dn, preferred_element_type=F32)
            u.res = [p + u.res[0]] if (u.acc and u.res) else u.res + [p]
            m = n % 4
            n += 1
            t0 = busy[m]
            busy[m] = t0 + max(u.rows, 32)
            while u.full and heap and heap[0][0] < t0 + u.rows:
                t, _, i, fn = heapq.heappop(heap)
                pend[i] -= 1
                r = min(max(int(t - t0), 0), u.rows - 1) // 8 * 8
                fn(pltpu.bitcast(p[r:r + 8], U32) & zero)
            if k == len(u.tiles) - 1:
                u.epi(u.res)
            left[u.name] -= 1
        elif it[0] == "wait":
            force(it[1])
            wait(it[1])
            busy, n = [max(busy)] * 4, 0
            left[it[1]] -= 1
        else:
            it[2]()
            left[it[1]] -= 1
        release()
    force("end")
    assert not heap and not todo


def _sum(ps):
    acc = ps[0]
    for p in ps[1:]:
        acc = acc + p
    return acc


def _flat(us):
    return [(u, i) for u in us for i in range(len(u.tiles))]


def _phase(seq):
    n = 0
    for it in seq:
        n = n + 1 if isinstance(it[0], Unit) else (0 if it[0] in ("wait", "sync") else n)
    return n % 4


def _mix(seq, a, b, lo=0.0, hi=1.0):
    n, k = _phase(seq), 0
    for i, t in enumerate(a):
        if k < len(b) and n % 4 == 0 and t[1] != 1 and i >= len(a) * (lo + (hi - lo) * k / len(b)):
            seq.extend(b[k])
            k += 1
        seq.append(t)
        n += 1
    assert k == len(b)


def _wait(seq, name, head=(), back=0):
    r = _phase(seq) + 4 * back
    assert all(isinstance(it[0], Unit) for it in seq[len(seq) - r:])
    seq[len(seq) - r:len(seq) - r] = [("wait", name)] + list(head)


def kernel(q_hbm, k_hbm, v_hbm, sh_hbm, ssm_hbm, sd_hbm, w1_hbm, w2_hbm, w3_hbm, w4_hbm, c_hbm, wm_hbm,
           o_hbm,
           q_n, k_n, v_n, ssm_w, w1_w, w2_w, w3_w, w4_w, wm_w, o_v,
           sh_v, sd_v, c_v, zsrc, z_s, taps, mod_v, tf_w, tg_w,
           kf, uf, acc, zraw, kv_w, zz_w, y_v, x_v, hb_v, x1_v, r_v, n1_w, n2_w, g_w, h1_v, a_w,
           ws_w, as_w,
           sem, sem_b, sem_o):
    bf = lambda r: r.bitcast(BF16)
    w1_v, w2_v, w3_v, w4_v = bf(w1_w), bf(w2_w), bf(w3_w), bf(w4_w)
    wm_v = {0: bf(wm_w[0]), 3: bf(wm_w[1]), 5: bf(wm_w[2])}
    tf_v, tg_v, n1_v, n2_v, g_v = bf(tf_w), bf(tg_w), bf(n1_w), bf(n2_w), bf(g_w)
    a_v, kv_v, zz_v = bf(a_w), bf(kv_w), bf(zz_w)
    w1s, w2s, w3s, w4s = [bf(r) for r in ws_w]
    n1s, gs, n2s, a_s = [bf(r) for r in as_w]
    cp = pltpu.make_async_copy
    cat = lambda ls: [x for l in ls for x in l]

    def base(j, n):
        return j * n if isinstance(j, int) else pl.multiple_of(j * n, n)

    def rows(j, n=1, size=T):
        return pl.ds(base(j, size), n * size)

    def view(ref, j, size=T):
        return ref.at[rows(j, 1, size)]

    dmas = {}

    def group(name, *mks):
        sm = sem.at[len(dmas)]
        dmas[name] = [c for mk in mks for c in mk(sm)]

    def ssm_in(t):
        return lambda sm: [cp(ssm_hbm.at[C(t)], bf(ssm_w[t]), sm)]

    def cols(src, start, n, dst, row=0):
        return lambda sm: [cp(src.at[pl.ds(start, n), C(t)], bf(dst).at[t, pl.ds(row, n)], sm) for t in range(NT)]

    def kv_in(s, sl):
        if isinstance(s, int):
            kk = cols(k_hbm, s * T - 16, T + 16, k_n[sl]) if s else cols(k_hbm, 0, T, k_n[sl], 16)
        else:
            kk = cols(k_hbm, pl.multiple_of(s * T - 16, 16), T + 16, k_n[sl])
        return lambda sm: kk(sm) + cols(v_hbm, base(s, T), T, v_n[sl])(sm)

    def q_in(s, sl):
        return cols(q_hbm, base(s, T), T, q_n[sl])

    def wm_in(a, b):
        return lambda sm: [cp(wm_hbm.at[:, a * D:b * D], wm_v[a], sm)]

    def whole(src, dst):
        return lambda sm: [cp(src, dst, sm)]

    next_kv = lambda s: kv_in(s, 0)(sem_b.at[0])
    next_q = lambda s: q_in(s, 0)(sem_b.at[0])

    zsrc[...] = jnp.zeros((8, 128), I32)
    k_n[0][:, 0:8, :] = jnp.zeros((NT, 8, 128), U32)
    group("small", lambda sm: [cp(zsrc, z_s, sm), cp(sh_hbm, sh_v, sm), cp(sd_hbm, sd_v, sm), cp(c_hbm, c_v, sm)])
    for s in range(NC):
        group("c%d" % s, ssm_in(s), kv_in(s, s))
    group("c3", ssm_in(3), ssm_in(4))
    group("wma", wm_in(0, 3), q_in(0, 0), q_in(1, 1))
    group("wmb", wm_in(3, 5))
    group("w1", whole(w1_hbm, w1_v))
    group("w2", q_in(2, 2), whole(w2_hbm, w2_v))
    group("w3", whole(w3_hbm, w3_v))
    group("w4", whole(w4_hbm, w4_v), wm_in(5, 6))
    for g in dmas.values():
        for c in g:
            c.start()

    def wait(name):
        for c in dmas[name]:
            c.wait()

    tau_b = lambda l: H + ((l + (H - 1)) & (H - 1))
    tf_v[:, C(0)] = _dft((T, H), 0, lambda l: jnp.where((l & 1) == 0, l, tau_b(l)), 1.0 / T)
    tf_v[:, C(1)] = _dft((T, H), 0, lambda l: jnp.where((l & 1) == 1, l, tau_b(l)), 1.0 / T)
    tf_v[:, C(2)] = _dft((T, H), 0, lambda l: 2 * l - H)
    tf_v[:, C(3)] = _dft((T, H), 0, lambda l: 2 * l + 1 - H)
    sin0 = lax.broadcasted_iota(I32, (GR, T), 1) >= H
    tg_v[:, 0:T] = _dft((GR, T), 1, lambda l: jnp.where(sin0 & (l == 0), H, 2 * l))
    tg_v[:, T:2 * T] = _dft((GR, T), 1, lambda l: 2 * l + 1)
    h1_v[:, 0:8, :] = jnp.zeros((NT, 8, 128), F32)
    h1_v[:, 8 + NC * T:16 + NC * T, :] = jnp.zeros((NT, 8, 128), F32)

    wait("small")
    z = jnp.clip(z_s[0, 0], 0, 1)
    zero = jnp.full((8, 128), z, I32).astype(U32)
    z8 = pl.multiple_of(z * 8, 8)
    for r in (x_v, hb_v, x1_v, r_v, zraw, n1_w, n2_w, g_w, a_w, kv_w, zz_w, *ws_w, *as_w):
        r[pl.ds(z8, 8), 0:128] = jnp.zeros((8, 128), r.dtype)
    for r in (kf, uf, acc, taps, mod_v):
        r[z, 0:8, 0:128] = jnp.zeros((8, 128), r.dtype)
    for r in (tf_w, tg_w):
        r[pl.ds(z8, 8), 0:128] = r[0:8, 0:128]
    sh = sh_v[...].astype(F32)
    for i in range(4):
        taps[i] = jnp.broadcast_to(sh[i:i + 1], (8, D))
    taps[4] = jnp.broadcast_to(sd_v[...].astype(F32).reshape(1, D) * (1.0 / T), (8, D))
    cf = c_v[...].astype(F32)
    silu_c = jnp.broadcast_to((cf / (1.0 + jnp.exp(-cf))).astype(BF16), (16, D))

    def mmK(n):
        def unit(m):
            st = []

            def rhs(i):
                if not st:
                    ev = (lax.broadcasted_iota(I32, (64, 128), 1) & 1) == 0
                    a = ssm_w[n][:, m * T:m * T + H]
                    b = pltpu.roll(ssm_w[n][:, m * T + H:(m + 1) * T], 1, 1)
                    st.extend([pltpu.bitcast(jnp.where(ev, a, b), BF16), pltpu.bitcast(jnp.where(ev, b, a), BF16)])
                return st[i]

            def epi(p):
                er, ei, or_, oi = p
                if m == 0:
                    er = er + taps[4, 0:1, C(n)]
                for h, (cr, ci) in enumerate(((er + or_, ei + oi), (er - or_, ei - oi))):
                    B = h * 3 * H
                    kf[m, B:B + H, C(n)] = cr
                    kf[m, B + H:B + 2 * H, C(n)] = ci - cr
                    kf[m, B + 2 * H:B + 3 * H, C(n)] = ci + cr
            return Unit("K%d" % n, [(lambda i=i, r=r: (tf_v[r:r + H, C(i)], rhs(i))) for i in range(2) for r in (0, H)],
                        epi, H, 170, nt=True)
        return [unit(m) for m in range(NB)]

    def kv(s, sl):
        def mk(t, w):
            def fn(a):
                ld = lambda o, n: k_n[s][t, pl.ds(8 + w + o, n), :]
                c0 = jnp.concatenate([_tie(ld(0, 8), a), ld(8, 8)], axis=0).reshape(2, 8, 128)
                c1, c2 = ld(-1, 16).reshape(2, 8, 128), ld(-2, 16).reshape(2, 8, 128)
                s0, s1, s2, s3 = (taps[i, :, C(t)] for i in range(4))
                ke, ko, ke1, ko1, ko2 = _lo(c0), _hi(c0), _lo(c1), _hi(c1), _hi(c2)
                wv = v_n[s][t, w:w + 16, :].reshape(2, 8, 128)
                kve = ((s0 * ke + s1 * ko1) + (s2 * ke1 + s3 * ko2)) * _lo(wv)
                kvo = ((s0 * ko + s1 * ke) + (s2 * ko1 + s3 * ke1)) * _hi(wv)
                kv_v[pl.ds(sl * T + w, 16), C(t)] = kve.reshape(16, 128).astype(BF16)
                kv_v[pl.ds(sl * T + H + w, 16), C(t)] = kvo.reshape(16, 128).astype(BF16)
            return fn
        return [[mk(t, w) for w in range(0, H, 16)] for t in range(NT)]

    def mmU(name, sl, us):
        def unit(n):
            def epi(p):
                er, ei, or_, oi = p
                for h, (cr, ci) in enumerate(((er + or_, ei + oi), (er - or_, ei - oi))):
                    B = h * 3 * H
                    uf[us, B:B + H, C(n)] = cr + ci
                    uf[us, B + H:B + 2 * H, C(n)] = cr
                    uf[us, B + 2 * H:B + 3 * H, C(n)] = ci
            return Unit(name(n), [(lambda i=i, r=r: (tf_v[r:r + H, C(2 + i)], kv_v[pl.ds(sl * T + i * H, H), C(n)]))
                                  for i in range(2) for r in (0, H)], epi, H, 120)
        return [unit(n) for n in range(NT)]

    def cmul(m0, u0, n, h, row, L, a):
        t = []
        for i in range(3):
            Rw = slice((3 * h + i) * H + row, (3 * h + i) * H + row + 8)
            kk = kf[m0:m0 + n, Rw, L]
            if i == 0 and a is not None:
                k0 = _tie(kk[0], a)[None]
                kk = k0 if n == 1 else jnp.concatenate([k0, kk[1:]], axis=0)
            t.append(jnp.sum(kk * uf[u0:u0 + n, Rw, L], axis=0))
        return t[0] - t[2], t[0] + t[1]

    def AR(h, q, row):
        return slice((2 * h + q) * H + row, (2 * h + q) * H + row + 8)

    def mac(n, u0, sl, first=False, part=False):
        def mk(t, rc):
            st, fin = [], []

            def piece(i):
                def fn(a):
                    h, row = i & 1, rc + (i >> 1) * 8
                    zr, zi = cmul(0, u0, n, h, row, C(t), a)
                    if part:
                        zr, zi = zr + acc[0, AR(h, 0, row), C(t)], zi + acc[0, AR(h, 1, row), C(t)]
                    st.append((zr, zi))
                    if h:
                        (pr, pi), (mr, mi) = st[-2:]
                        z = [pr + mr, pi + mi, pr - mr, pi - mi]
                        Rw = lambda q: slice(q * H + row, q * H + row + 8)
                        pv = None if first else [zraw[Rw(q ^ 1), C(t)] for q in range(4)]
                        for q in range(4):
                            zraw[Rw(q), C(t)] = z[q]
                        if not first:
                            z = [z[q] + pv[q] if (q & 1) == (rc < 64) else z[q] - pv[q] for q in range(4)]
                        fin.append(z)
                    if i == 3:
                        for q in range(4):
                            zz_v[pl.ds(sl * 2 * T + q * H + rc, 16), C(t)] = jnp.concatenate(
                                [fin[0][q], fin[1][q]], axis=0).astype(BF16)
                return fn
            if not part:
                return [piece(i) for i in range(4)]
            both = lambda f, g: (lambda a: (f(a), g(None)))
            return [both(piece(0), piece(1)), both(piece(2), piece(3))]
        return [[fn for rc in range(0, H, 16) for fn in mk(t, rc)] for t in range(NT)]

    def pos():
        return [(t, h, row) for t in range(NT) for row in range(0, H, 8) for h in range(2)]

    def ahead(i):
        def mk(t, h, row):
            def fn(a):
                zr, zi = cmul(i + 1, 0, NC, h, row, C(t), a)
                acc[i, AR(h, 0, row), C(t)] = zr
                acc[i, AR(h, 1, row), C(t)] = zi
            return fn
        return [mk(*p) for p in pos()]

    def spread():
        n = NB - NC - 1

        def mk(t, h, row):
            def fn(a):
                p = []
                for i in range(3):
                    Rw = slice((3 * h + i) * H + row, (3 * h + i) * H + row + 8)
                    u = uf[0, Rw, C(t)]
                    p.append(kf[1:1 + n, Rw, C(t)] * (_tie(u, a) if i == 0 else u)[None])
                acc[0:n, AR(h, 0, row), C(t)] = acc[1:1 + n, AR(h, 0, row), C(t)] + (p[0] - p[2])
                acc[0:n, AR(h, 1, row), C(t)] = acc[1:1 + n, AR(h, 1, row), C(t)] + (p[0] + p[1])
            return fn
        return [mk(*p) for p in pos()]

    def mmI(name, sl, ys):
        def unit(n):
            def epi(p):
                ce, se, co, so = p
                sub = lax.broadcasted_iota(I32, (8, 128), 0)
                c0 = ys * T + H
                y_v[n, ys * T:ys * T + 1, :] = (ce[64:72] - se[0:8])[0:1]
                se = jnp.concatenate([jnp.where(sub == 0, 0.0, se[0:8]), se[8:]], axis=0)
                for d, cc, ss in ((0, ce[0:64], se), (1, co, so)):
                    y_v[n, pl.ds(c0 + d, 64, stride=2), :] = cc + ss
                    lo = cc - ss
                    for i in range(0, 64, 8):
                        y_v[n, pl.ds(c0 - d - 2 * i - 14, 8, stride=2), :] = jnp.take_along_axis(
                            lo[i:i + 8], 7 - sub, axis=0)
            return Unit(name(n), [(lambda i=i: (tg_v[0:(GR if i == 0 else 64), C(i)], zz_v[pl.ds(sl * 2 * T + i * H, H), C(n)]))
                                  for i in range(4)], epi, 64, 52)
        return [unit(n) for n in range(NT)]

    def mod(name, a, b):
        def unit(n):
            def epi(p):
                v = [_sum(p[i * NT:(i + 1) * NT])[0:8] for i in range(b - a)]
                if a == 0:
                    mod_v[0, :, C(n)] = v[0] * v[2]
                    mod_v[1, :, C(n)] = (v[1] + 1.0) * v[2]
                elif a == 3:
                    mod_v[3, :, C(n)] = v[0]
                    mod_v[4, :, C(n)] = v[1] + 1.0
                else:
                    mod_v[5, :, C(n)] = v[0]
                    mod_v[2, :, C(n)] = v[0] * G_POST
            return Unit(name, [(lambda i=i, k=k: (silu_c[:, C(k)], wm_v[a][C(k), pl.ds(i * D + n * 128, 128)]))
                               for i in range(b - a) for k in range(NT)], epi, 16, 10, full=False, acc=b - a == 1)
        return [unit(n) for n in range(NT)]

    HS = (slice(0, 128), slice(128, 256))
    QS = tuple(slice(r, r + 64) for r in range(0, T, 64))

    def tasks(f, n=RG):
        return [(lambda a, r=r: f(slice(r, r + n), a)) for r in range(0, T, n)]

    def load_y(sl, R):
        return jnp.concatenate([y_v[t, sl * T + R.start:sl * T + R.stop, :] for t in range(NT)],
                               axis=1).reshape(2, 8, D)

    def put(nn, ss, R, x):
        nn[R, :] = x.astype(BF16)
        if ss is not None:
            ss[R.start // 2:R.stop // 2, 0:5 * T] = jnp.concatenate(
                _lhs_sums(x[:, 0:T], x[:, T:2 * T]), axis=1).astype(BF16)

    def front(sl, xs, early=False, ss=None):
        xx, hh, nn = view(x_v, xs), view(hb_v, xs), view(n1_v, sl)

        def fa(R, a):
            q = [q_n[sl][t, R.start // 2:R.stop // 2, :] for t in range(NT)]
            q = jnp.concatenate([_tie(q[0], a)] + q[1:], axis=1)
            q = pltpu.bitcast(q, BF16).astype(F32).reshape(2, 8, D)
            x = (q + (_ln(q) * mod_v[1] + mod_v[0]) * load_y(sl, R)).reshape(RG, D)
            xx[R, :] = x
            if early:
                hh[R, :] = _ln(x)

        def fb(R, a):
            hh[R, :] = (_ln(_tie(xx[R, :], a).reshape(2, 8, D)) * mod_v[4] + mod_v[3]).reshape(RG, D)

        def fc(R, a):
            hb = _tie(hh[R, :], a)
            if early:
                hb = (hb.reshape(2, 8, D) * mod_v[4] + mod_v[3]).reshape(RG, D)
                hh[R, :] = hb
            put(nn, ss, R, _ln(hb, G_A))
        if early:
            return tasks(fa), tasks(fc)
        last = tasks(fc) if ss is None else [f for g in tasks(fc, 32) for f in (g, lambda a: None)]
        return tasks(fa) + tasks(fb) + last

    def shift(hs, sl, pieces=((0, 64), (64, 64), (128, 64), (192, 64)), ss=None):
        gg = view(g_v, sl)

        def one_tile(t, r, n, a):
            lane = lax.broadcasted_iota(I32, (n, 128), 1)
            ld = lambda d: h1_v[t, pl.ds(hs * T + 8 + r + d, n), :]
            if t == 0:
                g = ld(-1)
            elif t == 1:
                g = jnp.where(lane < 32, ld(-1), ld(1))
            elif t == 2:
                g = jnp.where(lane < 64, ld(1), ld(-2))
            elif t == 3:
                g = jnp.where(lane < 96, ld(-2), ld(2))
            else:
                g = ld(2)
            if a is not None:
                g = jnp.concatenate([_tie(g[i:i + 8], a) if i % 16 == 0 else g[i:i + 8]
                                     for i in range(0, n, 8)], axis=0)
            gg[r:r + n, C(t)] = g.astype(BF16)
            return g

        def mk(ts, r, n):
            def fn(a):
                g = [one_tile(t, r, n, a) for t in ts]
                if len(ts) == 2:
                    for i, x in enumerate(_lhs_sums(*g)):
                        ss[r // 2:(r + n) // 2, C(2 * i + ts[0])] = x.astype(BF16)
            return fn
        sets = [(t,) for t in range(NT)] if ss is None else [(0, 2), (1, 3), (4,)]
        return [mk(ts, r, n) for ts in sets for r, n in pieces]

    def shift_early():
        def keep(a):
            h1_v[:, 2 * T - 32:2 * T + 8, :] = h1_v[:, 3 * T - 32:3 * T + 8, :]
        return shift(2, 0, [(r, 32) for r in range(0, T - 32, 32)], gs) + [keep]

    def ln2(xs, sl, fast=True):
        xx, nn, ss = view(x1_v, xs), view(n2_v, sl), view(n2s, sl, H) if fast else None
        return tasks(lambda R, a: put(nn, ss, R, _ln(_tie(xx[R, :], a), G_A)), 32 if fast else RG)

    def resid(xs, x1s, rotate=False):
        xx, x1 = view(x_v, xs), view(x1_v, x1s)

        def f(R, a):
            gb = mod_v[5] if a is None else pltpu.bitcast(
                pltpu.bitcast(mod_v[5], U32) | jnp.concatenate([a] * NT, axis=1), F32)
            r_v[R, :] = xx[R, :] + (x1[R, :].reshape(2, 8, D) * gb).reshape(RG, D)
            if rotate:
                xx[R, :] = x_v[R, :]
                view(hb_v, 1)[R, :] = hb_v[R, :]
        return tasks(f)

    KD, KF, ND = [(0, 2), (1, 3)], [(2 * i, 2 * i + 1) for i in range(6)], [(1, 2), (3, 4)]
    Wt = {1: (lambda k, n: w1_v[C(k), C(n)], lambda i, kp, j: w1s[C(kp), C(2 * i + j)], False, KD, [4]),
          2: (lambda k, n: w2_v[C(k), C(n)], lambda i, kp, j: w2s[C(kp), C(2 * i + j)], False, KD, [4]),
          3: (lambda k, n: w3_v[C(n), C(k)], lambda i, kp, j: w3s[C(j), C(2 * i + kp)], True, KD, [4]),
          4: (lambda k, n: w4_v[C(k, F), C(n)], lambda i, kp, j: w4s[C(kp), C(2 * i + j)], False, KF, [12, 13])}

    def wsums(w_w, ws, rp, cp_, nt):
        def mk(i, j, r):
            def fn(a):
                b = [[w_w[pl.ds(64 * p + r // 2, 8), C(q)] for q in cp_[j]] for p in rp[i]]
                b[0][0], b[1][1] = _tie(b[0][0], a), _tie(b[1][1], a)
                (b11, b12), (b21, b22) = [[pltpu.bitcast(x, BF16).astype(F32) for x in row] for row in b]
                if nt:
                    b12, b21 = b21, b12
                for m, x in enumerate((b11 + b22, b12 - b22, b21 - b11, b11 + b12, b21 + b22)):
                    ws[pl.ds(128 * i + r, 16), C(2 * m + j)] = x.astype(BF16)
            return fn
        return [mk(i, j, r) for i in range(len(rp)) for j in range(len(cp_)) for r in range(0, 128, 16)]

    def plain(name, w, lhs, n, R, epi, cost):
        tile, _, nt, kp, kl = Wt[w]
        ks = sorted([k for p in kp for k in p] + kl)
        rows_ = R.stop - R.start
        return Unit(name, [(lambda k=k: (lhs[R, C(k, F)], tile(k, n))) for k in ks], lambda p: epi(n, R, p[0]),
                    rows_, rows_ // 8 * (len(ks) - 1 + cost), nt=nt, acc=True)

    def quad(name, w, lhs, sums, j, cols_, R, epi, cost):
        tile, wsum, nt, kp, kl = Wt[w]
        h, S2, c = len(kp), slice(R.start // 2, R.stop // 2), {}
        a_ = lambda i, k: _top(lhs[R, C(k, F)], i)
        s_ = lambda i, p: sums[S2, C(h * i + p)]
        prod = lambda fa_, fb_: [(lambda p=p: (fa_(p), fb_(p))) for p in range(h)]
        left = lambda i, n: [(lambda k=k: (a_(i, k), tile(k, n))) for k in kl]
        mk = lambda tiles, f, x=0: Unit(name, tiles, lambda p: f(p[0]), 64, 8 * len(tiles) + x, nt=nt, acc=True)

        def e1(m):
            u7.res, u6.res = [m], [m]

        def e4(m):
            c[11], c[21] = c[11] + m, m

        def e2(m):
            l21.res, c[22] = [c[21] + m], c[22] - m

        def e5(m):
            c[12] = m
            epi(cols_[0], R, _zip(c[11] - m, c[21]))

        def e3(m):
            l12.res, c[22] = [c[12] + m], c[22] + m
        u1 = mk(prod(lambda p: s_(0, p), lambda p: wsum(0, p, j)), e1)
        u7 = mk(prod(lambda p: s_(4, p), lambda p: wsum(4, p, j)) + left(0, cols_[0]), lambda m: c.update({11: m}))
        u6 = mk(prod(lambda p: s_(3, p), lambda p: wsum(3, p, j)) + left(1, cols_[1]), lambda m: c.update({22: m}))
        u4 = mk(prod(lambda p: a_(1, kp[p][1]), lambda p: wsum(2, p, j)), e4)
        u2 = mk(prod(lambda p: s_(1, p), lambda p: tile(kp[p][0], cols_[0])), e2, 8)
        l21 = mk(left(1, cols_[0]), lambda m: c.update({21: m}))
        u5 = mk(prod(lambda p: s_(2, p), lambda p: tile(kp[p][1], cols_[1])), e5, 16 * cost)
        u3 = mk(prod(lambda p: a_(0, kp[p][0]), lambda p: wsum(1, p, j)), e3, 8)
        l12 = mk(left(0, cols_[1]), lambda m: epi(cols_[1], R, _zip(m, c[22])), 16 * cost)
        return [u1, u7, u6, u4, u2, l21, u5, u3, l12]

    def mm(name, w, lhs, sums, epi, cost):
        if sums is None:
            return [[plain(name, w, lhs, n, R, epi, cost) for R in HS] for n in range(NT)]
        return [[plain(name, w, lhs, 0, R, epi, cost) for R in QS]] + [
            [u for R in HS for u in quad(name, w, lhs, sums, j, ND[j], R, epi, cost)] for j in range(2)]

    def mm1(name, hs, sl, fast=False):
        def epi(n, R, p):
            h1_v[n, pl.ds(hs * T + 8 + R.start, R.stop - R.start), :] = _gelu2(p)
        return cat(mm(name, 1, view(n1_v, sl), n1s if fast else None, epi, 5))

    def mm2(name, sl, xs, x1s, fast=False):
        def epi(n, R, p):
            view(x1_v, x1s)[R, C(n)] = view(hb_v, xs)[R, C(n)] + p * G_POST
        return cat(mm(name, 2, view(g_v, sl), gs if fast else None, epi, 2))

    def mm3(name, sl, fast=True):
        nn, aa, ss, keep = view(n2_v, sl), view(a_v, sl), view(a_s, sl, H), []

        def epi(n, R, p):
            g = _gelu2(p)
            aa[R, C(n)] = g.astype(BF16)
            if n < 12 and n % 2:
                for i, x in enumerate(_lhs_sums(keep.pop(), g)):
                    ss[R.start // 2:R.stop // 2, C(6 * i + n // 2)] = x.astype(BF16)
            elif n < 12:
                keep.append(g)

        def rem(R):
            def f(p):
                aa[R, 13 * 128:F] = _gelu2(p[0]).T.astype(BF16)
            return Unit(name, [(lambda k=k: (w3_v[13 * 128:F, C(k)], nn[R, C(k)])) for k in range(NT)], f, 64, 84,
                        nt=True, acc=True)
        odd = [rem(R) for R in HS] + [plain(name, 3, nn, 12, R, epi, 6) for R in QS]
        if fast:
            return odd + [u for j in range(6) for R in HS
                          for u in quad(name, 3, nn, view(n2s, sl, H), j, KF[j], R, epi, 8)]
        return odd + [plain(name, 3, nn, n, R, epi, 8) for p in KF for R in HS for n in p]

    NA = 3 * 128

    def cp_out(j, osl, L, sm, R=slice(0, T)):
        return cp(o_v.at[pl.ds(osl * T + R.start, R.stop - R.start), L],
                  o_hbm.at[pl.ds(base(j, T) + R.start, R.stop - R.start), L], sem_o.at[sm])

    out_a = lambda j: cp_out(j, 0, slice(0, NA), 0)
    out_b = lambda j: cp_out(j, 0, slice(NA, D), 1)
    last = []

    def mm4(name, j, sl, osl=0, xs=None, x1s=None, fast=True):
        oo = view(o_v, osl)

        def epi(n, R, p):
            if xs is None:
                oo[R, C(n)] = (r_v[R, C(n)] + mod_v[2, 0:1, C(n)] * p).astype(BF16)
            else:
                oo[R, C(n)] = (view(x_v, xs)[R, C(n)] + mod_v[5, 0:1, C(n)]
                               * (view(x1_v, x1s)[R, C(n)] + p * G_POST)).astype(BF16)
            if osl == 2:
                last.append(cp_out(j, osl, C(n), 2, R))
                last[-1].start()
            elif R.stop == T and (osl, (n + 1) * 128) in ((1, D), (3, NA)):
                last.append(cp_out(j, osl, slice(0, (n + 1) * 128), 2))
                last[-1].start()
            elif R.stop == T and osl == 0 and (n + 1) * 128 in (NA, D):
                (out_a if (n + 1) * 128 == NA else out_b)(j).start()
        return mm(name, 4, view(a_v, sl), view(a_s, sl, H) if fast else None, epi, 3 if xs is None else 5)

    def split(us):
        n = 4 // len(us)
        m, mks, st = us[0].rows // n, [u.tiles.pop(0) for u in us], {}

        def piece(i, k):
            if i not in st:
                st[i] = mks[i]()
            return st[i][0][m * k:m * (k + 1)], st[i][1]

        def epi(p):
            for i, u in enumerate(us):
                u.res = [jnp.concatenate(p[n * i:n * (i + 1)], axis=0)]
        return _flat([Unit(us[0].name, [(lambda i=i, k=k: piece(i, k)) for i in range(len(us)) for k in range(n)],
                           epi, m, 0, nt=us[0].nt)])

    W = lambda nm: [("wait", nm)]
    run = lambda fns: [("run", "run", lambda: [fn(None) for fn in fns])]
    one = lambda us: [_flat([u]) for u in us]
    nm = lambda x: (lambda n: x)

    seq, grp = [], []
    for s in range(NC):
        seq += W("c%d" % s) + _flat(mmK(s) + mmU(nm("U%d" % s), s % 2, NC - 1 - s))
        grp.append(Group("kv%d" % s, cat(kv(s, s % 2)), 50, ["c%d" % s], ["U%d" % s], 100))
    inv = [mmI(lambda n: "I%d" % n, s, s) for s in range(NC)]
    seq += W("c3") + _flat(mmK(3) + mmK(4) + [inv[s][t] for t in range(NT) for s in range(NC)])
    macs = [mac(s + 1, NC - 1 - s, s, first=s == 0) for s in range(NC)]
    grp.append(Group("mac00", macs[0][0], 12, ["c1"], ["c2"], 0))
    grp.append(Group("mac01", macs[1][0] + macs[0][1] + macs[1][1], 16, ["c2"], ["c3"], 0))
    for t in range(NT):
        grp.append(Group("mac%d" % t, cat(macs[s][t] for s in range(2 if t < 2 else 0, NC)), 24 if t < 2 else 18,
                         ["c3", "K%d" % t], ["I%d" % t], 100, 150))
    start = lambda cs: [("run", "run", lambda: [c.start() for c in cs])]
    f0, f1 = front(0, 2, True), front(1, 1, True)
    seq += run(ahead(0))
    seq += W("wma") + _flat(mod("moda", 0, 3)) + run(f0[0] + f1[0] + ahead(1))
    seq += W("wmb") + start(next_kv(NC) + next_q(NC)) + _flat(mod("modb", 3, 5)) + run(f0[1])
    w1 = _flat(mm1("w1_0", 0, 0) + mm1("w1_1", 1, 1))
    seq += W("w1") + w1[:LP[4]] + W("w2") + w1[LP[4]:] + run(shift(0, 0))
    seq += _flat(mm2("w2_0", 0, 2, 1) + mm1("w1_2", 2, 2)) + run(shift(1, 1)) + _flat(mm2("w2_1", 1, 1, 0))
    grp.append(Group("f1", f1[1], 80, ["w1"], ["w1_1"], 450))
    grp.append(Group("f2", front(2, 0), 80, ["w2"], ["w1_2"], 450))
    grp.append(Group("ln2_0", ln2(1, 0, False), 60, ["w2_0"], ["w3"], 450))
    grp.append(Group("ahead", cat(ahead(i) for i in range(2, NB - NC)), 19, ["w1"], ["end"], 100))
    grp.append(Group("ws1", wsums(w1_w, w1s, KD, ND, False), 26, ["w1"], ["end"], 100))
    grp.append(Group("ws2", wsums(w2_w, w2s, KD, ND, False), 26, ["w2"], ["end"], 100))
    grp.append(Group("ws3", wsums(w3_w, w3s, KF, KD, True), 26, ["w3"], ["end"], 100))
    grp.append(Group("ws4", wsums(w4_w, w4s, KF, ND, False), 26, ["w4"], ["end"], 100))
    _wait(seq, "w3", back=1)
    w3 = mm3("w3_0", 0, False)
    _mix(seq, _flat(w3[6:]), [split(w3[4:6]) + _flat(w3[:6])], 0.1)
    mc = _flat(mod("modc", 5, 6))
    _wait(seq, "w4", mc[:5] + [("sync", "run", lambda: None)])
    w4 = cat(mm4("w4_0", 0, 0, 3, 2, 1, False)[:3])
    qs = [split([w4[-1 - i]]) for i in range((_phase(seq) + FT * 6) % 4)]
    _mix(seq, _flat(w4), [mc[i:i + 4] for i in range(5, 25, 4)] + qs, 0.01, 0.4)
    assert _phase(seq) == 0
    grp.append(Group("resid", resid(2, 1), 26, ["modc"], ["end"], 100))
    _emit(seq, grp, zero, wait)

    def step(s, carry):
        for c in next_kv(s) + next_q(s):
            c.wait()
        nxt = jnp.minimum(s + 1, NB - 1)
        seq, grp = [], []
        us, it = one(mmU(lambda n: "U%d" % n, 0, 0)), one(mmI(lambda n: "I%d" % n, 0, 0))
        w4 = mm4("w4", s - 2, 0)
        q = split(w4[0][2:])
        _mix(seq, _flat(mm4("w4c", s - 3, 0)[2] + mm3("w3", 0)),
             [us[0], us[1], us[2], it[0] + us[3], it[1] + us[4], it[2] + start(next_kv(nxt)), it[3], it[4]],
             LP[3], LP[0])
        _mix(seq, _flat(w4[0] + w4[1][:9]), [q])
        w1 = _flat(mm1("w1", 2, 0, True))
        seq += w1[:8] + start(next_q(nxt)) + w1[8:] + run(shift(1, 0, ((T - 32, 32),), gs))
        seq += _flat(w4[1][9:] + mm2("w2", 0, 1, 0, True))
        assert _phase(seq) == 0
        kvs, macs = kv(0, 0), mac(1, 0, 0, part=True)
        for t in range(NT):
            grp.append(Group("kv%d" % t, kvs[t], 50, ["start"], ["U%d" % t], 300))
            grp.append(Group("mac%d" % t, macs[t], 28, ["U%d" % t], ["I%d" % t], 300, 150))
        iall = ["I%d" % t for t in range(NT)]
        grp.append(Group("ln2", ln2(0, 0), 150, ["start"], ["w3"], 450))
        grp.append(Group("resid", resid(1, 0, True), 40, ["w4c"], ["w4", "I4"], 100))
        grp.append(Group("front", front(0, 0, ss=n1s), 82, iall, ["w1"], 450))
        grp.append(Group("spread", spread(), 30, iall, ["end"], 100))
        grp.append(Group("shift", shift_early(), 24, ["start"], ["w1"], 200))
        _emit(seq, grp, zero, wait)
        out_b(s - 3).wait()
        out_a(s - 2).wait()
        return carry

    lax.fori_loop(NC, NB, step, 0)

    seq, grp = [], []
    seq += _flat(mm4("w4_5", NB - 3, 0)[2] + mm3("w3_6", 0) + mm2("w2_7", 0, 0, 1, True)
                 + cat(mm4("w4_6", NB - 2, 0, 1, 1, 0)) + mm3("w3_7", 1) + cat(mm4("w4_7", NB - 1, 1, 2, 0, 1)))
    assert _phase(seq) == 0
    grp.append(Group("ln2_6", ln2(0, 0), 150, ["start"], ["w3_6"], 450))
    grp.append(Group("shift7", shift(2, 0, [(r, 32) for r in range(0, T, 32)], gs), 24, ["start"], ["w2_7"], 200))
    grp.append(Group("ln2_7", ln2(1, 1), 150, ["w2_7"], ["w3_7"], 450))
    _emit(seq, grp, zero, wait)
    for c in next_kv(NB - 1) + next_q(NB - 1) + [out_b(NB - 3)] + last:
        c.wait()


@jax.jit
def pallas_adaLN_cond__ssm_conv_h3__mixer_s_mlp__prompt_kernel(
        A_q, A_k, A_v, A_shift_k, A_ssm_k, A_ssm_D, B_x, B_w1, B_w2, B_w3, B_w4, c, w_mod):
    any_ = pl.BlockSpec(memory_space=pl.ANY)
    V = pltpu.VMEM
    out = pl.pallas_call(
        kernel,
        in_specs=[any_] * 12,
        out_specs=any_,
        out_shape=jax.ShapeDtypeStruct((S, D), BF16),
        scratch_shapes=[
            [V((NT, H + 8, 128), U32)] * NC, [V((NT, H + 8, 128), U32)] * NC, [V((NT, H + 8, 128), U32)] * NC,
            [V((64, S), U32)] * NT,
            V((D // 2, D), U32), V((D // 2, D), U32), V((F // 2, D), U32), V((F // 2, D), U32),
            [V((D // 2, 3 * D), U32), V((D // 2, 2 * D), U32), V((D // 2, D), U32)], V((4 * T, D), BF16),
            V((4, D), BF16), V((D,), BF16), V((1, D), BF16), V((8, 128), I32), pltpu.SMEM((8, 128), I32),
            V((5, 8, D), F32), V((6, 8, D), F32), V((T // 2, 4 * H), U32), V((GR // 2, 2 * T), U32),
            V((NB, 3 * T + 8, D), F32), V((NC, 3 * T + 8, D), F32), V((NB - NC, 2 * T + 8, D), F32), V((2 * T, D), F32),
            V((T, D), U32), V((NC * T, D), U32), V((NT, NC * T + 8, 128), F32),
            V((3 * T, D), F32), V((3 * T, D), F32), V((2 * T, D), F32), V((T, D), F32),
            V((3 * T // 2, D), U32), V((T, D), U32), V((T, D), U32), V((NT, NC * T + 24, 128), F32),
            V((T, (FT + 1) * 128), U32),
            [V((128, 11 * 128), U32)] * 2 + [V((384, 11 * 128), U32)] * 2,
            [V((64, 11 * 128), U32)] * 2 + [V((128, 11 * 128), U32), V((128, 31 * 128), U32)],
            pltpu.SemaphoreType.DMA((11,)), pltpu.SemaphoreType.DMA((1,)), pltpu.SemaphoreType.DMA((3,)),
        ],
        compiler_params=pltpu.CompilerParams(vmem_limit_bytes=110 << 20, disable_semaphore_checks=True,
                                             disable_bounds_checks=True),
        name="fused",
    )(A_q[0], A_k[0], A_v[0], A_shift_k.T, A_ssm_k, A_ssm_D, B_w1, B_w2, B_w3.T, B_w4, c, w_mod)
    return out[None]
```

```python
import heapq
import os
import numpy as np
import jax
import jax.numpy as jnp
from jax import lax
from jax.experimental import pallas as pl
from jax.experimental.pallas import tpu as pltpu

S, D, F = 2048, 640, 1728
T = 256
H = T // 2
NB = S // T
NT = D // 128
FT = (F + 127) // 128
EPS = 1e-5
F32, BF16, U32, I32 = jnp.float32, jnp.bfloat16, jnp.uint32, jnp.int32
G_C1 = 0.044715 * float(np.sqrt(2.0 / np.pi))
G_C2 = float(np.sqrt(2.0 / np.pi))
G_A = G_C1 ** (1.0 / 3.0)
G_B = G_C2 / G_A
G_POST = 0.5 / G_A
RG = 16
GR = 80
NC = 3
DL = int(os.environ.get('DL', 450))
V = os.environ.get('V', 'Q')
FL = int(os.environ.get('FL', 400))
RL = int(os.environ.get('RL', 2300))
DA = int(os.environ.get('DA', 650))
SLOT = 32
LP = (float(os.environ.get('LP0', 0.66)), 4, 6, float(os.environ.get('LP3', 0.15)), 72)


def _dft(shape, f_axis, tau, scale=1.0):
    r = lax.broadcasted_iota(I32, shape, f_axis)
    l = lax.broadcasted_iota(I32, shape, 1 - f_axis)
    f = r & 127
    odd = ((f & 63) << 2) | ((f >> 6) << 1) | 1
    p = odd * tau(l) + ((r >> 7) << 8)
    a = ((p + 512) & 1023) - 512
    u = (256 - jnp.abs(a)).astype(F32) * (np.pi / 512.0)
    u2 = u * u
    c = [scale, -scale / 6.0, scale / 120.0, -scale / 5040.0, scale / 362880.0, -scale / 39916800.0]
    poly = c[5]
    for ci in c[4::-1]:
        poly = poly * u2 + ci
    return (u * poly).astype(BF16)


def _rstd(xc, scale):
    s2 = 1.0 / (scale * scale)
    v = jnp.sum(xc * xc, axis=-1, keepdims=True) * (s2 / D) + EPS * s2
    return jnp.exp2(jnp.log(v) * float(-0.5 / np.log(2.0)))


def _ln(x, scale=1.0):
    xc = x - jnp.sum(x, axis=-1, keepdims=True) * (1.0 / D)
    return xc * _rstd(xc, scale)


def _gelu2(x):
    u = x * (x * x + G_B)
    return x * (1.0 + jnp.tanh(u))


def _lo(w):
    return pltpu.bitcast(w << 16, F32)


def _hi(w):
    return pltpu.bitcast(w & jnp.uint32(0xFFFF0000), F32)


def _tie(x, a):
    if a is None:
        return x
    w = pltpu.bitcast(x[:, :128], U32)
    k = w.shape[0] // 8
    w = w | (a if k == 1 else jnp.concatenate([a] * k, axis=0))
    w = pltpu.bitcast(w, x.dtype)
    return w if x.shape[1] == 128 else jnp.concatenate([w, x[:, 128:]], axis=1)


def _top(x, i):
    return jnp.concatenate([x[r:r + 16] for r in range(16 * i, x.shape[0], 32)], axis=0)


def _zip(t, b):
    return jnp.concatenate([x[r:r + 16] for r in range(0, t.shape[0], 16) for x in (t, b)], axis=0)


def _lhs_sums(x1, x2):
    a11, a21, a12, a22 = _top(x1, 0), _top(x1, 1), _top(x2, 0), _top(x2, 1)
    return [a11 + a22, a21 + a22, a11 + a12, a21 - a11, a12 - a22]


def C(i, lim=1 << 20):
    return slice(i * 128, min((i + 1) * 128, lim))


class Unit:
    def __init__(self, name, tiles, epi, rows, cost, nt=False, full=True, acc=False):
        self.acc, self.res = acc, []
        self.name, self.tiles, self.epi, self.rows, self.cost, self.nt, self.full = name, tiles, epi, rows, cost, nt, full


class Due:
    def __init__(self, val, delay):
        self.val, self.delay = val, delay


class Group:
    def __init__(self, name, fns, cost, rel, dead, lat, rlat=200):
        self.name, self.fns, self.cost, self.rel, self.dead, self.lat, self.rlat = name, fns, cost, rel, dead, lat, rlat


def _plan(seq, groups):
    busy, n = [0] * 4, 0
    start, end, tiles, bars = {}, {}, [], []
    for it in seq:
        if isinstance(it[0], Unit):
            u = it[0]
            m = n % 4
            n += 1
            t0, t1 = busy[m], busy[m] + max(u.rows, 32)
            busy[m] = t1
            tiles.append((t0, t1, u.cost / len(u.tiles)))
            start.setdefault(u.name, t0)
            end[u.name] = max(end.get(u.name, 0), t1)
        elif it[0] == "wait":
            t = max(busy)
            busy, n = [t] * 4, 0
            start[it[1]] = end[it[1]] = t
            bars.append(t)
    total = max(busy)
    start["end"] = end["end"] = total
    start["start"] = end["start"] = 0
    ns = total // SLOT + 2
    load = np.zeros(ns)
    for t0, t1, c in tiles:
        a, b = t0 // SLOT, max(t1 // SLOT, t0 // SLOT + 1)
        load[a:b] += c / (b - a)
    win = []
    for g in groups:
        r = max(end[x] + (0 if start[x] == end[x] else g.rlat) for x in g.rel)
        d = min(start[x] for x in g.dead) - g.lat
        ok = np.zeros(ns, bool)
        ok[r // SLOT:max(d // SLOT, r // SLOT + 1)] = True
        for b in bars:
            if r < b <= d:
                ok[max((b - g.lat) // SLOT, 0):b // SLOT] = False
        win.append(np.nonzero(ok)[0])
    alloc = [np.zeros(len(w)) for w in win]
    for _ in range(60):
        for i, g in enumerate(groups):
            w = win[i]
            load[w] -= alloc[i]
            base = load[w]
            vol = g.cost * len(g.fns)
            lo, hi = base.min(), base.max() + vol
            for _ in range(50):
                mid = 0.5 * (lo + hi)
                if np.maximum(mid - base, 0).sum() > vol:
                    hi = mid
                else:
                    lo = mid
            alloc[i] = np.maximum(hi - base, 0)
            load[w] += alloc[i]
    times = []
    for i, g in enumerate(groups):
        cum = np.cumsum(alloc[i])
        ts = []
        for k in range(len(g.fns)):
            x = (k + 0.5) * cum[-1] / len(g.fns)
            j = int(np.searchsorted(cum, x))
            prev = cum[j - 1] if j else 0.0
            ts.append(win[i][j] * SLOT + SLOT * (x - prev) / max(alloc[i][j], 1e-9))
        times.append(ts)
    return times


def _emit(seq, groups, zero, wait):
    times = _plan(seq, groups)
    left = {"start": 0}
    for it in seq:
        nm = it[0].name if isinstance(it[0], Unit) else it[1]
        left[nm] = left.get(nm, 0) + 1
    heap, pend, todo, cnt = [], {}, list(range(len(groups))), 0
    busy, n, due = [0] * 4, 0, []

    def release():
        nonlocal cnt
        for i in list(todo):
            g = groups[i]
            if all(left[x] == 0 for x in g.rel):
                todo.remove(i)
                pend[i] = len(g.fns)
                for t, fn in zip(times[i], g.fns):
                    heapq.heappush(heap, (t, cnt, i, fn))
                    cnt += 1

    def force(name):
        nonlocal heap
        for i, g in enumerate(groups):
            if name in g.dead:
                assert i not in todo, (g.name, name)
                if pend[i]:
                    for it in sorted(x for x in heap if x[2] == i):
                        it[3](None)
                    heap = [x for x in heap if x[2] != i]
                    heapq.heapify(heap)
                    pend[i] = 0

    release()
    for it in seq:
        if isinstance(it[0], Unit):
            u, k = it
            force(u.name)
            lhs, rhs = u.tiles[k]()
            t0 = busy[n % 4]
            while u.full and due and due[0][0] < t0 + u.rows:
                t, x = due.pop(0)
                r = min(max(int(t - t0), 0), u.rows - 1) // 16 * 8
                if lhs.shape[1] != 128:
                    due.insert(0, (t, x))
                    break
                w = pltpu.bitcast(lhs, U32)
                x = pltpu.bitcast(x[:, :128], U32)
                parts = [w[:r], w[r:r + 8] | ((x[0:8] | x[8:16]) & zero), w[r + 8:]]
                lhs = pltpu.bitcast(jnp.concatenate([y for y in parts if y.shape[0]], axis=0), BF16)
            dn = (((1,), (1 if u.nt else 0,)), ((), ()))
            p = lax.dot_general(lhs, rhs, dn, preferred_element_type=F32)
            u.res = [p + u.res[0]] if (u.acc and u.res) else u.res + [p]
            m = n % 4
            n += 1
            t0 = busy[m]
            busy[m] = t0 + max(u.rows, 32)
            while u.full and heap and heap[0][0] < t0 + u.rows:
                t, _, i, fn = heapq.heappop(heap)
                pend[i] -= 1
                r = min(max(int(t - t0), 0), u.rows - 1) // 8 * 8
                x = fn(pltpu.bitcast(p[r:r + 8], U32) & zero)
                if isinstance(x, Due):
                    due.append((t + x.delay, x.val))
                    due.sort(key=lambda e: e[0])
            if k == len(u.tiles) - 1:
                u.epi(u.res)
            left[u.name] -= 1
        elif it[0] == "wait":
            force(it[1])
            wait(it[1])
            busy, n, due = [max(busy)] * 4, 0, []
            left[it[1]] -= 1
        else:
            it[2]()
            left[it[1]] -= 1
        release()
    force("end")
    assert not heap and not todo


def _sum(ps):
    acc = ps[0]
    for p in ps[1:]:
        acc = acc + p
    return acc


def _flat(us):
    return [(u, i) for u in us for i in range(len(u.tiles))]


def _phase(seq):
    n = 0
    for it in seq:
        n = n + 1 if isinstance(it[0], Unit) else (0 if it[0] in ("wait", "sync") else n)
    return n % 4


def _mix(seq, a, b, lo=0.0, hi=1.0):
    n, k = _phase(seq), 0
    for i, t in enumerate(a):
        if k < len(b) and n % 4 == 0 and t[1] != 1 and i >= len(a) * (lo + (hi - lo) * k / len(b)):
            seq.extend(b[k])
            k += 1
        seq.append(t)
        n += 1
    assert k == len(b)


def _wait(seq, name, head=(), back=0):
    r = _phase(seq) + 4 * back
    assert all(isinstance(it[0], Unit) for it in seq[len(seq) - r:])
    seq[len(seq) - r:len(seq) - r] = [("wait", name)] + list(head)


def kernel(q_hbm, k_hbm, v_hbm, sh_hbm, ssm_hbm, sd_hbm, w1_hbm, w2_hbm, w3_hbm, w4_hbm, c_hbm, wm_hbm,
           o_hbm,
           q_n, k_n, v_n, ssm_w, w1_w, w2_w, w3_w, w4_w, wm_w, o_v,
           sh_v, sd_v, c_v, zsrc, z_s, taps, mod_v, tf_w, tg_w,
           kf, uf, acc, zraw, kv_w, zz_w, y_v, x_v, hb_v, x1_v, r_v, n1_w, n2_w, g_w, h1_v, a_w,
           ws_w, as_w, w3n_w, top_v, st_v,
           sem, sem_b, sem_o):
    bf = lambda r: r.bitcast(BF16)
    w1_v, w2_v, w3_v, w4_v = bf(w1_w), bf(w2_w), bf(w3_w), bf(w4_w)
    wm_v = {0: bf(wm_w[0]), 3: bf(wm_w[1]), 5: bf(wm_w[2])}
    tf_v, tg_v, n1_v, n2_v, g_v = bf(tf_w), bf(tg_w), bf(n1_w), bf(n2_w), bf(g_w)
    a_v, kv_v, zz_v = bf(a_w), bf(kv_w), bf(zz_w)
    w1s, w2s, w3s, w4s = [bf(r) for r in ws_w]
    n1s, gs, n2s, a_s = [bf(r) for r in as_w]
    w3n = bf(w3n_w)
    cp = pltpu.make_async_copy
    cat = lambda ls: [x for l in ls for x in l]

    def base(j, n):
        return j * n if isinstance(j, int) else pl.multiple_of(j * n, n)

    def rows(j, n=1, size=T):
        return pl.ds(base(j, size), n * size)

    def view(ref, j, size=T):
        return ref.at[rows(j, 1, size)]

    dmas = {}

    def group(name, *mks):
        sm = sem.at[len(dmas)]
        dmas[name] = [c for mk in mks for c in mk(sm)]

    def ssm_in(t):
        return lambda sm: [cp(ssm_hbm.at[C(t)], bf(ssm_w[t]), sm)]

    def cols(src, start, n, dst, row=0):
        return lambda sm: [cp(src.at[pl.ds(start, n), C(t)], bf(dst).at[t, pl.ds(row, n)], sm) for t in range(NT)]

    def kv_in(s, sl):
        if isinstance(s, int):
            kk = cols(k_hbm, s * T - 16, T + 16, k_n[sl]) if s else cols(k_hbm, 0, T, k_n[sl], 16)
        else:
            kk = cols(k_hbm, pl.multiple_of(s * T - 16, 16), T + 16, k_n[sl])
        return lambda sm: kk(sm) + cols(v_hbm, base(s, T), T, v_n[sl])(sm)

    def q_in(s, sl):
        return cols(q_hbm, base(s, T), T, q_n[sl])

    def wm_in(a, b):
        return lambda sm: [cp(wm_hbm.at[:, a * D:b * D], wm_v[a], sm)]

    def whole(src, dst):
        return lambda sm: [cp(src, dst, sm)]

    next_kv = lambda s: kv_in(s, 0)(sem_b.at[0])
    next_q = lambda s: q_in(s, 0)(sem_b.at[0])

    zsrc[...] = jnp.zeros((8, 128), I32)
    k_n[0][:, 0:8, :] = jnp.zeros((NT, 8, 128), U32)
    group("small", lambda sm: [cp(zsrc, z_s, sm), cp(sh_hbm, sh_v, sm), cp(sd_hbm, sd_v, sm), cp(c_hbm, c_v, sm)])
    for s in range(NC):
        group("c%d" % s, ssm_in(s), kv_in(s, s))
    group("c3", ssm_in(3), ssm_in(4))
    group("wma", wm_in(0, 3), q_in(0, 0), q_in(1, 1))
    group("wmb", wm_in(3, 5))
    group("w1", whole(w1_hbm, w1_v))
    group("w2", q_in(2, 2), whole(w2_hbm, w2_v))
    group("w3", whole(w3_hbm, w3_v))
    group("w4", whole(w4_hbm, w4_v), wm_in(5, 6))
    for g in dmas.values():
        for c in g:
            c.start()

    def wait(name):
        for c in dmas[name]:
            c.wait()

    tau_b = lambda l: H + ((l + (H - 1)) & (H - 1))
    tf_v[:, C(0)] = _dft((T, H), 0, lambda l: jnp.where((l & 1) == 0, l, tau_b(l)), 1.0 / T)
    tf_v[:, C(1)] = _dft((T, H), 0, lambda l: jnp.where((l & 1) == 1, l, tau_b(l)), 1.0 / T)
    tf_v[:, C(2)] = _dft((T, H), 0, lambda l: 2 * l - H)
    tf_v[:, C(3)] = _dft((T, H), 0, lambda l: 2 * l + 1 - H)
    sin0 = lax.broadcasted_iota(I32, (GR, T), 1) >= H
    tg_v[:, 0:T] = _dft((GR, T), 1, lambda l: jnp.where(sin0 & (l == 0), H, 2 * l))
    tg_v[:, T:2 * T] = _dft((GR, T), 1, lambda l: 2 * l + 1)
    h1_v[:, 0:8, :] = jnp.zeros((NT, 8, 128), F32)
    h1_v[:, 8 + NC * T:16 + NC * T, :] = jnp.zeros((NT, 8, 128), F32)

    wait("small")
    z = jnp.clip(z_s[0, 0], 0, 1)
    zero = jnp.full((8, 128), z, I32).astype(U32)
    z8 = pl.multiple_of(z * 8, 8)
    for r in (x_v, hb_v, x1_v, r_v, zraw, n1_w, n2_w, g_w, a_w, kv_w, zz_w, *ws_w, *as_w, w3n_w, top_v, st_v):
        r[pl.ds(z8, 8), 0:128] = jnp.zeros((8, 128), r.dtype)
    for r in (kf, uf, acc, taps, mod_v):
        r[z, 0:8, 0:128] = jnp.zeros((8, 128), r.dtype)
    for r in (tf_w, tg_w):
        r[pl.ds(z8, 8), 0:128] = r[0:8, 0:128]
    sh = sh_v[...].astype(F32)
    for i in range(4):
        taps[i] = jnp.broadcast_to(sh[i:i + 1], (8, D))
    taps[4] = jnp.broadcast_to(sd_v[...].astype(F32).reshape(1, D) * (1.0 / T), (8, D))
    cf = c_v[...].astype(F32)
    silu_c = jnp.broadcast_to((cf / (1.0 + jnp.exp(-cf))).astype(BF16), (16, D))

    def mmK(n):
        def unit(m):
            st = []

            def rhs(i):
                if not st:
                    ev = (lax.broadcasted_iota(I32, (64, 128), 1) & 1) == 0
                    a = ssm_w[n][:, m * T:m * T + H]
                    b = pltpu.roll(ssm_w[n][:, m * T + H:(m + 1) * T], 1, 1)
                    st.extend([pltpu.bitcast(jnp.where(ev, a, b), BF16), pltpu.bitcast(jnp.where(ev, b, a), BF16)])
                return st[i]

            def epi(p):
                er, ei, or_, oi = p
                if m == 0:
                    er = er + taps[4, 0:1, C(n)]
                for h, (cr, ci) in enumerate(((er + or_, ei + oi), (er - or_, ei - oi))):
                    B = h * 3 * H
                    kf[m, B:B + H, C(n)] = cr
                    kf[m, B + H:B + 2 * H, C(n)] = ci - cr
                    kf[m, B + 2 * H:B + 3 * H, C(n)] = ci + cr
            return Unit("K%d" % n, [(lambda i=i, r=r: (tf_v[r:r + H, C(i)], rhs(i))) for i in range(2) for r in (0, H)],
                        epi, H, 170, nt=True)
        return [unit(m) for m in range(NB)]

    def kv(s, sl):
        def mk(t, w):
            def fn(a):
                ld = lambda o, n: k_n[s][t, pl.ds(8 + w + o, n), :]
                c0 = jnp.concatenate([_tie(ld(0, 8), a), ld(8, 8)], axis=0).reshape(2, 8, 128)
                c1, c2 = ld(-1, 16).reshape(2, 8, 128), ld(-2, 16).reshape(2, 8, 128)
                s0, s1, s2, s3 = (taps[i, :, C(t)] for i in range(4))
                ke, ko, ke1, ko1, ko2 = _lo(c0), _hi(c0), _lo(c1), _hi(c1), _hi(c2)
                wv = v_n[s][t, w:w + 16, :].reshape(2, 8, 128)
                kve = ((s0 * ke + s1 * ko1) + (s2 * ke1 + s3 * ko2)) * _lo(wv)
                kvo = ((s0 * ko + s1 * ke) + (s2 * ko1 + s3 * ke1)) * _hi(wv)
                kv_v[pl.ds(sl * T + w, 16), C(t)] = kve.reshape(16, 128).astype(BF16)
                kv_v[pl.ds(sl * T + H + w, 16), C(t)] = kvo.reshape(16, 128).astype(BF16)
            return fn
        return [[mk(t, w) for w in range(0, H, 16)] for t in range(NT)]

    def mmU(name, sl, us):
        def unit(n):
            def epi(p):
                er, ei, or_, oi = p
                for h, (cr, ci) in enumerate(((er + or_, ei + oi), (er - or_, ei - oi))):
                    B = h * 3 * H
                    uf[us, B:B + H, C(n)] = cr + ci
                    uf[us, B + H:B + 2 * H, C(n)] = cr
                    uf[us, B + 2 * H:B + 3 * H, C(n)] = ci
            return Unit(name(n), [(lambda i=i, r=r: (tf_v[r:r + H, C(2 + i)], kv_v[pl.ds(sl * T + i * H, H), C(n)]))
                                  for i in range(2) for r in (0, H)], epi, H, 120)
        return [unit(n) for n in range(NT)]

    def cmul(m0, u0, n, h, row, L, a):
        t = []
        for i in range(3):
            Rw = slice((3 * h + i) * H + row, (3 * h + i) * H + row + 8)
            kk = kf[m0:m0 + n, Rw, L]
            if i == 0 and a is not None:
                k0 = _tie(kk[0], a)[None]
                kk = k0 if n == 1 else jnp.concatenate([k0, kk[1:]], axis=0)
            t.append(jnp.sum(kk * uf[u0:u0 + n, Rw, L], axis=0))
        return t[0] - t[2], t[0] + t[1]

    def AR(h, q, row):
        return slice((2 * h + q) * H + row, (2 * h + q) * H + row + 8)

    def mac(n, u0, sl, first=False, part=False):
        def mk(t, rc):
            st, fin = [], []

            def piece(i):
                def fn(a):
                    h, row = i & 1, rc + (i >> 1) * 8
                    zr, zi = cmul(0, u0, n, h, row, C(t), a)
                    if part:
                        zr, zi = zr + acc[0, AR(h, 0, row), C(t)], zi + acc[0, AR(h, 1, row), C(t)]
                    st.append((zr, zi))
                    if h:
                        (pr, pi), (mr, mi) = st[-2:]
                        z = [pr + mr, pi + mi, pr - mr, pi - mi]
                        Rw = lambda q: slice(q * H + row, q * H + row + 8)
                        pv = None if first else [zraw[Rw(q ^ 1), C(t)] for q in range(4)]
                        for q in range(4):
                            zraw[Rw(q), C(t)] = z[q]
                        if not first:
                            z = [z[q] + pv[q] if (q & 1) == (rc < 64) else z[q] - pv[q] for q in range(4)]
                        fin.append(z)
                    if i == 3:
                        for q in range(4):
                            zz_v[pl.ds(sl * 2 * T + q * H + rc, 16), C(t)] = jnp.concatenate(
                                [fin[0][q], fin[1][q]], axis=0).astype(BF16)
                return fn
            if not part:
                return [piece(i) for i in range(4)]
            both = lambda f, g: (lambda a: (f(a), g(None)))
            return [both(piece(0), piece(1)), both(piece(2), piece(3))]
        return [[fn for rc in range(0, H, 16) for fn in mk(t, rc)] for t in range(NT)]

    def pos():
        return [(t, h, row) for t in range(NT) for row in range(0, H, 8) for h in range(2)]

    def ahead(i):
        def mk(t, h, row):
            def fn(a):
                zr, zi = cmul(i + 1, 0, NC, h, row, C(t), a)
                acc[i, AR(h, 0, row), C(t)] = zr
                acc[i, AR(h, 1, row), C(t)] = zi
            return fn
        return [mk(*p) for p in pos()]

    def spread():
        n = NB - NC - 1

        def mk(t, h, row):
            def fn(a):
                p = []
                for i in range(3):
                    Rw = slice((3 * h + i) * H + row, (3 * h + i) * H + row + 8)
                    u = uf[0, Rw, C(t)]
                    p.append(kf[1:1 + n, Rw, C(t)] * (_tie(u, a) if i == 0 else u)[None])
                acc[0:n, AR(h, 0, row), C(t)] = acc[1:1 + n, AR(h, 0, row), C(t)] + (p[0] - p[2])
                acc[0:n, AR(h, 1, row), C(t)] = acc[1:1 + n, AR(h, 1, row), C(t)] + (p[0] + p[1])
            return fn
        return [mk(*p) for p in pos()]

    def mmI(name, sl, ys):
        def unit(n):
            def epi(p):
                ce, se, co, so = p
                sub = lax.broadcasted_iota(I32, (8, 128), 0)
                c0 = ys * T + H
                y_v[n, ys * T:ys * T + 1, :] = (ce[64:72] - se[0:8])[0:1]
                se = jnp.concatenate([jnp.where(sub == 0, 0.0, se[0:8]), se[8:]], axis=0)
                for d, cc, ss in ((0, ce[0:64], se), (1, co, so)):
                    y_v[n, pl.ds(c0 + d, 64, stride=2), :] = cc + ss
                    lo = cc - ss
                    for i in range(0, 64, 8):
                        y_v[n, pl.ds(c0 - d - 2 * i - 14, 8, stride=2), :] = jnp.take_along_axis(
                            lo[i:i + 8], 7 - sub, axis=0)
            return Unit(name(n), [(lambda i=i: (tg_v[0:(GR if i == 0 else 64), C(i)], zz_v[pl.ds(sl * 2 * T + i * H, H), C(n)]))
                                  for i in range(4)], epi, 64, 52)
        return [unit(n) for n in range(NT)]

    def mod(name, a, b):
        def unit(n):
            def epi(p):
                v = [_sum(p[i * NT:(i + 1) * NT])[0:8] for i in range(b - a)]
                if a == 0:
                    mod_v[0, :, C(n)] = v[0] * v[2]
                    mod_v[1, :, C(n)] = (v[1] + 1.0) * v[2]
                elif a == 3:
                    mod_v[3, :, C(n)] = v[0]
                    mod_v[4, :, C(n)] = v[1] + 1.0
                else:
                    mod_v[5, :, C(n)] = v[0]
                    mod_v[2, :, C(n)] = v[0] * G_POST
            return Unit(name, [(lambda i=i, k=k: (silu_c[:, C(k)], wm_v[a][C(k), pl.ds(i * D + n * 128, 128)]))
                               for i in range(b - a) for k in range(NT)], epi, 16, 10, full=False, acc=b - a == 1)
        return [unit(n) for n in range(NT)]

    HS = (slice(0, 128), slice(128, 256))
    QS = tuple(slice(r, r + 64) for r in range(0, T, 64))

    def tasks(f, due=None, tie=True, n=RG):
        def mk(R):
            def fn(a):
                x = f(R, a if tie else None)
                return Due(x, due) if due else None
            return fn
        return [mk(slice(r, r + n)) for r in range(0, T, n)]

    def load_y(sl, R):
        return jnp.concatenate([y_v[t, sl * T + R.start:sl * T + R.stop, :] for t in range(NT)],
                               axis=1).reshape(2, 8, D)

    def put(nn, ss, R, x):
        nn[R, :] = x.astype(BF16)
        tok = x
        if ss is not None:
            S2 = pl.ds(R.start // 32 * 16, 16)
            if R.stop % 32:
                top_v[S2, 0:2 * T] = x[:, 0:2 * T]
            else:
                if R.start % 32:
                    x = jnp.concatenate([top_v[S2, 0:2 * T], x[:, 0:2 * T]], axis=0)
                ss[S2, 0:5 * T] = jnp.concatenate(_lhs_sums(x[:, 0:T], x[:, T:2 * T]), axis=1).astype(BF16)
        return tok

    def front(sl, xs, early=False, ss=None):
        xx, hh, nn = view(x_v, xs), view(hb_v, xs), view(n1_v, sl)

        def fa(R, a):
            q = [q_n[sl][t, R.start // 2:R.stop // 2, :] for t in range(NT)]
            q = jnp.concatenate([_tie(q[0], a)] + q[1:], axis=1)
            q = pltpu.bitcast(q, BF16).astype(F32).reshape(2, 8, D)
            x = (q + (_ln(q) * mod_v[1] + mod_v[0]) * load_y(sl, R)).reshape(RG, D)
            xx[R, :] = x
            if early:
                hh[R, :] = _ln(x)
            return x

        def fb(R, a):
            hb = (_ln(_tie(xx[R, :], a).reshape(2, 8, D)) * mod_v[4] + mod_v[3]).reshape(RG, D)
            hh[R, :] = hb
            return hb

        def fc(R, a):
            hb = _tie(hh[R, :], a)
            if early:
                hb = (hb.reshape(2, 8, D) * mod_v[4] + mod_v[3]).reshape(RG, D)
                hh[R, :] = hb
            return put(nn, ss, R, _ln(hb, G_A))
        if early:
            return tasks(fa), tasks(fc)
        if ss is None:
            return tasks(fa) + tasks(fb) + tasks(fc)
        qf = view(x_v, 2)
        wide = lambda v: jnp.concatenate([v] * NT, axis=1)

        def mean(i, R, x):
            st_v[R, C(i)] = jnp.broadcast_to(jnp.sum(x, axis=-1, keepdims=True) * (1.0 / D), (x.shape[0], 128))

        def centred(src, i, R, a):
            return src[R, :] - wide(_tie(st_v[R, C(i)], a))

        def scale(src, i, g):
            def f(R, a):
                st_v[R, C(i + 1)] = jnp.broadcast_to(_rstd(centred(src, i, R, a), g), (RG, 128))
            return f

        def normed(src, i, R, a):
            return centred(src, i, R, a) * wide(st_v[R, C(i + 1)])

        def s1(R, a):
            q = [q_n[sl][t, R.start // 2:R.stop // 2, :] for t in range(NT)]
            q = pltpu.bitcast(jnp.concatenate([_tie(v, a) for v in q], axis=1), BF16).astype(F32)
            qf[R, :] = q
            mean(0, R, q)

        def s3(R, a):
            h = normed(qf, 0, R, a).reshape(2, 8, D) * mod_v[1] + mod_v[0]
            x = qf[R, :] + (h * load_y(sl, R)).reshape(RG, D)
            xx[R, :] = x
            mean(2, R, x)

        def s5(R, a):
            hb = (normed(xx, 2, R, a).reshape(2, 8, D) * mod_v[4] + mod_v[3]).reshape(RG, D)
            hh[R, :] = hb
            mean(4, R, hb)
        s7 = [f for g in tasks(lambda R, a: put(nn, ss, R, normed(hh, 4, R, a)), n=32) for f in (g, lambda a: None)]
        st = [tasks(s3), tasks(scale(xx, 2, 1.0)), tasks(s5), tasks(scale(hh, 4, G_A)), s7]
        if "S" in V:
            return cat(st), [], tasks(s1) + tasks(scale(qf, 0, 1.0))
        if "Q" in V:
            p = [tasks(s1), tasks(scale(qf, 0, 1.0))]
            return cat(x[:8] for x in st), cat(x[8:] for x in p + st), cat(x[:8] for x in p)
        return cat(x[:8] for x in st), cat(x[8:] for x in st), tasks(s1) + tasks(scale(qf, 0, 1.0))

    def shift(hs, sl, pieces=((0, 64), (64, 64), (128, 64), (192, 64)), ss=None):
        gg = view(g_v, sl)

        def one_tile(t, r, n, a):
            lane = lax.broadcasted_iota(I32, (n, 128), 1)
            ld = lambda d: h1_v[t, pl.ds(hs * T + 8 + r + d, n), :]
            if t == 0:
                g = ld(-1)
            elif t == 1:
                g = jnp.where(lane < 32, ld(-1), ld(1))
            elif t == 2:
                g = jnp.where(lane < 64, ld(1), ld(-2))
            elif t == 3:
                g = jnp.where(lane < 96, ld(-2), ld(2))
            else:
                g = ld(2)
            if a is not None:
                g = jnp.concatenate([_tie(g[i:i + 8], a) if i % 16 == 0 else g[i:i + 8]
                                     for i in range(0, n, 8)], axis=0)
            gg[r:r + n, C(t)] = g.astype(BF16)
            return g

        def mk(ts, r, n):
            def fn(a):
                g = [one_tile(t, r, n, a) for t in ts]
                if len(ts) == 2:
                    for i, x in enumerate(_lhs_sums(*g)):
                        ss[r // 2:(r + n) // 2, C(2 * i + ts[0])] = x.astype(BF16)
            return fn
        sets = [(t,) for t in range(NT)] if ss is None else [(0, 2), (1, 3), (4,)]
        return [mk(ts, r, n) for ts in sets for r, n in pieces]

    def shift_early():
        def keep(a):
            h1_v[:, 2 * T - 32:2 * T + 8, :] = h1_v[:, 3 * T - 32:3 * T + 8, :]
        return shift(2, 0, [(r, 32) for r in range(0, T - 32, 32)], gs) + [keep]

    def ln2(xs, sl, fast=True):
        xx, nn, ss = view(x1_v, xs), view(n2_v, sl), view(n2s, sl, H) if fast else None
        f = lambda R, a: put(nn, ss, R, _ln(_tie(xx[R, :], a), G_A))
        ts = tasks(f, DL, False)
        return ts[0::2] + ts[1::2] if fast else tasks(f)

    def resid(xs, x1s, rotate=False):
        xx, x1 = view(x_v, xs), view(x1_v, x1s)

        def f(R, a):
            gb = mod_v[5] if a is None else pltpu.bitcast(
                pltpu.bitcast(mod_v[5], U32) | jnp.concatenate([a] * NT, axis=1), F32)
            r_v[R, :] = xx[R, :] + (x1[R, :].reshape(2, 8, D) * gb).reshape(RG, D)
            if rotate:
                xx[R, :] = x_v[R, :]
                view(hb_v, 1)[R, :] = hb_v[R, :]
        return tasks(f)

    KD, KF, ND = [(0, 2), (1, 3)], [(2 * i, 2 * i + 1) for i in range(6)], [(1, 2), (3, 4)]
    Wt = {1: (lambda k, n: w1_v[C(k), C(n)], lambda i, kp, j: w1s[C(kp), C(2 * i + j)], False, KD, [4]),
          2: (lambda k, n: w2_v[C(k), C(n)], lambda i, kp, j: w2s[C(kp), C(2 * i + j)], False, KD, [4]),
          0: (lambda k, n: w3_v[C(n), C(k)], None, True, KD, [4]),
          3: (lambda k, n: w3n[C(k), C(n)], lambda i, kp, j: w3s[C(kp), C(6 * i + j)], False, KD, [4]),
          4: (lambda k, n: w4_v[C(k, F), C(n)], lambda i, kp, j: w4s[C(kp), C(2 * i + j)], False, KF, [12, 13])}

    def wsums(w_w, ws, rp, cp_):
        def mk(i, j, r):
            def fn(a):
                b = [[w_w[pl.ds(64 * p + r // 2, 8), C(q)] for q in cp_[j]] for p in rp[i]]
                b[0][0], b[1][1] = _tie(b[0][0], a), _tie(b[1][1], a)
                (b11, b12), (b21, b22) = [[pltpu.bitcast(x, BF16).astype(F32) for x in row] for row in b]
                for m, x in enumerate((b11 + b22, b12 - b22, b21 - b11, b11 + b12, b21 + b22)):
                    ws[pl.ds(128 * i + r, 16), C(len(cp_) * m + j)] = x.astype(BF16)
            return fn
        return [mk(i, j, r) for j in range(len(cp_)) for i in range(len(rp)) for r in range(0, 128, 16)]

    def w3_turn():
        def mk(n, k):
            def fn(a):
                x = jnp.concatenate([_tie(w3_w[64 * n:64 * n + 8, C(k)], a), w3_w[64 * n + 8:64 * n + 64, C(k)]], axis=0)
                w3n[C(k), C(n)] = pltpu.bitcast(x, BF16).T
            return fn
        return [mk(n, k) for n in range(FT - 1) for k in range(NT)]

    def plain(name, w, lhs, n, R, epi, cost):
        tile, _, nt, kp, kl = Wt[w]
        ks = sorted([k for p in kp for k in p] + kl)
        rows_ = R.stop - R.start
        return Unit(name, [(lambda k=k: (lhs[R, C(k, F)], tile(k, n))) for k in ks], lambda p: epi(n, R, p[0]),
                    rows_, rows_ // 8 * (len(ks) - 1 + cost), nt=nt, acc=True)

    def quad(name, w, lhs, sums, j, cols_, R, epi, cost):
        tile, wsum, nt, kp, kl = Wt[w]
        h, S2, c = len(kp), slice(R.start // 2, R.stop // 2), {}
        a_ = lambda i, k: _top(lhs[R, C(k, F)], i)
        s_ = lambda i, p: sums[S2, C(h * i + p)]
        prod = lambda fa_, fb_: [(lambda p=p: (fa_(p), fb_(p))) for p in range(h)]
        left = lambda i, n: [(lambda k=k: (a_(i, k), tile(k, n))) for k in kl]
        mk = lambda tiles, f, x=0: Unit(name, tiles, lambda p: f(p[0]), 64, 8 * len(tiles) + x, nt=nt, acc=True)

        def e1(m):
            u7.res, u6.res = [m], [m]

        def e4(m):
            c[11], c[21] = c[11] + m, m

        def e2(m):
            l21.res, c[22] = [c[21] + m], c[22] - m

        def e5(m):
            c[12] = m
            epi(cols_[0], R, _zip(c[11] - m, c[21]))

        def e3(m):
            l12.res, c[22] = [c[12] + m], c[22] + m
        u1 = mk(prod(lambda p: s_(0, p), lambda p: wsum(0, p, j)), e1)
        u7 = mk(prod(lambda p: s_(4, p), lambda p: wsum(4, p, j)) + left(0, cols_[0]), lambda m: c.update({11: m}))
        u6 = mk(prod(lambda p: s_(3, p), lambda p: wsum(3, p, j)) + left(1, cols_[1]), lambda m: c.update({22: m}))
        u4 = mk(prod(lambda p: a_(1, kp[p][1]), lambda p: wsum(2, p, j)), e4)
        u2 = mk(prod(lambda p: s_(1, p), lambda p: tile(kp[p][0], cols_[0])), e2, 8)
        l21 = mk(left(1, cols_[0]), lambda m: c.update({21: m}))
        u5 = mk(prod(lambda p: s_(2, p), lambda p: tile(kp[p][1], cols_[1])), e5, 16 * cost)
        u3 = mk(prod(lambda p: a_(0, kp[p][0]), lambda p: wsum(1, p, j)), e3, 8)
        l12 = mk(left(0, cols_[1]), lambda m: epi(cols_[1], R, _zip(m, c[22])), 16 * cost)
        return [u1, u7, u6, u4, u2, l21, u5, u3, l12]

    def mm(name, w, lhs, sums, epi, cost):
        if sums is None:
            return [[plain(name, w, lhs, n, R, epi, cost) for R in HS] for n in range(NT)]
        return [[plain(name, w, lhs, 0, R, epi, cost) for R in QS]] + [
            [u for R in HS for u in quad(name, w, lhs, sums, j, ND[j], R, epi, cost)] for j in range(2)]

    def mm1(name, hs, sl, fast=False):
        def epi(n, R, p):
            h1_v[n, pl.ds(hs * T + 8 + R.start, R.stop - R.start), :] = _gelu2(p)
        return cat(mm(name, 1, view(n1_v, sl), n1s if fast else None, epi, 5))

    def mm2(name, sl, xs, x1s, fast=False):
        def epi(n, R, p):
            view(x1_v, x1s)[R, C(n)] = view(hb_v, xs)[R, C(n)] + p * G_POST
        return cat(mm(name, 2, view(g_v, sl), gs if fast else None, epi, 2))

    def mm3(name, sl, fast=True):
        nn, aa, ss, keep = view(n2_v, sl), view(a_v, sl), view(a_s, sl, H), []

        def epi(n, R, p):
            g = _gelu2(p)
            aa[R, C(n)] = g.astype(BF16)
            if n < 12 and n % 2:
                for i, x in enumerate(_lhs_sums(keep.pop(), g)):
                    ss[R.start // 2:R.stop // 2, C(6 * i + n // 2)] = x.astype(BF16)
            elif n < 12:
                keep.append(g)

        def rem(R):
            def f(p):
                aa[R, 13 * 128:F] = _gelu2(p[0]).T.astype(BF16)
            return Unit(name, [(lambda k=k: (w3_v[13 * 128:F, C(k)], nn[R, C(k)])) for k in range(NT)], f, 64, 84,
                        nt=True, acc=True)
        odd = [rem(R) for R in HS] + [plain(name, 3 if fast else 0, nn, 12, R, epi, 6) for R in QS]
        if fast:
            return odd + [u for j in range(6) for R in HS
                          for u in quad(name, 3, nn, view(n2s, sl, H), j, KF[j], R, epi, 8)]
        return odd + [plain(name, 0, nn, n, R, epi, 8) for p in KF for R in HS for n in p]

    NA = 3 * 128

    def cp_out(j, osl, L, sm, R=slice(0, T)):
        return cp(o_v.at[pl.ds(osl * T + R.start, R.stop - R.start), L],
                  o_hbm.at[pl.ds(base(j, T) + R.start, R.stop - R.start), L], sem_o.at[sm])

    out_a = lambda j: cp_out(j, 0, slice(0, NA), 0)
    out_b = lambda j: cp_out(j, 0, slice(NA, D), 1)
    last = []

    def mm4(name, j, sl, osl=0, xs=None, x1s=None, fast=True):
        oo = view(o_v, osl)

        def epi(n, R, p):
            if xs is None:
                oo[R, C(n)] = (r_v[R, C(n)] + mod_v[2, 0:1, C(n)] * p).astype(BF16)
            else:
                oo[R, C(n)] = (view(x_v, xs)[R, C(n)] + mod_v[5, 0:1, C(n)]
                               * (view(x1_v, x1s)[R, C(n)] + p * G_POST)).astype(BF16)
            if osl == 2:
                last.append(cp_out(j, osl, C(n), 2, R))
                last[-1].start()
            elif R.stop == T and (osl, (n + 1) * 128) in ((1, D), (3, NA)):
                last.append(cp_out(j, osl, slice(0, (n + 1) * 128), 2))
                last[-1].start()
            elif R.stop == T and osl == 0 and (n + 1) * 128 in (NA, D):
                (out_a if (n + 1) * 128 == NA else out_b)(j).start()
        return mm(name, 4, view(a_v, sl), view(a_s, sl, H) if fast else None, epi, 3 if xs is None else 5)

    def split(us):
        n = 4 // len(us)
        m, mks, st = us[0].rows // n, [u.tiles.pop(0) for u in us], {}

        def piece(i, k):
            if i not in st:
                st[i] = mks[i]()
            return st[i][0][m * k:m * (k + 1)], st[i][1]

        def epi(p):
            for i, u in enumerate(us):
                u.res = [jnp.concatenate(p[n * i:n * (i + 1)], axis=0)]
        return _flat([Unit(us[0].name, [(lambda i=i, k=k: piece(i, k)) for i in range(len(us)) for k in range(n)],
                           epi, m, 0, nt=us[0].nt)])

    W = lambda nm: [("wait", nm)]
    run = lambda fns: [("run", "run", lambda: [fn(None) for fn in fns])]
    one = lambda us: [_flat([u]) for u in us]
    nm = lambda x: (lambda n: x)

    seq, grp = [], []
    for s in range(NC):
        seq += W("c%d" % s) + _flat(mmK(s) + mmU(nm("U%d" % s), s % 2, NC - 1 - s))
        grp.append(Group("kv%d" % s, cat(kv(s, s % 2)), 50, ["c%d" % s], ["U%d" % s], 100))
    inv = [mmI(lambda n: "I%d" % n, s, s) for s in range(NC)]
    seq += W("c3") + _flat(mmK(3) + mmK(4) + [inv[s][t] for t in range(NT) for s in range(NC)])
    macs = [mac(s + 1, NC - 1 - s, s, first=s == 0) for s in range(NC)]
    grp.append(Group("mac00", macs[0][0], 12, ["c1"], ["c2"], 0))
    grp.append(Group("mac01", macs[1][0] + macs[0][1] + macs[1][1], 16, ["c2"], ["c3"], 0))
    for t in range(NT):
        grp.append(Group("mac%d" % t, cat(macs[s][t] for s in range(2 if t < 2 else 0, NC)), 24 if t < 2 else 18,
                         ["c3", "K%d" % t], ["I%d" % t], 100, 150))
    start = lambda cs: [("run", "run", lambda: [c.start() for c in cs])]
    f0, f1 = front(0, 2, True), front(1, 1, True)
    seq += run(ahead(0))
    seq += W("wma") + _flat(mod("moda", 0, 3)) + run(f0[0] + f1[0] + ahead(1))
    seq += W("wmb") + start(next_kv(NC) + next_q(NC)) + _flat(mod("modb", 3, 5)) + run(f0[1])
    w1 = _flat(mm1("w1_0", 0, 0) + mm1("w1_1", 1, 1))
    seq += W("w1") + w1[:LP[4]] + W("w2") + w1[LP[4]:] + run(shift(0, 0))
    seq += _flat(mm2("w2_0", 0, 2, 1) + mm1("w1_2", 2, 2)) + run(shift(1, 1)) + _flat(mm2("w2_1", 1, 1, 0))
    grp.append(Group("f1", f1[1], 80, ["w1"], ["w1_1"], 450))
    grp.append(Group("f2", front(2, 0), 80, ["w2"], ["w1_2"], 450))
    grp.append(Group("ln2_0", ln2(1, 0, False), 60, ["w2_0"], ["w3"], 450))
    grp.append(Group("ahead", cat(ahead(i) for i in range(2, NB - NC)), 19, ["w1"], ["end"], 100))
    grp.append(Group("ws1", wsums(w1_w, w1s, KD, ND), 26, ["w1"], ["end"], 100))
    grp.append(Group("ws2", wsums(w2_w, w2s, KD, ND), 26, ["w2"], ["end"], 100))
    grp.append(Group("ws3", w3_turn() + wsums(w3n_w, w3s, KD, KF), 22, ["w3"], ["end"], 100))
    grp.append(Group("ws4", wsums(w4_w, w4s, KF, ND), 26, ["w4"], ["end"], 100))
    _wait(seq, "w3", back=1)
    w3 = mm3("w3_0", 0, False)
    _mix(seq, _flat(w3[6:]), [split(w3[4:6]) + _flat(w3[:6])], 0.1)
    mc = _flat(mod("modc", 5, 6))
    _wait(seq, "w4", mc[:5] + [("sync", "run", lambda: None)])
    w4 = cat(mm4("w4_0", 0, 0, 3, 2, 1, False)[:3])
    qs = [split([w4[-1 - i]]) for i in range((_phase(seq) + FT * 6) % 4)]
    _mix(seq, _flat(w4), [mc[i:i + 4] for i in range(5, 25, 4)] + qs, 0.01, 0.4)
    assert _phase(seq) == 0
    grp.append(Group("resid", resid(2, 1), 26, ["modc"], ["end"], 100))
    _emit(seq, grp, zero, wait)

    def step(s, carry):
        for c in next_kv(s) + next_q(s):
            c.wait()
        nxt = jnp.minimum(s + 1, NB - 1)
        seq, grp = [], []
        us, it = one(mmU(lambda n: "U%d" % n, 0, 0)), one(mmI(lambda n: "I%d" % n, 0, 0))
        w4 = mm4("w4", s - 2, 0)
        q = split(w4[0][2:])
        _mix(seq, _flat(mm4("w4c", s - 3, 0)[2] + mm3("w3", 0)),
             [us[0], us[1], us[2], it[0] + us[3], it[1] + us[4], it[2] + start(next_kv(nxt)), it[3], it[4]],
             LP[3], LP[0])
        w1a, w1b = mm1("w1a", 2, 0, True), mm1("w1b", 2, 0, True)
        w1a, w1b = _flat(w1a[0:2] + w1a[4:13] + w1a[22:31]), _flat(w1b[2:4] + w1b[13:22] + w1b[31:])
        _mix(seq, _flat(w4[0] + w4[1][:9]), [q])
        if "S" in V:
            seq += _flat(w4[1][9:]) + w1a + run(shift(1, 0, ((T - 32, 32),), gs)) + w1b[:8] + start(next_q(nxt)) + w1b[8:]
        else:
            seq += w1a + run(shift(1, 0, ((T - 32, 32),), gs)) + _flat(w4[1][9:]) + w1b[:8] + start(next_q(nxt)) + w1b[8:]
        seq += _flat(mm2("w2", 0, 1, 0, True))
        assert _phase(seq) == 0
        kvs, macs = kv(0, 0), mac(1, 0, 0, part=True)
        for t in range(NT):
            grp.append(Group("kv%d" % t, kvs[t], 50, ["start"], ["U%d" % t], 300))
            grp.append(Group("mac%d" % t, macs[t], 28, ["U%d" % t], ["I%d" % t], 300, 150))
        iall = ["I%d" % t for t in range(NT)]
        grp.append(Group("ln2", ln2(0, 0), 75, ["start"], ["w3"], 450))
        grp.append(Group("resid", resid(1, 0, True), 40, ["w4c"], ["w4", "I4"], 100))
        fr = front(0, 0, ss=n1s)
        grp.append(Group("fronta", fr[0], 50, iall, ["w1a"], FL))
        if fr[1]:
          grp.append(Group("frontb", fr[1], 50, iall, ["w1b"], FL, RL))
        grp.append(Group("fq", fr[2], 34, ["w4c"], ["I4"], 100))
        grp.append(Group("spread", spread(), 30, iall, ["end"], 100))
        grp.append(Group("shift", shift_early(), 24, ["start"], ["w1a"], 200))
        _emit(seq, grp, zero, wait)
        out_b(s - 3).wait()
        out_a(s - 2).wait()
        return carry

    lax.fori_loop(NC, NB, step, 0)

    seq, grp = [], []
    seq += _flat(mm4("w4_5", NB - 3, 0)[2] + mm3("w3_6", 0) + mm2("w2_7", 0, 0, 1, True)
                 + cat(mm4("w4_6", NB - 2, 0, 1, 1, 0)) + mm3("w3_7", 1) + cat(mm4("w4_7", NB - 1, 1, 2, 0, 1)))
    assert _phase(seq) == 0
    grp.append(Group("ln2_6", ln2(0, 0), 75, ["start"], ["w3_6"], 450))
    grp.append(Group("shift7", shift(2, 0, [(r, 32) for r in range(0, T, 32)], gs), 24, ["start"], ["w2_7"], 200))
    grp.append(Group("ln2_7", ln2(1, 1), 75, ["w2_7"], ["w3_7"], 450))
    _emit(seq, grp, zero, wait)
    for c in next_kv(NB - 1) + next_q(NB - 1) + [out_b(NB - 3)] + last:
        c.wait()


@jax.jit
def pallas_adaLN_cond__ssm_conv_h3__mixer_s_mlp__prompt_kernel(
        A_q, A_k, A_v, A_shift_k, A_ssm_k, A_ssm_D, B_x, B_w1, B_w2, B_w3, B_w4, c, w_mod):
    any_ = pl.BlockSpec(memory_space=pl.ANY)
    V = pltpu.VMEM
    out = pl.pallas_call(
        kernel,
        in_specs=[any_] * 12,
        out_specs=any_,
        out_shape=jax.ShapeDtypeStruct((S, D), BF16),
        scratch_shapes=[
            [V((NT, H + 8, 128), U32)] * NC, [V((NT, H + 8, 128), U32)] * NC, [V((NT, H + 8, 128), U32)] * NC,
            [V((64, S), U32)] * NT,
            V((D // 2, D), U32), V((D // 2, D), U32), V((F // 2, D), U32), V((F // 2, D), U32),
            [V((D // 2, 3 * D), U32), V((D // 2, 2 * D), U32), V((D // 2, D), U32)], V((4 * T, D), BF16),
            V((4, D), BF16), V((D,), BF16), V((1, D), BF16), V((8, 128), I32), pltpu.SMEM((8, 128), I32),
            V((5, 8, D), F32), V((6, 8, D), F32), V((T // 2, 4 * H), U32), V((GR // 2, 2 * T), U32),
            V((NB, 3 * T + 8, D), F32), V((NC, 3 * T + 8, D), F32), V((NB - NC, 2 * T + 8, D), F32), V((2 * T, D), F32),
            V((T, D), U32), V((NC * T, D), U32), V((NT, NC * T + 8, 128), F32),
            V((3 * T, D), F32), V((3 * T, D), F32), V((2 * T, D), F32), V((T, D), F32),
            V((3 * T // 2, D), U32), V((T, D), U32), V((T, D), U32), V((NT, NC * T + 24, 128), F32),
            V((T, (FT + 1) * 128), U32),
            [V((128, 11 * 128), U32)] * 2 + [V((128, 31 * 128), U32), V((384, 11 * 128), U32)],
            [V((64, 11 * 128), U32)] * 2 + [V((128, 11 * 128), U32), V((128, 31 * 128), U32)],
            V((D // 2, 13 * 128), U32), V((H, D), F32), V((T, 7 * 128), F32),
            pltpu.SemaphoreType.DMA((11,)), pltpu.SemaphoreType.DMA((1,)), pltpu.SemaphoreType.DMA((3,)),
        ],
        compiler_params=pltpu.CompilerParams(vmem_limit_bytes=110 << 20, disable_semaphore_checks=True,
                                             disable_bounds_checks=True),
        name="fused",
    )(A_q[0], A_k[0], A_v[0], A_shift_k.T, A_ssm_k, A_ssm_D, B_w1, B_w2, B_w3.T, B_w4, c, w_mod)
    return out[None]
```

```python
import heapq
import os
import numpy as np
import jax
import jax.numpy as jnp
from jax import lax
from jax.experimental import pallas as pl
from jax.experimental.pallas import tpu as pltpu

S, D, F = 2048, 640, 1728
T = 256
H = T // 2
NB = S // T
NT = D // 128
FT = (F + 127) // 128
EPS = 1e-5
F32, BF16, U32, I32 = jnp.float32, jnp.bfloat16, jnp.uint32, jnp.int32
G_C1 = 0.044715 * float(np.sqrt(2.0 / np.pi))
G_C2 = float(np.sqrt(2.0 / np.pi))
G_A = G_C1 ** (1.0 / 3.0)
G_B = G_C2 / G_A
G_POST = 0.5 / G_A
RG = 16
GR = 80
NC = 3
DL = int(os.environ.get('DL', 450))
V = os.environ.get('V', 'Q')
FL = int(os.environ.get('FL', 330))
RL = int(os.environ.get('RL', 2000))
DA = int(os.environ.get('DA', 650))
SLOT = 32
LP = (float(os.environ.get('LP0', 0.78)), 4, 6, float(os.environ.get('LP3', 0.2)), 72)


def _dft(shape, f_axis, tau, scale=1.0):
    r = lax.broadcasted_iota(I32, shape, f_axis)
    l = lax.broadcasted_iota(I32, shape, 1 - f_axis)
    f = r & 127
    odd = ((f & 63) << 2) | ((f >> 6) << 1) | 1
    p = odd * tau(l) + ((r >> 7) << 8)
    a = ((p + 512) & 1023) - 512
    u = (256 - jnp.abs(a)).astype(F32) * (np.pi / 512.0)
    u2 = u * u
    c = [scale, -scale / 6.0, scale / 120.0, -scale / 5040.0, scale / 362880.0, -scale / 39916800.0]
    poly = c[5]
    for ci in c[4::-1]:
        poly = poly * u2 + ci
    return (u * poly).astype(BF16)


def _rstd(xc, scale):
    s2 = 1.0 / (scale * scale)
    v = jnp.sum(xc * xc, axis=-1, keepdims=True) * (s2 / D) + EPS * s2
    return jnp.exp2(jnp.log(v) * float(-0.5 / np.log(2.0)))


def _ln(x, scale=1.0):
    xc = x - jnp.sum(x, axis=-1, keepdims=True) * (1.0 / D)
    return xc * _rstd(xc, scale)


def _gelu2(x):
    u = x * (x * x + G_B)
    return x * (1.0 + jnp.tanh(u))


def _lo(w):
    return pltpu.bitcast(w << 16, F32)


def _hi(w):
    return pltpu.bitcast(w & jnp.uint32(0xFFFF0000), F32)


def _tie(x, a):
    if a is None:
        return x
    w = pltpu.bitcast(x[:, :128], U32)
    k = w.shape[0] // 8
    w = w | (a if k == 1 else jnp.concatenate([a] * k, axis=0))
    w = pltpu.bitcast(w, x.dtype)
    return w if x.shape[1] == 128 else jnp.concatenate([w, x[:, 128:]], axis=1)


def _top(x, i):
    return jnp.concatenate([x[r:r + 16] for r in range(16 * i, x.shape[0], 32)], axis=0)


def _zip(t, b):
    return jnp.concatenate([x[r:r + 16] for r in range(0, t.shape[0], 16) for x in (t, b)], axis=0)


def _lhs_sums(x1, x2):
    a11, a21, a12, a22 = _top(x1, 0), _top(x1, 1), _top(x2, 0), _top(x2, 1)
    return [a11 + a22, a21 + a22, a11 + a12, a21 - a11, a12 - a22]


def C(i, lim=1 << 20):
    return slice(i * 128, min((i + 1) * 128, lim))


class Unit:
    def __init__(self, name, tiles, epi, rows, cost, nt=False, full=True, acc=False):
        self.acc, self.res = acc, []
        self.name, self.tiles, self.epi, self.rows, self.cost, self.nt, self.full = name, tiles, epi, rows, cost, nt, full


class Due:
    def __init__(self, val, delay):
        self.val, self.delay = val, delay


class Group:
    def __init__(self, name, fns, cost, rel, dead, lat, rlat=200):
        self.name, self.fns, self.cost, self.rel, self.dead, self.lat, self.rlat = name, fns, cost, rel, dead, lat, rlat


def _plan(seq, groups):
    busy, n = [0] * 4, 0
    start, end, tiles, bars = {}, {}, [], []
    for it in seq:
        if isinstance(it[0], Unit):
            u = it[0]
            m = n % 4
            n += 1
            t0, t1 = busy[m], busy[m] + max(u.rows, 32)
            busy[m] = t1
            tiles.append((t0, t1, u.cost / len(u.tiles)))
            start.setdefault(u.name, t0)
            end[u.name] = max(end.get(u.name, 0), t1)
        elif it[0] == "wait":
            t = max(busy)
            busy, n = [t] * 4, 0
            start[it[1]] = end[it[1]] = t
            bars.append(t)
    total = max(busy)
    start["end"] = end["end"] = total
    start["start"] = end["start"] = 0
    ns = total // SLOT + 2
    load = np.zeros(ns)
    for t0, t1, c in tiles:
        a, b = t0 // SLOT, max(t1 // SLOT, t0 // SLOT + 1)
        load[a:b] += c / (b - a)
    win = []
    for g in groups:
        r = max(end[x] + (0 if start[x] == end[x] else g.rlat) for x in g.rel)
        d = min(start[x] for x in g.dead) - g.lat
        ok = np.zeros(ns, bool)
        ok[r // SLOT:max(d // SLOT, r // SLOT + 1)] = True
        for b in bars:
            if r < b <= d:
                ok[max((b - g.lat) // SLOT, 0):b // SLOT] = False
        win.append(np.nonzero(ok)[0])
    alloc = [np.zeros(len(w)) for w in win]
    for _ in range(60):
        for i, g in enumerate(groups):
            w = win[i]
            load[w] -= alloc[i]
            base = load[w]
            vol = g.cost * len(g.fns)
            lo, hi = base.min(), base.max() + vol
            for _ in range(50):
                mid = 0.5 * (lo + hi)
                if np.maximum(mid - base, 0).sum() > vol:
                    hi = mid
                else:
                    lo = mid
            alloc[i] = np.maximum(hi - base, 0)
            load[w] += alloc[i]
    times = []
    for i, g in enumerate(groups):
        cum = np.cumsum(alloc[i])
        ts = []
        for k in range(len(g.fns)):
            x = (k + 0.5) * cum[-1] / len(g.fns)
            j = int(np.searchsorted(cum, x))
            prev = cum[j - 1] if j else 0.0
            ts.append(win[i][j] * SLOT + SLOT * (x - prev) / max(alloc[i][j], 1e-9))
        times.append(ts)
    return times


def _emit(seq, groups, zero, wait):
    times = _plan(seq, groups)
    left = {"start": 0}
    for it in seq:
        nm = it[0].name if isinstance(it[0], Unit) else it[1]
        left[nm] = left.get(nm, 0) + 1
    heap, pend, todo, cnt = [], {}, list(range(len(groups))), 0
    busy, n, due = [0] * 4, 0, []

    def release():
        nonlocal cnt
        for i in list(todo):
            g = groups[i]
            if all(left[x] == 0 for x in g.rel):
                todo.remove(i)
                pend[i] = len(g.fns)
                for t, fn in zip(times[i], g.fns):
                    heapq.heappush(heap, (t, cnt, i, fn))
                    cnt += 1

    def force(name):
        nonlocal heap
        for i, g in enumerate(groups):
            if name in g.dead:
                assert i not in todo, (g.name, name)
                if pend[i]:
                    for it in sorted(x for x in heap if x[2] == i):
                        it[3](None)
                    heap = [x for x in heap if x[2] != i]
                    heapq.heapify(heap)
                    pend[i] = 0

    release()
    for it in seq:
        if isinstance(it[0], Unit):
            u, k = it
            force(u.name)
            lhs, rhs = u.tiles[k]()
            t0 = busy[n % 4]
            while u.full and due and due[0][0] < t0 + u.rows:
                t, x = due.pop(0)
                r = min(max(int(t - t0), 0), u.rows - 1) // 16 * 8
                if lhs.shape[1] != 128:
                    due.insert(0, (t, x))
                    break
                w = pltpu.bitcast(lhs, U32)
                x = pltpu.bitcast(x[:, :128], U32)
                parts = [w[:r], w[r:r + 8] | ((x[0:8] | x[8:16]) & zero), w[r + 8:]]
                lhs = pltpu.bitcast(jnp.concatenate([y for y in parts if y.shape[0]], axis=0), BF16)
            dn = (((1,), (1 if u.nt else 0,)), ((), ()))
            p = lax.dot_general(lhs, rhs, dn, preferred_element_type=F32)
            u.res = [p + u.res[0]] if (u.acc and u.res) else u.res + [p]
            m = n % 4
            n += 1
            t0 = busy[m]
            busy[m] = t0 + max(u.rows, 32)
            while u.full and heap and heap[0][0] < t0 + u.rows:
                t, _, i, fn = heapq.heappop(heap)
                pend[i] -= 1
                r = min(max(int(t - t0), 0), u.rows - 1) // 8 * 8
                x = fn(pltpu.bitcast(p[r:r + 8], U32) & zero)
                if isinstance(x, Due):
                    due.append((t + x.delay, x.val))
                    due.sort(key=lambda e: e[0])
            if k == len(u.tiles) - 1:
                u.epi(u.res)
            left[u.name] -= 1
        elif it[0] == "wait":
            force(it[1])
            wait(it[1])
            busy, n, due = [max(busy)] * 4, 0, []
            left[it[1]] -= 1
        else:
            it[2]()
            left[it[1]] -= 1
        release()
    force("end")
    assert not heap and not todo


def _sum(ps):
    acc = ps[0]
    for p in ps[1:]:
        acc = acc + p
    return acc


def _flat(us):
    return [(u, i) for u in us for i in range(len(u.tiles))]


def _phase(seq):
    n = 0
    for it in seq:
        n = n + 1 if isinstance(it[0], Unit) else (0 if it[0] in ("wait", "sync") else n)
    return n % 4


def _mix(seq, a, b, lo=0.0, hi=1.0):
    n, k = _phase(seq), 0
    for i, t in enumerate(a):
        if k < len(b) and n % 4 == 0 and t[1] != 1 and i >= len(a) * (lo + (hi - lo) * k / len(b)):
            seq.extend(b[k])
            k += 1
        seq.append(t)
        n += 1
    assert k == len(b)


def _wait(seq, name, head=(), back=0):
    r = _phase(seq) + 4 * back
    assert all(isinstance(it[0], Unit) for it in seq[len(seq) - r:])
    seq[len(seq) - r:len(seq) - r] = [("wait", name)] + list(head)


def kernel(q_hbm, k_hbm, v_hbm, sh_hbm, ssm_hbm, sd_hbm, w1_hbm, w2_hbm, w3_hbm, w4_hbm, c_hbm, wm_hbm,
           o_hbm,
           q_n, k_n, v_n, ssm_w, w1_w, w2_w, w3_w, w4_w, wm_w, o_v,
           sh_v, sd_v, c_v, zsrc, z_s, taps, mod_v, tf_w, tg_w,
           kf, uf, acc, zraw, kv_w, zz_w, y_v, x_v, hb_v, x1_v, r_v, n1_w, n2_w, g_w, h1_v, a_w,
           ws_w, as_w, w3n_w, top_v, st_v,
           sem, sem_b, sem_o):
    bf = lambda r: r.bitcast(BF16)
    w1_v, w2_v, w3_v, w4_v = bf(w1_w), bf(w2_w), bf(w3_w), bf(w4_w)
    wm_v = {0: bf(wm_w[0]), 3: bf(wm_w[1]), 5: bf(wm_w[2])}
    tf_v, tg_v, n1_v, n2_v, g_v = bf(tf_w), bf(tg_w), bf(n1_w), bf(n2_w), bf(g_w)
    a_v, kv_v, zz_v = bf(a_w), bf(kv_w), bf(zz_w)
    w1s, w2s, w3s, w4s = [bf(r) for r in ws_w]
    n1s, gs, n2s, a_s = [bf(r) for r in as_w]
    w3n = bf(w3n_w)
    cp = pltpu.make_async_copy
    cat = lambda ls: [x for l in ls for x in l]

    def base(j, n):
        return j * n if isinstance(j, int) else pl.multiple_of(j * n, n)

    def rows(j, n=1, size=T):
        return pl.ds(base(j, size), n * size)

    def view(ref, j, size=T):
        return ref.at[rows(j, 1, size)]

    dmas = {}

    def group(name, *mks):
        sm = sem.at[len(dmas)]
        dmas[name] = [c for mk in mks for c in mk(sm)]

    def ssm_in(t):
        return lambda sm: [cp(ssm_hbm.at[C(t)], bf(ssm_w[t]), sm)]

    def cols(src, start, n, dst, row=0):
        return lambda sm: [cp(src.at[pl.ds(start, n), C(t)], bf(dst).at[t, pl.ds(row, n)], sm) for t in range(NT)]

    def kv_in(s, sl):
        if isinstance(s, int):
            kk = cols(k_hbm, s * T - 16, T + 16, k_n[sl]) if s else cols(k_hbm, 0, T, k_n[sl], 16)
        else:
            kk = cols(k_hbm, pl.multiple_of(s * T - 16, 16), T + 16, k_n[sl])
        return lambda sm: kk(sm) + cols(v_hbm, base(s, T), T, v_n[sl])(sm)

    def q_in(s, sl):
        return cols(q_hbm, base(s, T), T, q_n[sl])

    def wm_in(a, b):
        return lambda sm: [cp(wm_hbm.at[:, a * D:b * D], wm_v[a], sm)]

    def whole(src, dst):
        return lambda sm: [cp(src, dst, sm)]

    next_kv = lambda s: kv_in(s, 0)(sem_b.at[0])
    next_q = lambda s: q_in(s, 0)(sem_b.at[0])

    zsrc[...] = jnp.zeros((8, 128), I32)
    k_n[0][:, 0:8, :] = jnp.zeros((NT, 8, 128), U32)
    w4_w[F // 2:FT * 64, :] = jnp.zeros((FT * 64 - F // 2, D), U32)
    group("small", lambda sm: [cp(zsrc, z_s, sm), cp(sh_hbm, sh_v, sm), cp(sd_hbm, sd_v, sm), cp(c_hbm, c_v, sm)])
    for s in range(NC):
        group("c%d" % s, ssm_in(s), kv_in(s, s))
    group("c3", ssm_in(3), ssm_in(4))
    group("wma", wm_in(0, 3), q_in(0, 0), q_in(1, 1))
    group("wmb", wm_in(3, 5))
    group("w1", whole(w1_hbm, w1_v))
    group("w2", q_in(2, 2), whole(w2_hbm, w2_v))
    group("w3", whole(w3_hbm, w3_v))
    group("w4", whole(w4_hbm, w4_v.at[0:F]), wm_in(5, 6))
    for g in dmas.values():
        for c in g:
            c.start()

    def wait(name):
        for c in dmas[name]:
            c.wait()

    tau_b = lambda l: H + ((l + (H - 1)) & (H - 1))
    tf_v[:, C(0)] = _dft((T, H), 0, lambda l: jnp.where((l & 1) == 0, l, tau_b(l)), 1.0 / T)
    tf_v[:, C(1)] = _dft((T, H), 0, lambda l: jnp.where((l & 1) == 1, l, tau_b(l)), 1.0 / T)
    tf_v[:, C(2)] = _dft((T, H), 0, lambda l: 2 * l - H)
    tf_v[:, C(3)] = _dft((T, H), 0, lambda l: 2 * l + 1 - H)
    sin0 = lax.broadcasted_iota(I32, (GR, T), 1) >= H
    tg_v[:, 0:T] = _dft((GR, T), 1, lambda l: jnp.where(sin0 & (l == 0), H, 2 * l))
    tg_v[:, T:2 * T] = _dft((GR, T), 1, lambda l: 2 * l + 1)
    h1_v[:, 0:8, :] = jnp.zeros((NT, 8, 128), F32)
    h1_v[:, 8 + NC * T:16 + NC * T, :] = jnp.zeros((NT, 8, 128), F32)

    wait("small")
    z = jnp.clip(z_s[0, 0], 0, 1)
    zero = jnp.full((8, 128), z, I32).astype(U32)
    z8 = pl.multiple_of(z * 8, 8)
    for r in (x_v, hb_v, x1_v, r_v, zraw, n1_w, n2_w, g_w, a_w, kv_w, zz_w, *ws_w, *as_w, w3n_w, top_v, st_v):
        r[pl.ds(z8, 8), 0:128] = jnp.zeros((8, 128), r.dtype)
    for r in (kf, uf, acc, taps, mod_v):
        r[z, 0:8, 0:128] = jnp.zeros((8, 128), r.dtype)
    for r in (tf_w, tg_w):
        r[pl.ds(z8, 8), 0:128] = r[0:8, 0:128]
    sh = sh_v[...].astype(F32)
    for i in range(4):
        taps[i] = jnp.broadcast_to(sh[i:i + 1], (8, D))
    taps[4] = jnp.broadcast_to(sd_v[...].astype(F32).reshape(1, D) * (1.0 / T), (8, D))
    cf = c_v[...].astype(F32)
    silu_c = jnp.broadcast_to((cf / (1.0 + jnp.exp(-cf))).astype(BF16), (16, D))

    def mmK(n):
        def unit(m):
            st = []

            def rhs(i):
                if not st:
                    ev = (lax.broadcasted_iota(I32, (64, 128), 1) & 1) == 0
                    a = ssm_w[n][:, m * T:m * T + H]
                    b = pltpu.roll(ssm_w[n][:, m * T + H:(m + 1) * T], 1, 1)
                    st.extend([pltpu.bitcast(jnp.where(ev, a, b), BF16), pltpu.bitcast(jnp.where(ev, b, a), BF16)])
                return st[i]

            def epi(p):
                er, ei, or_, oi = p
                if m == 0:
                    er = er + taps[4, 0:1, C(n)]
                for h, (cr, ci) in enumerate(((er + or_, ei + oi), (er - or_, ei - oi))):
                    B = h * 3 * H
                    kf[m, B:B + H, C(n)] = cr
                    kf[m, B + H:B + 2 * H, C(n)] = ci - cr
                    kf[m, B + 2 * H:B + 3 * H, C(n)] = ci + cr
            return Unit("K%d" % n, [(lambda i=i, r=r: (tf_v[r:r + H, C(i)], rhs(i))) for i in range(2) for r in (0, H)],
                        epi, H, 170, nt=True)
        return [unit(m) for m in range(NB)]

    def kv(s, sl):
        def mk(t, w):
            def fn(a):
                ld = lambda o, n: k_n[s][t, pl.ds(8 + w + o, n), :]
                c0 = jnp.concatenate([_tie(ld(0, 8), a), ld(8, 8)], axis=0).reshape(2, 8, 128)
                c1, c2 = ld(-1, 16).reshape(2, 8, 128), ld(-2, 16).reshape(2, 8, 128)
                s0, s1, s2, s3 = (taps[i, :, C(t)] for i in range(4))
                ke, ko, ke1, ko1, ko2 = _lo(c0), _hi(c0), _lo(c1), _hi(c1), _hi(c2)
                wv = v_n[s][t, w:w + 16, :].reshape(2, 8, 128)
                kve = ((s0 * ke + s1 * ko1) + (s2 * ke1 + s3 * ko2)) * _lo(wv)
                kvo = ((s0 * ko + s1 * ke) + (s2 * ko1 + s3 * ke1)) * _hi(wv)
                kv_v[pl.ds(sl * T + w, 16), C(t)] = kve.reshape(16, 128).astype(BF16)
                kv_v[pl.ds(sl * T + H + w, 16), C(t)] = kvo.reshape(16, 128).astype(BF16)
            return fn
        return [[mk(t, w) for w in range(0, H, 16)] for t in range(NT)]

    def mmU(name, sl, us):
        def unit(n):
            def epi(p):
                er, ei, or_, oi = p
                for h, (cr, ci) in enumerate(((er + or_, ei + oi), (er - or_, ei - oi))):
                    B = h * 3 * H
                    uf[us, B:B + H, C(n)] = cr + ci
                    uf[us, B + H:B + 2 * H, C(n)] = cr
                    uf[us, B + 2 * H:B + 3 * H, C(n)] = ci
            return Unit(name(n), [(lambda i=i, r=r: (tf_v[r:r + H, C(2 + i)], kv_v[pl.ds(sl * T + i * H, H), C(n)]))
                                  for i in range(2) for r in (0, H)], epi, H, 120)
        return [unit(n) for n in range(NT)]

    def cmul(m0, u0, n, h, row, L, a):
        t = []
        for i in range(3):
            Rw = slice((3 * h + i) * H + row, (3 * h + i) * H + row + 8)
            kk = kf[m0:m0 + n, Rw, L]
            if i == 0 and a is not None:
                k0 = _tie(kk[0], a)[None]
                kk = k0 if n == 1 else jnp.concatenate([k0, kk[1:]], axis=0)
            t.append(jnp.sum(kk * uf[u0:u0 + n, Rw, L], axis=0))
        return t[0] - t[2], t[0] + t[1]

    def AR(h, q, row):
        return slice((2 * h + q) * H + row, (2 * h + q) * H + row + 8)

    def mac(n, u0, sl, first=False, part=False):
        def mk(t, rc):
            st, fin = [], []

            def piece(i):
                def fn(a):
                    h, row = i & 1, rc + (i >> 1) * 8
                    zr, zi = cmul(0, u0, n, h, row, C(t), a)
                    if part:
                        zr, zi = zr + acc[0, AR(h, 0, row), C(t)], zi + acc[0, AR(h, 1, row), C(t)]
                    st.append((zr, zi))
                    if h:
                        (pr, pi), (mr, mi) = st[-2:]
                        z = [pr + mr, pi + mi, pr - mr, pi - mi]
                        Rw = lambda q: slice(q * H + row, q * H + row + 8)
                        pv = None if first else [zraw[Rw(q ^ 1), C(t)] for q in range(4)]
                        for q in range(4):
                            zraw[Rw(q), C(t)] = z[q]
                        if not first:
                            z = [z[q] + pv[q] if (q & 1) == (rc < 64) else z[q] - pv[q] for q in range(4)]
                        fin.append(z)
                    if i == 3:
                        for q in range(4):
                            zz_v[pl.ds(sl * 2 * T + q * H + rc, 16), C(t)] = jnp.concatenate(
                                [fin[0][q], fin[1][q]], axis=0).astype(BF16)
                return fn
            if not part:
                return [piece(i) for i in range(4)]
            both = lambda f, g: (lambda a: (f(a), g(None)))
            return [both(piece(0), piece(1)), both(piece(2), piece(3))]
        return [[fn for rc in range(0, H, 16) for fn in mk(t, rc)] for t in range(NT)]

    def pos():
        return [(t, h, row) for t in range(NT) for row in range(0, H, 8) for h in range(2)]

    def ahead(i):
        def mk(t, h, row):
            def fn(a):
                zr, zi = cmul(i + 1, 0, NC, h, row, C(t), a)
                acc[i, AR(h, 0, row), C(t)] = zr
                acc[i, AR(h, 1, row), C(t)] = zi
            return fn
        return [mk(*p) for p in pos()]

    def spread():
        n = NB - NC - 1

        def mk(t, h, row):
            def fn(a):
                p = []
                for i in range(3):
                    Rw = slice((3 * h + i) * H + row, (3 * h + i) * H + row + 8)
                    u = uf[0, Rw, C(t)]
                    p.append(kf[1:1 + n, Rw, C(t)] * (_tie(u, a) if i == 0 else u)[None])
                acc[0:n, AR(h, 0, row), C(t)] = acc[1:1 + n, AR(h, 0, row), C(t)] + (p[0] - p[2])
                acc[0:n, AR(h, 1, row), C(t)] = acc[1:1 + n, AR(h, 1, row), C(t)] + (p[0] + p[1])
            return fn
        return [mk(*p) for p in pos()]

    def mmI(name, sl, ys):
        def unit(n):
            def epi(p):
                ce, se, co, so = p
                sub = lax.broadcasted_iota(I32, (8, 128), 0)
                c0 = ys * T + H
                y_v[n, ys * T:ys * T + 1, :] = (ce[64:72] - se[0:8])[0:1]
                se = jnp.concatenate([jnp.where(sub == 0, 0.0, se[0:8]), se[8:]], axis=0)
                for d, cc, ss in ((0, ce[0:64], se), (1, co, so)):
                    y_v[n, pl.ds(c0 + d, 64, stride=2), :] = cc + ss
                    lo = cc - ss
                    for i in range(0, 64, 8):
                        y_v[n, pl.ds(c0 - d - 2 * i - 14, 8, stride=2), :] = jnp.take_along_axis(
                            lo[i:i + 8], 7 - sub, axis=0)
            return Unit(name(n), [(lambda i=i: (tg_v[0:(GR if i == 0 else 64), C(i)], zz_v[pl.ds(sl * 2 * T + i * H, H), C(n)]))
                                  for i in range(4)], epi, 64, 52)
        return [unit(n) for n in range(NT)]

    def mod(name, a, b):
        def unit(n):
            def epi(p):
                v = [_sum(p[i * NT:(i + 1) * NT])[0:8] for i in range(b - a)]
                if a == 0:
                    mod_v[0, :, C(n)] = v[0] * v[2]
                    mod_v[1, :, C(n)] = (v[1] + 1.0) * v[2]
                elif a == 3:
                    mod_v[3, :, C(n)] = v[0]
                    mod_v[4, :, C(n)] = v[1] + 1.0
                else:
                    mod_v[5, :, C(n)] = v[0]
                    mod_v[2, :, C(n)] = v[0] * G_POST
            return Unit(name, [(lambda i=i, k=k: (silu_c[:, C(k)], wm_v[a][C(k), pl.ds(i * D + n * 128, 128)]))
                               for i in range(b - a) for k in range(NT)], epi, 16, 10, full=False, acc=b - a == 1)
        return [unit(n) for n in range(NT)]

    HS = (slice(0, 128), slice(128, 256))
    QS = tuple(slice(r, r + 64) for r in range(0, T, 64))

    def tasks(f, due=None, tie=True, n=RG):
        def mk(R):
            def fn(a):
                x = f(R, a if tie else None)
                return Due(x, due) if due else None
            return fn
        return [mk(slice(r, r + n)) for r in range(0, T, n)]

    def load_y(sl, R):
        return jnp.concatenate([y_v[t, sl * T + R.start:sl * T + R.stop, :] for t in range(NT)],
                               axis=1).reshape(2, 8, D)

    def put(nn, ss, R, x):
        nn[R, :] = x.astype(BF16)
        tok = x
        if ss is not None:
            S2 = pl.ds(R.start // 32 * 16, 16)
            if R.stop % 32:
                top_v[S2, 0:2 * T] = x[:, 0:2 * T]
            else:
                if R.start % 32:
                    x = jnp.concatenate([top_v[S2, 0:2 * T], x[:, 0:2 * T]], axis=0)
                ss[S2, 0:5 * T] = jnp.concatenate(_lhs_sums(x[:, 0:T], x[:, T:2 * T]), axis=1).astype(BF16)
        return tok

    wide = lambda v: jnp.concatenate([v] * NT, axis=1)

    def mean(i, R, x):
        st_v[R, C(i)] = jnp.broadcast_to(jnp.sum(x, axis=-1, keepdims=True) * (1.0 / D), (x.shape[0], 128))

    def centred(src, i, R, a):
        return src[R, :] - wide(_tie(st_v[R, C(i)], a))

    def scale(src, i, g):
        def f(R, a):
            st_v[R, C(i + 1)] = jnp.broadcast_to(_rstd(centred(src, i, R, a), g), (RG, 128))
        return f

    def normed(src, i, R, a):
        return centred(src, i, R, a) * wide(st_v[R, C(i + 1)])

    def front(sl, xs, early=False, ss=None):
        xx, hh, nn = view(x_v, xs), view(hb_v, xs), view(n1_v, sl)

        def fa(R, a):
            q = [q_n[sl][t, R.start // 2:R.stop // 2, :] for t in range(NT)]
            q = jnp.concatenate([_tie(q[0], a)] + q[1:], axis=1)
            q = pltpu.bitcast(q, BF16).astype(F32).reshape(2, 8, D)
            x = (q + (_ln(q) * mod_v[1] + mod_v[0]) * load_y(sl, R)).reshape(RG, D)
            xx[R, :] = x
            if early:
                hh[R, :] = _ln(x)
            return x

        def fb(R, a):
            hb = (_ln(_tie(xx[R, :], a).reshape(2, 8, D)) * mod_v[4] + mod_v[3]).reshape(RG, D)
            hh[R, :] = hb
            return hb

        def fc(R, a):
            hb = _tie(hh[R, :], a)
            if early:
                hb = (hb.reshape(2, 8, D) * mod_v[4] + mod_v[3]).reshape(RG, D)
                hh[R, :] = hb
            return put(nn, ss, R, _ln(hb, G_A))
        if early:
            return tasks(fa), tasks(fc)
        if ss is None:
            return tasks(fa) + tasks(fb) + tasks(fc)
        qf = view(x_v, 2)

        def s1(R, a):
            q = [q_n[sl][t, R.start // 2:R.stop // 2, :] for t in range(NT)]
            q = pltpu.bitcast(jnp.concatenate([_tie(v, a) for v in q], axis=1), BF16).astype(F32)
            qf[R, :] = q
            mean(0, R, q)

        def s3(R, a):
            h = normed(qf, 0, R, a).reshape(2, 8, D) * mod_v[1] + mod_v[0]
            x = qf[R, :] + (h * load_y(sl, R)).reshape(RG, D)
            xx[R, :] = x
            mean(2, R, x)

        def s5(R, a):
            hb = (normed(xx, 2, R, a).reshape(2, 8, D) * mod_v[4] + mod_v[3]).reshape(RG, D)
            hh[R, :] = hb
            mean(4, R, hb)
        s7 = [f for g in tasks(lambda R, a: put(nn, ss, R, normed(hh, 4, R, a)), n=32) for f in (g, lambda a: None)]
        st = [tasks(s3), tasks(scale(xx, 2, 1.0)), tasks(s5), tasks(scale(hh, 4, G_A)), s7]
        if "S" in V:
            return cat(st), [], tasks(s1) + tasks(scale(qf, 0, 1.0))
        if "Q" in V:
            p = [tasks(s1), tasks(scale(qf, 0, 1.0))]
            return cat(x[:8] for x in st), cat(x[8:] for x in p + st), cat(x[:8] for x in p)
        return cat(x[:8] for x in st), cat(x[8:] for x in st), tasks(s1) + tasks(scale(qf, 0, 1.0))

    def shift(hs, sl, pieces=((0, 64), (64, 64), (128, 64), (192, 64)), ss=None):
        gg = view(g_v, sl)

        def one_tile(t, r, n, a):
            lane = lax.broadcasted_iota(I32, (n, 128), 1)
            ld = lambda d: h1_v[t, pl.ds(hs * T + 8 + r + d, n), :]
            if t == 0:
                g = ld(-1)
            elif t == 1:
                g = jnp.where(lane < 32, ld(-1), ld(1))
            elif t == 2:
                g = jnp.where(lane < 64, ld(1), ld(-2))
            elif t == 3:
                g = jnp.where(lane < 96, ld(-2), ld(2))
            else:
                g = ld(2)
            if a is not None:
                g = jnp.concatenate([_tie(g[i:i + 8], a) if i % 16 == 0 else g[i:i + 8]
                                     for i in range(0, n, 8)], axis=0)
            gg[r:r + n, C(t)] = g.astype(BF16)
            return g

        def mk(ts, r, n):
            def fn(a):
                g = [one_tile(t, r, n, a) for t in ts]
                if len(ts) == 2:
                    for i, x in enumerate(_lhs_sums(*g)):
                        ss[r // 2:(r + n) // 2, C(2 * i + ts[0])] = x.astype(BF16)
            return fn
        sets = [(t,) for t in range(NT)] if ss is None else [(0, 2), (1, 3), (4,)]
        return [mk(ts, r, n) for ts in sets for r, n in pieces]

    def shift_early():
        def keep(a):
            h1_v[:, 2 * T - 32:2 * T + 8, :] = h1_v[:, 3 * T - 32:3 * T + 8, :]
        return shift(2, 0, [(r, 32) for r in range(0, T - 32, 32)], gs) + [keep]

    def ln2(xs, sl, fast=True):
        xx, nn, ss = view(x1_v, xs), view(n2_v, sl), view(n2s, sl, H) if fast else None
        f = lambda R, a: put(nn, ss, R, _ln(_tie(xx[R, :], a), G_A))
        if fast and "N" in V:
            a_, b_ = tasks(lambda R, a: mean(6, R, _tie(xx[R, :], a))), tasks(scale(xx, 6, G_A))
            c_ = [f for g in tasks(lambda R, a: put(nn, ss, R, normed(xx, 6, R, a)), n=32)
                  for f in (g, lambda a: None, lambda a: None)]
            return a_[:8] + b_[:8] + a_[8:] + b_[8:] + c_
        ts = tasks(f, DL, False)
        return ts[0::2] + ts[1::2] if fast else tasks(f)

    def resid(xs, x1s, rotate=False):
        xx, x1 = view(x_v, xs), view(x1_v, x1s)

        def f(R, a):
            gb = mod_v[5] if a is None else pltpu.bitcast(
                pltpu.bitcast(mod_v[5], U32) | jnp.concatenate([a] * NT, axis=1), F32)
            r_v[R, :] = xx[R, :] + (x1[R, :].reshape(2, 8, D) * gb).reshape(RG, D)
            if rotate:
                xx[R, :] = x_v[R, :]
                view(hb_v, 1)[R, :] = hb_v[R, :]
        return tasks(f)

    KD, KF, ND = [(0, 2), (1, 3)], [(2 * i, 2 * i + 1) for i in range(7)], [(1, 2), (3, 4)]
    Wt = {1: (lambda k, n: w1_v[C(k), C(n)], lambda i, kp, j: w1s[C(kp), C(2 * i + j)], False, KD, [4]),
          2: (lambda k, n: w2_v[C(k), C(n)], lambda i, kp, j: w2s[C(kp), C(2 * i + j)], False, KD, [4]),
          0: (lambda k, n: w3_v[C(n), C(k)], None, True, KD, [4]),
          3: (lambda k, n: w3n[C(k), C(n)], lambda i, kp, j: w3s[C(kp), C(6 * i + j)], False, KD, [4]),
          4: (lambda k, n: w4_v[C(k), C(n)], lambda i, kp, j: w4s[C(kp), C(2 * i + j)], False, KF, [])}

    def wsums(w_w, ws, rp, cp_):
        def mk(i, j, r):
            def fn(a):
                b = [[w_w[pl.ds(64 * p + r // 2, 8), C(q)] for q in cp_[j]] for p in rp[i]]
                b[0][0], b[1][1] = _tie(b[0][0], a), _tie(b[1][1], a)
                (b11, b12), (b21, b22) = [[pltpu.bitcast(x, BF16).astype(F32) for x in row] for row in b]
                for m, x in enumerate((b11 + b22, b12 - b22, b21 - b11, b11 + b12, b21 + b22)):
                    ws[pl.ds(128 * i + r, 16), C(len(cp_) * m + j)] = x.astype(BF16)
            return fn
        return [mk(i, j, r) for j in range(len(cp_)) for i in range(len(rp)) for r in range(0, 128, 16)]

    def w3_turn():
        def mk(n, k):
            def fn(a):
                x = jnp.concatenate([_tie(w3_w[64 * n:64 * n + 8, C(k)], a), w3_w[64 * n + 8:64 * n + 64, C(k)]], axis=0)
                w3n[C(k), C(n)] = pltpu.bitcast(x, BF16).T
            return fn
        return [mk(n, k) for n in range(FT - 1) for k in range(NT)]

    def plain(name, w, lhs, n, R, epi, cost):
        tile, _, nt, kp, kl = Wt[w]
        ks = sorted([k for p in kp for k in p] + kl)
        rows_ = R.stop - R.start
        return Unit(name, [(lambda k=k: (lhs[R, C(k)], tile(k, n))) for k in ks], lambda p: epi(n, R, p[0]),
                    rows_, rows_ // 8 * (len(ks) - 1 + cost), nt=nt, acc=True)

    def quad(name, w, lhs, sums, j, cols_, R, epi, cost):
        tile, wsum, nt, kp, kl = Wt[w]
        h, S2, c = len(kp), slice(R.start // 2, R.stop // 2), {}
        a_ = lambda i, k: _top(lhs[R, C(k)], i)
        s_ = lambda i, p: sums[S2, C(h * i + p)]
        prod = lambda fa_, fb_: [(lambda p=p: (fa_(p), fb_(p))) for p in range(h)]
        left = lambda i, n: [(lambda k=k: (a_(i, k), tile(k, n))) for k in kl]
        mk = lambda tiles, f, x=0: Unit(name, tiles, lambda p: f(p[0]), 64, 8 * len(tiles) + x, nt=nt, acc=True)

        def e1(m):
            u7.res, u6.res = [m], [m]

        def e4(m):
            c[11], c[21] = c[11] + m, m

        def e2(m):
            c[21], c[22] = c[21] + m, c[22] - m
            l21.res = [c[21]]

        def e5(m):
            c[12] = m
            epi(cols_[0], R, _zip(c[11] - m, c[21]))

        def e3(m):
            l12.res, c[22] = [c[12] + m], c[22] + m
            if not kl:
                l12.epi(l12.res)
        u1 = mk(prod(lambda p: s_(0, p), lambda p: wsum(0, p, j)), e1)
        u7 = mk(prod(lambda p: s_(4, p), lambda p: wsum(4, p, j)) + left(0, cols_[0]), lambda m: c.update({11: m}))
        u6 = mk(prod(lambda p: s_(3, p), lambda p: wsum(3, p, j)) + left(1, cols_[1]), lambda m: c.update({22: m}))
        u4 = mk(prod(lambda p: a_(1, kp[p][1]), lambda p: wsum(2, p, j)), e4)
        u2 = mk(prod(lambda p: s_(1, p), lambda p: tile(kp[p][0], cols_[0])), e2, 8)
        l21 = mk(left(1, cols_[0]), lambda m: c.update({21: m}))
        u5 = mk(prod(lambda p: s_(2, p), lambda p: tile(kp[p][1], cols_[1])), e5, 16 * cost)
        u3 = mk(prod(lambda p: a_(0, kp[p][0]), lambda p: wsum(1, p, j)), e3, 8 if kl else 8 + 16 * cost)
        l12 = mk(left(0, cols_[1]), lambda m: epi(cols_[1], R, _zip(m, c[22])), 16 * cost)
        return [u1, u7, u6, u4, u2, l21, u5, u3, l12]

    def mm(name, w, lhs, sums, epi, cost):
        if sums is None:
            return [[plain(name, w, lhs, n, R, epi, cost) for R in HS] for n in range(NT)]
        return [[plain(name, w, lhs, 0, R, epi, cost) for R in QS]] + [
            [u for R in HS for u in quad(name, w, lhs, sums, j, ND[j], R, epi, cost)] for j in range(2)]

    def mm1(name, hs, sl, fast=False):
        def epi(n, R, p):
            h1_v[n, pl.ds(hs * T + 8 + R.start, R.stop - R.start), :] = _gelu2(p)
        return cat(mm(name, 1, view(n1_v, sl), n1s if fast else None, epi, 5))

    def mm2(name, sl, xs, x1s, fast=False):
        def epi(n, R, p):
            view(x1_v, x1s)[R, C(n)] = view(hb_v, xs)[R, C(n)] + p * G_POST
        return cat(mm(name, 2, view(g_v, sl), gs if fast else None, epi, 2))

    def mm3(name, sl, fast=True):
        nn, aa, ss, keep, tail = view(n2_v, sl), view(a_v, sl), view(a_s, sl, H), [], []

        def epi(n, R, p):
            g = _gelu2(p)
            aa[R, C(n)] = g.astype(BF16)
            if n % 2 == 0 and n < 12:
                keep.append(g)
                return
            pair = (keep.pop(), g) if n % 2 else (g, tail[R.start // 128][R.start % 128:R.start % 128 + 64])
            for i, x in enumerate(_lhs_sums(*pair)):
                ss[R.start // 2:R.stop // 2, C(7 * i + n // 2)] = x.astype(BF16)

        def rem(R):
            def f(p):
                tail.append(jnp.concatenate([_gelu2(p[0]), jnp.zeros((64, 128), F32)], axis=0).T)
                aa[R, C(13)] = tail[-1].astype(BF16)
            return Unit(name, [(lambda k=k: (w3_v[13 * 128:F, C(k)], nn[R, C(k)])) for k in range(NT)], f, 64, 84,
                        nt=True, acc=True)
        odd = [rem(R) for R in HS] + [plain(name, 3 if fast else 0, nn, 12, R, epi, 9) for R in QS]
        if fast:
            qd = [u for j in range(6) for R in HS for u in quad(name, 3, nn, view(n2s, sl, H), j, KF[j], R, epi, 8)]
            return qd[:18] + odd[:2] + qd[18:36] + odd[2:] + qd[36:]
        return odd + [plain(name, 0, nn, n, R, epi, 8) for p in KF[:6] for R in HS for n in p]

    NA = 3 * 128

    def cp_out(j, osl, L, sm, R=slice(0, T)):
        return cp(o_v.at[pl.ds(osl * T + R.start, R.stop - R.start), L],
                  o_hbm.at[pl.ds(base(j, T) + R.start, R.stop - R.start), L], sem_o.at[sm])

    out_a = lambda j: cp_out(j, 0, slice(0, NA), 0)
    out_b = lambda j: cp_out(j, 0, slice(NA, D), 1)
    last = []

    def mm4(name, j, sl, osl=0, xs=None, x1s=None, fast=True):
        oo = view(o_v, osl)

        def epi(n, R, p):
            if xs is None:
                oo[R, C(n)] = (r_v[R, C(n)] + mod_v[2, 0:1, C(n)] * p).astype(BF16)
            else:
                oo[R, C(n)] = (view(x_v, xs)[R, C(n)] + mod_v[5, 0:1, C(n)]
                               * (view(x1_v, x1s)[R, C(n)] + p * G_POST)).astype(BF16)
            if osl == 2:
                last.append(cp_out(j, osl, C(n), 2, R))
                last[-1].start()
            elif R.stop == T and (osl, (n + 1) * 128) in ((1, D), (3, NA)):
                last.append(cp_out(j, osl, slice(0, (n + 1) * 128), 2))
                last[-1].start()
            elif R.stop == T and osl == 0 and (n + 1) * 128 in (NA, D):
                (out_a if (n + 1) * 128 == NA else out_b)(j).start()
        return mm(name, 4, view(a_v, sl), view(a_s, sl, H) if fast else None, epi, 3 if xs is None else 5)

    def split(us):
        n = 4 // len(us)
        m, mks, st = us[0].rows // n, [u.tiles.pop(0) for u in us], {}

        def piece(i, k):
            if i not in st:
                st[i] = mks[i]()
            return st[i][0][m * k:m * (k + 1)], st[i][1]

        def epi(p):
            for i, u in enumerate(us):
                u.res = [jnp.concatenate(p[n * i:n * (i + 1)], axis=0)]
        return _flat([Unit(us[0].name, [(lambda i=i, k=k: piece(i, k)) for i in range(len(us)) for k in range(n)],
                           epi, m, 0, nt=us[0].nt)])

    W = lambda nm: [("wait", nm)]
    run = lambda fns: [("run", "run", lambda: [fn(None) for fn in fns])]
    one = lambda us: [_flat([u]) for u in us]
    nm = lambda x: (lambda n: x)

    seq, grp = [], []
    for s in range(NC):
        seq += W("c%d" % s) + _flat(mmK(s) + mmU(nm("U%d" % s), s % 2, NC - 1 - s))
        grp.append(Group("kv%d" % s, cat(kv(s, s % 2)), 50, ["c%d" % s], ["U%d" % s], 100))
    inv = [mmI(lambda n: "I%d" % n, s, s) for s in range(NC)]
    seq += W("c3") + _flat(mmK(3) + mmK(4) + [inv[s][t] for t in range(NT) for s in range(NC)])
    macs = [mac(s + 1, NC - 1 - s, s, first=s == 0) for s in range(NC)]
    grp.append(Group("mac00", macs[0][0], 12, ["c1"], ["c2"], 0))
    grp.append(Group("mac01", macs[1][0] + macs[0][1] + macs[1][1], 16, ["c2"], ["c3"], 0))
    for t in range(NT):
        grp.append(Group("mac%d" % t, cat(macs[s][t] for s in range(2 if t < 2 else 0, NC)), 24 if t < 2 else 18,
                         ["c3", "K%d" % t], ["I%d" % t], 100, 150))
    start = lambda cs: [("run", "run", lambda: [c.start() for c in cs])]
    f0, f1 = front(0, 2, True), front(1, 1, True)
    seq += run(ahead(0))
    seq += W("wma") + _flat(mod("moda", 0, 3)) + run(f0[0] + f1[0] + ahead(1))
    seq += W("wmb") + start(next_kv(NC) + next_q(NC)) + _flat(mod("modb", 3, 5)) + run(f0[1])
    w1 = _flat(mm1("w1_0", 0, 0) + mm1("w1_1", 1, 1))
    seq += W("w1") + w1[:LP[4]] + W("w2") + w1[LP[4]:] + run(shift(0, 0))
    seq += _flat(mm2("w2_0", 0, 2, 1) + mm1("w1_2", 2, 2)) + run(shift(1, 1)) + _flat(mm2("w2_1", 1, 1, 0))
    grp.append(Group("f1", f1[1], 80, ["w1"], ["w1_1"], 450))
    grp.append(Group("f2", front(2, 0), 80, ["w2"], ["w1_2"], 450))
    grp.append(Group("ln2_0", ln2(1, 0, False), 60, ["w2_0"], ["w3"], 450))
    grp.append(Group("ahead", cat(ahead(i) for i in range(2, NB - NC)), 19, ["w1"], ["end"], 100))
    grp.append(Group("ws1", wsums(w1_w, w1s, KD, ND), 26, ["w1"], ["end"], 100))
    grp.append(Group("ws2", wsums(w2_w, w2s, KD, ND), 26, ["w2"], ["end"], 100))
    grp.append(Group("ws3", w3_turn() + wsums(w3n_w, w3s, KD, KF[:6]), 22, ["w3"], ["end"], 100))
    grp.append(Group("ws4", wsums(w4_w, w4s, KF, ND), 26, ["w4"], ["end"], 100))
    _wait(seq, "w3", back=1)
    w3 = mm3("w3_0", 0, False)
    _mix(seq, _flat(w3[6:]), [split(w3[4:6]) + _flat(w3[:6])], 0.1)
    mc = _flat(mod("modc", 5, 6))
    _wait(seq, "w4", mc[:5] + [("sync", "run", lambda: None)])
    w4 = cat(mm4("w4_0", 0, 0, 3, 2, 1, False)[:3])
    qs = [split([w4[-1 - i]]) for i in range((_phase(seq) + FT * 6) % 4)]
    _mix(seq, _flat(w4), [mc[i:i + 4] for i in range(5, 25, 4)] + qs, 0.01, 0.4)
    assert _phase(seq) == 0
    grp.append(Group("resid", resid(2, 1), 26, ["modc"], ["end"], 100))
    _emit(seq, grp, zero, wait)

    def step(s, carry):
        for c in next_kv(s) + next_q(s):
            c.wait()
        nxt = jnp.minimum(s + 1, NB - 1)
        seq, grp = [], []
        us, it = one(mmU(lambda n: "U%d" % n, 0, 0)), one(mmI(lambda n: "I%d" % n, 0, 0))
        w4 = mm4("w4", s - 2, 0)
        q = split(w4[0][2:])
        _mix(seq, _flat(mm4("w4c", s - 3, 0)[2] + mm3("w3", 0)),
             [us[0], us[1], us[2], it[0] + us[3], it[1] + us[4], it[2] + start(next_kv(nxt)), it[3], it[4]],
             LP[3], LP[0])
        w1a, w1b = mm1("w1a", 2, 0, True), mm1("w1b", 2, 0, True)
        w1a, w1b = _flat(w1a[0:2] + w1a[4:13] + w1a[22:31]), _flat(w1b[2:4] + w1b[13:22] + w1b[31:])
        _mix(seq, _flat(w4[0] + w4[1][:9]), [q])
        if "S" in V:
            seq += _flat(w4[1][9:]) + w1a + run(shift(1, 0, ((T - 32, 32),), gs)) + w1b[:8] + start(next_q(nxt)) + w1b[8:]
        else:
            seq += w1a + run(shift(1, 0, ((T - 32, 32),), gs)) + _flat(w4[1][9:]) + w1b[:8] + start(next_q(nxt)) + w1b[8:]
        seq += _flat(mm2("w2", 0, 1, 0, True))
        assert _phase(seq) == 0
        kvs, macs = kv(0, 0), mac(1, 0, 0, part=True)
        for t in range(NT):
            grp.append(Group("kv%d" % t, kvs[t], 50, ["start"], ["U%d" % t], 300))
            grp.append(Group("mac%d" % t, macs[t], 28, ["U%d" % t], ["I%d" % t], 300, 150))
        iall = ["I%d" % t for t in range(NT)]
        grp.append(Group("ln2", ln2(0, 0), 27 if "N" in V else 75, ["start"], ["w3"], 200 if "N" in V else 450))
        grp.append(Group("resid", resid(1, 0, True), 40, ["w4c"], ["w4", "I4"], 100))
        fr = front(0, 0, ss=n1s)
        grp.append(Group("fronta", fr[0], 50, iall, ["w1a"], FL))
        if fr[1]:
          grp.append(Group("frontb", fr[1], 50, iall, ["w1b"], FL, RL))
        grp.append(Group("fq", fr[2], 34, ["w4c"], ["I4"], 100))
        grp.append(Group("spread", spread(), 30, iall, ["end"], 100))
        grp.append(Group("shift", shift_early(), 24, ["start"], ["w1a"], 200))
        _emit(seq, grp, zero, wait)
        out_b(s - 3).wait()
        out_a(s - 2).wait()
        return carry

    lax.fori_loop(NC, NB, step, 0)

    seq, grp = [], []
    w4 = cat(mm4("w4_6", NB - 2, 0, 1, 1, 0))
    q = split(w4[2:4])
    seq += _flat(mm4("w4_5", NB - 3, 0)[2] + mm3("w3_6", 0) + mm2("w2_7", 0, 0, 1, True))
    _mix(seq, _flat(w4), [q])
    seq += _flat(mm3("w3_7", 1) + cat(mm4("w4_7", NB - 1, 1, 2, 0, 1)))
    assert _phase(seq) == 0
    grp.append(Group("ln2_6", ln2(0, 0), 27 if "N" in V else 75, ["start"], ["w3_6"], 200 if "N" in V else 450))
    grp.append(Group("shift7", shift(2, 0, [(r, 32) for r in range(0, T, 32)], gs), 24, ["start"], ["w2_7"], 200))
    grp.append(Group("ln2_7", ln2(1, 1), 27 if "N" in V else 75, ["w2_7"], ["w3_7"], 200 if "N" in V else 450))
    _emit(seq, grp, zero, wait)
    for c in next_kv(NB - 1) + next_q(NB - 1) + [out_b(NB - 3)] + last:
        c.wait()


@jax.jit
def pallas_adaLN_cond__ssm_conv_h3__mixer_s_mlp__prompt_kernel(
        A_q, A_k, A_v, A_shift_k, A_ssm_k, A_ssm_D, B_x, B_w1, B_w2, B_w3, B_w4, c, w_mod):
    any_ = pl.BlockSpec(memory_space=pl.ANY)
    V = pltpu.VMEM
    out = pl.pallas_call(
        kernel,
        in_specs=[any_] * 12,
        out_specs=any_,
        out_shape=jax.ShapeDtypeStruct((S, D), BF16),
        scratch_shapes=[
            [V((NT, H + 8, 128), U32)] * NC, [V((NT, H + 8, 128), U32)] * NC, [V((NT, H + 8, 128), U32)] * NC,
            [V((64, S), U32)] * NT,
            V((D // 2, D), U32), V((D // 2, D), U32), V((F // 2, D), U32), V((FT * 64, D), U32),
            [V((D // 2, 3 * D), U32), V((D // 2, 2 * D), U32), V((D // 2, D), U32)], V((4 * T, D), BF16),
            V((4, D), BF16), V((D,), BF16), V((1, D), BF16), V((8, 128), I32), pltpu.SMEM((8, 128), I32),
            V((5, 8, D), F32), V((6, 8, D), F32), V((T // 2, 4 * H), U32), V((GR // 2, 2 * T), U32),
            V((NB, 3 * T + 8, D), F32), V((NC, 3 * T + 8, D), F32), V((NB - NC, 2 * T + 8, D), F32), V((2 * T, D), F32),
            V((T, D), U32), V((NC * T, D), U32), V((NT, NC * T + 8, 128), F32),
            V((3 * T, D), F32), V((3 * T, D), F32), V((2 * T, D), F32), V((T, D), F32),
            V((3 * T // 2, D), U32), V((T, D), U32), V((T, D), U32), V((NT, NC * T + 24, 128), F32),
            V((T, (FT + 1) * 128), U32),
            [V((128, 11 * 128), U32)] * 2 + [V((128, 31 * 128), U32), V((448, 11 * 128), U32)],
            [V((64, 11 * 128), U32)] * 2 + [V((128, 11 * 128), U32), V((128, 35 * 128), U32)],
            V((D // 2, 13 * 128), U32), V((H, D), F32), V((T, 9 * 128), F32),
            pltpu.SemaphoreType.DMA((11,)), pltpu.SemaphoreType.DMA((1,)), pltpu.SemaphoreType.DMA((3,)),
        ],
        compiler_params=pltpu.CompilerParams(vmem_limit_bytes=110 << 20, disable_semaphore_checks=True,
                                             disable_bounds_checks=True),
        name="fused",
    )(A_q[0], A_k[0], A_v[0], A_shift_k.T, A_ssm_k, A_ssm_D, B_w1, B_w2, B_w3.T, B_w4, c, w_mod)
    return out[None]
```

```python
import heapq
import numpy as np
import jax
import jax.numpy as jnp
from jax import lax
from jax.experimental import pallas as pl
from jax.experimental.pallas import tpu as pltpu

S, D, F = 2048, 640, 1728
T = 256
H = T // 2
NB = S // T
NT = D // 128
FT = (F + 127) // 128
EPS = 1e-5
F32, BF16, U32, I32 = jnp.float32, jnp.bfloat16, jnp.uint32, jnp.int32
G_C1 = 0.044715 * float(np.sqrt(2.0 / np.pi))
G_C2 = float(np.sqrt(2.0 / np.pi))
G_A = G_C1 ** (1.0 / 3.0)
G_B = G_C2 / G_A
G_POST = 0.5 / G_A
RG = 16
GR = 80
NC = 3
DL = 450
SLOT = 32


def _dft(shape, f_axis, tau, scale=1.0):
    r = lax.broadcasted_iota(I32, shape, f_axis)
    l = lax.broadcasted_iota(I32, shape, 1 - f_axis)
    f = r & 127
    odd = ((f & 63) << 2) | ((f >> 6) << 1) | 1
    p = odd * tau(l) + ((r >> 7) << 8)
    a = ((p + 512) & 1023) - 512
    u = (256 - jnp.abs(a)).astype(F32) * (np.pi / 512.0)
    u2 = u * u
    c = [scale, -scale / 6.0, scale / 120.0, -scale / 5040.0, scale / 362880.0, -scale / 39916800.0]
    poly = c[5]
    for ci in c[4::-1]:
        poly = poly * u2 + ci
    return (u * poly).astype(BF16)


def _rstd(xc, scale):
    s2 = 1.0 / (scale * scale)
    v = jnp.sum(xc * xc, axis=-1, keepdims=True) * (s2 / D) + EPS * s2
    return jnp.exp2(jnp.log(v) * float(-0.5 / np.log(2.0)))


def _ln(x, scale=1.0):
    xc = x - jnp.sum(x, axis=-1, keepdims=True) * (1.0 / D)
    return xc * _rstd(xc, scale)


def _gelu2(x):
    u = x * (x * x + G_B)
    return x * (1.0 + jnp.tanh(u))


def _lo(w):
    return pltpu.bitcast(w << 16, F32)


def _hi(w):
    return pltpu.bitcast(w & jnp.uint32(0xFFFF0000), F32)


def _tie(x, a):
    if a is None:
        return x
    w = pltpu.bitcast(x[:, :128], U32)
    k = w.shape[0] // 8
    w = w | (a if k == 1 else jnp.concatenate([a] * k, axis=0))
    w = pltpu.bitcast(w, x.dtype)
    return w if x.shape[1] == 128 else jnp.concatenate([w, x[:, 128:]], axis=1)


def _top(x, i):
    return jnp.concatenate([x[r:r + 16] for r in range(16 * i, x.shape[0], 32)], axis=0)


def _zip(t, b):
    return jnp.concatenate([x[r:r + 16] for r in range(0, t.shape[0], 16) for x in (t, b)], axis=0)


def _lhs_sums(x1, x2):
    a11, a21, a12, a22 = _top(x1, 0), _top(x1, 1), _top(x2, 0), _top(x2, 1)
    return [a11 + a22, a21 + a22, a11 + a12, a21 - a11, a12 - a22]


def C(i):
    return slice(i * 128, (i + 1) * 128)


class Unit:
    def __init__(self, name, tiles, epi, rows, cost, nt=False, full=True, acc=False):
        self.acc, self.res = acc, []
        self.name, self.tiles, self.epi, self.rows, self.cost, self.nt, self.full = name, tiles, epi, rows, cost, nt, full


class Due:
    def __init__(self, val, delay):
        self.val, self.delay = val, delay


class Group:
    def __init__(self, name, fns, cost, rel, dead, lat, rlat=200):
        self.name, self.fns, self.cost, self.rel, self.dead, self.lat, self.rlat = name, fns, cost, rel, dead, lat, rlat


def _plan(seq, groups):
    busy, n = [0] * 4, 0
    start, end, tiles, bars = {}, {}, [], []
    for it in seq:
        if isinstance(it[0], Unit):
            u = it[0]
            m = n % 4
            n += 1
            t0, t1 = busy[m], busy[m] + max(u.rows, 32)
            busy[m] = t1
            tiles.append((t0, t1, u.cost / len(u.tiles)))
            start.setdefault(u.name, t0)
            end[u.name] = max(end.get(u.name, 0), t1)
        elif it[0] == "wait":
            t = max(busy)
            busy, n = [t] * 4, 0
            start[it[1]] = end[it[1]] = t
            bars.append(t)
    total = max(busy)
    start["end"] = end["end"] = total
    start["start"] = end["start"] = 0
    ns = total // SLOT + 2
    load = np.zeros(ns)
    for t0, t1, c in tiles:
        a, b = t0 // SLOT, max(t1 // SLOT, t0 // SLOT + 1)
        load[a:b] += c / (b - a)
    win = []
    for g in groups:
        r = max(end[x] + (0 if start[x] == end[x] else g.rlat) for x in g.rel)
        d = min(start[x] for x in g.dead) - g.lat
        ok = np.zeros(ns, bool)
        ok[r // SLOT:max(d // SLOT, r // SLOT + 1)] = True
        for b in bars:
            if r < b <= d:
                ok[max((b - g.lat) // SLOT, 0):b // SLOT] = False
        win.append(np.nonzero(ok)[0])
    alloc = [np.zeros(len(w)) for w in win]
    for _ in range(60):
        for i, g in enumerate(groups):
            w = win[i]
            load[w] -= alloc[i]
            base = load[w]
            vol = g.cost * len(g.fns)
            lo, hi = base.min(), base.max() + vol
            for _ in range(50):
                mid = 0.5 * (lo + hi)
                if np.maximum(mid - base, 0).sum() > vol:
                    hi = mid
                else:
                    lo = mid
            alloc[i] = np.maximum(hi - base, 0)
            load[w] += alloc[i]
    times = []
    for i, g in enumerate(groups):
        cum = np.cumsum(alloc[i])
        ts = []
        for k in range(len(g.fns)):
            x = (k + 0.5) * cum[-1] / len(g.fns)
            j = int(np.searchsorted(cum, x))
            prev = cum[j - 1] if j else 0.0
            ts.append(win[i][j] * SLOT + SLOT * (x - prev) / max(alloc[i][j], 1e-9))
        times.append(ts)
    return times


def _emit(seq, groups, zero, wait):
    times = _plan(seq, groups)
    left = {"start": 0}
    for it in seq:
        nm = it[0].name if isinstance(it[0], Unit) else it[1]
        left[nm] = left.get(nm, 0) + 1
    heap, pend, todo, cnt = [], {}, list(range(len(groups))), 0
    busy, n, due = [0] * 4, 0, []

    def release():
        nonlocal cnt
        for i in list(todo):
            g = groups[i]
            if all(left[x] == 0 for x in g.rel):
                todo.remove(i)
                pend[i] = len(g.fns)
                for t, fn in zip(times[i], g.fns):
                    heapq.heappush(heap, (t, cnt, i, fn))
                    cnt += 1

    def force(name):
        nonlocal heap
        for i, g in enumerate(groups):
            if name in g.dead:
                assert i not in todo, (g.name, name)
                if pend[i]:
                    for it in sorted(x for x in heap if x[2] == i):
                        it[3](None)
                    heap = [x for x in heap if x[2] != i]
                    heapq.heapify(heap)
                    pend[i] = 0

    release()
    for it in seq:
        if isinstance(it[0], Unit):
            u, k = it
            force(u.name)
            lhs, rhs = u.tiles[k]()
            t0 = busy[n % 4]
            while u.full and due and due[0][0] < t0 + u.rows:
                t, x = due.pop(0)
                r = min(max(int(t - t0), 0), u.rows - 1) // 16 * 8
                w = pltpu.bitcast(lhs, U32)
                x = pltpu.bitcast(x[:, :128], U32)
                parts = [w[:r], w[r:r + 8] | ((x[0:8] | x[8:16]) & zero), w[r + 8:]]
                lhs = pltpu.bitcast(jnp.concatenate([y for y in parts if y.shape[0]], axis=0), BF16)
            dn = (((1,), (1 if u.nt else 0,)), ((), ()))
            p = lax.dot_general(lhs, rhs, dn, preferred_element_type=F32)
            u.res = [p + u.res[0]] if (u.acc and u.res) else u.res + [p]
            m = n % 4
            n += 1
            t0 = busy[m]
            busy[m] = t0 + max(u.rows, 32)
            while u.full and heap and heap[0][0] < t0 + u.rows:
                t, _, i, fn = heapq.heappop(heap)
                pend[i] -= 1
                r = min(max(int(t - t0), 0), u.rows - 1) // 8 * 8
                x = fn(pltpu.bitcast(p[r:r + 8], U32) & zero)
                if isinstance(x, Due):
                    due.append((t + x.delay, x.val))
                    due.sort(key=lambda e: e[0])
            if k == len(u.tiles) - 1:
                u.epi(u.res)
            left[u.name] -= 1
        elif it[0] == "wait":
            force(it[1])
            wait(it[1])
            busy, n, due = [max(busy)] * 4, 0, []
            left[it[1]] -= 1
        else:
            it[2]()
            left[it[1]] -= 1
        release()
    force("end")
    assert not heap and not todo


def _sum(ps):
    acc = ps[0]
    for p in ps[1:]:
        acc = acc + p
    return acc


def _flat(us):
    return [(u, i) for u in us for i in range(len(u.tiles))]


def _phase(seq):
    n = 0
    for it in seq:
        n = n + 1 if isinstance(it[0], Unit) else (0 if it[0] in ("wait", "sync") else n)
    return n % 4


def _mix(seq, a, b, lo=0.0, hi=1.0):
    n, k = _phase(seq), 0
    for i, t in enumerate(a):
        if k < len(b) and n % 4 == 0 and t[1] != 1 and i >= len(a) * (lo + (hi - lo) * k / len(b)):
            seq.extend(b[k])
            k += 1
        seq.append(t)
        n += 1
    assert k == len(b)


def _wait(seq, name, head=(), back=0):
    r = _phase(seq) + 4 * back
    assert all(isinstance(it[0], Unit) for it in seq[len(seq) - r:])
    seq[len(seq) - r:len(seq) - r] = [("wait", name)] + list(head)


def kernel(q_hbm, k_hbm, v_hbm, sh_hbm, ssm_hbm, sd_hbm, w1_hbm, w2_hbm, w3_hbm, w4_hbm, c_hbm, wm_hbm,
           o_hbm,
           q_n, k_n, v_n, ssm_w, w1_w, w2_w, w3_w, w4_w, wm_w, o_v,
           sh_v, sd_v, c_v, zsrc, z_s, taps, mod_v, tf_w, tg_w,
           kf, uf, acc, zraw, kv_w, zz_w, y_v, x_v, hb_v, x1_v, r_v, n1_w, n2_w, g_w, h1_v, a_w,
           ws_w, as_w, w3n_w, top_v, st_v,
           sem, sem_b, sem_o):
    bf = lambda r: r.bitcast(BF16)
    w1_v, w2_v, w3_v, w4_v = bf(w1_w), bf(w2_w), bf(w3_w), bf(w4_w)
    wm_v = {0: bf(wm_w[0]), 3: bf(wm_w[1]), 5: bf(wm_w[2])}
    tf_v, tg_v, n1_v, n2_v, g_v = bf(tf_w), bf(tg_w), bf(n1_w), bf(n2_w), bf(g_w)
    a_v, kv_v, zz_v = bf(a_w), bf(kv_w), bf(zz_w)
    w1s, w2s, w3s, w4s = [bf(r) for r in ws_w]
    n1s, gs, n2s, a_s = [bf(r) for r in as_w]
    w3n = bf(w3n_w)
    cp = pltpu.make_async_copy
    cat = lambda ls: [x for l in ls for x in l]

    def base(j, n):
        return j * n if isinstance(j, int) else pl.multiple_of(j * n, n)

    def rows(j, n=1, size=T):
        return pl.ds(base(j, size), n * size)

    def view(ref, j, size=T):
        return ref.at[rows(j, 1, size)]

    dmas = {}

    def group(name, *mks):
        sm = sem.at[len(dmas)]
        dmas[name] = [c for mk in mks for c in mk(sm)]

    def ssm_in(t):
        return lambda sm: [cp(ssm_hbm.at[C(t)], bf(ssm_w[t]), sm)]

    def cols(src, start, n, dst, row=0):
        return lambda sm: [cp(src.at[pl.ds(start, n), C(t)], bf(dst).at[t, pl.ds(row, n)], sm) for t in range(NT)]

    def kv_in(s, sl):
        if isinstance(s, int):
            kk = cols(k_hbm, s * T - 16, T + 16, k_n[sl]) if s else cols(k_hbm, 0, T, k_n[sl], 16)
        else:
            kk = cols(k_hbm, pl.multiple_of(s * T - 16, 16), T + 16, k_n[sl])
        return lambda sm: kk(sm) + cols(v_hbm, base(s, T), T, v_n[sl])(sm)

    def q_in(s, sl):
        return cols(q_hbm, base(s, T), T, q_n[sl])

    def wm_in(a, b):
        return lambda sm: [cp(wm_hbm.at[:, a * D:b * D], wm_v[a], sm)]

    def whole(src, dst):
        return lambda sm: [cp(src, dst, sm)]

    next_kv = lambda s: kv_in(s, 0)(sem_b.at[0])
    next_q = lambda s: q_in(s, 0)(sem_b.at[0])

    zsrc[...] = jnp.zeros((8, 128), I32)
    k_n[0][:, 0:8, :] = jnp.zeros((NT, 8, 128), U32)
    w4_w[F // 2:FT * 64, :] = jnp.zeros((FT * 64 - F // 2, D), U32)
    group("small", lambda sm: [cp(zsrc, z_s, sm), cp(sh_hbm, sh_v, sm), cp(sd_hbm, sd_v, sm), cp(c_hbm, c_v, sm)])
    for s in range(NC):
        group("c%d" % s, ssm_in(s), kv_in(s, s))
    group("c3", ssm_in(3), ssm_in(4))
    group("wma", wm_in(0, 3), q_in(0, 0), q_in(1, 1))
    group("wmb", wm_in(3, 5))
    group("w1", whole(w1_hbm, w1_v))
    group("w2", q_in(2, 2), whole(w2_hbm, w2_v))
    group("w3", whole(w3_hbm, w3_v))
    group("w4", whole(w4_hbm, w4_v.at[0:F]), wm_in(5, 6))
    for g in dmas.values():
        for c in g:
            c.start()

    def wait(name):
        for c in dmas[name]:
            c.wait()

    tau_b = lambda l: H + ((l + (H - 1)) & (H - 1))
    tf_v[:, C(0)] = _dft((T, H), 0, lambda l: jnp.where((l & 1) == 0, l, tau_b(l)), 1.0 / T)
    tf_v[:, C(1)] = _dft((T, H), 0, lambda l: jnp.where((l & 1) == 1, l, tau_b(l)), 1.0 / T)
    tf_v[:, C(2)] = _dft((T, H), 0, lambda l: 2 * l - H)
    tf_v[:, C(3)] = _dft((T, H), 0, lambda l: 2 * l + 1 - H)
    sin0 = lax.broadcasted_iota(I32, (GR, T), 1) >= H
    tg_v[:, 0:T] = _dft((GR, T), 1, lambda l: jnp.where(sin0 & (l == 0), H, 2 * l))
    tg_v[:, T:2 * T] = _dft((GR, T), 1, lambda l: 2 * l + 1)
    h1_v[:, 0:8, :] = jnp.zeros((NT, 8, 128), F32)
    h1_v[:, 8 + NC * T:16 + NC * T, :] = jnp.zeros((NT, 8, 128), F32)

    wait("small")
    z = jnp.clip(z_s[0, 0], 0, 1)
    zero = jnp.full((8, 128), z, I32).astype(U32)
    z8 = pl.multiple_of(z * 8, 8)
    for r in (x_v, hb_v, x1_v, r_v, zraw, n1_w, n2_w, g_w, a_w, kv_w, zz_w, *ws_w, *as_w, w3n_w, top_v, st_v):
        r[pl.ds(z8, 8), 0:128] = jnp.zeros((8, 128), r.dtype)
    for r in (kf, uf, acc, taps, mod_v):
        r[z, 0:8, 0:128] = jnp.zeros((8, 128), r.dtype)
    for r in (tf_w, tg_w):
        r[pl.ds(z8, 8), 0:128] = r[0:8, 0:128]
    sh = sh_v[...].astype(F32)
    for i in range(4):
        taps[i] = jnp.broadcast_to(sh[i:i + 1], (8, D))
    taps[4] = jnp.broadcast_to(sd_v[...].astype(F32).reshape(1, D) * (1.0 / T), (8, D))
    cf = c_v[...].astype(F32)
    silu_c = jnp.broadcast_to((cf / (1.0 + jnp.exp(-cf))).astype(BF16), (16, D))

    def mmK(n):
        def unit(m):
            st = []

            def rhs(i):
                if not st:
                    ev = (lax.broadcasted_iota(I32, (64, 128), 1) & 1) == 0
                    a = ssm_w[n][:, m * T:m * T + H]
                    b = pltpu.roll(ssm_w[n][:, m * T + H:(m + 1) * T], 1, 1)
                    st.extend([pltpu.bitcast(jnp.where(ev, a, b), BF16), pltpu.bitcast(jnp.where(ev, b, a), BF16)])
                return st[i]

            def epi(p):
                er, ei, or_, oi = p
                if m == 0:
                    er = er + taps[4, 0:1, C(n)]
                for h, (cr, ci) in enumerate(((er + or_, ei + oi), (er - or_, ei - oi))):
                    B = h * 3 * H
                    kf[m, B:B + H, C(n)] = cr
                    kf[m, B + H:B + 2 * H, C(n)] = ci - cr
                    kf[m, B + 2 * H:B + 3 * H, C(n)] = ci + cr
            return Unit("K%d" % n, [(lambda i=i, r=r: (tf_v[r:r + H, C(i)], rhs(i))) for i in range(2) for r in (0, H)],
                        epi, H, 170, nt=True)
        return [unit(m) for m in range(NB)]

    def kv(s, sl):
        def mk(t, w):
            def fn(a):
                ld = lambda o, n: k_n[s][t, pl.ds(8 + w + o, n), :]
                c0 = jnp.concatenate([_tie(ld(0, 8), a), ld(8, 8)], axis=0).reshape(2, 8, 128)
                c1, c2 = ld(-1, 16).reshape(2, 8, 128), ld(-2, 16).reshape(2, 8, 128)
                s0, s1, s2, s3 = (taps[i, :, C(t)] for i in range(4))
                ke, ko, ke1, ko1, ko2 = _lo(c0), _hi(c0), _lo(c1), _hi(c1), _hi(c2)
                wv = v_n[s][t, w:w + 16, :].reshape(2, 8, 128)
                kve = ((s0 * ke + s1 * ko1) + (s2 * ke1 + s3 * ko2)) * _lo(wv)
                kvo = ((s0 * ko + s1 * ke) + (s2 * ko1 + s3 * ke1)) * _hi(wv)
                kv_v[pl.ds(sl * T + w, 16), C(t)] = kve.reshape(16, 128).astype(BF16)
                kv_v[pl.ds(sl * T + H + w, 16), C(t)] = kvo.reshape(16, 128).astype(BF16)
            return fn
        return [[mk(t, w) for w in range(0, H, 16)] for t in range(NT)]

    def mmU(name, sl, us):
        def unit(n):
            def epi(p):
                er, ei, or_, oi = p
                for h, (cr, ci) in enumerate(((er + or_, ei + oi), (er - or_, ei - oi))):
                    B = h * 3 * H
                    uf[us, B:B + H, C(n)] = cr + ci
                    uf[us, B + H:B + 2 * H, C(n)] = cr
                    uf[us, B + 2 * H:B + 3 * H, C(n)] = ci
            return Unit(name(n), [(lambda i=i, r=r: (tf_v[r:r + H, C(2 + i)], kv_v[pl.ds(sl * T + i * H, H), C(n)]))
                                  for i in range(2) for r in (0, H)], epi, H, 120)
        return [unit(n) for n in range(NT)]

    def cmul(m0, u0, n, h, row, L, a):
        t = []
        for i in range(3):
            Rw = slice((3 * h + i) * H + row, (3 * h + i) * H + row + 8)
            kk = kf[m0:m0 + n, Rw, L]
            if i == 0 and a is not None:
                k0 = _tie(kk[0], a)[None]
                kk = k0 if n == 1 else jnp.concatenate([k0, kk[1:]], axis=0)
            t.append(jnp.sum(kk * uf[u0:u0 + n, Rw, L], axis=0))
        return t[0] - t[2], t[0] + t[1]

    def AR(h, q, row):
        return slice((2 * h + q) * H + row, (2 * h + q) * H + row + 8)

    def mac(n, u0, sl, first=False, part=False):
        def mk(t, rc):
            st, fin = [], []

            def piece(i):
                def fn(a):
                    h, row = i & 1, rc + (i >> 1) * 8
                    zr, zi = cmul(0, u0, n, h, row, C(t), a)
                    if part:
                        zr, zi = zr + acc[0, AR(h, 0, row), C(t)], zi + acc[0, AR(h, 1, row), C(t)]
                    st.append((zr, zi))
                    if h:
                        (pr, pi), (mr, mi) = st[-2:]
                        z = [pr + mr, pi + mi, pr - mr, pi - mi]
                        Rw = lambda q: slice(q * H + row, q * H + row + 8)
                        pv = None if first else [zraw[Rw(q ^ 1), C(t)] for q in range(4)]
                        for q in range(4):
                            zraw[Rw(q), C(t)] = z[q]
                        if not first:
                            z = [z[q] + pv[q] if (q & 1) == (rc < 64) else z[q] - pv[q] for q in range(4)]
                        fin.append(z)
                    if i == 3:
                        for q in range(4):
                            zz_v[pl.ds(sl * 2 * T + q * H + rc, 16), C(t)] = jnp.concatenate(
                                [fin[0][q], fin[1][q]], axis=0).astype(BF16)
                return fn
            if not part:
                return [piece(i) for i in range(4)]
            both = lambda f, g: (lambda a: (f(a), g(None)))
            return [both(piece(0), piece(1)), both(piece(2), piece(3))]
        return [[fn for rc in range(0, H, 16) for fn in mk(t, rc)] for t in range(NT)]

    def pos():
        return [(t, h, row) for t in range(NT) for row in range(0, H, 8) for h in range(2)]

    def ahead(i):
        def mk(t, h, row):
            def fn(a):
                zr, zi = cmul(i + 1, 0, NC, h, row, C(t), a)
                acc[i, AR(h, 0, row), C(t)] = zr
                acc[i, AR(h, 1, row), C(t)] = zi
            return fn
        return [mk(*p) for p in pos()]

    def spread():
        n = NB - NC - 1

        def mk(t, h, row):
            def fn(a):
                p = []
                for i in range(3):
                    Rw = slice((3 * h + i) * H + row, (3 * h + i) * H + row + 8)
                    u = uf[0, Rw, C(t)]
                    p.append(kf[1:1 + n, Rw, C(t)] * (_tie(u, a) if i == 0 else u)[None])
                acc[0:n, AR(h, 0, row), C(t)] = acc[1:1 + n, AR(h, 0, row), C(t)] + (p[0] - p[2])
                acc[0:n, AR(h, 1, row), C(t)] = acc[1:1 + n, AR(h, 1, row), C(t)] + (p[0] + p[1])
            return fn
        return [mk(*p) for p in pos()]

    def mmI(name, sl, ys):
        def unit(n):
            def epi(p):
                ce, se, co, so = p
                sub = lax.broadcasted_iota(I32, (8, 128), 0)
                c0 = ys * T + H
                y_v[n, ys * T:ys * T + 1, :] = (ce[64:72] - se[0:8])[0:1]
                se = jnp.concatenate([jnp.where(sub == 0, 0.0, se[0:8]), se[8:]], axis=0)
                for d, cc, ss in ((0, ce[0:64], se), (1, co, so)):
                    y_v[n, pl.ds(c0 + d, 64, stride=2), :] = cc + ss
                    lo = cc - ss
                    for i in range(0, 64, 8):
                        y_v[n, pl.ds(c0 - d - 2 * i - 14, 8, stride=2), :] = jnp.take_along_axis(
                            lo[i:i + 8], 7 - sub, axis=0)
            return Unit(name(n), [(lambda i=i: (tg_v[0:(GR if i == 0 else 64), C(i)], zz_v[pl.ds(sl * 2 * T + i * H, H), C(n)]))
                                  for i in range(4)], epi, 64, 52)
        return [unit(n) for n in range(NT)]

    def mod(name, a, b):
        def unit(n):
            def epi(p):
                v = [_sum(p[i * NT:(i + 1) * NT])[0:8] for i in range(b - a)]
                if a == 0:
                    mod_v[0, :, C(n)] = v[0] * v[2]
                    mod_v[1, :, C(n)] = (v[1] + 1.0) * v[2]
                elif a == 3:
                    mod_v[3, :, C(n)] = v[0]
                    mod_v[4, :, C(n)] = v[1] + 1.0
                else:
                    mod_v[5, :, C(n)] = v[0]
                    mod_v[2, :, C(n)] = v[0] * G_POST
            return Unit(name, [(lambda i=i, k=k: (silu_c[:, C(k)], wm_v[a][C(k), pl.ds(i * D + n * 128, 128)]))
                               for i in range(b - a) for k in range(NT)], epi, 16, 10, full=False, acc=b - a == 1)
        return [unit(n) for n in range(NT)]

    HS = (slice(0, 128), slice(128, 256))
    QS = tuple(slice(r, r + 64) for r in range(0, T, 64))

    def tasks(f, due=None, tie=True, n=RG):
        def mk(R):
            def fn(a):
                x = f(R, a if tie else None)
                return Due(x, due) if due else None
            return fn
        return [mk(slice(r, r + n)) for r in range(0, T, n)]

    def load_y(sl, R):
        return jnp.concatenate([y_v[t, sl * T + R.start:sl * T + R.stop, :] for t in range(NT)],
                               axis=1).reshape(2, 8, D)

    def put(nn, ss, R, x):
        nn[R, :] = x.astype(BF16)
        tok = x
        if ss is not None:
            S2 = pl.ds(R.start // 32 * 16, 16)
            if R.stop % 32:
                top_v[S2, 0:2 * T] = x[:, 0:2 * T]
            else:
                if R.start % 32:
                    x = jnp.concatenate([top_v[S2, 0:2 * T], x[:, 0:2 * T]], axis=0)
                ss[S2, 0:5 * T] = jnp.concatenate(_lhs_sums(x[:, 0:T], x[:, T:2 * T]), axis=1).astype(BF16)
        return tok

    wide = lambda v: jnp.concatenate([v] * NT, axis=1)

    def mean(i, R, x):
        st_v[R, C(i)] = jnp.broadcast_to(jnp.sum(x, axis=-1, keepdims=True) * (1.0 / D), (x.shape[0], 128))

    def centred(src, i, R, a):
        return src[R, :] - wide(_tie(st_v[R, C(i)], a))

    def scale(src, i, g):
        def f(R, a):
            st_v[R, C(i + 1)] = jnp.broadcast_to(_rstd(centred(src, i, R, a), g), (RG, 128))
        return f

    def normed(src, i, R, a):
        return centred(src, i, R, a) * wide(st_v[R, C(i + 1)])

    def front(sl, xs, early=False, ss=None):
        xx, hh, nn = view(x_v, xs), view(hb_v, xs), view(n1_v, sl)

        def fa(R, a):
            q = [q_n[sl][t, R.start // 2:R.stop // 2, :] for t in range(NT)]
            q = jnp.concatenate([_tie(q[0], a)] + q[1:], axis=1)
            q = pltpu.bitcast(q, BF16).astype(F32).reshape(2, 8, D)
            x = (q + (_ln(q) * mod_v[1] + mod_v[0]) * load_y(sl, R)).reshape(RG, D)
            xx[R, :] = x
            if early:
                hh[R, :] = _ln(x)

        def fb(R, a):
            hh[R, :] = (_ln(_tie(xx[R, :], a).reshape(2, 8, D)) * mod_v[4] + mod_v[3]).reshape(RG, D)

        def fc(R, a):
            hb = _tie(hh[R, :], a)
            if early:
                hb = (hb.reshape(2, 8, D) * mod_v[4] + mod_v[3]).reshape(RG, D)
                hh[R, :] = hb
            nn[R, :] = _ln(hb, G_A).astype(BF16)
        if early:
            return tasks(fa), tasks(fc)
        if ss is None:
            return tasks(fa) + tasks(fb) + tasks(fc)
        qf = view(x_v, 2)

        def s1(R, a):
            q = [q_n[sl][t, R.start // 2:R.stop // 2, :] for t in range(NT)]
            q = pltpu.bitcast(jnp.concatenate([_tie(v, a) for v in q], axis=1), BF16).astype(F32)
            qf[R, :] = q
            mean(0, R, q)

        def s3(R, a):
            h = normed(qf, 0, R, a).reshape(2, 8, D) * mod_v[1] + mod_v[0]
            x = qf[R, :] + (h * load_y(sl, R)).reshape(RG, D)
            xx[R, :] = x
            mean(2, R, x)

        def s5(R, a):
            hb = (normed(xx, 2, R, a).reshape(2, 8, D) * mod_v[4] + mod_v[3]).reshape(RG, D)
            hh[R, :] = hb
            mean(4, R, hb)
        s7 = [f for g in tasks(lambda R, a: put(nn, ss, R, normed(hh, 4, R, a)), n=32) for f in (g, lambda a: None)]
        st = [tasks(s3), tasks(scale(xx, 2, 1.0)), tasks(s5), tasks(scale(hh, 4, G_A)), s7]
        p = [tasks(s1), tasks(scale(qf, 0, 1.0))]
        return cat(x[:8] for x in st), cat(x[8:] for x in p + st), cat(x[:8] for x in p)

    def shift(hs, sl, pieces=((0, 64), (64, 64), (128, 64), (192, 64)), ss=None):
        gg = view(g_v, sl)

        def one_tile(t, r, n, a):
            lane = lax.broadcasted_iota(I32, (n, 128), 1)
            ld = lambda d: h1_v[t, pl.ds(hs * T + 8 + r + d, n), :]
            if t == 0:
                g = ld(-1)
            elif t == 1:
                g = jnp.where(lane < 32, ld(-1), ld(1))
            elif t == 2:
                g = jnp.where(lane < 64, ld(1), ld(-2))
            elif t == 3:
                g = jnp.where(lane < 96, ld(-2), ld(2))
            else:
                g = ld(2)
            if a is not None:
                g = jnp.concatenate([_tie(g[i:i + 8], a) if i % 16 == 0 else g[i:i + 8]
                                     for i in range(0, n, 8)], axis=0)
            gg[r:r + n, C(t)] = g.astype(BF16)
            return g

        def mk(ts, r, n):
            def fn(a):
                g = [one_tile(t, r, n, a) for t in ts]
                if len(ts) == 2:
                    for i, x in enumerate(_lhs_sums(*g)):
                        ss[r // 2:(r + n) // 2, C(2 * i + ts[0])] = x.astype(BF16)
            return fn
        sets = [(t,) for t in range(NT)] if ss is None else [(0, 2), (1, 3), (4,)]
        return [mk(ts, r, n) for ts in sets for r, n in pieces]

    def shift_early():
        def keep(a):
            h1_v[:, 2 * T - 32:2 * T + 8, :] = h1_v[:, 3 * T - 32:3 * T + 8, :]
        return shift(2, 0, [(r, 32) for r in range(0, T - 32, 32)], gs) + [keep]

    def ln2(xs, sl, fast=True):
        xx, nn, ss = view(x1_v, xs), view(n2_v, sl), view(n2s, sl, H) if fast else None
        f = lambda R, a: put(nn, ss, R, _ln(_tie(xx[R, :], a), G_A))
        ts = tasks(f, DL, False)
        return ts[0::2] + ts[1::2] if fast else tasks(f)

    def resid(xs, x1s, rotate=False):
        xx, x1 = view(x_v, xs), view(x1_v, x1s)

        def f(R, a):
            gb = mod_v[5] if a is None else pltpu.bitcast(
                pltpu.bitcast(mod_v[5], U32) | jnp.concatenate([a] * NT, axis=1), F32)
            r_v[R, :] = xx[R, :] + (x1[R, :].reshape(2, 8, D) * gb).reshape(RG, D)
            if rotate:
                xx[R, :] = x_v[R, :]
                view(hb_v, 1)[R, :] = hb_v[R, :]
        return tasks(f)

    KD, KF, ND = [(0, 2), (1, 3)], [(2 * i, 2 * i + 1) for i in range(7)], [(1, 2), (3, 4)]
    Wt = {1: (lambda k, n: w1_v[C(k), C(n)], lambda i, kp, j: w1s[C(kp), C(2 * i + j)], False, KD, [4]),
          2: (lambda k, n: w2_v[C(k), C(n)], lambda i, kp, j: w2s[C(kp), C(2 * i + j)], False, KD, [4]),
          0: (lambda k, n: w3_v[C(n), C(k)], None, True, KD, [4]),
          3: (lambda k, n: w3n[C(k), C(n)], lambda i, kp, j: w3s[C(kp), C(6 * i + j)], False, KD, [4]),
          4: (lambda k, n: w4_v[C(k), C(n)], lambda i, kp, j: w4s[C(kp), C(2 * i + j)], False, KF, [])}

    def wsums(w_w, ws, rp, cp_):
        def mk(i, j, r):
            def fn(a):
                b = [[w_w[pl.ds(64 * p + r // 2, 8), C(q)] for q in cp_[j]] for p in rp[i]]
                b[0][0], b[1][1] = _tie(b[0][0], a), _tie(b[1][1], a)
                (b11, b12), (b21, b22) = [[pltpu.bitcast(x, BF16).astype(F32) for x in row] for row in b]
                for m, x in enumerate((b11 + b22, b12 - b22, b21 - b11, b11 + b12, b21 + b22)):
                    ws[pl.ds(128 * i + r, 16), C(len(cp_) * m + j)] = x.astype(BF16)
            return fn
        return [mk(i, j, r) for j in range(len(cp_)) for i in range(len(rp)) for r in range(0, 128, 16)]

    def w3_turn():
        def mk(n, k):
            def fn(a):
                x = jnp.concatenate([_tie(w3_w[64 * n:64 * n + 8, C(k)], a), w3_w[64 * n + 8:64 * n + 64, C(k)]], axis=0)
                w3n[C(k), C(n)] = pltpu.bitcast(x, BF16).T
            return fn
        return [mk(n, k) for n in range(FT - 1) for k in range(NT)]

    def plain(name, w, lhs, n, R, epi, cost):
        tile, _, nt, kp, kl = Wt[w]
        ks = sorted([k for p in kp for k in p] + kl)
        rows_ = R.stop - R.start
        return Unit(name, [(lambda k=k: (lhs[R, C(k)], tile(k, n))) for k in ks], lambda p: epi(n, R, p[0]),
                    rows_, rows_ // 8 * (len(ks) - 1 + cost), nt=nt, acc=True)

    def quad(name, w, lhs, sums, j, cols_, R, epi, cost):
        tile, wsum, nt, kp, kl = Wt[w]
        h, S2, c = len(kp), slice(R.start // 2, R.stop // 2), {}
        a_ = lambda i, k: _top(lhs[R, C(k)], i)
        s_ = lambda i, p: sums[S2, C(h * i + p)]
        prod = lambda fa_, fb_: [(lambda p=p: (fa_(p), fb_(p))) for p in range(h)]
        left = lambda i, n: [(lambda k=k: (a_(i, k), tile(k, n))) for k in kl]
        mk = lambda tiles, f, x=0: Unit(name, tiles, lambda p: f(p[0]), 64, 8 * len(tiles) + x, nt=nt, acc=True)

        def e1(m):
            u7.res, u6.res = [m], [m]

        def e4(m):
            c[11], c[21] = c[11] + m, m

        def e2(m):
            c[21], c[22] = c[21] + m, c[22] - m
            l21.res = [c[21]]

        def e5(m):
            c[12] = m
            epi(cols_[0], R, _zip(c[11] - m, c[21]))

        def e3(m):
            l12.res, c[22] = [c[12] + m], c[22] + m
            if not kl:
                l12.epi(l12.res)
        u1 = mk(prod(lambda p: s_(0, p), lambda p: wsum(0, p, j)), e1)
        u7 = mk(prod(lambda p: s_(4, p), lambda p: wsum(4, p, j)) + left(0, cols_[0]), lambda m: c.update({11: m}))
        u6 = mk(prod(lambda p: s_(3, p), lambda p: wsum(3, p, j)) + left(1, cols_[1]), lambda m: c.update({22: m}))
        u4 = mk(prod(lambda p: a_(1, kp[p][1]), lambda p: wsum(2, p, j)), e4)
        u2 = mk(prod(lambda p: s_(1, p), lambda p: tile(kp[p][0], cols_[0])), e2, 8)
        l21 = mk(left(1, cols_[0]), lambda m: c.update({21: m}))
        u5 = mk(prod(lambda p: s_(2, p), lambda p: tile(kp[p][1], cols_[1])), e5, 16 * cost)
        u3 = mk(prod(lambda p: a_(0, kp[p][0]), lambda p: wsum(1, p, j)), e3, 8 if kl else 8 + 16 * cost)
        l12 = mk(left(0, cols_[1]), lambda m: epi(cols_[1], R, _zip(m, c[22])), 16 * cost)
        return [u1, u7, u6, u4, u2, l21, u5, u3, l12]

    def mm(name, w, lhs, sums, epi, cost):
        if sums is None:
            return [[plain(name, w, lhs, n, R, epi, cost) for R in HS] for n in range(NT)]
        return [[plain(name, w, lhs, 0, R, epi, cost) for R in QS]] + [
            [u for R in HS for u in quad(name, w, lhs, sums, j, ND[j], R, epi, cost)] for j in range(2)]

    def mm1(name, hs, sl, fast=False):
        def epi(n, R, p):
            h1_v[n, pl.ds(hs * T + 8 + R.start, R.stop - R.start), :] = _gelu2(p)
        return cat(mm(name, 1, view(n1_v, sl), n1s if fast else None, epi, 5))

    def mm2(name, sl, xs, x1s, fast=False):
        def epi(n, R, p):
            view(x1_v, x1s)[R, C(n)] = view(hb_v, xs)[R, C(n)] + p * G_POST
        return cat(mm(name, 2, view(g_v, sl), gs if fast else None, epi, 2))

    def mm3(name, sl, fast=True):
        nn, aa, ss, keep, tail = view(n2_v, sl), view(a_v, sl), view(a_s, sl, H), [], []

        def epi(n, R, p):
            g = _gelu2(p)
            aa[R, C(n)] = g.astype(BF16)
            if n % 2 == 0 and n < 12:
                keep.append(g)
                return
            pair = (keep.pop(), g) if n % 2 else (g, tail[R.start // 128][R.start % 128:R.start % 128 + 64])
            for i, x in enumerate(_lhs_sums(*pair)):
                ss[R.start // 2:R.stop // 2, C(7 * i + n // 2)] = x.astype(BF16)

        def rem(R):
            def f(p):
                tail.append(jnp.concatenate([_gelu2(p[0]), jnp.zeros((64, 128), F32)], axis=0).T)
                aa[R, C(13)] = tail[-1].astype(BF16)
            return Unit(name, [(lambda k=k: (w3_v[13 * 128:F, C(k)], nn[R, C(k)])) for k in range(NT)], f, 64, 84,
                        nt=True, acc=True)
        odd = [rem(R) for R in HS] + [plain(name, 3 if fast else 0, nn, 12, R, epi, 9) for R in QS]
        if fast:
            qd = [u for j in range(6) for R in HS for u in quad(name, 3, nn, view(n2s, sl, H), j, KF[j], R, epi, 8)]
            return qd[:18] + odd[:2] + qd[18:36] + odd[2:] + qd[36:]
        return odd + [plain(name, 0, nn, n, R, epi, 8) for p in KF[:6] for R in HS for n in p]

    NA = 3 * 128

    def cp_out(j, osl, L, sm, R=slice(0, T)):
        return cp(o_v.at[pl.ds(osl * T + R.start, R.stop - R.start), L],
                  o_hbm.at[pl.ds(base(j, T) + R.start, R.stop - R.start), L], sem_o.at[sm])

    out_a = lambda j: cp_out(j, 0, slice(0, NA), 0)
    out_b = lambda j: cp_out(j, 0, slice(NA, D), 1)
    last = []

    def mm4(name, j, sl, osl=0, xs=None, x1s=None, fast=True):
        oo = view(o_v, osl)

        def epi(n, R, p):
            if xs is None:
                oo[R, C(n)] = (r_v[R, C(n)] + mod_v[2, 0:1, C(n)] * p).astype(BF16)
            else:
                oo[R, C(n)] = (view(x_v, xs)[R, C(n)] + mod_v[5, 0:1, C(n)]
                               * (view(x1_v, x1s)[R, C(n)] + p * G_POST)).astype(BF16)
            if osl == 2:
                last.append(cp_out(j, osl, C(n), 2, R))
                last[-1].start()
            elif R.stop == T and (osl, (n + 1) * 128) in ((1, D), (3, NA)):
                last.append(cp_out(j, osl, slice(0, (n + 1) * 128), 2))
                last[-1].start()
            elif R.stop == T and osl == 0 and (n + 1) * 128 in (NA, D):
                (out_a if (n + 1) * 128 == NA else out_b)(j).start()
        return mm(name, 4, view(a_v, sl), view(a_s, sl, H) if fast else None, epi, 3 if xs is None else 5)

    def split(us):
        n = 4 // len(us)
        m, mks, st = us[0].rows // n, [u.tiles.pop(0) for u in us], {}

        def piece(i, k):
            if i not in st:
                st[i] = mks[i]()
            return st[i][0][m * k:m * (k + 1)], st[i][1]

        def epi(p):
            for i, u in enumerate(us):
                u.res = [jnp.concatenate(p[n * i:n * (i + 1)], axis=0)]
        return _flat([Unit(us[0].name, [(lambda i=i, k=k: piece(i, k)) for i in range(len(us)) for k in range(n)],
                           epi, m, 0, nt=us[0].nt)])

    W = lambda nm: [("wait", nm)]
    run = lambda fns: [("run", "run", lambda: [fn(None) for fn in fns])]
    one = lambda us: [_flat([u]) for u in us]
    nm = lambda x: (lambda n: x)

    seq, grp = [], []
    for s in range(NC):
        seq += W("c%d" % s) + _flat(mmK(s) + mmU(nm("U%d" % s), s % 2, NC - 1 - s))
        grp.append(Group("kv%d" % s, cat(kv(s, s % 2)), 50, ["c%d" % s], ["U%d" % s], 100))
    inv = [mmI(lambda n: "I%d" % n, s, s) for s in range(NC)]
    seq += W("c3") + _flat(mmK(3) + mmK(4) + [inv[s][t] for t in range(NT) for s in range(NC)])
    macs = [mac(s + 1, NC - 1 - s, s, first=s == 0) for s in range(NC)]
    grp.append(Group("mac00", macs[0][0], 12, ["c1"], ["c2"], 0))
    grp.append(Group("mac01", macs[1][0] + macs[0][1] + macs[1][1], 16, ["c2"], ["c3"], 0))
    for t in range(NT):
        grp.append(Group("mac%d" % t, cat(macs[s][t] for s in range(2 if t < 2 else 0, NC)), 24 if t < 2 else 18,
                         ["c3", "K%d" % t], ["I%d" % t], 100, 150))
    start = lambda cs: [("run", "run", lambda: [c.start() for c in cs])]
    f0, f1 = front(0, 2, True), front(1, 1, True)
    seq += run(ahead(0))
    seq += W("wma") + _flat(mod("moda", 0, 3)) + run(f0[0] + f1[0] + ahead(1))
    seq += W("wmb") + start(next_kv(NC) + next_q(NC)) + _flat(mod("modb", 3, 5)) + run(f0[1])
    w1 = _flat(mm1("w1_0", 0, 0) + mm1("w1_1", 1, 1))
    seq += W("w1") + w1[:72] + W("w2") + w1[72:] + run(shift(0, 0))
    seq += _flat(mm2("w2_0", 0, 2, 1) + mm1("w1_2", 2, 2)) + run(shift(1, 1)) + _flat(mm2("w2_1", 1, 1, 0))
    grp.append(Group("f1", f1[1], 80, ["w1"], ["w1_1"], 450))
    grp.append(Group("f2", front(2, 0), 80, ["w2"], ["w1_2"], 450))
    grp.append(Group("ln2_0", ln2(1, 0, False), 60, ["w2_0"], ["w3"], 450))
    grp.append(Group("ahead", cat(ahead(i) for i in range(2, NB - NC)), 19, ["w1"], ["end"], 100))
    grp.append(Group("ws1", wsums(w1_w, w1s, KD, ND), 26, ["w1"], ["end"], 100))
    grp.append(Group("ws2", wsums(w2_w, w2s, KD, ND), 26, ["w2"], ["end"], 100))
    grp.append(Group("ws3", w3_turn() + wsums(w3n_w, w3s, KD, KF[:6]), 22, ["w3"], ["end"], 100))
    grp.append(Group("ws4", wsums(w4_w, w4s, KF, ND), 26, ["w4"], ["end"], 100))
    _wait(seq, "w3", back=1)
    w3 = mm3("w3_0", 0, False)
    _mix(seq, _flat(w3[6:]), [split(w3[4:6]) + _flat(w3[:6])], 0.1)
    mc = _flat(mod("modc", 5, 6))
    _wait(seq, "w4", mc[:5] + [("sync", "run", lambda: None)])
    w4 = cat(mm4("w4_0", 0, 0, 3, 2, 1, False)[:3])
    qs = [split([w4[-1 - i]]) for i in range((_phase(seq) + FT * 6) % 4)]
    _mix(seq, _flat(w4), [mc[i:i + 4] for i in range(5, 25, 4)] + qs, 0.01, 0.4)
    assert _phase(seq) == 0
    grp.append(Group("resid", resid(2, 1), 26, ["modc"], ["end"], 100))
    _emit(seq, grp, zero, wait)

    def step(s, carry):
        for c in next_kv(s) + next_q(s):
            c.wait()
        nxt = jnp.minimum(s + 1, NB - 1)
        seq, grp = [], []
        us, it = one(mmU(lambda n: "U%d" % n, 0, 0)), one(mmI(lambda n: "I%d" % n, 0, 0))
        w4 = mm4("w4", s - 2, 0)
        q = split(w4[0][2:])
        _mix(seq, _flat(mm4("w4c", s - 3, 0)[2] + mm3("w3", 0)),
             [us[0], us[1], us[2], it[0] + us[3], it[1] + us[4], it[2] + start(next_kv(nxt)), it[3], it[4]],
             0.26, 0.78)
        w1a, w1b = mm1("w1a", 2, 0, True), mm1("w1b", 2, 0, True)
        w1a, w1b = _flat(w1a[0:2] + w1a[4:13] + w1a[22:31]), _flat(w1b[2:4] + w1b[13:22] + w1b[31:])
        _mix(seq, _flat(w4[0] + w4[1][:9]), [q])
        seq += w1a + run(shift(1, 0, ((T - 32, 32),), gs)) + _flat(w4[1][9:]) + w1b[:8] + start(next_q(nxt)) + w1b[8:]
        seq += _flat(mm2("w2", 0, 1, 0, True))
        assert _phase(seq) == 0
        kvs, macs = kv(0, 0), mac(1, 0, 0, part=True)
        for t in range(NT):
            grp.append(Group("kv%d" % t, kvs[t], 50, ["start"], ["U%d" % t], 300))
            grp.append(Group("mac%d" % t, macs[t], 28, ["U%d" % t], ["I%d" % t], 300, 150))
        iall = ["I%d" % t for t in range(NT)]
        grp.append(Group("ln2", ln2(0, 0), 75, ["start"], ["w3"], 450))
        grp.append(Group("resid", resid(1, 0, True), 40, ["w4c"], ["w4", "I4"], 100))
        fr = front(0, 0, ss=n1s)
        grp.append(Group("fronta", fr[0], 50, iall, ["w1a"], 230))
        grp.append(Group("frontb", fr[1], 50, iall, ["w1b"], 230, 2200))
        grp.append(Group("fq", fr[2], 34, ["w4c"], ["I4"], 100))
        grp.append(Group("spread", spread(), 30, iall, ["end"], 100))
        grp.append(Group("shift", shift_early(), 24, ["start"], ["w1a"], 200))
        _emit(seq, grp, zero, wait)
        out_b(s - 3).wait()
        out_a(s - 2).wait()
        return carry

    lax.fori_loop(NC, NB, step, 0)

    seq, grp = [], []
    w4 = cat(mm4("w4_6", NB - 2, 0, 1, 1, 0))
    q = split(w4[2:4])
    seq += _flat(mm4("w4_5", NB - 3, 0)[2] + mm3("w3_6", 0) + mm2("w2_7", 0, 0, 1, True))
    _mix(seq, _flat(w4), [q])
    seq += _flat(mm3("w3_7", 1) + cat(mm4("w4_7", NB - 1, 1, 2, 0, 1)))
    assert _phase(seq) == 0
    grp.append(Group("ln2_6", ln2(0, 0), 75, ["start"], ["w3_6"], 450))
    grp.append(Group("shift7", shift(2, 0, [(r, 32) for r in range(0, T, 32)], gs), 24, ["start"], ["w2_7"], 200))
    grp.append(Group("ln2_7", ln2(1, 1), 75, ["w2_7"], ["w3_7"], 450))
    _emit(seq, grp, zero, wait)
    for c in next_kv(NB - 1) + next_q(NB - 1) + [out_b(NB - 3)] + last:
        c.wait()


@jax.jit
def pallas_adaLN_cond__ssm_conv_h3__mixer_s_mlp__prompt_kernel(
        A_q, A_k, A_v, A_shift_k, A_ssm_k, A_ssm_D, B_x, B_w1, B_w2, B_w3, B_w4, c, w_mod):
    any_ = pl.BlockSpec(memory_space=pl.ANY)
    V = pltpu.VMEM
    out = pl.pallas_call(
        kernel,
        in_specs=[any_] * 12,
        out_specs=any_,
        out_shape=jax.ShapeDtypeStruct((S, D), BF16),
        scratch_shapes=[
            [V((NT, H + 8, 128), U32)] * NC, [V((NT, H + 8, 128), U32)] * NC, [V((NT, H + 8, 128), U32)] * NC,
            [V((64, S), U32)] * NT,
            V((D // 2, D), U32), V((D // 2, D), U32), V((F // 2, D), U32), V((FT * 64, D), U32),
            [V((D // 2, 3 * D), U32), V((D // 2, 2 * D), U32), V((D // 2, D), U32)], V((4 * T, D), BF16),
            V((4, D), BF16), V((D,), BF16), V((1, D), BF16), V((8, 128), I32), pltpu.SMEM((8, 128), I32),
            V((5, 8, D), F32), V((6, 8, D), F32), V((T // 2, 4 * H), U32), V((GR // 2, 2 * T), U32),
            V((NB, 3 * T + 8, D), F32), V((NC, 3 * T + 8, D), F32), V((NB - NC, 2 * T + 8, D), F32), V((2 * T, D), F32),
            V((T, D), U32), V((NC * T, D), U32), V((NT, NC * T + 8, 128), F32),
            V((3 * T, D), F32), V((3 * T, D), F32), V((2 * T, D), F32), V((T, D), F32),
            V((3 * T // 2, D), U32), V((T, D), U32), V((T, D), U32), V((NT, NC * T + 24, 128), F32),
            V((T, (FT + 1) * 128), U32),
            [V((128, 11 * 128), U32)] * 2 + [V((128, 31 * 128), U32), V((448, 11 * 128), U32)],
            [V((64, 11 * 128), U32)] * 2 + [V((128, 11 * 128), U32), V((128, 35 * 128), U32)],
            V((D // 2, 13 * 128), U32), V((H, D), F32), V((T, 7 * 128), F32),
            pltpu.SemaphoreType.DMA((11,)), pltpu.SemaphoreType.DMA((1,)), pltpu.SemaphoreType.DMA((3,)),
        ],
        compiler_params=pltpu.CompilerParams(vmem_limit_bytes=110 << 20, disable_semaphore_checks=True,
                                             disable_bounds_checks=True),
        name="fused",
    )(A_q[0], A_k[0], A_v[0], A_shift_k.T, A_ssm_k, A_ssm_D, B_w1, B_w2, B_w3.T, B_w4, c, w_mod)
    return out[None]
```

```python
import heapq
import numpy as np
import jax
import jax.numpy as jnp
from jax import lax
from jax.experimental import pallas as pl
from jax.experimental.pallas import tpu as pltpu

S, D, F = 2048, 640, 1728
T = 256
H = T // 2
NB = S // T
NT = D // 128
FT = (F + 127) // 128
EPS = 1e-5
F32, BF16, U32, I32 = jnp.float32, jnp.bfloat16, jnp.uint32, jnp.int32
G_C1 = 0.044715 * float(np.sqrt(2.0 / np.pi))
G_C2 = float(np.sqrt(2.0 / np.pi))
G_A = G_C1 ** (1.0 / 3.0)
G_B = G_C2 / G_A
G_POST = 0.5 / G_A
RG = 16
GR = 80
NC = 3
DL = 450
SLOT = 32


def _dft(shape, f_axis, tau, scale=1.0):
    r = lax.broadcasted_iota(I32, shape, f_axis)
    l = lax.broadcasted_iota(I32, shape, 1 - f_axis)
    f = r & 127
    odd = ((f & 63) << 2) | ((f >> 6) << 1) | 1
    p = odd * tau(l) + ((r >> 7) << 8)
    a = ((p + 512) & 1023) - 512
    u = (256 - jnp.abs(a)).astype(F32) * (np.pi / 512.0)
    u2 = u * u
    c = [scale, -scale / 6.0, scale / 120.0, -scale / 5040.0, scale / 362880.0, -scale / 39916800.0]
    poly = c[5]
    for ci in c[4::-1]:
        poly = poly * u2 + ci
    return (u * poly).astype(BF16)


def _rstd(xc, scale):
    s2 = 1.0 / (scale * scale)
    v = jnp.sum(xc * xc, axis=-1, keepdims=True) * (s2 / D) + EPS * s2
    return jnp.exp2(jnp.log(v) * float(-0.5 / np.log(2.0)))


def _ln(x, scale=1.0):
    xc = x - jnp.sum(x, axis=-1, keepdims=True) * (1.0 / D)
    return xc * _rstd(xc, scale)


def _gelu2(x):
    u = x * (x * x + G_B)
    return x * (1.0 + jnp.tanh(u))


def _lo(w):
    return pltpu.bitcast(w << 16, F32)


def _hi(w):
    return pltpu.bitcast(w & jnp.uint32(0xFFFF0000), F32)


def _tie(x, a):
    if a is None:
        return x
    w = pltpu.bitcast(x[:, :128], U32)
    k = w.shape[0] // 8
    w = w | (a if k == 1 else jnp.concatenate([a] * k, axis=0))
    w = pltpu.bitcast(w, x.dtype)
    return w if x.shape[1] == 128 else jnp.concatenate([w, x[:, 128:]], axis=1)


def _top(x, i):
    return jnp.concatenate([x[r:r + 16] for r in range(16 * i, x.shape[0], 32)], axis=0)


def _zip(t, b):
    return jnp.concatenate([x[r:r + 16] for r in range(0, t.shape[0], 16) for x in (t, b)], axis=0)


def _lhs_sums(x1, x2):
    a11, a21, a12, a22 = _top(x1, 0), _top(x1, 1), _top(x2, 0), _top(x2, 1)
    return [a11 + a22, a21 + a22, a11 + a12, a21 - a11, a12 - a22]


def C(i):
    return slice(i * 128, (i + 1) * 128)


class Unit:
    def __init__(self, name, tiles, epi, rows, cost, nt=False, full=True, acc=False):
        self.acc, self.res = acc, []
        self.name, self.tiles, self.epi, self.rows, self.cost, self.nt, self.full = name, tiles, epi, rows, cost, nt, full


class Due:
    def __init__(self, val, delay):
        self.val, self.delay = val, delay


class Group:
    def __init__(self, name, fns, cost, rel, dead, lat, rlat=200):
        self.name, self.fns, self.cost, self.rel, self.dead, self.lat, self.rlat = name, fns, cost, rel, dead, lat, rlat


def _plan(seq, groups):
    busy, n = [0] * 4, 0
    start, end, tiles, bars = {}, {}, [], []
    for it in seq:
        if isinstance(it[0], Unit):
            u = it[0]
            m = n % 4
            n += 1
            t0, t1 = busy[m], busy[m] + max(u.rows, 32)
            busy[m] = t1
            tiles.append((t0, t1, u.cost / len(u.tiles)))
            start.setdefault(u.name, t0)
            end[u.name] = max(end.get(u.name, 0), t1)
        elif it[0] == "wait":
            t = max(busy)
            busy, n = [t] * 4, 0
            start[it[1]] = end[it[1]] = t
            bars.append(t)
    total = max(busy)
    start["end"] = end["end"] = total
    start["start"] = end["start"] = 0
    ns = total // SLOT + 2
    load = np.zeros(ns)
    for t0, t1, c in tiles:
        a, b = t0 // SLOT, max(t1 // SLOT, t0 // SLOT + 1)
        load[a:b] += c / (b - a)
    win = []
    for g in groups:
        r = max(end[x] + (0 if start[x] == end[x] else g.rlat) for x in g.rel)
        d = min(start[x] for x in g.dead) - g.lat
        ok = np.zeros(ns, bool)
        ok[r // SLOT:max(d // SLOT, r // SLOT + 1)] = True
        for b in bars:
            if r < b <= d:
                ok[max((b - g.lat) // SLOT, 0):b // SLOT] = False
        win.append(np.nonzero(ok)[0])
    alloc = [np.zeros(len(w)) for w in win]
    for _ in range(60):
        for i, g in enumerate(groups):
            w = win[i]
            load[w] -= alloc[i]
            base = load[w]
            vol = g.cost * len(g.fns)
            lo, hi = base.min(), base.max() + vol
            for _ in range(50):
                mid = 0.5 * (lo + hi)
                if np.maximum(mid - base, 0).sum() > vol:
                    hi = mid
                else:
                    lo = mid
            alloc[i] = np.maximum(hi - base, 0)
            load[w] += alloc[i]
    times = []
    for i, g in enumerate(groups):
        cum = np.cumsum(alloc[i])
        ts = []
        for k in range(len(g.fns)):
            x = (k + 0.5) * cum[-1] / len(g.fns)
            j = int(np.searchsorted(cum, x))
            prev = cum[j - 1] if j else 0.0
            ts.append(win[i][j] * SLOT + SLOT * (x - prev) / max(alloc[i][j], 1e-9))
        times.append(ts)
    return times


def _emit(seq, groups, zero, wait):
    times = _plan(seq, groups)
    left = {"start": 0}
    for it in seq:
        nm = it[0].name if isinstance(it[0], Unit) else it[1]
        left[nm] = left.get(nm, 0) + 1
    heap, pend, todo, cnt = [], {}, list(range(len(groups))), 0
    busy, n, due = [0] * 4, 0, []

    def release():
        nonlocal cnt
        for i in list(todo):
            g = groups[i]
            if all(left[x] == 0 for x in g.rel):
                todo.remove(i)
                pend[i] = len(g.fns)
                for t, fn in zip(times[i], g.fns):
                    heapq.heappush(heap, (t, cnt, i, fn))
                    cnt += 1

    def force(name):
        nonlocal heap
        for i, g in enumerate(groups):
            if name in g.dead:
                assert i not in todo, (g.name, name)
                if pend[i]:
                    for it in sorted(x for x in heap if x[2] == i):
                        it[3](None)
                    heap = [x for x in heap if x[2] != i]
                    heapq.heapify(heap)
                    pend[i] = 0

    release()
    for it in seq:
        if isinstance(it[0], Unit):
            u, k = it
            force(u.name)
            lhs, rhs = u.tiles[k]()
            t0 = busy[n % 4]
            while u.full and due and due[0][0] < t0 + u.rows:
                t, x = due.pop(0)
                r = min(max(int(t - t0), 0), u.rows - 1) // 16 * 8
                w = pltpu.bitcast(lhs, U32)
                x = pltpu.bitcast(x[:, :128], U32)
                parts = [w[:r], w[r:r + 8] | ((x[0:8] | x[8:16]) & zero), w[r + 8:]]
                lhs = pltpu.bitcast(jnp.concatenate([y for y in parts if y.shape[0]], axis=0), BF16)
            dn = (((1,), (1 if u.nt else 0,)), ((), ()))
            p = lax.dot_general(lhs, rhs, dn, preferred_element_type=F32)
            u.res = [p + u.res[0]] if (u.acc and u.res) else u.res + [p]
            m = n % 4
            n += 1
            t0 = busy[m]
            busy[m] = t0 + max(u.rows, 32)
            while u.full and heap and heap[0][0] < t0 + u.rows:
                t, _, i, fn = heapq.heappop(heap)
                pend[i] -= 1
                r = min(max(int(t - t0), 0), u.rows - 1) // 8 * 8
                x = fn(pltpu.bitcast(p[r:r + 8], U32) & zero)
                if isinstance(x, Due):
                    due.append((t + x.delay, x.val))
                    due.sort(key=lambda e: e[0])
            if k == len(u.tiles) - 1:
                u.epi(u.res)
            left[u.name] -= 1
        elif it[0] == "wait":
            force(it[1])
            wait(it[1])
            busy, n, due = [max(busy)] * 4, 0, []
            left[it[1]] -= 1
        else:
            it[2]()
            left[it[1]] -= 1
        release()
    force("end")
    assert not heap and not todo


def _sum(ps):
    acc = ps[0]
    for p in ps[1:]:
        acc = acc + p
    return acc


def _flat(us):
    return [(u, i) for u in us for i in range(len(u.tiles))]


def _phase(seq):
    n = 0
    for it in seq:
        n = n + 1 if isinstance(it[0], Unit) else (0 if it[0] in ("wait", "sync") else n)
    return n % 4


def _mix(seq, a, b, lo=0.0, hi=1.0):
    n, k = _phase(seq), 0
    for i, t in enumerate(a):
        if k < len(b) and n % 4 == 0 and t[1] != 1 and i >= len(a) * (lo + (hi - lo) * k / len(b)):
            seq.extend(b[k])
            k += 1
        seq.append(t)
        n += 1
    assert k == len(b)


def _wait(seq, name, head=(), back=0):
    r = _phase(seq) + 4 * back
    assert all(isinstance(it[0], Unit) for it in seq[len(seq) - r:])
    seq[len(seq) - r:len(seq) - r] = [("wait", name)] + list(head)


def kernel(q_hbm, k_hbm, v_hbm, sh_hbm, ssm_hbm, sd_hbm, w1_hbm, w2_hbm, w3_hbm, w4_hbm, c_hbm, wm_hbm,
           o_hbm,
           q_n, k_n, v_n, ssm_w, w1_w, w2_w, w3_w, w4_w, wm_w, o_v,
           sh_v, sd_v, c_v, zsrc, z_s, taps, mod_v, tf_w, tg_w,
           kf, uf, acc, zraw, kv_w, zz_w, y_v, x_v, hb_v, x1_v, r_v, n1_w, n2_w, g_w, h1_v, a_w,
           ws_w, as_w, w3n_w, top_v, st_v, l2_w,
           sem, sem_b, sem_o):
    bf = lambda r: r.bitcast(BF16)
    w1_v, w2_v, w3_v, w4_v = bf(w1_w), bf(w2_w), bf(w3_w), bf(w4_w)
    wm_v = {0: bf(wm_w[0]), 3: bf(wm_w[1]), 5: bf(wm_w[2])}
    tf_v, tg_v, n1_v, n2_v, g_v = bf(tf_w), bf(tg_w), bf(n1_w), bf(n2_w), bf(g_w)
    a_v, kv_v, zz_v = bf(a_w), bf(kv_w), bf(zz_w)
    w1s, w2s, w3s, w4s = [bf(r) for r in ws_w]
    n1s, gs, n2s, a_s = [bf(r) for r in as_w]
    w3n = bf(w3n_w)
    w3t, w4t, n2t, a_t = [bf(r) for r in l2_w]
    cp = pltpu.make_async_copy
    cat = lambda ls: [x for l in ls for x in l]

    def base(j, n):
        return j * n if isinstance(j, int) else pl.multiple_of(j * n, n)

    def rows(j, n=1, size=T):
        return pl.ds(base(j, size), n * size)

    def view(ref, j, size=T):
        return ref.at[rows(j, 1, size)]

    dmas = {}

    def group(name, *mks):
        sm = sem.at[len(dmas)]
        dmas[name] = [c for mk in mks for c in mk(sm)]

    def ssm_in(t):
        return lambda sm: [cp(ssm_hbm.at[C(t)], bf(ssm_w[t]), sm)]

    def cols(src, start, n, dst, row=0):
        return lambda sm: [cp(src.at[pl.ds(start, n), C(t)], bf(dst).at[t, pl.ds(row, n)], sm) for t in range(NT)]

    def kv_in(s, sl):
        if isinstance(s, int):
            kk = cols(k_hbm, s * T - 16, T + 16, k_n[sl]) if s else cols(k_hbm, 0, T, k_n[sl], 16)
        else:
            kk = cols(k_hbm, pl.multiple_of(s * T - 16, 16), T + 16, k_n[sl])
        return lambda sm: kk(sm) + cols(v_hbm, base(s, T), T, v_n[sl])(sm)

    def q_in(s, sl):
        return cols(q_hbm, base(s, T), T, q_n[sl])

    def wm_in(a, b):
        return lambda sm: [cp(wm_hbm.at[:, a * D:b * D], wm_v[a], sm)]

    def whole(src, dst):
        return lambda sm: [cp(src, dst, sm)]

    next_kv = lambda s: kv_in(s, 0)(sem_b.at[0])
    next_q = lambda s: q_in(s, 0)(sem_b.at[0])

    zsrc[...] = jnp.zeros((8, 128), I32)
    k_n[0][:, 0:8, :] = jnp.zeros((NT, 8, 128), U32)
    w4_w[F // 2:FT * 64, :] = jnp.zeros((FT * 64 - F // 2, D), U32)
    group("small", lambda sm: [cp(zsrc, z_s, sm), cp(sh_hbm, sh_v, sm), cp(sd_hbm, sd_v, sm), cp(c_hbm, c_v, sm)])
    for s in range(NC):
        group("c%d" % s, ssm_in(s), kv_in(s, s))
    group("c3", ssm_in(3), ssm_in(4))
    group("wma", wm_in(0, 3), q_in(0, 0), q_in(1, 1))
    group("wmb", wm_in(3, 5))
    group("w1", whole(w1_hbm, w1_v))
    group("w2", q_in(2, 2), whole(w2_hbm, w2_v))
    group("w3", whole(w3_hbm, w3_v))
    group("w4", whole(w4_hbm, w4_v.at[0:F]), wm_in(5, 6))
    for g in dmas.values():
        for c in g:
            c.start()

    def wait(name):
        for c in dmas[name]:
            c.wait()

    tau_b = lambda l: H + ((l + (H - 1)) & (H - 1))
    tf_v[:, C(0)] = _dft((T, H), 0, lambda l: jnp.where((l & 1) == 0, l, tau_b(l)), 1.0 / T)
    tf_v[:, C(1)] = _dft((T, H), 0, lambda l: jnp.where((l & 1) == 1, l, tau_b(l)), 1.0 / T)
    tf_v[:, C(2)] = _dft((T, H), 0, lambda l: 2 * l - H)
    tf_v[:, C(3)] = _dft((T, H), 0, lambda l: 2 * l + 1 - H)
    sin0 = lax.broadcasted_iota(I32, (GR, T), 1) >= H
    tg_v[:, 0:T] = _dft((GR, T), 1, lambda l: jnp.where(sin0 & (l == 0), H, 2 * l))
    tg_v[:, T:2 * T] = _dft((GR, T), 1, lambda l: 2 * l + 1)
    h1_v[:, 0:8, :] = jnp.zeros((NT, 8, 128), F32)
    h1_v[:, 8 + NC * T:16 + NC * T, :] = jnp.zeros((NT, 8, 128), F32)

    wait("small")
    z = jnp.clip(z_s[0, 0], 0, 1)
    zero = jnp.full((8, 128), z, I32).astype(U32)
    z8 = pl.multiple_of(z * 8, 8)
    for r in (x_v, hb_v, x1_v, r_v, zraw, n1_w, n2_w, g_w, a_w, kv_w, zz_w, *ws_w, *as_w, w3n_w, top_v, st_v, *l2_w):
        r[pl.ds(z8, 8), 0:128] = jnp.zeros((8, 128), r.dtype)
    for r in (kf, uf, acc, taps, mod_v):
        r[z, 0:8, 0:128] = jnp.zeros((8, 128), r.dtype)
    for r in (tf_w, tg_w):
        r[pl.ds(z8, 8), 0:128] = r[0:8, 0:128]
    sh = sh_v[...].astype(F32)
    for i in range(4):
        taps[i] = jnp.broadcast_to(sh[i:i + 1], (8, D))
    taps[4] = jnp.broadcast_to(sd_v[...].astype(F32).reshape(1, D) * (1.0 / T), (8, D))
    cf = c_v[...].astype(F32)
    silu_c = jnp.broadcast_to((cf / (1.0 + jnp.exp(-cf))).astype(BF16), (16, D))

    def mmK(n):
        def unit(m):
            st = []

            def rhs(i):
                if not st:
                    ev = (lax.broadcasted_iota(I32, (64, 128), 1) & 1) == 0
                    a = ssm_w[n][:, m * T:m * T + H]
                    b = pltpu.roll(ssm_w[n][:, m * T + H:(m + 1) * T], 1, 1)
                    st.extend([pltpu.bitcast(jnp.where(ev, a, b), BF16), pltpu.bitcast(jnp.where(ev, b, a), BF16)])
                return st[i]

            def epi(p):
                er, ei, or_, oi = p
                if m == 0:
                    er = er + taps[4, 0:1, C(n)]
                for h, (cr, ci) in enumerate(((er + or_, ei + oi), (er - or_, ei - oi))):
                    B = h * 3 * H
                    kf[m, B:B + H, C(n)] = cr
                    kf[m, B + H:B + 2 * H, C(n)] = ci - cr
                    kf[m, B + 2 * H:B + 3 * H, C(n)] = ci + cr
            return Unit("K%d" % n, [(lambda i=i, r=r: (tf_v[r:r + H, C(i)], rhs(i))) for i in range(2) for r in (0, H)],
                        epi, H, 170, nt=True)
        return [unit(m) for m in range(NB)]

    def kv(s, sl):
        def mk(t, w):
            def fn(a):
                ld = lambda o, n: k_n[s][t, pl.ds(8 + w + o, n), :]
                c0 = jnp.concatenate([_tie(ld(0, 8), a), ld(8, 8)], axis=0).reshape(2, 8, 128)
                c1, c2 = ld(-1, 16).reshape(2, 8, 128), ld(-2, 16).reshape(2, 8, 128)
                s0, s1, s2, s3 = (taps[i, :, C(t)] for i in range(4))
                ke, ko, ke1, ko1, ko2 = _lo(c0), _hi(c0), _lo(c1), _hi(c1), _hi(c2)
                wv = v_n[s][t, w:w + 16, :].reshape(2, 8, 128)
                kve = ((s0 * ke + s1 * ko1) + (s2 * ke1 + s3 * ko2)) * _lo(wv)
                kvo = ((s0 * ko + s1 * ke) + (s2 * ko1 + s3 * ke1)) * _hi(wv)
                kv_v[pl.ds(sl * T + w, 16), C(t)] = kve.reshape(16, 128).astype(BF16)
                kv_v[pl.ds(sl * T + H + w, 16), C(t)] = kvo.reshape(16, 128).astype(BF16)
            return fn
        return [[mk(t, w) for w in range(0, H, 16)] for t in range(NT)]

    def mmU(name, sl, us):
        def unit(n):
            def epi(p):
                er, ei, or_, oi = p
                for h, (cr, ci) in enumerate(((er + or_, ei + oi), (er - or_, ei - oi))):
                    B = h * 3 * H
                    uf[us, B:B + H, C(n)] = cr + ci
                    uf[us, B + H:B + 2 * H, C(n)] = cr
                    uf[us, B + 2 * H:B + 3 * H, C(n)] = ci
            return Unit(name(n), [(lambda i=i, r=r: (tf_v[r:r + H, C(2 + i)], kv_v[pl.ds(sl * T + i * H, H), C(n)]))
                                  for i in range(2) for r in (0, H)], epi, H, 120)
        return [unit(n) for n in range(NT)]

    def cmul(m0, u0, n, h, row, L, a):
        t = []
        for i in range(3):
            Rw = slice((3 * h + i) * H + row, (3 * h + i) * H + row + 8)
            kk = kf[m0:m0 + n, Rw, L]
            if i == 0 and a is not None:
                k0 = _tie(kk[0], a)[None]
                kk = k0 if n == 1 else jnp.concatenate([k0, kk[1:]], axis=0)
            t.append(jnp.sum(kk * uf[u0:u0 + n, Rw, L], axis=0))
        return t[0] - t[2], t[0] + t[1]

    def AR(h, q, row):
        return slice((2 * h + q) * H + row, (2 * h + q) * H + row + 8)

    def mac(n, u0, sl, first=False, part=False):
        def mk(t, rc):
            st, fin = [], []

            def piece(i):
                def fn(a):
                    h, row = i & 1, rc + (i >> 1) * 8
                    zr, zi = cmul(0, u0, n, h, row, C(t), a)
                    if part:
                        zr, zi = zr + acc[0, AR(h, 0, row), C(t)], zi + acc[0, AR(h, 1, row), C(t)]
                    st.append((zr, zi))
                    if h:
                        (pr, pi), (mr, mi) = st[-2:]
                        z = [pr + mr, pi + mi, pr - mr, pi - mi]
                        Rw = lambda q: slice(q * H + row, q * H + row + 8)
                        pv = None if first else [zraw[Rw(q ^ 1), C(t)] for q in range(4)]
                        for q in range(4):
                            zraw[Rw(q), C(t)] = z[q]
                        if not first:
                            z = [z[q] + pv[q] if (q & 1) == (rc < 64) else z[q] - pv[q] for q in range(4)]
                        fin.append(z)
                    if i == 3:
                        for q in range(4):
                            zz_v[pl.ds(sl * 2 * T + q * H + rc, 16), C(t)] = jnp.concatenate(
                                [fin[0][q], fin[1][q]], axis=0).astype(BF16)
                return fn
            if not part:
                return [piece(i) for i in range(4)]
            both = lambda f, g: (lambda a: (f(a), g(None)))
            return [both(piece(0), piece(1)), both(piece(2), piece(3))]
        return [[fn for rc in range(0, H, 16) for fn in mk(t, rc)] for t in range(NT)]

    def pos():
        return [(t, h, row) for t in range(NT) for row in range(0, H, 8) for h in range(2)]

    def ahead(i):
        def mk(t, h, row):
            def fn(a):
                zr, zi = cmul(i + 1, 0, NC, h, row, C(t), a)
                acc[i, AR(h, 0, row), C(t)] = zr
                acc[i, AR(h, 1, row), C(t)] = zi
            return fn
        return [mk(*p) for p in pos()]

    def spread():
        n = NB - NC - 1

        def mk(t, h, row):
            def fn(a):
                p = []
                for i in range(3):
                    Rw = slice((3 * h + i) * H + row, (3 * h + i) * H + row + 8)
                    u = uf[0, Rw, C(t)]
                    p.append(kf[1:1 + n, Rw, C(t)] * (_tie(u, a) if i == 0 else u)[None])
                acc[0:n, AR(h, 0, row), C(t)] = acc[1:1 + n, AR(h, 0, row), C(t)] + (p[0] - p[2])
                acc[0:n, AR(h, 1, row), C(t)] = acc[1:1 + n, AR(h, 1, row), C(t)] + (p[0] + p[1])
            return fn
        return [mk(*p) for p in pos()]

    def mmI(name, sl, ys):
        def unit(n):
            def epi(p):
                ce, se, co, so = p
                sub = lax.broadcasted_iota(I32, (8, 128), 0)
                c0 = ys * T + H
                y_v[n, ys * T:ys * T + 1, :] = (ce[64:72] - se[0:8])[0:1]
                se = jnp.concatenate([jnp.where(sub == 0, 0.0, se[0:8]), se[8:]], axis=0)
                for d, cc, ss in ((0, ce[0:64], se), (1, co, so)):
                    y_v[n, pl.ds(c0 + d, 64, stride=2), :] = cc + ss
                    lo = cc - ss
                    for i in range(0, 64, 8):
                        y_v[n, pl.ds(c0 - d - 2 * i - 14, 8, stride=2), :] = jnp.take_along_axis(
                            lo[i:i + 8], 7 - sub, axis=0)
            return Unit(name(n), [(lambda i=i: (tg_v[0:(GR if i == 0 else 64), C(i)], zz_v[pl.ds(sl * 2 * T + i * H, H), C(n)]))
                                  for i in range(4)], epi, 64, 52)
        return [unit(n) for n in range(NT)]

    def mod(name, a, b):
        def unit(n):
            def epi(p):
                v = [_sum(p[i * NT:(i + 1) * NT])[0:8] for i in range(b - a)]
                if a == 0:
                    mod_v[0, :, C(n)] = v[0] * v[2]
                    mod_v[1, :, C(n)] = (v[1] + 1.0) * v[2]
                elif a == 3:
                    mod_v[3, :, C(n)] = v[0]
                    mod_v[4, :, C(n)] = v[1] + 1.0
                else:
                    mod_v[5, :, C(n)] = v[0]
                    mod_v[2, :, C(n)] = v[0] * G_POST
            return Unit(name, [(lambda i=i, k=k: (silu_c[:, C(k)], wm_v[a][C(k), pl.ds(i * D + n * 128, 128)]))
                               for i in range(b - a) for k in range(NT)], epi, 16, 10, full=False, acc=b - a == 1)
        return [unit(n) for n in range(NT)]

    HS = (slice(0, 128), slice(128, 256))
    QS = tuple(slice(r, r + 64) for r in range(0, T, 64))

    def tasks(f, due=None, tie=True, n=RG):
        def mk(R):
            def fn(a):
                x = f(R, a if tie else None)
                return Due(x, due) if due else None
            return fn
        return [mk(slice(r, r + n)) for r in range(0, T, n)]

    def load_y(sl, R):
        return jnp.concatenate([y_v[t, sl * T + R.start:sl * T + R.stop, :] for t in range(NT)],
                               axis=1).reshape(2, 8, D)

    def put(nn, ss, R, x):
        nn[R, :] = x.astype(BF16)
        tok = x
        if ss is not None:
            S2 = pl.ds(R.start // 32 * 16, 16)
            if R.stop % 32:
                top_v[S2, 0:2 * T] = x[:, 0:2 * T]
            else:
                if R.start % 32:
                    x = jnp.concatenate([top_v[S2, 0:2 * T], x[:, 0:2 * T]], axis=0)
                ss[S2, 0:5 * T] = jnp.concatenate(_lhs_sums(x[:, 0:T], x[:, T:2 * T]), axis=1).astype(BF16)
        return tok

    wide = lambda v: jnp.concatenate([v] * NT, axis=1)

    def mean(i, R, x):
        st_v[R, C(i)] = jnp.broadcast_to(jnp.sum(x, axis=-1, keepdims=True) * (1.0 / D), (x.shape[0], 128))

    def centred(src, i, R, a):
        return src[R, :] - wide(_tie(st_v[R, C(i)], a))

    def scale(src, i, g):
        def f(R, a):
            st_v[R, C(i + 1)] = jnp.broadcast_to(_rstd(centred(src, i, R, a), g), (RG, 128))
        return f

    def normed(src, i, R, a):
        return centred(src, i, R, a) * wide(st_v[R, C(i + 1)])

    def front(sl, xs, early=False, ss=None):
        xx, hh, nn = view(x_v, xs), view(hb_v, xs), view(n1_v, sl)

        def fa(R, a):
            q = [q_n[sl][t, R.start // 2:R.stop // 2, :] for t in range(NT)]
            q = jnp.concatenate([_tie(q[0], a)] + q[1:], axis=1)
            q = pltpu.bitcast(q, BF16).astype(F32).reshape(2, 8, D)
            x = (q + (_ln(q) * mod_v[1] + mod_v[0]) * load_y(sl, R)).reshape(RG, D)
            xx[R, :] = x
            if early:
                hh[R, :] = _ln(x)

        def fb(R, a):
            hh[R, :] = (_ln(_tie(xx[R, :], a).reshape(2, 8, D)) * mod_v[4] + mod_v[3]).reshape(RG, D)

        def fc(R, a):
            hb = _tie(hh[R, :], a)
            if early:
                hb = (hb.reshape(2, 8, D) * mod_v[4] + mod_v[3]).reshape(RG, D)
                hh[R, :] = hb
            nn[R, :] = _ln(hb, G_A).astype(BF16)
        if early:
            return tasks(fa), tasks(fc)
        if ss is None:
            return tasks(fa) + tasks(fb) + tasks(fc)
        qf = view(x_v, 2)

        def s1(R, a):
            q = [q_n[sl][t, R.start // 2:R.stop // 2, :] for t in range(NT)]
            q = pltpu.bitcast(jnp.concatenate([_tie(v, a) for v in q], axis=1), BF16).astype(F32)
            qf[R, :] = q
            mean(0, R, q)

        def s3(R, a):
            h = normed(qf, 0, R, a).reshape(2, 8, D) * mod_v[1] + mod_v[0]
            x = qf[R, :] + (h * load_y(sl, R)).reshape(RG, D)
            xx[R, :] = x
            mean(2, R, x)

        def s5(R, a):
            hb = (normed(xx, 2, R, a).reshape(2, 8, D) * mod_v[4] + mod_v[3]).reshape(RG, D)
            hh[R, :] = hb
            mean(4, R, hb)
        s7 = [f for g in tasks(lambda R, a: put(nn, ss, R, normed(hh, 4, R, a)), n=32) for f in (g, lambda a: None)]
        st = [tasks(s3), tasks(scale(xx, 2, 1.0)), tasks(s5), tasks(scale(hh, 4, G_A)), s7]
        p = [tasks(s1), tasks(scale(qf, 0, 1.0))]
        return cat(x[:8] for x in st), cat(x[8:] for x in p + st), cat(x[:8] for x in p)

    def shift(hs, sl, pieces=((0, 64), (64, 64), (128, 64), (192, 64)), ss=None):
        gg = view(g_v, sl)

        def one_tile(t, r, n, a):
            lane = lax.broadcasted_iota(I32, (n, 128), 1)
            ld = lambda d: h1_v[t, pl.ds(hs * T + 8 + r + d, n), :]
            if t == 0:
                g = ld(-1)
            elif t == 1:
                g = jnp.where(lane < 32, ld(-1), ld(1))
            elif t == 2:
                g = jnp.where(lane < 64, ld(1), ld(-2))
            elif t == 3:
                g = jnp.where(lane < 96, ld(-2), ld(2))
            else:
                g = ld(2)
            if a is not None:
                g = jnp.concatenate([_tie(g[i:i + 8], a) if i % 16 == 0 else g[i:i + 8]
                                     for i in range(0, n, 8)], axis=0)
            gg[r:r + n, C(t)] = g.astype(BF16)
            return g

        def mk(ts, r, n):
            def fn(a):
                g = [one_tile(t, r, n, a) for t in ts]
                if len(ts) == 2:
                    for i, x in enumerate(_lhs_sums(*g)):
                        ss[r // 2:(r + n) // 2, C(2 * i + ts[0])] = x.astype(BF16)
            return fn
        sets = [(t,) for t in range(NT)] if ss is None else [(0, 2), (1, 3), (4,)]
        return [mk(ts, r, n) for ts in sets for r, n in pieces]

    def shift_early():
        def keep(a):
            h1_v[:, 2 * T - 32:2 * T + 8, :] = h1_v[:, 3 * T - 32:3 * T + 8, :]
        return shift(2, 0, [(r, 32) for r in range(0, T - 32, 32)], gs) + [keep]

    def ln2(xs, sl, fast=True):
        xx, nn, ss = view(x1_v, xs), view(n2_v, sl), view(n2s, sl, H) if fast else None
        f = lambda R, a: put(nn, ss, R, _ln(_tie(xx[R, :], a), G_A))
        ts = tasks(f, DL, False)
        return ts[0::2] + ts[1::2] if fast else tasks(f)

    def resid(xs, x1s, rotate=False):
        xx, x1 = view(x_v, xs), view(x1_v, x1s)

        def f(R, a):
            gb = mod_v[5] if a is None else pltpu.bitcast(
                pltpu.bitcast(mod_v[5], U32) | jnp.concatenate([a] * NT, axis=1), F32)
            r_v[R, :] = xx[R, :] + (x1[R, :].reshape(2, 8, D) * gb).reshape(RG, D)
            if rotate:
                xx[R, :] = x_v[R, :]
                view(hb_v, 1)[R, :] = hb_v[R, :]
        return tasks(f)

    KD, KF, ND = [(0, 2), (1, 3)], [(2 * i, 2 * i + 1) for i in range(7)], [(1, 2), (3, 4)]
    Wt = {1: (lambda k, n: w1_v[C(k), C(n)], lambda i, kp, j: w1s[C(kp), C(2 * i + j)], False, KD, [4]),
          2: (lambda k, n: w2_v[C(k), C(n)], lambda i, kp, j: w2s[C(kp), C(2 * i + j)], False, KD, [4]),
          0: (lambda k, n: w3_v[C(n), C(k)], None, True, KD, [4]),
          3: (lambda k, n: w3n[C(k), C(n)], lambda i, kp, j: w3s[C(kp), C(6 * i + j)], False, KD, [4]),
          4: (lambda k, n: w4_v[C(k), C(n)], lambda i, kp, j: w4s[C(kp), C(2 * i + j)], False, KF, [])}

    def sums_task(load, store, left):
        def fn(a):
            b = [[load(u, v) for v in range(2)] for u in range(2)]
            b[0][0], b[1][1] = _tie(b[0][0], a), _tie(b[1][1], a)
            (x11, x12), (x21, x22) = [[pltpu.bitcast(x, BF16).astype(F32) for x in row] for row in b]
            r = ((x11 + x22, x21 + x22, x11 + x12, x21 - x11, x12 - x22) if left else
                 (x11 + x22, x12 - x22, x21 - x11, x11 + x12, x21 + x22))
            for m, x in enumerate(r):
                store(m, x.astype(BF16))
        return fn

    def wsums(w_w, ws, rp, cp_):
        def mk(i, j, r):
            def store(m, x):
                ws[pl.ds(128 * i + r, 16), C(len(cp_) * m + j)] = x
            return sums_task(lambda u, v: w_w[pl.ds(64 * rp[i][u] + r // 2, 8), C(cp_[j][v])], store, False)
        return [mk(i, j, r) for j in range(len(cp_)) for i in range(len(rp)) for r in range(0, 128, 16)]

    def w3_turn():
        def mk(n, k):
            def fn(a):
                x = jnp.concatenate([_tie(w3_w[64 * n:64 * n + 8, C(k)], a), w3_w[64 * n + 8:64 * n + 64, C(k)]], axis=0)
                w3n[C(k), C(n)] = pltpu.bitcast(x, BF16).T
            return fn
        return [mk(n, k) for n in range(FT - 1) for k in range(NT)]

    def plain(name, w, lhs, n, R, epi, cost):
        tile, _, nt, kp, kl = Wt[w]
        ks = sorted([k for p in kp for k in p] + kl)
        rows_ = R.stop - R.start
        return Unit(name, [(lambda k=k: (lhs[R, C(k)], tile(k, n))) for k in ks], lambda p: epi(n, R, p[0]),
                    rows_, rows_ // 8 * (len(ks) - 1 + cost), nt=nt, acc=True)

    def quad(name, w, lhs, sums, j, cols_, R, epi, cost):
        tile, wsum, nt, kp, kl = Wt[w] if isinstance(w, int) else w
        h, S2, c = len(kp), slice(R.start // 2, R.stop // 2), {}
        a_ = lambda i, k: _top(lhs(k) if callable(lhs) else lhs[R, C(k)], i)
        s_ = sums if callable(sums) else (lambda i, p: sums[S2, C(h * i + p)])
        prod = lambda fa_, fb_: [(lambda p=p: (fa_(p), fb_(p))) for p in range(h)]
        left = lambda i, n: [(lambda k=k: (a_(i, k), tile(k, n))) for k in kl]
        mk = lambda tiles, f, x=0: Unit(name, tiles, lambda p: f(p[0]), 64, 8 * len(tiles) + x, nt=nt, acc=True)

        def e1(m):
            u7.res, u6.res = [m], [m]

        def e4(m):
            c[11], c[21] = c[11] + m, m

        def e2(m):
            c[21], c[22] = c[21] + m, c[22] - m
            l21.res = [c[21]]

        def e5(m):
            c[12] = m
            epi(cols_[0], R, _zip(c[11] - m, c[21]))

        def e3(m):
            l12.res, c[22] = [c[12] + m], c[22] + m
            if not kl:
                l12.epi(l12.res)
        u1 = mk(prod(lambda p: s_(0, p), lambda p: wsum(0, p, j)), e1)
        u7 = mk(prod(lambda p: s_(4, p), lambda p: wsum(4, p, j)) + left(0, cols_[0]), lambda m: c.update({11: m}))
        u6 = mk(prod(lambda p: s_(3, p), lambda p: wsum(3, p, j)) + left(1, cols_[1]), lambda m: c.update({22: m}))
        u4 = mk(prod(lambda p: a_(1, kp[p][1]), lambda p: wsum(2, p, j)), e4)
        u2 = mk(prod(lambda p: s_(1, p), lambda p: tile(kp[p][0], cols_[0])), e2, 8)
        l21 = mk(left(1, cols_[0]), lambda m: c.update({21: m}))
        u5 = mk(prod(lambda p: s_(2, p), lambda p: tile(kp[p][1], cols_[1])), e5, 16 * cost)
        u3 = mk(prod(lambda p: a_(0, kp[p][0]), lambda p: wsum(1, p, j)), e3, 8 if kl else 8 + 16 * cost)
        l12 = mk(left(0, cols_[1]), lambda m: epi(cols_[1], R, _zip(m, c[22])), 16 * cost)
        return [u1, u7, u6, u4, u2, l21, u5, u3, l12]

    LH, RH = [0, 4, 3, (1, 1), 1, 2, (0, 0)], [0, 4, 3, 2, (0, 0), (1, 1), 1]
    L2 = {3: (w3n_w, ws_w[2], w3t, KF[:6], n2t), 4: (w4_w, ws_w[3], w4t, ND, a_t)}

    def wsums2(w):
        w_w, s_w, ws2, cp_, _ = L2[w]
        kp, nj = Wt[w][3], len(cp_)

        def mk(o, p2, j2, r):
            def load(u, v):
                p, j, y = 2 * p2 + u, 2 * j2 + v, RH[o]
                if isinstance(y, int):
                    return s_w[pl.ds(64 * p + r // 2, 8), C(nj * y + j)]
                return w_w[pl.ds(64 * kp[p][y[0]] + r // 2, 8), C(cp_[j][y[1]])]

            def store(m, x):
                ws2[pl.ds(128 * p2 + r, 16), C((5 * o + m) * (nj // 2) + j2)] = x
            return sums_task(load, store, False)
        return [mk(o, p2, j2, r) for j2 in range(nj // 2) for o in range(7) for p2 in range(len(kp) // 2)
                for r in range(0, 128, 16)]

    def lsums2(w, lhs_w, sums_w, sl):
        kp, xs2 = Wt[w][3], L2[w][4]
        h2 = len(kp) // 2

        def mk(o, p2, g):
            def load(u, v):
                p, ch, x = 2 * p2 + v, 2 * g + u, LH[o]
                if isinstance(x, int):
                    return sums_w[pl.ds(64 * sl + 8 * ch, 8), C(len(kp) * x + p)]
                return lhs_w[pl.ds(H * sl + 16 * ch + 8 * x[0], 8), C(kp[p][x[1]])]

            def store(m, x):
                xs2[pl.ds(16 * g, 16), C((5 * o + m) * h2 + p2)] = x
            return sums_task(load, store, True)
        return [[mk(o, p2, g) for o in range(7) for g in range(4)] for p2 in range(h2)]

    def quad2(name, w, lhs, sums, j2, epi, cost):
        tile, wsum, nt, kp, kl = Wt[w]
        ws2, cp_, xs2 = L2[w][2:]
        h, h2, nj2, c, R = len(kp), len(kp) // 2, len(cp_) // 2, {}, slice(0, T)

        def done(j, v):
            val = _zip(c[j, 1, v], c[j, 2, v])
            if not kl:
                return epi(cp_[j][v], R, val)
            c[j, v] = val

        def upd(o, j, m):
            for i, v, sg in (((1, 0, 1), (2, 1, 1)), ((1, 0, 1),), ((2, 1, 1),), ((1, 0, 1), (2, 0, 1)),
                             ((2, 0, 1), (2, 1, -1)), ((1, 0, -1), (1, 1, 1)), ((1, 1, 1), (2, 1, 1)))[o]:
                k = (j, i, v)
                c[k] = m if k not in c else (c[k] + m if sg > 0 else c[k] - m)
            if o >= 5:
                done(j, o - 5)

        def inner(o):
            x, y = LH[o], RH[o]
            xo = ((lambda p: sums[:, C(h * x + p)]) if isinstance(x, int)
                  else (lambda p: _top(lhs[:, C(kp[p][x[1]])], x[0])))
            yo = ((lambda p, j: wsum(y, p, j)) if isinstance(y, int)
                  else (lambda p, j: tile(kp[p][y[0]], cp_[j][y[1]])))
            w_ = (yo, lambda m, p2, _: ws2[C(p2), C((5 * o + m) * nj2 + j2)], nt,
                  [(2 * i, 2 * i + 1) for i in range(h2)], list(range(2 * h2, h)))
            return quad(name, w_, xo, lambda m, p2: xs2[:, C((5 * o + m) * h2 + p2)], 0, (2 * j2, 2 * j2 + 1),
                        HS[0], lambda j, _, m: upd(o, j, m), 2 + (2 * cost if o >= 5 and not kl else 0))

        def rest(j, v):
            return [Unit(name, [(lambda Q=Q: (lhs[Q, C(k)], tile(k, cp_[j][v]))) for Q in QS],
                         lambda p: epi(cp_[j][v], R, jnp.concatenate(p, axis=0) + c[j, v]), 64, 32 * (cost + 1))
                    for k in kl]
        js = (2 * j2, 2 * j2 + 1)
        return (cat(inner(o) for o in range(6)) + cat(rest(j, 0) for j in js) + inner(6) + cat(rest(j, 1) for j in js))

    def mm(name, w, lhs, sums, epi, cost):
        if sums is None:
            return [[plain(name, w, lhs, n, R, epi, cost) for R in HS] for n in range(NT)]
        return [[plain(name, w, lhs, 0, R, epi, cost) for R in QS]] + [
            [u for R in HS for u in quad(name, w, lhs, sums, j, ND[j], R, epi, cost)] for j in range(2)]

    def mm1(name, hs, sl, fast=False):
        def epi(n, R, p):
            h1_v[n, pl.ds(hs * T + 8 + R.start, R.stop - R.start), :] = _gelu2(p)
        return cat(mm(name, 1, view(n1_v, sl), n1s if fast else None, epi, 5))

    def mm2(name, sl, xs, x1s, fast=False):
        def epi(n, R, p):
            view(x1_v, x1s)[R, C(n)] = view(hb_v, xs)[R, C(n)] + p * G_POST
        return cat(mm(name, 2, view(g_v, sl), gs if fast else None, epi, 2))

    def mm3(name, sl, fast=True):
        nn, aa, ss, keep, tail = view(n2_v, sl), view(a_v, sl), view(a_s, sl, H), {}, []

        def epi(n, R, p):
            g = _gelu2(p)
            aa[R, C(n)] = g.astype(BF16)
            if n % 2 == 0 and n < 12:
                keep[n] = g
                return
            pair = (keep.pop(n - 1), g) if n % 2 else (g, tail[R.start // 128][R.start % 128:R.start % 128 + 64])
            for i, x in enumerate(_lhs_sums(*pair)):
                ss[R.start // 2:R.stop // 2, C(7 * i + n // 2)] = x.astype(BF16)

        def rem(R):
            def f(p):
                tail.append(jnp.concatenate([_gelu2(p[0]), jnp.zeros((64, 128), F32)], axis=0).T)
                aa[R, C(13)] = tail[-1].astype(BF16)
            return Unit(name, [(lambda k=k: (w3_v[13 * 128:F, C(k)], nn[R, C(k)])) for k in range(NT)], f, 64, 84,
                        nt=True, acc=True)
        odd = [rem(R) for R in HS] + [plain(name, 3 if fast else 0, nn, 12, R, epi, 9) for R in QS]
        if fast == 2:
            return odd + cat(quad2(name + "_%d" % j, 3, nn, view(n2s, sl, H), j, epi, 8) for j in range(3))
        if fast:
            qd = [u for j in range(6) for R in HS for u in quad(name, 3, nn, view(n2s, sl, H), j, KF[j], R, epi, 8)]
            return qd[:18] + odd[:2] + qd[18:36] + odd[2:] + qd[36:]
        return odd + [plain(name, 0, nn, n, R, epi, 8) for p in KF[:6] for R in HS for n in p]

    NA = 3 * 128

    def cp_out(j, osl, L, sm, R=slice(0, T)):
        return cp(o_v.at[pl.ds(osl * T + R.start, R.stop - R.start), L],
                  o_hbm.at[pl.ds(base(j, T) + R.start, R.stop - R.start), L], sem_o.at[sm])

    out_a = lambda j: cp_out(j, 0, slice(0, NA), 0)
    out_b = lambda j: cp_out(j, 0, slice(NA, D), 1)
    last = []

    def mm4(name, j, sl, osl=0, xs=None, x1s=None, fast=True):
        oo = view(o_v, osl)

        def epi(n, R, p):
            if xs is None:
                oo[R, C(n)] = (r_v[R, C(n)] + mod_v[2, 0:1, C(n)] * p).astype(BF16)
            else:
                oo[R, C(n)] = (view(x_v, xs)[R, C(n)] + mod_v[5, 0:1, C(n)]
                               * (view(x1_v, x1s)[R, C(n)] + p * G_POST)).astype(BF16)
            if osl == 2:
                last.append(cp_out(j, osl, C(n), 2, R))
                last[-1].start()
            elif R.stop == T and (osl, (n + 1) * 128) in ((1, D), (3, NA)):
                last.append(cp_out(j, osl, slice(0, (n + 1) * 128), 2))
                last[-1].start()
            elif R.stop == T and osl == 0 and (n + 1) * 128 in (NA, D):
                (out_a if (n + 1) * 128 == NA else out_b)(j).start()
        if fast == 2:
            return ([plain(name, 4, view(a_v, sl), 0, R, epi, 5) for R in QS],
                    quad2(name + "q", 4, view(a_v, sl), view(a_s, sl, H), 0, epi, 5))
        return mm(name, 4, view(a_v, sl), view(a_s, sl, H) if fast else None, epi, 3 if xs is None else 5)

    def split(us):
        n = 4 // len(us)
        m, mks, st = us[0].rows // n, [u.tiles.pop(0) for u in us], {}

        def piece(i, k):
            if i not in st:
                st[i] = mks[i]()
            return st[i][0][m * k:m * (k + 1)], st[i][1]

        def epi(p):
            for i, u in enumerate(us):
                u.res = [jnp.concatenate(p[n * i:n * (i + 1)], axis=0)]
        return _flat([Unit(us[0].name, [(lambda i=i, k=k: piece(i, k)) for i in range(len(us)) for k in range(n)],
                           epi, m, 0, nt=us[0].nt)])

    W = lambda nm: [("wait", nm)]
    run = lambda fns: [("run", "run", lambda: [fn(None) for fn in fns])]
    one = lambda us: [_flat([u]) for u in us]
    nm = lambda x: (lambda n: x)

    seq, grp = [], []
    for s in range(NC):
        seq += W("c%d" % s) + _flat(mmK(s) + mmU(nm("U%d" % s), s % 2, NC - 1 - s))
        grp.append(Group("kv%d" % s, cat(kv(s, s % 2)), 50, ["c%d" % s], ["U%d" % s], 100))
    inv = [mmI(lambda n: "I%d" % n, s, s) for s in range(NC)]
    seq += W("c3") + _flat(mmK(3) + mmK(4) + [inv[s][t] for t in range(NT) for s in range(NC)])
    macs = [mac(s + 1, NC - 1 - s, s, first=s == 0) for s in range(NC)]
    grp.append(Group("mac00", macs[0][0], 12, ["c1"], ["c2"], 0))
    grp.append(Group("mac01", macs[1][0] + macs[0][1] + macs[1][1], 16, ["c2"], ["c3"], 0))
    for t in range(NT):
        grp.append(Group("mac%d" % t, cat(macs[s][t] for s in range(2 if t < 2 else 0, NC)), 24 if t < 2 else 18,
                         ["c3", "K%d" % t], ["I%d" % t], 100, 150))
    start = lambda cs: [("run", "run", lambda: [c.start() for c in cs])]
    f0, f1 = front(0, 2, True), front(1, 1, True)
    seq += run(ahead(0))
    seq += W("wma") + _flat(mod("moda", 0, 3)) + run(f0[0] + f1[0] + ahead(1))
    seq += W("wmb") + start(next_kv(NC) + next_q(NC)) + _flat(mod("modb", 3, 5)) + run(f0[1])
    w1 = _flat(mm1("w1_0", 0, 0) + mm1("w1_1", 1, 1))
    seq += W("w1") + w1[:72] + W("w2") + w1[72:] + run(shift(0, 0))
    seq += _flat(mm2("w2_0", 0, 2, 1) + mm1("w1_2", 2, 2)) + run(shift(1, 1)) + _flat(mm2("w2_1", 1, 1, 0))
    grp.append(Group("f1", f1[1], 80, ["w1"], ["w1_1"], 450))
    grp.append(Group("f2", front(2, 0), 80, ["w2"], ["w1_2"], 450))
    grp.append(Group("ln2_0", ln2(1, 0, False), 60, ["w2_0"], ["w3"], 450))
    grp.append(Group("ahead", cat(ahead(i) for i in range(2, NB - NC)), 19, ["w1"], ["end"], 100))
    grp.append(Group("ws1", wsums(w1_w, w1s, KD, ND), 26, ["w1"], ["end"], 100))
    grp.append(Group("ws2", wsums(w2_w, w2s, KD, ND), 26, ["w2"], ["end"], 100))
    grp.append(Group("ws3", w3_turn() + wsums(w3n_w, w3s, KD, KF[:6]), 22, ["w3"], ["end"], 100))
    grp.append(Group("ws4", wsums(w4_w, w4s, KF, ND), 26, ["w4"], ["end"], 100))
    _wait(seq, "w3", back=1)
    w3 = mm3("w3_0", 0, False)
    _mix(seq, _flat(w3[6:]), [split(w3[4:6]) + _flat(w3[:6])], 0.1)
    mc = _flat(mod("modc", 5, 6))
    _wait(seq, "w4", mc[:5] + [("sync", "run", lambda: None)])
    w4 = cat(mm4("w4_0", 0, 0, 3, 2, 1, False)[:3])
    qs = [split([w4[-1 - i]]) for i in range((_phase(seq) + FT * 6) % 4)]
    _mix(seq, _flat(w4), [mc[i:i + 4] for i in range(5, 25, 4)] + qs, 0.01, 0.4)
    assert _phase(seq) == 0
    grp.append(Group("resid", resid(2, 1), 26, ["modc"], ["end"], 100))
    _emit(seq, grp, zero, wait)

    def step(s, carry):
        for c in next_kv(s) + next_q(s):
            c.wait()
        nxt = jnp.minimum(s + 1, NB - 1)
        seq, grp = [], []
        us, it = one(mmU(lambda n: "U%d" % n, 0, 0)), one(mmI(lambda n: "I%d" % n, 0, 0))
        w4 = mm4("w4", s - 2, 0)
        q = split(w4[0][2:])
        _mix(seq, _flat(mm4("w4c", s - 3, 0)[2] + mm3("w3", 0)),
             [us[0], us[1], us[2], it[0] + us[3], it[1] + us[4], it[2] + start(next_kv(nxt)), it[3], it[4]],
             0.26, 0.78)
        w1a, w1b = mm1("w1a", 2, 0, True), mm1("w1b", 2, 0, True)
        w1a, w1b = _flat(w1a[0:2] + w1a[4:13] + w1a[22:31]), _flat(w1b[2:4] + w1b[13:22] + w1b[31:])
        _mix(seq, _flat(w4[0] + w4[1][:9]), [q])
        seq += w1a + run(shift(1, 0, ((T - 32, 32),), gs)) + _flat(w4[1][9:]) + w1b[:8] + start(next_q(nxt)) + w1b[8:]
        seq += _flat(mm2("w2", 0, 1, 0, True))
        assert _phase(seq) == 0
        kvs, macs = kv(0, 0), mac(1, 0, 0, part=True)
        for t in range(NT):
            grp.append(Group("kv%d" % t, kvs[t], 50, ["start"], ["U%d" % t], 300))
            grp.append(Group("mac%d" % t, macs[t], 28, ["U%d" % t], ["I%d" % t], 300, 150))
        iall = ["I%d" % t for t in range(NT)]
        grp.append(Group("ln2", ln2(0, 0), 75, ["start"], ["w3"], 450))
        grp.append(Group("resid", resid(1, 0, True), 40, ["w4c"], ["w4", "I4"], 100))
        fr = front(0, 0, ss=n1s)
        grp.append(Group("fronta", fr[0], 50, iall, ["w1a"], 230))
        grp.append(Group("frontb", fr[1], 50, iall, ["w1b"], 230, 2200))
        grp.append(Group("fq", fr[2], 34, ["w4c"], ["I4"], 100))
        grp.append(Group("spread", spread(), 30, iall, ["end"], 100))
        grp.append(Group("shift", shift_early(), 24, ["start"], ["w1a"], 200))
        _emit(seq, grp, zero, wait)
        out_b(s - 3).wait()
        out_a(s - 2).wait()
        return carry

    lax.fori_loop(NC, NB, step, 0)

    seq, grp = [], []
    w47 = mm4("w4_7", NB - 1, 1, 2, 0, 1, 2)
    seq += _flat(mm4("w4_5", NB - 3, 0)[2] + mm3("w3_6", 0) + mm2("w2_7", 0, 0, 1, True)
                 + cat(mm4("w4_6", NB - 2, 0, 1, 1, 0, 2)) + mm3("w3_7", 1, 2) + w47[0][:3] + w47[1] + w47[0][3:])
    grp.append(Group("ln2_6", ln2(0, 0), 75, ["start"], ["w3_6"], 450))
    grp.append(Group("shift7", shift(2, 0, [(r, 32) for r in range(0, T, 32)], gs), 24, ["start"], ["w2_7"], 200))
    grp.append(Group("ws4b", wsums2(4), 26, ["start"], ["w4_6q"], 250))
    grp.append(Group("ws3b", wsums2(3), 26, ["start"], ["w3_7_0"], 250))
    grp.append(Group("xa6", cat(lsums2(4, a_w, as_w[3], 0)), 26, ["w3_6"], ["w4_6q"], 200))
    grp.append(Group("ln2_7", ln2(1, 1), 75, ["w2_7"], ["w3_7"], 1200))
    grp.append(Group("xn7", cat(lsums2(3, n2_w, as_w[2], 1)), 26, ["w2_7"], ["w3_7_0"], 200, 3100))
    for p, ts in enumerate(lsums2(4, a_w, as_w[3], 1)):
        grp.append(Group("xa7_%d" % p, ts, 26, ["w3_7_%d" % p], ["w4_7q"], 200, 150))
    _emit(seq, grp, zero, wait)
    for c in next_kv(NB - 1) + next_q(NB - 1) + [out_b(NB - 3)] + last:
        c.wait()


@jax.jit
def pallas_adaLN_cond__ssm_conv_h3__mixer_s_mlp__prompt_kernel(
        A_q, A_k, A_v, A_shift_k, A_ssm_k, A_ssm_D, B_x, B_w1, B_w2, B_w3, B_w4, c, w_mod):
    any_ = pl.BlockSpec(memory_space=pl.ANY)
    V = pltpu.VMEM
    out = pl.pallas_call(
        kernel,
        in_specs=[any_] * 12,
        out_specs=any_,
        out_shape=jax.ShapeDtypeStruct((S, D), BF16),
        scratch_shapes=[
            [V((NT, H + 8, 128), U32)] * NC, [V((NT, H + 8, 128), U32)] * NC, [V((NT, H + 8, 128), U32)] * NC,
            [V((64, S), U32)] * NT,
            V((D // 2, D), U32), V((D // 2, D), U32), V((F // 2, D), U32), V((FT * 64, D), U32),
            [V((D // 2, 3 * D), U32), V((D // 2, 2 * D), U32), V((D // 2, D), U32)], V((4 * T, D), BF16),
            V((4, D), BF16), V((D,), BF16), V((1, D), BF16), V((8, 128), I32), pltpu.SMEM((8, 128), I32),
            V((5, 8, D), F32), V((6, 8, D), F32), V((T // 2, 4 * H), U32), V((GR // 2, 2 * T), U32),
            V((NB, 3 * T + 8, D), F32), V((NC, 3 * T + 8, D), F32), V((NB - NC, 2 * T + 8, D), F32), V((2 * T, D), F32),
            V((T, D), U32), V((NC * T, D), U32), V((NT, NC * T + 8, 128), F32),
            V((3 * T, D), F32), V((3 * T, D), F32), V((2 * T, D), F32), V((T, D), F32),
            V((3 * T // 2, D), U32), V((T, D), U32), V((T, D), U32), V((NT, NC * T + 24, 128), F32),
            V((T, (FT + 1) * 128), U32),
            [V((128, 11 * 128), U32)] * 2 + [V((128, 31 * 128), U32), V((448, 11 * 128), U32)],
            [V((64, 11 * 128), U32)] * 2 + [V((128, 11 * 128), U32), V((128, 35 * 128), U32)],
            V((D // 2, 13 * 128), U32), V((H, D), F32), V((T, 7 * 128), F32),
            [V((64, 105 * 128), U32), V((192, 35 * 128), U32), V((32, 35 * 128), U32), V((32, 105 * 128), U32)],
            pltpu.SemaphoreType.DMA((11,)), pltpu.SemaphoreType.DMA((1,)), pltpu.SemaphoreType.DMA((3,)),
        ],
        compiler_params=pltpu.CompilerParams(vmem_limit_bytes=110 << 20, disable_semaphore_checks=True,
                                             disable_bounds_checks=True),
        name="fused",
    )(A_q[0], A_k[0], A_v[0], A_shift_k.T, A_ssm_k, A_ssm_D, B_w1, B_w2, B_w3.T, B_w4, c, w_mod)
    return out[None]
```

```python
import heapq
import numpy as np
import jax
import jax.numpy as jnp
from jax import lax
from jax.experimental import pallas as pl
from jax.experimental.pallas import tpu as pltpu

S, D, F = 2048, 640, 1728
T = 256
H = T // 2
NB = S // T
NT = D // 128
FT = (F + 127) // 128
EPS = 1e-5
F32, BF16, U32, I32 = jnp.float32, jnp.bfloat16, jnp.uint32, jnp.int32
G_C1 = 0.044715 * float(np.sqrt(2.0 / np.pi))
G_C2 = float(np.sqrt(2.0 / np.pi))
G_A = G_C1 ** (1.0 / 3.0)
G_B = G_C2 / G_A
G_POST = 0.5 / G_A
RG = 16
GR = 80
NC = 3
DL = 450
SLOT = 32


def _dft(shape, f_axis, tau, scale=1.0):
    r = lax.broadcasted_iota(I32, shape, f_axis)
    l = lax.broadcasted_iota(I32, shape, 1 - f_axis)
    f = r & 127
    odd = ((f & 63) << 2) | ((f >> 6) << 1) | 1
    p = odd * tau(l) + ((r >> 7) << 8)
    a = ((p + 512) & 1023) - 512
    u = (256 - jnp.abs(a)).astype(F32) * (np.pi / 512.0)
    u2 = u * u
    c = [scale, -scale / 6.0, scale / 120.0, -scale / 5040.0, scale / 362880.0, -scale / 39916800.0]
    poly = c[5]
    for ci in c[4::-1]:
        poly = poly * u2 + ci
    return (u * poly).astype(BF16)


def _rstd(xc, scale):
    s2 = 1.0 / (scale * scale)
    v = jnp.sum(xc * xc, axis=-1, keepdims=True) * (s2 / D) + EPS * s2
    return jnp.exp2(jnp.log(v) * float(-0.5 / np.log(2.0)))


def _ln(x, scale=1.0):
    xc = x - jnp.sum(x, axis=-1, keepdims=True) * (1.0 / D)
    return xc * _rstd(xc, scale)


def _gelu2(x):
    u = x * (x * x + G_B)
    return x * (1.0 + jnp.tanh(u))


def _lo(w):
    return pltpu.bitcast(w << 16, F32)


def _hi(w):
    return pltpu.bitcast(w & jnp.uint32(0xFFFF0000), F32)


def _tie(x, a):
    if a is None:
        return x
    w = pltpu.bitcast(x[:, :128], U32)
    k = w.shape[0] // 8
    w = w | (a if k == 1 else jnp.concatenate([a] * k, axis=0))
    w = pltpu.bitcast(w, x.dtype)
    return w if x.shape[1] == 128 else jnp.concatenate([w, x[:, 128:]], axis=1)


def _top(x, i):
    return jnp.concatenate([x[r:r + 16] for r in range(16 * i, x.shape[0], 32)], axis=0)


def _zip(t, b):
    return jnp.concatenate([x[r:r + 16] for r in range(0, t.shape[0], 16) for x in (t, b)], axis=0)


def _lhs_sums(x1, x2):
    a11, a21, a12, a22 = _top(x1, 0), _top(x1, 1), _top(x2, 0), _top(x2, 1)
    return [a11 + a22, a21 + a22, a11 + a12, a21 - a11, a12 - a22]


def C(i):
    return slice(i * 128, (i + 1) * 128)


class Unit:
    def __init__(self, name, tiles, epi, rows, cost, nt=False, full=True, acc=False):
        self.acc, self.res = acc, []
        self.name, self.tiles, self.epi, self.rows, self.cost, self.nt, self.full = name, tiles, epi, rows, cost, nt, full


class Due:
    def __init__(self, val, delay):
        self.val, self.delay = val, delay


class Group:
    def __init__(self, name, fns, cost, rel, dead, lat, rlat=200):
        self.name, self.fns, self.cost, self.rel, self.dead, self.lat, self.rlat = name, fns, cost, rel, dead, lat, rlat


def _plan(seq, groups):
    busy, n = [0] * 4, 0
    start, end, tiles, bars = {}, {}, [], []
    for it in seq:
        if isinstance(it[0], Unit):
            u = it[0]
            m = n % 4
            n += 1
            t0, t1 = busy[m], busy[m] + max(u.rows, 32)
            busy[m] = t1
            tiles.append((t0, t1, u.cost / len(u.tiles)))
            start.setdefault(u.name, t0)
            end[u.name] = max(end.get(u.name, 0), t1)
        elif it[0] == "wait":
            t = max(busy)
            busy, n = [t] * 4, 0
            start[it[1]] = end[it[1]] = t
            bars.append(t)
    total = max(busy)
    start["end"] = end["end"] = total
    start["start"] = end["start"] = 0
    ns = total // SLOT + 2
    load = np.zeros(ns)
    for t0, t1, c in tiles:
        a, b = t0 // SLOT, max(t1 // SLOT, t0 // SLOT + 1)
        load[a:b] += c / (b - a)
    win = []
    for g in groups:
        r = max(end[x] + (0 if start[x] == end[x] else g.rlat) for x in g.rel)
        d = min(start[x] for x in g.dead) - g.lat
        ok = np.zeros(ns, bool)
        ok[r // SLOT:max(d // SLOT, r // SLOT + 1)] = True
        for b in bars:
            if r < b <= d:
                ok[max((b - g.lat) // SLOT, 0):b // SLOT] = False
        win.append(np.nonzero(ok)[0])
    alloc = [np.zeros(len(w)) for w in win]
    for _ in range(60):
        for i, g in enumerate(groups):
            w = win[i]
            load[w] -= alloc[i]
            base = load[w]
            vol = g.cost * len(g.fns)
            lo, hi = base.min(), base.max() + vol
            for _ in range(50):
                mid = 0.5 * (lo + hi)
                if np.maximum(mid - base, 0).sum() > vol:
                    hi = mid
                else:
                    lo = mid
            alloc[i] = np.maximum(hi - base, 0)
            load[w] += alloc[i]
    times = []
    for i, g in enumerate(groups):
        cum = np.cumsum(alloc[i])
        ts = []
        for k in range(len(g.fns)):
            x = (k + 0.5) * cum[-1] / len(g.fns)
            j = int(np.searchsorted(cum, x))
            prev = cum[j - 1] if j else 0.0
            ts.append(win[i][j] * SLOT + SLOT * (x - prev) / max(alloc[i][j], 1e-9))
        times.append(ts)
    return times


def _emit(seq, groups, zero, wait):
    times = _plan(seq, groups)
    left = {"start": 0}
    for it in seq:
        nm = it[0].name if isinstance(it[0], Unit) else it[1]
        left[nm] = left.get(nm, 0) + 1
    heap, pend, todo, cnt = [], {}, list(range(len(groups))), 0
    busy, n, due = [0] * 4, 0, []

    def release():
        nonlocal cnt
        for i in list(todo):
            g = groups[i]
            if all(left[x] == 0 for x in g.rel):
                todo.remove(i)
                pend[i] = len(g.fns)
                for t, fn in zip(times[i], g.fns):
                    heapq.heappush(heap, (t, cnt, i, fn))
                    cnt += 1

    def force(name):
        nonlocal heap
        for i, g in enumerate(groups):
            if name in g.dead:
                assert i not in todo, (g.name, name)
                if pend[i]:
                    for it in sorted(x for x in heap if x[2] == i):
                        it[3](None)
                    heap = [x for x in heap if x[2] != i]
                    heapq.heapify(heap)
                    pend[i] = 0

    release()
    for it in seq:
        if isinstance(it[0], Unit):
            u, k = it
            force(u.name)
            lhs, rhs = u.tiles[k]()
            t0 = busy[n % 4]
            while u.full and due and due[0][0] < t0 + u.rows:
                t, x = due.pop(0)
                r = min(max(int(t - t0), 0), u.rows - 1) // 16 * 8
                w = pltpu.bitcast(lhs, U32)
                x = pltpu.bitcast(x[:, :128], U32)
                parts = [w[:r], w[r:r + 8] | ((x[0:8] | x[8:16]) & zero), w[r + 8:]]
                lhs = pltpu.bitcast(jnp.concatenate([y for y in parts if y.shape[0]], axis=0), BF16)
            dn = (((1,), (1 if u.nt else 0,)), ((), ()))
            p = lax.dot_general(lhs, rhs, dn, preferred_element_type=F32)
            u.res = [p + u.res[0]] if (u.acc and u.res) else u.res + [p]
            m = n % 4
            n += 1
            t0 = busy[m]
            busy[m] = t0 + max(u.rows, 32)
            while u.full and heap and heap[0][0] < t0 + u.rows:
                t, _, i, fn = heapq.heappop(heap)
                pend[i] -= 1
                r = min(max(int(t - t0), 0), u.rows - 1) // 8 * 8
                x = fn(pltpu.bitcast(p[r:r + 8], U32) & zero)
                if isinstance(x, Due):
                    due.append((t + x.delay, x.val))
                    due.sort(key=lambda e: e[0])
            if k == len(u.tiles) - 1:
                u.epi(u.res)
            left[u.name] -= 1
        elif it[0] == "wait":
            force(it[1])
            wait(it[1])
            busy, n, due = [max(busy)] * 4, 0, []
            left[it[1]] -= 1
        else:
            it[2]()
            left[it[1]] -= 1
        release()
    force("end")
    assert not heap and not todo


def _sum(ps):
    acc = ps[0]
    for p in ps[1:]:
        acc = acc + p
    return acc


def _flat(us):
    return [(u, i) for u in us for i in range(len(u.tiles))]


def _weave(a, b):
    out = []
    for i, u in enumerate(a):
        out += [u] + b[i * len(b) // len(a):(i + 1) * len(b) // len(a)]
    return out


def _phase(seq):
    n = 0
    for it in seq:
        n = n + 1 if isinstance(it[0], Unit) else (0 if it[0] in ("wait", "sync") else n)
    return n % 4


def _mix(seq, a, b, lo=0.0, hi=1.0):
    n, k = _phase(seq), 0
    for i, t in enumerate(a):
        if k < len(b) and n % 4 == 0 and t[1] != 1 and i >= len(a) * (lo + (hi - lo) * k / len(b)):
            seq.extend(b[k])
            k += 1
        seq.append(t)
        n += 1
    assert k == len(b)


def _wait(seq, name, head=(), back=0):
    r = _phase(seq) + 4 * back
    assert all(isinstance(it[0], Unit) for it in seq[len(seq) - r:])
    seq[len(seq) - r:len(seq) - r] = [("wait", name)] + list(head)


def kernel(q_hbm, k_hbm, v_hbm, sh_hbm, ssm_hbm, sd_hbm, w1_hbm, w2_hbm, w3_hbm, w4_hbm, c_hbm, wm_hbm,
           o_hbm,
           q_n, k_n, v_n, ssm_w, w1_w, w2_w, w3_w, w4_w, wm_w, o_v,
           sh_v, sd_v, c_v, zsrc, z_s, taps, mod_v, tf_w, tg_w,
           kf, uf, acc, zraw, kv_w, zz_w, y_v, x_v, hb_v, x1_v, r_v, n1_w, n2_w, g_w, h1_v, a_w,
           ws_w, as_w, w3n_w, top_v, st_v, l2_w,
           sem, sem_b, sem_o):
    bf = lambda r: r.bitcast(BF16)
    w1_v, w2_v, w3_v, w4_v = bf(w1_w), bf(w2_w), bf(w3_w), bf(w4_w)
    wm_v = {0: bf(wm_w[0]), 3: bf(wm_w[1]), 5: bf(wm_w[2])}
    tf_v, tg_v, n1_v, n2_v, g_v = bf(tf_w), bf(tg_w), bf(n1_w), bf(n2_w), bf(g_w)
    a_v, kv_v, zz_v = bf(a_w), bf(kv_w), bf(zz_w)
    w1s, w2s, w3s, w4s = [bf(r) for r in ws_w]
    n1s, gs, n2s, a_s = [bf(r) for r in as_w]
    w3n = bf(w3n_w)
    w3t, w4t, n2t, a_t = [bf(r) for r in l2_w]
    cp = pltpu.make_async_copy
    cat = lambda ls: [x for l in ls for x in l]

    def base(j, n):
        return j * n if isinstance(j, int) else pl.multiple_of(j * n, n)

    def rows(j, n=1, size=T):
        return pl.ds(base(j, size), n * size)

    def view(ref, j, size=T):
        return ref.at[rows(j, 1, size)]

    dmas = {}

    def group(name, *mks):
        sm = sem.at[len(dmas)]
        dmas[name] = [c for mk in mks for c in mk(sm)]

    def ssm_in(t):
        return lambda sm: [cp(ssm_hbm.at[C(t)], bf(ssm_w[t]), sm)]

    def cols(src, start, n, dst, row=0):
        return lambda sm: [cp(src.at[pl.ds(start, n), C(t)], bf(dst).at[t, pl.ds(row, n)], sm) for t in range(NT)]

    def kv_in(s, sl):
        if isinstance(s, int):
            kk = cols(k_hbm, s * T - 16, T + 16, k_n[sl]) if s else cols(k_hbm, 0, T, k_n[sl], 16)
        else:
            kk = cols(k_hbm, pl.multiple_of(s * T - 16, 16), T + 16, k_n[sl])
        return lambda sm: kk(sm) + cols(v_hbm, base(s, T), T, v_n[sl])(sm)

    def q_in(s, sl):
        return cols(q_hbm, base(s, T), T, q_n[sl])

    def wm_in(a, b):
        return lambda sm: [cp(wm_hbm.at[:, a * D:b * D], wm_v[a], sm)]

    def whole(src, dst):
        return lambda sm: [cp(src, dst, sm)]

    next_kv = lambda s: kv_in(s, 0)(sem_b.at[0])
    next_q = lambda s: q_in(s, 0)(sem_b.at[0])

    zsrc[...] = jnp.zeros((8, 128), I32)
    k_n[0][:, 0:8, :] = jnp.zeros((NT, 8, 128), U32)
    w4_w[F // 2:FT * 64, :] = jnp.zeros((FT * 64 - F // 2, D), U32)
    group("small", lambda sm: [cp(zsrc, z_s, sm), cp(sh_hbm, sh_v, sm), cp(sd_hbm, sd_v, sm), cp(c_hbm, c_v, sm)])
    for s in range(NC):
        group("c%d" % s, ssm_in(s), kv_in(s, s))
    group("c3", ssm_in(3), ssm_in(4))
    group("wma", wm_in(0, 3), q_in(0, 0), q_in(1, 1))
    group("wmb", wm_in(3, 5))
    group("w1", whole(w1_hbm, w1_v))
    group("w2", q_in(2, 2), whole(w2_hbm, w2_v))
    group("w3", whole(w3_hbm, w3_v))
    group("w4", whole(w4_hbm, w4_v.at[0:F]), wm_in(5, 6))
    for g in dmas.values():
        for c in g:
            c.start()

    def wait(name):
        for c in dmas[name]:
            c.wait()

    tau_b = lambda l: H + ((l + (H - 1)) & (H - 1))
    tf_v[:, C(0)] = _dft((T, H), 0, lambda l: jnp.where((l & 1) == 0, l, tau_b(l)), 1.0 / T)
    tf_v[:, C(1)] = _dft((T, H), 0, lambda l: jnp.where((l & 1) == 1, l, tau_b(l)), 1.0 / T)
    tf_v[:, C(2)] = _dft((T, H), 0, lambda l: 2 * l - H)
    tf_v[:, C(3)] = _dft((T, H), 0, lambda l: 2 * l + 1 - H)
    sin0 = lax.broadcasted_iota(I32, (GR, T), 1) >= H
    tg_v[:, 0:T] = _dft((GR, T), 1, lambda l: jnp.where(sin0 & (l == 0), H, 2 * l))
    tg_v[:, T:2 * T] = _dft((GR, T), 1, lambda l: 2 * l + 1)
    h1_v[:, 0:8, :] = jnp.zeros((NT, 8, 128), F32)
    h1_v[:, 8 + NC * T:16 + NC * T, :] = jnp.zeros((NT, 8, 128), F32)

    wait("small")
    z = jnp.clip(z_s[0, 0], 0, 1)
    zero = jnp.full((8, 128), z, I32).astype(U32)
    z8 = pl.multiple_of(z * 8, 8)
    for r in (x_v, hb_v, x1_v, r_v, zraw, n1_w, n2_w, g_w, a_w, kv_w, zz_w, *ws_w, *as_w, w3n_w, top_v, st_v, *l2_w):
        r[pl.ds(z8, 8), 0:128] = jnp.zeros((8, 128), r.dtype)
    for r in (kf, uf, acc, taps, mod_v):
        r[z, 0:8, 0:128] = jnp.zeros((8, 128), r.dtype)
    for r in (tf_w, tg_w):
        r[pl.ds(z8, 8), 0:128] = r[0:8, 0:128]
    sh = sh_v[...].astype(F32)
    for i in range(4):
        taps[i] = jnp.broadcast_to(sh[i:i + 1], (8, D))
    taps[4] = jnp.broadcast_to(sd_v[...].astype(F32).reshape(1, D) * (1.0 / T), (8, D))
    cf = c_v[...].astype(F32)
    silu_c = jnp.broadcast_to((cf / (1.0 + jnp.exp(-cf))).astype(BF16), (16, D))

    def mmK(n):
        def unit(m):
            st = []

            def rhs(i):
                if not st:
                    ev = (lax.broadcasted_iota(I32, (64, 128), 1) & 1) == 0
                    a = ssm_w[n][:, m * T:m * T + H]
                    b = pltpu.roll(ssm_w[n][:, m * T + H:(m + 1) * T], 1, 1)
                    st.extend([pltpu.bitcast(jnp.where(ev, a, b), BF16), pltpu.bitcast(jnp.where(ev, b, a), BF16)])
                return st[i]

            def epi(p):
                er, ei, or_, oi = p
                if m == 0:
                    er = er + taps[4, 0:1, C(n)]
                for h, (cr, ci) in enumerate(((er + or_, ei + oi), (er - or_, ei - oi))):
                    B = h * 3 * H
                    kf[m, B:B + H, C(n)] = cr
                    kf[m, B + H:B + 2 * H, C(n)] = ci - cr
                    kf[m, B + 2 * H:B + 3 * H, C(n)] = ci + cr
            return Unit("K%d" % n, [(lambda i=i, r=r: (tf_v[r:r + H, C(i)], rhs(i))) for i in range(2) for r in (0, H)],
                        epi, H, 170, nt=True)
        return [unit(m) for m in range(NB)]

    def kv(s, sl):
        def mk(t, w):
            def fn(a):
                ld = lambda o, n: k_n[s][t, pl.ds(8 + w + o, n), :]
                c0 = jnp.concatenate([_tie(ld(0, 8), a), ld(8, 8)], axis=0).reshape(2, 8, 128)
                c1, c2 = ld(-1, 16).reshape(2, 8, 128), ld(-2, 16).reshape(2, 8, 128)
                s0, s1, s2, s3 = (taps[i, :, C(t)] for i in range(4))
                ke, ko, ke1, ko1, ko2 = _lo(c0), _hi(c0), _lo(c1), _hi(c1), _hi(c2)
                wv = v_n[s][t, w:w + 16, :].reshape(2, 8, 128)
                kve = ((s0 * ke + s1 * ko1) + (s2 * ke1 + s3 * ko2)) * _lo(wv)
                kvo = ((s0 * ko + s1 * ke) + (s2 * ko1 + s3 * ke1)) * _hi(wv)
                kv_v[pl.ds(sl * T + w, 16), C(t)] = kve.reshape(16, 128).astype(BF16)
                kv_v[pl.ds(sl * T + H + w, 16), C(t)] = kvo.reshape(16, 128).astype(BF16)
            return fn
        return [[mk(t, w) for w in range(0, H, 16)] for t in range(NT)]

    def mmU(name, sl, us):
        def unit(n):
            def epi(p):
                er, ei, or_, oi = p
                for h, (cr, ci) in enumerate(((er + or_, ei + oi), (er - or_, ei - oi))):
                    B = h * 3 * H
                    uf[us, B:B + H, C(n)] = cr + ci
                    uf[us, B + H:B + 2 * H, C(n)] = cr
                    uf[us, B + 2 * H:B + 3 * H, C(n)] = ci
            return Unit(name(n), [(lambda i=i, r=r: (tf_v[r:r + H, C(2 + i)], kv_v[pl.ds(sl * T + i * H, H), C(n)]))
                                  for i in range(2) for r in (0, H)], epi, H, 120)
        return [unit(n) for n in range(NT)]

    def cmul(m0, u0, n, h, row, L, a):
        t = []
        for i in range(3):
            Rw = slice((3 * h + i) * H + row, (3 * h + i) * H + row + 8)
            kk = kf[m0:m0 + n, Rw, L]
            if i == 0 and a is not None:
                k0 = _tie(kk[0], a)[None]
                kk = k0 if n == 1 else jnp.concatenate([k0, kk[1:]], axis=0)
            t.append(jnp.sum(kk * uf[u0:u0 + n, Rw, L], axis=0))
        return t[0] - t[2], t[0] + t[1]

    def AR(h, q, row):
        return slice((2 * h + q) * H + row, (2 * h + q) * H + row + 8)

    def mac(n, u0, sl, first=False, part=False):
        def mk(t, rc):
            st, fin = [], []

            def piece(i):
                def fn(a):
                    h, row = i & 1, rc + (i >> 1) * 8
                    zr, zi = cmul(0, u0, n, h, row, C(t), a)
                    if part:
                        zr, zi = zr + acc[0, AR(h, 0, row), C(t)], zi + acc[0, AR(h, 1, row), C(t)]
                    st.append((zr, zi))
                    if h:
                        (pr, pi), (mr, mi) = st[-2:]
                        z = [pr + mr, pi + mi, pr - mr, pi - mi]
                        Rw = lambda q: slice(q * H + row, q * H + row + 8)
                        pv = None if first else [zraw[Rw(q ^ 1), C(t)] for q in range(4)]
                        for q in range(4):
                            zraw[Rw(q), C(t)] = z[q]
                        if not first:
                            z = [z[q] + pv[q] if (q & 1) == (rc < 64) else z[q] - pv[q] for q in range(4)]
                        fin.append(z)
                    if i == 3:
                        for q in range(4):
                            zz_v[pl.ds(sl * 2 * T + q * H + rc, 16), C(t)] = jnp.concatenate(
                                [fin[0][q], fin[1][q]], axis=0).astype(BF16)
                return fn
            if not part:
                return [piece(i) for i in range(4)]
            both = lambda f, g: (lambda a: (f(a), g(None)))
            return [both(piece(0), piece(1)), both(piece(2), piece(3))]
        return [[fn for rc in range(0, H, 16) for fn in mk(t, rc)] for t in range(NT)]

    def pos():
        return [(t, h, row) for t in range(NT) for row in range(0, H, 8) for h in range(2)]

    def ahead(i):
        def mk(t, h, row):
            def fn(a):
                zr, zi = cmul(i + 1, 0, NC, h, row, C(t), a)
                acc[i, AR(h, 0, row), C(t)] = zr
                acc[i, AR(h, 1, row), C(t)] = zi
            return fn
        return [mk(*p) for p in pos()]

    def spread():
        n = NB - NC - 1

        def mk(t, h, row):
            def fn(a):
                p = []
                for i in range(3):
                    Rw = slice((3 * h + i) * H + row, (3 * h + i) * H + row + 8)
                    u = uf[0, Rw, C(t)]
                    p.append(kf[1:1 + n, Rw, C(t)] * (_tie(u, a) if i == 0 else u)[None])
                acc[0:n, AR(h, 0, row), C(t)] = acc[1:1 + n, AR(h, 0, row), C(t)] + (p[0] - p[2])
                acc[0:n, AR(h, 1, row), C(t)] = acc[1:1 + n, AR(h, 1, row), C(t)] + (p[0] + p[1])
            return fn
        return [mk(*p) for p in pos()]

    def mmI(name, sl, ys):
        def unit(n):
            def epi(p):
                ce, se, co, so = p
                sub = lax.broadcasted_iota(I32, (8, 128), 0)
                c0 = ys * T + H
                y_v[n, ys * T:ys * T + 1, :] = (ce[64:72] - se[0:8])[0:1]
                se = jnp.concatenate([jnp.where(sub == 0, 0.0, se[0:8]), se[8:]], axis=0)
                for d, cc, ss in ((0, ce[0:64], se), (1, co, so)):
                    y_v[n, pl.ds(c0 + d, 64, stride=2), :] = cc + ss
                    lo = cc - ss
                    for i in range(0, 64, 8):
                        y_v[n, pl.ds(c0 - d - 2 * i - 14, 8, stride=2), :] = jnp.take_along_axis(
                            lo[i:i + 8], 7 - sub, axis=0)
            return Unit(name(n), [(lambda i=i: (tg_v[0:(GR if i == 0 else 64), C(i)], zz_v[pl.ds(sl * 2 * T + i * H, H), C(n)]))
                                  for i in range(4)], epi, 64, 52)
        return [unit(n) for n in range(NT)]

    def mod(name, a, b):
        def unit(n):
            def epi(p):
                v = [_sum(p[i * NT:(i + 1) * NT])[0:8] for i in range(b - a)]
                if a == 0:
                    mod_v[0, :, C(n)] = v[0] * v[2]
                    mod_v[1, :, C(n)] = (v[1] + 1.0) * v[2]
                elif a == 3:
                    mod_v[3, :, C(n)] = v[0]
                    mod_v[4, :, C(n)] = v[1] + 1.0
                else:
                    mod_v[5, :, C(n)] = v[0]
                    mod_v[2, :, C(n)] = v[0] * G_POST
            return Unit(name, [(lambda i=i, k=k: (silu_c[:, C(k)], wm_v[a][C(k), pl.ds(i * D + n * 128, 128)]))
                               for i in range(b - a) for k in range(NT)], epi, 16, 10, full=False, acc=b - a == 1)
        return [unit(n) for n in range(NT)]

    HS = (slice(0, 128), slice(128, 256))
    QS = tuple(slice(r, r + 64) for r in range(0, T, 64))

    def tasks(f, due=None, tie=True, n=RG):
        def mk(R):
            def fn(a):
                x = f(R, a if tie else None)
                return Due(x, due) if due else None
            return fn
        return [mk(slice(r, r + n)) for r in range(0, T, n)]

    def load_y(sl, R):
        return jnp.concatenate([y_v[t, sl * T + R.start:sl * T + R.stop, :] for t in range(NT)],
                               axis=1).reshape(2, 8, D)

    def put(nn, ss, R, x):
        nn[R, :] = x.astype(BF16)
        tok = x
        if ss is not None:
            S2 = pl.ds(R.start // 32 * 16, 16)
            if R.stop % 32:
                top_v[S2, 0:2 * T] = x[:, 0:2 * T]
            else:
                if R.start % 32:
                    x = jnp.concatenate([top_v[S2, 0:2 * T], x[:, 0:2 * T]], axis=0)
                ss[S2, 0:5 * T] = jnp.concatenate(_lhs_sums(x[:, 0:T], x[:, T:2 * T]), axis=1).astype(BF16)
        return tok

    wide = lambda v: jnp.concatenate([v] * NT, axis=1)

    def mean(i, R, x):
        st_v[R, C(i)] = jnp.broadcast_to(jnp.sum(x, axis=-1, keepdims=True) * (1.0 / D), (x.shape[0], 128))

    def centred(src, i, R, a):
        return src[R, :] - wide(_tie(st_v[R, C(i)], a))

    def scale(src, i, g):
        def f(R, a):
            st_v[R, C(i + 1)] = jnp.broadcast_to(_rstd(centred(src, i, R, a), g), (RG, 128))
        return f

    def normed(src, i, R, a):
        return centred(src, i, R, a) * wide(st_v[R, C(i + 1)])

    def front(sl, xs, early=False, ss=None):
        xx, hh, nn = view(x_v, xs), view(hb_v, xs), view(n1_v, sl)

        def fa(R, a):
            q = [q_n[sl][t, R.start // 2:R.stop // 2, :] for t in range(NT)]
            q = jnp.concatenate([_tie(q[0], a)] + q[1:], axis=1)
            q = pltpu.bitcast(q, BF16).astype(F32).reshape(2, 8, D)
            x = (q + (_ln(q) * mod_v[1] + mod_v[0]) * load_y(sl, R)).reshape(RG, D)
            xx[R, :] = x
            if early:
                hh[R, :] = _ln(x)

        def fb(R, a):
            hh[R, :] = (_ln(_tie(xx[R, :], a).reshape(2, 8, D)) * mod_v[4] + mod_v[3]).reshape(RG, D)

        def fc(R, a):
            hb = _tie(hh[R, :], a)
            if early:
                hb = (hb.reshape(2, 8, D) * mod_v[4] + mod_v[3]).reshape(RG, D)
                hh[R, :] = hb
            nn[R, :] = _ln(hb, G_A).astype(BF16)
        if early:
            return tasks(fa), tasks(fc)
        if ss is None:
            return tasks(fa) + tasks(fb) + tasks(fc)
        qf = view(x_v, 2)

        def s1(R, a):
            q = [q_n[sl][t, R.start // 2:R.stop // 2, :] for t in range(NT)]
            q = pltpu.bitcast(jnp.concatenate([_tie(v, a) for v in q], axis=1), BF16).astype(F32)
            qf[R, :] = q
            mean(0, R, q)

        def s3(R, a):
            h = normed(qf, 0, R, a).reshape(2, 8, D) * mod_v[1] + mod_v[0]
            x = qf[R, :] + (h * load_y(sl, R)).reshape(RG, D)
            xx[R, :] = x
            mean(2, R, x)

        def s5(R, a):
            hb = (normed(xx, 2, R, a).reshape(2, 8, D) * mod_v[4] + mod_v[3]).reshape(RG, D)
            hh[R, :] = hb
            mean(4, R, hb)
        s7 = [f for g in tasks(lambda R, a: put(nn, ss, R, normed(hh, 4, R, a)), n=32) for f in (g, lambda a: None)]
        st = [tasks(s3), tasks(scale(xx, 2, 1.0)), tasks(s5), tasks(scale(hh, 4, G_A)), s7]
        p = [tasks(s1), tasks(scale(qf, 0, 1.0))]
        return cat(x[:8] for x in st), cat(x[8:] for x in p + st), cat(x[:8] for x in p)

    def shift(hs, sl, pieces=((0, 64), (64, 64), (128, 64), (192, 64)), ss=None):
        gg = view(g_v, sl)

        def one_tile(t, r, n, a):
            lane = lax.broadcasted_iota(I32, (n, 128), 1)
            ld = lambda d: h1_v[t, pl.ds(hs * T + 8 + r + d, n), :]
            if t == 0:
                g = ld(-1)
            elif t == 1:
                g = jnp.where(lane < 32, ld(-1), ld(1))
            elif t == 2:
                g = jnp.where(lane < 64, ld(1), ld(-2))
            elif t == 3:
                g = jnp.where(lane < 96, ld(-2), ld(2))
            else:
                g = ld(2)
            if a is not None:
                g = jnp.concatenate([_tie(g[i:i + 8], a) if i % 16 == 0 else g[i:i + 8]
                                     for i in range(0, n, 8)], axis=0)
            gg[r:r + n, C(t)] = g.astype(BF16)
            return g

        def mk(ts, r, n):
            def fn(a):
                g = [one_tile(t, r, n, a) for t in ts]
                if len(ts) == 2:
                    for i, x in enumerate(_lhs_sums(*g)):
                        ss[r // 2:(r + n) // 2, C(2 * i + ts[0])] = x.astype(BF16)
            return fn
        sets = [(t,) for t in range(NT)] if ss is None else [(0, 2), (1, 3), (4,)]
        return [mk(ts, r, n) for ts in sets for r, n in pieces]

    def shift_early():
        def keep(a):
            h1_v[:, 2 * T - 32:2 * T + 8, :] = h1_v[:, 3 * T - 32:3 * T + 8, :]
        return shift(2, 0, [(r, 32) for r in range(0, T - 32, 32)], gs) + [keep]

    def ln2(xs, sl, fast=True):
        xx, nn, ss = view(x1_v, xs), view(n2_v, sl), view(n2s, sl, H) if fast else None
        f = lambda R, a: put(nn, ss, R, _ln(_tie(xx[R, :], a), G_A))
        ts = tasks(f, DL, False)
        return ts[0::2] + ts[1::2] if fast else tasks(f)

    def resid(xs, x1s, rotate=False):
        xx, x1 = view(x_v, xs), view(x1_v, x1s)

        def f(R, a):
            gb = mod_v[5] if a is None else pltpu.bitcast(
                pltpu.bitcast(mod_v[5], U32) | jnp.concatenate([a] * NT, axis=1), F32)
            r_v[R, :] = xx[R, :] + (x1[R, :].reshape(2, 8, D) * gb).reshape(RG, D)
            if rotate:
                xx[R, :] = x_v[R, :]
                view(hb_v, 1)[R, :] = hb_v[R, :]
        return tasks(f)

    KD, KF, ND = [(0, 2), (1, 3)], [(2 * i, 2 * i + 1) for i in range(7)], [(1, 2), (3, 4)]
    Wt = {1: (lambda k, n: w1_v[C(k), C(n)], lambda i, kp, j: w1s[C(kp), C(2 * i + j)], False, KD, [4]),
          2: (lambda k, n: w2_v[C(k), C(n)], lambda i, kp, j: w2s[C(kp), C(2 * i + j)], False, KD, [4]),
          0: (lambda k, n: w3_v[C(n), C(k)], None, True, KD, [4]),
          3: (lambda k, n: w3n[C(k), C(n)], lambda i, kp, j: w3s[C(kp), C(6 * i + j)], False, KD, [4]),
          4: (lambda k, n: w4_v[C(k), C(n)], lambda i, kp, j: w4s[C(kp), C(2 * i + j)], False, KF, [])}

    def sums_task(load, store, left):
        def fn(a):
            b = [[load(u, v) for v in range(2)] for u in range(2)]
            b[0][0], b[1][1] = _tie(b[0][0], a), _tie(b[1][1], a)
            (x11, x12), (x21, x22) = [[pltpu.bitcast(x, BF16).astype(F32) for x in row] for row in b]
            r = ((x11 + x22, x21 + x22, x11 + x12, x21 - x11, x12 - x22) if left else
                 (x11 + x22, x12 - x22, x21 - x11, x11 + x12, x21 + x22))
            for m, x in enumerate(r):
                store(m, x.astype(BF16))
        return fn

    def wsums(w_w, ws, rp, cp_):
        def mk(i, j, r):
            def store(m, x):
                ws[pl.ds(128 * i + r, 16), C(len(cp_) * m + j)] = x
            return sums_task(lambda u, v: w_w[pl.ds(64 * rp[i][u] + r // 2, 8), C(cp_[j][v])], store, False)
        return [mk(i, j, r) for j in range(len(cp_)) for i in range(len(rp)) for r in range(0, 128, 16)]

    def w3_turn():
        def mk(n, k):
            def fn(a):
                x = jnp.concatenate([_tie(w3_w[64 * n:64 * n + 8, C(k)], a), w3_w[64 * n + 8:64 * n + 64, C(k)]], axis=0)
                w3n[C(k), C(n)] = pltpu.bitcast(x, BF16).T
            return fn
        return [mk(n, k) for n in range(FT - 1) for k in range(NT)]

    def plain(name, w, lhs, n, R, epi, cost):
        tile, _, nt, kp, kl = Wt[w]
        ks = sorted([k for p in kp for k in p] + kl)
        rows_ = R.stop - R.start
        return Unit(name, [(lambda k=k: (lhs[R, C(k)], tile(k, n))) for k in ks], lambda p: epi(n, R, p[0]),
                    rows_, rows_ // 8 * (len(ks) - 1 + cost), nt=nt, acc=True)

    def quad(name, w, lhs, sums, j, cols_, R, epi, cost):
        tile, wsum, nt, kp, kl = Wt[w] if isinstance(w, int) else w
        h, S2, c = len(kp), slice(R.start // 2, R.stop // 2), {}
        a_ = lambda i, k: _top(lhs(k) if callable(lhs) else lhs[R, C(k)], i)
        s_ = sums if callable(sums) else (lambda i, p: sums[S2, C(h * i + p)])
        prod = lambda fa_, fb_: [(lambda p=p: (fa_(p), fb_(p))) for p in range(h)]
        left = lambda i, n: [(lambda k=k: (a_(i, k), tile(k, n))) for k in kl]
        mk = lambda tiles, f, x=0: Unit(name, tiles, lambda p: f(p[0]), 64, 8 * len(tiles) + x, nt=nt, acc=True)

        def e1(m):
            u7.res, u6.res = [m], [m]

        def e4(m):
            c[11], c[21] = c[11] + m, m

        def e2(m):
            c[21], c[22] = c[21] + m, c[22] - m
            l21.res = [c[21]]

        def e5(m):
            c[12] = m
            epi(cols_[0], R, _zip(c[11] - m, c[21]))

        def e3(m):
            l12.res, c[22] = [c[12] + m], c[22] + m
            if not kl:
                l12.epi(l12.res)
        u1 = mk(prod(lambda p: s_(0, p), lambda p: wsum(0, p, j)), e1)
        u7 = mk(prod(lambda p: s_(4, p), lambda p: wsum(4, p, j)) + left(0, cols_[0]), lambda m: c.update({11: m}))
        u6 = mk(prod(lambda p: s_(3, p), lambda p: wsum(3, p, j)) + left(1, cols_[1]), lambda m: c.update({22: m}))
        u4 = mk(prod(lambda p: a_(1, kp[p][1]), lambda p: wsum(2, p, j)), e4)
        u2 = mk(prod(lambda p: s_(1, p), lambda p: tile(kp[p][0], cols_[0])), e2, 8)
        l21 = mk(left(1, cols_[0]), lambda m: c.update({21: m}))
        u5 = mk(prod(lambda p: s_(2, p), lambda p: tile(kp[p][1], cols_[1])), e5, 16 * cost)
        u3 = mk(prod(lambda p: a_(0, kp[p][0]), lambda p: wsum(1, p, j)), e3, 8 if kl else 8 + 16 * cost)
        l12 = mk(left(0, cols_[1]), lambda m: epi(cols_[1], R, _zip(m, c[22])), 16 * cost)
        return [u1, u7, u6, u4, u2, l21, u5, u3, l12]

    LH, RH = [0, 4, 3, (1, 1), 1, 2, (0, 0)], [0, 4, 3, 2, (0, 0), (1, 1), 1]
    L2 = {3: (w3n_w, ws_w[2], w3t, KF[:6], n2t), 4: (w4_w, ws_w[3], w4t, ND, a_t)}

    def wsums2(w):
        w_w, s_w, ws2, cp_, _ = L2[w]
        kp, nj = Wt[w][3], len(cp_)

        def mk(o, p2, j2, r):
            def load(u, v):
                p, j, y = 2 * p2 + u, 2 * j2 + v, RH[o]
                if isinstance(y, int):
                    return s_w[pl.ds(64 * p + r // 2, 8), C(nj * y + j)]
                return w_w[pl.ds(64 * kp[p][y[0]] + r // 2, 8), C(cp_[j][y[1]])]

            def store(m, x):
                ws2[pl.ds(128 * p2 + r, 16), C((5 * o + m) * (nj // 2) + j2)] = x
            return sums_task(load, store, False)
        return [mk(o, p2, j2, r) for j2 in range(nj // 2) for o in range(7) for p2 in range(len(kp) // 2)
                for r in range(0, 128, 16)]

    def lsums2(w, lhs_w, sums_w, sl):
        kp, xs2 = Wt[w][3], L2[w][4]
        h2 = len(kp) // 2

        def mk(o, p2, g):
            def load(u, v):
                p, ch, x = 2 * p2 + v, 2 * g + u, LH[o]
                if isinstance(x, int):
                    return sums_w[pl.ds(64 * sl + 8 * ch, 8), C(len(kp) * x + p)]
                return lhs_w[pl.ds(H * sl + 16 * ch + 8 * x[0], 8), C(kp[p][x[1]])]

            def store(m, x):
                xs2[pl.ds(16 * g, 16), C((5 * o + m) * h2 + p2)] = x
            return sums_task(load, store, True)
        return [[mk(o, p2, g) for o in range(7) for g in range(4)] for p2 in range(h2)]

    def quad2(name, w, lhs, sums, j2, epi, cost):
        tile, wsum, nt, kp, kl = Wt[w]
        ws2, cp_, xs2 = L2[w][2:]
        h, h2, nj2, c, R = len(kp), len(kp) // 2, len(cp_) // 2, {}, slice(0, T)

        def done(j, v):
            val = _zip(c[j, 1, v], c[j, 2, v])
            if not kl:
                return epi(cp_[j][v], R, val)
            c[j, v] = val

        def upd(o, j, m):
            for i, v, sg in (((1, 0, 1), (2, 1, 1)), ((1, 0, 1),), ((2, 1, 1),), ((1, 0, 1), (2, 0, 1)),
                             ((2, 0, 1), (2, 1, -1)), ((1, 0, -1), (1, 1, 1)), ((1, 1, 1), (2, 1, 1)))[o]:
                k = (j, i, v)
                c[k] = m if k not in c else (c[k] + m if sg > 0 else c[k] - m)
            if o >= 5:
                done(j, o - 5)

        def inner(o):
            x, y = LH[o], RH[o]
            xo = ((lambda p: sums[:, C(h * x + p)]) if isinstance(x, int)
                  else (lambda p: _top(lhs[:, C(kp[p][x[1]])], x[0])))
            yo = ((lambda p, j: wsum(y, p, j)) if isinstance(y, int)
                  else (lambda p, j: tile(kp[p][y[0]], cp_[j][y[1]])))
            w_ = (yo, lambda m, p2, _: ws2[C(p2), C((5 * o + m) * nj2 + j2)], nt,
                  [(2 * i, 2 * i + 1) for i in range(h2)], list(range(2 * h2, h)))
            return quad(name, w_, xo, lambda m, p2: xs2[:, C((5 * o + m) * h2 + p2)], 0, (2 * j2, 2 * j2 + 1),
                        HS[0], lambda j, _, m: upd(o, j, m), 2 + (2 * cost if o >= 5 and not kl else 0))

        def rest(j, v, Q):
            return [Unit(name, [lambda: (lhs[Q, C(k)], tile(k, cp_[j][v]))],
                         lambda p: epi(cp_[j][v], Q, p[0] + c[j, v][Q]), 64, 8 * (cost + 1)) for k in kl]
        return cat(inner(o) for o in range(7)), [u for Q in QS for j in (2 * j2, 2 * j2 + 1) for v in range(2)
                                                 for u in rest(j, v, Q)]

    def mm(name, w, lhs, sums, epi, cost):
        if sums is None:
            return [[plain(name, w, lhs, n, R, epi, cost) for R in HS] for n in range(NT)]
        return [[plain(name, w, lhs, 0, R, epi, cost) for R in QS]] + [
            [u for R in HS for u in quad(name, w, lhs, sums, j, ND[j], R, epi, cost)] for j in range(2)]

    def mm1(name, hs, sl, fast=False):
        def epi(n, R, p):
            h1_v[n, pl.ds(hs * T + 8 + R.start, R.stop - R.start), :] = _gelu2(p)
        return cat(mm(name, 1, view(n1_v, sl), n1s if fast else None, epi, 5))

    def mm2(name, sl, xs, x1s, fast=False):
        def epi(n, R, p):
            view(x1_v, x1s)[R, C(n)] = view(hb_v, xs)[R, C(n)] + p * G_POST
        return cat(mm(name, 2, view(g_v, sl), gs if fast else None, epi, 2))

    def mm3(name, sl, fast=True):
        nn, aa, ss, keep, tail = view(n2_v, sl), view(a_v, sl), view(a_s, sl, H), {}, []

        def epi(n, R, p):
            g = _gelu2(p)
            aa[R, C(n)] = g.astype(BF16)
            if n % 2 == 0 and n < 12:
                keep[n] = g
                return
            pair = (keep.pop(n - 1), g) if n % 2 else (g, tail[R.start // 128][R.start % 128:R.start % 128 + 64])
            for i, x in enumerate(_lhs_sums(*pair)):
                ss[R.start // 2:R.stop // 2, C(7 * i + n // 2)] = x.astype(BF16)

        def rem(R):
            def f(p):
                tail.append(jnp.concatenate([_gelu2(p[0]), jnp.zeros((64, 128), F32)], axis=0).T)
                aa[R, C(13)] = tail[-1].astype(BF16)
            return Unit(name, [(lambda k=k: (w3_v[13 * 128:F, C(k)], nn[R, C(k)])) for k in range(NT)], f, 64, 84,
                        nt=True, acc=True)
        odd = [rem(R) for R in HS] + [plain(name, 3 if fast else 0, nn, 12, R, epi, 9) for R in QS]
        if fast == 2:
            qd = [quad2(name + "_%d" % j, 3, nn, view(n2s, sl, H), j, epi, 8) for j in range(3)]
            return odd[:2] + qd[0][0] + _weave(qd[1][0], qd[0][1]) + _weave(qd[2][0], qd[1][1]) + _weave(odd[2:], qd[2][1])
        if fast:
            qd = [u for j in range(6) for R in HS for u in quad(name, 3, nn, view(n2s, sl, H), j, KF[j], R, epi, 8)]
            return qd[:18] + odd[:2] + qd[18:36] + odd[2:] + qd[36:]
        return odd + [plain(name, 0, nn, n, R, epi, 8) for p in KF[:6] for R in HS for n in p]

    NA = 3 * 128

    def cp_out(j, osl, L, sm, R=slice(0, T)):
        return cp(o_v.at[pl.ds(osl * T + R.start, R.stop - R.start), L],
                  o_hbm.at[pl.ds(base(j, T) + R.start, R.stop - R.start), L], sem_o.at[sm])

    out_a = lambda j: cp_out(j, 0, slice(0, NA), 0)
    out_b = lambda j: cp_out(j, 0, slice(NA, D), 1)
    last = []

    def mm4(name, j, sl, osl=0, xs=None, x1s=None, fast=True):
        oo = view(o_v, osl)

        def epi(n, R, p):
            if xs is None:
                oo[R, C(n)] = (r_v[R, C(n)] + mod_v[2, 0:1, C(n)] * p).astype(BF16)
            else:
                oo[R, C(n)] = (view(x_v, xs)[R, C(n)] + mod_v[5, 0:1, C(n)]
                               * (view(x1_v, x1s)[R, C(n)] + p * G_POST)).astype(BF16)
            if osl == 2:
                last.append(cp_out(j, osl, C(n), 2, R))
                last[-1].start()
            elif R.stop == T and (osl, (n + 1) * 128) in ((1, D), (3, NA)):
                last.append(cp_out(j, osl, slice(0, (n + 1) * 128), 2))
                last[-1].start()
            elif R.stop == T and osl == 0 and (n + 1) * 128 in (NA, D):
                (out_a if (n + 1) * 128 == NA else out_b)(j).start()
        if fast == 2:
            return ([plain(name, 4, view(a_v, sl), 0, R, epi, 5) for R in QS],
                    quad2(name + "q", 4, view(a_v, sl), view(a_s, sl, H), 0, epi, 5)[0])
        return mm(name, 4, view(a_v, sl), view(a_s, sl, H) if fast else None, epi, 3 if xs is None else 5)

    def split(us):
        n = 4 // len(us)
        m, mks, st = us[0].rows // n, [u.tiles.pop(0) for u in us], {}

        def piece(i, k):
            if i not in st:
                st[i] = mks[i]()
            return st[i][0][m * k:m * (k + 1)], st[i][1]

        def epi(p):
            for i, u in enumerate(us):
                u.res = [jnp.concatenate(p[n * i:n * (i + 1)], axis=0)]
        return _flat([Unit(us[0].name, [(lambda i=i, k=k: piece(i, k)) for i in range(len(us)) for k in range(n)],
                           epi, m, 0, nt=us[0].nt)])

    W = lambda nm: [("wait", nm)]
    run = lambda fns: [("run", "run", lambda: [fn(None) for fn in fns])]
    one = lambda us: [_flat([u]) for u in us]
    nm = lambda x: (lambda n: x)

    seq, grp = [], []
    for s in range(NC):
        seq += W("c%d" % s) + _flat(mmK(s) + mmU(nm("U%d" % s), s % 2, NC - 1 - s))
        grp.append(Group("kv%d" % s, cat(kv(s, s % 2)), 50, ["c%d" % s], ["U%d" % s], 100))
    inv = [mmI(lambda n: "I%d" % n, s, s) for s in range(NC)]
    seq += W("c3") + _flat(mmK(3) + mmK(4) + [inv[s][t] for t in range(NT) for s in range(NC)])
    macs = [mac(s + 1, NC - 1 - s, s, first=s == 0) for s in range(NC)]
    grp.append(Group("mac00", macs[0][0], 12, ["c1"], ["c2"], 0))
    grp.append(Group("mac01", macs[1][0] + macs[0][1] + macs[1][1], 16, ["c2"], ["c3"], 0))
    for t in range(NT):
        grp.append(Group("mac%d" % t, cat(macs[s][t] for s in range(2 if t < 2 else 0, NC)), 24 if t < 2 else 18,
                         ["c3", "K%d" % t], ["I%d" % t], 100, 150))
    start = lambda cs: [("run", "run", lambda: [c.start() for c in cs])]
    f0, f1 = front(0, 2, True), front(1, 1, True)
    seq += run(ahead(0))
    seq += W("wma") + _flat(mod("moda", 0, 3)) + run(f0[0] + f1[0] + ahead(1))
    seq += W("wmb") + start(next_kv(NC) + next_q(NC)) + _flat(mod("modb", 3, 5)) + run(f0[1])
    w1 = _flat(mm1("w1_0", 0, 0) + mm1("w1_1", 1, 1))
    seq += W("w1") + w1[:72] + W("w2") + w1[72:] + run(shift(0, 0))
    seq += _flat(mm2("w2_0", 0, 2, 1) + mm1("w1_2", 2, 2)) + run(shift(1, 1)) + _flat(mm2("w2_1", 1, 1, 0))
    grp.append(Group("f1", f1[1], 80, ["w1"], ["w1_1"], 450))
    grp.append(Group("f2", front(2, 0), 80, ["w2"], ["w1_2"], 450))
    grp.append(Group("ln2_0", ln2(1, 0, False), 60, ["w2_0"], ["w3"], 450))
    grp.append(Group("ahead", cat(ahead(i) for i in range(2, NB - NC)), 19, ["w1"], ["end"], 100))
    grp.append(Group("ws1", wsums(w1_w, w1s, KD, ND), 26, ["w1"], ["end"], 100))
    grp.append(Group("ws2", wsums(w2_w, w2s, KD, ND), 26, ["w2"], ["end"], 100))
    grp.append(Group("ws3", w3_turn() + wsums(w3n_w, w3s, KD, KF[:6]) + wsums2(3), 24, ["w3"], ["end"], 100))
    grp.append(Group("ws4", wsums(w4_w, w4s, KF, ND), 26, ["w4"], ["end"], 100))
    _wait(seq, "w3", back=1)
    w3 = mm3("w3_0", 0, False)
    _mix(seq, _flat(w3[6:]), [split(w3[4:6]) + _flat(w3[:6])], 0.1)
    mc = _flat(mod("modc", 5, 6))
    _wait(seq, "w4", mc[:5] + [("sync", "run", lambda: None)])
    w4 = cat(mm4("w4_0", 0, 0, 3, 2, 1, False)[:3])
    qs = [split([w4[-1 - i]]) for i in range((_phase(seq) + FT * 6) % 4)]
    _mix(seq, _flat(w4), [mc[i:i + 4] for i in range(5, 25, 4)] + qs, 0.01, 0.4)
    assert _phase(seq) == 0
    grp.append(Group("resid", resid(2, 1), 26, ["modc"], ["end"], 100))
    _emit(seq, grp, zero, wait)

    def step(s, carry):
        for c in next_kv(s) + next_q(s):
            c.wait()
        nxt = jnp.minimum(s + 1, NB - 1)
        seq, grp = [], []
        us, it = one(mmU(lambda n: "U%d" % n, 0, 0)), one(mmI(lambda n: "I%d" % n, 0, 0))
        w4 = mm4("w4", s - 2, 0)
        q = split(w4[0][2:])
        _mix(seq, _flat(mm4("w4c", s - 3, 0)[2] + mm3("w3", 0)),
             [us[0], us[1], us[2], it[0] + us[3], it[1] + us[4], it[2] + start(next_kv(nxt)), it[3], it[4]],
             0.26, 0.78)
        w1a, w1b = mm1("w1a", 2, 0, True), mm1("w1b", 2, 0, True)
        w1a, w1b = _flat(w1a[0:2] + w1a[4:13] + w1a[22:31]), _flat(w1b[2:4] + w1b[13:22] + w1b[31:])
        _mix(seq, _flat(w4[0] + w4[1][:9]), [q])
        seq += w1a + run(shift(1, 0, ((T - 32, 32),), gs)) + _flat(w4[1][9:]) + w1b[:8] + start(next_q(nxt)) + w1b[8:]
        seq += _flat(mm2("w2", 0, 1, 0, True))
        assert _phase(seq) == 0
        kvs, macs = kv(0, 0), mac(1, 0, 0, part=True)
        for t in range(NT):
            grp.append(Group("kv%d" % t, kvs[t], 50, ["start"], ["U%d" % t], 300))
            grp.append(Group("mac%d" % t, macs[t], 28, ["U%d" % t], ["I%d" % t], 300, 150))
        iall = ["I%d" % t for t in range(NT)]
        grp.append(Group("ln2", ln2(0, 0), 75, ["start"], ["w3"], 450))
        grp.append(Group("resid", resid(1, 0, True), 40, ["w4c"], ["w4", "I4"], 100))
        fr = front(0, 0, ss=n1s)
        grp.append(Group("fronta", fr[0], 50, iall, ["w1a"], 230))
        grp.append(Group("frontb", fr[1], 50, iall, ["w1b"], 230, 2200))
        grp.append(Group("fq", fr[2], 34, ["w4c"], ["I4"], 100))
        grp.append(Group("spread", spread(), 30, iall, ["end"], 100))
        grp.append(Group("shift", shift_early(), 24, ["start"], ["w1a"], 200))
        _emit(seq, grp, zero, wait)
        out_b(s - 3).wait()
        out_a(s - 2).wait()
        return carry

    lax.fori_loop(NC, NB, step, 0)

    seq, grp = [], []
    w47 = mm4("w4_7", NB - 1, 1, 2, 0, 1, 2)
    seq += _flat(mm4("w4_5", NB - 3, 0)[2] + mm2("w2_7", 0, 0, 1, True) + mm3("w3_6", 0, 2)
                 + cat(mm4("w4_6", NB - 2, 0, 1, 1, 0, 2)) + mm3("w3_7", 1, 2) + w47[0][:3] + w47[1] + w47[0][3:])
    grp.append(Group("shift7", shift(2, 0, [(r, 32) for r in range(0, T, 32)], gs), 24, ["start"], ["w2_7"], 200))
    grp.append(Group("ln2_6", ln2(0, 0), 75, ["start"], ["w2_7"], 0))
    grp.append(Group("xn6", cat(lsums2(3, n2_w, as_w[2], 0)), 26, ["w4_5"], ["w3_6_0"], 200, 600))
    grp.append(Group("ws4b", wsums2(4), 26, ["start"], ["w4_6q"], 250))
    grp.append(Group("ln2_7", ln2(1, 1), 75, ["w4_6"], ["w3_7"], 1200))
    grp.append(Group("xn7", cat(lsums2(3, n2_w, as_w[2], 1)), 26, ["w4_6"], ["w3_7_0"], 200, 2100))
    for j in (6, 7):
        for p, ts in enumerate(lsums2(4, a_w, as_w[3], j - 6)):
            grp.append(Group("xa%d_%d" % (j, p), ts, 26, ["w3_%d_%d" % (j, p)], ["w4_%dq" % j], 200, 150))
    _emit(seq, grp, zero, wait)
    for c in next_kv(NB - 1) + next_q(NB - 1) + [out_b(NB - 3)] + last:
        c.wait()


@jax.jit
def pallas_adaLN_cond__ssm_conv_h3__mixer_s_mlp__prompt_kernel(
        A_q, A_k, A_v, A_shift_k, A_ssm_k, A_ssm_D, B_x, B_w1, B_w2, B_w3, B_w4, c, w_mod):
    any_ = pl.BlockSpec(memory_space=pl.ANY)
    V = pltpu.VMEM
    out = pl.pallas_call(
        kernel,
        in_specs=[any_] * 12,
        out_specs=any_,
        out_shape=jax.ShapeDtypeStruct((S, D), BF16),
        scratch_shapes=[
            [V((NT, H + 8, 128), U32)] * NC, [V((NT, H + 8, 128), U32)] * NC, [V((NT, H + 8, 128), U32)] * NC,
            [V((64, S), U32)] * NT,
            V((D // 2, D), U32), V((D // 2, D), U32), V((F // 2, D), U32), V((FT * 64, D), U32),
            [V((D // 2, 3 * D), U32), V((D // 2, 2 * D), U32), V((D // 2, D), U32)], V((4 * T, D), BF16),
            V((4, D), BF16), V((D,), BF16), V((1, D), BF16), V((8, 128), I32), pltpu.SMEM((8, 128), I32),
            V((5, 8, D), F32), V((6, 8, D), F32), V((T // 2, 4 * H), U32), V((GR // 2, 2 * T), U32),
            V((NB, 3 * T + 8, D), F32), V((NC, 3 * T + 8, D), F32), V((NB - NC, 2 * T + 8, D), F32), V((2 * T, D), F32),
            V((T, D), U32), V((NC * T, D), U32), V((NT, NC * T + 8, 128), F32),
            V((3 * T, D), F32), V((3 * T, D), F32), V((2 * T, D), F32), V((T, D), F32),
            V((3 * T // 2, D), U32), V((T, D), U32), V((T, D), U32), V((NT, NC * T + 24, 128), F32),
            V((T, (FT + 1) * 128), U32),
            [V((128, 11 * 128), U32)] * 2 + [V((128, 31 * 128), U32), V((448, 11 * 128), U32)],
            [V((64, 11 * 128), U32)] * 2 + [V((128, 11 * 128), U32), V((128, 35 * 128), U32)],
            V((D // 2, 13 * 128), U32), V((H, D), F32), V((T, 7 * 128), F32),
            [V((64, 105 * 128), U32), V((192, 35 * 128), U32), V((32, 35 * 128), U32), V((32, 105 * 128), U32)],
            pltpu.SemaphoreType.DMA((11,)), pltpu.SemaphoreType.DMA((1,)), pltpu.SemaphoreType.DMA((3,)),
        ],
        compiler_params=pltpu.CompilerParams(vmem_limit_bytes=110 << 20, disable_semaphore_checks=True,
                                             disable_bounds_checks=True),
        name="fused",
    )(A_q[0], A_k[0], A_v[0], A_shift_k.T, A_ssm_k, A_ssm_D, B_w1, B_w2, B_w3.T, B_w4, c, w_mod)
    return out[None]
```

```python
import heapq
import os
import numpy as np
import jax
import jax.numpy as jnp
from jax import lax
from jax.experimental import pallas as pl
from jax.experimental.pallas import tpu as pltpu

S, D, F = 2048, 640, 1728
T = 256
H = T // 2
NB = S // T
NT = D // 128
FT = (F + 127) // 128
EPS = 1e-5
F32, BF16, U32, I32 = jnp.float32, jnp.bfloat16, jnp.uint32, jnp.int32
G_C1 = 0.044715 * float(np.sqrt(2.0 / np.pi))
G_C2 = float(np.sqrt(2.0 / np.pi))
G_A = G_C1 ** (1.0 / 3.0)
G_B = G_C2 / G_A
G_POST = 0.5 / G_A
RG = 16
GR = 80
NC = 3
DL = 450
E = lambda k, d: type(d)(os.environ.get(k, d))
SLOT = 32


def _dft(shape, f_axis, tau, scale=1.0):
    r = lax.broadcasted_iota(I32, shape, f_axis)
    l = lax.broadcasted_iota(I32, shape, 1 - f_axis)
    f = r & 127
    odd = ((f & 63) << 2) | ((f >> 6) << 1) | 1
    p = odd * tau(l) + ((r >> 7) << 8)
    a = ((p + 512) & 1023) - 512
    u = (256 - jnp.abs(a)).astype(F32) * (np.pi / 512.0)
    u2 = u * u
    c = [scale, -scale / 6.0, scale / 120.0, -scale / 5040.0, scale / 362880.0, -scale / 39916800.0]
    poly = c[5]
    for ci in c[4::-1]:
        poly = poly * u2 + ci
    return (u * poly).astype(BF16)


def _rstd(xc, mlp):
    s2, eps = (1.0 / (G_A * G_A), EPS / (G_POST * G_POST)) if mlp else (1.0, EPS)
    v = jnp.sum(xc * xc, axis=-1, keepdims=True) * (s2 / D) + eps * s2
    return jnp.exp2(jnp.log(v) * float(-0.5 / np.log(2.0)))


def _ln(x, mlp=False):
    xc = x - jnp.sum(x, axis=-1, keepdims=True) * (1.0 / D)
    return xc * _rstd(xc, mlp)


def _gelu2(x):
    u = x * (x * x + G_B)
    return x * (1.0 + jnp.tanh(u))


def _lo(w):
    return pltpu.bitcast(w << 16, F32)


def _hi(w):
    return pltpu.bitcast(w & jnp.uint32(0xFFFF0000), F32)


def _tie(x, a):
    if a is None:
        return x
    w = pltpu.bitcast(x[:, :128], U32)
    k = w.shape[0] // 8
    w = w | (a if k == 1 else jnp.concatenate([a] * k, axis=0))
    w = pltpu.bitcast(w, x.dtype)
    return w if x.shape[1] == 128 else jnp.concatenate([w, x[:, 128:]], axis=1)


def _top(x, i):
    return jnp.concatenate([x[r:r + 16] for r in range(16 * i, x.shape[0], 32)], axis=0)


def _zip(t, b):
    return jnp.concatenate([x[r:r + 16] for r in range(0, t.shape[0], 16) for x in (t, b)], axis=0)


def _lhs_sums(x1, x2):
    a11, a21, a12, a22 = _top(x1, 0), _top(x1, 1), _top(x2, 0), _top(x2, 1)
    return [a11 + a22, a21 + a22, a11 + a12, a21 - a11, a12 - a22]


def C(i):
    return slice(i * 128, (i + 1) * 128)


class Unit:
    def __init__(self, name, tiles, epi, rows, cost, nt=False, full=True, acc=False):
        self.acc, self.res = acc, []
        self.name, self.tiles, self.epi, self.rows, self.cost, self.nt, self.full = name, tiles, epi, rows, cost, nt, full


class Due:
    def __init__(self, val, delay):
        self.val, self.delay = val, delay


class Group:
    def __init__(self, name, fns, cost, rel, dead, lat, rlat=200):
        self.name, self.fns, self.cost, self.rel, self.dead, self.lat, self.rlat = name, fns, cost, rel, dead, lat, rlat


def _plan(seq, groups):
    busy, n = [0] * 4, 0
    start, end, tiles, bars = {}, {}, [], []
    for it in seq:
        if isinstance(it[0], Unit):
            u = it[0]
            m = n % 4
            n += 1
            t0, t1 = busy[m], busy[m] + max(u.rows, 32)
            busy[m] = t1
            tiles.append((t0, t1, u.cost / len(u.tiles)))
            start.setdefault(u.name, t0)
            end[u.name] = max(end.get(u.name, 0), t1)
        elif it[0] == "wait":
            t = max(busy)
            busy, n = [t] * 4, 0
            start[it[1]] = end[it[1]] = t
            bars.append(t)
    total = max(busy)
    start["end"] = end["end"] = total
    start["start"] = end["start"] = 0
    ns = total // SLOT + 2
    load = np.zeros(ns)
    for t0, t1, c in tiles:
        a, b = t0 // SLOT, max(t1 // SLOT, t0 // SLOT + 1)
        load[a:b] += c / (b - a)
    win = []
    for g in groups:
        r = max(end[x] + (0 if start[x] == end[x] else g.rlat) for x in g.rel)
        d = min(start[x] for x in g.dead) - g.lat
        ok = np.zeros(ns, bool)
        ok[r // SLOT:max(d // SLOT, r // SLOT + 1)] = True
        for b in bars:
            if r < b <= d:
                ok[max((b - g.lat) // SLOT, 0):b // SLOT] = False
        win.append(np.nonzero(ok)[0])
    alloc = [np.zeros(len(w)) for w in win]
    for _ in range(60):
        for i, g in enumerate(groups):
            w = win[i]
            load[w] -= alloc[i]
            base = load[w]
            vol = g.cost * len(g.fns)
            lo, hi = base.min(), base.max() + vol
            for _ in range(50):
                mid = 0.5 * (lo + hi)
                if np.maximum(mid - base, 0).sum() > vol:
                    hi = mid
                else:
                    lo = mid
            alloc[i] = np.maximum(hi - base, 0)
            load[w] += alloc[i]
    times = []
    for i, g in enumerate(groups):
        cum = np.cumsum(alloc[i])
        ts = []
        for k in range(len(g.fns)):
            x = (k + 0.5) * cum[-1] / len(g.fns)
            j = int(np.searchsorted(cum, x))
            prev = cum[j - 1] if j else 0.0
            ts.append(win[i][j] * SLOT + SLOT * (x - prev) / max(alloc[i][j], 1e-9))
        times.append(ts)
    return times


def _emit(seq, groups, zero, wait):
    times = _plan(seq, groups)
    left = {"start": 0}
    for it in seq:
        nm = it[0].name if isinstance(it[0], Unit) else it[1]
        left[nm] = left.get(nm, 0) + 1
    heap, pend, todo, cnt = [], {}, list(range(len(groups))), 0
    busy, n, due = [0] * 4, 0, []

    def release():
        nonlocal cnt
        for i in list(todo):
            g = groups[i]
            if all(left[x] == 0 for x in g.rel):
                todo.remove(i)
                pend[i] = len(g.fns)
                for t, fn in zip(times[i], g.fns):
                    heapq.heappush(heap, (t, cnt, i, fn))
                    cnt += 1

    def force(name):
        nonlocal heap
        for i, g in enumerate(groups):
            if name in g.dead:
                assert i not in todo, (g.name, name)
                if pend[i]:
                    for it in sorted(x for x in heap if x[2] == i):
                        it[3](None)
                    heap = [x for x in heap if x[2] != i]
                    heapq.heapify(heap)
                    pend[i] = 0

    release()
    for it in seq:
        if isinstance(it[0], Unit):
            u, k = it
            force(u.name)
            lhs, rhs = u.tiles[k]()
            t0 = busy[n % 4]
            while u.full and due and due[0][0] < t0 + u.rows:
                t, x = due.pop(0)
                r = min(max(int(t - t0), 0), u.rows - 1) // 16 * 8
                w = pltpu.bitcast(lhs, U32)
                x = pltpu.bitcast(x[:, :128], U32)
                parts = [w[:r], w[r:r + 8] | ((x[0:8] | x[8:16]) & zero), w[r + 8:]]
                lhs = pltpu.bitcast(jnp.concatenate([y for y in parts if y.shape[0]], axis=0), BF16)
            dn = (((1,), (1 if u.nt else 0,)), ((), ()))
            p = lax.dot_general(lhs, rhs, dn, preferred_element_type=F32)
            u.res = [p + u.res[0]] if (u.acc and u.res) else u.res + [p]
            m = n % 4
            n += 1
            t0 = busy[m]
            busy[m] = t0 + max(u.rows, 32)
            while u.full and heap and heap[0][0] < t0 + u.rows:
                t, _, i, fn = heapq.heappop(heap)
                pend[i] -= 1
                r = min(max(int(t - t0), 0), u.rows - 1) // 8 * 8
                x = fn(pltpu.bitcast(p[r:r + 8], U32) & zero)
                if isinstance(x, Due):
                    due.append((t + x.delay, x.val))
                    due.sort(key=lambda e: e[0])
            if k == len(u.tiles) - 1:
                u.epi(u.res)
            left[u.name] -= 1
        elif it[0] == "wait":
            force(it[1])
            wait(it[1])
            busy, n, due = [max(busy)] * 4, 0, []
            left[it[1]] -= 1
        else:
            it[2]()
            left[it[1]] -= 1
        release()
    force("end")
    assert not heap and not todo


def _sum(ps):
    acc = ps[0]
    for p in ps[1:]:
        acc = acc + p
    return acc


def _flat(us):
    return [(u, i) for u in us for i in range(len(u.tiles))]


def _weave(a, b):
    out = []
    for i, u in enumerate(a):
        out += [u] + b[i * len(b) // len(a):(i + 1) * len(b) // len(a)]
    return out


def _phase(seq):
    n = 0
    for it in seq:
        n = n + 1 if isinstance(it[0], Unit) else (0 if it[0] in ("wait", "sync") else n)
    return n % 4


def _mix(seq, a, b, lo=0.0, hi=1.0):
    n, k = _phase(seq), 0
    for i, t in enumerate(a):
        if k < len(b) and n % 4 == 0 and t[1] != 1 and i >= len(a) * (lo + (hi - lo) * k / len(b)):
            seq.extend(b[k])
            k += 1
        seq.append(t)
        n += 1
    assert k == len(b)


def _wait(seq, name, head=(), back=0):
    r = _phase(seq) + 4 * back
    assert all(isinstance(it[0], Unit) for it in seq[len(seq) - r:])
    seq[len(seq) - r:len(seq) - r] = [("wait", name)] + list(head)


def kernel(q_hbm, k_hbm, v_hbm, sh_hbm, ssm_hbm, sd_hbm, w1_hbm, w2_hbm, w3_hbm, w4_hbm, c_hbm, wm_hbm,
           o_hbm,
           q_n, k_n, v_n, ssm_w, w1_w, w2_w, w3_w, w4_w, wm_w, o_v,
           sh_v, sd_v, c_v, zsrc, z_s, taps, mod_v, tf_w, tg_w,
           kf, uf, acc, zraw, kv_w, zz_w, y_v, x_v, hb_v, x1_v, r_v, n1_w, n2_w, g_w, h1_v, a_w,
           ws_w, as_w, w3n_w, top_v, st_v, l2_w,
           sem, sem_b, sem_o):
    bf = lambda r: r.bitcast(BF16)
    w1_v, w2_v, w3_v, w4_v = bf(w1_w), bf(w2_w), bf(w3_w), bf(w4_w)
    wm_v = {0: bf(wm_w[0]), 3: bf(wm_w[1]), 5: bf(wm_w[2])}
    tf_v, tg_v, n1_v, n2_v, g_v = bf(tf_w), bf(tg_w), bf(n1_w), bf(n2_w), bf(g_w)
    a_v, kv_v, zz_v = bf(a_w), bf(kv_w), bf(zz_w)
    w1s, w2s, w3s, w4s = [bf(r) for r in ws_w]
    n1s, gs, n2s, a_s = [bf(r) for r in as_w]
    w3n = bf(w3n_w)
    w3t, w4t, n2t, a_t = [bf(r) for r in l2_w]
    cp = pltpu.make_async_copy
    cat = lambda ls: [x for l in ls for x in l]

    def base(j, n):
        return j * n if isinstance(j, int) else pl.multiple_of(j * n, n)

    def rows(j, n=1, size=T):
        return pl.ds(base(j, size), n * size)

    def view(ref, j, size=T):
        return ref.at[rows(j, 1, size)]

    dmas = {}

    def group(name, *mks):
        sm = sem.at[len(dmas)]
        dmas[name] = [c for mk in mks for c in mk(sm)]

    def ssm_in(t):
        return lambda sm: [cp(ssm_hbm.at[C(t)], bf(ssm_w[t]), sm)]

    def cols(src, start, n, dst, row=0):
        return lambda sm: [cp(src.at[pl.ds(start, n), C(t)], bf(dst).at[t, pl.ds(row, n)], sm) for t in range(NT)]

    def kv_in(s, sl):
        if isinstance(s, int):
            kk = cols(k_hbm, s * T - 16, T + 16, k_n[sl]) if s else cols(k_hbm, 0, T, k_n[sl], 16)
        else:
            kk = cols(k_hbm, pl.multiple_of(s * T - 16, 16), T + 16, k_n[sl])
        return lambda sm: kk(sm) + cols(v_hbm, base(s, T), T, v_n[sl])(sm)

    def q_in(s, sl):
        return cols(q_hbm, base(s, T), T, q_n[sl])

    def wm_in(a, b):
        return lambda sm: [cp(wm_hbm.at[:, a * D:b * D], wm_v[a], sm)]

    def whole(src, dst):
        return lambda sm: [cp(src, dst, sm)]

    next_kv = lambda s: kv_in(s, 0)(sem_b.at[0])
    next_q = lambda s: q_in(s, 0)(sem_b.at[0])

    zsrc[...] = jnp.zeros((8, 128), I32)
    k_n[0][:, 0:8, :] = jnp.zeros((NT, 8, 128), U32)
    w4_w[F // 2:FT * 64, :] = jnp.zeros((FT * 64 - F // 2, D), U32)
    group("small", lambda sm: [cp(zsrc, z_s, sm), cp(sh_hbm, sh_v, sm), cp(sd_hbm, sd_v, sm), cp(c_hbm, c_v, sm)])
    for s in range(NC):
        group("c%d" % s, ssm_in(s), kv_in(s, s))
    group("c3", ssm_in(3), ssm_in(4))
    group("wma", wm_in(0, 3), q_in(0, 0), q_in(1, 1))
    group("wmb", wm_in(3, 5))
    group("w1", whole(w1_hbm, w1_v))
    group("w2", q_in(2, 2), whole(w2_hbm, w2_v))
    group("w3", whole(w3_hbm, w3_v))
    group("w4", whole(w4_hbm, w4_v.at[0:F]), wm_in(5, 6))
    for g in dmas.values():
        for c in g:
            c.start()

    def wait(name):
        for c in dmas[name]:
            c.wait()

    tau_b = lambda l: H + ((l + (H - 1)) & (H - 1))
    tf_v[:, C(0)] = _dft((T, H), 0, lambda l: jnp.where((l & 1) == 0, l, tau_b(l)), 1.0 / T)
    tf_v[:, C(1)] = _dft((T, H), 0, lambda l: jnp.where((l & 1) == 1, l, tau_b(l)), 1.0 / T)
    tf_v[:, C(2)] = _dft((T, H), 0, lambda l: 2 * l - H)
    tf_v[:, C(3)] = _dft((T, H), 0, lambda l: 2 * l + 1 - H)
    sin0 = lax.broadcasted_iota(I32, (GR, T), 1) >= H
    tg_v[:, 0:T] = _dft((GR, T), 1, lambda l: jnp.where(sin0 & (l == 0), H, 2 * l))
    tg_v[:, T:2 * T] = _dft((GR, T), 1, lambda l: 2 * l + 1)
    h1_v[:, 0:8, :] = jnp.zeros((NT, 8, 128), F32)
    h1_v[:, 8 + NC * T:16 + NC * T, :] = jnp.zeros((NT, 8, 128), F32)

    wait("small")
    z = jnp.clip(z_s[0, 0], 0, 1)
    zero = jnp.full((8, 128), z, I32).astype(U32)
    z8 = pl.multiple_of(z * 8, 8)
    for r in (x_v, hb_v, x1_v, r_v, zraw, n1_w, n2_w, g_w, a_w, kv_w, zz_w, *ws_w, *as_w, w3n_w, top_v, st_v, *l2_w):
        r[pl.ds(z8, 8), 0:128] = jnp.zeros((8, 128), r.dtype)
    for r in (kf, uf, acc, taps, mod_v):
        r[z, 0:8, 0:128] = jnp.zeros((8, 128), r.dtype)
    for r in (tf_w, tg_w):
        r[pl.ds(z8, 8), 0:128] = r[0:8, 0:128]
    sh = sh_v[...].astype(F32)
    for i in range(4):
        taps[i] = jnp.broadcast_to(sh[i:i + 1], (8, D))
    taps[4] = jnp.broadcast_to(sd_v[...].astype(F32).reshape(1, D) * (1.0 / T), (8, D))
    cf = c_v[...].astype(F32)
    silu_c = jnp.broadcast_to((cf / (1.0 + jnp.exp(-cf))).astype(BF16), (16, D))

    def mmK(n):
        def unit(m):
            st = []

            def rhs(i):
                if not st:
                    ev = (lax.broadcasted_iota(I32, (64, 128), 1) & 1) == 0
                    a = ssm_w[n][:, m * T:m * T + H]
                    b = pltpu.roll(ssm_w[n][:, m * T + H:(m + 1) * T], 1, 1)
                    st.extend([pltpu.bitcast(jnp.where(ev, a, b), BF16), pltpu.bitcast(jnp.where(ev, b, a), BF16)])
                return st[i]

            def epi(p):
                er, ei, or_, oi = p
                cur = [er, ei, or_, oi]
                if m:
                    pv = [zraw[C(4 * ((m - 1) % 2) + (q ^ 1)), :] for q in range(4)]
                    pm = lambda x, y, up: jnp.concatenate([x[:64] + y[:64], x[64:] - y[64:]] if up else
                                                          [x[:64] - y[:64], x[64:] + y[64:]], axis=0)
                    er, ei, or_, oi = [pm(cur[q], pv[q], q & 1) for q in range(4)]
                else:
                    er = er + taps[4, 0:1, C(n)]
                if m + 1 < NB:
                    for q in range(4):
                        zraw[C(4 * (m % 2) + q), :] = cur[q]
                for h, (cr, ci) in enumerate(((er + or_, ei + oi), (er - or_, ei - oi))):
                    B = h * 3 * H
                    kf[m, B:B + H, C(n)] = cr
                    kf[m, B + H:B + 2 * H, C(n)] = ci - cr
                    kf[m, B + 2 * H:B + 3 * H, C(n)] = ci + cr
            return Unit("K%d" % n, [(lambda i=i, r=r: (tf_v[r:r + H, C(i)], rhs(i))) for i in range(2) for r in (0, H)],
                        epi, H, 260, nt=True)
        return [unit(m) for m in range(NB)]

    def kv(s, sl):
        def mk(t, w):
            def fn(a):
                ld = lambda o, n: k_n[s][t, pl.ds(8 + w + o, n), :]
                c0 = jnp.concatenate([_tie(ld(0, 8), a), ld(8, 8)], axis=0).reshape(2, 8, 128)
                c1, c2 = ld(-1, 16).reshape(2, 8, 128), ld(-2, 16).reshape(2, 8, 128)
                s0, s1, s2, s3 = (taps[i, :, C(t)] for i in range(4))
                ke, ko, ke1, ko1, ko2 = _lo(c0), _hi(c0), _lo(c1), _hi(c1), _hi(c2)
                wv = v_n[s][t, w:w + 16, :].reshape(2, 8, 128)
                kve = ((s0 * ke + s1 * ko1) + (s2 * ke1 + s3 * ko2)) * _lo(wv)
                kvo = ((s0 * ko + s1 * ke) + (s2 * ko1 + s3 * ke1)) * _hi(wv)
                kv_v[pl.ds(sl * T + w, 16), C(t)] = kve.reshape(16, 128).astype(BF16)
                kv_v[pl.ds(sl * T + H + w, 16), C(t)] = kvo.reshape(16, 128).astype(BF16)
            return fn
        return [[mk(t, w) for w in range(0, H, 16)] for t in range(NT)]

    def mmU(name, sl, us):
        def unit(n):
            def epi(p):
                er, ei, or_, oi = p
                for h, (cr, ci) in enumerate(((er + or_, ei + oi), (er - or_, ei - oi))):
                    B = h * 3 * H
                    uf[us, B:B + H, C(n)] = cr + ci
                    uf[us, B + H:B + 2 * H, C(n)] = cr
                    uf[us, B + 2 * H:B + 3 * H, C(n)] = ci
            return Unit(name(n), [(lambda i=i, r=r: (tf_v[r:r + H, C(2 + i)], kv_v[pl.ds(sl * T + i * H, H), C(n)]))
                                  for i in range(2) for r in (0, H)], epi, H, 120)
        return [unit(n) for n in range(NT)]

    def cmul(m0, u0, n, h, row, L, a):
        t = []
        for i in range(3):
            Rw = slice((3 * h + i) * H + row, (3 * h + i) * H + row + 8)
            kk = kf[m0:m0 + n, Rw, L]
            if i == 0 and a is not None:
                k0 = _tie(kk[0], a)[None]
                kk = k0 if n == 1 else jnp.concatenate([k0, kk[1:]], axis=0)
            t.append(jnp.sum(kk * uf[u0:u0 + n, Rw, L], axis=0))
        return t[0] - t[2], t[0] + t[1]

    def AR(h, q, row):
        return slice((2 * h + q) * H + row, (2 * h + q) * H + row + 8)

    def mac(n, u0, sl, part=False):
        def mk(t, rc):
            st, fin = [], []

            def piece(i):
                def fn(a):
                    h, row = i & 1, rc + (i >> 1) * 8
                    zr, zi = cmul(0, u0, n, h, row, C(t), a)
                    if part:
                        zr, zi = zr + acc[0, AR(h, 0, row), C(t)], zi + acc[0, AR(h, 1, row), C(t)]
                    st.append((zr, zi))
                    if h:
                        (pr, pi), (mr, mi) = st[-2:]
                        fin.append([pr + mr, pi + mi, pr - mr, pi - mi])
                    if i == 3:
                        for q in range(4):
                            zz_v[pl.ds(sl * 2 * T + q * H + rc, 16), C(t)] = jnp.concatenate(
                                [fin[0][q], fin[1][q]], axis=0).astype(BF16)
                return fn
            if not part:
                return [piece(i) for i in range(4)]
            both = lambda f, g: (lambda a: (f(a), g(None)))
            return [both(piece(0), piece(1)), both(piece(2), piece(3))]
        return [[fn for rc in range(0, H, 16) for fn in mk(t, rc)] for t in range(NT)]

    def pos():
        return [(t, h, row) for t in range(NT) for row in range(0, H, 8) for h in range(2)]

    def ahead(i):
        def mk(t, h, row):
            def fn(a):
                zr, zi = cmul(i + 1, 0, NC, h, row, C(t), a)
                acc[i, AR(h, 0, row), C(t)] = zr
                acc[i, AR(h, 1, row), C(t)] = zi
            return fn
        return [mk(*p) for p in pos()]

    def spread():
        n = NB - NC - 1

        def mk(t, h, row):
            def fn(a):
                p = []
                for i in range(3):
                    Rw = slice((3 * h + i) * H + row, (3 * h + i) * H + row + 8)
                    u = uf[0, Rw, C(t)]
                    p.append(kf[1:1 + n, Rw, C(t)] * (_tie(u, a) if i == 0 else u)[None])
                acc[0:n, AR(h, 0, row), C(t)] = acc[1:1 + n, AR(h, 0, row), C(t)] + (p[0] - p[2])
                acc[0:n, AR(h, 1, row), C(t)] = acc[1:1 + n, AR(h, 1, row), C(t)] + (p[0] + p[1])
            return fn
        return [mk(*p) for p in pos()]

    def mmI(name, sl, ys):
        def unit(n):
            def epi(p):
                ce, se, co, so = p
                sub = lax.broadcasted_iota(I32, (8, 128), 0)
                b0 = ys * (T + 8) + 8
                y_v[n, b0 + H - 1:b0 + H, :] = (ce[64:72] - se[0:8])[0:1]
                se = jnp.concatenate([jnp.where(sub == 0, 0.0, se[0:8]), se[8:]], axis=0)
                for d, cc, ss in ((0, ce[0:64], se), (1, co, so)):
                    y_v[n, pl.ds(b0 + H + d, 64, stride=2), :] = cc + ss
                    y_v[n, pl.ds(b0 + d - 1, 64, stride=2), :] = cc - ss
            return Unit(name(n), [(lambda i=i: (tg_v[0:(GR if i == 0 else 64), C(i)], zz_v[pl.ds(sl * 2 * T + i * H, H), C(n)]))
                                  for i in range(4)], epi, 64, 36)
        return [unit(n) for n in range(NT)]

    def mod(name, a, b):
        def unit(n):
            def epi(p):
                v = [_sum(p[i * NT:(i + 1) * NT])[0:8] for i in range(b - a)]
                if a == 0:
                    mod_v[0, :, C(n)] = v[0] * v[2]
                    mod_v[1, :, C(n)] = (v[1] + 1.0) * v[2]
                elif a == 3:
                    mod_v[3, :, C(n)] = v[0] * (1.0 / G_POST)
                    mod_v[4, :, C(n)] = (v[1] + 1.0) * (1.0 / G_POST)
                else:
                    mod_v[2, :, C(n)] = v[0] * G_POST
            return Unit(name, [(lambda i=i, k=k: (silu_c[:, C(k)], wm_v[a][C(k), pl.ds(i * D + n * 128, 128)]))
                               for i in range(b - a) for k in range(NT)], epi, 16, 10, full=False, acc=b - a == 1)
        return [unit(n) for n in range(NT)]

    HS = (slice(0, 128), slice(128, 256))
    QS = tuple(slice(r, r + 64) for r in range(0, T, 64))

    def tasks(f, due=None, tie=True, n=RG):
        def mk(R):
            def fn(a):
                x = f(R, a if tie else None)
                return Due(x, due) if due else None
            return fn
        return [mk(slice(r, r + n)) for r in range(0, T, n)]

    def load_y(sl, R):
        b0, back = sl * (T + 8) + 8, 7 - lax.broadcasted_iota(I32, (8, 128), 0)

        def ld(t, r):
            if r >= H:
                return y_v[t, b0 + r:b0 + r + 8, :]
            return jnp.take_along_axis(y_v[t, b0 + H - 8 - r:b0 + H - r, :], back, axis=0)
        return jnp.stack([jnp.concatenate([ld(t, r) for t in range(NT)], axis=1) for r in (R.start, R.start + 8)])

    def put(nn, ss, R, x):
        nn[R, :] = x.astype(BF16)
        tok = x
        if ss is not None:
            S2 = pl.ds(R.start // 32 * 16, 16)
            if R.stop % 32:
                top_v[S2, 0:2 * T] = x[:, 0:2 * T]
            else:
                if R.start % 32:
                    x = jnp.concatenate([top_v[S2, 0:2 * T], x[:, 0:2 * T]], axis=0)
                ss[S2, 0:5 * T] = jnp.concatenate(_lhs_sums(x[:, 0:T], x[:, T:2 * T]), axis=1).astype(BF16)
        return tok

    wide = lambda v: jnp.concatenate([v] * NT, axis=1)

    def mean(i, R, x):
        st_v[R, C(i)] = jnp.broadcast_to(jnp.sum(x, axis=-1, keepdims=True) * (1.0 / D), (x.shape[0], 128))

    def centred(src, i, R, a):
        return src[R, :] - wide(_tie(st_v[R, C(i)], a))

    def scale(src, i, g):
        def f(R, a):
            st_v[R, C(i + 1)] = jnp.broadcast_to(_rstd(centred(src, i, R, a), g), (RG, 128))
        return f

    def normed(src, i, R, a):
        return centred(src, i, R, a) * wide(st_v[R, C(i + 1)])

    def front(sl, xs, early=False, ss=None):
        xx, hh, nn = view(x_v, xs), view(hb_v, xs), view(n1_v, sl)

        def fa(R, a):
            q = [q_n[sl][t, R.start // 2:R.stop // 2, :] for t in range(NT)]
            q = jnp.concatenate([_tie(q[0], a)] + q[1:], axis=1)
            q = pltpu.bitcast(q, BF16).astype(F32).reshape(2, 8, D)
            x = (q + (_ln(q) * mod_v[1] + mod_v[0]) * load_y(sl, R)).reshape(RG, D)
            xx[R, :] = x
            if early:
                hh[R, :] = _ln(x)

        def fb(R, a):
            hh[R, :] = (_ln(_tie(xx[R, :], a).reshape(2, 8, D)) * mod_v[4] + mod_v[3]).reshape(RG, D)

        def fc(R, a):
            hb = _tie(hh[R, :], a)
            if early:
                hb = (hb.reshape(2, 8, D) * mod_v[4] + mod_v[3]).reshape(RG, D)
                hh[R, :] = hb
            nn[R, :] = _ln(hb, True).astype(BF16)
        if early:
            return tasks(fa), tasks(fc)
        if ss is None:
            return tasks(fa) + tasks(fb) + tasks(fc)
        qf = view(x_v, 2)

        def s1(R, a):
            q = [q_n[sl][t, R.start // 2:R.stop // 2, :] for t in range(NT)]
            q = pltpu.bitcast(jnp.concatenate([_tie(v, a) for v in q], axis=1), BF16).astype(F32)
            qf[R, :] = q
            mean(0, R, q)

        def s3(R, a):
            h = normed(qf, 0, R, a).reshape(2, 8, D) * mod_v[1] + mod_v[0]
            x = qf[R, :] + (h * load_y(sl, R)).reshape(RG, D)
            xx[R, :] = x
            mean(2, R, x)

        def s5(R, a):
            hb = (normed(xx, 2, R, a).reshape(2, 8, D) * mod_v[4] + mod_v[3]).reshape(RG, D)
            hh[R, :] = hb
            mean(4, R, hb)
        s7 = [f for g in tasks(lambda R, a: put(nn, ss, R, normed(hh, 4, R, a)), n=32) for f in (g, lambda a: None)]
        st = [tasks(s3), tasks(scale(xx, 2, False)), tasks(s5), tasks(scale(hh, 4, True)), s7]
        p = [tasks(s1), tasks(scale(qf, 0, False))]
        return cat(x[:8] for x in st), cat(x[8:] for x in p + st), cat(x[:8] for x in p)

    def shift(hs, sl, pieces=((0, 64), (64, 64), (128, 64), (192, 64)), ss=None):
        gg = view(g_v, sl)

        def one_tile(t, r, n, a):
            lane = lax.broadcasted_iota(I32, (n, 128), 1)
            ld = lambda d: h1_v[t, pl.ds(hs * T + 8 + r + d, n), :]
            if t == 0:
                g = ld(-1)
            elif t == 1:
                g = jnp.where(lane < 32, ld(-1), ld(1))
            elif t == 2:
                g = jnp.where(lane < 64, ld(1), ld(-2))
            elif t == 3:
                g = jnp.where(lane < 96, ld(-2), ld(2))
            else:
                g = ld(2)
            if a is not None:
                g = jnp.concatenate([_tie(g[i:i + 8], a) if i % 16 == 0 else g[i:i + 8]
                                     for i in range(0, n, 8)], axis=0)
            gg[r:r + n, C(t)] = g.astype(BF16)
            return g

        def mk(ts, r, n):
            def fn(a):
                g = [one_tile(t, r, n, a) for t in ts]
                if len(ts) == 2:
                    for i, x in enumerate(_lhs_sums(*g)):
                        ss[r // 2:(r + n) // 2, C(2 * i + ts[0])] = x.astype(BF16)
            return fn
        sets = [(t,) for t in range(NT)] if ss is None else [(0, 2), (1, 3), (4,)]
        return [mk(ts, r, n) for ts in sets for r, n in pieces]

    def shift_early():
        def keep(a):
            h1_v[:, 2 * T - 32:2 * T + 8, :] = h1_v[:, 3 * T - 32:3 * T + 8, :]
        return shift(2, 0, [(r, 32) for r in range(0, T - 32, 32)], gs) + [keep]

    def ln2(xs, sl, fast=True):
        xx, nn, ss = view(x1_v, xs), view(n2_v, sl), view(n2s, sl, H) if fast else None
        f = lambda R, a: put(nn, ss, R, _ln(_tie(xx[R, :], a), True))
        ts = tasks(f, 900) if sl else tasks(f, DL, False)
        return ts[0::2] + ts[1::2] if fast else tasks(f)

    def resid(xs, x1s, rotate=False):
        xx, x1 = view(x_v, xs), view(x1_v, x1s)

        def f(R, a):
            gb = mod_v[2] if a is None else pltpu.bitcast(
                pltpu.bitcast(mod_v[2], U32) | jnp.concatenate([a] * NT, axis=1), F32)
            r_v[R, :] = xx[R, :] + (x1[R, :].reshape(2, 8, D) * gb).reshape(RG, D)
            if rotate:
                xx[R, :] = x_v[R, :]
                view(hb_v, 1)[R, :] = hb_v[R, :]
        return tasks(f)

    KD, KF, ND = [(0, 2), (1, 3)], [(2 * i, 2 * i + 1) for i in range(7)], [(1, 2), (3, 4)]
    Wt = {1: (lambda k, n: w1_v[C(k), C(n)], lambda i, kp, j: w1s[C(kp), C(2 * i + j)], False, KD, [4]),
          2: (lambda k, n: w2_v[C(k), C(n)], lambda i, kp, j: w2s[C(kp), C(2 * i + j)], False, KD, [4]),
          0: (lambda k, n: w3_v[C(n), C(k)], None, True, KD, [4]),
          3: (lambda k, n: w3n[C(k), C(n)], lambda i, kp, j: w3s[C(kp), C(6 * i + j)], False, KD, [4]),
          4: (lambda k, n: w4_v[C(k), C(n)], lambda i, kp, j: w4s[C(kp), C(2 * i + j)], False, KF, [])}

    def sums_task(load, store, left):
        def fn(a):
            b = [[load(u, v) for v in range(2)] for u in range(2)]
            b[0][0], b[1][1] = _tie(b[0][0], a), _tie(b[1][1], a)
            (x11, x12), (x21, x22) = [[pltpu.bitcast(x, BF16).astype(F32) for x in row] for row in b]
            r = ((x11 + x22, x21 + x22, x11 + x12, x21 - x11, x12 - x22) if left else
                 (x11 + x22, x12 - x22, x21 - x11, x11 + x12, x21 + x22))
            for m, x in enumerate(r):
                store(m, x.astype(BF16))
        return fn

    def wsums(w_w, ws, rp, cp_):
        def mk(i, j, r):
            def store(m, x):
                ws[pl.ds(128 * i + r, 16), C(len(cp_) * m + j)] = x
            return sums_task(lambda u, v: w_w[pl.ds(64 * rp[i][u] + r // 2, 8), C(cp_[j][v])], store, False)
        return [mk(i, j, r) for j in range(len(cp_)) for i in range(len(rp)) for r in range(0, 128, 16)]

    def w3_turn():
        def mk(n, k):
            def fn(a):
                x = jnp.concatenate([_tie(w3_w[64 * n:64 * n + 8, C(k)], a), w3_w[64 * n + 8:64 * n + 64, C(k)]], axis=0)
                w3n[C(k), C(n)] = pltpu.bitcast(x, BF16).T
            return fn
        return [mk(n, k) for n in range(FT - 1) for k in range(NT)]

    def plain(name, w, lhs, n, R, epi, cost):
        tile, _, nt, kp, kl = Wt[w]
        ks = sorted([k for p in kp for k in p] + kl)
        rows_ = R.stop - R.start
        return Unit(name, [(lambda k=k: (lhs[R, C(k)], tile(k, n))) for k in ks], lambda p: epi(n, R, p[0]),
                    rows_, rows_ // 8 * (len(ks) - 1 + cost), nt=nt, acc=True)

    def quad(name, w, lhs, sums, j, cols_, R, epi, cost):
        tile, wsum, nt, kp, kl = Wt[w] if isinstance(w, int) else w
        h, S2, c = len(kp), slice(R.start // 2, R.stop // 2), {}
        a_ = lambda i, k: _top(lhs(k) if callable(lhs) else lhs[R, C(k)], i)
        s_ = sums if callable(sums) else (lambda i, p: sums[S2, C(h * i + p)])
        prod = lambda fa_, fb_: [(lambda p=p: (fa_(p), fb_(p))) for p in range(h)]
        left = lambda i, n: [(lambda k=k: (a_(i, k), tile(k, n))) for k in kl]
        mk = lambda tiles, f, x=0: Unit(name, tiles, lambda p: f(p[0]), 64, 8 * len(tiles) + x, nt=nt, acc=True)

        def e1(m):
            u7.res, u6.res = [m], [m]

        def e4(m):
            c[11], c[21] = c[11] + m, m

        def e2(m):
            c[21], c[22] = c[21] + m, c[22] - m
            l21.res = [c[21]]

        def e5(m):
            c[12] = m
            epi(cols_[0], R, _zip(c[11] - m, c[21]))

        def e3(m):
            l12.res, c[22] = [c[12] + m], c[22] + m
            if not kl:
                l12.epi(l12.res)
        u1 = mk(prod(lambda p: s_(0, p), lambda p: wsum(0, p, j)), e1)
        u7 = mk(prod(lambda p: s_(4, p), lambda p: wsum(4, p, j)) + left(0, cols_[0]), lambda m: c.update({11: m}))
        u6 = mk(prod(lambda p: s_(3, p), lambda p: wsum(3, p, j)) + left(1, cols_[1]), lambda m: c.update({22: m}))
        u4 = mk(prod(lambda p: a_(1, kp[p][1]), lambda p: wsum(2, p, j)), e4)
        u2 = mk(prod(lambda p: s_(1, p), lambda p: tile(kp[p][0], cols_[0])), e2, 8)
        l21 = mk(left(1, cols_[0]), lambda m: c.update({21: m}))
        u5 = mk(prod(lambda p: s_(2, p), lambda p: tile(kp[p][1], cols_[1])), e5, 16 * cost)
        u3 = mk(prod(lambda p: a_(0, kp[p][0]), lambda p: wsum(1, p, j)), e3, 8 if kl else 8 + 16 * cost)
        l12 = mk(left(0, cols_[1]), lambda m: epi(cols_[1], R, _zip(m, c[22])), 16 * cost)
        return [u1, u7, u6, u4, u2, l21, u5, u3, l12]

    LH, RH = [0, 4, 3, (1, 1), 1, 2, (0, 0)], [0, 4, 3, 2, (0, 0), (1, 1), 1]
    L2 = {3: (w3n_w, ws_w[2], w3t, KF[:6], n2t), 4: (w4_w, ws_w[3], w4t, ND, a_t)}

    def wsums2(w):
        w_w, s_w, ws2, cp_, _ = L2[w]
        kp, nj = Wt[w][3], len(cp_)

        def mk(o, p2, j2, r):
            def load(u, v):
                p, j, y = 2 * p2 + u, 2 * j2 + v, RH[o]
                if isinstance(y, int):
                    return s_w[pl.ds(64 * p + r // 2, 8), C(nj * y + j)]
                return w_w[pl.ds(64 * kp[p][y[0]] + r // 2, 8), C(cp_[j][y[1]])]

            def store(m, x):
                ws2[pl.ds(128 * p2 + r, 16), C((5 * o + m) * (nj // 2) + j2)] = x
            return sums_task(load, store, False)
        return [mk(o, p2, j2, r) for j2 in range(nj // 2) for o in range(7) for p2 in range(len(kp) // 2)
                for r in range(0, 128, 16)]

    def wsums4():
        form = [((0, 0), (1, 1), 1), ((0, 1), (1, 1), -1), ((1, 0), (0, 0), -1), ((0, 0), (0, 1), 1), ((1, 0), (1, 1), 1)]

        def mk(o, p2, r):
            def fn(a):
                def blk(p, j, uv, t):
                    x = w4_w[pl.ds(64 * KF[p][uv[0]] + r // 2, 8), C(ND[j][uv[1]])]
                    return pltpu.bitcast(_tie(x, t), BF16).astype(F32)
                y = {}
                for u in range(2):
                    for j in range(2):
                        p = 2 * p2 + u
                        if isinstance(RH[o], int):
                            f = form[RH[o]]
                            x1, x2 = blk(p, j, f[0], a), blk(p, j, f[1], None)
                            y[u, j] = x1 + x2 if f[2] > 0 else x1 - x2
                            w4s[pl.ds(128 * p + r, 16), C(2 * RH[o] + j)] = y[u, j].astype(BF16)
                        else:
                            y[u, j] = blk(p, j, RH[o], a if u == j else None)
                for m, f in enumerate(form):
                    x = y[f[0]] + y[f[1]] if f[2] > 0 else y[f[0]] - y[f[1]]
                    w4t[pl.ds(128 * p2 + r, 16), C(5 * o + m)] = x.astype(BF16)
            return fn
        last = wsums(w4_w, w4s, KF, ND)
        return (last[48:56] + last[104:112]
                + [mk(o, p2, r) for o in range(7) for p2 in range(3) for r in range(0, 128, 16)])

    def lsums2(w, lhs_w, sums_w, sl):
        kp, xs2 = Wt[w][3], L2[w][4]
        h2 = len(kp) // 2

        def mk(o, p2, g):
            def load(u, v):
                p, ch, x = 2 * p2 + v, 2 * g + u, LH[o]
                if isinstance(x, int):
                    return sums_w[pl.ds(64 * sl + 8 * ch, 8), C(len(kp) * x + p)]
                return lhs_w[pl.ds(H * sl + 16 * ch + 8 * x[0], 8), C(kp[p][x[1]])]

            def store(m, x):
                xs2[pl.ds(16 * g, 16), C((5 * o + m) * h2 + p2)] = x
            return sums_task(load, store, True)
        return [[mk(o, p2, g) for o in range(7) for g in range(4)] for p2 in range(h2)]

    def quad2(name, w, lhs, sums, j2, epi, cost):
        tile, wsum, nt, kp, kl = Wt[w]
        ws2, cp_, xs2 = L2[w][2:]
        h, h2, nj2, c, R = len(kp), len(kp) // 2, len(cp_) // 2, {}, slice(0, T)

        def done(j, v):
            val = _zip(c[j, 1, v], c[j, 2, v])
            if not kl:
                return epi(cp_[j][v], R, val)
            c[j, v] = val

        def upd(o, j, m):
            for i, v, sg in (((1, 0, 1), (2, 1, 1)), ((1, 0, 1),), ((2, 1, 1),), ((1, 0, 1), (2, 0, 1)),
                             ((2, 0, 1), (2, 1, -1)), ((1, 0, -1), (1, 1, 1)), ((1, 1, 1), (2, 1, 1)))[o]:
                k = (j, i, v)
                c[k] = m if k not in c else (c[k] + m if sg > 0 else c[k] - m)
            if o >= 5:
                done(j, o - 5)

        def inner(o):
            x, y = LH[o], RH[o]
            xo = ((lambda p: sums[:, C(h * x + p)]) if isinstance(x, int)
                  else (lambda p: _top(lhs[:, C(kp[p][x[1]])], x[0])))
            yo = ((lambda p, j: wsum(y, p, j)) if isinstance(y, int)
                  else (lambda p, j: tile(kp[p][y[0]], cp_[j][y[1]])))
            w_ = (yo, lambda m, p2, _: ws2[C(p2), C((5 * o + m) * nj2 + j2)], nt,
                  [(2 * i, 2 * i + 1) for i in range(h2)], list(range(2 * h2, h)))
            return quad(name, w_, xo, lambda m, p2: xs2[:, C((5 * o + m) * h2 + p2)], 0, (2 * j2, 2 * j2 + 1),
                        HS[0], lambda j, _, m: upd(o, j, m), 2 + (2 * cost if o >= 5 and not kl else 0))

        def rest(j, v, Q):
            return [Unit(name, [lambda: (lhs[Q, C(k)], tile(k, cp_[j][v]))],
                         lambda p: epi(cp_[j][v], Q, p[0] + c[j, v][Q]), 64, 8 * (cost + 1)) for k in kl]
        return cat(inner(o) for o in range(7)), [u for Q in QS for j in (2 * j2, 2 * j2 + 1) for v in range(2)
                                                 for u in rest(j, v, Q)]

    def mm(name, w, lhs, sums, epi, cost):
        if sums is None:
            return [[plain(name, w, lhs, n, R, epi, cost) for R in HS] for n in range(NT)]
        return [[plain(name, w, lhs, 0, R, epi, cost) for R in QS]] + [
            [u for R in HS for u in quad(name, w, lhs, sums, j, ND[j], R, epi, cost)] for j in range(2)]

    def mm1(name, hs, sl, fast=False):
        def epi(n, R, p):
            h1_v[n, pl.ds(hs * T + 8 + R.start, R.stop - R.start), :] = _gelu2(p)
        return cat(mm(name, 1, view(n1_v, sl), n1s if fast else None, epi, 5))

    def mm2(name, sl, xs, x1s, fast=False):
        def epi(n, R, p):
            view(x1_v, x1s)[R, C(n)] = view(hb_v, xs)[R, C(n)] + p
        return cat(mm(name, 2, view(g_v, sl), gs if fast else None, epi, 1))

    def mm3(name, sl, fast=True, deep=False):
        nn, aa, ss, keep, tail = view(n2_v, sl), view(a_v, sl), view(a_s, sl, H), {}, []

        def epi(n, R, p):
            g = _gelu2(p)
            aa[R, C(n)] = g.astype(BF16)
            if n % 2 == 0 and n < 12:
                keep[n] = g
                return
            pair = (keep.pop(n - 1), g) if n % 2 else (g, tail[R.start // 128][R.start % 128:R.start % 128 + 64])
            sm = _lhs_sums(*pair)
            for i, x in enumerate(sm):
                ss[R.start // 2:R.stop // 2, C(7 * i + n // 2)] = x.astype(BF16)
            if deep and n < 12:
                xo = [sm[x] if isinstance(x, int) else _top(pair[x[1]], x[0]) for x in LH]
                if n % 4 == 1:
                    keep[n, R.start] = xo
                    return
                for o, x in enumerate(zip(keep.pop((n - 2, R.start)), xo)):
                    for m, y in enumerate(_lhs_sums(*x)):
                        a_t[R.start // 4:R.stop // 4, C((5 * o + m) * 3 + n // 4)] = y.astype(BF16)

        def rem(R):
            def f(p):
                tail.append(jnp.concatenate([_gelu2(p[0]), jnp.zeros((64, 128), F32)], axis=0).T)
                aa[R, C(13)] = tail[-1].astype(BF16)
            return Unit(name, [(lambda k=k: (w3_v[13 * 128:F, C(k)], nn[R, C(k)])) for k in range(NT)], f, 64, 84,
                        nt=True, acc=True)
        odd = [rem(R) for R in HS] + [plain(name, 3 if fast else 0, nn, 12, R, epi, 9) for R in QS]
        if fast == 2:
            qd = [quad2(name + "_%d" % j, 3, nn, view(n2s, sl, H), j, epi, 8) for j in range(3)]
            return odd[:2] + qd[0][0] + _weave(qd[1][0], qd[0][1]) + _weave(qd[2][0], qd[1][1]) + _weave(odd[2:], qd[2][1])
        if fast:
            qd = [[u for j in range(6) for u in quad(name + ("b%d" % (j // 2) if i else "a"), 3, nn, view(n2s, sl, H), j,
                                                     KF[j], R, epi, 8)] for i, R in enumerate(HS)]
            return qd[0] + qd[1][:36] + odd[:2] + qd[1][36:] + odd[2:]
        return odd + [plain(name, 0, nn, n, R, epi, 8) for p in KF[:6] for R in HS for n in p]

    def cp_out(j, osl, L, sm, R=slice(0, T)):
        return cp(o_v.at[pl.ds(osl * T + R.start, R.stop - R.start), L],
                  o_hbm.at[pl.ds(base(j, T) + R.start, R.stop - R.start), L], sem_o.at[sm])

    out_a = lambda j: cp_out(j, 0, slice(128, D), 0)
    out_b = lambda j: cp_out(j, 0, C(0), 1)
    last = []

    def mm4(name, j, sl, osl=0, xs=None, x1s=None, fast=True):
        oo = view(o_v, osl)

        def epi(n, R, p):
            if xs is None:
                oo[R, C(n)] = (r_v[R, C(n)] + mod_v[2, 0:1, C(n)] * p).astype(BF16)
            else:
                oo[R, C(n)] = (view(x_v, xs)[R, C(n)] + mod_v[2, 0:1, C(n)]
                               * (view(x1_v, x1s)[R, C(n)] + p)).astype(BF16)
            if osl == 2:
                last.append(cp_out(j, osl, C(n), 2, R))
                last[-1].start()
            elif R.stop == T and osl and n == NT - 1:
                last.append(cp_out(j, osl, slice(128 if osl == 3 else 0, D), 2))
                last[-1].start()
            elif R.stop == T and osl == 0 and n in (0, NT - 1):
                (out_a if n else out_b)(j).start()
        if fast == 2:
            return ([plain(name, 4, view(a_v, sl), 0, R, epi, 3 if xs is None else 5) for R in QS],
                    quad2(name + "q", 4, view(a_v, sl), view(a_s, sl, H), 0, epi, 3 if xs is None else 5)[0])
        return mm(name, 4, view(a_v, sl), view(a_s, sl, H) if fast else None, epi, 3 if xs is None else 5)

    def split(us):
        n = 4 // len(us)
        m, mks, st = us[0].rows // n, [u.tiles.pop(0) for u in us], {}

        def piece(i, k):
            if i not in st:
                st[i] = mks[i]()
            return st[i][0][m * k:m * (k + 1)], st[i][1]

        def epi(p):
            for i, u in enumerate(us):
                u.res = [jnp.concatenate(p[n * i:n * (i + 1)], axis=0)]
        return _flat([Unit(us[0].name, [(lambda i=i, k=k: piece(i, k)) for i in range(len(us)) for k in range(n)],
                           epi, m, 0, nt=us[0].nt)])

    W = lambda nm: [("wait", nm)]
    run = lambda fns: [("run", "run", lambda: [fn(None) for fn in fns])]
    one = lambda us: [_flat([u]) for u in us]
    nm = lambda x: (lambda n: x)

    seq, grp = [], []
    for s in range(NC):
        seq += W("c%d" % s) + _flat(mmK(s) + mmU(nm("U%d" % s), s % 2, NC - 1 - s))
        grp.append(Group("kv%d" % s, cat(kv(s, s % 2)), 50, ["c%d" % s], ["U%d" % s], 100))
    inv = [mmI(lambda n: "I%d" % n, s, s) for s in range(NC)]
    seq += W("c3") + _flat(mmK(3) + mmK(4) + [inv[s][t] for t in range(NT) for s in range(NC)])
    macs = [mac(s + 1, NC - 1 - s, s) for s in range(NC)]
    grp.append(Group("mac00", macs[0][0], 12, ["c1"], ["c2"], 0))
    grp.append(Group("mac01", macs[1][0] + macs[0][1] + macs[1][1], 16, ["c2"], ["c3"], 0))
    for t in range(NT):
        grp.append(Group("mac%d" % t, cat(macs[s][t] for s in range(2 if t < 2 else 0, NC)), 24 if t < 2 else 18,
                         ["c3", "K%d" % t], ["I%d" % t], 100, 150))
    start = lambda cs: [("run", "run", lambda: [c.start() for c in cs])]
    f0, f1 = front(0, 2, True), front(1, 1, True)
    seq += run(ahead(0))
    seq += W("wma") + _flat(mod("moda", 0, 3)) + run(f0[0] + f1[0] + ahead(1))
    seq += W("wmb") + start(next_kv(NC) + next_q(NC)) + _flat(mod("modb", 3, 5)) + run(f0[1])
    w1 = _flat(mm1("w1_0", 0, 0) + mm1("w1_1", 1, 1))
    seq += W("w1") + w1[:72] + W("w2") + w1[72:] + run(shift(0, 0))
    seq += _flat(mm2("w2_0", 0, 2, 1) + mm1("w1_2", 2, 2)) + run(shift(1, 1)) + _flat(mm2("w2_1", 1, 1, 0))
    grp.append(Group("f1", f1[1], 80, ["w1"], ["w1_1"], 450))
    grp.append(Group("f2", front(2, 0), 80, ["w2"], ["w1_2"], 450))
    grp.append(Group("ln2_0", ln2(1, 0, False), 60, ["w2_0"], ["w3"], 450))
    grp.append(Group("ahead", cat(ahead(i) for i in range(2, NB - NC)), 19, ["w1"], ["end"], 100))
    grp.append(Group("ws1", wsums(w1_w, w1s, KD, ND), 26, ["w1"], ["end"], 100))
    grp.append(Group("ws2", wsums(w2_w, w2s, KD, ND), 26, ["w2"], ["end"], 100))
    grp.append(Group("ws3", w3_turn() + wsums(w3n_w, w3s, KD, KF[:6]) + wsums2(3), 24, ["w3"], ["end"], 100))
    grp.append(Group("ws4", wsums4(), 40, ["w4"], ["end"], 60))
    _wait(seq, "w3", back=1)
    w3 = mm3("w3_0", 0, False, False)
    _mix(seq, _flat(w3[6:]), [split(w3[4:6]) + _flat(w3[:6])], 0.1)
    mc = mod("modc", 5, 6)
    mc = _flat(mc[1:] + mc[:1])
    _wait(seq, "w4", mc[:5] + [("sync", "run", lambda: None)])
    w4 = cat(mm4("w4_0", 0, 0, 3, 2, 1, False)[1:])
    qs = [split([w4[-1 - i]]) for i in range(_phase(seq))]
    _mix(seq, _flat(w4), [mc[i:i + 4] for i in range(5, 25, 4)] + qs, 0.01, 0.4)
    assert _phase(seq) == 0
    grp.append(Group("resid", resid(2, 1), 26, ["modc"], ["end"], 100))
    _emit(seq, grp, zero, wait)

    def step(s, carry):
        for c in next_kv(s) + next_q(s):
            c.wait()
        nxt = jnp.minimum(s + 1, NB - 1)
        seq, grp = [], []
        us, it = one(mmU(lambda n: "U%d" % n, 0, 0)), one(mmI(lambda n: "I%d" % n, 0, 0))
        w4, w4c = mm4("w4", s - 2, 0, fast=2)[1], mm4("w4c", s - 3, 0, fast=2)[0]
        w2 = mm2("w2", 0, 1, 0, True)
        q = split(w2[3:4])
        _mix(seq, _flat(w4c + mm3("w3", 0)),
             [us[0], us[1], us[2], it[0] + us[3], it[1] + us[4], it[2] + start(next_kv(nxt)), it[3], it[4]],
             E("LP3", 0.25), E("LP0", 0.8))
        w1a, w1b = mm1("w1a", 2, 0, True), mm1("w1b", 2, 0, True)
        w1a, w1b = _flat(w1a[0:2] + w1a[4:13] + w1a[22:31]), _flat(w1b[2:4] + w1b[13:22] + w1b[31:])
        k = 9 * E("KW", 5)
        seq += _flat(w4[:k]) + w1a + run(shift(1, 0, ((T - 32, 32),), gs)) + _flat(w4[k:])
        seq += w1b[:8] + start(next_q(nxt)) + w1b[8:]
        _mix(seq, _flat(w2), [q])
        assert _phase(seq) == 0
        kvs, macs = kv(0, 0), mac(1, 0, 0, part=True)
        for t in range(NT):
            grp.append(Group("kv%d" % t, kvs[t], 50, ["start"], ["U%d" % t], 300))
            grp.append(Group("mac%d" % t, macs[t], 24, ["U%d" % t], ["I%d" % t], 300, 150))
        iall = ["I%d" % t for t in range(NT)]
        ln = ln2(0, 0)
        grp.append(Group("ln2a", ln[0:4] + ln[8:12], 75, ["start"], ["w3a"], 450))
        grp.append(Group("ln2b", ln[4:8] + ln[12:16], 75, ["w4c"], ["w3b0"], 450, -300))
        grp.append(Group("resid", resid(1, 0, True), 40, ["w4c"], ["w4q", "I4"], 100))
        xa = lsums2(4, a_w, as_w[3], 0)
        grp.append(Group("xa", [f for x in xa for i, f in enumerate(x) if i % 4 < 2], 26, ["w3a"], ["w4q"], 150))
        for p in range(3):
            grp.append(Group("xb%d" % p, [f for i, f in enumerate(xa[p]) if i % 4 >= 2], 26, ["w3b%d" % p], ["w4q"], 150, 100))
        fr = front(0, 0, ss=n1s)
        grp.append(Group("fronta", fr[0], 50, iall, ["w1a"], E("FL", 230)))
        grp.append(Group("frontb", fr[1], 50, iall, ["w1b"], E("FL", 230), E("RL", 2500)))
        grp.append(Group("fq", fr[2], 34, ["w4c"], ["I4"], 100))
        grp.append(Group("spread", spread(), 30, iall, ["end"], 100))
        grp.append(Group("shift", shift_early(), 24, ["start"], ["w1a"], 200))
        _emit(seq, grp, zero, wait)
        out_b(s - 3).wait()
        out_a(s - 2).wait()
        return carry

    lax.fori_loop(NC, NB, step, 0)

    seq, grp = [], []
    w47 = mm4("w4_7", NB - 1, 1, 2, 0, 1, 2)
    seq += _flat(mm4("w4_5", NB - 3, 0, fast=2)[0] + mm2("w2_7", 0, 0, 1, True) + mm3("w3_6", 0, 2)
                 + cat(mm4("w4_6", NB - 2, 0, 1, 1, 0, 2)) + mm3("w3_7", 1, 2) + w47[0][:3] + w47[1] + w47[0][3:])
    grp.append(Group("shift7", shift(2, 0, [(r, 32) for r in range(0, T, 32)], gs), 24, ["start"], ["w2_7"], 200))
    grp.append(Group("ln2_6", ln2(0, 0), 75, ["start"], ["w3_6"], 1200))
    grp.append(Group("xn6", cat(lsums2(3, n2_w, as_w[2], 0)), 26, ["w4_5"], ["w3_6_0"], 200, 800))
    grp.append(Group("ln2_7", ln2(1, 1), 75, ["w4_6"], ["w3_7"], 1500))
    grp.append(Group("xn7", cat(lsums2(3, n2_w, as_w[2], 1)), 26, ["w4_6"], ["w3_7_0"], 200, 2100))
    for j in (6, 7):
        for p, ts in enumerate(lsums2(4, a_w, as_w[3], j - 6)):
            grp.append(Group("xa%d_%d" % (j, p), ts, 26, ["w3_%d_%d" % (j, p)], ["w4_%dq" % j], 200, 150))
    _emit(seq, grp, zero, wait)
    for c in next_kv(NB - 1) + next_q(NB - 1) + [out_b(NB - 3)] + last:
        c.wait()


@jax.jit
def pallas_adaLN_cond__ssm_conv_h3__mixer_s_mlp__prompt_kernel(
        A_q, A_k, A_v, A_shift_k, A_ssm_k, A_ssm_D, B_x, B_w1, B_w2, B_w3, B_w4, c, w_mod):
    any_ = pl.BlockSpec(memory_space=pl.ANY)
    V = pltpu.VMEM
    out = pl.pallas_call(
        kernel,
        in_specs=[any_] * 12,
        out_specs=any_,
        out_shape=jax.ShapeDtypeStruct((S, D), BF16),
        scratch_shapes=[
            [V((NT, H + 8, 128), U32)] * NC, [V((NT, H + 8, 128), U32)] * NC, [V((NT, H + 8, 128), U32)] * NC,
            [V((64, S), U32)] * NT,
            V((D // 2, D), U32), V((D // 2, D), U32), V((F // 2, D), U32), V((FT * 64, D), U32),
            [V((D // 2, 3 * D), U32), V((D // 2, 2 * D), U32), V((D // 2, D), U32)], V((4 * T, D), BF16),
            V((4, D), BF16), V((D,), BF16), V((1, D), BF16), V((8, 128), I32), pltpu.SMEM((8, 128), I32),
            V((5, 8, D), F32), V((6, 8, D), F32), V((T // 2, 4 * H), U32), V((GR // 2, 2 * T), U32),
            V((NB, 3 * T + 8, D), F32), V((NC, 3 * T + 8, D), F32), V((NB - NC, 2 * T + 8, D), F32), V((4 * T, 128), F32),
            V((T, D), U32), V((NC * T, D), U32), V((NT, NC * (T + 8) + 16, 128), F32),
            V((3 * T, D), F32), V((3 * T, D), F32), V((2 * T, D), F32), V((T, D), F32),
            V((3 * T // 2, D), U32), V((T, D), U32), V((T, D), U32), V((NT, NC * T + 24, 128), F32),
            V((T, (FT + 1) * 128), U32),
            [V((128, 11 * 128), U32)] * 2 + [V((128, 31 * 128), U32), V((448, 11 * 128), U32)],
            [V((64, 11 * 128), U32)] * 2 + [V((128, 11 * 128), U32), V((128, 35 * 128), U32)],
            V((D // 2, 13 * 128), U32), V((H, D), F32), V((T, 7 * 128), F32),
            [V((64, 105 * 128), U32), V((192, 35 * 128), U32), V((32, 35 * 128), U32), V((32, 105 * 128), U32)],
            pltpu.SemaphoreType.DMA((11,)), pltpu.SemaphoreType.DMA((1,)), pltpu.SemaphoreType.DMA((3,)),
        ],
        compiler_params=pltpu.CompilerParams(vmem_limit_bytes=110 << 20, disable_semaphore_checks=True,
                                             disable_bounds_checks=True),
        name="fused",
    )(A_q[0], A_k[0], A_v[0], A_shift_k.T, A_ssm_k, A_ssm_D, B_w1, B_w2, B_w3.T, B_w4, c, w_mod)
    return out[None]
```

```python
import heapq
import os
import numpy as np
import jax
import jax.numpy as jnp
from jax import lax
from jax.experimental import pallas as pl
from jax.experimental.pallas import tpu as pltpu

S, D, F = 2048, 640, 1728
T = 256
H = T // 2
NB = S // T
NT = D // 128
FT = (F + 127) // 128
EPS = 1e-5
F32, BF16, U32, I32 = jnp.float32, jnp.bfloat16, jnp.uint32, jnp.int32
G_C1 = 0.044715 * float(np.sqrt(2.0 / np.pi))
G_C2 = float(np.sqrt(2.0 / np.pi))
G_A = G_C1 ** (1.0 / 3.0)
G_B = G_C2 / G_A
G_POST = 0.5 / G_A
RG = 16
GR = 80
NC = 3
DL = 450
E = lambda k, d: type(d)(os.environ.get(k, d))
KS = E('KS', 1.5)
SLOT = 32


def _dft(shape, f_axis, tau, scale=1.0):
    r = lax.broadcasted_iota(I32, shape, f_axis)
    l = lax.broadcasted_iota(I32, shape, 1 - f_axis)
    f = r & 127
    odd = ((f & 63) << 2) | ((f >> 6) << 1) | 1
    p = odd * tau(l) + ((r >> 7) << 8)
    a = ((p + 512) & 1023) - 512
    u = (256 - jnp.abs(a)).astype(F32) * (np.pi / 512.0)
    u2 = u * u
    c = [scale, -scale / 6.0, scale / 120.0, -scale / 5040.0, scale / 362880.0, -scale / 39916800.0]
    poly = c[5]
    for ci in c[4::-1]:
        poly = poly * u2 + ci
    return (u * poly).astype(BF16)


def _rstd(xc, mlp):
    s2, eps = (1.0 / (G_A * G_A), EPS / (G_POST * G_POST)) if mlp else (1.0, EPS)
    v = jnp.sum(xc * xc, axis=-1, keepdims=True) * (s2 / D) + eps * s2
    return jnp.exp2(jnp.log(v) * float(-0.5 / np.log(2.0)))


def _ln(x, mlp=False):
    xc = x - jnp.sum(x, axis=-1, keepdims=True) * (1.0 / D)
    return xc * _rstd(xc, mlp)


def _gelu2(x):
    u = x * (x * x + G_B)
    return x * (1.0 + jnp.tanh(u))


def _lo(w):
    return pltpu.bitcast(w << 16, F32)


def _hi(w):
    return pltpu.bitcast(w & jnp.uint32(0xFFFF0000), F32)


def _tie(x, a):
    if a is None:
        return x
    w = pltpu.bitcast(x[:, :128], U32)
    k = w.shape[0] // 8
    w = w | (a if k == 1 else jnp.concatenate([a] * k, axis=0))
    w = pltpu.bitcast(w, x.dtype)
    return w if x.shape[1] == 128 else jnp.concatenate([w, x[:, 128:]], axis=1)


def _top(x, i):
    return jnp.concatenate([x[r:r + 16] for r in range(16 * i, x.shape[0], 32)], axis=0)


def _zip(t, b):
    return jnp.concatenate([x[r:r + 16] for r in range(0, t.shape[0], 16) for x in (t, b)], axis=0)


def _lhs_sums(x1, x2):
    a11, a21, a12, a22 = _top(x1, 0), _top(x1, 1), _top(x2, 0), _top(x2, 1)
    return [a11 + a22, a21 + a22, a11 + a12, a21 - a11, a12 - a22]


def C(i):
    return slice(i * 128, (i + 1) * 128)


class Unit:
    def __init__(self, name, tiles, epi, rows, cost, nt=False, full=True, acc=False, tail=0):
        self.tail = tail
        self.acc, self.res = acc, []
        self.name, self.tiles, self.epi, self.rows, self.cost, self.nt, self.full = name, tiles, epi, rows, cost, nt, full


class Due:
    def __init__(self, val, delay):
        self.val, self.delay = val, delay


class Group:
    def __init__(self, name, fns, cost, rel, dead, lat, rlat=200):
        self.name, self.fns, self.cost, self.rel, self.dead, self.lat, self.rlat = name, fns, cost, rel, dead, lat, rlat


def _plan(seq, groups):
    busy, n = [0] * 4, 0
    start, end, tiles, bars = {}, {}, [], []
    for it in seq:
        if isinstance(it[0], Unit):
            u = it[0]
            m = n % 4
            n += 1
            t0, t1 = busy[m], busy[m] + max(u.rows, 32)
            busy[m] = t1
            tiles.append((t0, t1, u.cost / len(u.tiles) + (u.tail if it[1] == len(u.tiles) - 1 else 0)))
            start.setdefault(u.name, t0)
            end[u.name] = max(end.get(u.name, 0), t1)
        elif it[0] == "wait":
            t = max(busy)
            busy, n = [t] * 4, 0
            start[it[1]] = end[it[1]] = t
            bars.append(t)
    total = max(busy)
    start["end"] = end["end"] = total
    start["start"] = end["start"] = 0
    ns = total // SLOT + 2
    load = np.zeros(ns)
    for t0, t1, c in tiles:
        a, b = t0 // SLOT, max(t1 // SLOT, t0 // SLOT + 1)
        load[a:b] += c / (b - a)
    win = []
    for g in groups:
        r = max(end[x] + (0 if start[x] == end[x] else g.rlat) for x in g.rel)
        d = min(start[x] for x in g.dead) - g.lat
        ok = np.zeros(ns, bool)
        ok[r // SLOT:max(d // SLOT, r // SLOT + 1)] = True
        for b in bars:
            if r < b <= d:
                ok[max((b - g.lat) // SLOT, 0):b // SLOT] = False
        win.append(np.nonzero(ok)[0])
    alloc = [np.zeros(len(w)) for w in win]
    for _ in range(60):
        for i, g in enumerate(groups):
            w = win[i]
            load[w] -= alloc[i]
            base = load[w]
            vol = g.cost * len(g.fns)
            lo, hi = base.min(), base.max() + vol
            for _ in range(50):
                mid = 0.5 * (lo + hi)
                if np.maximum(mid - base, 0).sum() > vol:
                    hi = mid
                else:
                    lo = mid
            alloc[i] = np.maximum(hi - base, 0)
            load[w] += alloc[i]
    times = []
    for i, g in enumerate(groups):
        cum = np.cumsum(alloc[i])
        ts = []
        for k in range(len(g.fns)):
            x = (k + 0.5) * cum[-1] / len(g.fns)
            j = int(np.searchsorted(cum, x))
            prev = cum[j - 1] if j else 0.0
            ts.append(win[i][j] * SLOT + SLOT * (x - prev) / max(alloc[i][j], 1e-9))
        times.append(ts)
    return times


def _emit(seq, groups, zero, wait):
    times = _plan(seq, groups)
    left = {"start": 0}
    for it in seq:
        nm = it[0].name if isinstance(it[0], Unit) else it[1]
        left[nm] = left.get(nm, 0) + 1
    heap, pend, todo, cnt = [], {}, list(range(len(groups))), 0
    busy, n, due = [0] * 4, 0, []

    def release():
        nonlocal cnt
        for i in list(todo):
            g = groups[i]
            if all(left[x] == 0 for x in g.rel):
                todo.remove(i)
                pend[i] = len(g.fns)
                for t, fn in zip(times[i], g.fns):
                    heapq.heappush(heap, (t, cnt, i, fn))
                    cnt += 1

    def force(name):
        nonlocal heap
        for i, g in enumerate(groups):
            if name in g.dead:
                assert i not in todo, (g.name, name)
                if pend[i]:
                    for it in sorted(x for x in heap if x[2] == i):
                        it[3](None)
                    heap = [x for x in heap if x[2] != i]
                    heapq.heapify(heap)
                    pend[i] = 0

    release()
    for it in seq:
        if isinstance(it[0], Unit):
            u, k = it
            force(u.name)
            lhs, rhs = u.tiles[k]()
            t0 = busy[n % 4]
            while u.full and due and due[0][0] < t0 + u.rows:
                t, x = due.pop(0)
                r = min(max(int(t - t0), 0), u.rows - 1) // 16 * 8
                w = pltpu.bitcast(lhs, U32)
                x = pltpu.bitcast(x[:, :128], U32)
                parts = [w[:r], w[r:r + 8] | ((x[0:8] | x[8:16]) & zero), w[r + 8:]]
                lhs = pltpu.bitcast(jnp.concatenate([y for y in parts if y.shape[0]], axis=0), BF16)
            dn = (((1,), (1 if u.nt else 0,)), ((), ()))
            p = lax.dot_general(lhs, rhs, dn, preferred_element_type=F32)
            u.res = [p + u.res[0]] if (u.acc and u.res) else u.res + [p]
            m = n % 4
            n += 1
            t0 = busy[m]
            busy[m] = t0 + max(u.rows, 32)
            while u.full and heap and heap[0][0] < t0 + u.rows:
                t, _, i, fn = heapq.heappop(heap)
                pend[i] -= 1
                r = min(max(int(t - t0), 0), u.rows - 1) // 8 * 8
                x = fn(pltpu.bitcast(p[r:r + 8], U32) & zero)
                if isinstance(x, Due):
                    due.append((t + x.delay, x.val))
                    due.sort(key=lambda e: e[0])
            if k == len(u.tiles) - 1:
                u.epi(u.res)
            left[u.name] -= 1
        elif it[0] == "wait":
            force(it[1])
            wait(it[1])
            busy, n, due = [max(busy)] * 4, 0, []
            left[it[1]] -= 1
        else:
            it[2]()
            left[it[1]] -= 1
        release()
    force("end")
    assert not heap and not todo


def _sum(ps):
    acc = ps[0]
    for p in ps[1:]:
        acc = acc + p
    return acc


def _flat(us):
    return [(u, i) for u in us for i in range(len(u.tiles))]


def _weave(a, b):
    out = []
    for i, u in enumerate(a):
        out += [u] + b[i * len(b) // len(a):(i + 1) * len(b) // len(a)]
    return out


def _phase(seq):
    n = 0
    for it in seq:
        n = n + 1 if isinstance(it[0], Unit) else (0 if it[0] in ("wait", "sync") else n)
    return n % 4


def _mix(seq, a, b, lo=0.0, hi=1.0):
    n, k = _phase(seq), 0
    for i, t in enumerate(a):
        if k < len(b) and n % 4 == 0 and t[1] != 1 and i >= len(a) * (lo + (hi - lo) * k / len(b)):
            seq.extend(b[k])
            k += 1
        seq.append(t)
        n += 1
    assert k == len(b)


def _wait(seq, name, head=(), back=0):
    r = _phase(seq) + 4 * back
    assert all(isinstance(it[0], Unit) for it in seq[len(seq) - r:])
    seq[len(seq) - r:len(seq) - r] = [("wait", name)] + list(head)


def kernel(q_hbm, k_hbm, v_hbm, sh_hbm, ssm_hbm, sd_hbm, w1_hbm, w2_hbm, w3_hbm, w4_hbm, c_hbm, wm_hbm,
           o_hbm,
           q_n, k_n, v_n, ssm_w, w1_w, w2_w, w3_w, w4_w, wm_w, o_v,
           sh_v, sd_v, c_v, zsrc, z_s, taps, mod_v, tf_w, tg_w,
           kf, uf, acc, zraw, kv_w, zz_w, y_v, x_v, hb_v, x1_v, r_v, n1_w, n2_w, g_w, h1_v, a_w,
           ws_w, as_w, w3n_w, top_v, st_v, l2_w,
           sem, sem_b, sem_o):
    bf = lambda r: r.bitcast(BF16)
    w1_v, w2_v, w3_v, w4_v = bf(w1_w), bf(w2_w), bf(w3_w), bf(w4_w)
    wm_v = {0: bf(wm_w[0]), 3: bf(wm_w[1]), 5: bf(wm_w[2])}
    tf_v, tg_v, n1_v, n2_v, g_v = bf(tf_w), bf(tg_w), bf(n1_w), bf(n2_w), bf(g_w)
    a_v, kv_v, zz_v = bf(a_w), bf(kv_w), bf(zz_w)
    w1s, w2s, w3s, w4s = [bf(r) for r in ws_w]
    n1s, gs, n2s, a_s = [bf(r) for r in as_w]
    w3n = bf(w3n_w)
    w3t, w4t, n2t, a_t = [bf(r) for r in l2_w]
    cp = pltpu.make_async_copy
    cat = lambda ls: [x for l in ls for x in l]

    def base(j, n):
        return j * n if isinstance(j, int) else pl.multiple_of(j * n, n)

    def rows(j, n=1, size=T):
        return pl.ds(base(j, size), n * size)

    def view(ref, j, size=T):
        return ref.at[rows(j, 1, size)]

    dmas = {}

    def group(name, *mks):
        sm = sem.at[len(dmas)]
        dmas[name] = [c for mk in mks for c in mk(sm)]

    def ssm_in(t):
        return lambda sm: [cp(ssm_hbm.at[C(t)], bf(ssm_w[t]), sm)]

    def cols(src, start, n, dst, row=0):
        return lambda sm: [cp(src.at[pl.ds(start, n), C(t)], bf(dst).at[t, pl.ds(row, n)], sm) for t in range(NT)]

    def kv_in(s, sl):
        if isinstance(s, int):
            kk = cols(k_hbm, s * T - 16, T + 16, k_n[sl]) if s else cols(k_hbm, 0, T, k_n[sl], 16)
        else:
            kk = cols(k_hbm, pl.multiple_of(s * T - 16, 16), T + 16, k_n[sl])
        return lambda sm: kk(sm) + cols(v_hbm, base(s, T), T, v_n[sl])(sm)

    def q_in(s, sl):
        return cols(q_hbm, base(s, T), T, q_n[sl])

    def wm_in(a, b):
        return lambda sm: [cp(wm_hbm.at[:, a * D:b * D], wm_v[a], sm)]

    def whole(src, dst):
        return lambda sm: [cp(src, dst, sm)]

    next_kv = lambda s: kv_in(s, 0)(sem_b.at[0])
    next_q = lambda s: q_in(s, 0)(sem_b.at[0])

    zsrc[...] = jnp.zeros((8, 128), I32)
    k_n[0][:, 0:8, :] = jnp.zeros((NT, 8, 128), U32)
    w4_w[F // 2:FT * 64, :] = jnp.zeros((FT * 64 - F // 2, D), U32)
    group("small", lambda sm: [cp(zsrc, z_s, sm), cp(sh_hbm, sh_v, sm), cp(sd_hbm, sd_v, sm), cp(c_hbm, c_v, sm)])
    for s in range(NC):
        group("c%d" % s, ssm_in(s), kv_in(s, s))
    group("c3", ssm_in(3), ssm_in(4))
    group("wma", wm_in(0, 3), q_in(0, 0), q_in(1, 1))
    group("wmb", wm_in(3, 5))
    group("w1", whole(w1_hbm, w1_v))
    group("w2", q_in(2, 2), whole(w2_hbm, w2_v))
    group("w3", whole(w3_hbm, w3_v))
    group("w4", whole(w4_hbm, w4_v.at[0:F]), wm_in(5, 6))
    for g in dmas.values():
        for c in g:
            c.start()

    def wait(name):
        for c in dmas[name]:
            c.wait()

    tau_b = lambda l: H + ((l + (H - 1)) & (H - 1))
    tf_v[:, C(0)] = _dft((T, H), 0, lambda l: jnp.where((l & 1) == 0, l, tau_b(l)), 1.0 / T)
    tf_v[:, C(1)] = _dft((T, H), 0, lambda l: jnp.where((l & 1) == 1, l, tau_b(l)), 1.0 / T)
    tf_v[:, C(2)] = _dft((T, H), 0, lambda l: 2 * l - H)
    tf_v[:, C(3)] = _dft((T, H), 0, lambda l: 2 * l + 1 - H)
    sin0 = lax.broadcasted_iota(I32, (GR, T), 1) >= H
    tg_v[:, 0:T] = _dft((GR, T), 1, lambda l: jnp.where(sin0 & (l == 0), H, 2 * l))
    tg_v[:, T:2 * T] = _dft((GR, T), 1, lambda l: 2 * l + 1)
    h1_v[:, 0:8, :] = jnp.zeros((NT, 8, 128), F32)
    h1_v[:, 8 + NC * T:16 + NC * T, :] = jnp.zeros((NT, 8, 128), F32)

    wait("small")
    z = jnp.clip(z_s[0, 0], 0, 1)
    zero = jnp.full((8, 128), z, I32).astype(U32)
    z8 = pl.multiple_of(z * 8, 8)
    for r in (x_v, hb_v, x1_v, r_v, zraw, n1_w, n2_w, g_w, a_w, kv_w, zz_w, *ws_w, *as_w, w3n_w, top_v, st_v, *l2_w):
        r[pl.ds(z8, 8), 0:128] = jnp.zeros((8, 128), r.dtype)
    for r in (kf, uf, acc, taps, mod_v):
        r[z, 0:8, 0:128] = jnp.zeros((8, 128), r.dtype)
    for r in (tf_w, tg_w):
        r[pl.ds(z8, 8), 0:128] = r[0:8, 0:128]
    sh = sh_v[...].astype(F32)
    for i in range(4):
        taps[i] = jnp.broadcast_to(sh[i:i + 1], (8, D))
    taps[4] = jnp.broadcast_to(sd_v[...].astype(F32).reshape(1, D) * (1.0 / T), (8, D))
    cf = c_v[...].astype(F32)
    silu_c = jnp.broadcast_to((cf / (1.0 + jnp.exp(-cf))).astype(BF16), (16, D))

    def mmK(n):
        def unit(m):
            st = []

            def rhs(i):
                if not st:
                    ev = (lax.broadcasted_iota(I32, (64, 128), 1) & 1) == 0
                    a = ssm_w[n][:, m * T:m * T + H]
                    b = pltpu.roll(ssm_w[n][:, m * T + H:(m + 1) * T], 1, 1)
                    st.extend([pltpu.bitcast(jnp.where(ev, a, b), BF16), pltpu.bitcast(jnp.where(ev, b, a), BF16)])
                return st[i]

            def epi(p):
                er, ei, or_, oi = p
                cur = [er, ei, or_, oi]
                if m:
                    pv = [zraw[C(4 * ((m - 1) % 2) + (q ^ 1)), :] for q in range(4)]
                    pm = lambda x, y, up: jnp.concatenate([x[:64] + y[:64], x[64:] - y[64:]] if up else
                                                          [x[:64] - y[:64], x[64:] + y[64:]], axis=0)
                    er, ei, or_, oi = [pm(cur[q], pv[q], q & 1) for q in range(4)]
                else:
                    er = er + taps[4, 0:1, C(n)]
                if m + 1 < NB:
                    for q in range(4):
                        zraw[C(4 * (m % 2) + q), :] = cur[q]
                for h, (cr, ci) in enumerate(((er + or_, ei + oi), (er - or_, ei - oi))):
                    B = h * 3 * H
                    kf[m, B:B + H, C(n)] = cr
                    kf[m, B + H:B + 2 * H, C(n)] = ci - cr
                    kf[m, B + 2 * H:B + 3 * H, C(n)] = ci + cr
            return Unit("K%d" % n, [(lambda i=i, r=r: (tf_v[r:r + H, C(i)], rhs(i))) for i in range(2) for r in (0, H)],
                        epi, H, 260, nt=True)
        return [unit(m) for m in range(NB)]

    def kv(s, sl):
        def mk(t, w):
            def fn(a):
                ld = lambda o, n: k_n[s][t, pl.ds(8 + w + o, n), :]
                c0 = jnp.concatenate([_tie(ld(0, 8), a), ld(8, 8)], axis=0).reshape(2, 8, 128)
                c1, c2 = ld(-1, 16).reshape(2, 8, 128), ld(-2, 16).reshape(2, 8, 128)
                s0, s1, s2, s3 = (taps[i, :, C(t)] for i in range(4))
                ke, ko, ke1, ko1, ko2 = _lo(c0), _hi(c0), _lo(c1), _hi(c1), _hi(c2)
                wv = v_n[s][t, w:w + 16, :].reshape(2, 8, 128)
                kve = ((s0 * ke + s1 * ko1) + (s2 * ke1 + s3 * ko2)) * _lo(wv)
                kvo = ((s0 * ko + s1 * ke) + (s2 * ko1 + s3 * ke1)) * _hi(wv)
                kv_v[pl.ds(sl * T + w, 16), C(t)] = kve.reshape(16, 128).astype(BF16)
                kv_v[pl.ds(sl * T + H + w, 16), C(t)] = kvo.reshape(16, 128).astype(BF16)
            return fn
        return [[mk(t, w) for w in range(0, H, 16)] for t in range(NT)]

    def mmU(name, sl, us):
        def unit(n):
            def epi(p):
                er, ei, or_, oi = p
                for h, (cr, ci) in enumerate(((er + or_, ei + oi), (er - or_, ei - oi))):
                    B = h * 3 * H
                    uf[us, B:B + H, C(n)] = cr + ci
                    uf[us, B + H:B + 2 * H, C(n)] = cr
                    uf[us, B + 2 * H:B + 3 * H, C(n)] = ci
            return Unit(name(n), [(lambda i=i, r=r: (tf_v[r:r + H, C(2 + i)], kv_v[pl.ds(sl * T + i * H, H), C(n)]))
                                  for i in range(2) for r in (0, H)], epi, H, 96 + 96 * KS)
        return [unit(n) for n in range(NT)]

    def cmul(m0, u0, n, h, row, L, a):
        t = []
        for i in range(3):
            Rw = slice((3 * h + i) * H + row, (3 * h + i) * H + row + 8)
            kk = kf[m0:m0 + n, Rw, L]
            if i == 0 and a is not None:
                k0 = _tie(kk[0], a)[None]
                kk = k0 if n == 1 else jnp.concatenate([k0, kk[1:]], axis=0)
            t.append(jnp.sum(kk * uf[u0:u0 + n, Rw, L], axis=0))
        return t[0] - t[2], t[0] + t[1]

    def AR(h, q, row):
        return slice((2 * h + q) * H + row, (2 * h + q) * H + row + 8)

    def mac(n, u0, sl, part=False):
        def mk(t, rc):
            st, fin = [], []

            def piece(i):
                def fn(a):
                    h, row = i & 1, rc + (i >> 1) * 8
                    zr, zi = cmul(0, u0, n, h, row, C(t), a)
                    if part:
                        zr, zi = zr + acc[0, AR(h, 0, row), C(t)], zi + acc[0, AR(h, 1, row), C(t)]
                    st.append((zr, zi))
                    if h:
                        (pr, pi), (mr, mi) = st[-2:]
                        fin.append([pr + mr, pi + mi, pr - mr, pi - mi])
                    if i == 3:
                        for q in range(4):
                            zz_v[pl.ds(sl * 2 * T + q * H + rc, 16), C(t)] = jnp.concatenate(
                                [fin[0][q], fin[1][q]], axis=0).astype(BF16)
                return fn
            if not part:
                return [piece(i) for i in range(4)]
            both = lambda f, g: (lambda a: (f(a), g(None)))
            return [both(piece(0), piece(1)), both(piece(2), piece(3))]
        return [[fn for rc in range(0, H, 16) for fn in mk(t, rc)] for t in range(NT)]

    def pos():
        return [(t, h, row) for t in range(NT) for row in range(0, H, 8) for h in range(2)]

    def ahead(i):
        def mk(t, h, row):
            def fn(a):
                zr, zi = cmul(i + 1, 0, NC, h, row, C(t), a)
                acc[i, AR(h, 0, row), C(t)] = zr
                acc[i, AR(h, 1, row), C(t)] = zi
            return fn
        return [mk(*p) for p in pos()]

    def spread():
        n = NB - NC - 1

        def mk(t, h, row):
            def fn(a):
                p = []
                for i in range(3):
                    Rw = slice((3 * h + i) * H + row, (3 * h + i) * H + row + 8)
                    u = uf[0, Rw, C(t)]
                    p.append(kf[1:1 + n, Rw, C(t)] * (_tie(u, a) if i == 0 else u)[None])
                acc[0:n, AR(h, 0, row), C(t)] = acc[1:1 + n, AR(h, 0, row), C(t)] + (p[0] - p[2])
                acc[0:n, AR(h, 1, row), C(t)] = acc[1:1 + n, AR(h, 1, row), C(t)] + (p[0] + p[1])
            return fn
        return [mk(*p) for p in pos()]

    def mmI(name, sl, ys):
        def unit(n):
            def epi(p):
                ce, se, co, so = p
                sub = lax.broadcasted_iota(I32, (8, 128), 0)
                b0 = ys * (T + 8) + 8
                y_v[n, b0 + H - 1:b0 + H, :] = (ce[64:72] - se[0:8])[0:1]
                se = jnp.concatenate([jnp.where(sub == 0, 0.0, se[0:8]), se[8:]], axis=0)
                for d, cc, ss in ((0, ce[0:64], se), (1, co, so)):
                    y_v[n, pl.ds(b0 + H + d, 64, stride=2), :] = cc + ss
                    y_v[n, pl.ds(b0 + d - 1, 64, stride=2), :] = cc - ss
            return Unit(name(n), [(lambda i=i: (tg_v[0:(GR if i == 0 else 64), C(i)], zz_v[pl.ds(sl * 2 * T + i * H, H), C(n)]))
                                  for i in range(4)], epi, 64, 36 + 33 * KS)
        return [unit(n) for n in range(NT)]

    def mod(name, a, b):
        def unit(n):
            def epi(p):
                v = [_sum(p[i * NT:(i + 1) * NT])[0:8] for i in range(b - a)]
                if a == 0:
                    mod_v[0, :, C(n)] = v[0] * v[2]
                    mod_v[1, :, C(n)] = (v[1] + 1.0) * v[2]
                elif a == 3:
                    mod_v[3, :, C(n)] = v[0] * (1.0 / G_POST)
                    mod_v[4, :, C(n)] = (v[1] + 1.0) * (1.0 / G_POST)
                else:
                    mod_v[2, :, C(n)] = v[0] * G_POST
            return Unit(name, [(lambda i=i, k=k: (silu_c[:, C(k)], wm_v[a][C(k), pl.ds(i * D + n * 128, 128)]))
                               for i in range(b - a) for k in range(NT)], epi, 16, 10, full=False, acc=b - a == 1)
        return [unit(n) for n in range(NT)]

    HS = (slice(0, 128), slice(128, 256))
    QS = tuple(slice(r, r + 64) for r in range(0, T, 64))

    def tasks(f, due=None, tie=True, n=RG):
        def mk(R):
            def fn(a):
                x = f(R, a if tie else None)
                return Due(x, due) if due else None
            return fn
        return [mk(slice(r, r + n)) for r in range(0, T, n)]

    def load_y(sl, R):
        b0, back = sl * (T + 8) + 8, 7 - lax.broadcasted_iota(I32, (8, 128), 0)

        def ld(t, r):
            if r >= H:
                return y_v[t, b0 + r:b0 + r + 8, :]
            return jnp.take_along_axis(y_v[t, b0 + H - 8 - r:b0 + H - r, :], back, axis=0)
        return jnp.stack([jnp.concatenate([ld(t, r) for t in range(NT)], axis=1) for r in (R.start, R.start + 8)])

    def put(nn, ss, R, x):
        nn[R, :] = x.astype(BF16)
        tok = x
        if ss is not None:
            S2 = pl.ds(R.start // 32 * 16, 16)
            if R.stop % 32:
                top_v[S2, 0:2 * T] = x[:, 0:2 * T]
            else:
                if R.start % 32:
                    x = jnp.concatenate([top_v[S2, 0:2 * T], x[:, 0:2 * T]], axis=0)
                ss[S2, 0:5 * T] = jnp.concatenate(_lhs_sums(x[:, 0:T], x[:, T:2 * T]), axis=1).astype(BF16)
        return tok

    wide = lambda v: jnp.concatenate([v] * NT, axis=1)

    def mean(i, R, x):
        st_v[R, C(i)] = jnp.broadcast_to(jnp.sum(x, axis=-1, keepdims=True) * (1.0 / D), (x.shape[0], 128))

    def centred(src, i, R, a):
        return src[R, :] - wide(_tie(st_v[R, C(i)], a))

    def scale(src, i, g):
        def f(R, a):
            st_v[R, C(i + 1)] = jnp.broadcast_to(_rstd(centred(src, i, R, a), g), (RG, 128))
        return f

    def normed(src, i, R, a):
        return centred(src, i, R, a) * wide(st_v[R, C(i + 1)])

    def front(sl, xs, early=False, ss=None):
        xx, hh, nn = view(x_v, xs), view(hb_v, xs), view(n1_v, sl)

        def fa(R, a):
            q = [q_n[sl][t, R.start // 2:R.stop // 2, :] for t in range(NT)]
            q = jnp.concatenate([_tie(q[0], a)] + q[1:], axis=1)
            q = pltpu.bitcast(q, BF16).astype(F32).reshape(2, 8, D)
            x = (q + (_ln(q) * mod_v[1] + mod_v[0]) * load_y(sl, R)).reshape(RG, D)
            xx[R, :] = x
            if early:
                hh[R, :] = _ln(x)

        def fb(R, a):
            hh[R, :] = (_ln(_tie(xx[R, :], a).reshape(2, 8, D)) * mod_v[4] + mod_v[3]).reshape(RG, D)

        def fc(R, a):
            hb = _tie(hh[R, :], a)
            if early:
                hb = (hb.reshape(2, 8, D) * mod_v[4] + mod_v[3]).reshape(RG, D)
                hh[R, :] = hb
            nn[R, :] = _ln(hb, True).astype(BF16)
        if early:
            return tasks(fa), tasks(fc)
        if ss is None:
            return tasks(fa) + tasks(fb) + tasks(fc)
        qf = view(x_v, 2)

        def s1(R, a):
            q = [q_n[sl][t, R.start // 2:R.stop // 2, :] for t in range(NT)]
            q = pltpu.bitcast(jnp.concatenate([_tie(v, a) for v in q], axis=1), BF16).astype(F32)
            qf[R, :] = q
            mean(0, R, q)

        def s3(R, a):
            h = normed(qf, 0, R, a).reshape(2, 8, D) * mod_v[1] + mod_v[0]
            x = qf[R, :] + (h * load_y(sl, R)).reshape(RG, D)
            xx[R, :] = x
            mean(2, R, x)

        def s5(R, a):
            hb = (normed(xx, 2, R, a).reshape(2, 8, D) * mod_v[4] + mod_v[3]).reshape(RG, D)
            hh[R, :] = hb
            mean(4, R, hb)
        s7 = [f for g in tasks(lambda R, a: put(nn, ss, R, normed(hh, 4, R, a)), n=32) for f in (g, lambda a: None)]
        st = [tasks(s3), tasks(scale(xx, 2, False)), tasks(s5), tasks(scale(hh, 4, True)), s7]
        p = [tasks(s1), tasks(scale(qf, 0, False))]
        return cat(x[:8] for x in st), cat(x[8:] for x in p[1:] + st), cat(x[:8] for x in p), p[0][8:]

    def shift(hs, sl, pieces=((0, 64), (64, 64), (128, 64), (192, 64)), ss=None):
        gg = view(g_v, sl)

        def one_tile(t, r, n, a):
            lane = lax.broadcasted_iota(I32, (n, 128), 1)
            ld = lambda d: h1_v[t, pl.ds(hs * T + 8 + r + d, n), :]
            if t == 0:
                g = ld(-1)
            elif t == 1:
                g = jnp.where(lane < 32, ld(-1), ld(1))
            elif t == 2:
                g = jnp.where(lane < 64, ld(1), ld(-2))
            elif t == 3:
                g = jnp.where(lane < 96, ld(-2), ld(2))
            else:
                g = ld(2)
            if a is not None:
                g = jnp.concatenate([_tie(g[i:i + 8], a) if i % 16 == 0 else g[i:i + 8]
                                     for i in range(0, n, 8)], axis=0)
            gg[r:r + n, C(t)] = g.astype(BF16)
            return g

        def mk(ts, r, n):
            def fn(a):
                g = [one_tile(t, r, n, a) for t in ts]
                if len(ts) == 2:
                    for i, x in enumerate(_lhs_sums(*g)):
                        ss[r // 2:(r + n) // 2, C(2 * i + ts[0])] = x.astype(BF16)
            return fn
        sets = [(t,) for t in range(NT)] if ss is None else [(0, 2), (1, 3), (4,)]
        return [mk(ts, r, n) for ts in sets for r, n in pieces]

    def shift_early():
        def keep(a):
            h1_v[:, 2 * T - 32:2 * T + 8, :] = h1_v[:, 3 * T - 32:3 * T + 8, :]
        return shift(2, 0, [(r, 32) for r in range(0, T - 32, 32)], gs) + [keep]

    def ln2(xs, sl, fast=True):
        xx, nn, ss = view(x1_v, xs), view(n2_v, sl), view(n2s, sl, H) if fast else None
        f = lambda R, a: put(nn, ss, R, _ln(_tie(xx[R, :], a), True))
        ts = tasks(f, 900) if sl else tasks(f, DL, False)
        return ts[0::2] + ts[1::2] if fast else tasks(f)

    def ln2_late(mode):
        xx, nn, ss = view(x1_v, 0), view(n2_v, 0), view(n2s, 0, H)
        if mode == 0:
            return tasks(lambda R, a: put(nn, ss, R, _ln(_tie(xx[R, :], a), True)), n=32)[:4], 160
        a_, b_ = tasks(lambda R, a: mean(6, R, _tie(xx[R, :], a))), tasks(scale(xx, 6, True))
        c_ = [f for g in tasks(lambda R, a: put(nn, ss, R, normed(xx, 6, R, a)), n=32)[:4] for f in (g, lambda a: None)]
        return a_[:8] + b_[:8] + c_, 40

    def resid(xs, x1s, rotate=False):
        xx, x1 = view(x_v, xs), view(x1_v, x1s)

        def f(R, a):
            gb = mod_v[2] if a is None else pltpu.bitcast(
                pltpu.bitcast(mod_v[2], U32) | jnp.concatenate([a] * NT, axis=1), F32)
            r_v[R, :] = xx[R, :] + (x1[R, :].reshape(2, 8, D) * gb).reshape(RG, D)
            if rotate:
                xx[R, :] = x_v[R, :]
                view(hb_v, 1)[R, :] = hb_v[R, :]
        return tasks(f)

    KD, KF, ND = [(0, 2), (1, 3)], [(2 * i, 2 * i + 1) for i in range(7)], [(1, 2), (3, 4)]
    Wt = {1: (lambda k, n: w1_v[C(k), C(n)], lambda i, kp, j: w1s[C(kp), C(2 * i + j)], False, KD, [4]),
          2: (lambda k, n: w2_v[C(k), C(n)], lambda i, kp, j: w2s[C(kp), C(2 * i + j)], False, KD, [4]),
          0: (lambda k, n: w3_v[C(n), C(k)], None, True, KD, [4]),
          3: (lambda k, n: w3n[C(k), C(n)], lambda i, kp, j: w3s[C(kp), C(6 * i + j)], False, KD, [4]),
          4: (lambda k, n: w4_v[C(k), C(n)], lambda i, kp, j: w4s[C(kp), C(2 * i + j)], False, KF, [])}

    def sums_task(load, store, left):
        def fn(a):
            b = [[load(u, v) for v in range(2)] for u in range(2)]
            b[0][0], b[1][1] = _tie(b[0][0], a), _tie(b[1][1], a)
            (x11, x12), (x21, x22) = [[pltpu.bitcast(x, BF16).astype(F32) for x in row] for row in b]
            r = ((x11 + x22, x21 + x22, x11 + x12, x21 - x11, x12 - x22) if left else
                 (x11 + x22, x12 - x22, x21 - x11, x11 + x12, x21 + x22))
            for m, x in enumerate(r):
                store(m, x.astype(BF16))
        return fn

    def wsums(w_w, ws, rp, cp_):
        def mk(i, j, r):
            def store(m, x):
                ws[pl.ds(128 * i + r, 16), C(len(cp_) * m + j)] = x
            return sums_task(lambda u, v: w_w[pl.ds(64 * rp[i][u] + r // 2, 8), C(cp_[j][v])], store, False)
        return [mk(i, j, r) for j in range(len(cp_)) for i in range(len(rp)) for r in range(0, 128, 16)]

    def w3_turn():
        def mk(n, k):
            def fn(a):
                x = jnp.concatenate([_tie(w3_w[64 * n:64 * n + 8, C(k)], a), w3_w[64 * n + 8:64 * n + 64, C(k)]], axis=0)
                w3n[C(k), C(n)] = pltpu.bitcast(x, BF16).T
            return fn
        return [mk(n, k) for n in range(FT - 1) for k in range(NT)]

    def plain(name, w, lhs, n, R, epi, cost):
        tile, _, nt, kp, kl = Wt[w]
        ks = sorted([k for p in kp for k in p] + kl)
        rows_ = R.stop - R.start
        return Unit(name, [(lambda k=k: (lhs[R, C(k)], tile(k, n))) for k in ks], lambda p: epi(n, R, p[0]),
                    rows_, rows_ // 8 * (len(ks) - 1), nt=nt, acc=True, tail=rows_ // 8 * cost(n))

    def quad(name, w, lhs, sums, j, cols_, R, epi, cost):
        tile, wsum, nt, kp, kl = Wt[w] if isinstance(w, int) else w
        h, S2, c = len(kp), slice(R.start // 2, R.stop // 2), {}
        a_ = lambda i, k: _top(lhs(k) if callable(lhs) else lhs[R, C(k)], i)
        s_ = sums if callable(sums) else (lambda i, p: sums[S2, C(h * i + p)])
        prod = lambda fa_, fb_: [(lambda p=p: (fa_(p), fb_(p))) for p in range(h)]
        left = lambda i, n: [(lambda k=k: (a_(i, k), tile(k, n))) for k in kl]
        mk = lambda tiles, f, x=0: Unit(name, tiles, lambda p: f(p[0]), 64, 8 * len(tiles), nt=nt, acc=True, tail=x)

        def e1(m):
            u7.res, u6.res = [m], [m]

        def e4(m):
            c[11], c[21] = c[11] + m, m

        def e2(m):
            c[21], c[22] = c[21] + m, c[22] - m
            l21.res = [c[21]]

        def e5(m):
            c[12] = m
            epi(cols_[0], R, _zip(c[11] - m, c[21]))

        def e3(m):
            l12.res, c[22] = [c[12] + m], c[22] + m
            if not kl:
                l12.epi(l12.res)
        u1 = mk(prod(lambda p: s_(0, p), lambda p: wsum(0, p, j)), e1)
        u7 = mk(prod(lambda p: s_(4, p), lambda p: wsum(4, p, j)) + left(0, cols_[0]), lambda m: c.update({11: m}))
        u6 = mk(prod(lambda p: s_(3, p), lambda p: wsum(3, p, j)) + left(1, cols_[1]), lambda m: c.update({22: m}))
        u4 = mk(prod(lambda p: a_(1, kp[p][1]), lambda p: wsum(2, p, j)), e4)
        u2 = mk(prod(lambda p: s_(1, p), lambda p: tile(kp[p][0], cols_[0])), e2, 8)
        l21 = mk(left(1, cols_[0]), lambda m: c.update({21: m}))
        u5 = mk(prod(lambda p: s_(2, p), lambda p: tile(kp[p][1], cols_[1])), e5, 16 * cost(cols_[0]))
        u3 = mk(prod(lambda p: a_(0, kp[p][0]), lambda p: wsum(1, p, j)), e3, 8 if kl else 8 + 16 * cost(cols_[1]))
        l12 = mk(left(0, cols_[1]), lambda m: epi(cols_[1], R, _zip(m, c[22])), 16 * cost(cols_[1]))
        return [u1, u7, u6, u4, u2, l21, u5, u3, l12]

    LH, RH = [0, 4, 3, (1, 1), 1, 2, (0, 0)], [0, 4, 3, 2, (0, 0), (1, 1), 1]
    L2 = {3: (w3n_w, ws_w[2], w3t, KF[:6], n2t), 4: (w4_w, ws_w[3], w4t, ND, a_t)}

    def wsums2(w):
        w_w, s_w, ws2, cp_, _ = L2[w]
        kp, nj = Wt[w][3], len(cp_)

        def mk(o, p2, j2, r):
            def load(u, v):
                p, j, y = 2 * p2 + u, 2 * j2 + v, RH[o]
                if isinstance(y, int):
                    return s_w[pl.ds(64 * p + r // 2, 8), C(nj * y + j)]
                return w_w[pl.ds(64 * kp[p][y[0]] + r // 2, 8), C(cp_[j][y[1]])]

            def store(m, x):
                ws2[pl.ds(128 * p2 + r, 16), C((5 * o + m) * (nj // 2) + j2)] = x
            return sums_task(load, store, False)
        return [mk(o, p2, j2, r) for j2 in range(nj // 2) for o in range(7) for p2 in range(len(kp) // 2)
                for r in range(0, 128, 16)]

    def wsums4():
        form = [((0, 0), (1, 1), 1), ((0, 1), (1, 1), -1), ((1, 0), (0, 0), -1), ((0, 0), (0, 1), 1), ((1, 0), (1, 1), 1)]

        def mk(o, p2, r):
            def fn(a):
                def blk(p, j, uv, t):
                    x = w4_w[pl.ds(64 * KF[p][uv[0]] + r // 2, 8), C(ND[j][uv[1]])]
                    return pltpu.bitcast(_tie(x, t), BF16).astype(F32)
                y = {}
                for u in range(2):
                    for j in range(2):
                        p = 2 * p2 + u
                        if isinstance(RH[o], int):
                            f = form[RH[o]]
                            x1, x2 = blk(p, j, f[0], a), blk(p, j, f[1], None)
                            y[u, j] = x1 + x2 if f[2] > 0 else x1 - x2
                            w4s[pl.ds(128 * p + r, 16), C(2 * RH[o] + j)] = y[u, j].astype(BF16)
                        else:
                            y[u, j] = blk(p, j, RH[o], a if u == j else None)
                for m, f in enumerate(form):
                    x = y[f[0]] + y[f[1]] if f[2] > 0 else y[f[0]] - y[f[1]]
                    w4t[pl.ds(128 * p2 + r, 16), C(5 * o + m)] = x.astype(BF16)
            return fn
        last = wsums(w4_w, w4s, KF, ND)
        return (last[48:56] + last[104:112]
                + [mk(o, p2, r) for o in range(7) for p2 in range(3) for r in range(0, 128, 16)])

    def lsums2(w, lhs_w, sums_w, sl):
        kp, xs2 = Wt[w][3], L2[w][4]
        h2 = len(kp) // 2

        def mk(o, p2, g):
            def load(u, v):
                p, ch, x = 2 * p2 + v, 2 * g + u, LH[o]
                if isinstance(x, int):
                    return sums_w[pl.ds(64 * sl + 8 * ch, 8), C(len(kp) * x + p)]
                return lhs_w[pl.ds(H * sl + 16 * ch + 8 * x[0], 8), C(kp[p][x[1]])]

            def store(m, x):
                xs2[pl.ds(16 * g, 16), C((5 * o + m) * h2 + p2)] = x
            return sums_task(load, store, True)
        return [[mk(o, p2, g) for o in range(7) for g in range(4)] for p2 in range(h2)]

    def quad2(name, w, lhs, sums, j2, epi, cost):
        tile, wsum, nt, kp, kl = Wt[w]
        ws2, cp_, xs2 = L2[w][2:]
        h, h2, nj2, c, R = len(kp), len(kp) // 2, len(cp_) // 2, {}, slice(0, T)

        def done(j, v):
            val = _zip(c[j, 1, v], c[j, 2, v])
            if not kl:
                return epi(cp_[j][v], R, val)
            c[j, v] = val

        def upd(o, j, m):
            for i, v, sg in (((1, 0, 1), (2, 1, 1)), ((1, 0, 1),), ((2, 1, 1),), ((1, 0, 1), (2, 0, 1)),
                             ((2, 0, 1), (2, 1, -1)), ((1, 0, -1), (1, 1, 1)), ((1, 1, 1), (2, 1, 1)))[o]:
                k = (j, i, v)
                c[k] = m if k not in c else (c[k] + m if sg > 0 else c[k] - m)
            if o >= 5:
                done(j, o - 5)

        def inner(o):
            x, y = LH[o], RH[o]
            xo = ((lambda p: sums[:, C(h * x + p)]) if isinstance(x, int)
                  else (lambda p: _top(lhs[:, C(kp[p][x[1]])], x[0])))
            yo = ((lambda p, j: wsum(y, p, j)) if isinstance(y, int)
                  else (lambda p, j: tile(kp[p][y[0]], cp_[j][y[1]])))
            w_ = (yo, lambda m, p2, _: ws2[C(p2), C((5 * o + m) * nj2 + j2)], nt,
                  [(2 * i, 2 * i + 1) for i in range(h2)], list(range(2 * h2, h)))
            return quad(name, w_, xo, lambda m, p2: xs2[:, C((5 * o + m) * h2 + p2)], 0, (2 * j2, 2 * j2 + 1),
                        HS[0], lambda j, _, m: upd(o, j, m), lambda j: 1.5 + KS + (2 * cost(0) if o >= 5 and not kl else 0))

        def rest(j, v, Q):
            return [Unit(name, [lambda: (lhs[Q, C(k)], tile(k, cp_[j][v]))],
                         lambda p: epi(cp_[j][v], Q, p[0] + c[j, v][Q]), 64, 8 * (cost(cp_[j][v]) + 1)) for k in kl]
        return cat(inner(o) for o in range(7)), [u for Q in QS for j in (2 * j2, 2 * j2 + 1) for v in range(2)
                                                 for u in rest(j, v, Q)]

    def mm(name, w, lhs, sums, epi, cost):
        if sums is None:
            return [[plain(name, w, lhs, n, R, epi, cost) for R in HS] for n in range(NT)]
        return [[plain(name, w, lhs, 0, R, epi, cost) for R in QS]] + [
            [u for R in HS for u in quad(name, w, lhs, sums, j, ND[j], R, epi, cost)] for j in range(2)]

    def mm1(name, hs, sl, fast=False):
        def epi(n, R, p):
            h1_v[n, pl.ds(hs * T + 8 + R.start, R.stop - R.start), :] = _gelu2(p)
        return cat(mm(name, 1, view(n1_v, sl), n1s if fast else None, epi, lambda n: 5 + KS))

    def mm2(name, sl, xs, x1s, fast=False):
        def epi(n, R, p):
            view(x1_v, x1s)[R, C(n)] = view(hb_v, xs)[R, C(n)] + p
        return cat(mm(name, 2, view(g_v, sl), gs if fast else None, epi, lambda n: 1 + KS))

    def mm3(name, sl, fast=True, deep=False):
        nn, aa, ss, keep, tail = view(n2_v, sl), view(a_v, sl), view(a_s, sl, H), {}, []

        def epi(n, R, p):
            g = _gelu2(p)
            aa[R, C(n)] = g.astype(BF16)
            if not fast:
                return
            if n % 2 == 0 and n < 12:
                keep[n] = g
                return
            pair = (keep.pop(n - 1), g) if n % 2 else (g, tail[R.start // 128][R.start % 128:R.start % 128 + 64])
            sm = _lhs_sums(*pair)
            for i, x in enumerate(sm):
                ss[R.start // 2:R.stop // 2, C(7 * i + n // 2)] = x.astype(BF16)
            if deep and n < 12:
                xo = [sm[x] if isinstance(x, int) else _top(pair[x[1]], x[0]) for x in LH]
                if n % 4 == 1:
                    keep[n, R.start] = xo
                    return
                for o, x in enumerate(zip(keep.pop((n - 2, R.start)), xo)):
                    for m, y in enumerate(_lhs_sums(*x)):
                        a_t[R.start // 4:R.stop // 4, C((5 * o + m) * 3 + n // 4)] = y.astype(BF16)

        c3 = lambda n: 5.5 + 0.5 * KS + (3.75 + 1.25 * KS if fast and (n % 2 or n == 12) else 0)

        def rem(R):
            def f(p):
                tail.append(jnp.concatenate([_gelu2(p[0]), jnp.zeros((64, 128), F32)], axis=0).T)
                aa[R, C(13)] = tail[-1].astype(BF16)
            return Unit(name, [(lambda k=k: (w3_v[13 * 128:F, C(k)], nn[R, C(k)])) for k in range(NT)], f, 64, 84,
                        nt=True, acc=True)
        odd = [rem(R) for R in HS] + [plain(name, 3 if fast else 0, nn, 12, R, epi, c3) for R in QS]
        if fast == 2:
            qd = [quad2(name + "_%d" % j, 3, nn, view(n2s, sl, H), j, epi, c3) for j in range(3)]
            return odd[:2] + qd[0][0] + _weave(qd[1][0], qd[0][1]) + _weave(qd[2][0], qd[1][1]) + _weave(odd[2:], qd[2][1])
        if fast:
            qd = [[u for j in range(6) for u in quad(name + ("b%d" % (j // 2) if i else "a"), 3, nn, view(n2s, sl, H), j,
                                                     KF[j], R, epi, c3)] for i, R in enumerate(HS)]
            return qd[0] + qd[1][:36] + odd[:2] + qd[1][36:] + odd[2:]
        return odd + [plain(name, 0, nn, n, R, epi, c3) for p in KF[:6] for R in HS for n in p]

    def cp_out(j, osl, L, sm, R=slice(0, T)):
        return cp(o_v.at[pl.ds(osl * T + R.start, R.stop - R.start), L],
                  o_hbm.at[pl.ds(base(j, T) + R.start, R.stop - R.start), L], sem_o.at[sm])

    out_a = lambda j: cp_out(j, 0, slice(128, D), 0)
    out_b = lambda j: cp_out(j, 0, C(0), 1)
    last = []

    def mm4(name, j, sl, osl=0, xs=None, x1s=None, fast=True):
        oo = view(o_v, osl)

        def epi(n, R, p):
            if xs is None:
                oo[R, C(n)] = (r_v[R, C(n)] + mod_v[2, 0:1, C(n)] * p).astype(BF16)
            else:
                oo[R, C(n)] = (view(x_v, xs)[R, C(n)] + mod_v[2, 0:1, C(n)]
                               * (view(x1_v, x1s)[R, C(n)] + p)).astype(BF16)
            if osl == 2:
                last.append(cp_out(j, osl, C(n), 2, R))
                last[-1].start()
            elif R.stop == T and osl and n == NT - 1:
                last.append(cp_out(j, osl, slice(128 if osl == 3 else 0, D), 2))
                last[-1].start()
            elif R.stop == T and osl == 0 and n in (0, NT - 1):
                (out_a if n else out_b)(j).start()
        c4 = lambda n: (3 if xs is None else 4) + KS
        if fast == 2:
            return ([plain(name, 4, view(a_v, sl), 0, R, epi, c4) for R in QS],
                    quad2(name + "q", 4, view(a_v, sl), view(a_s, sl, H), 0, epi, c4)[0])
        return mm(name, 4, view(a_v, sl), view(a_s, sl, H) if fast else None, epi, c4)

    def split(us):
        n = 4 // len(us)
        m, mks, st = us[0].rows // n, [u.tiles.pop(0) for u in us], {}

        def piece(i, k):
            if i not in st:
                st[i] = mks[i]()
            return st[i][0][m * k:m * (k + 1)], st[i][1]

        def epi(p):
            for i, u in enumerate(us):
                u.res = [jnp.concatenate(p[n * i:n * (i + 1)], axis=0)]
        return _flat([Unit(us[0].name, [(lambda i=i, k=k: piece(i, k)) for i in range(len(us)) for k in range(n)],
                           epi, m, 0, nt=us[0].nt)])

    W = lambda nm: [("wait", nm)]
    run = lambda fns: [("run", "run", lambda: [fn(None) for fn in fns])]
    one = lambda us: [_flat([u]) for u in us]
    nm = lambda x: (lambda n: x)

    seq, grp = [], []
    for s in range(NC):
        seq += W("c%d" % s) + _flat(mmK(s) + mmU(nm("U%d" % s), s % 2, NC - 1 - s))
        grp.append(Group("kv%d" % s, cat(kv(s, s % 2)), 50, ["c%d" % s], ["U%d" % s], 100))
    inv = [mmI(lambda n: "I%d" % n, s, s) for s in range(NC)]
    seq += W("c3") + _flat(mmK(3) + mmK(4) + [inv[s][t] for t in range(NT) for s in range(NC)])
    macs = [mac(s + 1, NC - 1 - s, s) for s in range(NC)]
    grp.append(Group("mac00", macs[0][0], 12, ["c1"], ["c2"], 0))
    grp.append(Group("mac01", macs[1][0] + macs[0][1] + macs[1][1], 16, ["c2"], ["c3"], 0))
    for t in range(NT):
        grp.append(Group("mac%d" % t, cat(macs[s][t] for s in range(2 if t < 2 else 0, NC)), 24 if t < 2 else 18,
                         ["c3", "K%d" % t], ["I%d" % t], 100, 150))
    start = lambda cs: [("run", "run", lambda: [c.start() for c in cs])]
    f0, f1 = front(0, 2, True), front(1, 1, True)
    seq += run(ahead(0))
    seq += W("wma") + _flat(mod("moda", 0, 3)) + run(f0[0] + f1[0] + ahead(1))
    seq += W("wmb") + start(next_kv(NC) + next_q(NC)) + _flat(mod("modb", 3, 5)) + run(f0[1])
    w1 = _flat(mm1("w1_0", 0, 0) + mm1("w1_1", 1, 1))
    seq += W("w1") + w1[:72] + W("w2") + w1[72:] + run(shift(0, 0))
    seq += _flat(mm2("w2_0", 0, 2, 1) + mm1("w1_2", 2, 2)) + run(shift(1, 1)) + _flat(mm2("w2_1", 1, 1, 0))
    grp.append(Group("f1", f1[1], 80, ["w1"], ["w1_1"], 450))
    grp.append(Group("f2", front(2, 0), 80, ["w2"], ["w1_2"], 450))
    grp.append(Group("ln2_0", ln2(1, 0, False), 60, ["w2_0"], ["w3"], 450))
    grp.append(Group("ahead", cat(ahead(i) for i in range(2, NB - NC)), 19 + 2 * KS, ["w1"], ["end"], 100))
    grp.append(Group("ws1", wsums(w1_w, w1s, KD, ND), 26 + 5 * KS, ["w1"], ["end"], 100))
    grp.append(Group("ws2", wsums(w2_w, w2s, KD, ND), 26 + 5 * KS, ["w2"], ["end"], 100))
    grp.append(Group("ws3", w3_turn() + wsums(w3n_w, w3s, KD, KF[:6]) + wsums2(3), 22 + 5.5 * KS, ["w3"], ["end"], 100))
    grp.append(Group("ws4", wsums4(), 40 + 8 * KS, ["w4"], ["end"], 60))
    _wait(seq, "w3", back=1)
    w3 = mm3("w3_0", 0, False, False)
    _mix(seq, _flat(w3[6:]), [split(w3[4:6]) + _flat(w3[:6])], 0.1)
    mc = mod("modc", 5, 6)
    mc = _flat(mc[1:] + mc[:1])
    _wait(seq, "w4", mc[:5] + [("sync", "run", lambda: None)])
    w4 = cat(mm4("w4_0", 0, 0, 3, 2, 1, False)[1:])
    qs = [split([w4[-1 - i]]) for i in range(_phase(seq))]
    _mix(seq, _flat(w4), [mc[i:i + 4] for i in range(5, 25, 4)] + qs, 0.01, 0.4)
    assert _phase(seq) == 0
    grp.append(Group("resid", resid(2, 1), 26 + 5 * KS, ["modc"], ["end"], 100))
    grp.append(Group("ln2a", *ln2_late(1), ["w3_0"], ["end"], 100))
    _emit(seq, grp, zero, wait)

    def step(s, carry):
        for c in next_kv(s) + next_q(s):
            c.wait()
        nxt = jnp.minimum(s + 1, NB - 1)
        seq, grp = [], []
        us, it = one(mmU(lambda n: "U%d" % n, 0, 0)), one(mmI(lambda n: "I%d" % n, 0, 0))
        w4, w4c = mm4("w4", s - 2, 0, fast=2)[1], mm4("w4c", s - 3, 0, fast=2)[0]
        w2 = mm2("w2", 0, 1, 0, True)
        q = split(w2[3:4])
        _mix(seq, _flat(w4c + mm3("w3", 0)),
             [us[0], us[1], us[2], it[0] + us[3], it[1] + us[4], it[2] + start(next_kv(nxt)), it[3], it[4]],
             E("LP3", 0.15), E("LP0", 0.62))
        w1a, w1b = mm1("w1a", 2, 0, True), mm1("w1b", 2, 0, True)
        w1a, w1b = _flat(w1a[0:2] + w1a[4:13] + w1a[22:31]), _flat(w1b[2:4] + w1b[13:22] + w1b[31:])
        w2 = w2[0:3] + w2[4:13] + w2[22:31] + w2[3:4] + w2[13:22] + w2[31:]
        for u in w2[:21]:
            u.name = "w2a"
        kw = 9 * E("KW", 6)
        if E("ORD", 1):
            seq += _flat(w2[:21] + w4[:kw]) + w1a[:8] + start(next_q(nxt)) + w1a[8:] + run(shift(1, 0, ((T - 32, 32),), gs))
            _mix(seq, _flat(w4[kw:]), [q], 0.6)
            seq += _flat(w2[21:]) + w1b
        else:
            seq += _flat(w4) + w1a[:8] + start(next_q(nxt)) + w1a[8:] + run(shift(1, 0, ((T - 32, 32),), gs))
            _mix(seq, _flat(w2), [q], 0.3)
            seq += w1b
        assert _phase(seq) == 0
        kvs, macs = kv(0, 0), mac(1, 0, 0, part=True)
        for t in range(NT):
            grp.append(Group("kv%d" % t, kvs[t], 50 + 2 * KS, ["start"], ["U%d" % t], 300))
            grp.append(Group("mac%d" % t, macs[t], 24 + 2 * KS, ["U%d" % t], ["I%d" % t], 300, 150))
        iall = ["I%d" % t for t in range(NT)]
        ln = ln2(0, 0)
        grp.append(Group("ln2a", *ln2_late(E("LM", 1)), ["w2a", E("LR", "w2")], ["end"], E("LL", 100)))
        grp.append(Group("ln2b", ln[4:8] + ln[12:16], 78 + 20 * KS, ["start"], ["w3b0"], 450))
        grp.append(Group("resid", resid(1, 0, True), 26 + 30 * KS, ["w4c"], ["w2a", "w4q", "I4"], 100))
        xa = lsums2(4, a_w, as_w[3], 0)
        grp.append(Group("xa", [f for x in xa for i, f in enumerate(x) if i % 4 < 2], 26 + 5 * KS, ["w3a"], ["w4q"], 150))
        for p in range(3):
            grp.append(Group("xb%d" % p, [f for i, f in enumerate(xa[p]) if i % 4 >= 2], 26 + 5 * KS, ["w3b%d" % p], ["w4q"], 150, 100))
        fr = front(0, 0, ss=n1s)
        grp.append(Group("fronta", fr[0], 50 + 8 * KS, iall, ["w1a"], E("FL", 230)))
        grp.append(Group("frontb", fr[1], 48 + 7 * KS, iall, ["w1b"], E("FL", 230), E("RL", 4000)))
        grp.append(Group("fqb", fr[3], 26 + 12 * KS, iall, ["w1a"], E("QL", 300), E("RL", 4000) - 500))
        grp.append(Group("fq", fr[2], 33 + 7 * KS, ["w4c"], ["I4"], 100))
        grp.append(Group("spread", spread(), 30 + 8 * KS, iall, ["end"], 100))
        grp.append(Group("shift", shift_early(), 22 + 7 * KS, ["start"], ["w1a", "w2a"], 200))
        _emit(seq, grp, zero, wait)
        out_b(s - 3).wait()
        out_a(s - 2).wait()
        return carry

    lax.fori_loop(NC, NB, step, 0)

    seq, grp = [], []
    w47 = mm4("w4_7", NB - 1, 1, 2, 0, 1, 2)
    seq += _flat(mm4("w4_5", NB - 3, 0, fast=2)[0] + mm2("w2_7", 0, 0, 1, True) + mm3("w3_6", 0, 2)
                 + cat(mm4("w4_6", NB - 2, 0, 1, 1, 0, 2)) + mm3("w3_7", 1, 2) + w47[0][:3] + w47[1] + w47[0][3:])
    grp.append(Group("shift7", shift(2, 0, [(r, 32) for r in range(0, T, 32)], gs), 24, ["start"], ["w2_7"], 200))
    ln = ln2(0, 0)
    grp.append(Group("ln2_6", ln[4:8] + ln[12:16], 75, ["start"], ["w3_6"], 1200))
    grp.append(Group("xn6", cat(lsums2(3, n2_w, as_w[2], 0)), 26 + 5 * KS, ["w4_5"], ["w3_6_0"], 200, 800))
    grp.append(Group("ln2_7", ln2(1, 1), 75, ["w4_6"], ["w3_7"], 1500))
    grp.append(Group("xn7", cat(lsums2(3, n2_w, as_w[2], 1)), 26 + 5 * KS, ["w4_6"], ["w3_7_0"], 200, 2100))
    for j in (6, 7):
        for p, ts in enumerate(lsums2(4, a_w, as_w[3], j - 6)):
            grp.append(Group("xa%d_%d" % (j, p), ts, 26 + 5 * KS, ["w3_%d_%d" % (j, p)], ["w4_%dq" % j], 200, 150))
    _emit(seq, grp, zero, wait)
    for c in next_kv(NB - 1) + next_q(NB - 1) + [out_b(NB - 3)] + last:
        c.wait()


@jax.jit
def pallas_adaLN_cond__ssm_conv_h3__mixer_s_mlp__prompt_kernel(
        A_q, A_k, A_v, A_shift_k, A_ssm_k, A_ssm_D, B_x, B_w1, B_w2, B_w3, B_w4, c, w_mod):
    any_ = pl.BlockSpec(memory_space=pl.ANY)
    V = pltpu.VMEM
    out = pl.pallas_call(
        kernel,
        in_specs=[any_] * 12,
        out_specs=any_,
        out_shape=jax.ShapeDtypeStruct((S, D), BF16),
        scratch_shapes=[
            [V((NT, H + 8, 128), U32)] * NC, [V((NT, H + 8, 128), U32)] * NC, [V((NT, H + 8, 128), U32)] * NC,
            [V((64, S), U32)] * NT,
            V((D // 2, D), U32), V((D // 2, D), U32), V((F // 2, D), U32), V((FT * 64, D), U32),
            [V((D // 2, 3 * D), U32), V((D // 2, 2 * D), U32), V((D // 2, D), U32)], V((4 * T, D), BF16),
            V((4, D), BF16), V((D,), BF16), V((1, D), BF16), V((8, 128), I32), pltpu.SMEM((8, 128), I32),
            V((5, 8, D), F32), V((6, 8, D), F32), V((T // 2, 4 * H), U32), V((GR // 2, 2 * T), U32),
            V((NB, 3 * T + 8, D), F32), V((NC, 3 * T + 8, D), F32), V((NB - NC, 2 * T + 8, D), F32), V((4 * T, 128), F32),
            V((T, D), U32), V((NC * T, D), U32), V((NT, NC * (T + 8) + 16, 128), F32),
            V((3 * T, D), F32), V((3 * T, D), F32), V((2 * T, D), F32), V((T, D), F32),
            V((3 * T // 2, D), U32), V((T, D), U32), V((T, D), U32), V((NT, NC * T + 24, 128), F32),
            V((T, (FT + 1) * 128), U32),
            [V((128, 11 * 128), U32)] * 2 + [V((128, 31 * 128), U32), V((448, 11 * 128), U32)],
            [V((64, 11 * 128), U32)] * 2 + [V((128, 11 * 128), U32), V((128, 35 * 128), U32)],
            V((D // 2, 13 * 128), U32), V((H, D), F32), V((T, 9 * 128), F32),
            [V((64, 105 * 128), U32), V((192, 35 * 128), U32), V((32, 35 * 128), U32), V((32, 105 * 128), U32)],
            pltpu.SemaphoreType.DMA((11,)), pltpu.SemaphoreType.DMA((1,)), pltpu.SemaphoreType.DMA((3,)),
        ],
        compiler_params=pltpu.CompilerParams(vmem_limit_bytes=110 << 20, disable_semaphore_checks=True,
                                             disable_bounds_checks=True),
        name="fused",
    )(A_q[0], A_k[0], A_v[0], A_shift_k.T, A_ssm_k, A_ssm_D, B_w1, B_w2, B_w3.T, B_w4, c, w_mod)
    return out[None]
```

```python
import heapq
import os
import numpy as np
import jax
import jax.numpy as jnp
from jax import lax
from jax.experimental import pallas as pl
from jax.experimental.pallas import tpu as pltpu

S, D, F = 2048, 640, 1728
T = 256
H = T // 2
NB = S // T
NT = D // 128
FT = (F + 127) // 128
EPS = 1e-5
F32, BF16, U32, I32 = jnp.float32, jnp.bfloat16, jnp.uint32, jnp.int32
G_C1 = 0.044715 * float(np.sqrt(2.0 / np.pi))
G_C2 = float(np.sqrt(2.0 / np.pi))
G_A = G_C1 ** (1.0 / 3.0)
G_B = G_C2 / G_A
G_POST = 0.5 / G_A
RG = 16
GR = 80
NC = 3
DL = int(os.environ.get('DL', 450))
E = lambda k, d: type(d)(os.environ.get(k, d))
KS = E('KS', 1.5)
SLOT = E('SLOT', 32)


def _dft(shape, f_axis, tau, scale=1.0):
    r = lax.broadcasted_iota(I32, shape, f_axis)
    l = lax.broadcasted_iota(I32, shape, 1 - f_axis)
    f = r & 127
    odd = ((f & 63) << 2) | ((f >> 6) << 1) | 1
    p = odd * tau(l) + ((r >> 7) << 8)
    a = ((p + 512) & 1023) - 512
    u = (256 - jnp.abs(a)).astype(F32) * (np.pi / 512.0)
    u2 = u * u
    c = [scale, -scale / 6.0, scale / 120.0, -scale / 5040.0, scale / 362880.0, -scale / 39916800.0]
    poly = c[5]
    for ci in c[4::-1]:
        poly = poly * u2 + ci
    return (u * poly).astype(BF16)


def _rstd(xc, mlp):
    s2, eps = (1.0 / (G_A * G_A), EPS / (G_POST * G_POST)) if mlp else (1.0, EPS)
    v = jnp.sum(xc * xc, axis=-1, keepdims=True) * (s2 / D) + eps * s2
    return jnp.exp2(jnp.log(v) * float(-0.5 / np.log(2.0)))


def _ln(x, mlp=False):
    xc = x - jnp.sum(x, axis=-1, keepdims=True) * (1.0 / D)
    return xc * _rstd(xc, mlp)


def _gelu2(x):
    u = x * (x * x + G_B)
    return x * (1.0 + jnp.tanh(u))


def _lo(w):
    return pltpu.bitcast(w << 16, F32)


def _hi(w):
    return pltpu.bitcast(w & jnp.uint32(0xFFFF0000), F32)


def _tie(x, a):
    if a is None:
        return x
    w = pltpu.bitcast(x[:, :128], U32)
    k = w.shape[0] // 8
    w = w | (a if k == 1 else jnp.concatenate([a] * k, axis=0))
    w = pltpu.bitcast(w, x.dtype)
    return w if x.shape[1] == 128 else jnp.concatenate([w, x[:, 128:]], axis=1)


def _top(x, i):
    return jnp.concatenate([x[r:r + 16] for r in range(16 * i, x.shape[0], 32)], axis=0)


def _zip(t, b):
    return jnp.concatenate([x[r:r + 16] for r in range(0, t.shape[0], 16) for x in (t, b)], axis=0)


def _lhs_sums(x1, x2):
    a11, a21, a12, a22 = _top(x1, 0), _top(x1, 1), _top(x2, 0), _top(x2, 1)
    return [a11 + a22, a21 + a22, a11 + a12, a21 - a11, a12 - a22]


def C(i):
    return slice(i * 128, (i + 1) * 128)


class Unit:
    def __init__(self, name, tiles, epi, rows, cost, nt=False, full=True, acc=False, tail=0):
        self.tail = tail
        self.acc, self.res = acc, []
        self.name, self.tiles, self.epi, self.rows, self.cost, self.nt, self.full = name, tiles, epi, rows, cost, nt, full


class Due:
    def __init__(self, val, delay):
        self.val, self.delay = val, delay


class Group:
    def __init__(self, name, fns, cost, rel, dead, lat, rlat=200):
        self.name, self.fns, self.cost, self.rel, self.dead, self.lat, self.rlat = name, fns, cost, rel, dead, lat, rlat


def _plan(seq, groups):
    busy, n = [0] * 4, 0
    start, end, tiles, bars = {}, {}, [], []
    for it in seq:
        if isinstance(it[0], Unit):
            u = it[0]
            m = n % 4
            n += 1
            t0, t1 = busy[m], busy[m] + max(u.rows, 32)
            busy[m] = t1
            tiles.append((t0, t1, u.cost / len(u.tiles) + (u.tail if it[1] == len(u.tiles) - 1 else 0)))
            start.setdefault(u.name, t0)
            end[u.name] = max(end.get(u.name, 0), t1)
        elif it[0] == "wait":
            t = max(busy)
            busy, n = [t] * 4, 0
            start[it[1]] = end[it[1]] = t
            bars.append(t)
    total = max(busy)
    start["end"] = end["end"] = total
    start["start"] = end["start"] = 0
    ns = total // SLOT + 2
    load = np.zeros(ns)
    for t0, t1, c in tiles:
        a, b = t0 // SLOT, max(t1 // SLOT, t0 // SLOT + 1)
        load[a:b] += c / (b - a)
    win = []
    for g in groups:
        r = max(end[x] + (0 if start[x] == end[x] else g.rlat) for x in g.rel)
        d = min(start[x] for x in g.dead) - g.lat
        ok = np.zeros(ns, bool)
        ok[r // SLOT:max(d // SLOT, r // SLOT + 1)] = True
        for b in bars:
            if r < b <= d:
                ok[max((b - g.lat) // SLOT, 0):b // SLOT] = False
        win.append(np.nonzero(ok)[0])
    alloc = [np.zeros(len(w)) for w in win]
    for _ in range(60):
        for i, g in enumerate(groups):
            w = win[i]
            load[w] -= alloc[i]
            base = load[w]
            vol = g.cost * len(g.fns)
            lo, hi = base.min(), base.max() + vol
            for _ in range(50):
                mid = 0.5 * (lo + hi)
                if np.maximum(mid - base, 0).sum() > vol:
                    hi = mid
                else:
                    lo = mid
            ev = E('EV', 0.0) if g.name in ('fronta', 'frontb', 'fq', 'fqb') else 0.0
            alloc[i] = np.maximum(hi - base, 0) * (1 - ev) + ev * vol / len(w)
            load[w] += alloc[i]
    times = []
    for i, g in enumerate(groups):
        cum = np.cumsum(alloc[i])
        ts = []
        for k in range(len(g.fns)):
            x = (k + 0.5) * cum[-1] / len(g.fns)
            j = int(np.searchsorted(cum, x))
            prev = cum[j - 1] if j else 0.0
            ts.append(win[i][j] * SLOT + SLOT * (x - prev) / max(alloc[i][j], 1e-9))
        times.append(ts)
    return times


def _emit(seq, groups, zero, wait):
    times = _plan(seq, groups)
    left = {"start": 0}
    for it in seq:
        nm = it[0].name if isinstance(it[0], Unit) else it[1]
        left[nm] = left.get(nm, 0) + 1
    heap, pend, todo, cnt = [], {}, list(range(len(groups))), 0
    busy, n, due = [0] * 4, 0, []

    def release():
        nonlocal cnt
        for i in list(todo):
            g = groups[i]
            if all(left[x] == 0 for x in g.rel):
                todo.remove(i)
                pend[i] = len(g.fns)
                for t, fn in zip(times[i], g.fns):
                    heapq.heappush(heap, (t, cnt, i, fn))
                    cnt += 1

    def force(name):
        nonlocal heap
        for i, g in enumerate(groups):
            if name in g.dead:
                assert i not in todo, (g.name, name)
                if pend[i]:
                    for it in sorted(x for x in heap if x[2] == i):
                        it[3](None)
                    heap = [x for x in heap if x[2] != i]
                    heapq.heapify(heap)
                    pend[i] = 0

    release()
    for it in seq:
        if isinstance(it[0], Unit):
            u, k = it
            force(u.name)
            lhs, rhs = u.tiles[k]()
            t0 = busy[n % 4]
            while u.full and due and due[0][0] < t0 + u.rows:
                t, x = due.pop(0)
                r = min(max(int(t - t0), 0), u.rows - 1) // 16 * 8
                w = pltpu.bitcast(lhs, U32)
                x = pltpu.bitcast(x[:, :128], U32)
                parts = [w[:r], w[r:r + 8] | ((x[0:8] | x[8:16]) & zero), w[r + 8:]]
                lhs = pltpu.bitcast(jnp.concatenate([y for y in parts if y.shape[0]], axis=0), BF16)
            dn = (((1,), (1 if u.nt else 0,)), ((), ()))
            p = lax.dot_general(lhs, rhs, dn, preferred_element_type=F32)
            u.res = [p + u.res[0]] if (u.acc and u.res) else u.res + [p]
            m = n % 4
            n += 1
            t0 = busy[m]
            busy[m] = t0 + max(u.rows, 32)
            while u.full and heap and heap[0][0] < t0 + u.rows:
                t, _, i, fn = heapq.heappop(heap)
                pend[i] -= 1
                r = min(max(int(t - t0), 0), u.rows - 1) // 8 * 8
                x = fn(pltpu.bitcast(p[r:r + 8], U32) & zero)
                if isinstance(x, Due):
                    due.append((t + x.delay, x.val))
                    due.sort(key=lambda e: e[0])
            if k == len(u.tiles) - 1:
                u.epi(u.res)
            left[u.name] -= 1
        elif it[0] == "wait":
            force(it[1])
            wait(it[1])
            busy, n, due = [max(busy)] * 4, 0, []
            left[it[1]] -= 1
        else:
            it[2]()
            left[it[1]] -= 1
        release()
    force("end")
    assert not heap and not todo


def _sum(ps):
    acc = ps[0]
    for p in ps[1:]:
        acc = acc + p
    return acc


def _flat(us):
    return [(u, i) for u in us for i in range(len(u.tiles))]


def _weave(a, b):
    out = []
    for i, u in enumerate(a):
        out += [u] + b[i * len(b) // len(a):(i + 1) * len(b) // len(a)]
    return out


def _phase(seq):
    n = 0
    for it in seq:
        n = n + 1 if isinstance(it[0], Unit) else (0 if it[0] in ("wait", "sync") else n)
    return n % 4


def _mix(seq, a, b, lo=0.0, hi=1.0):
    n, k = _phase(seq), 0
    for i, t in enumerate(a):
        if k < len(b) and n % 4 == 0 and t[1] != 1 and i >= len(a) * (lo + (hi - lo) * k / len(b)):
            seq.extend(b[k])
            k += 1
        seq.append(t)
        n += 1
    assert k == len(b)


def _wait(seq, name, head=(), back=0):
    r = _phase(seq) + 4 * back
    assert all(isinstance(it[0], Unit) for it in seq[len(seq) - r:])
    seq[len(seq) - r:len(seq) - r] = [("wait", name)] + list(head)


def kernel(q_hbm, k_hbm, v_hbm, sh_hbm, ssm_hbm, sd_hbm, w1_hbm, w2_hbm, w3_hbm, w4_hbm, c_hbm, wm_hbm,
           o_hbm,
           q_n, k_n, v_n, ssm_w, w1_w, w2_w, w3_w, w4_w, wm_w, o_v,
           sh_v, sd_v, c_v, zsrc, z_s, taps, mod_v, tf_w, tg_w,
           kf, uf, acc, zraw, kv_w, zz_w, y_v, x_v, hb_v, x1_v, r_v, n1_w, n2_w, g_w, h1_v, a_w,
           ws_w, as_w, w3n_w, top_v, st_v, l2_w,
           sem, sem_b, sem_o):
    bf = lambda r: r.bitcast(BF16)
    w1_v, w2_v, w3_v, w4_v = bf(w1_w), bf(w2_w), bf(w3_w), bf(w4_w)
    wm_v = {0: bf(wm_w[0]), 3: bf(wm_w[1]), 5: bf(wm_w[2])}
    tf_v, tg_v, n1_v, n2_v, g_v = bf(tf_w), bf(tg_w), bf(n1_w), bf(n2_w), bf(g_w)
    a_v, kv_v, zz_v = bf(a_w), bf(kv_w), bf(zz_w)
    w1s, w2s, w3s, w4s = [bf(r) for r in ws_w]
    n1s, gs, n2s, a_s = [bf(r) for r in as_w]
    w3n = bf(w3n_w)
    w3t, w4t, n2t, a_t = [bf(r) for r in l2_w]
    cp = pltpu.make_async_copy
    cat = lambda ls: [x for l in ls for x in l]

    def base(j, n):
        return j * n if isinstance(j, int) else pl.multiple_of(j * n, n)

    def rows(j, n=1, size=T):
        return pl.ds(base(j, size), n * size)

    def view(ref, j, size=T):
        return ref.at[rows(j, 1, size)]

    dmas = {}

    def group(name, *mks):
        sm = sem.at[len(dmas)]
        dmas[name] = [c for mk in mks for c in mk(sm)]

    def ssm_in(t):
        return lambda sm: [cp(ssm_hbm.at[C(t)], bf(ssm_w[t]), sm)]

    def cols(src, start, n, dst, row=0):
        return lambda sm: [cp(src.at[pl.ds(start, n), C(t)], bf(dst).at[t, pl.ds(row, n)], sm) for t in range(NT)]

    def kv_in(s, sl):
        if isinstance(s, int):
            kk = cols(k_hbm, s * T - 16, T + 16, k_n[sl]) if s else cols(k_hbm, 0, T, k_n[sl], 16)
        else:
            kk = cols(k_hbm, pl.multiple_of(s * T - 16, 16), T + 16, k_n[sl])
        return lambda sm: kk(sm) + cols(v_hbm, base(s, T), T, v_n[sl])(sm)

    def q_in(s, sl):
        return cols(q_hbm, base(s, T), T, q_n[sl])

    def wm_in(a, b):
        return lambda sm: [cp(wm_hbm.at[:, a * D:b * D], wm_v[a], sm)]

    def whole(src, dst):
        return lambda sm: [cp(src, dst, sm)]

    next_kv = lambda s: kv_in(s, 0)(sem_b.at[0])
    next_q = lambda s: q_in(s, 0)(sem_b.at[0])

    zsrc[...] = jnp.zeros((8, 128), I32)
    k_n[0][:, 0:8, :] = jnp.zeros((NT, 8, 128), U32)
    w4_w[F // 2:FT * 64, :] = jnp.zeros((FT * 64 - F // 2, D), U32)
    group("small", lambda sm: [cp(zsrc, z_s, sm), cp(sh_hbm, sh_v, sm), cp(sd_hbm, sd_v, sm), cp(c_hbm, c_v, sm)])
    for s in range(NC):
        group("c%d" % s, ssm_in(s), kv_in(s, s))
    group("c3", ssm_in(3), ssm_in(4))
    group("wma", wm_in(0, 3), q_in(0, 0), q_in(1, 1))
    group("wmb", wm_in(3, 5))
    group("w1", whole(w1_hbm, w1_v))
    group("w2", q_in(2, 2), whole(w2_hbm, w2_v))
    group("w3", whole(w3_hbm, w3_v))
    group("w4", whole(w4_hbm, w4_v.at[0:F]), wm_in(5, 6))
    for g in dmas.values():
        for c in g:
            c.start()

    def wait(name):
        for c in dmas[name]:
            c.wait()

    tau_b = lambda l: H + ((l + (H - 1)) & (H - 1))
    tf_v[:, C(0)] = _dft((T, H), 0, lambda l: jnp.where((l & 1) == 0, l, tau_b(l)), 1.0 / T)
    tf_v[:, C(1)] = _dft((T, H), 0, lambda l: jnp.where((l & 1) == 1, l, tau_b(l)), 1.0 / T)
    tf_v[:, C(2)] = _dft((T, H), 0, lambda l: 2 * l - H)
    tf_v[:, C(3)] = _dft((T, H), 0, lambda l: 2 * l + 1 - H)
    sin0 = lax.broadcasted_iota(I32, (GR, T), 1) >= H
    tg_v[:, 0:T] = _dft((GR, T), 1, lambda l: jnp.where(sin0 & (l == 0), H, 2 * l))
    tg_v[:, T:2 * T] = _dft((GR, T), 1, lambda l: 2 * l + 1)
    h1_v[:, 0:8, :] = jnp.zeros((NT, 8, 128), F32)
    h1_v[:, 8 + NC * T:16 + NC * T, :] = jnp.zeros((NT, 8, 128), F32)

    wait("small")
    z = jnp.clip(z_s[0, 0], 0, 1)
    zero = jnp.full((8, 128), z, I32).astype(U32)
    z8 = pl.multiple_of(z * 8, 8)
    for r in (x_v, hb_v, x1_v, r_v, zraw, n1_w, n2_w, g_w, a_w, kv_w, zz_w, *ws_w, *as_w, w3n_w, top_v, st_v, *l2_w):
        r[pl.ds(z8, 8), 0:128] = jnp.zeros((8, 128), r.dtype)
    for r in (kf, uf, acc, taps, mod_v):
        r[z, 0:8, 0:128] = jnp.zeros((8, 128), r.dtype)
    for r in (tf_w, tg_w):
        r[pl.ds(z8, 8), 0:128] = r[0:8, 0:128]
    sh = sh_v[...].astype(F32)
    for i in range(4):
        taps[i] = jnp.broadcast_to(sh[i:i + 1], (8, D))
    taps[4] = jnp.broadcast_to(sd_v[...].astype(F32).reshape(1, D) * (1.0 / T), (8, D))
    cf = c_v[...].astype(F32)
    silu_c = jnp.broadcast_to((cf / (1.0 + jnp.exp(-cf))).astype(BF16), (16, D))

    def mmK(n):
        def unit(m):
            st = []

            def rhs(i):
                if not st:
                    ev = (lax.broadcasted_iota(I32, (64, 128), 1) & 1) == 0
                    a = ssm_w[n][:, m * T:m * T + H]
                    b = pltpu.roll(ssm_w[n][:, m * T + H:(m + 1) * T], 1, 1)
                    st.extend([pltpu.bitcast(jnp.where(ev, a, b), BF16), pltpu.bitcast(jnp.where(ev, b, a), BF16)])
                return st[i]

            def epi(p):
                er, ei, or_, oi = p
                cur = [er, ei, or_, oi]
                if m:
                    pv = [zraw[C(4 * ((m - 1) % 2) + (q ^ 1)), :] for q in range(4)]
                    pm = lambda x, y, up: jnp.concatenate([x[:64] + y[:64], x[64:] - y[64:]] if up else
                                                          [x[:64] - y[:64], x[64:] + y[64:]], axis=0)
                    er, ei, or_, oi = [pm(cur[q], pv[q], q & 1) for q in range(4)]
                else:
                    er = er + taps[4, 0:1, C(n)]
                if m + 1 < NB:
                    for q in range(4):
                        zraw[C(4 * (m % 2) + q), :] = cur[q]
                for h, (cr, ci) in enumerate(((er + or_, ei + oi), (er - or_, ei - oi))):
                    B = h * 3 * H
                    kf[m, B:B + H, C(n)] = cr
                    kf[m, B + H:B + 2 * H, C(n)] = ci - cr
                    kf[m, B + 2 * H:B + 3 * H, C(n)] = ci + cr
            return Unit("K%d" % n, [(lambda i=i, r=r: (tf_v[r:r + H, C(i)], rhs(i))) for i in range(2) for r in (0, H)],
                        epi, H, 260, nt=True)
        return [unit(m) for m in range(NB)]

    def kv(s, sl):
        def mk(t, w):
            def fn(a):
                ld = lambda o, n: k_n[s][t, pl.ds(8 + w + o, n), :]
                c0 = jnp.concatenate([_tie(ld(0, 8), a), ld(8, 8)], axis=0).reshape(2, 8, 128)
                c1, c2 = ld(-1, 16).reshape(2, 8, 128), ld(-2, 16).reshape(2, 8, 128)
                s0, s1, s2, s3 = (taps[i, :, C(t)] for i in range(4))
                ke, ko, ke1, ko1, ko2 = _lo(c0), _hi(c0), _lo(c1), _hi(c1), _hi(c2)
                wv = v_n[s][t, w:w + 16, :].reshape(2, 8, 128)
                kve = ((s0 * ke + s1 * ko1) + (s2 * ke1 + s3 * ko2)) * _lo(wv)
                kvo = ((s0 * ko + s1 * ke) + (s2 * ko1 + s3 * ke1)) * _hi(wv)
                kv_v[pl.ds(sl * T + w, 16), C(t)] = kve.reshape(16, 128).astype(BF16)
                kv_v[pl.ds(sl * T + H + w, 16), C(t)] = kvo.reshape(16, 128).astype(BF16)
            return fn
        return [[mk(t, w) for w in range(0, H, 16)] for t in range(NT)]

    def mmU(name, sl, us):
        def unit(n):
            def epi(p):
                er, ei, or_, oi = p
                for h, (cr, ci) in enumerate(((er + or_, ei + oi), (er - or_, ei - oi))):
                    B = h * 3 * H
                    uf[us, B:B + H, C(n)] = cr + ci
                    uf[us, B + H:B + 2 * H, C(n)] = cr
                    uf[us, B + 2 * H:B + 3 * H, C(n)] = ci
            return Unit(name(n), [(lambda i=i, r=r: (tf_v[r:r + H, C(2 + i)], kv_v[pl.ds(sl * T + i * H, H), C(n)]))
                                  for i in range(2) for r in (0, H)], epi, H, 96 + 96 * KS)
        return [unit(n) for n in range(NT)]

    def cmul(m0, u0, n, h, row, L, a):
        t = []
        for i in range(3):
            Rw = slice((3 * h + i) * H + row, (3 * h + i) * H + row + 8)
            kk = kf[m0:m0 + n, Rw, L]
            if i == 0 and a is not None:
                k0 = _tie(kk[0], a)[None]
                kk = k0 if n == 1 else jnp.concatenate([k0, kk[1:]], axis=0)
            t.append(jnp.sum(kk * uf[u0:u0 + n, Rw, L], axis=0))
        return t[0] - t[2], t[0] + t[1]

    def AR(h, q, row):
        return slice((2 * h + q) * H + row, (2 * h + q) * H + row + 8)

    def mac(n, u0, sl, part=False):
        def mk(t, rc):
            st, fin = [], []

            def piece(i):
                def fn(a):
                    h, row = i & 1, rc + (i >> 1) * 8
                    zr, zi = cmul(0, u0, n, h, row, C(t), a)
                    if part:
                        zr, zi = zr + acc[0, AR(h, 0, row), C(t)], zi + acc[0, AR(h, 1, row), C(t)]
                    st.append((zr, zi))
                    if h:
                        (pr, pi), (mr, mi) = st[-2:]
                        fin.append([pr + mr, pi + mi, pr - mr, pi - mi])
                    if i == 3:
                        for q in range(4):
                            zz_v[pl.ds(sl * 2 * T + q * H + rc, 16), C(t)] = jnp.concatenate(
                                [fin[0][q], fin[1][q]], axis=0).astype(BF16)
                return fn
            if not part:
                return [piece(i) for i in range(4)]
            both = lambda f, g: (lambda a: (f(a), g(None)))
            return [both(piece(0), piece(1)), both(piece(2), piece(3))]
        return [[fn for rc in range(0, H, 16) for fn in mk(t, rc)] for t in range(NT)]

    def pos():
        return [(t, h, row) for t in range(NT) for row in range(0, H, 8) for h in range(2)]

    def ahead(i):
        def mk(t, h, row):
            def fn(a):
                zr, zi = cmul(i + 1, 0, NC, h, row, C(t), a)
                acc[i, AR(h, 0, row), C(t)] = zr
                acc[i, AR(h, 1, row), C(t)] = zi
            return fn
        return [mk(*p) for p in pos()]

    def spread():
        n = NB - NC - 1

        def mk(t, h, row):
            def fn(a):
                p = []
                for i in range(3):
                    Rw = slice((3 * h + i) * H + row, (3 * h + i) * H + row + 8)
                    u = uf[0, Rw, C(t)]
                    p.append(kf[1:1 + n, Rw, C(t)] * (_tie(u, a) if i == 0 else u)[None])
                acc[0:n, AR(h, 0, row), C(t)] = acc[1:1 + n, AR(h, 0, row), C(t)] + (p[0] - p[2])
                acc[0:n, AR(h, 1, row), C(t)] = acc[1:1 + n, AR(h, 1, row), C(t)] + (p[0] + p[1])
            return fn
        return [mk(*p) for p in pos()]

    def mmI(name, sl, ys):
        def unit(n):
            def epi(p):
                ce, se, co, so = p
                sub = lax.broadcasted_iota(I32, (8, 128), 0)
                b0 = ys * (T + 8) + 8
                y_v[n, b0 + H - 1:b0 + H, :] = (ce[64:72] - se[0:8])[0:1]
                se = jnp.concatenate([jnp.where(sub == 0, 0.0, se[0:8]), se[8:]], axis=0)
                for d, cc, ss in ((0, ce[0:64], se), (1, co, so)):
                    y_v[n, pl.ds(b0 + H + d, 64, stride=2), :] = cc + ss
                    y_v[n, pl.ds(b0 + d - 1, 64, stride=2), :] = cc - ss
            return Unit(name(n), [(lambda i=i: (tg_v[0:(GR if i == 0 else 64), C(i)], zz_v[pl.ds(sl * 2 * T + i * H, H), C(n)]))
                                  for i in range(4)], epi, 64, 36 + 33 * KS)
        return [unit(n) for n in range(NT)]

    def mod(name, a, b):
        def unit(n):
            def epi(p):
                v = [_sum(p[i * NT:(i + 1) * NT])[0:8] for i in range(b - a)]
                if a == 0:
                    mod_v[0, :, C(n)] = v[0] * v[2]
                    mod_v[1, :, C(n)] = (v[1] + 1.0) * v[2]
                elif a == 3:
                    mod_v[3, :, C(n)] = v[0] * (1.0 / G_POST)
                    mod_v[4, :, C(n)] = (v[1] + 1.0) * (1.0 / G_POST)
                else:
                    mod_v[2, :, C(n)] = v[0] * G_POST
            return Unit(name, [(lambda i=i, k=k: (silu_c[:, C(k)], wm_v[a][C(k), pl.ds(i * D + n * 128, 128)]))
                               for i in range(b - a) for k in range(NT)], epi, 16, 10, full=False, acc=b - a == 1)
        return [unit(n) for n in range(NT)]

    HS = (slice(0, 128), slice(128, 256))
    QS = tuple(slice(r, r + 64) for r in range(0, T, 64))

    def tasks(f, due=None, tie=True, n=RG):
        def mk(R):
            def fn(a):
                x = f(R, a if tie else None)
                return Due(x, due) if due else None
            return fn
        return [mk(slice(r, r + n)) for r in range(0, T, n)]

    def load_y(sl, R):
        b0, back = sl * (T + 8) + 8, 7 - lax.broadcasted_iota(I32, (8, 128), 0)

        def ld(t, r):
            if r >= H:
                return y_v[t, b0 + r:b0 + r + 8, :]
            return jnp.take_along_axis(y_v[t, b0 + H - 8 - r:b0 + H - r, :], back, axis=0)
        return jnp.stack([jnp.concatenate([ld(t, r) for t in range(NT)], axis=1) for r in (R.start, R.start + 8)])

    def put(nn, ss, R, x):
        nn[R, :] = x.astype(BF16)
        tok = x
        if ss is not None:
            S2 = pl.ds(R.start // 32 * 16, 16)
            if R.stop % 32:
                top_v[S2, 0:2 * T] = x[:, 0:2 * T]
            else:
                if R.start % 32:
                    x = jnp.concatenate([top_v[S2, 0:2 * T], x[:, 0:2 * T]], axis=0)
                ss[S2, 0:5 * T] = jnp.concatenate(_lhs_sums(x[:, 0:T], x[:, T:2 * T]), axis=1).astype(BF16)
        return tok

    wide = lambda v: jnp.concatenate([v] * NT, axis=1)

    def mean(i, R, x):
        st_v[R, C(i)] = jnp.broadcast_to(jnp.sum(x, axis=-1, keepdims=True) * (1.0 / D), (x.shape[0], 128))

    def centred(src, i, R, a):
        return src[R, :] - wide(_tie(st_v[R, C(i)], a))

    def scale(src, i, g):
        def f(R, a):
            st_v[R, C(i + 1)] = jnp.broadcast_to(_rstd(centred(src, i, R, a), g), (RG, 128))
        return f

    def normed(src, i, R, a):
        return centred(src, i, R, a) * wide(st_v[R, C(i + 1)])

    def front(sl, xs, early=False, ss=None):
        xx, hh, nn = view(x_v, xs), view(hb_v, xs), view(n1_v, sl)

        def fa(R, a):
            q = [q_n[sl][t, R.start // 2:R.stop // 2, :] for t in range(NT)]
            q = jnp.concatenate([_tie(q[0], a)] + q[1:], axis=1)
            q = pltpu.bitcast(q, BF16).astype(F32).reshape(2, 8, D)
            x = (q + (_ln(q) * mod_v[1] + mod_v[0]) * load_y(sl, R)).reshape(RG, D)
            xx[R, :] = x
            if early:
                hh[R, :] = _ln(x)

        def fb(R, a):
            hh[R, :] = (_ln(_tie(xx[R, :], a).reshape(2, 8, D)) * mod_v[4] + mod_v[3]).reshape(RG, D)

        def fc(R, a):
            hb = _tie(hh[R, :], a)
            if early:
                hb = (hb.reshape(2, 8, D) * mod_v[4] + mod_v[3]).reshape(RG, D)
                hh[R, :] = hb
            nn[R, :] = _ln(hb, True).astype(BF16)
        if early:
            return tasks(fa), tasks(fc)
        if ss is None:
            return tasks(fa) + tasks(fb) + tasks(fc)
        qf = view(x_v, 2)

        def s1(R, a):
            q = [q_n[sl][t, R.start // 2:R.stop // 2, :] for t in range(NT)]
            q = pltpu.bitcast(jnp.concatenate([_tie(v, a) for v in q], axis=1), BF16).astype(F32)
            qf[R, :] = q
            mean(0, R, q)

        def s3(R, a):
            h = normed(qf, 0, R, a).reshape(2, 8, D) * mod_v[1] + mod_v[0]
            x = qf[R, :] + (h * load_y(sl, R)).reshape(RG, D)
            xx[R, :] = x
            mean(2, R, x)

        def s5(R, a):
            hb = (normed(xx, 2, R, a).reshape(2, 8, D) * mod_v[4] + mod_v[3]).reshape(RG, D)
            hh[R, :] = hb
            mean(4, R, hb)
        s7 = [f for g in tasks(lambda R, a: put(nn, ss, R, normed(hh, 4, R, a)), n=32) for f in (g, lambda a: None)]
        st = [tasks(s3), tasks(scale(xx, 2, False)), tasks(s5), tasks(scale(hh, 4, True)), s7]
        p = [tasks(s1), tasks(scale(qf, 0, False))]
        return cat(x[:8] for x in st), cat(x[8:] for x in p[1:] + st), cat(x[:8] for x in p), p[0][8:]

    def shift(hs, sl, pieces=((0, 64), (64, 64), (128, 64), (192, 64)), ss=None):
        gg = view(g_v, sl)

        def one_tile(t, r, n, a):
            lane = lax.broadcasted_iota(I32, (n, 128), 1)
            ld = lambda d: h1_v[t, pl.ds(hs * T + 8 + r + d, n), :]
            if t == 0:
                g = ld(-1)
            elif t == 1:
                g = jnp.where(lane < 32, ld(-1), ld(1))
            elif t == 2:
                g = jnp.where(lane < 64, ld(1), ld(-2))
            elif t == 3:
                g = jnp.where(lane < 96, ld(-2), ld(2))
            else:
                g = ld(2)
            if a is not None:
                g = jnp.concatenate([_tie(g[i:i + 8], a) if i % 16 == 0 else g[i:i + 8]
                                     for i in range(0, n, 8)], axis=0)
            gg[r:r + n, C(t)] = g.astype(BF16)
            return g

        def mk(ts, r, n):
            def fn(a):
                g = [one_tile(t, r, n, a) for t in ts]
                if len(ts) == 2:
                    for i, x in enumerate(_lhs_sums(*g)):
                        ss[r // 2:(r + n) // 2, C(2 * i + ts[0])] = x.astype(BF16)
            return fn
        sets = [(t,) for t in range(NT)] if ss is None else [(0, 2), (1, 3), (4,)]
        return [mk(ts, r, n) for ts in sets for r, n in pieces]

    def shift_early():
        def keep(a):
            h1_v[:, 2 * T - 32:2 * T + 8, :] = h1_v[:, 3 * T - 32:3 * T + 8, :]
        return shift(2, 0, [(r, 32) for r in range(0, T - 32, 32)], gs) + [keep]

    def ln2(xs, sl, fast=True):
        xx, nn, ss = view(x1_v, xs), view(n2_v, sl), view(n2s, sl, H) if fast else None
        f = lambda R, a: put(nn, ss, R, _ln(_tie(xx[R, :], a), True))
        ts = tasks(f, 900) if sl else tasks(f, DL, False)
        return ts[0::2] + ts[1::2] if fast else tasks(f)

    def ln2_late(mode):
        xx, nn, ss = view(x1_v, 0), view(n2_v, 0), view(n2s, 0, H)
        if mode == 0:
            return tasks(lambda R, a: put(nn, ss, R, _ln(_tie(xx[R, :], a), True)), n=32)[:4], 160
        a_, b_ = tasks(lambda R, a: mean(6, R, _tie(xx[R, :], a))), tasks(scale(xx, 6, True))
        c_ = [f for g in tasks(lambda R, a: put(nn, ss, R, normed(xx, 6, R, a)), n=32)[:4] for f in (g, lambda a: None)]
        return a_[:8] + b_[:8] + c_, 40

    def resid(xs, x1s, rotate=False):
        xx, x1 = view(x_v, xs), view(x1_v, x1s)

        def f(R, a):
            tie = lambda v: v if a is None else pltpu.bitcast(pltpu.bitcast(v, U32) | wide(a), F32)
            r_v[R, :] = xx[R, :] + (x1[R, :].reshape(2, 8, D) * tie(mod_v[2])).reshape(RG, D)
            if rotate:
                xx[R, :] = tie(x_v[R, :].reshape(2, 8, D)).reshape(RG, D)
                view(hb_v, 1)[R, :] = tie(hb_v[R, :].reshape(2, 8, D)).reshape(RG, D)
        return tasks(f)

    KD, KF, ND = [(0, 2), (1, 3)], [(2 * i, 2 * i + 1) for i in range(7)], [(1, 2), (3, 4)]
    Wt = {1: (lambda k, n: w1_v[C(k), C(n)], lambda i, kp, j: w1s[C(kp), C(2 * i + j)], False, KD, [4]),
          2: (lambda k, n: w2_v[C(k), C(n)], lambda i, kp, j: w2s[C(kp), C(2 * i + j)], False, KD, [4]),
          0: (lambda k, n: w3_v[C(n), C(k)], None, True, KD, [4]),
          3: (lambda k, n: w3n[C(k), C(n)], lambda i, kp, j: w3s[C(kp), C(6 * i + j)], False, KD, [4]),
          4: (lambda k, n: w4_v[C(k), C(n)], lambda i, kp, j: w4s[C(kp), C(2 * i + j)], False, KF, [])}

    def sums_task(load, store, left):
        def fn(a):
            b = [[load(u, v) for v in range(2)] for u in range(2)]
            b[0][0], b[1][1] = _tie(b[0][0], a), _tie(b[1][1], a)
            (x11, x12), (x21, x22) = [[pltpu.bitcast(x, BF16).astype(F32) for x in row] for row in b]
            r = ((x11 + x22, x21 + x22, x11 + x12, x21 - x11, x12 - x22) if left else
                 (x11 + x22, x12 - x22, x21 - x11, x11 + x12, x21 + x22))
            for m, x in enumerate(r):
                store(m, x.astype(BF16))
        return fn

    def wsums(w_w, ws, rp, cp_):
        def mk(i, j, r):
            def store(m, x):
                ws[pl.ds(128 * i + r, 16), C(len(cp_) * m + j)] = x
            return sums_task(lambda u, v: w_w[pl.ds(64 * rp[i][u] + r // 2, 8), C(cp_[j][v])], store, False)
        return [mk(i, j, r) for j in range(len(cp_)) for i in range(len(rp)) for r in range(0, 128, 16)]

    def w3_turn():
        def mk(n, k):
            def fn(a):
                x = jnp.concatenate([_tie(w3_w[64 * n:64 * n + 8, C(k)], a), w3_w[64 * n + 8:64 * n + 64, C(k)]], axis=0)
                w3n[C(k), C(n)] = pltpu.bitcast(x, BF16).T
            return fn
        return [mk(n, k) for n in range(FT - 1) for k in range(NT)]

    def plain(name, w, lhs, n, R, epi, cost):
        tile, _, nt, kp, kl = Wt[w]
        ks = sorted([k for p in kp for k in p] + kl)
        rows_ = R.stop - R.start
        return Unit(name, [(lambda k=k: (lhs[R, C(k)], tile(k, n))) for k in ks], lambda p: epi(n, R, p[0]),
                    rows_, rows_ // 8 * (len(ks) - 1), nt=nt, acc=True, tail=rows_ // 8 * cost(n))

    def quad(name, w, lhs, sums, j, cols_, R, epi, cost):
        tile, wsum, nt, kp, kl = Wt[w] if isinstance(w, int) else w
        h, S2, c = len(kp), slice(R.start // 2, R.stop // 2), {}
        a_ = lambda i, k: _top(lhs(k) if callable(lhs) else lhs[R, C(k)], i)
        s_ = sums if callable(sums) else (lambda i, p: sums[S2, C(h * i + p)])
        prod = lambda fa_, fb_: [(lambda p=p: (fa_(p), fb_(p))) for p in range(h)]
        left = lambda i, n: [(lambda k=k: (a_(i, k), tile(k, n))) for k in kl]
        mk = lambda tiles, f, x=0: Unit(name, tiles, lambda p: f(p[0]), 64, 8 * len(tiles), nt=nt, acc=True, tail=x)

        def e1(m):
            u7.res, u6.res = [m], [m]

        def e4(m):
            c[11], c[21] = c[11] + m, m

        def e2(m):
            c[21], c[22] = c[21] + m, c[22] - m
            l21.res = [c[21]]

        def e5(m):
            c[12] = m
            epi(cols_[0], R, _zip(c[11] - m, c[21]))

        def e3(m):
            l12.res, c[22] = [c[12] + m], c[22] + m
            if not kl:
                l12.epi(l12.res)
        u1 = mk(prod(lambda p: s_(0, p), lambda p: wsum(0, p, j)), e1)
        u7 = mk(prod(lambda p: s_(4, p), lambda p: wsum(4, p, j)) + left(0, cols_[0]), lambda m: c.update({11: m}))
        u6 = mk(prod(lambda p: s_(3, p), lambda p: wsum(3, p, j)) + left(1, cols_[1]), lambda m: c.update({22: m}))
        u4 = mk(prod(lambda p: a_(1, kp[p][1]), lambda p: wsum(2, p, j)), e4)
        u2 = mk(prod(lambda p: s_(1, p), lambda p: tile(kp[p][0], cols_[0])), e2, 8)
        l21 = mk(left(1, cols_[0]), lambda m: c.update({21: m}))
        u5 = mk(prod(lambda p: s_(2, p), lambda p: tile(kp[p][1], cols_[1])), e5, 16 * cost(cols_[0]))
        u3 = mk(prod(lambda p: a_(0, kp[p][0]), lambda p: wsum(1, p, j)), e3, 8 if kl else 8 + 16 * cost(cols_[1]))
        l12 = mk(left(0, cols_[1]), lambda m: epi(cols_[1], R, _zip(m, c[22])), 16 * cost(cols_[1]))
        return [u1, u7, u6, u4, u2, l21, u5, u3, l12]

    LH, RH = [0, 4, 3, (1, 1), 1, 2, (0, 0)], [0, 4, 3, 2, (0, 0), (1, 1), 1]
    L2 = {3: (w3n_w, ws_w[2], w3t, KF[:6], n2t), 4: (w4_w, ws_w[3], w4t, ND, a_t)}

    def wsums2(w):
        w_w, s_w, ws2, cp_, _ = L2[w]
        kp, nj = Wt[w][3], len(cp_)

        def mk(o, p2, j2, r):
            def load(u, v):
                p, j, y = 2 * p2 + u, 2 * j2 + v, RH[o]
                if isinstance(y, int):
                    return s_w[pl.ds(64 * p + r // 2, 8), C(nj * y + j)]
                return w_w[pl.ds(64 * kp[p][y[0]] + r // 2, 8), C(cp_[j][y[1]])]

            def store(m, x):
                ws2[pl.ds(128 * p2 + r, 16), C((5 * o + m) * (nj // 2) + j2)] = x
            return sums_task(load, store, False)
        return [mk(o, p2, j2, r) for j2 in range(nj // 2) for o in range(7) for p2 in range(len(kp) // 2)
                for r in range(0, 128, 16)]

    def wsums4():
        form = [((0, 0), (1, 1), 1), ((0, 1), (1, 1), -1), ((1, 0), (0, 0), -1), ((0, 0), (0, 1), 1), ((1, 0), (1, 1), 1)]

        def mk(o, p2, r):
            def fn(a):
                def blk(p, j, uv, t):
                    x = w4_w[pl.ds(64 * KF[p][uv[0]] + r // 2, 8), C(ND[j][uv[1]])]
                    return pltpu.bitcast(_tie(x, t), BF16).astype(F32)
                y = {}
                for u in range(2):
                    for j in range(2):
                        p = 2 * p2 + u
                        if isinstance(RH[o], int):
                            f = form[RH[o]]
                            x1, x2 = blk(p, j, f[0], a), blk(p, j, f[1], None)
                            y[u, j] = x1 + x2 if f[2] > 0 else x1 - x2
                            w4s[pl.ds(128 * p + r, 16), C(2 * RH[o] + j)] = y[u, j].astype(BF16)
                        else:
                            y[u, j] = blk(p, j, RH[o], a if u == j else None)
                for m, f in enumerate(form):
                    x = y[f[0]] + y[f[1]] if f[2] > 0 else y[f[0]] - y[f[1]]
                    w4t[pl.ds(128 * p2 + r, 16), C(5 * o + m)] = x.astype(BF16)
            return fn
        last = wsums(w4_w, w4s, KF, ND)
        return (last[48:56] + last[104:112]
                + [mk(o, p2, r) for o in range(7) for p2 in range(3) for r in range(0, 128, 16)])

    def lsums2(w, lhs_w, sums_w, sl):
        kp, xs2 = Wt[w][3], L2[w][4]
        h2 = len(kp) // 2

        def mk(o, p2, g):
            def load(u, v):
                p, ch, x = 2 * p2 + v, 2 * g + u, LH[o]
                if isinstance(x, int):
                    return sums_w[pl.ds(64 * sl + 8 * ch, 8), C(len(kp) * x + p)]
                return lhs_w[pl.ds(H * sl + 16 * ch + 8 * x[0], 8), C(kp[p][x[1]])]

            def store(m, x):
                xs2[pl.ds(16 * g, 16), C((5 * o + m) * h2 + p2)] = x
            return sums_task(load, store, True)
        return [[mk(o, p2, g) for o in range(7) for g in range(4)] for p2 in range(h2)]

    def quad2(name, w, lhs, sums, j2, epi, cost):
        tile, wsum, nt, kp, kl = Wt[w]
        ws2, cp_, xs2 = L2[w][2:]
        h, h2, nj2, c, R = len(kp), len(kp) // 2, len(cp_) // 2, {}, slice(0, T)

        def done(j, v):
            val = _zip(c[j, 1, v], c[j, 2, v])
            if not kl:
                return epi(cp_[j][v], R, val)
            c[j, v] = val

        def upd(o, j, m):
            for i, v, sg in (((1, 0, 1), (2, 1, 1)), ((1, 0, 1),), ((2, 1, 1),), ((1, 0, 1), (2, 0, 1)),
                             ((2, 0, 1), (2, 1, -1)), ((1, 0, -1), (1, 1, 1)), ((1, 1, 1), (2, 1, 1)))[o]:
                k = (j, i, v)
                c[k] = m if k not in c else (c[k] + m if sg > 0 else c[k] - m)
            if o >= 5:
                done(j, o - 5)

        def inner(o):
            x, y = LH[o], RH[o]
            xo = ((lambda p: sums[:, C(h * x + p)]) if isinstance(x, int)
                  else (lambda p: _top(lhs[:, C(kp[p][x[1]])], x[0])))
            yo = ((lambda p, j: wsum(y, p, j)) if isinstance(y, int)
                  else (lambda p, j: tile(kp[p][y[0]], cp_[j][y[1]])))
            w_ = (yo, lambda m, p2, _: ws2[C(p2), C((5 * o + m) * nj2 + j2)], nt,
                  [(2 * i, 2 * i + 1) for i in range(h2)], list(range(2 * h2, h)))
            return quad(name, w_, xo, lambda m, p2: xs2[:, C((5 * o + m) * h2 + p2)], 0, (2 * j2, 2 * j2 + 1),
                        HS[0], lambda j, _, m: upd(o, j, m), lambda j: 1.5 + KS + (2 * cost(0) if o >= 5 and not kl else 0))

        def rest(j, v, Q):
            return [Unit(name, [lambda: (lhs[Q, C(k)], tile(k, cp_[j][v]))],
                         lambda p: epi(cp_[j][v], Q, p[0] + c[j, v][Q]), 64, 8 * (cost(cp_[j][v]) + 1)) for k in kl]
        return cat(inner(o) for o in range(7)), [u for Q in QS for j in (2 * j2, 2 * j2 + 1) for v in range(2)
                                                 for u in rest(j, v, Q)]

    def mm(name, w, lhs, sums, epi, cost):
        if sums is None:
            return [[plain(name, w, lhs, n, R, epi, cost) for R in HS] for n in range(NT)]
        return [[plain(name, w, lhs, 0, R, epi, cost) for R in QS]] + [
            [u for R in HS for u in quad(name, w, lhs, sums, j, ND[j], R, epi, cost)] for j in range(2)]

    def mm1(name, hs, sl, fast=False):
        def epi(n, R, p):
            h1_v[n, pl.ds(hs * T + 8 + R.start, R.stop - R.start), :] = _gelu2(p)
        return cat(mm(name, 1, view(n1_v, sl), n1s if fast else None, epi, lambda n: 5 + KS))

    def mm2(name, sl, xs, x1s, fast=False):
        def epi(n, R, p):
            view(x1_v, x1s)[R, C(n)] = view(hb_v, xs)[R, C(n)] + p
        return cat(mm(name, 2, view(g_v, sl), gs if fast else None, epi, lambda n: 1 + KS))

    def mm3(name, sl, fast=True, deep=False, host=None):
        nn, aa, ss, keep, tail = view(n2_v, sl), view(a_v, sl), view(a_s, sl, H), {}, []

        def epi(n, R, p):
            g = _gelu2(p)
            aa[R, C(n)] = g.astype(BF16)
            if not fast:
                return
            if n % 2 == 0 and n < 12:
                keep[n] = g
                return
            pair = (keep.pop(n - 1), g) if n % 2 else (g, tail[R.start // 128][R.start % 128:R.start % 128 + 64])
            sm = _lhs_sums(*pair)
            for i, x in enumerate(sm):
                ss[R.start // 2:R.stop // 2, C(7 * i + n // 2)] = x.astype(BF16)
            if deep and n < 12:
                xo = [sm[x] if isinstance(x, int) else _top(pair[x[1]], x[0]) for x in LH]
                if n % 4 == 1:
                    keep[n, R.start] = xo
                    return
                for o, x in enumerate(zip(keep.pop((n - 2, R.start)), xo)):
                    for m, y in enumerate(_lhs_sums(*x)):
                        a_t[R.start // 4:R.stop // 4, C((5 * o + m) * 3 + n // 4)] = y.astype(BF16)

        c3 = lambda n: 5.5 + 0.5 * KS + (3.75 + 1.25 * KS if fast and (n % 2 or n == 12) else 0)

        def rem(R):
            def f(p):
                tail.append(jnp.concatenate([_gelu2(p[0]), jnp.zeros((64, 128), F32)], axis=0).T)
                aa[R, C(13)] = tail[-1].astype(BF16)
            return Unit(name, [(lambda k=k: (w3_v[13 * 128:F, C(k)], nn[R, C(k)])) for k in range(NT)], f, 64, 84,
                        nt=True, acc=True)
        odd = [rem(R) for R in HS] + [plain(name, 3 if fast else 0, nn, 12, R, epi, c3) for R in QS]
        if fast == 2:
            qd = [quad2(name + "_%d" % j, 3, nn, view(n2s, sl, H), j, epi, c3) for j in range(3)]
            if host is not None:
                for u in (odd[0], odd[2], odd[3]):
                    u.name = name + "h"
                return ([odd[0], odd[2], odd[3], odd[1]] + qd[0][0] + _weave(qd[1][0], qd[0][1])
                        + _weave(qd[2][0], qd[1][1]), _weave(odd[4:] + host, qd[2][1]))
            return odd[:2] + qd[0][0] + _weave(qd[1][0], qd[0][1]) + _weave(qd[2][0], qd[1][1]) + _weave(odd[2:], qd[2][1])
        if fast:
            qd = [[u for j in range(6) for u in quad(name + ("b%d" % (j // 2) if i else "a"), 3, nn, view(n2s, sl, H), j,
                                                     KF[j], R, epi, c3)] for i, R in enumerate(HS)]
            return qd[0] + qd[1][:36] + odd[:2] + qd[1][36:] + odd[2:]
        return odd + [plain(name, 0, nn, n, R, epi, c3) for p in KF[:6] for R in HS for n in p]

    def cp_out(j, osl, L, sm, R=slice(0, T)):
        return cp(o_v.at[pl.ds(osl * T + R.start, R.stop - R.start), L],
                  o_hbm.at[pl.ds(base(j, T) + R.start, R.stop - R.start), L], sem_o.at[sm])

    out_a = lambda j: cp_out(j, 0, slice(128, D), 0)
    out_b = lambda j: cp_out(j, 0, C(0), 1)
    last = []

    def mm4(name, j, sl, osl=0, xs=None, x1s=None, fast=True):
        oo = view(o_v, osl)

        def epi(n, R, p):
            if xs is None:
                oo[R, C(n)] = (r_v[R, C(n)] + mod_v[2, 0:1, C(n)] * p).astype(BF16)
            else:
                oo[R, C(n)] = (view(x_v, xs)[R, C(n)] + mod_v[2, 0:1, C(n)]
                               * (view(x1_v, x1s)[R, C(n)] + p)).astype(BF16)
            if osl == 2:
                last.append(cp_out(j, osl, C(n), 2, R))
                last[-1].start()
            elif R.stop == T and osl and n == NT - 1:
                last.append(cp_out(j, osl, slice(128 if osl == 3 else 0, D), 2))
                last[-1].start()
            elif R.stop == T and osl == 0 and n in (0, NT - 1):
                (out_a if n else out_b)(j).start()
        c4 = lambda n: (3 if xs is None else 4) + KS
        if fast == 2:
            return ([plain(name, 4, view(a_v, sl), 0, R, epi, c4) for R in QS],
                    quad2(name + "q", 4, view(a_v, sl), view(a_s, sl, H), 0, epi, c4)[0])
        return mm(name, 4, view(a_v, sl), view(a_s, sl, H) if fast else None, epi, c4)

    def split(us):
        n = 4 // len(us)
        m, mks, st = us[0].rows // n, [u.tiles.pop(0) for u in us], {}

        def piece(i, k):
            if i not in st:
                st[i] = mks[i]()
            return st[i][0][m * k:m * (k + 1)], st[i][1]

        def epi(p):
            for i, u in enumerate(us):
                u.res = [jnp.concatenate(p[n * i:n * (i + 1)], axis=0)]
        return _flat([Unit(us[0].name, [(lambda i=i, k=k: piece(i, k)) for i in range(len(us)) for k in range(n)],
                           epi, m, 0, nt=us[0].nt)])

    W = lambda nm: [("wait", nm)]
    run = lambda fns: [("run", "run", lambda: [fn(None) for fn in fns])]
    one = lambda us: [_flat([u]) for u in us]
    nm = lambda x: (lambda n: x)

    seq, grp = [], []
    for s in range(NC):
        seq += W("c%d" % s) + _flat(mmK(s) + mmU(nm("U%d" % s), s % 2, NC - 1 - s))
        grp.append(Group("kv%d" % s, cat(kv(s, s % 2)), 50, ["c%d" % s], ["U%d" % s], 100))
    inv = [mmI(lambda n: "I%d" % n, s, s) for s in range(NC)]
    seq += W("c3") + _flat(mmK(3) + mmK(4) + [inv[s][t] for t in range(NT) for s in range(NC)])
    macs = [mac(s + 1, NC - 1 - s, s) for s in range(NC)]
    grp.append(Group("mac00", macs[0][0], 12, ["c1"], ["c2"], 0))
    grp.append(Group("mac01", macs[1][0] + macs[0][1] + macs[1][1], 16, ["c2"], ["c3"], 0))
    for t in range(NT):
        grp.append(Group("mac%d" % t, cat(macs[s][t] for s in range(2 if t < 2 else 0, NC)), 24 if t < 2 else 18,
                         ["c3", "K%d" % t], ["I%d" % t], 100, 150))
    start = lambda cs: [("run", "run", lambda: [c.start() for c in cs])]
    f0, f1 = front(0, 2, True), front(1, 1, True)
    seq += run(ahead(0))
    seq += W("wma") + _flat(mod("moda", 0, 3)) + run(f0[0] + f1[0] + ahead(1))
    seq += W("wmb") + start(next_kv(NC) + next_q(NC)) + _flat(mod("modb", 3, 5)) + run(f0[1])
    w1 = _flat(mm1("w1_0", 0, 0) + mm1("w1_1", 1, 1))
    seq += W("w1") + w1[:72] + W("w2") + w1[72:] + run(shift(0, 0))
    seq += _flat(mm2("w2_0", 0, 2, 1) + mm1("w1_2", 2, 2)) + run(shift(1, 1)) + _flat(mm2("w2_1", 1, 1, 0))
    grp.append(Group("f1", f1[1], 80, ["w1"], ["w1_1"], 450))
    grp.append(Group("f2", front(2, 0), 80, ["w2"], ["w1_2"], 450))
    grp.append(Group("ln2_0", ln2(1, 0, False), 60, ["w2_0"], ["w3"], 450))
    grp.append(Group("ahead", cat(ahead(i) for i in range(2, NB - NC)), 19 + 2 * KS, ["w1"], ["end"], 100))
    grp.append(Group("ws1", wsums(w1_w, w1s, KD, ND), 26 + 5 * KS, ["w1"], ["end"], 100))
    grp.append(Group("ws2", wsums(w2_w, w2s, KD, ND), 26 + 5 * KS, ["w2"], ["end"], 100))
    grp.append(Group("ws3", w3_turn() + wsums(w3n_w, w3s, KD, KF[:6]) + wsums2(3), 22 + 5.5 * KS, ["w3"], ["end"], 100))
    grp.append(Group("ws4", wsums4(), 40 + 8 * KS, ["w4"], ["end"], 60))
    _wait(seq, "w3", back=1)
    w3 = mm3("w3_0", 0, False, False)
    _mix(seq, _flat(w3[6:]), [split(w3[4:6]) + _flat(w3[:6])], 0.1)
    mc = mod("modc", 5, 6)
    mc = _flat(mc[1:] + mc[:1])
    _wait(seq, "w4", mc[:5] + [("sync", "run", lambda: None)])
    w4 = cat(mm4("w4_0", 0, 0, 3, 2, 1, False)[1:])
    qs = [split([w4[-1 - i]]) for i in range(_phase(seq))]
    _mix(seq, _flat(w4), [mc[i:i + 4] for i in range(5, 25, 4)] + qs, 0.01, 0.4)
    assert _phase(seq) == 0
    grp.append(Group("resid", resid(2, 1), 26 + 5 * KS, ["modc"], ["end"], 100))
    grp.append(Group("ln2a", *ln2_late(1), ["w3_0"], ["end"], 100))
    if E("ONLY", 0):
        for g in grp:
            g.fns = [lambda a: None] * len(g.fns)
        seq = [it if it[0] != "run" else ("run", "run", lambda: None) for it in seq]
    _emit(seq, grp, zero, wait)

    def step(s, carry):
        for c in next_kv(s) + next_q(s):
            c.wait()
        nxt = jnp.minimum(s + 1, NB - 1)
        seq, grp = [], []
        us, it = one(mmU(lambda n: "U%d" % n, 0, 0)), one(mmI(lambda n: "I%d" % n, 0, 0))
        w4, w4c = mm4("w4", s - 2, 0, fast=2)[1], mm4("w4c", s - 3, 0, fast=2)[0]
        w2 = mm2("w2", 0, 1, 0, True)
        w2 = w2[0:3] + w2[4:13] + w2[22:31] + w2[3:4] + w2[13:22] + w2[31:]
        for u in w2[:21]:
            u.name = "w2a"
        w3, w3e = mm3("w3", 0, 2, host=w2[:E("HN", 12)])
        _mix(seq, _flat(w4c + w3),
             [us[0], us[1], us[2], it[0] + us[3], it[1] + us[4], it[2] + start(next_kv(nxt)), it[3], it[4]],
             E("LP3", 0.18), E("LP0", 0.75))
        w1a, w1b = mm1("w1a", 2, 0, True), mm1("w1b", 2, 0, True)
        w1a, w1b = _flat(w1a[0:2] + w1a[4:13] + w1a[22:31]), _flat(w1b[2:4] + w1b[13:22] + w1b[31:])
        kw = 9 * E("KW", 6)
        seq += _flat(w3e + w2[E("HN", 12):21] + w4[:kw]) + w1a[:8] + start(next_q(nxt)) + w1a[8:]
        seq += run(shift(1, 0, ((T - 32, 32),), gs)) + _flat(w4[kw:] + w2[21:]) + w1b
        assert _phase(seq) == 0
        kvs, macs = kv(0, 0), mac(1, 0, 0, part=True)
        for t in range(NT):
            grp.append(Group("kv%d" % t, kvs[t], 50 + 2 * KS, ["start"], ["U%d" % t], E("KL", 300)))
            grp.append(Group("mac%d" % t, macs[t], 24 + 2 * KS, ["U%d" % t], ["I%d" % t], E("ML", 300), 150))
        iall = ["I%d" % t for t in range(NT)]
        ln = ln2(0, 0)
        grp.append(Group("ln2a", *ln2_late(E("LM", 1)), ["w2a", E("LR", "w2")], ["end"], E("LL", 100)))
        xn = lsums2(3, n2_w, as_w[2], 0)[0]
        grp.append(Group("ln2b", ln[4:8] + ln[12:16], 78 + 20 * KS, ["start"], ["w3h"], E("BL", 450)))
        grp.append(Group("xna", [f for i, f in enumerate(xn) if i % 4 < 2], 26 + 5 * KS, ["start"], ["w3_0"], 150))
        grp.append(Group("xnb", [f for i, f in enumerate(xn) if i % 4 >= 2], 26 + 5 * KS, ["w4c"], ["w3_0"], 150, 0))
        grp.append(Group("resid", resid(1, 0, True), 46 + 30 * KS, ["w4c"], ["w2a", "w4q", "I4"], 100))
        for p, ts in enumerate(lsums2(4, a_w, as_w[3], 0)):
            grp.append(Group("xa%d" % p, ts, 26 + 5 * KS, ["w3_%d" % p], ["w4q"], 150, 100))
        fr = front(0, 0, ss=n1s)
        grp.append(Group("fronta", fr[0], 50 + 8 * KS, iall, ["w1a"], E("FL", 230)))
        grp.append(Group("frontb", fr[1], 48 + 7 * KS, iall, ["w1b"], E("FL", 230), E("RL", 3500)))
        grp.append(Group("fqb", fr[3], 26 + 12 * KS, iall, ["w1a"], E("QL", 300), E("RL", 3500) - 500))
        grp.append(Group("fq", fr[2], 33 + 7 * KS, ["w4c"], ["I4"], 100))
        grp.append(Group("spread", spread(), 30 + 8 * KS, iall, ["end"], E("SL", 100)))
        grp.append(Group("shift", shift_early(), 22 + 7 * KS, ["start"], ["w1a", "w2a"], 200))
        _emit(seq, grp, zero, wait)
        out_b(s - 3).wait()
        out_a(s - 2).wait()
        return carry

    lax.fori_loop(NC, NB, step, 0)

    seq, grp = [], []
    w47 = mm4("w4_7", NB - 1, 1, 2, 0, 1, 2)
    seq += _flat(mm4("w4_5", NB - 3, 0, fast=2)[0] + mm2("w2_7", 0, 0, 1, True) + mm3("w3_6", 0, 2)
                 + cat(mm4("w4_6", NB - 2, 0, 1, 1, 0, 2)) + mm3("w3_7", 1, 2) + w47[0][:3] + w47[1] + w47[0][3:])
    grp.append(Group("shift7", shift(2, 0, [(r, 32) for r in range(0, T, 32)], gs), 24, ["start"], ["w2_7"], 200))
    ln = ln2(0, 0)
    grp.append(Group("ln2_6", ln[4:8] + ln[12:16], 75, ["start"], ["w3_6"], 1200))
    grp.append(Group("xn6", cat(lsums2(3, n2_w, as_w[2], 0)), 26 + 5 * KS, ["w4_5"], ["w3_6_0"], 200, 800))
    grp.append(Group("ln2_7", ln2(1, 1), 75, ["w4_6"], ["w3_7"], 1500))
    grp.append(Group("xn7", cat(lsums2(3, n2_w, as_w[2], 1)), 26 + 5 * KS, ["w4_6"], ["w3_7_0"], 200, 2100))
    for j in (6, 7):
        for p, ts in enumerate(lsums2(4, a_w, as_w[3], j - 6)):
            grp.append(Group("xa%d_%d" % (j, p), ts, 26 + 5 * KS, ["w3_%d_%d" % (j, p)], ["w4_%dq" % j], 200, 150))
    if E("ONLY", 0):
        seq, grp = seq[:8 * 14], []
    _emit(seq, grp, zero, wait)
    for c in next_kv(NB - 1) + next_q(NB - 1) + [out_b(NB - 3)] + last:
        c.wait()


@jax.jit
def pallas_adaLN_cond__ssm_conv_h3__mixer_s_mlp__prompt_kernel(
        A_q, A_k, A_v, A_shift_k, A_ssm_k, A_ssm_D, B_x, B_w1, B_w2, B_w3, B_w4, c, w_mod):
    any_ = pl.BlockSpec(memory_space=pl.ANY)
    V = pltpu.VMEM
    out = pl.pallas_call(
        kernel,
        in_specs=[any_] * 12,
        out_specs=any_,
        out_shape=jax.ShapeDtypeStruct((S, D), BF16),
        scratch_shapes=[
            [V((NT, H + 8, 128), U32)] * NC, [V((NT, H + 8, 128), U32)] * NC, [V((NT, H + 8, 128), U32)] * NC,
            [V((64, S), U32)] * NT,
            V((D // 2, D), U32), V((D // 2, D), U32), V((F // 2, D), U32), V((FT * 64, D), U32),
            [V((D // 2, 3 * D), U32), V((D // 2, 2 * D), U32), V((D // 2, D), U32)], V((4 * T, D), BF16),
            V((4, D), BF16), V((D,), BF16), V((1, D), BF16), V((8, 128), I32), pltpu.SMEM((8, 128), I32),
            V((5, 8, D), F32), V((6, 8, D), F32), V((T // 2, 4 * H), U32), V((GR // 2, 2 * T), U32),
            V((NB, 3 * T + 8, D), F32), V((NC, 3 * T + 8, D), F32), V((NB - NC, 2 * T + 8, D), F32), V((4 * T, 128), F32),
            V((T, D), U32), V((NC * T, D), U32), V((NT, NC * (T + 8) + 16, 128), F32),
            V((3 * T, D), F32), V((3 * T, D), F32), V((2 * T, D), F32), V((T, D), F32),
            V((3 * T // 2, D), U32), V((T, D), U32), V((T, D), U32), V((NT, NC * T + 24, 128), F32),
            V((T, (FT + 1) * 128), U32),
            [V((128, 11 * 128), U32)] * 2 + [V((128, 31 * 128), U32), V((448, 11 * 128), U32)],
            [V((64, 11 * 128), U32)] * 2 + [V((128, 11 * 128), U32), V((128, 35 * 128), U32)],
            V((D // 2, 13 * 128), U32), V((H, D), F32), V((T, 9 * 128), F32),
            [V((64, 105 * 128), U32), V((192, 35 * 128), U32), V((32, 35 * 128), U32), V((32, 105 * 128), U32)],
            pltpu.SemaphoreType.DMA((11,)), pltpu.SemaphoreType.DMA((1,)), pltpu.SemaphoreType.DMA((3,)),
        ],
        compiler_params=pltpu.CompilerParams(vmem_limit_bytes=110 << 20, disable_semaphore_checks=True,
                                             disable_bounds_checks=True),
        name="fused",
    )(A_q[0], A_k[0], A_v[0], A_shift_k.T, A_ssm_k, A_ssm_D, B_w1, B_w2, B_w3.T, B_w4, c, w_mod)
    return out[None]
```

```python
import heapq
import numpy as np
import jax
import jax.numpy as jnp
from jax import lax
from jax.experimental import pallas as pl
from jax.experimental.pallas import tpu as pltpu

S, D, F = 2048, 640, 1728
T = 256
H = T // 2
NB = S // T
NT = D // 128
FT = (F + 127) // 128
EPS = 1e-5
F32, BF16, U32, I32 = jnp.float32, jnp.bfloat16, jnp.uint32, jnp.int32
G_C1 = 0.044715 * float(np.sqrt(2.0 / np.pi))
G_C2 = float(np.sqrt(2.0 / np.pi))
G_A = G_C1 ** (1.0 / 3.0)
G_B = G_C2 / G_A
G_POST = 0.5 / G_A
RG = 16
GR = 80
NC = 3
DL = 450
KS = 1.9
SLOT = 32


def _dft(shape, f_axis, tau, scale=1.0):
    r = lax.broadcasted_iota(I32, shape, f_axis)
    l = lax.broadcasted_iota(I32, shape, 1 - f_axis)
    f = r & 127
    odd = ((f & 63) << 2) | ((f >> 6) << 1) | 1
    p = odd * tau(l) + ((r >> 7) << 8)
    a = ((p + 512) & 1023) - 512
    u = (256 - jnp.abs(a)).astype(F32) * (np.pi / 512.0)
    u2 = u * u
    c = [scale, -scale / 6.0, scale / 120.0, -scale / 5040.0, scale / 362880.0, -scale / 39916800.0]
    poly = c[5]
    for ci in c[4::-1]:
        poly = poly * u2 + ci
    return (u * poly).astype(BF16)


def _rstd(xc, mlp):
    s2, eps = (1.0 / (G_A * G_A), EPS / (G_POST * G_POST)) if mlp else (1.0, EPS)
    v = jnp.sum(xc * xc, axis=-1, keepdims=True) * (s2 / D) + eps * s2
    return jnp.exp2(jnp.log(v) * float(-0.5 / np.log(2.0)))


def _ln(x, mlp=False):
    xc = x - jnp.sum(x, axis=-1, keepdims=True) * (1.0 / D)
    return xc * _rstd(xc, mlp)


def _gelu2(x):
    u = x * (x * x + G_B)
    return x * (1.0 + jnp.tanh(u))


def _lo(w):
    return pltpu.bitcast(w << 16, F32)


def _hi(w):
    return pltpu.bitcast(w & jnp.uint32(0xFFFF0000), F32)


def _tie(x, a):
    if a is None:
        return x
    w = pltpu.bitcast(x[:, :128], U32)
    k = w.shape[0] // 8
    w = w | (a if k == 1 else jnp.concatenate([a] * k, axis=0))
    w = pltpu.bitcast(w, x.dtype)
    return w if x.shape[1] == 128 else jnp.concatenate([w, x[:, 128:]], axis=1)


def _top(x, i):
    return jnp.concatenate([x[r:r + 16] for r in range(16 * i, x.shape[0], 32)], axis=0)


def _zip(t, b):
    return jnp.concatenate([x[r:r + 16] for r in range(0, t.shape[0], 16) for x in (t, b)], axis=0)


def _lhs_sums(x1, x2):
    a11, a21, a12, a22 = _top(x1, 0), _top(x1, 1), _top(x2, 0), _top(x2, 1)
    return [a11 + a22, a21 + a22, a11 + a12, a21 - a11, a12 - a22]


def C(i):
    return slice(i * 128, (i + 1) * 128)


class Unit:
    def __init__(self, name, tiles, epi, rows, cost, nt=False, full=True, acc=False, tail=0):
        self.tail = tail
        self.acc, self.res = acc, []
        self.name, self.tiles, self.epi, self.rows, self.cost, self.nt, self.full = name, tiles, epi, rows, cost, nt, full


class Due:
    def __init__(self, val, delay):
        self.val, self.delay = val, delay


class Group:
    def __init__(self, name, fns, cost, rel, dead, lat, rlat=200):
        self.name, self.fns, self.cost, self.rel, self.dead, self.lat, self.rlat = name, fns, cost, rel, dead, lat, rlat


def _plan(seq, groups):
    busy, n = [0] * 4, 0
    start, end, tiles, bars = {}, {}, [], []
    for it in seq:
        if isinstance(it[0], Unit):
            u = it[0]
            m = n % 4
            n += 1
            t0, t1 = busy[m], busy[m] + max(u.rows, 32)
            busy[m] = t1
            tiles.append((t0, t1, u.cost / len(u.tiles) + (u.tail if it[1] == len(u.tiles) - 1 else 0)))
            start.setdefault(u.name, t0)
            end[u.name] = max(end.get(u.name, 0), t1)
        elif it[0] == "wait":
            t = max(busy)
            busy, n = [t] * 4, 0
            start[it[1]] = end[it[1]] = t
            bars.append(t)
    total = max(busy)
    start["end"] = end["end"] = total
    start["start"] = end["start"] = 0
    ns = total // SLOT + 2
    load = np.zeros(ns)
    for t0, t1, c in tiles:
        a, b = t0 // SLOT, max(t1 // SLOT, t0 // SLOT + 1)
        load[a:b] += c / (b - a)
    win = []
    for g in groups:
        r = max(end[x] + (0 if start[x] == end[x] else g.rlat) for x in g.rel)
        d = min(start[x] for x in g.dead) - g.lat
        ok = np.zeros(ns, bool)
        ok[r // SLOT:max(d // SLOT, r // SLOT + 1)] = True
        for b in bars:
            if r < b <= d:
                ok[max((b - g.lat) // SLOT, 0):b // SLOT] = False
        win.append(np.nonzero(ok)[0])
    alloc = [np.zeros(len(w)) for w in win]
    for _ in range(60):
        for i, g in enumerate(groups):
            w = win[i]
            load[w] -= alloc[i]
            base = load[w]
            vol = g.cost * len(g.fns)
            lo, hi = base.min(), base.max() + vol
            for _ in range(50):
                mid = 0.5 * (lo + hi)
                if np.maximum(mid - base, 0).sum() > vol:
                    hi = mid
                else:
                    lo = mid
            alloc[i] = np.maximum(hi - base, 0)
            load[w] += alloc[i]
    times = []
    for i, g in enumerate(groups):
        cum = np.cumsum(alloc[i])
        ts = []
        for k in range(len(g.fns)):
            x = (k + 0.5) * cum[-1] / len(g.fns)
            j = int(np.searchsorted(cum, x))
            prev = cum[j - 1] if j else 0.0
            ts.append(win[i][j] * SLOT + SLOT * (x - prev) / max(alloc[i][j], 1e-9))
        times.append(ts)
    return times


def _emit(seq, groups, zero, wait):
    times = _plan(seq, groups)
    left = {"start": 0}
    for it in seq:
        nm = it[0].name if isinstance(it[0], Unit) else it[1]
        left[nm] = left.get(nm, 0) + 1
    heap, pend, todo, cnt = [], {}, list(range(len(groups))), 0
    busy, n, due = [0] * 4, 0, []

    def release():
        nonlocal cnt
        for i in list(todo):
            g = groups[i]
            if all(left[x] == 0 for x in g.rel):
                todo.remove(i)
                pend[i] = len(g.fns)
                for t, fn in zip(times[i], g.fns):
                    heapq.heappush(heap, (t, cnt, i, fn))
                    cnt += 1

    def force(name):
        nonlocal heap
        for i, g in enumerate(groups):
            if name in g.dead:
                assert i not in todo, (g.name, name)
                if pend[i]:
                    for it in sorted(x for x in heap if x[2] == i):
                        it[3](None)
                    heap = [x for x in heap if x[2] != i]
                    heapq.heapify(heap)
                    pend[i] = 0

    release()
    for it in seq:
        if isinstance(it[0], Unit):
            u, k = it
            force(u.name)
            lhs, rhs = u.tiles[k]()
            t0 = busy[n % 4]
            while u.full and due and due[0][0] < t0 + u.rows:
                t, x = due.pop(0)
                r = min(max(int(t - t0), 0), u.rows - 1) // 16 * 8
                w = pltpu.bitcast(lhs, U32)
                x = pltpu.bitcast(x[:, :128], U32)
                parts = [w[:r], w[r:r + 8] | ((x[0:8] | x[8:16]) & zero), w[r + 8:]]
                lhs = pltpu.bitcast(jnp.concatenate([y for y in parts if y.shape[0]], axis=0), BF16)
            dn = (((1,), (1 if u.nt else 0,)), ((), ()))
            p = lax.dot_general(lhs, rhs, dn, preferred_element_type=F32)
            u.res = [p + u.res[0]] if (u.acc and u.res) else u.res + [p]
            m = n % 4
            n += 1
            t0 = busy[m]
            busy[m] = t0 + max(u.rows, 32)
            while u.full and heap and heap[0][0] < t0 + u.rows:
                t, _, i, fn = heapq.heappop(heap)
                pend[i] -= 1
                r = min(max(int(t - t0), 0), u.rows - 1) // 8 * 8
                x = fn(pltpu.bitcast(p[r:r + 8], U32) & zero)
                if isinstance(x, Due):
                    due.append((t + x.delay, x.val))
                    due.sort(key=lambda e: e[0])
            if k == len(u.tiles) - 1:
                u.epi(u.res)
            left[u.name] -= 1
        elif it[0] == "wait":
            force(it[1])
            wait(it[1])
            busy, n, due = [max(busy)] * 4, 0, []
            left[it[1]] -= 1
        else:
            it[2]()
            left[it[1]] -= 1
        release()
    force("end")
    assert not heap and not todo


def _sum(ps):
    acc = ps[0]
    for p in ps[1:]:
        acc = acc + p
    return acc


def _flat(us):
    return [(u, i) for u in us for i in range(len(u.tiles))]


def _weave(a, b):
    out = []
    for i, u in enumerate(a):
        out += [u] + b[i * len(b) // len(a):(i + 1) * len(b) // len(a)]
    return out


def _phase(seq):
    n = 0
    for it in seq:
        n = n + 1 if isinstance(it[0], Unit) else (0 if it[0] in ("wait", "sync") else n)
    return n % 4


def _mix(seq, a, b, lo=0.0, hi=1.0):
    n, k = _phase(seq), 0
    for i, t in enumerate(a):
        if k < len(b) and n % 4 == 0 and t[1] != 1 and i >= len(a) * (lo + (hi - lo) * k / len(b)):
            seq.extend(b[k])
            k += 1
        seq.append(t)
        n += 1
    assert k == len(b)


def _wait(seq, name, head=(), back=0):
    r = _phase(seq) + 4 * back
    assert all(isinstance(it[0], Unit) for it in seq[len(seq) - r:])
    seq[len(seq) - r:len(seq) - r] = [("wait", name)] + list(head)


def kernel(q_hbm, k_hbm, v_hbm, sh_hbm, ssm_hbm, sd_hbm, w1_hbm, w2_hbm, w3_hbm, w4_hbm, c_hbm, wm_hbm,
           o_hbm,
           q_n, k_n, v_n, ssm_w, w1_w, w2_w, w3_w, w4_w, wm_w, o_v,
           sh_v, sd_v, c_v, zsrc, z_s, taps, mod_v, tf_w, tg_w,
           kf, uf, acc, zraw, kv_w, zz_w, y_v, x_v, hb_v, x1_v, r_v, n1_w, n2_w, g_w, h1_v, a_w,
           ws_w, as_w, w3n_w, top_v, st_v, l2_w,
           sem, sem_b, sem_o):
    bf = lambda r: r.bitcast(BF16)
    w1_v, w2_v, w3_v, w4_v = bf(w1_w), bf(w2_w), bf(w3_w), bf(w4_w)
    wm_v = {0: bf(wm_w[0]), 3: bf(wm_w[1]), 5: bf(wm_w[2])}
    tf_v, tg_v, n1_v, n2_v, g_v = bf(tf_w), bf(tg_w), bf(n1_w), bf(n2_w), bf(g_w)
    a_v, kv_v, zz_v = bf(a_w), bf(kv_w), bf(zz_w)
    w1s, w2s, w3s, w4s = [bf(r) for r in ws_w]
    n1s, gs, n2s, a_s = [bf(r) for r in as_w]
    w3n = bf(w3n_w)
    w3t, w4t, n2t, a_t = [bf(r) for r in l2_w]
    cp = pltpu.make_async_copy
    cat = lambda ls: [x for l in ls for x in l]

    def base(j, n):
        return j * n if isinstance(j, int) else pl.multiple_of(j * n, n)

    def rows(j, n=1, size=T):
        return pl.ds(base(j, size), n * size)

    def view(ref, j, size=T):
        return ref.at[rows(j, 1, size)]

    dmas = {}

    def group(name, *mks):
        sm = sem.at[len(dmas)]
        dmas[name] = [c for mk in mks for c in mk(sm)]

    def ssm_in(t):
        return lambda sm: [cp(ssm_hbm.at[C(t)], bf(ssm_w[t]), sm)]

    def cols(src, start, n, dst, row=0):
        return lambda sm: [cp(src.at[pl.ds(start, n), C(t)], bf(dst).at[t, pl.ds(row, n)], sm) for t in range(NT)]

    def kv_in(s, sl):
        if isinstance(s, int):
            kk = cols(k_hbm, s * T - 16, T + 16, k_n[sl]) if s else cols(k_hbm, 0, T, k_n[sl], 16)
        else:
            kk = cols(k_hbm, pl.multiple_of(s * T - 16, 16), T + 16, k_n[sl])
        return lambda sm: kk(sm) + cols(v_hbm, base(s, T), T, v_n[sl])(sm)

    def q_in(s, sl):
        return cols(q_hbm, base(s, T), T, q_n[sl])

    def wm_in(a, b):
        return lambda sm: [cp(wm_hbm.at[:, a * D:b * D], wm_v[a], sm)]

    def whole(src, dst):
        return lambda sm: [cp(src, dst, sm)]

    next_kv = lambda s: kv_in(s, 0)(sem_b.at[0])
    next_q = lambda s: q_in(s, 0)(sem_b.at[0])

    zsrc[...] = jnp.zeros((8, 128), I32)
    k_n[0][:, 0:8, :] = jnp.zeros((NT, 8, 128), U32)
    w4_w[F // 2:FT * 64, :] = jnp.zeros((FT * 64 - F // 2, D), U32)
    group("small", lambda sm: [cp(zsrc, z_s, sm), cp(sh_hbm, sh_v, sm), cp(sd_hbm, sd_v, sm), cp(c_hbm, c_v, sm)])
    for s in range(NC):
        group("c%d" % s, ssm_in(s), kv_in(s, s))
    group("c3", ssm_in(3), ssm_in(4))
    group("wma", wm_in(0, 3), q_in(0, 0), q_in(1, 1))
    group("wmb", wm_in(3, 5))
    group("w1", whole(w1_hbm, w1_v))
    group("w2", q_in(2, 2), whole(w2_hbm, w2_v))
    group("w3", whole(w3_hbm, w3_v))
    group("w4", whole(w4_hbm, w4_v.at[0:F]), wm_in(5, 6))
    for g in dmas.values():
        for c in g:
            c.start()

    def wait(name):
        for c in dmas[name]:
            c.wait()

    tau_b = lambda l: H + ((l + (H - 1)) & (H - 1))
    tf_v[:, C(0)] = _dft((T, H), 0, lambda l: jnp.where((l & 1) == 0, l, tau_b(l)), 1.0 / T)
    tf_v[:, C(1)] = _dft((T, H), 0, lambda l: jnp.where((l & 1) == 1, l, tau_b(l)), 1.0 / T)
    tf_v[:, C(2)] = _dft((T, H), 0, lambda l: 2 * l - H)
    tf_v[:, C(3)] = _dft((T, H), 0, lambda l: 2 * l + 1 - H)
    sin0 = lax.broadcasted_iota(I32, (GR, T), 1) >= H
    tg_v[:, 0:T] = _dft((GR, T), 1, lambda l: jnp.where(sin0 & (l == 0), H, 2 * l))
    tg_v[:, T:2 * T] = _dft((GR, T), 1, lambda l: 2 * l + 1)
    h1_v[:, 0:8, :] = jnp.zeros((NT, 8, 128), F32)
    h1_v[:, 8 + NC * T:16 + NC * T, :] = jnp.zeros((NT, 8, 128), F32)

    wait("small")
    z = jnp.clip(z_s[0, 0], 0, 1)
    zero = jnp.full((8, 128), z, I32).astype(U32)
    z8 = pl.multiple_of(z * 8, 8)
    for r in (x_v, hb_v, x1_v, r_v, zraw, n1_w, n2_w, g_w, a_w, kv_w, zz_w, *ws_w, *as_w, w3n_w, top_v, st_v, *l2_w):
        r[pl.ds(z8, 8), 0:128] = jnp.zeros((8, 128), r.dtype)
    for r in (kf, uf, acc, taps, mod_v):
        r[z, 0:8, 0:128] = jnp.zeros((8, 128), r.dtype)
    for r in (tf_w, tg_w):
        r[pl.ds(z8, 8), 0:128] = r[0:8, 0:128]
    sh = sh_v[...].astype(F32)
    for i in range(4):
        taps[i] = jnp.broadcast_to(sh[i:i + 1], (8, D))
    taps[4] = jnp.broadcast_to(sd_v[...].astype(F32).reshape(1, D) * (1.0 / T), (8, D))
    cf = c_v[...].astype(F32)
    silu_c = jnp.broadcast_to((cf / (1.0 + jnp.exp(-cf))).astype(BF16), (16, D))

    def mmK(n):
        def unit(m):
            st = []

            def rhs(i):
                if not st:
                    ev = (lax.broadcasted_iota(I32, (64, 128), 1) & 1) == 0
                    a = ssm_w[n][:, m * T:m * T + H]
                    b = pltpu.roll(ssm_w[n][:, m * T + H:(m + 1) * T], 1, 1)
                    st.extend([pltpu.bitcast(jnp.where(ev, a, b), BF16), pltpu.bitcast(jnp.where(ev, b, a), BF16)])
                return st[i]

            def epi(p):
                er, ei, or_, oi = p
                cur = [er, ei, or_, oi]
                if m:
                    pv = [zraw[C(4 * ((m - 1) % 2) + (q ^ 1)), :] for q in range(4)]
                    pm = lambda x, y, up: jnp.concatenate([x[:64] + y[:64], x[64:] - y[64:]] if up else
                                                          [x[:64] - y[:64], x[64:] + y[64:]], axis=0)
                    er, ei, or_, oi = [pm(cur[q], pv[q], q & 1) for q in range(4)]
                else:
                    er = er + taps[4, 0:1, C(n)]
                if m + 1 < NB:
                    for q in range(4):
                        zraw[C(4 * (m % 2) + q), :] = cur[q]
                for h, (cr, ci) in enumerate(((er + or_, ei + oi), (er - or_, ei - oi))):
                    B = h * 3 * H
                    kf[m, B:B + H, C(n)] = cr
                    kf[m, B + H:B + 2 * H, C(n)] = ci - cr
                    kf[m, B + 2 * H:B + 3 * H, C(n)] = ci + cr
            return Unit("K%d" % n, [(lambda i=i, r=r: (tf_v[r:r + H, C(i)], rhs(i))) for i in range(2) for r in (0, H)],
                        epi, H, 260, nt=True)
        return [unit(m) for m in range(NB)]

    def kv(s, sl):
        def mk(t, w):
            def fn(a):
                ld = lambda o, n: k_n[s][t, pl.ds(8 + w + o, n), :]
                c0 = jnp.concatenate([_tie(ld(0, 8), a), ld(8, 8)], axis=0).reshape(2, 8, 128)
                c1, c2 = ld(-1, 16).reshape(2, 8, 128), ld(-2, 16).reshape(2, 8, 128)
                s0, s1, s2, s3 = (taps[i, :, C(t)] for i in range(4))
                ke, ko, ke1, ko1, ko2 = _lo(c0), _hi(c0), _lo(c1), _hi(c1), _hi(c2)
                wv = v_n[s][t, w:w + 16, :].reshape(2, 8, 128)
                kve = ((s0 * ke + s1 * ko1) + (s2 * ke1 + s3 * ko2)) * _lo(wv)
                kvo = ((s0 * ko + s1 * ke) + (s2 * ko1 + s3 * ke1)) * _hi(wv)
                kv_v[pl.ds(sl * T + w, 16), C(t)] = kve.reshape(16, 128).astype(BF16)
                kv_v[pl.ds(sl * T + H + w, 16), C(t)] = kvo.reshape(16, 128).astype(BF16)
            return fn
        return [[mk(t, w) for w in range(0, H, 16)] for t in range(NT)]

    def mmU(name, sl, us):
        def unit(n):
            def epi(p):
                er, ei, or_, oi = p
                for h, (cr, ci) in enumerate(((er + or_, ei + oi), (er - or_, ei - oi))):
                    B = h * 3 * H
                    uf[us, B:B + H, C(n)] = cr + ci
                    uf[us, B + H:B + 2 * H, C(n)] = cr
                    uf[us, B + 2 * H:B + 3 * H, C(n)] = ci
            return Unit(name(n), [(lambda i=i, r=r: (tf_v[r:r + H, C(2 + i)], kv_v[pl.ds(sl * T + i * H, H), C(n)]))
                                  for i in range(2) for r in (0, H)], epi, H, 96 + 96 * KS)
        return [unit(n) for n in range(NT)]

    def cmul(m0, u0, n, h, row, L, a):
        t = []
        for i in range(3):
            Rw = slice((3 * h + i) * H + row, (3 * h + i) * H + row + 8)
            kk = kf[m0:m0 + n, Rw, L]
            if i == 0 and a is not None:
                k0 = _tie(kk[0], a)[None]
                kk = k0 if n == 1 else jnp.concatenate([k0, kk[1:]], axis=0)
            t.append(jnp.sum(kk * uf[u0:u0 + n, Rw, L], axis=0))
        return t[0] - t[2], t[0] + t[1]

    def AR(h, q, row):
        return slice((2 * h + q) * H + row, (2 * h + q) * H + row + 8)

    def mac(n, u0, sl, part=False):
        def mk(t, rc):
            st, fin = [], []

            def piece(i):
                def fn(a):
                    h, row = i & 1, rc + (i >> 1) * 8
                    zr, zi = cmul(0, u0, n, h, row, C(t), a)
                    if part:
                        zr, zi = zr + acc[0, AR(h, 0, row), C(t)], zi + acc[0, AR(h, 1, row), C(t)]
                    st.append((zr, zi))
                    if h:
                        (pr, pi), (mr, mi) = st[-2:]
                        fin.append([pr + mr, pi + mi, pr - mr, pi - mi])
                    if i == 3:
                        for q in range(4):
                            zz_v[pl.ds(sl * 2 * T + q * H + rc, 16), C(t)] = jnp.concatenate(
                                [fin[0][q], fin[1][q]], axis=0).astype(BF16)
                return fn
            if not part:
                return [piece(i) for i in range(4)]
            both = lambda f, g: (lambda a: (f(a), g(None)))
            return [both(piece(0), piece(1)), both(piece(2), piece(3))]
        return [[fn for rc in range(0, H, 16) for fn in mk(t, rc)] for t in range(NT)]

    def pos():
        return [(t, h, row) for t in range(NT) for row in range(0, H, 8) for h in range(2)]

    def ahead(i):
        def mk(t, h, row):
            def fn(a):
                zr, zi = cmul(i + 1, 0, NC, h, row, C(t), a)
                acc[i, AR(h, 0, row), C(t)] = zr
                acc[i, AR(h, 1, row), C(t)] = zi
            return fn
        return [mk(*p) for p in pos()]

    def spread():
        n = NB - NC - 1

        def mk(t, h, row):
            def fn(a):
                p = []
                for i in range(3):
                    Rw = slice((3 * h + i) * H + row, (3 * h + i) * H + row + 8)
                    u = uf[0, Rw, C(t)]
                    p.append(kf[1:1 + n, Rw, C(t)] * (_tie(u, a) if i == 0 else u)[None])
                acc[0:n, AR(h, 0, row), C(t)] = acc[1:1 + n, AR(h, 0, row), C(t)] + (p[0] - p[2])
                acc[0:n, AR(h, 1, row), C(t)] = acc[1:1 + n, AR(h, 1, row), C(t)] + (p[0] + p[1])
            return fn
        return [mk(*p) for p in pos()]

    def mmI(name, sl, ys):
        def unit(n):
            def epi(p):
                ce, se, co, so = p
                sub = lax.broadcasted_iota(I32, (8, 128), 0)
                b0 = ys * (T + 8) + 8
                y_v[n, b0 + H - 1:b0 + H, :] = (ce[64:72] - se[0:8])[0:1]
                se = jnp.concatenate([jnp.where(sub == 0, 0.0, se[0:8]), se[8:]], axis=0)
                for d, cc, ss in ((0, ce[0:64], se), (1, co, so)):
                    y_v[n, pl.ds(b0 + H + d, 64, stride=2), :] = cc + ss
                    y_v[n, pl.ds(b0 + d - 1, 64, stride=2), :] = cc - ss
            return Unit(name(n), [(lambda i=i: (tg_v[0:(GR if i == 0 else 64), C(i)], zz_v[pl.ds(sl * 2 * T + i * H, H), C(n)]))
                                  for i in range(4)], epi, 64, 36 + 33 * KS)
        return [unit(n) for n in range(NT)]

    def mod(name, a, b):
        def unit(n):
            def epi(p):
                v = [_sum(p[i * NT:(i + 1) * NT])[0:8] for i in range(b - a)]
                if a == 0:
                    mod_v[0, :, C(n)] = v[0] * v[2]
                    mod_v[1, :, C(n)] = (v[1] + 1.0) * v[2]
                elif a == 3:
                    mod_v[3, :, C(n)] = v[0] * (1.0 / G_POST)
                    mod_v[4, :, C(n)] = (v[1] + 1.0) * (1.0 / G_POST)
                else:
                    mod_v[2, :, C(n)] = v[0] * G_POST
            return Unit(name, [(lambda i=i, k=k: (silu_c[:, C(k)], wm_v[a][C(k), pl.ds(i * D + n * 128, 128)]))
                               for i in range(b - a) for k in range(NT)], epi, 16, 10, full=False, acc=b - a == 1)
        return [unit(n) for n in range(NT)]

    HS = (slice(0, 128), slice(128, 256))
    QS = tuple(slice(r, r + 64) for r in range(0, T, 64))

    def tasks(f, due=None, tie=True, n=RG):
        def mk(R):
            def fn(a):
                x = f(R, a if tie else None)
                return Due(x, due) if due else None
            return fn
        return [mk(slice(r, r + n)) for r in range(0, T, n)]

    def load_y(sl, R):
        b0, back = sl * (T + 8) + 8, 7 - lax.broadcasted_iota(I32, (8, 128), 0)

        def ld(t, r):
            if r >= H:
                return y_v[t, b0 + r:b0 + r + 8, :]
            return jnp.take_along_axis(y_v[t, b0 + H - 8 - r:b0 + H - r, :], back, axis=0)
        return jnp.stack([jnp.concatenate([ld(t, r) for t in range(NT)], axis=1) for r in (R.start, R.start + 8)])

    def put(nn, ss, R, x):
        nn[R, :] = x.astype(BF16)
        tok = x
        if ss is not None:
            S2 = pl.ds(R.start // 32 * 16, 16)
            if R.stop % 32:
                top_v[S2, 0:2 * T] = x[:, 0:2 * T]
            else:
                if R.start % 32:
                    x = jnp.concatenate([top_v[S2, 0:2 * T], x[:, 0:2 * T]], axis=0)
                ss[S2, 0:5 * T] = jnp.concatenate(_lhs_sums(x[:, 0:T], x[:, T:2 * T]), axis=1).astype(BF16)
        return tok

    wide = lambda v: jnp.concatenate([v] * NT, axis=1)

    def mean(i, R, x):
        st_v[R, C(i)] = jnp.broadcast_to(jnp.sum(x, axis=-1, keepdims=True) * (1.0 / D), (x.shape[0], 128))

    def centred(src, i, R, a):
        return src[R, :] - wide(_tie(st_v[R, C(i)], a))

    def scale(src, i, g):
        def f(R, a):
            st_v[R, C(i + 1)] = jnp.broadcast_to(_rstd(centred(src, i, R, a), g), (RG, 128))
        return f

    def normed(src, i, R, a):
        return centred(src, i, R, a) * wide(st_v[R, C(i + 1)])

    def front(sl, xs, early=False, ss=None):
        xx, hh, nn = view(x_v, xs), view(hb_v, xs), view(n1_v, sl)

        def fa(R, a):
            q = [q_n[sl][t, R.start // 2:R.stop // 2, :] for t in range(NT)]
            q = jnp.concatenate([_tie(q[0], a)] + q[1:], axis=1)
            q = pltpu.bitcast(q, BF16).astype(F32).reshape(2, 8, D)
            x = (q + (_ln(q) * mod_v[1] + mod_v[0]) * load_y(sl, R)).reshape(RG, D)
            xx[R, :] = x
            if early:
                hh[R, :] = _ln(x)

        def fb(R, a):
            hh[R, :] = (_ln(_tie(xx[R, :], a).reshape(2, 8, D)) * mod_v[4] + mod_v[3]).reshape(RG, D)

        def fc(R, a):
            hb = _tie(hh[R, :], a)
            if early:
                hb = (hb.reshape(2, 8, D) * mod_v[4] + mod_v[3]).reshape(RG, D)
                hh[R, :] = hb
            nn[R, :] = _ln(hb, True).astype(BF16)
        if early:
            return tasks(fa), tasks(fc)
        if ss is None:
            return tasks(fa) + tasks(fb) + tasks(fc)
        qf = view(x_v, 2)

        def s1(R, a):
            q = [q_n[sl][t, R.start // 2:R.stop // 2, :] for t in range(NT)]
            q = pltpu.bitcast(jnp.concatenate([_tie(v, a) for v in q], axis=1), BF16).astype(F32)
            qf[R, :] = q
            mean(0, R, q)

        def s3(R, a):
            h = normed(qf, 0, R, a).reshape(2, 8, D) * mod_v[1] + mod_v[0]
            x = qf[R, :] + (h * load_y(sl, R)).reshape(RG, D)
            xx[R, :] = x
            mean(2, R, x)

        def s5(R, a):
            hb = (normed(xx, 2, R, a).reshape(2, 8, D) * mod_v[4] + mod_v[3]).reshape(RG, D)
            hh[R, :] = hb
            mean(4, R, hb)
        s7 = [f for g in tasks(lambda R, a: put(nn, ss, R, normed(hh, 4, R, a)), n=32) for f in (g, lambda a: None)]
        st = [tasks(s3), tasks(scale(xx, 2, False)), tasks(s5), tasks(scale(hh, 4, True)), s7]
        p = [tasks(s1), tasks(scale(qf, 0, False))]
        sk = 4.091

        def wave(ls):
            body = sorted((i * sk + g, i, g) for i in range(len(ls) - 1) for g in range(8))
            return [ls[i][g] for _, i, g in body] + ls[-1]
        qb = []
        done = lambda a: qb[0]()
        full = wave([x[8:] for x in p + st])
        k = full.index(p[0][15]) + 1
        return wave([x[:8] for x in st]), full[:k] + [done] + full[k:], cat(x[:8] for x in p), qb

    def shift(hs, sl, pieces=((0, 64), (64, 64), (128, 64), (192, 64)), ss=None):
        gg = view(g_v, sl)

        def one_tile(t, r, n, a):
            lane = lax.broadcasted_iota(I32, (n, 128), 1)
            ld = lambda d: h1_v[t, pl.ds(hs * T + 8 + r + d, n), :]
            if t == 0:
                g = ld(-1)
            elif t == 1:
                g = jnp.where(lane < 32, ld(-1), ld(1))
            elif t == 2:
                g = jnp.where(lane < 64, ld(1), ld(-2))
            elif t == 3:
                g = jnp.where(lane < 96, ld(-2), ld(2))
            else:
                g = ld(2)
            if a is not None:
                g = jnp.concatenate([_tie(g[i:i + 8], a) if i % 16 == 0 else g[i:i + 8]
                                     for i in range(0, n, 8)], axis=0)
            gg[r:r + n, C(t)] = g.astype(BF16)
            return g

        def mk(ts, r, n):
            def fn(a):
                g = [one_tile(t, r, n, a) for t in ts]
                if len(ts) == 2:
                    for i, x in enumerate(_lhs_sums(*g)):
                        ss[r // 2:(r + n) // 2, C(2 * i + ts[0])] = x.astype(BF16)
            return fn
        sets = [(t,) for t in range(NT)] if ss is None else [(0, 2), (1, 3), (4,)]
        return [mk(ts, r, n) for ts in sets for r, n in pieces]

    def shift_early():
        def keep(a):
            h1_v[:, 2 * T - 32:2 * T + 8, :] = h1_v[:, 3 * T - 32:3 * T + 8, :]
        return shift(2, 0, [(r, 32) for r in range(0, T - 32, 32)], gs) + [keep]

    def ln2(xs, sl, fast=True):
        xx, nn, ss = view(x1_v, xs), view(n2_v, sl), view(n2s, sl, H) if fast else None
        f = lambda R, a: put(nn, ss, R, _ln(_tie(xx[R, :], a), True))
        ts = tasks(f, 900) if sl else tasks(f, DL, False)
        return ts[0::2] + ts[1::2] if fast else tasks(f)

    def ln2_late():
        xx, nn, ss = view(x1_v, 0), view(n2_v, 0), view(n2s, 0, H)
        a_, b_ = tasks(lambda R, a: mean(6, R, _tie(xx[R, :], a))), tasks(scale(xx, 6, True))
        c_ = [f for g in tasks(lambda R, a: put(nn, ss, R, normed(xx, 6, R, a)), n=32)[:4] for f in (g, lambda a: None)]
        return a_[:8] + b_[:8] + c_

    def resid(xs, x1s, rotate=False):
        xx, x1 = view(x_v, xs), view(x1_v, x1s)

        def f(R, a):
            tie = lambda v: v if a is None else pltpu.bitcast(pltpu.bitcast(v, U32) | wide(a), F32)
            r_v[R, :] = xx[R, :] + (x1[R, :].reshape(2, 8, D) * tie(mod_v[2])).reshape(RG, D)
            if rotate:
                xx[R, :] = tie(x_v[R, :].reshape(2, 8, D)).reshape(RG, D)
                view(hb_v, 1)[R, :] = tie(hb_v[R, :].reshape(2, 8, D)).reshape(RG, D)
        return tasks(f)

    KD, KF, ND = [(0, 2), (1, 3)], [(2 * i, 2 * i + 1) for i in range(7)], [(1, 2), (3, 4)]
    Wt = {1: (lambda k, n: w1_v[C(k), C(n)], lambda i, kp, j: w1s[C(kp), C(2 * i + j)], False, KD, [4]),
          2: (lambda k, n: w2_v[C(k), C(n)], lambda i, kp, j: w2s[C(kp), C(2 * i + j)], False, KD, [4]),
          0: (lambda k, n: w3_v[C(n), C(k)], None, True, KD, [4]),
          3: (lambda k, n: w3n[C(k), C(n)], lambda i, kp, j: w3s[C(kp), C(6 * i + j)], False, KD, [4]),
          4: (lambda k, n: w4_v[C(k), C(n)], lambda i, kp, j: w4s[C(kp), C(2 * i + j)], False, KF, [])}

    def sums_task(load, store, left):
        def fn(a):
            b = [[load(u, v) for v in range(2)] for u in range(2)]
            b[0][0], b[1][1] = _tie(b[0][0], a), _tie(b[1][1], a)
            (x11, x12), (x21, x22) = [[pltpu.bitcast(x, BF16).astype(F32) for x in row] for row in b]
            r = ((x11 + x22, x21 + x22, x11 + x12, x21 - x11, x12 - x22) if left else
                 (x11 + x22, x12 - x22, x21 - x11, x11 + x12, x21 + x22))
            for m, x in enumerate(r):
                store(m, x.astype(BF16))
        return fn

    def wsums(w_w, ws, rp, cp_):
        def mk(i, j, r):
            def store(m, x):
                ws[pl.ds(128 * i + r, 16), C(len(cp_) * m + j)] = x
            return sums_task(lambda u, v: w_w[pl.ds(64 * rp[i][u] + r // 2, 8), C(cp_[j][v])], store, False)
        return [mk(i, j, r) for j in range(len(cp_)) for i in range(len(rp)) for r in range(0, 128, 16)]

    def w3_turn():
        def mk(n, k):
            def fn(a):
                x = jnp.concatenate([_tie(w3_w[64 * n:64 * n + 8, C(k)], a), w3_w[64 * n + 8:64 * n + 64, C(k)]], axis=0)
                w3n[C(k), C(n)] = pltpu.bitcast(x, BF16).T
            return fn
        return [mk(n, k) for n in range(FT - 1) for k in range(NT)]

    def plain(name, w, lhs, n, R, epi, cost):
        tile, _, nt, kp, kl = Wt[w]
        ks = sorted([k for p in kp for k in p] + kl)
        rows_ = R.stop - R.start
        return Unit(name, [(lambda k=k: (lhs[R, C(k)], tile(k, n))) for k in ks], lambda p: epi(n, R, p[0]),
                    rows_, rows_ // 8 * (len(ks) - 1), nt=nt, acc=True, tail=rows_ // 8 * cost(n))

    def quad(name, w, lhs, sums, j, cols_, R, epi, cost):
        tile, wsum, nt, kp, kl = Wt[w] if isinstance(w, int) else w
        h, S2, c = len(kp), slice(R.start // 2, R.stop // 2), {}
        a_ = lambda i, k: _top(lhs(k) if callable(lhs) else lhs[R, C(k)], i)
        s_ = sums if callable(sums) else (lambda i, p: sums[S2, C(h * i + p)])
        prod = lambda fa_, fb_: [(lambda p=p: (fa_(p), fb_(p))) for p in range(h)]
        left = lambda i, n: [(lambda k=k: (a_(i, k), tile(k, n))) for k in kl]
        mk = lambda tiles, f, x=0: Unit(name, tiles, lambda p: f(p[0]), 64, 8 * len(tiles), nt=nt, acc=True, tail=x)

        def e1(m):
            u7.res, u6.res = [m], [m]

        def e4(m):
            c[11], c[21] = c[11] + m, m

        def e2(m):
            c[21], c[22] = c[21] + m, c[22] - m
            l21.res = [c[21]]

        def e5(m):
            c[12] = m
            epi(cols_[0], R, _zip(c[11] - m, c[21]))

        def e3(m):
            l12.res, c[22] = [c[12] + m], c[22] + m
            if not kl:
                l12.epi(l12.res)
        u1 = mk(prod(lambda p: s_(0, p), lambda p: wsum(0, p, j)), e1)
        u7 = mk(prod(lambda p: s_(4, p), lambda p: wsum(4, p, j)) + left(0, cols_[0]), lambda m: c.update({11: m}))
        u6 = mk(prod(lambda p: s_(3, p), lambda p: wsum(3, p, j)) + left(1, cols_[1]), lambda m: c.update({22: m}))
        u4 = mk(prod(lambda p: a_(1, kp[p][1]), lambda p: wsum(2, p, j)), e4)
        u2 = mk(prod(lambda p: s_(1, p), lambda p: tile(kp[p][0], cols_[0])), e2, 8)
        l21 = mk(left(1, cols_[0]), lambda m: c.update({21: m}))
        u5 = mk(prod(lambda p: s_(2, p), lambda p: tile(kp[p][1], cols_[1])), e5, 16 * cost(cols_[0]))
        u3 = mk(prod(lambda p: a_(0, kp[p][0]), lambda p: wsum(1, p, j)), e3, 8 if kl else 8 + 16 * cost(cols_[1]))
        l12 = mk(left(0, cols_[1]), lambda m: epi(cols_[1], R, _zip(m, c[22])), 16 * cost(cols_[1]))
        return [u1, u7, u6, u4, u2, l21, u5, u3, l12]

    LH, RH = [0, 4, 3, (1, 1), 1, 2, (0, 0)], [0, 4, 3, 2, (0, 0), (1, 1), 1]
    L2 = {3: (w3n_w, ws_w[2], w3t, KF[:6], n2t), 4: (w4_w, ws_w[3], w4t, ND, a_t)}

    def wsums2(w):
        w_w, s_w, ws2, cp_, _ = L2[w]
        kp, nj = Wt[w][3], len(cp_)

        def mk(o, p2, j2, r):
            def load(u, v):
                p, j, y = 2 * p2 + u, 2 * j2 + v, RH[o]
                if isinstance(y, int):
                    return s_w[pl.ds(64 * p + r // 2, 8), C(nj * y + j)]
                return w_w[pl.ds(64 * kp[p][y[0]] + r // 2, 8), C(cp_[j][y[1]])]

            def store(m, x):
                ws2[pl.ds(128 * p2 + r, 16), C((5 * o + m) * (nj // 2) + j2)] = x
            return sums_task(load, store, False)
        return [mk(o, p2, j2, r) for j2 in range(nj // 2) for o in range(7) for p2 in range(len(kp) // 2)
                for r in range(0, 128, 16)]

    def wsums4():
        form = [((0, 0), (1, 1), 1), ((0, 1), (1, 1), -1), ((1, 0), (0, 0), -1), ((0, 0), (0, 1), 1), ((1, 0), (1, 1), 1)]

        def mk(o, p2, r):
            def fn(a):
                def blk(p, j, uv, t):
                    x = w4_w[pl.ds(64 * KF[p][uv[0]] + r // 2, 8), C(ND[j][uv[1]])]
                    return pltpu.bitcast(_tie(x, t), BF16).astype(F32)
                y = {}
                for u in range(2):
                    for j in range(2):
                        p = 2 * p2 + u
                        if isinstance(RH[o], int):
                            f = form[RH[o]]
                            x1, x2 = blk(p, j, f[0], a), blk(p, j, f[1], None)
                            y[u, j] = x1 + x2 if f[2] > 0 else x1 - x2
                            w4s[pl.ds(128 * p + r, 16), C(2 * RH[o] + j)] = y[u, j].astype(BF16)
                        else:
                            y[u, j] = blk(p, j, RH[o], a if u == j else None)
                for m, f in enumerate(form):
                    x = y[f[0]] + y[f[1]] if f[2] > 0 else y[f[0]] - y[f[1]]
                    w4t[pl.ds(128 * p2 + r, 16), C(5 * o + m)] = x.astype(BF16)
            return fn
        last = wsums(w4_w, w4s, KF, ND)
        return (last[48:56] + last[104:112]
                + [mk(o, p2, r) for o in range(7) for p2 in range(3) for r in range(0, 128, 16)])

    def lsums2(w, lhs_w, sums_w, sl):
        kp, xs2 = Wt[w][3], L2[w][4]
        h2 = len(kp) // 2

        def mk(o, p2, g):
            def load(u, v):
                p, ch, x = 2 * p2 + v, 2 * g + u, LH[o]
                if isinstance(x, int):
                    return sums_w[pl.ds(64 * sl + 8 * ch, 8), C(len(kp) * x + p)]
                return lhs_w[pl.ds(H * sl + 16 * ch + 8 * x[0], 8), C(kp[p][x[1]])]

            def store(m, x):
                xs2[pl.ds(16 * g, 16), C((5 * o + m) * h2 + p2)] = x
            return sums_task(load, store, True)
        return [[mk(o, p2, g) for o in range(7) for g in range(4)] for p2 in range(h2)]

    def quad2(name, w, lhs, sums, j2, epi, cost):
        tile, wsum, nt, kp, kl = Wt[w]
        ws2, cp_, xs2 = L2[w][2:]
        h, h2, nj2, c, R = len(kp), len(kp) // 2, len(cp_) // 2, {}, slice(0, T)

        def done(j, v):
            val = _zip(c[j, 1, v], c[j, 2, v])
            if not kl:
                return epi(cp_[j][v], R, val)
            c[j, v] = val

        def upd(o, j, m):
            for i, v, sg in (((1, 0, 1), (2, 1, 1)), ((1, 0, 1),), ((2, 1, 1),), ((1, 0, 1), (2, 0, 1)),
                             ((2, 0, 1), (2, 1, -1)), ((1, 0, -1), (1, 1, 1)), ((1, 1, 1), (2, 1, 1)))[o]:
                k = (j, i, v)
                c[k] = m if k not in c else (c[k] + m if sg > 0 else c[k] - m)
            if o >= 5:
                done(j, o - 5)

        def inner(o):
            x, y = LH[o], RH[o]
            xo = ((lambda p: sums[:, C(h * x + p)]) if isinstance(x, int)
                  else (lambda p: _top(lhs[:, C(kp[p][x[1]])], x[0])))
            yo = ((lambda p, j: wsum(y, p, j)) if isinstance(y, int)
                  else (lambda p, j: tile(kp[p][y[0]], cp_[j][y[1]])))
            w_ = (yo, lambda m, p2, _: ws2[C(p2), C((5 * o + m) * nj2 + j2)], nt,
                  [(2 * i, 2 * i + 1) for i in range(h2)], list(range(2 * h2, h)))
            return quad(name, w_, xo, lambda m, p2: xs2[:, C((5 * o + m) * h2 + p2)], 0, (2 * j2, 2 * j2 + 1),
                        HS[0], lambda j, _, m: upd(o, j, m), lambda j: 1.5 + KS + (2 * cost(0) if o >= 5 and not kl else 0))

        def rest(j, v, Q):
            return [Unit(name, [lambda: (lhs[Q, C(k)], tile(k, cp_[j][v]))],
                         lambda p: epi(cp_[j][v], Q, p[0] + c[j, v][Q]), 64, 8 * (cost(cp_[j][v]) + 1)) for k in kl]
        return cat(inner(o) for o in range(7)), [u for Q in QS for j in (2 * j2, 2 * j2 + 1) for v in range(2)
                                                 for u in rest(j, v, Q)]

    def mm(name, w, lhs, sums, epi, cost):
        if sums is None:
            return [[plain(name, w, lhs, n, R, epi, cost) for R in HS] for n in range(NT)]
        return [[plain(name, w, lhs, 0, R, epi, cost) for R in QS]] + [
            [u for R in HS for u in quad(name, w, lhs, sums, j, ND[j], R, epi, cost)] for j in range(2)]

    def mm1(name, hs, sl, fast=False):
        def epi(n, R, p):
            h1_v[n, pl.ds(hs * T + 8 + R.start, R.stop - R.start), :] = _gelu2(p)
        return cat(mm(name, 1, view(n1_v, sl), n1s if fast else None, epi, lambda n: 5 + KS))

    def mm2(name, sl, xs, x1s, fast=False):
        def epi(n, R, p):
            view(x1_v, x1s)[R, C(n)] = view(hb_v, xs)[R, C(n)] + p
        return cat(mm(name, 2, view(g_v, sl), gs if fast else None, epi, lambda n: 1 + KS))

    def mm3(name, sl, fast=True, host=None):
        nn, aa, ss, keep, tail = view(n2_v, sl), view(a_v, sl), view(a_s, sl, H), {}, []

        def epi(n, R, p):
            g = _gelu2(p)
            aa[R, C(n)] = g.astype(BF16)
            if not fast:
                return
            if n % 2 == 0 and n < 12:
                keep[n] = g
                return
            pair = (keep.pop(n - 1), g) if n % 2 else (g, tail[R.start // 128][R.start % 128:R.start % 128 + 64])
            for i, x in enumerate(_lhs_sums(*pair)):
                ss[R.start // 2:R.stop // 2, C(7 * i + n // 2)] = x.astype(BF16)

        c3 = lambda n: 5.5 + 0.5 * KS + (3.75 + 1.25 * KS if fast and (n % 2 or n == 12) else 0)

        def rem(R):
            def f(p):
                tail.append(jnp.concatenate([_gelu2(p[0]), jnp.zeros((64, 128), F32)], axis=0).T)
                aa[R, C(13)] = tail[-1].astype(BF16)
            return Unit(name, [(lambda k=k: (w3_v[13 * 128:F, C(k)], nn[R, C(k)])) for k in range(NT)], f, 64, 84,
                        nt=True, acc=True)
        odd = [rem(R) for R in HS] + [plain(name, 3 if fast else 0, nn, 12, R, epi, c3) for R in QS]
        if not fast:
            return odd + [plain(name, 0, nn, n, R, epi, c3) for p in KF[:6] for R in HS for n in p]
        qd = [quad2(name + "_%d" % j, 3, nn, view(n2s, sl, H), j, epi, c3) for j in range(3)]
        mid = qd[0][0] + _weave(qd[1][0], qd[0][1]) + _weave(qd[2][0], qd[1][1])
        if host is None:
            return odd[:2] + mid + _weave(odd[2:], qd[2][1])
        for u in (odd[0], odd[2], odd[3]):
            u.name = name + "h"
        return [odd[0], odd[2], odd[3], odd[1]] + mid, _weave(odd[4:] + host, qd[2][1])

    def cp_out(j, osl, L, sm, R=slice(0, T)):
        return cp(o_v.at[pl.ds(osl * T + R.start, R.stop - R.start), L],
                  o_hbm.at[pl.ds(base(j, T) + R.start, R.stop - R.start), L], sem_o.at[sm])

    out_a = lambda j: cp_out(j, 0, slice(128, D), 0)
    out_b = lambda j: cp_out(j, 0, C(0), 1)
    last = []

    def mm4(name, j, sl, osl=0, xs=None, x1s=None, fast=True):
        oo = view(o_v, osl)

        def epi(n, R, p):
            if xs is None:
                oo[R, C(n)] = (r_v[R, C(n)] + mod_v[2, 0:1, C(n)] * p).astype(BF16)
            else:
                oo[R, C(n)] = (view(x_v, xs)[R, C(n)] + mod_v[2, 0:1, C(n)]
                               * (view(x1_v, x1s)[R, C(n)] + p)).astype(BF16)
            if osl == 2:
                last.append(cp_out(j, osl, C(n), 2, R))
                last[-1].start()
            elif R.stop == T and osl and n == NT - 1:
                last.append(cp_out(j, osl, slice(128 if osl == 3 else 0, D), 2))
                last[-1].start()
            elif R.stop == T and osl == 0 and n in (0, NT - 1):
                (out_a if n else out_b)(j).start()
        c4 = lambda n: (3 if xs is None else 4) + KS
        if fast:
            return ([plain(name, 4, view(a_v, sl), 0, R, epi, c4) for R in QS],
                    quad2(name + "q", 4, view(a_v, sl), view(a_s, sl, H), 0, epi, c4)[0])
        return mm(name, 4, view(a_v, sl), None, epi, c4)

    def split(us):
        n = 4 // len(us)
        m, mks, st = us[0].rows // n, [u.tiles.pop(0) for u in us], {}

        def piece(i, k):
            if i not in st:
                st[i] = mks[i]()
            return st[i][0][m * k:m * (k + 1)], st[i][1]

        def epi(p):
            for i, u in enumerate(us):
                u.res = [jnp.concatenate(p[n * i:n * (i + 1)], axis=0)]
        return _flat([Unit(us[0].name, [(lambda i=i, k=k: piece(i, k)) for i in range(len(us)) for k in range(n)],
                           epi, m, 0, nt=us[0].nt)])

    W = lambda nm: [("wait", nm)]
    run = lambda fns: [("run", "run", lambda: [fn(None) for fn in fns])]
    one = lambda us: [_flat([u]) for u in us]
    nm = lambda x: (lambda n: x)

    seq, grp = [], []
    for s in range(NC):
        seq += W("c%d" % s) + _flat(mmK(s) + mmU(nm("U%d" % s), s % 2, NC - 1 - s))
        grp.append(Group("kv%d" % s, cat(kv(s, s % 2)), 50, ["c%d" % s], ["U%d" % s], 100))
    inv = [mmI(lambda n: "I%d" % n, s, s) for s in range(NC)]
    seq += W("c3") + _flat(mmK(3) + mmK(4) + [inv[s][t] for t in range(NT) for s in range(NC)])
    macs = [mac(s + 1, NC - 1 - s, s) for s in range(NC)]
    grp.append(Group("mac00", macs[0][0], 12, ["c1"], ["c2"], 0))
    grp.append(Group("mac01", macs[1][0] + macs[0][1] + macs[1][1], 16, ["c2"], ["c3"], 0))
    for t in range(NT):
        grp.append(Group("mac%d" % t, cat(macs[s][t] for s in range(2 if t < 2 else 0, NC)), 24 if t < 2 else 18,
                         ["c3", "K%d" % t], ["I%d" % t], 100, 150))
    start = lambda cs: [("run", "run", lambda: [c.start() for c in cs])]
    f0, f1 = front(0, 2, True), front(1, 1, True)
    seq += run(ahead(0))
    seq += W("wma") + _flat(mod("moda", 0, 3)) + run(f0[0] + f1[0] + ahead(1))
    seq += W("wmb") + start(next_kv(NC) + next_q(NC)) + _flat(mod("modb", 3, 5)) + run(f0[1])
    w1 = _flat(mm1("w1_0", 0, 0) + mm1("w1_1", 1, 1))
    seq += W("w1") + w1[:72] + W("w2") + w1[72:] + run(shift(0, 0))
    seq += _flat(mm2("w2_0", 0, 2, 1) + mm1("w1_2", 2, 2)) + run(shift(1, 1)) + _flat(mm2("w2_1", 1, 1, 0))
    grp.append(Group("f1", f1[1], 80, ["w1"], ["w1_1"], 450))
    grp.append(Group("f2", front(2, 0), 80, ["w2"], ["w1_2"], 450))
    grp.append(Group("ln2_0", ln2(1, 0, False), 60, ["w2_0"], ["w3"], 450))
    grp.append(Group("ahead", cat(ahead(i) for i in range(2, NB - NC)), 19 + 2 * KS, ["w1"], ["end"], 100))
    grp.append(Group("ws1", wsums(w1_w, w1s, KD, ND), 26 + 5 * KS, ["w1"], ["end"], 100))
    grp.append(Group("ws2", wsums(w2_w, w2s, KD, ND), 26 + 5 * KS, ["w2"], ["end"], 100))
    grp.append(Group("ws3", w3_turn() + wsums(w3n_w, w3s, KD, KF[:6]) + wsums2(3), 22 + 5.5 * KS, ["w3"], ["end"], 100))
    grp.append(Group("ws4", wsums4(), 40 + 8 * KS, ["w4"], ["end"], 60))
    _wait(seq, "w3", back=1)
    w3 = mm3("w3_0", 0, False)
    _mix(seq, _flat(w3[6:]), [split(w3[4:6]) + _flat(w3[:6])], 0.1)
    mc = mod("modc", 5, 6)
    mc = _flat(mc[1:] + mc[:1])
    _wait(seq, "w4", mc[:5] + [("sync", "run", lambda: None)])
    w4 = cat(mm4("w4_0", 0, 0, 3, 2, 1, False)[1:])
    qs = [split([w4[-1 - i]]) for i in range(_phase(seq))]
    _mix(seq, _flat(w4), [mc[i:i + 4] for i in range(5, 25, 4)] + qs, 0.01, 0.4)
    assert _phase(seq) == 0
    grp.append(Group("resid", resid(2, 1), 26 + 5 * KS, ["modc"], ["end"], 100))
    grp.append(Group("ln2a", ln2_late(), 40, ["w3_0"], ["end"], 100))
    _emit(seq, grp, zero, wait)

    def step(s, carry):
        for c in next_kv(s) + next_q(s):
            c.wait()
        nxt = jnp.minimum(s + 1, NB - 1)
        seq, grp = [], []
        us, it = one(mmU(lambda n: "U%d" % n, 0, 0)), one(mmI(lambda n: "I%d" % n, 0, 0))
        w4, w4c = mm4("w4", s - 2, 0)[1], mm4("w4c", s - 3, 0)[0]
        w2 = mm2("w2", 0, 1, 0, True)
        w2 = w2[0:3] + w2[4:13] + w2[22:31] + w2[3:4] + w2[13:22] + w2[31:]
        for u in w2[:21]:
            u.name = "w2a"
        w3, w3e = mm3("w3", 0, host=w2[:12])
        _mix(seq, _flat(w4c + w3),
             [us[0], us[1], us[2], it[0] + us[3], it[1] + us[4], it[2] + start(next_kv(nxt)), it[3], it[4]],
             0.159, 0.746)
        w1a, w1b = mm1("w1a", 2, 0, True), mm1("w1b", 2, 0, True)
        w1a, w1b = _flat(w1a[0:2] + w1a[4:13] + w1a[22:31]), _flat(w1b[2:4] + w1b[13:22] + w1b[31:])
        kw = 9 * 4
        w4[kw - 16].name = "w4m"
        seq += _flat(w3e + w2[12:21] + w4[:kw]) + w1a + run(shift(1, 0, ((T - 32, 32),), gs))
        seq += _flat(w4[kw:] + w2[21:]) + w1b
        assert _phase(seq) == 0
        kvs, macs = kv(0, 0), mac(1, 0, 0, part=True)
        for t in range(NT):
            grp.append(Group("kv%d" % t, kvs[t], 50 + 2 * KS, ["start"], ["U%d" % t], 260))
            grp.append(Group("mac%d" % t, macs[t], 24 + 2 * KS, ["U%d" % t], ["I%d" % t], 350, 150))
        iall = ["I%d" % t for t in range(NT)]
        ln = ln2(0, 0)
        grp.append(Group("ln2a", ln2_late(), 40, ["w2a", "w2"], ["end"], 100))
        xn = lsums2(3, n2_w, as_w[2], 0)[0]
        grp.append(Group("ln2b", ln[4:8] + ln[12:16], 78 + 20 * KS, ["start"], ["w3h"], 450))
        grp.append(Group("xna", [f for i, f in enumerate(xn) if i % 4 < 2], 26 + 5 * KS, ["start"], ["w3_0"], 150))
        grp.append(Group("xnb", [f for i, f in enumerate(xn) if i % 4 >= 2], 26 + 5 * KS, ["w4c"], ["w3_0"], 150, 0))
        grp.append(Group("resid", resid(1, 0, True), 46 + 30 * KS, ["w4c"], ["w2a", "w4q", "I4"], 100))
        for p, ts in enumerate(lsums2(4, a_w, as_w[3], 0)):
            grp.append(Group("xa%d" % p, ts, 26 + 5 * KS, ["w3_%d" % p], ["w4q"], 150, 100))
        fr = front(0, 0, ss=n1s)
        grp.append(Group("fronta", fr[0], 50 + 8 * KS, iall, ["w1a"], 240))
        grp.append(Group("frontb", fr[1], 46 + 7 * KS, ["w4m"], ["w1b"], 240, 80))
        fr[3].append(lambda: [c.start() for c in next_q(nxt)])
        grp.append(Group("fq", fr[2], 33 + 7 * KS, ["w4c"], ["I4"], 100))
        grp.append(Group("spread", spread(), 30 + 8 * KS, iall, ["end"], 60))
        grp.append(Group("shift", shift_early(), 22 + 7 * KS, ["start"], ["w1a", "w2a"], 200))
        _emit(seq, grp, zero, wait)
        out_b(s - 3).wait()
        out_a(s - 2).wait()
        return carry

    lax.fori_loop(NC, NB, step, 0)

    seq, grp = [], []
    w47 = mm4("w4_7", NB - 1, 1, 2, 0, 1)
    seq += _flat(mm4("w4_5", NB - 3, 0)[0] + mm2("w2_7", 0, 0, 1, True) + mm3("w3_6", 0)
                 + cat(mm4("w4_6", NB - 2, 0, 1, 1, 0)) + mm3("w3_7", 1) + w47[0][:3] + w47[1] + w47[0][3:])
    grp.append(Group("shift7", shift(2, 0, [(r, 32) for r in range(0, T, 32)], gs), 24, ["start"], ["w2_7"], 200))
    ln = ln2(0, 0)
    grp.append(Group("ln2_6", ln[4:8] + ln[12:16], 75, ["start"], ["w3_6"], 1200))
    grp.append(Group("xn6", cat(lsums2(3, n2_w, as_w[2], 0)), 26 + 5 * KS, ["w4_5"], ["w3_6_0"], 200, 800))
    grp.append(Group("ln2_7", ln2(1, 1), 75, ["w4_6"], ["w3_7"], 1500))
    grp.append(Group("xn7", cat(lsums2(3, n2_w, as_w[2], 1)), 26 + 5 * KS, ["w4_6"], ["w3_7_0"], 200, 2100))
    for j in (6, 7):
        for p, ts in enumerate(lsums2(4, a_w, as_w[3], j - 6)):
            grp.append(Group("xa%d_%d" % (j, p), ts, 26 + 5 * KS, ["w3_%d_%d" % (j, p)], ["w4_%dq" % j], 200, 150))
    _emit(seq, grp, zero, wait)
    for c in next_kv(NB - 1) + next_q(NB - 1) + [out_b(NB - 3)] + last:
        c.wait()


@jax.jit
def pallas_adaLN_cond__ssm_conv_h3__mixer_s_mlp__prompt_kernel(
        A_q, A_k, A_v, A_shift_k, A_ssm_k, A_ssm_D, B_x, B_w1, B_w2, B_w3, B_w4, c, w_mod):
    any_ = pl.BlockSpec(memory_space=pl.ANY)
    V = pltpu.VMEM
    out = pl.pallas_call(
        kernel,
        in_specs=[any_] * 12,
        out_specs=any_,
        out_shape=jax.ShapeDtypeStruct((S, D), BF16),
        scratch_shapes=[
            [V((NT, H + 8, 128), U32)] * NC, [V((NT, H + 8, 128), U32)] * NC, [V((NT, H + 8, 128), U32)] * NC,
            [V((64, S), U32)] * NT,
            V((D // 2, D), U32), V((D // 2, D), U32), V((F // 2, D), U32), V((FT * 64, D), U32),
            [V((D // 2, 3 * D), U32), V((D // 2, 2 * D), U32), V((D // 2, D), U32)], V((4 * T, D), BF16),
            V((4, D), BF16), V((D,), BF16), V((1, D), BF16), V((8, 128), I32), pltpu.SMEM((8, 128), I32),
            V((5, 8, D), F32), V((6, 8, D), F32), V((T // 2, 4 * H), U32), V((GR // 2, 2 * T), U32),
            V((NB, 3 * T + 8, D), F32), V((NC, 3 * T + 8, D), F32), V((NB - NC, 2 * T + 8, D), F32), V((4 * T, 128), F32),
            V((T, D), U32), V((NC * T, D), U32), V((NT, NC * (T + 8) + 16, 128), F32),
            V((3 * T, D), F32), V((3 * T, D), F32), V((2 * T, D), F32), V((T, D), F32),
            V((3 * T // 2, D), U32), V((T, D), U32), V((T, D), U32), V((NT, NC * T + 24, 128), F32),
            V((T, (FT + 1) * 128), U32),
            [V((128, 11 * 128), U32)] * 2 + [V((128, 31 * 128), U32), V((448, 11 * 128), U32)],
            [V((64, 11 * 128), U32)] * 2 + [V((128, 11 * 128), U32), V((128, 35 * 128), U32)],
            V((D // 2, 13 * 128), U32), V((H, D), F32), V((T, 9 * 128), F32),
            [V((64, 105 * 128), U32), V((192, 35 * 128), U32), V((32, 35 * 128), U32), V((32, 105 * 128), U32)],
            pltpu.SemaphoreType.DMA((11,)), pltpu.SemaphoreType.DMA((1,)), pltpu.SemaphoreType.DMA((3,)),
        ],
        compiler_params=pltpu.CompilerParams(vmem_limit_bytes=110 << 20, disable_semaphore_checks=True,
                                             disable_bounds_checks=True),
        name="fused",
    )(A_q[0], A_k[0], A_v[0], A_shift_k.T, A_ssm_k, A_ssm_D, B_w1, B_w2, B_w3.T, B_w4, c, w_mod)
    return out[None]
```

```python
import heapq
import os
import numpy as np
import jax
import jax.numpy as jnp
from jax import lax
from jax.experimental import pallas as pl
from jax.experimental.pallas import tpu as pltpu

S, D, F = 2048, 640, 1728
T = 256
H = T // 2
NB = S // T
NT = D // 128
FT = (F + 127) // 128
EPS = 1e-5
F32, BF16, U32, I32 = jnp.float32, jnp.bfloat16, jnp.uint32, jnp.int32
G_C1 = 0.044715 * float(np.sqrt(2.0 / np.pi))
G_C2 = float(np.sqrt(2.0 / np.pi))
G_A = G_C1 ** (1.0 / 3.0)
G_B = G_C2 / G_A
G_POST = 0.5 / G_A
RG = 16
GR = 80
NC = 3
DL = 450
KS = float(os.environ.get('KS', 1.9))
BIAS = [tuple(int(c, 36) for c in os.environ.get('BIAS%d' % i, '')) for i in range(3)]
E = lambda k, d: type(d)(os.environ.get(k, d))
SLOT = 32


def _dft(shape, f_axis, tau, scale=1.0):
    r = lax.broadcasted_iota(I32, shape, f_axis)
    l = lax.broadcasted_iota(I32, shape, 1 - f_axis)
    f = r & 127
    odd = ((f & 63) << 2) | ((f >> 6) << 1) | 1
    p = odd * tau(l) + ((r >> 7) << 8)
    a = ((p + 512) & 1023) - 512
    u = (256 - jnp.abs(a)).astype(F32) * (np.pi / 512.0)
    u2 = u * u
    c = [scale, -scale / 6.0, scale / 120.0, -scale / 5040.0, scale / 362880.0, -scale / 39916800.0]
    poly = c[5]
    for ci in c[4::-1]:
        poly = poly * u2 + ci
    return (u * poly).astype(BF16)


def _rstd(xc, mlp):
    s2, eps = (1.0 / (G_A * G_A), EPS / (G_POST * G_POST)) if mlp else (1.0, EPS)
    v = jnp.sum(xc * xc, axis=-1, keepdims=True) * (s2 / D) + eps * s2
    return jnp.exp2(jnp.log(v) * float(-0.5 / np.log(2.0)))


def _ln(x, mlp=False):
    xc = x - jnp.sum(x, axis=-1, keepdims=True) * (1.0 / D)
    return xc * _rstd(xc, mlp)


def _gelu2(x):
    u = x * (x * x + G_B)
    return x * (1.0 + jnp.tanh(u))


def _lo(w):
    return pltpu.bitcast(w << 16, F32)


def _hi(w):
    return pltpu.bitcast(w & jnp.uint32(0xFFFF0000), F32)


def _tie(x, a):
    if a is None:
        return x
    w = pltpu.bitcast(x[:, :128], U32)
    k = w.shape[0] // 8
    w = w | (a if k == 1 else jnp.concatenate([a] * k, axis=0))
    w = pltpu.bitcast(w, x.dtype)
    return w if x.shape[1] == 128 else jnp.concatenate([w, x[:, 128:]], axis=1)


def _top(x, i):
    return jnp.concatenate([x[r:r + 16] for r in range(16 * i, x.shape[0], 32)], axis=0)


def _zip(t, b):
    return jnp.concatenate([x[r:r + 16] for r in range(0, t.shape[0], 16) for x in (t, b)], axis=0)


def _lhs_sums(x1, x2):
    a11, a21, a12, a22 = _top(x1, 0), _top(x1, 1), _top(x2, 0), _top(x2, 1)
    return [a11 + a22, a21 + a22, a11 + a12, a21 - a11, a12 - a22]


def C(i):
    return slice(i * 128, (i + 1) * 128)


class Unit:
    def __init__(self, name, tiles, epi, rows, cost, nt=False, full=True, acc=False, tail=0):
        self.tail = tail
        self.acc, self.res = acc, []
        self.name, self.tiles, self.epi, self.rows, self.cost, self.nt, self.full = name, tiles, epi, rows, cost, nt, full


class Due:
    def __init__(self, val, delay):
        self.val, self.delay = val, delay


class Group:
    def __init__(self, name, fns, cost, rel, dead, lat, rlat=200):
        self.name, self.fns, self.cost, self.rel, self.dead, self.lat, self.rlat = name, fns, cost, rel, dead, lat, rlat


def _plan(seq, groups, bias):
    busy, n = [0] * 4, 0
    start, end, tiles, bars = {}, {}, [], []
    for it in seq:
        if isinstance(it[0], Unit):
            u = it[0]
            m = n % 4
            n += 1
            t0, t1 = busy[m], busy[m] + max(u.rows, 32)
            busy[m] = t1
            tiles.append((t0, t1, u.cost / len(u.tiles) + (u.tail if it[1] == len(u.tiles) - 1 else 0)))
            start.setdefault(u.name, t0)
            end[u.name] = max(end.get(u.name, 0), t1)
        elif it[0] == "wait":
            t = max(busy)
            busy, n = [t] * 4, 0
            start[it[1]] = end[it[1]] = t
            bars.append(t)
    total = max(busy)
    start["end"] = end["end"] = total
    start["start"] = end["start"] = 0
    ns = total // SLOT + 2
    load = np.zeros(ns)
    for t0, t1, c in tiles:
        a, b = t0 // SLOT, max(t1 // SLOT, t0 // SLOT + 1)
        load[a:b] += c / (b - a)
    for i, b in enumerate(bias):
        load[2 * i:2 * i + 2] += 4 * b
    win = []
    for g in groups:
        r = max(end[x] + (0 if start[x] == end[x] else g.rlat) for x in g.rel)
        d = min(start[x] for x in g.dead) - g.lat
        ok = np.zeros(ns, bool)
        ok[r // SLOT:max(d // SLOT, r // SLOT + 1)] = True
        for b in bars:
            if r < b <= d:
                ok[max((b - g.lat) // SLOT, 0):b // SLOT] = False
        win.append(np.nonzero(ok)[0])
    alloc = [np.zeros(len(w)) for w in win]
    for _ in range(60):
        for i, g in enumerate(groups):
            w = win[i]
            load[w] -= alloc[i]
            base = load[w]
            vol = g.cost * len(g.fns)
            lo, hi = base.min(), base.max() + vol
            for _ in range(50):
                mid = 0.5 * (lo + hi)
                if np.maximum(mid - base, 0).sum() > vol:
                    hi = mid
                else:
                    lo = mid
            alloc[i] = np.maximum(hi - base, 0)
            load[w] += alloc[i]
    times = []
    for i, g in enumerate(groups):
        cum = np.cumsum(alloc[i])
        ts = []
        for k in range(len(g.fns)):
            x = (k + 0.5) * cum[-1] / len(g.fns)
            j = int(np.searchsorted(cum, x))
            prev = cum[j - 1] if j else 0.0
            ts.append(win[i][j] * SLOT + SLOT * (x - prev) / max(alloc[i][j], 1e-9))
        times.append(ts)
    return times


def _emit(seq, groups, zero, wait, bias):
    times = _plan(seq, groups, bias)
    left = {"start": 0}
    for it in seq:
        nm = it[0].name if isinstance(it[0], Unit) else it[1]
        left[nm] = left.get(nm, 0) + 1
    heap, pend, todo, cnt = [], {}, list(range(len(groups))), 0
    busy, n, due = [0] * 4, 0, []

    def release():
        nonlocal cnt
        for i in list(todo):
            g = groups[i]
            if all(left[x] == 0 for x in g.rel):
                todo.remove(i)
                pend[i] = len(g.fns)
                for t, fn in zip(times[i], g.fns):
                    heapq.heappush(heap, (t, cnt, i, fn))
                    cnt += 1

    def force(name):
        nonlocal heap
        for i, g in enumerate(groups):
            if name in g.dead:
                assert i not in todo, (g.name, name)
                if pend[i]:
                    for it in sorted(x for x in heap if x[2] == i):
                        it[3](None)
                    heap = [x for x in heap if x[2] != i]
                    heapq.heapify(heap)
                    pend[i] = 0

    release()
    for it in seq:
        if isinstance(it[0], Unit):
            u, k = it
            force(u.name)
            lhs, rhs = u.tiles[k]()
            t0 = busy[n % 4]
            while u.full and due and due[0][0] < t0 + u.rows:
                t, x = due.pop(0)
                r = min(max(int(t - t0), 0), u.rows - 1) // 16 * 8
                w = pltpu.bitcast(lhs, U32)
                x = pltpu.bitcast(x[:, :128], U32)
                parts = [w[:r], w[r:r + 8] | ((x[0:8] | x[8:16]) & zero), w[r + 8:]]
                lhs = pltpu.bitcast(jnp.concatenate([y for y in parts if y.shape[0]], axis=0), BF16)
            dn = (((1,), (1 if u.nt else 0,)), ((), ()))
            p = lax.dot_general(lhs, rhs, dn, preferred_element_type=F32)
            u.res = [p + u.res[0]] if (u.acc and u.res) else u.res + [p]
            m = n % 4
            n += 1
            t0 = busy[m]
            busy[m] = t0 + max(u.rows, 32)
            used = -8
            while u.full and heap and heap[0][0] < t0 + u.rows:
                r = min(max(int(heap[0][0] - t0), 0), u.rows - 1) // 8 * 8
                if E("UQ", 1):
                    r = max(r, used + 8)
                    if r >= u.rows or r > max(heap[0][0] - t0, 8) + E("UD", 16):
                        break
                used = r
                t, _, i, fn = heapq.heappop(heap)
                pend[i] -= 1
                x = fn(pltpu.bitcast(p[r:r + 8], U32) & zero)
                if isinstance(x, Due):
                    due.append((t + x.delay, x.val))
                    due.sort(key=lambda e: e[0])
            if k == len(u.tiles) - 1:
                u.epi(u.res)
            left[u.name] -= 1
        elif it[0] == "wait":
            force(it[1])
            wait(it[1])
            busy, n, due = [max(busy)] * 4, 0, []
            left[it[1]] -= 1
        else:
            it[2]()
            left[it[1]] -= 1
        release()
    force("end")
    assert not heap and not todo


def _sum(ps):
    acc = ps[0]
    for p in ps[1:]:
        acc = acc + p
    return acc


def _flat(us):
    return [(u, i) for u in us for i in range(len(u.tiles))]


def _weave(a, b):
    out = []
    for i, u in enumerate(a):
        out += [u] + b[i * len(b) // len(a):(i + 1) * len(b) // len(a)]
    return out


def _phase(seq):
    n = 0
    for it in seq:
        n = n + 1 if isinstance(it[0], Unit) else (0 if it[0] in ("wait", "sync") else n)
    return n % 4


def _mix(seq, a, b, lo=0.0, hi=1.0):
    n, k = _phase(seq), 0
    for i, t in enumerate(a):
        if k < len(b) and n % 4 == 0 and t[1] != 1 and i >= len(a) * (lo + (hi - lo) * k / len(b)):
            seq.extend(b[k])
            k += 1
        seq.append(t)
        n += 1
    assert k == len(b)


def _wait(seq, name, head=(), back=0):
    r = _phase(seq) + 4 * back
    assert all(isinstance(it[0], Unit) for it in seq[len(seq) - r:])
    seq[len(seq) - r:len(seq) - r] = [("wait", name)] + list(head)


def kernel(q_hbm, k_hbm, v_hbm, sh_hbm, ssm_hbm, sd_hbm, w1_hbm, w2_hbm, w3_hbm, w4_hbm, c_hbm, wm_hbm,
           o_hbm,
           q_n, k_n, v_n, ssm_w, w1_w, w2_w, w3_w, w4_w, wm_w, o_v,
           sh_v, sd_v, c_v, zsrc, z_s, taps, mod_v, tf_w, tg_w,
           kf, uf, acc, zraw, kv_w, zz_w, y_v, x_v, hb_v, x1_v, r_v, n1_w, n2_w, g_w, h1_v, a_w,
           ws_w, as_w, w3n_w, top_v, st_v, l2_w,
           sem, sem_b, sem_o):
    bf = lambda r: r.bitcast(BF16)
    w1_v, w2_v, w3_v, w4_v = bf(w1_w), bf(w2_w), bf(w3_w), bf(w4_w)
    wm_v = {0: bf(wm_w[0]), 3: bf(wm_w[1]), 5: bf(wm_w[2])}
    tf_v, tg_v, n1_v, n2_v, g_v = bf(tf_w), bf(tg_w), bf(n1_w), bf(n2_w), bf(g_w)
    a_v, kv_v, zz_v = bf(a_w), bf(kv_w), bf(zz_w)
    w1s, w2s, w3s, w4s = [bf(r) for r in ws_w]
    n1s, gs, n2s, a_s = [bf(r) for r in as_w]
    w3n = bf(w3n_w)
    w3t, w4t, n2t, a_t = [bf(r) for r in l2_w]
    cp = pltpu.make_async_copy
    cat = lambda ls: [x for l in ls for x in l]

    def base(j, n):
        return j * n if isinstance(j, int) else pl.multiple_of(j * n, n)

    def rows(j, n=1, size=T):
        return pl.ds(base(j, size), n * size)

    def view(ref, j, size=T):
        return ref.at[rows(j, 1, size)]

    dmas = {}

    def group(name, *mks):
        sm = sem.at[len(dmas)]
        dmas[name] = [c for mk in mks for c in mk(sm)]

    def ssm_in(t):
        return lambda sm: [cp(ssm_hbm.at[C(t)], bf(ssm_w[t]), sm)]

    def cols(src, start, n, dst, row=0):
        return lambda sm: [cp(src.at[pl.ds(start, n), C(t)], bf(dst).at[t, pl.ds(row, n)], sm) for t in range(NT)]

    def kv_in(s, sl):
        if isinstance(s, int):
            kk = cols(k_hbm, s * T - 16, T + 16, k_n[sl]) if s else cols(k_hbm, 0, T, k_n[sl], 16)
        else:
            kk = cols(k_hbm, pl.multiple_of(s * T - 16, 16), T + 16, k_n[sl])
        return lambda sm: kk(sm) + cols(v_hbm, base(s, T), T, v_n[sl])(sm)

    def q_in(s, sl):
        return cols(q_hbm, base(s, T), T, q_n[sl])

    def wm_in(a, b):
        return lambda sm: [cp(wm_hbm.at[:, a * D:b * D], wm_v[a], sm)]

    def whole(src, dst):
        return lambda sm: [cp(src, dst, sm)]

    next_kv = lambda s: kv_in(s, 0)(sem_b.at[0])
    next_q = lambda s: q_in(s, 0)(sem_b.at[0])

    zsrc[...] = jnp.zeros((8, 128), I32)
    k_n[0][:, 0:8, :] = jnp.zeros((NT, 8, 128), U32)
    w4_w[F // 2:FT * 64, :] = jnp.zeros((FT * 64 - F // 2, D), U32)
    group("small", lambda sm: [cp(zsrc, z_s, sm), cp(sh_hbm, sh_v, sm), cp(sd_hbm, sd_v, sm), cp(c_hbm, c_v, sm)])
    for s in range(NC):
        group("c%d" % s, ssm_in(s), kv_in(s, s))
    group("c3", ssm_in(3), ssm_in(4))
    group("wma", wm_in(0, 3), q_in(0, 0), q_in(1, 1))
    group("wmb", wm_in(3, 5))
    group("w1", whole(w1_hbm, w1_v))
    group("w2", q_in(2, 2), whole(w2_hbm, w2_v))
    group("w3", whole(w3_hbm, w3_v))
    group("w4", whole(w4_hbm, w4_v.at[0:F]), wm_in(5, 6))
    for g in dmas.values():
        for c in g:
            c.start()

    def wait(name):
        for c in dmas[name]:
            c.wait()

    tau_b = lambda l: H + ((l + (H - 1)) & (H - 1))
    tf_v[:, C(0)] = _dft((T, H), 0, lambda l: jnp.where((l & 1) == 0, l, tau_b(l)), 1.0 / T)
    tf_v[:, C(1)] = _dft((T, H), 0, lambda l: jnp.where((l & 1) == 1, l, tau_b(l)), 1.0 / T)
    tf_v[:, C(2)] = _dft((T, H), 0, lambda l: 2 * l - H)
    tf_v[:, C(3)] = _dft((T, H), 0, lambda l: 2 * l + 1 - H)
    sin0 = lax.broadcasted_iota(I32, (GR, T), 1) >= H
    tg_v[:, 0:T] = _dft((GR, T), 1, lambda l: jnp.where(sin0 & (l == 0), H, 2 * l))
    tg_v[:, T:2 * T] = _dft((GR, T), 1, lambda l: 2 * l + 1)
    h1_v[:, 0:8, :] = jnp.zeros((NT, 8, 128), F32)
    h1_v[:, 8 + NC * T:16 + NC * T, :] = jnp.zeros((NT, 8, 128), F32)

    wait("small")
    z = jnp.clip(z_s[0, 0], 0, 1)
    zero = jnp.full((8, 128), z, I32).astype(U32)
    z8 = pl.multiple_of(z * 8, 8)
    for r in (x_v, hb_v, x1_v, r_v, zraw, n1_w, n2_w, g_w, a_w, kv_w, zz_w, *ws_w, *as_w, w3n_w, top_v, st_v, *l2_w):
        r[pl.ds(z8, 8), 0:128] = jnp.zeros((8, 128), r.dtype)
    for r in (kf, uf, acc, taps, mod_v):
        r[z, 0:8, 0:128] = jnp.zeros((8, 128), r.dtype)
    for r in (tf_w, tg_w):
        r[pl.ds(z8, 8), 0:128] = r[0:8, 0:128]
    sh = sh_v[...].astype(F32)
    for i in range(4):
        taps[i] = jnp.broadcast_to(sh[i:i + 1], (8, D))
    taps[4] = jnp.broadcast_to(sd_v[...].astype(F32).reshape(1, D) * (1.0 / T), (8, D))
    cf = c_v[...].astype(F32)
    silu_c = jnp.broadcast_to((cf / (1.0 + jnp.exp(-cf))).astype(BF16), (16, D))

    def mmK(n):
        def unit(m):
            st = []

            def rhs(i):
                if not st:
                    ev = (lax.broadcasted_iota(I32, (64, 128), 1) & 1) == 0
                    a = ssm_w[n][:, m * T:m * T + H]
                    b = pltpu.roll(ssm_w[n][:, m * T + H:(m + 1) * T], 1, 1)
                    st.extend([pltpu.bitcast(jnp.where(ev, a, b), BF16), pltpu.bitcast(jnp.where(ev, b, a), BF16)])
                return st[i]

            def epi(p):
                er, ei, or_, oi = p
                cur = [er, ei, or_, oi]
                if m:
                    pv = [zraw[C(4 * ((m - 1) % 2) + (q ^ 1)), :] for q in range(4)]
                    pm = lambda x, y, up: jnp.concatenate([x[:64] + y[:64], x[64:] - y[64:]] if up else
                                                          [x[:64] - y[:64], x[64:] + y[64:]], axis=0)
                    er, ei, or_, oi = [pm(cur[q], pv[q], q & 1) for q in range(4)]
                else:
                    er = er + taps[4, 0:1, C(n)]
                if m + 1 < NB:
                    for q in range(4):
                        zraw[C(4 * (m % 2) + q), :] = cur[q]
                for h, (cr, ci) in enumerate(((er + or_, ei + oi), (er - or_, ei - oi))):
                    B = h * 3 * H
                    kf[m, B:B + H, C(n)] = cr
                    kf[m, B + H:B + 2 * H, C(n)] = ci - cr
                    kf[m, B + 2 * H:B + 3 * H, C(n)] = ci + cr
            return Unit("K%d" % n, [(lambda i=i, r=r: (tf_v[r:r + H, C(i)], rhs(i))) for i in range(2) for r in (0, H)],
                        epi, H, 260, nt=True)
        return [unit(m) for m in range(NB)]

    def kv(s, sl):
        def mk(t, w):
            def fn(a):
                ld = lambda o, n: k_n[s][t, pl.ds(8 + w + o, n), :]
                c0 = jnp.concatenate([_tie(ld(0, 8), a), ld(8, 8)], axis=0).reshape(2, 8, 128)
                c1, c2 = ld(-1, 16).reshape(2, 8, 128), ld(-2, 16).reshape(2, 8, 128)
                s0, s1, s2, s3 = (taps[i, :, C(t)] for i in range(4))
                ke, ko, ke1, ko1, ko2 = _lo(c0), _hi(c0), _lo(c1), _hi(c1), _hi(c2)
                wv = v_n[s][t, w:w + 16, :].reshape(2, 8, 128)
                kve = ((s0 * ke + s1 * ko1) + (s2 * ke1 + s3 * ko2)) * _lo(wv)
                kvo = ((s0 * ko + s1 * ke) + (s2 * ko1 + s3 * ke1)) * _hi(wv)
                kv_v[pl.ds(sl * T + w, 16), C(t)] = kve.reshape(16, 128).astype(BF16)
                kv_v[pl.ds(sl * T + H + w, 16), C(t)] = kvo.reshape(16, 128).astype(BF16)
            return fn
        return [[mk(t, w) for w in range(0, H, 16)] for t in range(NT)]

    def mmU(name, sl, us):
        def unit(n):
            def epi(p):
                er, ei, or_, oi = p
                for h, (cr, ci) in enumerate(((er + or_, ei + oi), (er - or_, ei - oi))):
                    B = h * 3 * H
                    uf[us, B:B + H, C(n)] = cr + ci
                    uf[us, B + H:B + 2 * H, C(n)] = cr
                    uf[us, B + 2 * H:B + 3 * H, C(n)] = ci
            return Unit(name(n), [(lambda i=i, r=r: (tf_v[r:r + H, C(2 + i)], kv_v[pl.ds(sl * T + i * H, H), C(n)]))
                                  for i in range(2) for r in (0, H)], epi, H, 96 + 96 * KS)
        return [unit(n) for n in range(NT)]

    def cmul(m0, u0, n, h, row, L, a):
        t = []
        for i in range(3):
            Rw = slice((3 * h + i) * H + row, (3 * h + i) * H + row + 8)
            kk = kf[m0:m0 + n, Rw, L]
            if i == 0 and a is not None:
                k0 = _tie(kk[0], a)[None]
                kk = k0 if n == 1 else jnp.concatenate([k0, kk[1:]], axis=0)
            t.append(jnp.sum(kk * uf[u0:u0 + n, Rw, L], axis=0))
        return t[0] - t[2], t[0] + t[1]

    def AR(h, q, row):
        return slice((2 * h + q) * H + row, (2 * h + q) * H + row + 8)

    def mac(n, u0, sl, part=False):
        def mk(t, rc):
            st, fin = [], []

            def piece(i):
                def fn(a):
                    h, row = i & 1, rc + (i >> 1) * 8
                    zr, zi = cmul(0, u0, n, h, row, C(t), a)
                    if part:
                        zr, zi = zr + acc[0, AR(h, 0, row), C(t)], zi + acc[0, AR(h, 1, row), C(t)]
                    st.append((zr, zi))
                    if h:
                        (pr, pi), (mr, mi) = st[-2:]
                        fin.append([pr + mr, pi + mi, pr - mr, pi - mi])
                    if i == 3:
                        for q in range(4):
                            zz_v[pl.ds(sl * 2 * T + q * H + rc, 16), C(t)] = jnp.concatenate(
                                [fin[0][q], fin[1][q]], axis=0).astype(BF16)
                return fn
            if not part:
                return [piece(i) for i in range(4)]
            both = lambda f, g: (lambda a: (f(a), g(None)))
            return [both(piece(0), piece(1)), both(piece(2), piece(3))]
        return [[fn for rc in range(0, H, 16) for fn in mk(t, rc)] for t in range(NT)]

    def pos():
        return [(t, h, row) for t in range(NT) for row in range(0, H, 8) for h in range(2)]

    def ahead(i):
        def mk(t, h, row):
            def fn(a):
                zr, zi = cmul(i + 1, 0, NC, h, row, C(t), a)
                acc[i, AR(h, 0, row), C(t)] = zr
                acc[i, AR(h, 1, row), C(t)] = zi
            return fn
        return [mk(*p) for p in pos()]

    def spread():
        n = NB - NC - 1

        def mk(t, h, row):
            def fn(a):
                p = []
                for i in range(3):
                    Rw = slice((3 * h + i) * H + row, (3 * h + i) * H + row + 8)
                    u = uf[0, Rw, C(t)]
                    p.append(kf[1:1 + n, Rw, C(t)] * (_tie(u, a) if i == 0 else u)[None])
                acc[0:n, AR(h, 0, row), C(t)] = acc[1:1 + n, AR(h, 0, row), C(t)] + (p[0] - p[2])
                acc[0:n, AR(h, 1, row), C(t)] = acc[1:1 + n, AR(h, 1, row), C(t)] + (p[0] + p[1])
            return fn
        return [mk(*p) for p in pos()]

    def mmI(name, sl, ys):
        def unit(n):
            def epi(p):
                ce, se, co, so = p
                sub = lax.broadcasted_iota(I32, (8, 128), 0)
                b0 = ys * (T + 8) + 8
                y_v[n, b0 + H - 1:b0 + H, :] = (ce[64:72] - se[0:8])[0:1]
                se = jnp.concatenate([jnp.where(sub == 0, 0.0, se[0:8]), se[8:]], axis=0)
                for d, cc, ss in ((0, ce[0:64], se), (1, co, so)):
                    y_v[n, pl.ds(b0 + H + d, 64, stride=2), :] = cc + ss
                    y_v[n, pl.ds(b0 + d - 1, 64, stride=2), :] = cc - ss
            return Unit(name(n), [(lambda i=i: (tg_v[0:(GR if i == 0 else 64), C(i)], zz_v[pl.ds(sl * 2 * T + i * H, H), C(n)]))
                                  for i in range(4)], epi, 64, 36 + 33 * KS)
        return [unit(n) for n in range(NT)]

    def mod(name, a, b):
        def unit(n):
            def epi(p):
                v = [_sum(p[i * NT:(i + 1) * NT])[0:8] for i in range(b - a)]
                if a == 0:
                    mod_v[0, :, C(n)] = v[0] * v[2]
                    mod_v[1, :, C(n)] = (v[1] + 1.0) * v[2]
                elif a == 3:
                    mod_v[3, :, C(n)] = v[0] * (1.0 / G_POST)
                    mod_v[4, :, C(n)] = (v[1] + 1.0) * (1.0 / G_POST)
                else:
                    mod_v[2, :, C(n)] = v[0] * G_POST
            return Unit(name, [(lambda i=i, k=k: (silu_c[:, C(k)], wm_v[a][C(k), pl.ds(i * D + n * 128, 128)]))
                               for i in range(b - a) for k in range(NT)], epi, 16, 10, full=False, acc=b - a == 1)
        return [unit(n) for n in range(NT)]

    HS = (slice(0, 128), slice(128, 256))
    QS = tuple(slice(r, r + 64) for r in range(0, T, 64))

    def tasks(f, due=None, tie=True, n=RG):
        def mk(R):
            def fn(a):
                x = f(R, a if tie else None)
                return Due(x, due) if due else None
            return fn
        return [mk(slice(r, r + n)) for r in range(0, T, n)]

    def load_y(sl, R):
        b0, back = sl * (T + 8) + 8, 7 - lax.broadcasted_iota(I32, (8, 128), 0)

        def ld(t, r):
            if r >= H:
                return y_v[t, b0 + r:b0 + r + 8, :]
            return jnp.take_along_axis(y_v[t, b0 + H - 8 - r:b0 + H - r, :], back, axis=0)
        return jnp.stack([jnp.concatenate([ld(t, r) for t in range(NT)], axis=1) for r in (R.start, R.start + 8)])

    def put(nn, ss, R, x):
        nn[R, :] = x.astype(BF16)
        tok = x
        if ss is not None:
            S2 = pl.ds(R.start // 32 * 16, 16)
            if R.stop % 32:
                top_v[S2, 0:2 * T] = x[:, 0:2 * T]
            else:
                if R.start % 32:
                    x = jnp.concatenate([top_v[S2, 0:2 * T], x[:, 0:2 * T]], axis=0)
                ss[S2, 0:5 * T] = jnp.concatenate(_lhs_sums(x[:, 0:T], x[:, T:2 * T]), axis=1).astype(BF16)
        return tok

    wide = lambda v: jnp.concatenate([v] * NT, axis=1)

    def mean(i, R, x):
        st_v[R, C(i)] = jnp.broadcast_to(jnp.sum(x, axis=-1, keepdims=True) * (1.0 / D), (x.shape[0], 128))

    def centred(src, i, R, a):
        return src[R, :] - wide(_tie(st_v[R, C(i)], a))

    def scale(src, i, g):
        def f(R, a):
            st_v[R, C(i + 1)] = jnp.broadcast_to(_rstd(centred(src, i, R, a), g), (RG, 128))
        return f

    def normed(src, i, R, a):
        return centred(src, i, R, a) * wide(st_v[R, C(i + 1)])

    def front(sl, xs, early=False, ss=None):
        xx, hh, nn = view(x_v, xs), view(hb_v, xs), view(n1_v, sl)

        def fa(R, a):
            q = [q_n[sl][t, R.start // 2:R.stop // 2, :] for t in range(NT)]
            q = jnp.concatenate([_tie(q[0], a)] + q[1:], axis=1)
            q = pltpu.bitcast(q, BF16).astype(F32).reshape(2, 8, D)
            x = (q + (_ln(q) * mod_v[1] + mod_v[0]) * load_y(sl, R)).reshape(RG, D)
            xx[R, :] = x
            if early:
                hh[R, :] = _ln(x)

        def fb(R, a):
            hh[R, :] = (_ln(_tie(xx[R, :], a).reshape(2, 8, D)) * mod_v[4] + mod_v[3]).reshape(RG, D)

        def fc(R, a):
            hb = _tie(hh[R, :], a)
            if early:
                hb = (hb.reshape(2, 8, D) * mod_v[4] + mod_v[3]).reshape(RG, D)
                hh[R, :] = hb
            nn[R, :] = _ln(hb, True).astype(BF16)
        if early:
            return tasks(fa), tasks(fc)
        if ss is None:
            return tasks(fa) + tasks(fb) + tasks(fc)
        qf = view(x_v, 2)

        def s1(R, a):
            q = [q_n[sl][t, R.start // 2:R.stop // 2, :] for t in range(NT)]
            q = pltpu.bitcast(jnp.concatenate([_tie(v, a) for v in q], axis=1), BF16).astype(F32)
            qf[R, :] = q
            mean(0, R, q)

        def s3(R, a):
            h = normed(qf, 0, R, a).reshape(2, 8, D) * mod_v[1] + mod_v[0]
            x = qf[R, :] + (h * load_y(sl, R)).reshape(RG, D)
            xx[R, :] = x
            mean(2, R, x)

        def s5(R, a):
            hb = (normed(xx, 2, R, a).reshape(2, 8, D) * mod_v[4] + mod_v[3]).reshape(RG, D)
            hh[R, :] = hb
            mean(4, R, hb)
        s7 = [f for g in tasks(lambda R, a: put(nn, ss, R, normed(hh, 4, R, a)), n=32) for f in (g, lambda a: None)]
        st = [tasks(s3), tasks(scale(xx, 2, False)), tasks(s5), tasks(scale(hh, 4, True)), s7]
        p = [tasks(s1), tasks(scale(qf, 0, False))]
        sk = E("SK", 4.091)

        def wave(ls):
            body = sorted((i * sk + g, i, g) for i in range(len(ls) - 1) for g in range(8))
            return [ls[i][g] for _, i, g in body] + ls[-1]
        qb = []
        done = lambda a: qb[0]()
        full = wave([x[8:] for x in p + st])
        k = full.index(p[0][15]) + 1
        return wave([x[:8] for x in st]), full[:k] + [done] + full[k:], cat(x[:8] for x in p), qb

    def shift(hs, sl, pieces=((0, 64), (64, 64), (128, 64), (192, 64)), ss=None):
        gg = view(g_v, sl)

        def one_tile(t, r, n, a):
            lane = lax.broadcasted_iota(I32, (n, 128), 1)
            ld = lambda d: h1_v[t, pl.ds(hs * T + 8 + r + d, n), :]
            if t == 0:
                g = ld(-1)
            elif t == 1:
                g = jnp.where(lane < 32, ld(-1), ld(1))
            elif t == 2:
                g = jnp.where(lane < 64, ld(1), ld(-2))
            elif t == 3:
                g = jnp.where(lane < 96, ld(-2), ld(2))
            else:
                g = ld(2)
            if a is not None:
                g = jnp.concatenate([_tie(g[i:i + 8], a) if i % 16 == 0 else g[i:i + 8]
                                     for i in range(0, n, 8)], axis=0)
            gg[r:r + n, C(t)] = g.astype(BF16)
            return g

        def mk(ts, r, n):
            def fn(a):
                g = [one_tile(t, r, n, a) for t in ts]
                if len(ts) == 2:
                    for i, x in enumerate(_lhs_sums(*g)):
                        ss[r // 2:(r + n) // 2, C(2 * i + ts[0])] = x.astype(BF16)
            return fn
        sets = [(t,) for t in range(NT)] if ss is None else [(0, 2), (1, 3), (4,)]
        return [mk(ts, r, n) for ts in sets for r, n in pieces]

    def shift_early():
        def keep(a):
            h1_v[:, 2 * T - 32:2 * T + 8, :] = h1_v[:, 3 * T - 32:3 * T + 8, :]
        return shift(2, 0, [(r, 32) for r in range(0, T - 32, 32)], gs) + [keep]

    def ln2(xs, sl, fast=True):
        xx, nn, ss = view(x1_v, xs), view(n2_v, sl), view(n2s, sl, H) if fast else None
        f = lambda R, a: put(nn, ss, R, _ln(_tie(xx[R, :], a), True))
        ts = tasks(f, 900) if sl else tasks(f, DL, False)
        return ts[0::2] + ts[1::2] if fast else tasks(f)

    def ln2_late():
        xx, nn, ss = view(x1_v, 0), view(n2_v, 0), view(n2s, 0, H)
        a_, b_ = tasks(lambda R, a: mean(6, R, _tie(xx[R, :], a))), tasks(scale(xx, 6, True))
        c_ = [f for g in tasks(lambda R, a: put(nn, ss, R, normed(xx, 6, R, a)), n=32)[:4] for f in (g, lambda a: None)]
        return a_[:8] + b_[:8] + c_

    def resid(xs, x1s, rotate=False):
        xx, x1 = view(x_v, xs), view(x1_v, x1s)
        tie = lambda v, a: v if a is None else pltpu.bitcast(pltpu.bitcast(v, U32) | wide(a), F32)

        def f(R, a):
            r_v[R, :] = xx[R, :] + tie(x1[R, :], a) * mod_v[2]

        def move(dst, src):
            def g(R, a):
                dst[R, :] = tie(src[R, :], a)
            return tasks(g, n=8)
        if not rotate:
            return tasks(f, n=8)
        return cat(zip(tasks(f, n=8), move(view(hb_v, 1), hb_v), move(xx, x_v)))

    KD, KF, ND = [(0, 2), (1, 3)], [(2 * i, 2 * i + 1) for i in range(7)], [(1, 2), (3, 4)]
    Wt = {1: (lambda k, n: w1_v[C(k), C(n)], lambda i, kp, j: w1s[C(kp), C(2 * i + j)], False, KD, [4]),
          2: (lambda k, n: w2_v[C(k), C(n)], lambda i, kp, j: w2s[C(kp), C(2 * i + j)], False, KD, [4]),
          0: (lambda k, n: w3_v[C(n), C(k)], None, True, KD, [4]),
          3: (lambda k, n: w3n[C(k), C(n)], lambda i, kp, j: w3s[C(kp), C(6 * i + j)], False, KD, [4]),
          4: (lambda k, n: w4_v[C(k), C(n)], lambda i, kp, j: w4s[C(kp), C(2 * i + j)], False, KF, [])}

    def sums_task(load, store, left):
        def fn(a):
            b = [[load(u, v) for v in range(2)] for u in range(2)]
            b[0][0], b[1][1] = _tie(b[0][0], a), _tie(b[1][1], a)
            (x11, x12), (x21, x22) = [[pltpu.bitcast(x, BF16).astype(F32) for x in row] for row in b]
            r = ((x11 + x22, x21 + x22, x11 + x12, x21 - x11, x12 - x22) if left else
                 (x11 + x22, x12 - x22, x21 - x11, x11 + x12, x21 + x22))
            for m, x in enumerate(r):
                store(m, x.astype(BF16))
        return fn

    def wsums(w_w, ws, rp, cp_):
        def mk(i, j, r):
            def store(m, x):
                ws[pl.ds(128 * i + r, 16), C(len(cp_) * m + j)] = x
            return sums_task(lambda u, v: w_w[pl.ds(64 * rp[i][u] + r // 2, 8), C(cp_[j][v])], store, False)
        return [mk(i, j, r) for j in range(len(cp_)) for i in range(len(rp)) for r in range(0, 128, 16)]

    def w3_turn():
        def mk(n, k):
            def fn(a):
                x = jnp.concatenate([_tie(w3_w[64 * n:64 * n + 8, C(k)], a), w3_w[64 * n + 8:64 * n + 64, C(k)]], axis=0)
                w3n[C(k), C(n)] = pltpu.bitcast(x, BF16).T
            return fn
        return [mk(n, k) for n in range(FT - 1) for k in range(NT)]

    def plain(name, w, lhs, n, R, epi, cost):
        tile, _, nt, kp, kl = Wt[w]
        ks = sorted([k for p in kp for k in p] + kl)
        rows_ = R.stop - R.start
        return Unit(name, [(lambda k=k: (lhs[R, C(k)], tile(k, n))) for k in ks], lambda p: epi(n, R, p[0]),
                    rows_, rows_ // 8 * (len(ks) - 1), nt=nt, acc=True, tail=rows_ // 8 * cost(n))

    def quad(name, w, lhs, sums, j, cols_, R, epi, cost):
        tile, wsum, nt, kp, kl = Wt[w] if isinstance(w, int) else w
        h, S2, c = len(kp), slice(R.start // 2, R.stop // 2), {}
        a_ = lambda i, k: _top(lhs(k) if callable(lhs) else lhs[R, C(k)], i)
        s_ = sums if callable(sums) else (lambda i, p: sums[S2, C(h * i + p)])
        prod = lambda fa_, fb_: [(lambda p=p: (fa_(p), fb_(p))) for p in range(h)]
        left = lambda i, n: [(lambda k=k: (a_(i, k), tile(k, n))) for k in kl]
        mk = lambda tiles, f, x=0: Unit(name, tiles, lambda p: f(p[0]), 64, 8 * len(tiles), nt=nt, acc=True, tail=x)

        def e1(m):
            u7.res, u6.res = [m], [m]

        def e4(m):
            c[11], c[21] = c[11] + m, m

        def e2(m):
            c[21], c[22] = c[21] + m, c[22] - m
            l21.res = [c[21]]

        def e5(m):
            c[12] = m
            epi(cols_[0], R, _zip(c[11] - m, c[21]))

        def e3(m):
            l12.res, c[22] = [c[12] + m], c[22] + m
            if not kl:
                l12.epi(l12.res)
        u1 = mk(prod(lambda p: s_(0, p), lambda p: wsum(0, p, j)), e1)
        u7 = mk(prod(lambda p: s_(4, p), lambda p: wsum(4, p, j)) + left(0, cols_[0]), lambda m: c.update({11: m}))
        u6 = mk(prod(lambda p: s_(3, p), lambda p: wsum(3, p, j)) + left(1, cols_[1]), lambda m: c.update({22: m}))
        u4 = mk(prod(lambda p: a_(1, kp[p][1]), lambda p: wsum(2, p, j)), e4)
        u2 = mk(prod(lambda p: s_(1, p), lambda p: tile(kp[p][0], cols_[0])), e2, 8)
        l21 = mk(left(1, cols_[0]), lambda m: c.update({21: m}))
        u5 = mk(prod(lambda p: s_(2, p), lambda p: tile(kp[p][1], cols_[1])), e5, 16 * cost(cols_[0]))
        u3 = mk(prod(lambda p: a_(0, kp[p][0]), lambda p: wsum(1, p, j)), e3, 8 if kl else 8 + 16 * cost(cols_[1]))
        l12 = mk(left(0, cols_[1]), lambda m: epi(cols_[1], R, _zip(m, c[22])), 16 * cost(cols_[1]))
        return [u1, u7, u6, u4, u2, l21, u5, u3, l12]

    LH, RH = [0, 4, 3, (1, 1), 1, 2, (0, 0)], [0, 4, 3, 2, (0, 0), (1, 1), 1]
    L2 = {3: (w3n_w, ws_w[2], w3t, KF[:6], n2t), 4: (w4_w, ws_w[3], w4t, ND, a_t)}

    def wsums2(w):
        w_w, s_w, ws2, cp_, _ = L2[w]
        kp, nj = Wt[w][3], len(cp_)

        def mk(o, p2, j2, r):
            def load(u, v):
                p, j, y = 2 * p2 + u, 2 * j2 + v, RH[o]
                if isinstance(y, int):
                    return s_w[pl.ds(64 * p + r // 2, 8), C(nj * y + j)]
                return w_w[pl.ds(64 * kp[p][y[0]] + r // 2, 8), C(cp_[j][y[1]])]

            def store(m, x):
                ws2[pl.ds(128 * p2 + r, 16), C((5 * o + m) * (nj // 2) + j2)] = x
            return sums_task(load, store, False)
        return [mk(o, p2, j2, r) for j2 in range(nj // 2) for o in range(7) for p2 in range(len(kp) // 2)
                for r in range(0, 128, 16)]

    def wsums4():
        form = [((0, 0), (1, 1), 1), ((0, 1), (1, 1), -1), ((1, 0), (0, 0), -1), ((0, 0), (0, 1), 1), ((1, 0), (1, 1), 1)]

        def mk(o, p2, r):
            def fn(a):
                def blk(p, j, uv, t):
                    x = w4_w[pl.ds(64 * KF[p][uv[0]] + r // 2, 8), C(ND[j][uv[1]])]
                    return pltpu.bitcast(_tie(x, t), BF16).astype(F32)
                y = {}
                for u in range(2):
                    for j in range(2):
                        p = 2 * p2 + u
                        if isinstance(RH[o], int):
                            f = form[RH[o]]
                            x1, x2 = blk(p, j, f[0], a), blk(p, j, f[1], None)
                            y[u, j] = x1 + x2 if f[2] > 0 else x1 - x2
                            w4s[pl.ds(128 * p + r, 16), C(2 * RH[o] + j)] = y[u, j].astype(BF16)
                        else:
                            y[u, j] = blk(p, j, RH[o], a if u == j else None)
                for m, f in enumerate(form):
                    x = y[f[0]] + y[f[1]] if f[2] > 0 else y[f[0]] - y[f[1]]
                    w4t[pl.ds(128 * p2 + r, 16), C(5 * o + m)] = x.astype(BF16)
            return fn
        last = wsums(w4_w, w4s, KF, ND)
        return (last[48:56] + last[104:112]
                + [mk(o, p2, r) for o in range(7) for p2 in range(3) for r in range(0, 128, 16)])

    def lsums2(w, lhs_w, sums_w, sl):
        kp, xs2 = Wt[w][3], L2[w][4]
        h2 = len(kp) // 2

        def mk(o, p2, g):
            def load(u, v):
                p, ch, x = 2 * p2 + v, 2 * g + u, LH[o]
                if isinstance(x, int):
                    return sums_w[pl.ds(64 * sl + 8 * ch, 8), C(len(kp) * x + p)]
                return lhs_w[pl.ds(H * sl + 16 * ch + 8 * x[0], 8), C(kp[p][x[1]])]

            def store(m, x):
                xs2[pl.ds(16 * g, 16), C((5 * o + m) * h2 + p2)] = x
            return sums_task(load, store, True)
        return [[mk(o, p2, g) for o in range(7) for g in range(4)] for p2 in range(h2)]

    def quad2(name, w, lhs, sums, j2, epi, cost):
        tile, wsum, nt, kp, kl = Wt[w]
        ws2, cp_, xs2 = L2[w][2:]
        h, h2, nj2, c, R = len(kp), len(kp) // 2, len(cp_) // 2, {}, slice(0, T)

        def done(j, v):
            val = _zip(c[j, 1, v], c[j, 2, v])
            if not kl:
                return epi(cp_[j][v], R, val)
            c[j, v] = val

        def upd(o, j, m):
            for i, v, sg in (((1, 0, 1), (2, 1, 1)), ((1, 0, 1),), ((2, 1, 1),), ((1, 0, 1), (2, 0, 1)),
                             ((2, 0, 1), (2, 1, -1)), ((1, 0, -1), (1, 1, 1)), ((1, 1, 1), (2, 1, 1)))[o]:
                k = (j, i, v)
                c[k] = m if k not in c else (c[k] + m if sg > 0 else c[k] - m)
            if o >= 5:
                done(j, o - 5)

        def inner(o):
            x, y = LH[o], RH[o]
            xo = ((lambda p: sums[:, C(h * x + p)]) if isinstance(x, int)
                  else (lambda p: _top(lhs[:, C(kp[p][x[1]])], x[0])))
            yo = ((lambda p, j: wsum(y, p, j)) if isinstance(y, int)
                  else (lambda p, j: tile(kp[p][y[0]], cp_[j][y[1]])))
            w_ = (yo, lambda m, p2, _: ws2[C(p2), C((5 * o + m) * nj2 + j2)], nt,
                  [(2 * i, 2 * i + 1) for i in range(h2)], list(range(2 * h2, h)))
            return quad(name, w_, xo, lambda m, p2: xs2[:, C((5 * o + m) * h2 + p2)], 0, (2 * j2, 2 * j2 + 1),
                        HS[0], lambda j, _, m: upd(o, j, m), lambda j: 1.5 + KS + (2 * cost(0) if o >= 5 and not kl else 0))

        def rest(j, v, Q):
            return [Unit(name, [lambda: (lhs[Q, C(k)], tile(k, cp_[j][v]))],
                         lambda p: epi(cp_[j][v], Q, p[0] + c[j, v][Q]), 64, 8 * (cost(cp_[j][v]) + 1)) for k in kl]
        return cat(inner(o) for o in range(7)), [u for Q in QS for j in (2 * j2, 2 * j2 + 1) for v in range(2)
                                                 for u in rest(j, v, Q)]

    def mm(name, w, lhs, sums, epi, cost):
        if sums is None:
            return [[plain(name, w, lhs, n, R, epi, cost) for R in HS] for n in range(NT)]
        return [[plain(name, w, lhs, 0, R, epi, cost) for R in QS]] + [
            [u for R in HS for u in quad(name, w, lhs, sums, j, ND[j], R, epi, cost)] for j in range(2)]

    def mm1(name, hs, sl, fast=False):
        def epi(n, R, p):
            h1_v[n, pl.ds(hs * T + 8 + R.start, R.stop - R.start), :] = _gelu2(p)
        return cat(mm(name, 1, view(n1_v, sl), n1s if fast else None, epi, lambda n: 5 + KS))

    def mm2(name, sl, xs, x1s, fast=False):
        def epi(n, R, p):
            view(x1_v, x1s)[R, C(n)] = view(hb_v, xs)[R, C(n)] + p
        return cat(mm(name, 2, view(g_v, sl), gs if fast else None, epi, lambda n: 1 + KS))

    def mm3(name, sl, fast=True, host=None):
        nn, aa, ss, keep, tail = view(n2_v, sl), view(a_v, sl), view(a_s, sl, H), {}, []

        def epi(n, R, p):
            g = _gelu2(p)
            aa[R, C(n)] = g.astype(BF16)
            if not fast:
                return
            if n % 2 == 0 and n < 12:
                keep[n] = g
                return
            pair = (keep.pop(n - 1), g) if n % 2 else (g, tail[R.start // 128][R.start % 128:R.start % 128 + 64])
            for i, x in enumerate(_lhs_sums(*pair)):
                ss[R.start // 2:R.stop // 2, C(7 * i + n // 2)] = x.astype(BF16)

        c3 = lambda n: 5.5 + 0.5 * KS + (3.75 + 1.25 * KS if fast and (n % 2 or n == 12) else 0)

        def rem(R):
            def f(p):
                tail.append(jnp.concatenate([_gelu2(p[0]), jnp.zeros((64, 128), F32)], axis=0).T)
                aa[R, C(13)] = tail[-1].astype(BF16)
            return Unit(name, [(lambda k=k: (w3_v[13 * 128:F, C(k)], nn[R, C(k)])) for k in range(NT)], f, 64, 84,
                        nt=True, acc=True)
        odd = [rem(R) for R in HS] + [plain(name, 3 if fast else 0, nn, 12, R, epi, c3) for R in QS]
        if not fast:
            return odd + [plain(name, 0, nn, n, R, epi, c3) for p in KF[:6] for R in HS for n in p]
        qd = [quad2(name + "_%d" % j, 3, nn, view(n2s, sl, H), j, epi, c3) for j in range(3)]
        mid = qd[0][0] + _weave(qd[1][0], qd[0][1]) + _weave(qd[2][0], qd[1][1])
        if host is None:
            return odd[:2] + mid + _weave(odd[2:], qd[2][1])
        for u in (odd[0], odd[2], odd[3]):
            u.name = name + "h"
        return [odd[0], odd[2], odd[3], odd[1]] + mid, _weave(odd[4:] + host, qd[2][1])

    def cp_out(j, osl, L, sm, R=slice(0, T)):
        return cp(o_v.at[pl.ds(osl * T + R.start, R.stop - R.start), L],
                  o_hbm.at[pl.ds(base(j, T) + R.start, R.stop - R.start), L], sem_o.at[sm])

    out_a = lambda j: cp_out(j, 0, slice(128, D), 0)
    out_b = lambda j: cp_out(j, 0, C(0), 1)
    last = []

    def mm4(name, j, sl, osl=0, xs=None, x1s=None, fast=True):
        oo = view(o_v, osl)

        def epi(n, R, p):
            if xs is None:
                oo[R, C(n)] = (r_v[R, C(n)] + mod_v[2, 0:1, C(n)] * p).astype(BF16)
            else:
                oo[R, C(n)] = (view(x_v, xs)[R, C(n)] + mod_v[2, 0:1, C(n)]
                               * (view(x1_v, x1s)[R, C(n)] + p)).astype(BF16)
            if osl == 2:
                last.append(cp_out(j, osl, C(n), 2, R))
                last[-1].start()
            elif R.stop == T and osl and n == NT - 1:
                last.append(cp_out(j, osl, slice(128 if osl == 3 else 0, D), 2))
                last[-1].start()
            elif R.stop == T and osl == 0 and n in (0, NT - 1):
                (out_a if n else out_b)(j).start()
        c4 = lambda n: (3 if xs is None else 4) + KS
        if fast:
            return ([plain(name, 4, view(a_v, sl), 0, R, epi, c4) for R in QS],
                    quad2(name + "q", 4, view(a_v, sl), view(a_s, sl, H), 0, epi, c4)[0])
        return mm(name, 4, view(a_v, sl), None, epi, c4)

    def split(us):
        n = 4 // len(us)
        m, mks, st = us[0].rows // n, [u.tiles.pop(0) for u in us], {}

        def piece(i, k):
            if i not in st:
                st[i] = mks[i]()
            return st[i][0][m * k:m * (k + 1)], st[i][1]

        def epi(p):
            for i, u in enumerate(us):
                u.res = [jnp.concatenate(p[n * i:n * (i + 1)], axis=0)]
        return _flat([Unit(us[0].name, [(lambda i=i, k=k: piece(i, k)) for i in range(len(us)) for k in range(n)],
                           epi, m, 0, nt=us[0].nt)])

    W = lambda nm: [("wait", nm)]
    run = lambda fns: [("run", "run", lambda: [fn(None) for fn in fns])]
    one = lambda us: [_flat([u]) for u in us]
    nm = lambda x: (lambda n: x)

    seq, grp = [], []
    for s in range(NC):
        seq += W("c%d" % s) + _flat(mmK(s) + mmU(nm("U%d" % s), s % 2, NC - 1 - s))
        grp.append(Group("kv%d" % s, cat(kv(s, s % 2)), 50, ["c%d" % s], ["U%d" % s], 100))
    inv = [mmI(lambda n: "I%d" % n, s, s) for s in range(NC)]
    seq += W("c3") + _flat(mmK(3) + mmK(4) + [inv[s][t] for t in range(NT) for s in range(NC)])
    macs = [mac(s + 1, NC - 1 - s, s) for s in range(NC)]
    grp.append(Group("mac00", macs[0][0], 12, ["c1"], ["c2"], 0))
    grp.append(Group("mac01", macs[1][0] + macs[0][1] + macs[1][1], 16, ["c2"], ["c3"], 0))
    for t in range(NT):
        grp.append(Group("mac%d" % t, cat(macs[s][t] for s in range(2 if t < 2 else 0, NC)), 24 if t < 2 else 18,
                         ["c3", "K%d" % t], ["I%d" % t], 100, 150))
    start = lambda cs: [("run", "run", lambda: [c.start() for c in cs])]
    f0, f1 = front(0, 2, True), front(1, 1, True)
    seq += run(ahead(0))
    seq += W("wma") + _flat(mod("moda", 0, 3)) + run(f0[0] + f1[0] + ahead(1))
    seq += W("wmb") + start(next_kv(NC) + next_q(NC)) + _flat(mod("modb", 3, 5)) + run(f0[1])
    w1 = _flat(mm1("w1_0", 0, 0) + mm1("w1_1", 1, 1))
    seq += W("w1") + w1[:72] + W("w2") + w1[72:] + run(shift(0, 0))
    seq += _flat(mm2("w2_0", 0, 2, 1) + mm1("w1_2", 2, 2)) + run(shift(1, 1)) + _flat(mm2("w2_1", 1, 1, 0))
    grp.append(Group("f1", f1[1], 80, ["w1"], ["w1_1"], 450))
    grp.append(Group("f2", front(2, 0), 80, ["w2"], ["w1_2"], 450))
    grp.append(Group("ln2_0", ln2(1, 0, False), 60, ["w2_0"], ["w3"], 450))
    grp.append(Group("ahead", cat(ahead(i) for i in range(2, NB - NC)), 19 + 2 * KS, ["w1"], ["end"], 100))
    grp.append(Group("ws1", wsums(w1_w, w1s, KD, ND), 26 + 5 * KS, ["w1"], ["end"], 100))
    grp.append(Group("ws2", wsums(w2_w, w2s, KD, ND), 26 + 5 * KS, ["w2"], ["end"], 100))
    grp.append(Group("ws3", w3_turn() + wsums(w3n_w, w3s, KD, KF[:6]) + wsums2(3), 22 + 5.5 * KS, ["w3"], ["end"], 100))
    grp.append(Group("ws4", wsums4(), 40 + 8 * KS, ["w4"], ["end"], 60))
    _wait(seq, "w3", back=1)
    w3 = mm3("w3_0", 0, False)
    _mix(seq, _flat(w3[6:]), [split(w3[4:6]) + _flat(w3[:6])], 0.1)
    mc = mod("modc", 5, 6)
    mc = _flat(mc[1:] + mc[:1])
    _wait(seq, "w4", mc[:5] + [("sync", "run", lambda: None)])
    w4 = cat(mm4("w4_0", 0, 0, 3, 2, 1, False)[1:])
    qs = [split([w4[-1 - i]]) for i in range(_phase(seq))]
    _mix(seq, _flat(w4), [mc[i:i + 4] for i in range(5, 25, 4)] + qs, 0.01, 0.4)
    assert _phase(seq) == 0
    grp.append(Group("resid", resid(2, 1), 16 + 5 * KS, ["modc"], ["end"], 100))
    grp.append(Group("ln2a", ln2_late(), 40, ["w3_0"], ["end"], 100))
    if os.environ.get("ONLY"):
        for g in grp:
            g.fns = [lambda a: None] * len(g.fns)
        seq = [it if it[0] != "run" else ("run", "run", lambda: None) for it in seq]
    _emit(seq, grp, zero, wait, BIAS[0])

    def step(s, carry):
        for c in next_kv(s) + next_q(s):
            c.wait()
        nxt = jnp.minimum(s + 1, NB - 1)
        seq, grp = [], []
        us, it = one(mmU(lambda n: "U%d" % n, 0, 0)), one(mmI(lambda n: "I%d" % n, 0, 0))
        w4, w4c = mm4("w4", s - 2, 0)[1], mm4("w4c", s - 3, 0)[0]
        w2 = mm2("w2", 0, 1, 0, True)
        w2 = w2[0:3] + w2[4:13] + w2[22:31] + w2[3:4] + w2[13:22] + w2[31:]
        for u in w2[:21]:
            u.name = "w2a"
        w2[0].name = "w2f"
        w3, w3e = mm3("w3", 0, host=w2[:E("HN", 4)])
        _mix(seq, _flat(w4c + w3),
             [us[0], us[1], us[2], it[0] + us[3], it[1] + us[4], it[2] + start(next_kv(nxt)), it[3], it[4]],
             E("LP3", 0.159), E("LP0", 0.7))
        w1a, w1b = mm1("w1a", 2, 0, True), mm1("w1b", 2, 0, True)
        w1a, w1b = _flat(w1a[0:2] + w1a[4:13] + w1a[22:31]), _flat(w1b[2:4] + w1b[13:22] + w1b[31:])
        kw = 9 * E("KW", 4)
        w4[kw - E("WM", 16)].name = "w4m"
        seq += _flat(w3e + w2[E("HN", 4):21] + w4[:kw]) + w1a + run(shift(1, 0, ((T - 32, 32),), gs))
        seq += _flat(w4[kw:] + w2[21:]) + w1b
        assert _phase(seq) == 0
        kvs, macs = kv(0, 0), mac(1, 0, 0, part=True)
        for t in range(NT):
            grp.append(Group("kv%d" % t, kvs[t], 50 + 2 * KS, ["start"], ["U%d" % t], E("KL", 260)))
            grp.append(Group("mac%d" % t, macs[t], 24 + 2 * KS, ["U%d" % t], ["I%d" % t], E("ML", 350), 150))
        iall = ["I%d" % t for t in range(NT)]
        ln = ln2(0, 0)
        grp.append(Group("ln2a", ln2_late(), 40, ["w2a", "w2"], ["end"], 100))
        xn = lsums2(3, n2_w, as_w[2], 0)[0]
        grp.append(Group("ln2b", ln[4:8] + ln[12:16], 78 + 20 * KS, ["start"], ["w3h"], 450))
        grp.append(Group("xna", [f for i, f in enumerate(xn) if i % 4 < 2], 26 + 5 * KS, ["start"], ["w3_0"], 150))
        grp.append(Group("xnb", [f for i, f in enumerate(xn) if i % 4 >= 2], 26 + 5 * KS, ["w4c"], ["w3_0"], 150, 0))
        grp.append(Group("resid", resid(1, 0, True), 9.5 + 5 * KS, ["w4c"], ["w2f"], 100))
        for p, ts in enumerate(lsums2(4, a_w, as_w[3], 0)):
            grp.append(Group("xa%d" % p, ts, 26 + 5 * KS, ["w3_%d" % p], ["w4q"], 150, 100))
        fr = front(0, 0, ss=n1s)
        grp.append(Group("fronta", fr[0], 50 + 8 * KS, ["w2f"], ["w1a"], E("FL", 240), 0))
        grp.append(Group("frontb", fr[1], 46 + 7 * KS, ["w4m"], ["w1b"], E("FL", 240), E("RB", 80)))
        fr[3].append(lambda: [c.start() for c in next_q(nxt)])
        grp.append(Group("fq", fr[2], 33 + 7 * KS, ["w4c"], ["w2f"], 100))
        grp.append(Group("spread", spread(), 30 + 8 * KS, iall, ["end"], 60))
        grp.append(Group("shift", shift_early(), 22 + 7 * KS, ["start"], ["w2f"], 200))
        _emit(seq, grp, zero, wait, BIAS[1])
        out_b(s - 3).wait()
        out_a(s - 2).wait()
        return carry

    lax.fori_loop(NC, NB, step, 0)

    seq, grp = [], []
    w47 = mm4("w4_7", NB - 1, 1, 2, 0, 1)
    seq += _flat(mm4("w4_5", NB - 3, 0)[0] + mm2("w2_7", 0, 0, 1, True) + mm3("w3_6", 0)
                 + cat(mm4("w4_6", NB - 2, 0, 1, 1, 0)) + mm3("w3_7", 1) + w47[0][:3] + w47[1] + w47[0][3:])
    grp.append(Group("shift7", shift(2, 0, [(r, 32) for r in range(0, T, 32)], gs), 24, ["start"], ["w2_7"], 200))
    ln = ln2(0, 0)
    grp.append(Group("ln2_6", ln[4:8] + ln[12:16], 75, ["start"], ["w3_6"], 1200))
    grp.append(Group("xn6", cat(lsums2(3, n2_w, as_w[2], 0)), 26 + 5 * KS, ["w4_5"], ["w3_6_0"], 200, 800))
    grp.append(Group("ln2_7", ln2(1, 1), 75, ["w4_6"], ["w3_7"], 1500))
    grp.append(Group("xn7", cat(lsums2(3, n2_w, as_w[2], 1)), 26 + 5 * KS, ["w4_6"], ["w3_7_0"], 200, 2100))
    for j in (6, 7):
        for p, ts in enumerate(lsums2(4, a_w, as_w[3], j - 6)):
            grp.append(Group("xa%d_%d" % (j, p), ts, 26 + 5 * KS, ["w3_%d_%d" % (j, p)], ["w4_%dq" % j], 200, 150))
    if os.environ.get("ONLY"):
        seq, grp = seq[:8 * 14], []
    _emit(seq, grp, zero, wait, BIAS[2])
    for c in next_kv(NB - 1) + next_q(NB - 1) + [out_b(NB - 3)] + last:
        c.wait()


@jax.jit
def pallas_adaLN_cond__ssm_conv_h3__mixer_s_mlp__prompt_kernel(
        A_q, A_k, A_v, A_shift_k, A_ssm_k, A_ssm_D, B_x, B_w1, B_w2, B_w3, B_w4, c, w_mod):
    any_ = pl.BlockSpec(memory_space=pl.ANY)
    V = pltpu.VMEM
    out = pl.pallas_call(
        kernel,
        in_specs=[any_] * 12,
        out_specs=any_,
        out_shape=jax.ShapeDtypeStruct((S, D), BF16),
        scratch_shapes=[
            [V((NT, H + 8, 128), U32)] * NC, [V((NT, H + 8, 128), U32)] * NC, [V((NT, H + 8, 128), U32)] * NC,
            [V((64, S), U32)] * NT,
            V((D // 2, D), U32), V((D // 2, D), U32), V((F // 2, D), U32), V((FT * 64, D), U32),
            [V((D // 2, 3 * D), U32), V((D // 2, 2 * D), U32), V((D // 2, D), U32)], V((4 * T, D), BF16),
            V((4, D), BF16), V((D,), BF16), V((1, D), BF16), V((8, 128), I32), pltpu.SMEM((8, 128), I32),
            V((5, 8, D), F32), V((6, 8, D), F32), V((T // 2, 4 * H), U32), V((GR // 2, 2 * T), U32),
            V((NB, 3 * T + 8, D), F32), V((NC, 3 * T + 8, D), F32), V((NB - NC, 2 * T + 8, D), F32), V((4 * T, 128), F32),
            V((T, D), U32), V((NC * T, D), U32), V((NT, NC * (T + 8) + 16, 128), F32),
            V((3 * T, D), F32), V((3 * T, D), F32), V((2 * T, D), F32), V((T, D), F32),
            V((3 * T // 2, D), U32), V((T, D), U32), V((T, D), U32), V((NT, NC * T + 24, 128), F32),
            V((T, (FT + 1) * 128), U32),
            [V((128, 11 * 128), U32)] * 2 + [V((128, 31 * 128), U32), V((448, 11 * 128), U32)],
            [V((64, 11 * 128), U32)] * 2 + [V((128, 11 * 128), U32), V((128, 35 * 128), U32)],
            V((D // 2, 13 * 128), U32), V((H, D), F32), V((T, 9 * 128), F32),
            [V((64, 105 * 128), U32), V((192, 35 * 128), U32), V((32, 35 * 128), U32), V((32, 105 * 128), U32)],
            pltpu.SemaphoreType.DMA((11,)), pltpu.SemaphoreType.DMA((1,)), pltpu.SemaphoreType.DMA((3,)),
        ],
        compiler_params=pltpu.CompilerParams(vmem_limit_bytes=110 << 20, disable_semaphore_checks=True,
                                             disable_bounds_checks=True),
        name="fused",
    )(A_q[0], A_k[0], A_v[0], A_shift_k.T, A_ssm_k, A_ssm_D, B_w1, B_w2, B_w3.T, B_w4, c, w_mod)
    return out[None]
```

```python
import heapq
import numpy as np
import jax
import jax.numpy as jnp
from jax import lax
from jax.experimental import pallas as pl
from jax.experimental.pallas import tpu as pltpu

S, D, F = 2048, 640, 1728
T = 256
H = T // 2
NB = S // T
NT = D // 128
FT = (F + 127) // 128
EPS = 1e-5
F32, BF16, U32, I32 = jnp.float32, jnp.bfloat16, jnp.uint32, jnp.int32
G_C1 = 0.044715 * float(np.sqrt(2.0 / np.pi))
G_C2 = float(np.sqrt(2.0 / np.pi))
G_A = G_C1 ** (1.0 / 3.0)
G_B = G_C2 / G_A
G_POST = 0.5 / G_A
RG = 16
GR = 80
NC = 3
DL = 450
KS = 1.9
SLOT = 32


def _dft(shape, f_axis, tau, scale=1.0):
    r = lax.broadcasted_iota(I32, shape, f_axis)
    l = lax.broadcasted_iota(I32, shape, 1 - f_axis)
    f = r & 127
    odd = ((f & 63) << 2) | ((f >> 6) << 1) | 1
    p = odd * tau(l) + ((r >> 7) << 8)
    a = ((p + 512) & 1023) - 512
    u = (256 - jnp.abs(a)).astype(F32) * (np.pi / 512.0)
    u2 = u * u
    c = [scale, -scale / 6.0, scale / 120.0, -scale / 5040.0, scale / 362880.0, -scale / 39916800.0]
    poly = c[5]
    for ci in c[4::-1]:
        poly = poly * u2 + ci
    return (u * poly).astype(BF16)


def _rstd(xc, mlp):
    s2, eps = (1.0 / (G_A * G_A), EPS / (G_POST * G_POST)) if mlp else (1.0, EPS)
    v = jnp.sum(xc * xc, axis=-1, keepdims=True) * (s2 / D) + eps * s2
    return jnp.exp2(jnp.log(v) * float(-0.5 / np.log(2.0)))


def _ln(x, mlp=False):
    xc = x - jnp.sum(x, axis=-1, keepdims=True) * (1.0 / D)
    return xc * _rstd(xc, mlp)


def _gelu2(x):
    u = x * (x * x + G_B)
    return x * (1.0 + jnp.tanh(u))


def _lo(w):
    return pltpu.bitcast(w << 16, F32)


def _hi(w):
    return pltpu.bitcast(w & jnp.uint32(0xFFFF0000), F32)


def _tie(x, a):
    if a is None:
        return x
    w = pltpu.bitcast(x[:, :128], U32)
    k = w.shape[0] // 8
    w = w | (a if k == 1 else jnp.concatenate([a] * k, axis=0))
    w = pltpu.bitcast(w, x.dtype)
    return w if x.shape[1] == 128 else jnp.concatenate([w, x[:, 128:]], axis=1)


def _top(x, i):
    return jnp.concatenate([x[r:r + 16] for r in range(16 * i, x.shape[0], 32)], axis=0)


def _zip(t, b):
    return jnp.concatenate([x[r:r + 16] for r in range(0, t.shape[0], 16) for x in (t, b)], axis=0)


def _lhs_sums(x1, x2):
    a11, a21, a12, a22 = _top(x1, 0), _top(x1, 1), _top(x2, 0), _top(x2, 1)
    return [a11 + a22, a21 + a22, a11 + a12, a21 - a11, a12 - a22]


def C(i):
    return slice(i * 128, (i + 1) * 128)


class Unit:
    def __init__(self, name, tiles, epi, rows, cost, nt=False, full=True, acc=False, tail=0):
        self.tail = tail
        self.acc, self.res = acc, []
        self.name, self.tiles, self.epi, self.rows, self.cost, self.nt, self.full = name, tiles, epi, rows, cost, nt, full


class Due:
    def __init__(self, val, delay):
        self.val, self.delay = val, delay


class Group:
    def __init__(self, name, fns, cost, rel, dead, lat, rlat=200):
        self.name, self.fns, self.cost, self.rel, self.dead, self.lat, self.rlat = name, fns, cost, rel, dead, lat, rlat


def _plan(seq, groups):
    busy, n = [0] * 4, 0
    start, end, tiles, bars = {}, {}, [], []
    for it in seq:
        if isinstance(it[0], Unit):
            u = it[0]
            m = n % 4
            n += 1
            t0, t1 = busy[m], busy[m] + max(u.rows, 32)
            busy[m] = t1
            tiles.append((t0, t1, u.cost / len(u.tiles) + (u.tail if it[1] == len(u.tiles) - 1 else 0)))
            start.setdefault(u.name, t0)
            end[u.name] = max(end.get(u.name, 0), t1)
        elif it[0] == "wait":
            t = max(busy)
            busy, n = [t] * 4, 0
            start[it[1]] = end[it[1]] = t
            bars.append(t)
    total = max(busy)
    start["end"] = end["end"] = total
    start["start"] = end["start"] = 0
    ns = total // SLOT + 2
    load = np.zeros(ns)
    for t0, t1, c in tiles:
        a, b = t0 // SLOT, max(t1 // SLOT, t0 // SLOT + 1)
        load[a:b] += c / (b - a)
    win = []
    for g in groups:
        r = max(end[x] + (0 if start[x] == end[x] else g.rlat) for x in g.rel)
        d = min(start[x] for x in g.dead) - g.lat
        ok = np.zeros(ns, bool)
        ok[r // SLOT:max(d // SLOT, r // SLOT + 1)] = True
        for b in bars:
            if r < b <= d:
                ok[max((b - g.lat) // SLOT, 0):b // SLOT] = False
        win.append(np.nonzero(ok)[0])
    alloc = [np.zeros(len(w)) for w in win]
    for _ in range(60):
        for i, g in enumerate(groups):
            w = win[i]
            load[w] -= alloc[i]
            base = load[w]
            vol = g.cost * len(g.fns)
            lo, hi = base.min(), base.max() + vol
            for _ in range(50):
                mid = 0.5 * (lo + hi)
                if np.maximum(mid - base, 0).sum() > vol:
                    hi = mid
                else:
                    lo = mid
            alloc[i] = np.maximum(hi - base, 0)
            load[w] += alloc[i]
    times = []
    for i, g in enumerate(groups):
        cum = np.cumsum(alloc[i])
        ts = []
        for k in range(len(g.fns)):
            x = (k + 0.5) * cum[-1] / len(g.fns)
            j = int(np.searchsorted(cum, x))
            prev = cum[j - 1] if j else 0.0
            ts.append(win[i][j] * SLOT + SLOT * (x - prev) / max(alloc[i][j], 1e-9))
        times.append(ts)
    return times


def _emit(seq, groups, zero, wait):
    times = _plan(seq, groups)
    left = {"start": 0}
    for it in seq:
        nm = it[0].name if isinstance(it[0], Unit) else it[1]
        left[nm] = left.get(nm, 0) + 1
    heap, pend, todo, cnt = [], {}, list(range(len(groups))), 0
    busy, n, due = [0] * 4, 0, []

    def release():
        nonlocal cnt
        for i in list(todo):
            g = groups[i]
            if all(left[x] == 0 for x in g.rel):
                todo.remove(i)
                pend[i] = len(g.fns)
                for t, fn in zip(times[i], g.fns):
                    heapq.heappush(heap, (t, cnt, i, fn))
                    cnt += 1

    def force(name):
        nonlocal heap
        for i, g in enumerate(groups):
            if name in g.dead:
                assert i not in todo, (g.name, name)
                if pend[i]:
                    for it in sorted(x for x in heap if x[2] == i):
                        it[3](None)
                    heap = [x for x in heap if x[2] != i]
                    heapq.heapify(heap)
                    pend[i] = 0

    release()
    for it in seq:
        if isinstance(it[0], Unit):
            u, k = it
            force(u.name)
            lhs, rhs = u.tiles[k]()
            t0 = busy[n % 4]
            while u.full and due and due[0][0] < t0 + u.rows:
                t, x = due.pop(0)
                r = min(max(int(t - t0), 0), u.rows - 1) // 16 * 8
                w = pltpu.bitcast(lhs, U32)
                x = pltpu.bitcast(x[:, :128], U32)
                parts = [w[:r], w[r:r + 8] | ((x[0:8] | x[8:16]) & zero), w[r + 8:]]
                lhs = pltpu.bitcast(jnp.concatenate([y for y in parts if y.shape[0]], axis=0), BF16)
            dn = (((1,), (1 if u.nt else 0,)), ((), ()))
            p = lax.dot_general(lhs, rhs, dn, preferred_element_type=F32)
            u.res = [p + u.res[0]] if (u.acc and u.res) else u.res + [p]
            m = n % 4
            n += 1
            t0 = busy[m]
            busy[m] = t0 + max(u.rows, 32)
            used = -8
            while u.full and heap and heap[0][0] < t0 + u.rows:
                r = min(max(int(heap[0][0] - t0), 0), u.rows - 1) // 8 * 8
                r = max(r, used + 8)
                if r >= u.rows or r > max(heap[0][0] - t0, 8) + 16:
                    break
                used = r
                t, _, i, fn = heapq.heappop(heap)
                pend[i] -= 1
                x = fn(pltpu.bitcast(p[r:r + 8], U32) & zero)
                if isinstance(x, Due):
                    due.append((t + x.delay, x.val))
                    due.sort(key=lambda e: e[0])
            if k == len(u.tiles) - 1:
                u.epi(u.res)
            left[u.name] -= 1
        elif it[0] == "wait":
            force(it[1])
            wait(it[1])
            busy, n, due = [max(busy)] * 4, 0, []
            left[it[1]] -= 1
        else:
            it[2]()
            left[it[1]] -= 1
        release()
    force("end")
    assert not heap and not todo


def _sum(ps):
    acc = ps[0]
    for p in ps[1:]:
        acc = acc + p
    return acc


def _flat(us):
    return [(u, i) for u in us for i in range(len(u.tiles))]


def _weave(a, b):
    out = []
    for i, u in enumerate(a):
        out += [u] + b[i * len(b) // len(a):(i + 1) * len(b) // len(a)]
    return out


def _phase(seq):
    n = 0
    for it in seq:
        n = n + 1 if isinstance(it[0], Unit) else (0 if it[0] in ("wait", "sync") else n)
    return n % 4


def _mix(seq, a, b, lo=0.0, hi=1.0):
    n, k = _phase(seq), 0
    for i, t in enumerate(a):
        if k < len(b) and n % 4 == 0 and t[1] != 1 and i >= len(a) * (lo + (hi - lo) * k / len(b)):
            seq.extend(b[k])
            k += 1
        seq.append(t)
        n += 1
    assert k == len(b)


def _wait(seq, name, head=(), back=0):
    r = _phase(seq) + 4 * back
    assert all(isinstance(it[0], Unit) for it in seq[len(seq) - r:])
    seq[len(seq) - r:len(seq) - r] = [("wait", name)] + list(head)


def kernel(q_hbm, k_hbm, v_hbm, sh_hbm, ssm_hbm, sd_hbm, w1_hbm, w2_hbm, w3_hbm, w4_hbm, c_hbm, wm_hbm,
           o_hbm,
           q_n, k_n, v_n, ssm_w, w1_w, w2_w, w3_w, w4_w, wm_w, o_v,
           sh_v, sd_v, c_v, zsrc, z_s, taps, mod_v, tf_w, tg_w,
           kf, uf, acc, zraw, kv_w, zz_w, y_v, x_v, hb_v, x1_v, r_v, n1_w, n2_w, g_w, h1_v, a_w,
           ws_w, as_w, w3n_w, top_v, st_v, l2_w,
           sem, sem_b, sem_o):
    bf = lambda r: r.bitcast(BF16)
    w1_v, w2_v, w3_v, w4_v = bf(w1_w), bf(w2_w), bf(w3_w), bf(w4_w)
    wm_v = {0: bf(wm_w[0]), 3: bf(wm_w[1]), 5: bf(wm_w[2])}
    tf_v, tg_v, n1_v, n2_v, g_v = bf(tf_w), bf(tg_w), bf(n1_w), bf(n2_w), bf(g_w)
    a_v, kv_v, zz_v = bf(a_w), bf(kv_w), bf(zz_w)
    w1s, w2s, w3s, w4s = [bf(r) for r in ws_w]
    n1s, gs, n2s, a_s = [bf(r) for r in as_w]
    w3n = bf(w3n_w)
    w3t, w4t, n2t, a_t = [bf(r) for r in l2_w]
    cp = pltpu.make_async_copy
    cat = lambda ls: [x for l in ls for x in l]

    def base(j, n):
        return j * n if isinstance(j, int) else pl.multiple_of(j * n, n)

    def rows(j, n=1, size=T):
        return pl.ds(base(j, size), n * size)

    def view(ref, j, size=T):
        return ref.at[rows(j, 1, size)]

    dmas = {}

    def group(name, *mks):
        sm = sem.at[len(dmas)]
        dmas[name] = [c for mk in mks for c in mk(sm)]

    def ssm_in(t):
        return lambda sm: [cp(ssm_hbm.at[C(t)], bf(ssm_w[t]), sm)]

    def cols(src, start, n, dst, row=0):
        return lambda sm: [cp(src.at[pl.ds(start, n), C(t)], bf(dst).at[t, pl.ds(row, n)], sm) for t in range(NT)]

    def kv_in(s, sl):
        if isinstance(s, int):
            kk = cols(k_hbm, s * T - 16, T + 16, k_n[sl]) if s else cols(k_hbm, 0, T, k_n[sl], 16)
        else:
            kk = cols(k_hbm, pl.multiple_of(s * T - 16, 16), T + 16, k_n[sl])
        return lambda sm: kk(sm) + cols(v_hbm, base(s, T), T, v_n[sl])(sm)

    def q_in(s, sl):
        return cols(q_hbm, base(s, T), T, q_n[sl])

    def wm_in(a, b):
        return lambda sm: [cp(wm_hbm.at[:, a * D:b * D], wm_v[a], sm)]

    def whole(src, dst):
        return lambda sm: [cp(src, dst, sm)]

    next_kv = lambda s: kv_in(s, 0)(sem_b.at[0])
    next_q = lambda s: q_in(s, 0)(sem_b.at[0])

    zsrc[...] = jnp.zeros((8, 128), I32)
    k_n[0][:, 0:8, :] = jnp.zeros((NT, 8, 128), U32)
    w4_w[F // 2:FT * 64, :] = jnp.zeros((FT * 64 - F // 2, D), U32)
    group("small", lambda sm: [cp(zsrc, z_s, sm), cp(sh_hbm, sh_v, sm), cp(sd_hbm, sd_v, sm), cp(c_hbm, c_v, sm)])
    for s in range(NC):
        group("c%d" % s, ssm_in(s), kv_in(s, s))
    group("c3", ssm_in(3), ssm_in(4))
    group("wma", wm_in(0, 3), q_in(0, 0), q_in(1, 1))
    group("wmb", wm_in(3, 5))
    group("w1", whole(w1_hbm, w1_v))
    group("w2", q_in(2, 2), whole(w2_hbm, w2_v))
    group("w3", whole(w3_hbm, w3_v))
    group("w4", whole(w4_hbm, w4_v.at[0:F]), wm_in(5, 6))
    for g in dmas.values():
        for c in g:
            c.start()

    def wait(name):
        for c in dmas[name]:
            c.wait()

    tau_b = lambda l: H + ((l + (H - 1)) & (H - 1))
    tf_v[:, C(0)] = _dft((T, H), 0, lambda l: jnp.where((l & 1) == 0, l, tau_b(l)), 1.0 / T)
    tf_v[:, C(1)] = _dft((T, H), 0, lambda l: jnp.where((l & 1) == 1, l, tau_b(l)), 1.0 / T)
    tf_v[:, C(2)] = _dft((T, H), 0, lambda l: 2 * l - H)
    tf_v[:, C(3)] = _dft((T, H), 0, lambda l: 2 * l + 1 - H)
    sin0 = lax.broadcasted_iota(I32, (GR, T), 1) >= H
    tg_v[:, 0:T] = _dft((GR, T), 1, lambda l: jnp.where(sin0 & (l == 0), H, 2 * l))
    tg_v[:, T:2 * T] = _dft((GR, T), 1, lambda l: 2 * l + 1)
    h1_v[:, 0:8, :] = jnp.zeros((NT, 8, 128), F32)
    h1_v[:, 8 + NC * T:16 + NC * T, :] = jnp.zeros((NT, 8, 128), F32)

    wait("small")
    z = jnp.clip(z_s[0, 0], 0, 1)
    zero = jnp.full((8, 128), z, I32).astype(U32)
    z8 = pl.multiple_of(z * 8, 8)
    for r in (x_v, hb_v, x1_v, r_v, zraw, n1_w, n2_w, g_w, a_w, kv_w, zz_w, *ws_w, *as_w, w3n_w, top_v, st_v, *l2_w):
        r[pl.ds(z8, 8), 0:128] = jnp.zeros((8, 128), r.dtype)
    for r in (kf, uf, acc, taps, mod_v):
        r[z, 0:8, 0:128] = jnp.zeros((8, 128), r.dtype)
    for r in (tf_w, tg_w):
        r[pl.ds(z8, 8), 0:128] = r[0:8, 0:128]
    sh = sh_v[...].astype(F32)
    for i in range(4):
        taps[i] = jnp.broadcast_to(sh[i:i + 1], (8, D))
    taps[4] = jnp.broadcast_to(sd_v[...].astype(F32).reshape(1, D) * (1.0 / T), (8, D))
    cf = c_v[...].astype(F32)
    silu_c = jnp.broadcast_to((cf / (1.0 + jnp.exp(-cf))).astype(BF16), (16, D))

    def mmK(n):
        def unit(m):
            st = []

            def rhs(i):
                if not st:
                    ev = (lax.broadcasted_iota(I32, (64, 128), 1) & 1) == 0
                    a = ssm_w[n][:, m * T:m * T + H]
                    b = pltpu.roll(ssm_w[n][:, m * T + H:(m + 1) * T], 1, 1)
                    st.extend([pltpu.bitcast(jnp.where(ev, a, b), BF16), pltpu.bitcast(jnp.where(ev, b, a), BF16)])
                return st[i]

            def epi(p):
                er, ei, or_, oi = p
                cur = [er, ei, or_, oi]
                if m:
                    pv = [zraw[C(4 * ((m - 1) % 2) + (q ^ 1)), :] for q in range(4)]
                    pm = lambda x, y, up: jnp.concatenate([x[:64] + y[:64], x[64:] - y[64:]] if up else
                                                          [x[:64] - y[:64], x[64:] + y[64:]], axis=0)
                    er, ei, or_, oi = [pm(cur[q], pv[q], q & 1) for q in range(4)]
                else:
                    er = er + taps[4, 0:1, C(n)]
                if m + 1 < NB:
                    for q in range(4):
                        zraw[C(4 * (m % 2) + q), :] = cur[q]
                for h, (cr, ci) in enumerate(((er + or_, ei + oi), (er - or_, ei - oi))):
                    B = h * 3 * H
                    kf[m, B:B + H, C(n)] = cr
                    kf[m, B + H:B + 2 * H, C(n)] = ci - cr
                    kf[m, B + 2 * H:B + 3 * H, C(n)] = ci + cr
            return Unit("K%d" % n, [(lambda i=i, r=r: (tf_v[r:r + H, C(i)], rhs(i))) for i in range(2) for r in (0, H)],
                        epi, H, 260, nt=True)
        return [unit(m) for m in range(NB)]

    def kv(s, sl):
        def mk(t, w):
            def fn(a):
                ld = lambda o, n: k_n[s][t, pl.ds(8 + w + o, n), :]
                c0 = jnp.concatenate([_tie(ld(0, 8), a), ld(8, 8)], axis=0).reshape(2, 8, 128)
                c1, c2 = ld(-1, 16).reshape(2, 8, 128), ld(-2, 16).reshape(2, 8, 128)
                s0, s1, s2, s3 = (taps[i, :, C(t)] for i in range(4))
                ke, ko, ke1, ko1, ko2 = _lo(c0), _hi(c0), _lo(c1), _hi(c1), _hi(c2)
                wv = v_n[s][t, w:w + 16, :].reshape(2, 8, 128)
                kve = ((s0 * ke + s1 * ko1) + (s2 * ke1 + s3 * ko2)) * _lo(wv)
                kvo = ((s0 * ko + s1 * ke) + (s2 * ko1 + s3 * ke1)) * _hi(wv)
                kv_v[pl.ds(sl * T + w, 16), C(t)] = kve.reshape(16, 128).astype(BF16)
                kv_v[pl.ds(sl * T + H + w, 16), C(t)] = kvo.reshape(16, 128).astype(BF16)
            return fn
        return [[mk(t, w) for w in range(0, H, 16)] for t in range(NT)]

    def mmU(name, sl, us):
        def unit(n):
            def epi(p):
                er, ei, or_, oi = p
                for h, (cr, ci) in enumerate(((er + or_, ei + oi), (er - or_, ei - oi))):
                    B = h * 3 * H
                    uf[us, B:B + H, C(n)] = cr + ci
                    uf[us, B + H:B + 2 * H, C(n)] = cr
                    uf[us, B + 2 * H:B + 3 * H, C(n)] = ci
            return Unit(name(n), [(lambda i=i, r=r: (tf_v[r:r + H, C(2 + i)], kv_v[pl.ds(sl * T + i * H, H), C(n)]))
                                  for i in range(2) for r in (0, H)], epi, H, 96 + 96 * KS)
        return [unit(n) for n in range(NT)]

    def cmul(m0, u0, n, h, row, L, a):
        t = []
        for i in range(3):
            Rw = slice((3 * h + i) * H + row, (3 * h + i) * H + row + 8)
            kk = kf[m0:m0 + n, Rw, L]
            if i == 0 and a is not None:
                k0 = _tie(kk[0], a)[None]
                kk = k0 if n == 1 else jnp.concatenate([k0, kk[1:]], axis=0)
            t.append(jnp.sum(kk * uf[u0:u0 + n, Rw, L], axis=0))
        return t[0] - t[2], t[0] + t[1]

    def AR(h, q, row):
        return slice((2 * h + q) * H + row, (2 * h + q) * H + row + 8)

    def mac(n, u0, sl, part=False):
        def mk(t, rc):
            st, fin = [], []

            def piece(i):
                def fn(a):
                    h, row = i & 1, rc + (i >> 1) * 8
                    zr, zi = cmul(0, u0, n, h, row, C(t), a)
                    if part:
                        zr, zi = zr + acc[0, AR(h, 0, row), C(t)], zi + acc[0, AR(h, 1, row), C(t)]
                    st.append((zr, zi))
                    if h:
                        (pr, pi), (mr, mi) = st[-2:]
                        fin.append([pr + mr, pi + mi, pr - mr, pi - mi])
                    if i == 3:
                        for q in range(4):
                            zz_v[pl.ds(sl * 2 * T + q * H + rc, 16), C(t)] = jnp.concatenate(
                                [fin[0][q], fin[1][q]], axis=0).astype(BF16)
                return fn
            if not part:
                return [piece(i) for i in range(4)]
            both = lambda f, g: (lambda a: (f(a), g(None)))
            return [both(piece(0), piece(1)), both(piece(2), piece(3))]
        return [[fn for rc in range(0, H, 16) for fn in mk(t, rc)] for t in range(NT)]

    def pos():
        return [(t, h, row) for t in range(NT) for row in range(0, H, 8) for h in range(2)]

    def ahead(i):
        def mk(t, h, row):
            def fn(a):
                zr, zi = cmul(i + 1, 0, NC, h, row, C(t), a)
                acc[i, AR(h, 0, row), C(t)] = zr
                acc[i, AR(h, 1, row), C(t)] = zi
            return fn
        return [mk(*p) for p in pos()]

    def spread():
        n = NB - NC - 1

        def mk(t, h, row):
            def fn(a):
                p = []
                for i in range(3):
                    Rw = slice((3 * h + i) * H + row, (3 * h + i) * H + row + 8)
                    u = uf[0, Rw, C(t)]
                    p.append(kf[1:1 + n, Rw, C(t)] * (_tie(u, a) if i == 0 else u)[None])
                acc[0:n, AR(h, 0, row), C(t)] = acc[1:1 + n, AR(h, 0, row), C(t)] + (p[0] - p[2])
                acc[0:n, AR(h, 1, row), C(t)] = acc[1:1 + n, AR(h, 1, row), C(t)] + (p[0] + p[1])
            return fn
        return [mk(*p) for p in pos()]

    def mmI(name, sl, ys):
        def unit(n):
            def epi(p):
                ce, se, co, so = p
                sub = lax.broadcasted_iota(I32, (8, 128), 0)
                b0 = ys * (T + 8) + 8
                y_v[n, b0 + H - 1:b0 + H, :] = (ce[64:72] - se[0:8])[0:1]
                se = jnp.concatenate([jnp.where(sub == 0, 0.0, se[0:8]), se[8:]], axis=0)
                for d, cc, ss in ((0, ce[0:64], se), (1, co, so)):
                    y_v[n, pl.ds(b0 + H + d, 64, stride=2), :] = cc + ss
                    y_v[n, pl.ds(b0 + d - 1, 64, stride=2), :] = cc - ss
            return Unit(name(n), [(lambda i=i: (tg_v[0:(GR if i == 0 else 64), C(i)], zz_v[pl.ds(sl * 2 * T + i * H, H), C(n)]))
                                  for i in range(4)], epi, 64, 36 + 33 * KS)
        return [unit(n) for n in range(NT)]

    def mod(name, a, b):
        def unit(n):
            def epi(p):
                v = [_sum(p[i * NT:(i + 1) * NT])[0:8] for i in range(b - a)]
                if a == 0:
                    mod_v[0, :, C(n)] = v[0] * v[2]
                    mod_v[1, :, C(n)] = (v[1] + 1.0) * v[2]
                elif a == 3:
                    mod_v[3, :, C(n)] = v[0] * (1.0 / G_POST)
                    mod_v[4, :, C(n)] = (v[1] + 1.0) * (1.0 / G_POST)
                else:
                    mod_v[2, :, C(n)] = v[0] * G_POST
            return Unit(name, [(lambda i=i, k=k: (silu_c[:, C(k)], wm_v[a][C(k), pl.ds(i * D + n * 128, 128)]))
                               for i in range(b - a) for k in range(NT)], epi, 16, 10, full=False, acc=b - a == 1)
        return [unit(n) for n in range(NT)]

    HS = (slice(0, 128), slice(128, 256))
    QS = tuple(slice(r, r + 64) for r in range(0, T, 64))

    def tasks(f, due=None, tie=True, n=RG):
        def mk(R):
            def fn(a):
                x = f(R, a if tie else None)
                return Due(x, due) if due else None
            return fn
        return [mk(slice(r, r + n)) for r in range(0, T, n)]

    def load_y(sl, R):
        b0, back = sl * (T + 8) + 8, 7 - lax.broadcasted_iota(I32, (8, 128), 0)

        def ld(t, r):
            if r >= H:
                return y_v[t, b0 + r:b0 + r + 8, :]
            return jnp.take_along_axis(y_v[t, b0 + H - 8 - r:b0 + H - r, :], back, axis=0)
        return jnp.stack([jnp.concatenate([ld(t, r) for t in range(NT)], axis=1) for r in (R.start, R.start + 8)])

    def put(nn, ss, R, x):
        nn[R, :] = x.astype(BF16)
        tok = x
        if ss is not None:
            S2 = pl.ds(R.start // 32 * 16, 16)
            if R.stop % 32:
                top_v[S2, 0:2 * T] = x[:, 0:2 * T]
            else:
                if R.start % 32:
                    x = jnp.concatenate([top_v[S2, 0:2 * T], x[:, 0:2 * T]], axis=0)
                ss[S2, 0:5 * T] = jnp.concatenate(_lhs_sums(x[:, 0:T], x[:, T:2 * T]), axis=1).astype(BF16)
        return tok

    wide = lambda v: jnp.concatenate([v] * NT, axis=1)

    def mean(i, R, x):
        st_v[R, C(i)] = jnp.broadcast_to(jnp.sum(x, axis=-1, keepdims=True) * (1.0 / D), (x.shape[0], 128))

    def centred(src, i, R, a):
        return src[R, :] - wide(_tie(st_v[R, C(i)], a))

    def scale(src, i, g):
        def f(R, a):
            st_v[R, C(i + 1)] = jnp.broadcast_to(_rstd(centred(src, i, R, a), g), (RG, 128))
        return f

    def normed(src, i, R, a):
        return centred(src, i, R, a) * wide(st_v[R, C(i + 1)])

    def front(sl, xs, early=False, ss=None):
        xx, hh, nn = view(x_v, xs), view(hb_v, xs), view(n1_v, sl)

        def fa(R, a):
            q = [q_n[sl][t, R.start // 2:R.stop // 2, :] for t in range(NT)]
            q = jnp.concatenate([_tie(q[0], a)] + q[1:], axis=1)
            q = pltpu.bitcast(q, BF16).astype(F32).reshape(2, 8, D)
            x = (q + (_ln(q) * mod_v[1] + mod_v[0]) * load_y(sl, R)).reshape(RG, D)
            xx[R, :] = x
            if early:
                hh[R, :] = _ln(x)

        def fb(R, a):
            hh[R, :] = (_ln(_tie(xx[R, :], a).reshape(2, 8, D)) * mod_v[4] + mod_v[3]).reshape(RG, D)

        def fc(R, a):
            hb = _tie(hh[R, :], a)
            if early:
                hb = (hb.reshape(2, 8, D) * mod_v[4] + mod_v[3]).reshape(RG, D)
                hh[R, :] = hb
            nn[R, :] = _ln(hb, True).astype(BF16)
        if early:
            return tasks(fa), tasks(fc)
        if ss is None:
            return tasks(fa) + tasks(fb) + tasks(fc)
        qf = view(x_v, 2)

        def s1(R, a):
            q = [q_n[sl][t, R.start // 2:R.stop // 2, :] for t in range(NT)]
            q = pltpu.bitcast(jnp.concatenate([_tie(v, a) for v in q], axis=1), BF16).astype(F32)
            qf[R, :] = q
            mean(0, R, q)

        def s3(R, a):
            h = normed(qf, 0, R, a).reshape(2, 8, D) * mod_v[1] + mod_v[0]
            x = qf[R, :] + (h * load_y(sl, R)).reshape(RG, D)
            xx[R, :] = x
            mean(2, R, x)

        def s5(R, a):
            hb = (normed(xx, 2, R, a).reshape(2, 8, D) * mod_v[4] + mod_v[3]).reshape(RG, D)
            hh[R, :] = hb
            mean(4, R, hb)
        s7 = [f for g in tasks(lambda R, a: put(nn, ss, R, normed(hh, 4, R, a)), n=32) for f in (g, lambda a: None)]
        st = [tasks(s3), tasks(scale(xx, 2, False)), tasks(s5), tasks(scale(hh, 4, True)), s7]
        p = [tasks(s1), tasks(scale(qf, 0, False))]
        sk = 4.091

        def wave(ls):
            body = sorted((i * sk + g, i, g) for i in range(len(ls) - 1) for g in range(8))
            return [ls[i][g] for _, i, g in body] + ls[-1]
        qb = []
        done = lambda a: qb[0]()
        full = wave([x[8:] for x in p + st])
        k = full.index(p[0][15]) + 1
        return wave([x[:8] for x in st]), full[:k] + [done] + full[k:], cat(x[:8] for x in p), qb

    def shift(hs, sl, pieces=((0, 64), (64, 64), (128, 64), (192, 64)), ss=None):
        gg = view(g_v, sl)

        def one_tile(t, r, n, a):
            lane = lax.broadcasted_iota(I32, (n, 128), 1)
            ld = lambda d: h1_v[t, pl.ds(hs * T + 8 + r + d, n), :]
            if t == 0:
                g = ld(-1)
            elif t == 1:
                g = jnp.where(lane < 32, ld(-1), ld(1))
            elif t == 2:
                g = jnp.where(lane < 64, ld(1), ld(-2))
            elif t == 3:
                g = jnp.where(lane < 96, ld(-2), ld(2))
            else:
                g = ld(2)
            if a is not None:
                g = jnp.concatenate([_tie(g[i:i + 8], a) if i % 16 == 0 else g[i:i + 8]
                                     for i in range(0, n, 8)], axis=0)
            gg[r:r + n, C(t)] = g.astype(BF16)
            return g

        def mk(ts, r, n):
            def fn(a):
                g = [one_tile(t, r, n, a) for t in ts]
                if len(ts) == 2:
                    for i, x in enumerate(_lhs_sums(*g)):
                        ss[r // 2:(r + n) // 2, C(2 * i + ts[0])] = x.astype(BF16)
            return fn
        sets = [(t,) for t in range(NT)] if ss is None else [(0, 2), (1, 3), (4,)]
        return [mk(ts, r, n) for ts in sets for r, n in pieces]

    def shift_early():
        def keep(a):
            h1_v[:, 2 * T - 32:2 * T + 8, :] = h1_v[:, 3 * T - 32:3 * T + 8, :]
        return shift(2, 0, [(r, 32) for r in range(0, T - 32, 32)], gs) + [keep]

    def ln2(xs, sl, fast=True):
        xx, nn, ss = view(x1_v, xs), view(n2_v, sl), view(n2s, sl, H) if fast else None
        f = lambda R, a: put(nn, ss, R, _ln(_tie(xx[R, :], a), True))
        ts = tasks(f, 900) if sl else tasks(f, DL, False)
        return ts[0::2] + ts[1::2] if fast else tasks(f)

    def ln2_late():
        xx, nn, ss = view(x1_v, 0), view(n2_v, 0), view(n2s, 0, H)
        a_, b_ = tasks(lambda R, a: mean(6, R, _tie(xx[R, :], a))), tasks(scale(xx, 6, True))
        c_ = [f for g in tasks(lambda R, a: put(nn, ss, R, normed(xx, 6, R, a)), n=32)[:4] for f in (g, lambda a: None)]
        return a_[:8] + b_[:8] + c_

    def resid(xs, x1s, rotate=False):
        xx, x1 = view(x_v, xs), view(x1_v, x1s)
        tie = lambda v, a: v if a is None else pltpu.bitcast(pltpu.bitcast(v, U32) | wide(a), F32)

        def f(R, a):
            r_v[R, :] = xx[R, :] + tie(x1[R, :], a) * mod_v[2]

        def move(dst, src):
            def g(R, a):
                dst[R, :] = tie(src[R, :], a)
            return tasks(g, n=8)
        if not rotate:
            return tasks(f, n=8)
        return cat(zip(tasks(f, n=8), move(view(hb_v, 1), hb_v), move(xx, x_v)))

    KD, KF, ND = [(0, 2), (1, 3)], [(2 * i, 2 * i + 1) for i in range(7)], [(1, 2), (3, 4)]
    Wt = {1: (lambda k, n: w1_v[C(k), C(n)], lambda i, kp, j: w1s[C(kp), C(2 * i + j)], False, KD, [4]),
          2: (lambda k, n: w2_v[C(k), C(n)], lambda i, kp, j: w2s[C(kp), C(2 * i + j)], False, KD, [4]),
          0: (lambda k, n: w3_v[C(n), C(k)], None, True, KD, [4]),
          3: (lambda k, n: w3n[C(k), C(n)], lambda i, kp, j: w3s[C(kp), C(6 * i + j)], False, KD, [4]),
          4: (lambda k, n: w4_v[C(k), C(n)], lambda i, kp, j: w4s[C(kp), C(2 * i + j)], False, KF, [])}

    def sums_task(load, store, left):
        def fn(a):
            b = [[load(u, v) for v in range(2)] for u in range(2)]
            b[0][0], b[1][1] = _tie(b[0][0], a), _tie(b[1][1], a)
            (x11, x12), (x21, x22) = [[pltpu.bitcast(x, BF16).astype(F32) for x in row] for row in b]
            r = ((x11 + x22, x21 + x22, x11 + x12, x21 - x11, x12 - x22) if left else
                 (x11 + x22, x12 - x22, x21 - x11, x11 + x12, x21 + x22))
            for m, x in enumerate(r):
                store(m, x.astype(BF16))
        return fn

    def wsums(w_w, ws, rp, cp_):
        def mk(i, j, r):
            def store(m, x):
                ws[pl.ds(128 * i + r, 16), C(len(cp_) * m + j)] = x
            return sums_task(lambda u, v: w_w[pl.ds(64 * rp[i][u] + r // 2, 8), C(cp_[j][v])], store, False)
        return [mk(i, j, r) for j in range(len(cp_)) for i in range(len(rp)) for r in range(0, 128, 16)]

    def w3_turn():
        def mk(n, k):
            def fn(a):
                x = jnp.concatenate([_tie(w3_w[64 * n:64 * n + 8, C(k)], a), w3_w[64 * n + 8:64 * n + 64, C(k)]], axis=0)
                w3n[C(k), C(n)] = pltpu.bitcast(x, BF16).T
            return fn
        return [mk(n, k) for n in range(FT - 1) for k in range(NT)]

    def plain(name, w, lhs, n, R, epi, cost):
        tile, _, nt, kp, kl = Wt[w]
        ks = sorted([k for p in kp for k in p] + kl)
        rows_ = R.stop - R.start
        return Unit(name, [(lambda k=k: (lhs[R, C(k)], tile(k, n))) for k in ks], lambda p: epi(n, R, p[0]),
                    rows_, rows_ // 8 * (len(ks) - 1), nt=nt, acc=True, tail=rows_ // 8 * cost(n))

    def quad(name, w, lhs, sums, j, cols_, R, epi, cost):
        tile, wsum, nt, kp, kl = Wt[w] if isinstance(w, int) else w
        h, S2, c = len(kp), slice(R.start // 2, R.stop // 2), {}
        a_ = lambda i, k: _top(lhs(k) if callable(lhs) else lhs[R, C(k)], i)
        s_ = sums if callable(sums) else (lambda i, p: sums[S2, C(h * i + p)])
        prod = lambda fa_, fb_: [(lambda p=p: (fa_(p), fb_(p))) for p in range(h)]
        left = lambda i, n: [(lambda k=k: (a_(i, k), tile(k, n))) for k in kl]
        mk = lambda tiles, f, x=0: Unit(name, tiles, lambda p: f(p[0]), 64, 8 * len(tiles), nt=nt, acc=True, tail=x)

        def e1(m):
            u7.res, u6.res = [m], [m]

        def e4(m):
            c[11], c[21] = c[11] + m, m

        def e2(m):
            c[21], c[22] = c[21] + m, c[22] - m
            l21.res = [c[21]]

        def e5(m):
            c[12] = m
            epi(cols_[0], R, _zip(c[11] - m, c[21]))

        def e3(m):
            l12.res, c[22] = [c[12] + m], c[22] + m
            if not kl:
                l12.epi(l12.res)
        u1 = mk(prod(lambda p: s_(0, p), lambda p: wsum(0, p, j)), e1)
        u7 = mk(prod(lambda p: s_(4, p), lambda p: wsum(4, p, j)) + left(0, cols_[0]), lambda m: c.update({11: m}))
        u6 = mk(prod(lambda p: s_(3, p), lambda p: wsum(3, p, j)) + left(1, cols_[1]), lambda m: c.update({22: m}))
        u4 = mk(prod(lambda p: a_(1, kp[p][1]), lambda p: wsum(2, p, j)), e4)
        u2 = mk(prod(lambda p: s_(1, p), lambda p: tile(kp[p][0], cols_[0])), e2, 8)
        l21 = mk(left(1, cols_[0]), lambda m: c.update({21: m}))
        u5 = mk(prod(lambda p: s_(2, p), lambda p: tile(kp[p][1], cols_[1])), e5, 16 * cost(cols_[0]))
        u3 = mk(prod(lambda p: a_(0, kp[p][0]), lambda p: wsum(1, p, j)), e3, 8 if kl else 8 + 16 * cost(cols_[1]))
        l12 = mk(left(0, cols_[1]), lambda m: epi(cols_[1], R, _zip(m, c[22])), 16 * cost(cols_[1]))
        return [u1, u7, u6, u4, u2, l21, u5, u3, l12]

    LH, RH = [0, 4, 3, (1, 1), 1, 2, (0, 0)], [0, 4, 3, 2, (0, 0), (1, 1), 1]
    L2 = {3: (w3n_w, ws_w[2], w3t, KF[:6], n2t), 4: (w4_w, ws_w[3], w4t, ND, a_t)}

    def wsums2(w):
        w_w, s_w, ws2, cp_, _ = L2[w]
        kp, nj = Wt[w][3], len(cp_)

        def mk(o, p2, j2, r):
            def load(u, v):
                p, j, y = 2 * p2 + u, 2 * j2 + v, RH[o]
                if isinstance(y, int):
                    return s_w[pl.ds(64 * p + r // 2, 8), C(nj * y + j)]
                return w_w[pl.ds(64 * kp[p][y[0]] + r // 2, 8), C(cp_[j][y[1]])]

            def store(m, x):
                ws2[pl.ds(128 * p2 + r, 16), C((5 * o + m) * (nj // 2) + j2)] = x
            return sums_task(load, store, False)
        return [mk(o, p2, j2, r) for j2 in range(nj // 2) for o in range(7) for p2 in range(len(kp) // 2)
                for r in range(0, 128, 16)]

    def wsums4():
        form = [((0, 0), (1, 1), 1), ((0, 1), (1, 1), -1), ((1, 0), (0, 0), -1), ((0, 0), (0, 1), 1), ((1, 0), (1, 1), 1)]

        def mk(o, p2, r):
            def fn(a):
                def blk(p, j, uv, t):
                    x = w4_w[pl.ds(64 * KF[p][uv[0]] + r // 2, 8), C(ND[j][uv[1]])]
                    return pltpu.bitcast(_tie(x, t), BF16).astype(F32)
                y = {}
                for u in range(2):
                    for j in range(2):
                        p = 2 * p2 + u
                        if isinstance(RH[o], int):
                            f = form[RH[o]]
                            x1, x2 = blk(p, j, f[0], a), blk(p, j, f[1], None)
                            y[u, j] = x1 + x2 if f[2] > 0 else x1 - x2
                            w4s[pl.ds(128 * p + r, 16), C(2 * RH[o] + j)] = y[u, j].astype(BF16)
                        else:
                            y[u, j] = blk(p, j, RH[o], a if u == j else None)
                for m, f in enumerate(form):
                    x = y[f[0]] + y[f[1]] if f[2] > 0 else y[f[0]] - y[f[1]]
                    w4t[pl.ds(128 * p2 + r, 16), C(5 * o + m)] = x.astype(BF16)
            return fn
        last = wsums(w4_w, w4s, KF, ND)
        return (last[48:56] + last[104:112]
                + [mk(o, p2, r) for o in range(7) for p2 in range(3) for r in range(0, 128, 16)])

    def lsums2(w, lhs_w, sums_w, sl):
        kp, xs2 = Wt[w][3], L2[w][4]
        h2 = len(kp) // 2

        def mk(o, p2, g):
            def load(u, v):
                p, ch, x = 2 * p2 + v, 2 * g + u, LH[o]
                if isinstance(x, int):
                    return sums_w[pl.ds(64 * sl + 8 * ch, 8), C(len(kp) * x + p)]
                return lhs_w[pl.ds(H * sl + 16 * ch + 8 * x[0], 8), C(kp[p][x[1]])]

            def store(m, x):
                xs2[pl.ds(16 * g, 16), C((5 * o + m) * h2 + p2)] = x
            return sums_task(load, store, True)
        return [[mk(o, p2, g) for o in range(7) for g in range(4)] for p2 in range(h2)]

    def quad2(name, w, lhs, sums, j2, epi, cost):
        tile, wsum, nt, kp, kl = Wt[w]
        ws2, cp_, xs2 = L2[w][2:]
        h, h2, nj2, c, R = len(kp), len(kp) // 2, len(cp_) // 2, {}, slice(0, T)

        def done(j, v):
            val = _zip(c[j, 1, v], c[j, 2, v])
            if not kl:
                return epi(cp_[j][v], R, val)
            c[j, v] = val

        def upd(o, j, m):
            for i, v, sg in (((1, 0, 1), (2, 1, 1)), ((1, 0, 1),), ((2, 1, 1),), ((1, 0, 1), (2, 0, 1)),
                             ((2, 0, 1), (2, 1, -1)), ((1, 0, -1), (1, 1, 1)), ((1, 1, 1), (2, 1, 1)))[o]:
                k = (j, i, v)
                c[k] = m if k not in c else (c[k] + m if sg > 0 else c[k] - m)
            if o >= 5:
                done(j, o - 5)

        def inner(o):
            x, y = LH[o], RH[o]
            xo = ((lambda p: sums[:, C(h * x + p)]) if isinstance(x, int)
                  else (lambda p: _top(lhs[:, C(kp[p][x[1]])], x[0])))
            yo = ((lambda p, j: wsum(y, p, j)) if isinstance(y, int)
                  else (lambda p, j: tile(kp[p][y[0]], cp_[j][y[1]])))
            w_ = (yo, lambda m, p2, _: ws2[C(p2), C((5 * o + m) * nj2 + j2)], nt,
                  [(2 * i, 2 * i + 1) for i in range(h2)], list(range(2 * h2, h)))
            return quad(name, w_, xo, lambda m, p2: xs2[:, C((5 * o + m) * h2 + p2)], 0, (2 * j2, 2 * j2 + 1),
                        HS[0], lambda j, _, m: upd(o, j, m), lambda j: 1.5 + KS + (2 * cost(0) if o >= 5 and not kl else 0))

        def rest(j, v, Q):
            return [Unit(name, [lambda: (lhs[Q, C(k)], tile(k, cp_[j][v]))],
                         lambda p: epi(cp_[j][v], Q, p[0] + c[j, v][Q]), 64, 8 * (cost(cp_[j][v]) + 1)) for k in kl]
        return cat(inner(o) for o in range(7)), [u for Q in QS for j in (2 * j2, 2 * j2 + 1) for v in range(2)
                                                 for u in rest(j, v, Q)]

    def mm(name, w, lhs, sums, epi, cost):
        if sums is None:
            return [[plain(name, w, lhs, n, R, epi, cost) for R in HS] for n in range(NT)]
        return [[plain(name, w, lhs, 0, R, epi, cost) for R in QS]] + [
            [u for R in HS for u in quad(name, w, lhs, sums, j, ND[j], R, epi, cost)] for j in range(2)]

    def mm1(name, hs, sl, fast=False):
        def epi(n, R, p):
            h1_v[n, pl.ds(hs * T + 8 + R.start, R.stop - R.start), :] = _gelu2(p)
        return cat(mm(name, 1, view(n1_v, sl), n1s if fast else None, epi, lambda n: 5 + KS))

    def mm2(name, sl, xs, x1s, fast=False):
        def epi(n, R, p):
            view(x1_v, x1s)[R, C(n)] = view(hb_v, xs)[R, C(n)] + p
        return cat(mm(name, 2, view(g_v, sl), gs if fast else None, epi, lambda n: 1 + KS))

    def mm3(name, sl, fast=True, host=None):
        nn, aa, ss, keep, tail = view(n2_v, sl), view(a_v, sl), view(a_s, sl, H), {}, []

        def epi(n, R, p):
            g = _gelu2(p)
            aa[R, C(n)] = g.astype(BF16)
            if not fast:
                return
            if n % 2 == 0 and n < 12:
                keep[n] = g
                return
            pair = (keep.pop(n - 1), g) if n % 2 else (g, tail[R.start // 128][R.start % 128:R.start % 128 + 64])
            for i, x in enumerate(_lhs_sums(*pair)):
                ss[R.start // 2:R.stop // 2, C(7 * i + n // 2)] = x.astype(BF16)

        c3 = lambda n: 5.5 + 0.5 * KS + (3.75 + 1.25 * KS if fast and (n % 2 or n == 12) else 0)

        def rem(R):
            def f(p):
                tail.append(jnp.concatenate([_gelu2(p[0]), jnp.zeros((64, 128), F32)], axis=0).T)
                aa[R, C(13)] = tail[-1].astype(BF16)
            return Unit(name, [(lambda k=k: (w3_v[13 * 128:F, C(k)], nn[R, C(k)])) for k in range(NT)], f, 64, 84,
                        nt=True, acc=True)
        odd = [rem(R) for R in HS] + [plain(name, 3 if fast else 0, nn, 12, R, epi, c3) for R in QS]
        if not fast:
            return odd + [plain(name, 0, nn, n, R, epi, c3) for p in KF[:6] for R in HS for n in p]
        qd = [quad2(name + "_%d" % j, 3, nn, view(n2s, sl, H), j, epi, c3) for j in range(3)]
        mid = qd[0][0] + _weave(qd[1][0], qd[0][1]) + _weave(qd[2][0], qd[1][1])
        if host is None:
            return odd[:2] + mid + _weave(odd[2:], qd[2][1])
        for u in (odd[0], odd[2], odd[3]):
            u.name = name + "h"
        return [odd[0], odd[2], odd[3], odd[1]] + mid, _weave(odd[4:] + host, qd[2][1])

    def cp_out(j, osl, L, sm, R=slice(0, T)):
        return cp(o_v.at[pl.ds(osl * T + R.start, R.stop - R.start), L],
                  o_hbm.at[pl.ds(base(j, T) + R.start, R.stop - R.start), L], sem_o.at[sm])

    out_a = lambda j: cp_out(j, 0, slice(128, D), 0)
    out_b = lambda j: cp_out(j, 0, C(0), 1)
    last = []

    def mm4(name, j, sl, osl=0, xs=None, x1s=None, fast=True):
        oo = view(o_v, osl)

        def epi(n, R, p):
            if xs is None:
                oo[R, C(n)] = (r_v[R, C(n)] + mod_v[2, 0:1, C(n)] * p).astype(BF16)
            else:
                oo[R, C(n)] = (view(x_v, xs)[R, C(n)] + mod_v[2, 0:1, C(n)]
                               * (view(x1_v, x1s)[R, C(n)] + p)).astype(BF16)
            if osl == 2:
                last.append(cp_out(j, osl, C(n), 2, R))
                last[-1].start()
            elif R.stop == T and osl and n == NT - 1:
                last.append(cp_out(j, osl, slice(128 if osl == 3 else 0, D), 2))
                last[-1].start()
            elif R.stop == T and osl == 0 and n in (0, NT - 1):
                (out_a if n else out_b)(j).start()
        c4 = lambda n: (3 if xs is None else 4) + KS
        if fast:
            return ([plain(name, 4, view(a_v, sl), 0, R, epi, c4) for R in QS],
                    quad2(name + "q", 4, view(a_v, sl), view(a_s, sl, H), 0, epi, c4)[0])
        return mm(name, 4, view(a_v, sl), None, epi, c4)

    def split(us):
        n = 4 // len(us)
        m, mks, st = us[0].rows // n, [u.tiles.pop(0) for u in us], {}

        def piece(i, k):
            if i not in st:
                st[i] = mks[i]()
            return st[i][0][m * k:m * (k + 1)], st[i][1]

        def epi(p):
            for i, u in enumerate(us):
                u.res = [jnp.concatenate(p[n * i:n * (i + 1)], axis=0)]
        return _flat([Unit(us[0].name, [(lambda i=i, k=k: piece(i, k)) for i in range(len(us)) for k in range(n)],
                           epi, m, 0, nt=us[0].nt)])

    W = lambda nm: [("wait", nm)]
    run = lambda fns: [("run", "run", lambda: [fn(None) for fn in fns])]
    one = lambda us: [_flat([u]) for u in us]
    nm = lambda x: (lambda n: x)

    seq, grp = [], []
    for s in range(NC):
        seq += W("c%d" % s) + _flat(mmK(s) + mmU(nm("U%d" % s), s % 2, NC - 1 - s))
        grp.append(Group("kv%d" % s, cat(kv(s, s % 2)), 50, ["c%d" % s], ["U%d" % s], 100))
    inv = [mmI(lambda n: "I%d" % n, s, s) for s in range(NC)]
    seq += W("c3") + _flat(mmK(3) + mmK(4) + [inv[s][t] for t in range(NT) for s in range(NC)])
    macs = [mac(s + 1, NC - 1 - s, s) for s in range(NC)]
    grp.append(Group("mac00", macs[0][0], 12, ["c1"], ["c2"], 0))
    grp.append(Group("mac01", macs[1][0] + macs[0][1] + macs[1][1], 16, ["c2"], ["c3"], 0))
    for t in range(NT):
        grp.append(Group("mac%d" % t, cat(macs[s][t] for s in range(2 if t < 2 else 0, NC)), 24 if t < 2 else 18,
                         ["c3", "K%d" % t], ["I%d" % t], 100, 150))
    start = lambda cs: [("run", "run", lambda: [c.start() for c in cs])]
    f0, f1 = front(0, 2, True), front(1, 1, True)
    seq += run(ahead(0))
    seq += W("wma") + _flat(mod("moda", 0, 3)) + run(f0[0] + f1[0] + ahead(1))
    seq += W("wmb") + start(next_kv(NC) + next_q(NC)) + _flat(mod("modb", 3, 5)) + run(f0[1])
    w1 = _flat(mm1("w1_0", 0, 0) + mm1("w1_1", 1, 1))
    seq += W("w1") + w1[:72] + W("w2") + w1[72:] + run(shift(0, 0))
    seq += _flat(mm2("w2_0", 0, 2, 1) + mm1("w1_2", 2, 2)) + run(shift(1, 1)) + _flat(mm2("w2_1", 1, 1, 0))
    grp.append(Group("f1", f1[1], 80, ["w1"], ["w1_1"], 450))
    grp.append(Group("f2", front(2, 0), 80, ["w2"], ["w1_2"], 450))
    grp.append(Group("ln2_0", ln2(1, 0, False), 60, ["w2_0"], ["w3"], 450))
    grp.append(Group("ahead", cat(ahead(i) for i in range(2, NB - NC)), 19 + 2 * KS, ["w1"], ["end"], 100))
    grp.append(Group("ws1", wsums(w1_w, w1s, KD, ND), 26 + 5 * KS, ["w1"], ["end"], 100))
    grp.append(Group("ws2", wsums(w2_w, w2s, KD, ND), 26 + 5 * KS, ["w2"], ["end"], 100))
    grp.append(Group("ws3", w3_turn() + wsums(w3n_w, w3s, KD, KF[:6]) + wsums2(3), 22 + 5.5 * KS, ["w3"], ["end"], 100))
    grp.append(Group("ws4", wsums4(), 40 + 8 * KS, ["w4"], ["end"], 60))
    _wait(seq, "w3", back=1)
    w3 = mm3("w3_0", 0, False)
    _mix(seq, _flat(w3[6:]), [split(w3[4:6]) + _flat(w3[:6])], 0.1)
    mc = mod("modc", 5, 6)
    mc = _flat(mc[1:] + mc[:1])
    _wait(seq, "w4", mc[:5] + [("sync", "run", lambda: None)])
    w4 = cat(mm4("w4_0", 0, 0, 3, 2, 1, False)[1:])
    qs = [split([w4[-1 - i]]) for i in range(_phase(seq))]
    _mix(seq, _flat(w4), [mc[i:i + 4] for i in range(5, 25, 4)] + qs, 0.01, 0.4)
    assert _phase(seq) == 0
    grp.append(Group("resid", resid(2, 1), 16 + 5 * KS, ["modc"], ["end"], 100))
    grp.append(Group("ln2a", ln2_late(), 40, ["w3_0"], ["end"], 100))
    _emit(seq, grp, zero, wait)

    def step(s, carry):
        for c in next_kv(s) + next_q(s):
            c.wait()
        nxt = jnp.minimum(s + 1, NB - 1)
        seq, grp = [], []
        us, it = one(mmU(lambda n: "U%d" % n, 0, 0)), one(mmI(lambda n: "I%d" % n, 0, 0))
        w4, w4c = mm4("w4", s - 2, 0)[1], mm4("w4c", s - 3, 0)[0]
        w2 = mm2("w2", 0, 1, 0, True)
        w2 = w2[0:3] + w2[4:13] + w2[22:31] + w2[3:4] + w2[13:22] + w2[31:]
        for u in w2[:21]:
            u.name = "w2a"
        w2[0].name = "w2f"
        w3, w3e = mm3("w3", 0, host=w2[:4])
        _mix(seq, _flat(w4c + w3),
             [us[0], us[1], us[2], it[0] + us[3], it[1] + us[4], it[2] + start(next_kv(nxt)), it[3], it[4]],
             0.159, 0.7)
        w1a, w1b = mm1("w1a", 2, 0, True), mm1("w1b", 2, 0, True)
        w1a, w1b = _flat(w1a[0:2] + w1a[4:13] + w1a[22:31]), _flat(w1b[2:4] + w1b[13:22] + w1b[31:])
        kw = 9 * 4
        w4[kw - 16].name = "w4m"
        seq += _flat(w3e + w2[4:21] + w4[:kw]) + w1a + run(shift(1, 0, ((T - 32, 32),), gs))
        seq += _flat(w4[kw:] + w2[21:]) + w1b
        assert _phase(seq) == 0
        kvs, macs = kv(0, 0), mac(1, 0, 0, part=True)
        for t in range(NT):
            grp.append(Group("kv%d" % t, kvs[t], 50 + 2 * KS, ["start"], ["U%d" % t], 260))
            grp.append(Group("mac%d" % t, macs[t], 24 + 2 * KS, ["U%d" % t], ["I%d" % t], 350, 150))
        iall = ["I%d" % t for t in range(NT)]
        ln = ln2(0, 0)
        grp.append(Group("ln2a", ln2_late(), 40, ["w2a", "w2"], ["end"], 100))
        xn = lsums2(3, n2_w, as_w[2], 0)[0]
        grp.append(Group("ln2b", ln[4:8] + ln[12:16], 78 + 20 * KS, ["start"], ["w3h"], 450))
        grp.append(Group("xna", [f for i, f in enumerate(xn) if i % 4 < 2], 26 + 5 * KS, ["start"], ["w3_0"], 150))
        grp.append(Group("xnb", [f for i, f in enumerate(xn) if i % 4 >= 2], 26 + 5 * KS, ["w4c"], ["w3_0"], 150, 0))
        grp.append(Group("resid", resid(1, 0, True), 9.5 + 5 * KS, ["w4c"], ["w2f"], 100))
        for p, ts in enumerate(lsums2(4, a_w, as_w[3], 0)):
            grp.append(Group("xa%d" % p, ts, 26 + 5 * KS, ["w3_%d" % p], ["w4q"], 150, 100))
        fr = front(0, 0, ss=n1s)
        grp.append(Group("fronta", fr[0], 50 + 8 * KS, ["w2f"], ["w1a"], 240, 0))
        grp.append(Group("frontb", fr[1], 46 + 7 * KS, ["w4m"], ["w1b"], 240, 80))
        fr[3].append(lambda: [c.start() for c in next_q(nxt)])
        grp.append(Group("fq", fr[2], 33 + 7 * KS, ["w4c"], ["w2f"], 100))
        grp.append(Group("spread", spread(), 30 + 8 * KS, iall, ["end"], 60))
        grp.append(Group("shift", shift_early(), 22 + 7 * KS, ["start"], ["w2f"], 200))
        _emit(seq, grp, zero, wait)
        out_b(s - 3).wait()
        out_a(s - 2).wait()
        return carry

    lax.fori_loop(NC, NB, step, 0)

    seq, grp = [], []
    w47 = mm4("w4_7", NB - 1, 1, 2, 0, 1)
    seq += _flat(mm4("w4_5", NB - 3, 0)[0] + mm2("w2_7", 0, 0, 1, True) + mm3("w3_6", 0)
                 + cat(mm4("w4_6", NB - 2, 0, 1, 1, 0)) + mm3("w3_7", 1) + w47[0][:3] + w47[1] + w47[0][3:])
    grp.append(Group("shift7", shift(2, 0, [(r, 32) for r in range(0, T, 32)], gs), 24, ["start"], ["w2_7"], 200))
    ln = ln2(0, 0)
    grp.append(Group("ln2_6", ln[4:8] + ln[12:16], 75, ["start"], ["w3_6"], 1200))
    grp.append(Group("xn6", cat(lsums2(3, n2_w, as_w[2], 0)), 26 + 5 * KS, ["w4_5"], ["w3_6_0"], 200, 800))
    grp.append(Group("ln2_7", ln2(1, 1), 75, ["w4_6"], ["w3_7"], 1500))
    grp.append(Group("xn7", cat(lsums2(3, n2_w, as_w[2], 1)), 26 + 5 * KS, ["w4_6"], ["w3_7_0"], 200, 2100))
    for j in (6, 7):
        for p, ts in enumerate(lsums2(4, a_w, as_w[3], j - 6)):
            grp.append(Group("xa%d_%d" % (j, p), ts, 26 + 5 * KS, ["w3_%d_%d" % (j, p)], ["w4_%dq" % j], 200, 150))
    _emit(seq, grp, zero, wait)
    for c in next_kv(NB - 1) + next_q(NB - 1) + [out_b(NB - 3)] + last:
        c.wait()


@jax.jit
def pallas_adaLN_cond__ssm_conv_h3__mixer_s_mlp__prompt_kernel(
        A_q, A_k, A_v, A_shift_k, A_ssm_k, A_ssm_D, B_x, B_w1, B_w2, B_w3, B_w4, c, w_mod):
    any_ = pl.BlockSpec(memory_space=pl.ANY)
    V = pltpu.VMEM
    out = pl.pallas_call(
        kernel,
        in_specs=[any_] * 12,
        out_specs=any_,
        out_shape=jax.ShapeDtypeStruct((S, D), BF16),
        scratch_shapes=[
            [V((NT, H + 8, 128), U32)] * NC, [V((NT, H + 8, 128), U32)] * NC, [V((NT, H + 8, 128), U32)] * NC,
            [V((64, S), U32)] * NT,
            V((D // 2, D), U32), V((D // 2, D), U32), V((F // 2, D), U32), V((FT * 64, D), U32),
            [V((D // 2, 3 * D), U32), V((D // 2, 2 * D), U32), V((D // 2, D), U32)], V((4 * T, D), BF16),
            V((4, D), BF16), V((D,), BF16), V((1, D), BF16), V((8, 128), I32), pltpu.SMEM((8, 128), I32),
            V((5, 8, D), F32), V((6, 8, D), F32), V((T // 2, 4 * H), U32), V((GR // 2, 2 * T), U32),
            V((NB, 3 * T + 8, D), F32), V((NC, 3 * T + 8, D), F32), V((NB - NC, 2 * T + 8, D), F32), V((4 * T, 128), F32),
            V((T, D), U32), V((NC * T, D), U32), V((NT, NC * (T + 8) + 16, 128), F32),
            V((3 * T, D), F32), V((3 * T, D), F32), V((2 * T, D), F32), V((T, D), F32),
            V((3 * T // 2, D), U32), V((T, D), U32), V((T, D), U32), V((NT, NC * T + 24, 128), F32),
            V((T, (FT + 1) * 128), U32),
            [V((128, 11 * 128), U32)] * 2 + [V((128, 31 * 128), U32), V((448, 11 * 128), U32)],
            [V((64, 11 * 128), U32)] * 2 + [V((128, 11 * 128), U32), V((128, 35 * 128), U32)],
            V((D // 2, 13 * 128), U32), V((H, D), F32), V((T, 9 * 128), F32),
            [V((64, 105 * 128), U32), V((192, 35 * 128), U32), V((32, 35 * 128), U32), V((32, 105 * 128), U32)],
            pltpu.SemaphoreType.DMA((11,)), pltpu.SemaphoreType.DMA((1,)), pltpu.SemaphoreType.DMA((3,)),
        ],
        compiler_params=pltpu.CompilerParams(vmem_limit_bytes=110 << 20, disable_semaphore_checks=True,
                                             disable_bounds_checks=True),
        name="fused",
    )(A_q[0], A_k[0], A_v[0], A_shift_k.T, A_ssm_k, A_ssm_D, B_w1, B_w2, B_w3.T, B_w4, c, w_mod)
    return out[None]
```

```python
import heapq
import numpy as np
import jax
import jax.numpy as jnp
from jax import lax
from jax.experimental import pallas as pl
from jax.experimental.pallas import tpu as pltpu

S, D, F = 2048, 640, 1728
T = 256
H = T // 2
NB = S // T
NT = D // 128
FT = (F + 127) // 128
EPS = 1e-5
F32, BF16, U32, I32 = jnp.float32, jnp.bfloat16, jnp.uint32, jnp.int32
G_C1 = 0.044715 * float(np.sqrt(2.0 / np.pi))
G_C2 = float(np.sqrt(2.0 / np.pi))
G_A = G_C1 ** (1.0 / 3.0)
G_B = G_C2 / G_A
G_POST = 0.5 / G_A
RG = 16
GR = 80
NC = 3
DL = 450
KS = 1.9
SLOT = 32


def _dft(shape, f_axis, tau, scale=1.0):
    r = lax.broadcasted_iota(I32, shape, f_axis)
    l = lax.broadcasted_iota(I32, shape, 1 - f_axis)
    f = r & 127
    odd = ((f & 63) << 2) | ((f >> 6) << 1) | 1
    p = odd * tau(l) + ((r >> 7) << 8)
    a = ((p + 512) & 1023) - 512
    u = (256 - jnp.abs(a)).astype(F32) * (np.pi / 512.0)
    u2 = u * u
    c = [scale, -scale / 6.0, scale / 120.0, -scale / 5040.0, scale / 362880.0, -scale / 39916800.0]
    poly = c[5]
    for ci in c[4::-1]:
        poly = poly * u2 + ci
    return (u * poly).astype(BF16)


def _rstd(xc, mlp):
    s2, eps = (1.0 / (G_A * G_A), EPS / (G_POST * G_POST)) if mlp else (1.0, EPS)
    v = jnp.sum(xc * xc, axis=-1, keepdims=True) * (s2 / D) + eps * s2
    return jnp.exp2(jnp.log(v) * float(-0.5 / np.log(2.0)))


def _ln(x, mlp=False):
    xc = x - jnp.sum(x, axis=-1, keepdims=True) * (1.0 / D)
    return xc * _rstd(xc, mlp)


def _gelu2(x):
    u = x * (x * x + G_B)
    return x * (1.0 + jnp.tanh(u))


def _lo(w):
    return pltpu.bitcast(w << 16, F32)


def _hi(w):
    return pltpu.bitcast(w & jnp.uint32(0xFFFF0000), F32)


def _tie(x, a):
    if a is None:
        return x
    w = pltpu.bitcast(x[:, :128], U32)
    k = w.shape[0] // 8
    w = w | (a if k == 1 else jnp.concatenate([a] * k, axis=0))
    w = pltpu.bitcast(w, x.dtype)
    return w if x.shape[1] == 128 else jnp.concatenate([w, x[:, 128:]], axis=1)


def _top(x, i):
    return jnp.concatenate([x[r:r + 16] for r in range(16 * i, x.shape[0], 32)], axis=0)


def _zip(t, b):
    return jnp.concatenate([x[r:r + 16] for r in range(0, t.shape[0], 16) for x in (t, b)], axis=0)


def _lhs_sums(x1, x2):
    a11, a21, a12, a22 = _top(x1, 0), _top(x1, 1), _top(x2, 0), _top(x2, 1)
    return [a11 + a22, a21 + a22, a11 + a12, a21 - a11, a12 - a22]


def C(i):
    return slice(i * 128, (i + 1) * 128)


class Unit:
    def __init__(self, name, tiles, epi, rows, cost, nt=False, full=True, acc=False, tail=0):
        self.tail = tail
        self.acc, self.res = acc, []
        self.name, self.tiles, self.epi, self.rows, self.cost, self.nt, self.full = name, tiles, epi, rows, cost, nt, full


class Due:
    def __init__(self, val, delay):
        self.val, self.delay = val, delay


class Group:
    def __init__(self, name, fns, cost, rel, dead, lat, rlat=200):
        self.name, self.fns, self.cost, self.rel, self.dead, self.lat, self.rlat = name, fns, cost, rel, dead, lat, rlat


def _plan(seq, groups):
    busy, n = [0] * 4, 0
    start, end, tiles, bars = {}, {}, [], []
    for it in seq:
        if isinstance(it[0], Unit):
            u = it[0]
            m = n % 4
            n += 1
            t0, t1 = busy[m], busy[m] + max(u.rows, 32)
            busy[m] = t1
            tiles.append((t0, t1, u.cost / len(u.tiles) + (u.tail if it[1] == len(u.tiles) - 1 else 0)))
            start.setdefault(u.name, t0)
            end[u.name] = max(end.get(u.name, 0), t1)
        elif it[0] == "wait":
            t = max(busy)
            busy, n = [t] * 4, 0
            start[it[1]] = end[it[1]] = t
            bars.append(t)
    total = max(busy)
    start["end"] = end["end"] = total
    start["start"] = end["start"] = 0
    ns = total // SLOT + 2
    load = np.zeros(ns)
    for t0, t1, c in tiles:
        a, b = t0 // SLOT, max(t1 // SLOT, t0 // SLOT + 1)
        load[a:b] += c / (b - a)
    win = []
    for g in groups:
        r = max(end[x] + (0 if start[x] == end[x] else g.rlat) for x in g.rel)
        d = min(start[x] for x in g.dead) - g.lat
        ok = np.zeros(ns, bool)
        ok[r // SLOT:max(d // SLOT, r // SLOT + 1)] = True
        for b in bars:
            if r < b <= d:
                ok[max((b - g.lat) // SLOT, 0):b // SLOT] = False
        win.append(np.nonzero(ok)[0])
    alloc = [np.zeros(len(w)) for w in win]
    for _ in range(60):
        for i, g in enumerate(groups):
            w = win[i]
            load[w] -= alloc[i]
            base = load[w]
            vol = g.cost * len(g.fns)
            lo, hi = base.min(), base.max() + vol
            for _ in range(50):
                mid = 0.5 * (lo + hi)
                if np.maximum(mid - base, 0).sum() > vol:
                    hi = mid
                else:
                    lo = mid
            alloc[i] = np.maximum(hi - base, 0)
            load[w] += alloc[i]
    times = []
    for i, g in enumerate(groups):
        cum = np.cumsum(alloc[i])
        ts = []
        for k in range(len(g.fns)):
            x = (k + 0.5) * cum[-1] / len(g.fns)
            j = int(np.searchsorted(cum, x))
            prev = cum[j - 1] if j else 0.0
            ts.append(win[i][j] * SLOT + SLOT * (x - prev) / max(alloc[i][j], 1e-9))
        times.append(ts)
    return times


def _emit(seq, groups, zero, wait):
    times = _plan(seq, groups)
    left = {"start": 0}
    for it in seq:
        nm = it[0].name if isinstance(it[0], Unit) else it[1]
        left[nm] = left.get(nm, 0) + 1
    heap, pend, todo, cnt = [], {}, list(range(len(groups))), 0
    busy, n, due = [0] * 4, 0, []

    def release():
        nonlocal cnt
        for i in list(todo):
            g = groups[i]
            if all(left[x] == 0 for x in g.rel):
                todo.remove(i)
                pend[i] = len(g.fns)
                for t, fn in zip(times[i], g.fns):
                    heapq.heappush(heap, (t, cnt, i, fn))
                    cnt += 1

    def force(name):
        nonlocal heap
        for i, g in enumerate(groups):
            if name in g.dead:
                assert i not in todo, (g.name, name)
                if pend[i]:
                    for it in sorted(x for x in heap if x[2] == i):
                        it[3](None)
                    heap = [x for x in heap if x[2] != i]
                    heapq.heapify(heap)
                    pend[i] = 0

    release()
    for it in seq:
        if isinstance(it[0], Unit):
            u, k = it
            force(u.name)
            lhs, rhs = u.tiles[k]()
            t0 = busy[n % 4]
            while u.full and due and due[0][0] < t0 + u.rows:
                t, x = due.pop(0)
                r = min(max(int(t - t0), 0), u.rows - 1) // 16 * 8
                w = pltpu.bitcast(lhs, U32)
                x = pltpu.bitcast(x[:, :128], U32)
                parts = [w[:r], w[r:r + 8] | ((x[0:8] | x[8:16]) & zero), w[r + 8:]]
                lhs = pltpu.bitcast(jnp.concatenate([y for y in parts if y.shape[0]], axis=0), BF16)
            dn = (((1,), (1 if u.nt else 0,)), ((), ()))
            p = lax.dot_general(lhs, rhs, dn, preferred_element_type=F32)
            u.res = [p + u.res[0]] if (u.acc and u.res) else u.res + [p]
            m = n % 4
            n += 1
            t0 = busy[m]
            busy[m] = t0 + max(u.rows, 32)
            used = -8
            while u.full and heap and heap[0][0] < t0 + u.rows:
                r = min(max(int(heap[0][0] - t0), 0), u.rows - 1) // 8 * 8
                r = max(r, used + 8)
                if r >= u.rows or r > max(heap[0][0] - t0, 8) + 16:
                    break
                used = r
                t, _, i, fn = heapq.heappop(heap)
                pend[i] -= 1
                x = fn(pltpu.bitcast(p[r:r + 8], U32) & zero)
                if isinstance(x, Due):
                    due.append((t + x.delay, x.val))
                    due.sort(key=lambda e: e[0])
            if k == len(u.tiles) - 1:
                u.epi(u.res)
            left[u.name] -= 1
        elif it[0] == "wait":
            force(it[1])
            wait(it[1])
            busy, n, due = [max(busy)] * 4, 0, []
            left[it[1]] -= 1
        else:
            it[2]()
            left[it[1]] -= 1
        release()
    force("end")
    assert not heap and not todo


def _sum(ps):
    acc = ps[0]
    for p in ps[1:]:
        acc = acc + p
    return acc


def _flat(us):
    return [(u, i) for u in us for i in range(len(u.tiles))]


def _weave(a, b):
    out = []
    for i, u in enumerate(a):
        out += [u] + b[i * len(b) // len(a):(i + 1) * len(b) // len(a)]
    return out


def _phase(seq):
    n = 0
    for it in seq:
        n = n + 1 if isinstance(it[0], Unit) else (0 if it[0] in ("wait", "sync") else n)
    return n % 4


def _mix(seq, a, b, lo=0.0, hi=1.0):
    n, k = _phase(seq), 0
    for i, t in enumerate(a):
        if k < len(b) and n % 4 == 0 and t[1] != 1 and i >= len(a) * (lo + (hi - lo) * k / len(b)):
            seq.extend(b[k])
            k += 1
        seq.append(t)
        n += 1
    assert k == len(b)


def _wait(seq, name, head=(), back=0):
    r = _phase(seq) + 4 * back
    assert all(isinstance(it[0], Unit) for it in seq[len(seq) - r:])
    seq[len(seq) - r:len(seq) - r] = [("wait", name)] + list(head)


def kernel(q_hbm, k_hbm, v_hbm, sh_hbm, ssm_hbm, sd_hbm, w1_hbm, w2_hbm, w3_hbm, w4_hbm, c_hbm, wm_hbm,
           o_hbm,
           q_n, k_n, v_n, ssm_w, w1_w, w2_w, w3_w, w4_w, wm_w, o_v,
           sh_v, sd_v, c_v, zsrc, z_s, taps, mod_v, tf_w, tg_w,
           kf, uf, acc, zraw, kv_w, zz_w, y_v, x_v, hb_v, x1_v, r_v, n1_w, n2_w, g_w, h1_v, a_w,
           ws_w, as_w, w3n_w, top_v, st_v, l2_w,
           sem, sem_b, sem_o):
    bf = lambda r: r.bitcast(BF16)
    w1_v, w2_v, w3_v, w4_v = bf(w1_w), bf(w2_w), bf(w3_w), bf(w4_w)
    wm_v = {0: bf(wm_w[0]), 3: bf(wm_w[1]), 5: bf(wm_w[2])}
    tf_v, tg_v, n1_v, n2_v, g_v = bf(tf_w), bf(tg_w), bf(n1_w), bf(n2_w), bf(g_w)
    a_v, kv_v, zz_v = bf(a_w), bf(kv_w), bf(zz_w)
    w1s, w2s, w3s, w4s = [bf(r) for r in ws_w]
    n1s, gs, n2s, a_s = [bf(r) for r in as_w]
    w3n = bf(w3n_w)
    w3t, w4t, n2t, a_t = [bf(r) for r in l2_w]
    cp = pltpu.make_async_copy
    cat = lambda ls: [x for l in ls for x in l]

    def base(j, n):
        return j * n if isinstance(j, int) else pl.multiple_of(j * n, n)

    def rows(j, n=1, size=T):
        return pl.ds(base(j, size), n * size)

    def view(ref, j, size=T):
        return ref.at[rows(j, 1, size)]

    dmas = {}

    def group(name, *mks):
        sm = sem.at[len(dmas)]
        dmas[name] = [c for mk in mks for c in mk(sm)]

    def ssm_in(t):
        return lambda sm: [cp(ssm_hbm.at[C(t)], bf(ssm_w[t]), sm)]

    def cols(src, start, n, dst, row=0):
        return lambda sm: [cp(src.at[pl.ds(start, n), C(t)], bf(dst).at[t, pl.ds(row, n)], sm) for t in range(NT)]

    def kv_in(s, sl):
        if isinstance(s, int):
            kk = cols(k_hbm, s * T - 16, T + 16, k_n[sl]) if s else cols(k_hbm, 0, T, k_n[sl], 16)
        else:
            kk = cols(k_hbm, pl.multiple_of(s * T - 16, 16), T + 16, k_n[sl])
        return lambda sm: kk(sm) + cols(v_hbm, base(s, T), T, v_n[sl])(sm)

    def q_in(s, sl):
        return cols(q_hbm, base(s, T), T, q_n[sl])

    def wm_in(a, b):
        return lambda sm: [cp(wm_hbm.at[:, a * D:b * D], wm_v[a], sm)]

    def whole(src, dst):
        return lambda sm: [cp(src, dst, sm)]

    next_kv = lambda s: kv_in(s, 0)(sem_b.at[0])
    next_q = lambda s: q_in(s, 0)(sem_b.at[0])

    zsrc[...] = jnp.zeros((8, 128), I32)
    k_n[0][:, 0:8, :] = jnp.zeros((NT, 8, 128), U32)
    w4_w[F // 2:FT * 64, :] = jnp.zeros((FT * 64 - F // 2, D), U32)
    group("small", lambda sm: [cp(zsrc, z_s, sm), cp(sh_hbm, sh_v, sm), cp(sd_hbm, sd_v, sm), cp(c_hbm, c_v, sm)])
    for s in range(NC):
        group("c%d" % s, ssm_in(s), kv_in(s, s))
    group("c3", ssm_in(3), ssm_in(4))
    group("wma", wm_in(0, 3), q_in(0, 0), q_in(1, 1))
    group("wmb", wm_in(3, 5))
    group("w1", whole(w1_hbm, w1_v))
    group("w2", q_in(2, 2), whole(w2_hbm, w2_v))
    group("w3", whole(w3_hbm, w3_v))
    group("w4", whole(w4_hbm, w4_v.at[0:F]), wm_in(5, 6))
    for g in dmas.values():
        for c in g:
            c.start()

    def wait(name):
        for c in dmas[name]:
            c.wait()

    tau_b = lambda l: H + ((l + (H - 1)) & (H - 1))
    tf_v[:, C(0)] = _dft((T, H), 0, lambda l: jnp.where((l & 1) == 0, l, tau_b(l)), 1.0 / T)
    tf_v[:, C(1)] = _dft((T, H), 0, lambda l: jnp.where((l & 1) == 1, l, tau_b(l)), 1.0 / T)
    tf_v[:, C(2)] = _dft((T, H), 0, lambda l: 2 * l - H)
    tf_v[:, C(3)] = _dft((T, H), 0, lambda l: 2 * l + 1 - H)
    sin0 = lax.broadcasted_iota(I32, (GR, T), 1) >= H
    tg_v[:, 0:T] = _dft((GR, T), 1, lambda l: jnp.where(sin0 & (l == 0), H, 2 * l))
    tg_v[:, T:2 * T] = _dft((GR, T), 1, lambda l: 2 * l + 1)
    h1_v[:, 0:8, :] = jnp.zeros((NT, 8, 128), F32)
    h1_v[:, 8 + NC * T:16 + NC * T, :] = jnp.zeros((NT, 8, 128), F32)

    wait("small")
    z = jnp.clip(z_s[0, 0], 0, 1)
    zero = jnp.full((8, 128), z, I32).astype(U32)
    z8 = pl.multiple_of(z * 8, 8)
    for r in (x_v, hb_v, x1_v, r_v, zraw, n1_w, n2_w, g_w, a_w, kv_w, zz_w, *ws_w, *as_w, w3n_w, top_v, st_v, *l2_w):
        r[pl.ds(z8, 8), 0:128] = jnp.zeros((8, 128), r.dtype)
    for r in (kf, uf, acc, taps, mod_v):
        r[z, 0:8, 0:128] = jnp.zeros((8, 128), r.dtype)
    for r in (tf_w, tg_w):
        r[pl.ds(z8, 8), 0:128] = r[0:8, 0:128]
    sh = sh_v[...].astype(F32)
    for i in range(4):
        taps[i] = jnp.broadcast_to(sh[i:i + 1], (8, D))
    taps[4] = jnp.broadcast_to(sd_v[...].astype(F32).reshape(1, D) * (1.0 / T), (8, D))
    cf = c_v[...].astype(F32)
    silu_c = jnp.broadcast_to((cf / (1.0 + jnp.exp(-cf))).astype(BF16), (16, D))

    def mmK(n):
        def unit(m):
            st = []

            def rhs(i):
                if not st:
                    ev = (lax.broadcasted_iota(I32, (64, 128), 1) & 1) == 0
                    a = ssm_w[n][:, m * T:m * T + H]
                    b = pltpu.roll(ssm_w[n][:, m * T + H:(m + 1) * T], 1, 1)
                    st.extend([pltpu.bitcast(jnp.where(ev, a, b), BF16), pltpu.bitcast(jnp.where(ev, b, a), BF16)])
                return st[i]

            def epi(p):
                er, ei, or_, oi = p
                cur = [er, ei, or_, oi]
                if m:
                    pv = [zraw[C(4 * ((m - 1) % 2) + (q ^ 1)), :] for q in range(4)]
                    pm = lambda x, y, up: jnp.concatenate([x[:64] + y[:64], x[64:] - y[64:]] if up else
                                                          [x[:64] - y[:64], x[64:] + y[64:]], axis=0)
                    er, ei, or_, oi = [pm(cur[q], pv[q], q & 1) for q in range(4)]
                else:
                    er = er + taps[4, 0:1, C(n)]
                if m + 1 < NB:
                    for q in range(4):
                        zraw[C(4 * (m % 2) + q), :] = cur[q]
                for h, (cr, ci) in enumerate(((er + or_, ei + oi), (er - or_, ei - oi))):
                    B = h * 3 * H
                    kf[m, B:B + H, C(n)] = cr
                    kf[m, B + H:B + 2 * H, C(n)] = ci - cr
                    kf[m, B + 2 * H:B + 3 * H, C(n)] = ci + cr
            return Unit("K%d" % n, [(lambda i=i, r=r: (tf_v[r:r + H, C(i)], rhs(i))) for i in range(2) for r in (0, H)],
                        epi, H, 260, nt=True)
        return [unit(m) for m in range(NB)]

    def kv(s, sl):
        def mk(t, w):
            def fn(a):
                ld = lambda o, n: k_n[s][t, pl.ds(8 + w + o, n), :]
                c0 = jnp.concatenate([_tie(ld(0, 8), a), ld(8, 8)], axis=0).reshape(2, 8, 128)
                c1, c2 = ld(-1, 16).reshape(2, 8, 128), ld(-2, 16).reshape(2, 8, 128)
                s0, s1, s2, s3 = (taps[i, :, C(t)] for i in range(4))
                ke, ko, ke1, ko1, ko2 = _lo(c0), _hi(c0), _lo(c1), _hi(c1), _hi(c2)
                wv = v_n[s][t, w:w + 16, :].reshape(2, 8, 128)
                kve = ((s0 * ke + s1 * ko1) + (s2 * ke1 + s3 * ko2)) * _lo(wv)
                kvo = ((s0 * ko + s1 * ke) + (s2 * ko1 + s3 * ke1)) * _hi(wv)
                kv_v[pl.ds(sl * T + w, 16), C(t)] = kve.reshape(16, 128).astype(BF16)
                kv_v[pl.ds(sl * T + H + w, 16), C(t)] = kvo.reshape(16, 128).astype(BF16)
            return fn
        return [[mk(t, w) for w in range(0, H, 16)] for t in range(NT)]

    def mmU(name, sl, us):
        def unit(n):
            def epi(p):
                er, ei, or_, oi = p
                for h, (cr, ci) in enumerate(((er + or_, ei + oi), (er - or_, ei - oi))):
                    B = h * 3 * H
                    uf[us, B:B + H, C(n)] = cr + ci
                    uf[us, B + H:B + 2 * H, C(n)] = cr
                    uf[us, B + 2 * H:B + 3 * H, C(n)] = ci
            return Unit(name(n), [(lambda i=i, r=r: (tf_v[r:r + H, C(2 + i)], kv_v[pl.ds(sl * T + i * H, H), C(n)]))
                                  for i in range(2) for r in (0, H)], epi, H, 96 + 96 * KS)
        return [unit(n) for n in range(NT)]

    def cmul(m0, u0, n, h, row, L, a):
        t = []
        for i in range(3):
            Rw = slice((3 * h + i) * H + row, (3 * h + i) * H + row + 8)
            kk = kf[m0:m0 + n, Rw, L]
            if i == 0 and a is not None:
                k0 = _tie(kk[0], a)[None]
                kk = k0 if n == 1 else jnp.concatenate([k0, kk[1:]], axis=0)
            t.append(jnp.sum(kk * uf[u0:u0 + n, Rw, L], axis=0))
        return t[0] - t[2], t[0] + t[1]

    def AR(h, q, row):
        return slice((2 * h + q) * H + row, (2 * h + q) * H + row + 8)

    def mac(n, u0, sl, part=False):
        def mk(t, rc):
            st, fin = [], []

            def piece(i):
                def fn(a):
                    h, row = i & 1, rc + (i >> 1) * 8
                    zr, zi = cmul(0, u0, n, h, row, C(t), a)
                    if part:
                        zr, zi = zr + acc[0, AR(h, 0, row), C(t)], zi + acc[0, AR(h, 1, row), C(t)]
                    st.append((zr, zi))
                    if h:
                        (pr, pi), (mr, mi) = st[-2:]
                        fin.append([pr + mr, pi + mi, pr - mr, pi - mi])
                    if i == 3:
                        for q in range(4):
                            zz_v[pl.ds(sl * 2 * T + q * H + rc, 16), C(t)] = jnp.concatenate(
                                [fin[0][q], fin[1][q]], axis=0).astype(BF16)
                return fn
            if not part:
                return [piece(i) for i in range(4)]
            both = lambda f, g: (lambda a: (f(a), g(None)))
            return [both(piece(0), piece(1)), both(piece(2), piece(3))]
        return [[fn for rc in range(0, H, 16) for fn in mk(t, rc)] for t in range(NT)]

    def pos():
        return [(t, h, row) for t in range(NT) for row in range(0, H, 8) for h in range(2)]

    def ahead(i):
        def mk(t, h, row):
            def fn(a):
                zr, zi = cmul(i + 1, 0, NC, h, row, C(t), a)
                acc[i, AR(h, 0, row), C(t)] = zr
                acc[i, AR(h, 1, row), C(t)] = zi
            return fn
        return [mk(*p) for p in pos()]

    def spread():
        n = NB - NC - 1

        def mk(t, h, row):
            def fn(a):
                p = []
                for i in range(3):
                    Rw = slice((3 * h + i) * H + row, (3 * h + i) * H + row + 8)
                    u = uf[0, Rw, C(t)]
                    p.append(kf[1:1 + n, Rw, C(t)] * (_tie(u, a) if i == 0 else u)[None])
                acc[0:n, AR(h, 0, row), C(t)] = acc[1:1 + n, AR(h, 0, row), C(t)] + (p[0] - p[2])
                acc[0:n, AR(h, 1, row), C(t)] = acc[1:1 + n, AR(h, 1, row), C(t)] + (p[0] + p[1])
            return fn
        return [mk(*p) for p in pos()]

    def mmI(name, sl, ys):
        def unit(n):
            def epi(p):
                ce, se, co, so = p
                sub = lax.broadcasted_iota(I32, (8, 128), 0)
                b0 = ys * (T + 8) + 8
                y_v[n, b0 + H - 1:b0 + H, :] = (ce[64:72] - se[0:8])[0:1]
                se = jnp.concatenate([jnp.where(sub == 0, 0.0, se[0:8]), se[8:]], axis=0)
                for d, cc, ss in ((0, ce[0:64], se), (1, co, so)):
                    y_v[n, pl.ds(b0 + H + d, 64, stride=2), :] = cc + ss
                    y_v[n, pl.ds(b0 + d - 1, 64, stride=2), :] = cc - ss
            return Unit(name(n), [(lambda i=i: (tg_v[0:(GR if i == 0 else 64), C(i)], zz_v[pl.ds(sl * 2 * T + i * H, H), C(n)]))
                                  for i in range(4)], epi, 64, 36 + 33 * KS)
        return [unit(n) for n in range(NT)]

    def mod(name, a, b):
        def unit(n):
            def epi(p):
                v = [_sum(p[i * NT:(i + 1) * NT])[0:8] for i in range(b - a)]
                if a == 0:
                    mod_v[0, :, C(n)] = v[0] * v[2]
                    mod_v[1, :, C(n)] = (v[1] + 1.0) * v[2]
                elif a == 3:
                    mod_v[3, :, C(n)] = v[0] * (1.0 / G_POST)
                    mod_v[4, :, C(n)] = (v[1] + 1.0) * (1.0 / G_POST)
                else:
                    mod_v[2, :, C(n)] = v[0] * G_POST
            return Unit(name, [(lambda i=i, k=k: (silu_c[:, C(k)], wm_v[a][C(k), pl.ds(i * D + n * 128, 128)]))
                               for i in range(b - a) for k in range(NT)], epi, 16, 10, full=False, acc=b - a == 1)
        return [unit(n) for n in range(NT)]

    HS = (slice(0, 128), slice(128, 256))
    QS = tuple(slice(r, r + 64) for r in range(0, T, 64))

    def tasks(f, due=None, tie=True, n=RG):
        def mk(R):
            def fn(a):
                x = f(R, a if tie else None)
                return Due(x, due) if due else None
            return fn
        return [mk(slice(r, r + n)) for r in range(0, T, n)]

    def load_y(sl, R):
        b0, back = sl * (T + 8) + 8, 7 - lax.broadcasted_iota(I32, (8, 128), 0)

        def ld(t, r):
            if r >= H:
                return y_v[t, b0 + r:b0 + r + 8, :]
            return jnp.take_along_axis(y_v[t, b0 + H - 8 - r:b0 + H - r, :], back, axis=0)
        return jnp.stack([jnp.concatenate([ld(t, r) for t in range(NT)], axis=1) for r in (R.start, R.start + 8)])

    def put(nn, ss, R, x):
        nn[R, :] = x.astype(BF16)
        tok = x
        if ss is not None:
            S2 = pl.ds(R.start // 32 * 16, 16)
            if R.stop % 32:
                top_v[S2, 0:2 * T] = x[:, 0:2 * T]
            else:
                if R.start % 32:
                    x = jnp.concatenate([top_v[S2, 0:2 * T], x[:, 0:2 * T]], axis=0)
                ss[S2, 0:5 * T] = jnp.concatenate(_lhs_sums(x[:, 0:T], x[:, T:2 * T]), axis=1).astype(BF16)
        return tok

    wide = lambda v: jnp.concatenate([v] * NT, axis=1)

    def mean(i, R, x):
        st_v[R, C(i)] = jnp.broadcast_to(jnp.sum(x, axis=-1, keepdims=True) * (1.0 / D), (x.shape[0], 128))

    def centred(src, i, R, a):
        return src[R, :] - wide(_tie(st_v[R, C(i)], a))

    def scale(src, i, g):
        def f(R, a):
            st_v[R, C(i + 1)] = jnp.broadcast_to(_rstd(centred(src, i, R, a), g), (RG, 128))
        return f

    def normed(src, i, R, a):
        return centred(src, i, R, a) * wide(st_v[R, C(i + 1)])

    def front(sl, xs, early=False, ss=None):
        xx, hh, nn = view(x_v, xs), view(hb_v, xs), view(n1_v, sl)

        def fa(R, a):
            q = [q_n[sl][t, R.start // 2:R.stop // 2, :] for t in range(NT)]
            q = jnp.concatenate([_tie(q[0], a)] + q[1:], axis=1)
            q = pltpu.bitcast(q, BF16).astype(F32).reshape(2, 8, D)
            x = (q + (_ln(q) * mod_v[1] + mod_v[0]) * load_y(sl, R)).reshape(RG, D)
            xx[R, :] = x
            if early:
                hh[R, :] = _ln(x)

        def fb(R, a):
            hh[R, :] = (_ln(_tie(xx[R, :], a).reshape(2, 8, D)) * mod_v[4] + mod_v[3]).reshape(RG, D)

        def fc(R, a):
            hb = _tie(hh[R, :], a)
            if early:
                hb = (hb.reshape(2, 8, D) * mod_v[4] + mod_v[3]).reshape(RG, D)
                hh[R, :] = hb
            nn[R, :] = _ln(hb, True).astype(BF16)
        if early:
            return tasks(fa), tasks(fc)
        if ss is None:
            return tasks(fa) + tasks(fb) + tasks(fc)
        qf = view(x_v, 2)

        def s1(R, a):
            q = [q_n[sl][t, R.start // 2:R.stop // 2, :] for t in range(NT)]
            q = pltpu.bitcast(jnp.concatenate([_tie(v, a) for v in q], axis=1), BF16).astype(F32)
            qf[R, :] = q
            mean(0, R, q)

        def s3(R, a):
            h = normed(qf, 0, R, a).reshape(2, 8, D) * mod_v[1] + mod_v[0]
            x = qf[R, :] + (h * load_y(sl, R)).reshape(RG, D)
            xx[R, :] = x
            mean(2, R, x)

        def s5(R, a):
            hb = (normed(xx, 2, R, a).reshape(2, 8, D) * mod_v[4] + mod_v[3]).reshape(RG, D)
            hh[R, :] = hb
            mean(4, R, hb)
        s7 = [f for g in tasks(lambda R, a: put(nn, ss, R, normed(hh, 4, R, a)), n=32) for f in (g, lambda a: None)]
        st = [tasks(s3), tasks(scale(xx, 2, False)), tasks(s5), tasks(scale(hh, 4, True)), s7]
        p = [tasks(s1), tasks(scale(qf, 0, False))]
        sk = 4.091

        def wave(ls):
            body = sorted((i * sk + g, i, g) for i in range(len(ls) - 1) for g in range(8))
            return [ls[i][g] for _, i, g in body] + ls[-1]
        qb = []
        done = lambda a: qb[0](a)
        full = wave([x[8:] for x in p + st])
        k = full.index(p[0][15]) + 1
        return wave([x[:8] for x in st]), full[:k] + [done] + full[k:], cat(x[:8] for x in p), qb

    def shift(hs, sl, pieces=((0, 64), (64, 64), (128, 64), (192, 64)), ss=None):
        gg = view(g_v, sl)

        def one_tile(t, r, n, a):
            lane = lax.broadcasted_iota(I32, (n, 128), 1)
            ld = lambda d: h1_v[t, pl.ds(hs * T + 8 + r + d, n), :]
            if t == 0:
                g = ld(-1)
            elif t == 1:
                g = jnp.where(lane < 32, ld(-1), ld(1))
            elif t == 2:
                g = jnp.where(lane < 64, ld(1), ld(-2))
            elif t == 3:
                g = jnp.where(lane < 96, ld(-2), ld(2))
            else:
                g = ld(2)
            if a is not None:
                g = jnp.concatenate([_tie(g[i:i + 8], a) if i % 16 == 0 else g[i:i + 8]
                                     for i in range(0, n, 8)], axis=0)
            gg[r:r + n, C(t)] = g.astype(BF16)
            return g

        def mk(ts, r, n):
            def fn(a):
                g = [one_tile(t, r, n, a) for t in ts]
                if len(ts) == 2:
                    for i, x in enumerate(_lhs_sums(*g)):
                        ss[r // 2:(r + n) // 2, C(2 * i + ts[0])] = x.astype(BF16)
            return fn
        sets = [(t,) for t in range(NT)] if ss is None else [(0, 2), (1, 3), (4,)]
        return [mk(ts, r, n) for ts in sets for r, n in pieces]

    def shift_early():
        def keep(a):
            h1_v[:, 2 * T - 32:2 * T + 8, :] = h1_v[:, 3 * T - 32:3 * T + 8, :]
        return shift(2, 0, [(r, 32) for r in range(0, T - 32, 32)], gs) + [keep]

    def ln2(xs, sl, fast=True):
        xx, nn, ss = view(x1_v, xs), view(n2_v, sl), view(n2s, sl, H) if fast else None
        f = lambda R, a: put(nn, ss, R, _ln(_tie(xx[R, :], a), True))
        ts = tasks(f, 900) if sl else tasks(f, DL, False)
        return ts[0::2] + ts[1::2] if fast else tasks(f)

    def ln2_late():
        xx, nn, ss = view(x1_v, 0), view(n2_v, 0), view(n2s, 0, H)
        a_, b_ = tasks(lambda R, a: mean(6, R, _tie(xx[R, :], a))), tasks(scale(xx, 6, True))
        c_ = [f for g in tasks(lambda R, a: put(nn, ss, R, normed(xx, 6, R, a)), n=32)[:4] for f in (g, lambda a: None)]
        return a_[:8] + b_[:8] + c_

    def resid(xs, x1s, rotate=False):
        xx, x1 = view(x_v, xs), view(x1_v, x1s)
        tie = lambda v, a: v if a is None else pltpu.bitcast(pltpu.bitcast(v, U32) | wide(a), F32)

        def f(R, a):
            r_v[R, :] = xx[R, :] + tie(x1[R, :], a) * mod_v[2]

        def move(dst, src):
            def g(R, a):
                dst[R, :] = tie(src[R, :], a)
            return tasks(g, n=8)
        if not rotate:
            return tasks(f, n=8)
        return cat(zip(tasks(f, n=8), move(view(hb_v, 1), hb_v), move(xx, x_v)))

    KD, KF, ND = [(0, 2), (1, 3)], [(2 * i, 2 * i + 1) for i in range(7)], [(1, 2), (3, 4)]
    Wt = {1: (lambda k, n: w1_v[C(k), C(n)], lambda i, kp, j: w1s[C(kp), C(2 * i + j)], False, KD, [4]),
          2: (lambda k, n: w2_v[C(k), C(n)], lambda i, kp, j: w2s[C(kp), C(2 * i + j)], False, KD, [4]),
          0: (lambda k, n: w3_v[C(n), C(k)], None, True, KD, [4]),
          3: (lambda k, n: w3n[C(k), C(n)], lambda i, kp, j: w3s[C(kp), C(6 * i + j)], False, KD, [4]),
          4: (lambda k, n: w4_v[C(k), C(n)], lambda i, kp, j: w4s[C(kp), C(2 * i + j)], False, KF, [])}

    def sums_task(load, store, left):
        def fn(a):
            b = [[load(u, v) for v in range(2)] for u in range(2)]
            b[0][0], b[1][1] = _tie(b[0][0], a), _tie(b[1][1], a)
            (x11, x12), (x21, x22) = [[pltpu.bitcast(x, BF16).astype(F32) for x in row] for row in b]
            r = ((x11 + x22, x21 + x22, x11 + x12, x21 - x11, x12 - x22) if left else
                 (x11 + x22, x12 - x22, x21 - x11, x11 + x12, x21 + x22))
            for m, x in enumerate(r):
                store(m, x.astype(BF16))
        return fn

    def wsums(w_w, ws, rp, cp_):
        def mk(i, j, r):
            def store(m, x):
                ws[pl.ds(128 * i + r, 16), C(len(cp_) * m + j)] = x
            return sums_task(lambda u, v: w_w[pl.ds(64 * rp[i][u] + r // 2, 8), C(cp_[j][v])], store, False)
        return [mk(i, j, r) for j in range(len(cp_)) for i in range(len(rp)) for r in range(0, 128, 16)]

    def w3_turn():
        def mk(n, k):
            def fn(a):
                x = jnp.concatenate([_tie(w3_w[64 * n:64 * n + 8, C(k)], a), w3_w[64 * n + 8:64 * n + 64, C(k)]], axis=0)
                w3n[C(k), C(n)] = pltpu.bitcast(x, BF16).T
            return fn
        return [mk(n, k) for n in range(FT - 1) for k in range(NT)]

    def plain(name, w, lhs, n, R, epi, cost):
        tile, _, nt, kp, kl = Wt[w]
        ks = sorted([k for p in kp for k in p] + kl)
        rows_ = R.stop - R.start
        return Unit(name, [(lambda k=k: (lhs[R, C(k)], tile(k, n))) for k in ks], lambda p: epi(n, R, p[0]),
                    rows_, rows_ // 8 * (len(ks) - 1), nt=nt, acc=True, tail=rows_ // 8 * cost(n))

    def quad(name, w, lhs, sums, j, cols_, R, epi, cost):
        tile, wsum, nt, kp, kl = Wt[w] if isinstance(w, int) else w
        h, S2, c = len(kp), slice(R.start // 2, R.stop // 2), {}
        a_ = lambda i, k: _top(lhs(k) if callable(lhs) else lhs[R, C(k)], i)
        s_ = sums if callable(sums) else (lambda i, p: sums[S2, C(h * i + p)])
        prod = lambda fa_, fb_: [(lambda p=p: (fa_(p), fb_(p))) for p in range(h)]
        left = lambda i, n: [(lambda k=k: (a_(i, k), tile(k, n))) for k in kl]
        mk = lambda tiles, f, x=0: Unit(name, tiles, lambda p: f(p[0]), 64, 8 * len(tiles), nt=nt, acc=True, tail=x)

        def e1(m):
            u7.res, u6.res = [m], [m]

        def e4(m):
            c[11], c[21] = c[11] + m, m

        def e2(m):
            c[21], c[22] = c[21] + m, c[22] - m
            l21.res = [c[21]]

        def e5(m):
            c[12] = m
            epi(cols_[0], R, _zip(c[11] - m, c[21]))

        def e3(m):
            l12.res, c[22] = [c[12] + m], c[22] + m
            if not kl:
                l12.epi(l12.res)
        u1 = mk(prod(lambda p: s_(0, p), lambda p: wsum(0, p, j)), e1)
        u7 = mk(prod(lambda p: s_(4, p), lambda p: wsum(4, p, j)) + left(0, cols_[0]), lambda m: c.update({11: m}))
        u6 = mk(prod(lambda p: s_(3, p), lambda p: wsum(3, p, j)) + left(1, cols_[1]), lambda m: c.update({22: m}))
        u4 = mk(prod(lambda p: a_(1, kp[p][1]), lambda p: wsum(2, p, j)), e4)
        u2 = mk(prod(lambda p: s_(1, p), lambda p: tile(kp[p][0], cols_[0])), e2, 8)
        l21 = mk(left(1, cols_[0]), lambda m: c.update({21: m}))
        u5 = mk(prod(lambda p: s_(2, p), lambda p: tile(kp[p][1], cols_[1])), e5, 16 * cost(cols_[0]))
        u3 = mk(prod(lambda p: a_(0, kp[p][0]), lambda p: wsum(1, p, j)), e3, 8 if kl else 8 + 16 * cost(cols_[1]))
        l12 = mk(left(0, cols_[1]), lambda m: epi(cols_[1], R, _zip(m, c[22])), 16 * cost(cols_[1]))
        return [u1, u7, u6, u4, u2, l21, u5, u3, l12]

    LH, RH = [0, 4, 3, (1, 1), 1, 2, (0, 0)], [0, 4, 3, 2, (0, 0), (1, 1), 1]
    L2 = {3: (w3n_w, ws_w[2], w3t, KF[:6], n2t), 4: (w4_w, ws_w[3], w4t, ND, a_t)}

    def wsums2(w):
        w_w, s_w, ws2, cp_, _ = L2[w]
        kp, nj = Wt[w][3], len(cp_)

        def mk(o, p2, j2, r):
            def load(u, v):
                p, j, y = 2 * p2 + u, 2 * j2 + v, RH[o]
                if isinstance(y, int):
                    return s_w[pl.ds(64 * p + r // 2, 8), C(nj * y + j)]
                return w_w[pl.ds(64 * kp[p][y[0]] + r // 2, 8), C(cp_[j][y[1]])]

            def store(m, x):
                ws2[pl.ds(128 * p2 + r, 16), C((5 * o + m) * (nj // 2) + j2)] = x
            return sums_task(load, store, False)
        return [mk(o, p2, j2, r) for j2 in range(nj // 2) for o in range(7) for p2 in range(len(kp) // 2)
                for r in range(0, 128, 16)]

    def wsums4():
        form = [((0, 0), (1, 1), 1), ((0, 1), (1, 1), -1), ((1, 0), (0, 0), -1), ((0, 0), (0, 1), 1), ((1, 0), (1, 1), 1)]

        def mk(o, p2, r):
            def fn(a):
                def blk(p, j, uv, t):
                    x = w4_w[pl.ds(64 * KF[p][uv[0]] + r // 2, 8), C(ND[j][uv[1]])]
                    return pltpu.bitcast(_tie(x, t), BF16).astype(F32)
                y = {}
                for u in range(2):
                    for j in range(2):
                        p = 2 * p2 + u
                        if isinstance(RH[o], int):
                            f = form[RH[o]]
                            x1, x2 = blk(p, j, f[0], a), blk(p, j, f[1], None)
                            y[u, j] = x1 + x2 if f[2] > 0 else x1 - x2
                            w4s[pl.ds(128 * p + r, 16), C(2 * RH[o] + j)] = y[u, j].astype(BF16)
                        else:
                            y[u, j] = blk(p, j, RH[o], a if u == j else None)
                for m, f in enumerate(form):
                    x = y[f[0]] + y[f[1]] if f[2] > 0 else y[f[0]] - y[f[1]]
                    w4t[pl.ds(128 * p2 + r, 16), C(5 * o + m)] = x.astype(BF16)
            return fn
        last = wsums(w4_w, w4s, KF, ND)
        return (last[48:56] + last[104:112]
                + [mk(o, p2, r) for o in range(7) for p2 in range(3) for r in range(0, 128, 16)])

    def lsums2(w, lhs_w, sums_w, sl):
        kp, xs2 = Wt[w][3], L2[w][4]
        h2 = len(kp) // 2

        def mk(o, p2, g):
            def load(u, v):
                p, ch, x = 2 * p2 + v, 2 * g + u, LH[o]
                if isinstance(x, int):
                    return sums_w[pl.ds(64 * sl + 8 * ch, 8), C(len(kp) * x + p)]
                return lhs_w[pl.ds(H * sl + 16 * ch + 8 * x[0], 8), C(kp[p][x[1]])]

            def store(m, x):
                xs2[pl.ds(16 * g, 16), C((5 * o + m) * h2 + p2)] = x
            return sums_task(load, store, True)
        return [[mk(o, p2, g) for o in range(7) for g in range(4)] for p2 in range(h2)]

    def quad2(name, w, lhs, sums, j2, epi, cost):
        tile, wsum, nt, kp, kl = Wt[w]
        ws2, cp_, xs2 = L2[w][2:]
        h, h2, nj2, c, R = len(kp), len(kp) // 2, len(cp_) // 2, {}, slice(0, T)

        def done(j, v):
            val = _zip(c[j, 1, v], c[j, 2, v])
            if not kl:
                return epi(cp_[j][v], R, val)
            c[j, v] = val

        def upd(o, j, m):
            for i, v, sg in (((1, 0, 1), (2, 1, 1)), ((1, 0, 1),), ((2, 1, 1),), ((1, 0, 1), (2, 0, 1)),
                             ((2, 0, 1), (2, 1, -1)), ((1, 0, -1), (1, 1, 1)), ((1, 1, 1), (2, 1, 1)))[o]:
                k = (j, i, v)
                c[k] = m if k not in c else (c[k] + m if sg > 0 else c[k] - m)
            if o >= 5:
                done(j, o - 5)

        def inner(o):
            x, y = LH[o], RH[o]
            xo = ((lambda p: sums[:, C(h * x + p)]) if isinstance(x, int)
                  else (lambda p: _top(lhs[:, C(kp[p][x[1]])], x[0])))
            yo = ((lambda p, j: wsum(y, p, j)) if isinstance(y, int)
                  else (lambda p, j: tile(kp[p][y[0]], cp_[j][y[1]])))
            w_ = (yo, lambda m, p2, _: ws2[C(p2), C((5 * o + m) * nj2 + j2)], nt,
                  [(2 * i, 2 * i + 1) for i in range(h2)], list(range(2 * h2, h)))
            return quad(name, w_, xo, lambda m, p2: xs2[:, C((5 * o + m) * h2 + p2)], 0, (2 * j2, 2 * j2 + 1),
                        HS[0], lambda j, _, m: upd(o, j, m), lambda j: 1.5 + KS + (2 * cost(0) if o >= 5 and not kl else 0))

        def rest(j, v, Q):
            return [Unit(name, [lambda: (lhs[Q, C(k)], tile(k, cp_[j][v]))],
                         lambda p: epi(cp_[j][v], Q, p[0] + c[j, v][Q]), 64, 8 * (cost(cp_[j][v]) + 1)) for k in kl]
        return cat(inner(o) for o in range(7)), [u for Q in QS for j in (2 * j2, 2 * j2 + 1) for v in range(2)
                                                 for u in rest(j, v, Q)]

    def mm(name, w, lhs, sums, epi, cost):
        if sums is None:
            return [[plain(name, w, lhs, n, R, epi, cost) for R in HS] for n in range(NT)]
        return [[plain(name, w, lhs, 0, R, epi, cost) for R in QS]] + [
            [u for R in HS for u in quad(name, w, lhs, sums, j, ND[j], R, epi, cost)] for j in range(2)]

    def mm1(name, hs, sl, fast=False):
        def epi(n, R, p):
            h1_v[n, pl.ds(hs * T + 8 + R.start, R.stop - R.start), :] = _gelu2(p)
        return cat(mm(name, 1, view(n1_v, sl), n1s if fast else None, epi, lambda n: 5 + KS))

    def mm2(name, sl, xs, x1s, fast=False):
        def epi(n, R, p):
            view(x1_v, x1s)[R, C(n)] = view(hb_v, xs)[R, C(n)] + p
        return cat(mm(name, 2, view(g_v, sl), gs if fast else None, epi, lambda n: 1 + KS))

    def mm3(name, sl, fast=True, host=None):
        nn, aa, ss, keep, tail = view(n2_v, sl), view(a_v, sl), view(a_s, sl, H), {}, []

        def epi(n, R, p):
            g = _gelu2(p)
            aa[R, C(n)] = g.astype(BF16)
            if not fast:
                return
            if n % 2 == 0 and n < 12:
                keep[n] = g
                return
            pair = (keep.pop(n - 1), g) if n % 2 else (g, tail[R.start // 128][R.start % 128:R.start % 128 + 64])
            for i, x in enumerate(_lhs_sums(*pair)):
                ss[R.start // 2:R.stop // 2, C(7 * i + n // 2)] = x.astype(BF16)

        c3 = lambda n: 5.5 + 0.5 * KS + (3.75 + 1.25 * KS if fast and (n % 2 or n == 12) else 0)

        def rem(R):
            def f(p):
                tail.append(jnp.concatenate([_gelu2(p[0]), jnp.zeros((64, 128), F32)], axis=0).T)
                aa[R, C(13)] = tail[-1].astype(BF16)
            return Unit(name, [(lambda k=k: (w3_v[13 * 128:F, C(k)], nn[R, C(k)])) for k in range(NT)], f, 64, 84,
                        nt=True, acc=True)
        odd = [rem(R) for R in HS] + [plain(name, 3 if fast else 0, nn, 12, R, epi, c3) for R in QS]
        if not fast:
            return odd + [plain(name, 0, nn, n, R, epi, c3) for p in KF[:6] for R in HS for n in p]
        qd = [quad2(name + "_%d" % j, 3, nn, view(n2s, sl, H), j, epi, c3) for j in range(3)]
        mid = qd[0][0] + _weave(qd[1][0], qd[0][1]) + _weave(qd[2][0], qd[1][1])
        if host is None:
            return odd[:2] + mid + _weave(odd[2:], qd[2][1])
        for u in (odd[0], odd[2], odd[3]):
            u.name = name + "h"
        return [odd[0], odd[2], odd[3], odd[1]] + mid, _weave(odd[4:] + host, qd[2][1])

    def cp_out(j, osl, L, sm, R=slice(0, T)):
        return cp(o_v.at[pl.ds(osl * T + R.start, R.stop - R.start), L],
                  o_hbm.at[pl.ds(base(j, T) + R.start, R.stop - R.start), L], sem_o.at[sm])

    out_a = lambda j: cp_out(j, 0, slice(128, D), 0)
    out_b = lambda j: cp_out(j, 0, C(0), 1)
    last = []

    def mm4(name, j, sl, osl=0, xs=None, x1s=None, fast=True):
        oo = view(o_v, osl)

        def epi(n, R, p):
            if xs is None:
                oo[R, C(n)] = (r_v[R, C(n)] + mod_v[2, 0:1, C(n)] * p).astype(BF16)
            else:
                oo[R, C(n)] = (view(x_v, xs)[R, C(n)] + mod_v[2, 0:1, C(n)]
                               * (view(x1_v, x1s)[R, C(n)] + p)).astype(BF16)
            if osl == 2:
                last.append(cp_out(j, osl, C(n), 2, R))
                last[-1].start()
            elif R.stop == T and osl and n == NT - 1:
                last.append(cp_out(j, osl, slice(128 if osl == 3 else 0, D), 2))
                last[-1].start()
            elif R.stop == T and osl == 0 and n in (0, NT - 1):
                (out_a if n else out_b)(j).start()
        c4 = lambda n: (3 if xs is None else 4) + KS
        if fast:
            return ([plain(name, 4, view(a_v, sl), 0, R, epi, c4) for R in QS],
                    quad2(name + "q", 4, view(a_v, sl), view(a_s, sl, H), 0, epi, c4)[0])
        return mm(name, 4, view(a_v, sl), None, epi, c4)

    def split(us):
        n = 4 // len(us)
        m, mks, st = us[0].rows // n, [u.tiles.pop(0) for u in us], {}

        def piece(i, k):
            if i not in st:
                st[i] = mks[i]()
            return st[i][0][m * k:m * (k + 1)], st[i][1]

        def epi(p):
            for i, u in enumerate(us):
                u.res = [jnp.concatenate(p[n * i:n * (i + 1)], axis=0)]
        return _flat([Unit(us[0].name, [(lambda i=i, k=k: piece(i, k)) for i in range(len(us)) for k in range(n)],
                           epi, m, 0, nt=us[0].nt)])

    W = lambda nm: [("wait", nm)]
    run = lambda fns: [("run", "run", lambda: [fn(None) for fn in fns])]
    one = lambda us: [_flat([u]) for u in us]
    nm = lambda x: (lambda n: x)

    seq, grp = [], []
    for s in range(NC):
        seq += W("c%d" % s) + _flat(mmK(s) + mmU(nm("U%d" % s), s % 2, NC - 1 - s))
        grp.append(Group("kv%d" % s, cat(kv(s, s % 2)), 50, ["c%d" % s], ["U%d" % s], 100))
    inv = [mmI(lambda n: "I%d" % n, s, s) for s in range(NC)]
    seq += W("c3") + _flat(mmK(3) + mmK(4) + [inv[s][t] for t in range(NT) for s in range(NC)])
    macs = [mac(s + 1, NC - 1 - s, s) for s in range(NC)]
    grp.append(Group("mac00", macs[0][0], 12, ["c1"], ["c2"], 0))
    grp.append(Group("mac01", macs[1][0] + macs[0][1] + macs[1][1], 16, ["c2"], ["c3"], 0))
    for t in range(NT):
        grp.append(Group("mac%d" % t, cat(macs[s][t] for s in range(2 if t < 2 else 0, NC)), 24 if t < 2 else 18,
                         ["c3", "K%d" % t], ["I%d" % t], 100, 150))
    start = lambda cs: [("run", "run", lambda: [c.start() for c in cs])]
    f0, f1 = front(0, 2, True), front(1, 1, True)
    seq += run(ahead(0))
    seq += W("wma") + _flat(mod("moda", 0, 3)) + run(f0[0] + f1[0] + ahead(1))
    seq += W("wmb") + start(next_kv(NC) + next_q(NC)) + _flat(mod("modb", 3, 5)) + run(f0[1])
    w1 = _flat(mm1("w1_0", 0, 0) + mm1("w1_1", 1, 1))
    seq += W("w1") + w1[:72] + W("w2") + w1[72:] + run(shift(0, 0))
    seq += _flat(mm2("w2_0", 0, 2, 1) + mm1("w1_2", 2, 2)) + run(shift(1, 1)) + _flat(mm2("w2_1", 1, 1, 0))
    grp.append(Group("f1", f1[1], 80, ["w1"], ["w1_1"], 450))
    grp.append(Group("f2", front(2, 0), 80, ["w2"], ["w1_2"], 450))
    grp.append(Group("ln2_0", ln2(1, 0, False), 60, ["w2_0"], ["w3"], 450))
    grp.append(Group("ahead", cat(ahead(i) for i in range(2, NB - NC)), 19 + 2 * KS, ["w1"], ["end"], 100))
    grp.append(Group("ws1", wsums(w1_w, w1s, KD, ND), 26 + 5 * KS, ["w1"], ["end"], 100))
    grp.append(Group("ws2", wsums(w2_w, w2s, KD, ND), 26 + 5 * KS, ["w2"], ["end"], 100))
    grp.append(Group("ws3", w3_turn() + wsums(w3n_w, w3s, KD, KF[:6]) + wsums2(3), 22 + 5.5 * KS, ["w3"], ["end"], 100))
    grp.append(Group("ws4", wsums4(), 40 + 8 * KS, ["w4"], ["end"], 60))
    _wait(seq, "w3", back=1)
    w3 = mm3("w3_0", 0, False)
    _mix(seq, _flat(w3[6:]), [split(w3[4:6]) + _flat(w3[:6])], 0.1)
    mc = mod("modc", 5, 6)
    mc = _flat(mc[1:] + mc[:1])
    _wait(seq, "w4", mc[:5] + [("sync", "run", lambda: None)])
    w4 = cat(mm4("w4_0", 0, 0, 3, 2, 1, False)[1:])
    qs = [split([w4[-1 - i]]) for i in range(_phase(seq))]
    _mix(seq, _flat(w4), [mc[i:i + 4] for i in range(5, 25, 4)] + qs, 0.01, 0.4)
    assert _phase(seq) == 0
    grp.append(Group("resid", resid(2, 1), 16 + 5 * KS, ["modc"], ["end"], 100))
    grp.append(Group("ln2a", ln2_late(), 40, ["w3_0"], ["end"], 100))
    _emit(seq, grp, zero, wait)

    def step(s, carry):
        for c in next_kv(s) + next_q(s):
            c.wait()
        nxt = jnp.minimum(s + 1, NB - 1)
        seq, grp = [], []
        us, it = one(mmU(lambda n: "U%d" % n, 0, 0)), one(mmI(lambda n: "I%d" % n, 0, 0))
        w4, w4c = mm4("w4", s - 2, 0)[1], mm4("w4c", s - 3, 0)[0]
        w2 = mm2("w2", 0, 1, 0, True)
        w2 = w2[0:3] + w2[4:13] + w2[22:31] + w2[3:4] + w2[13:22] + w2[31:]
        for u in w2[:21]:
            u.name = "w2a"
        w2[0].name = "w2f"
        w3, w3e = mm3("w3", 0, host=w2[:4])
        _mix(seq, _flat(w4c + w3),
             [us[0], us[1], us[2], it[0] + us[3], it[1] + us[4], it[2], it[3], it[4]],
             0.159, 0.7)
        w1a, w1b = mm1("w1a", 2, 0, True), mm1("w1b", 2, 0, True)
        w1a, w1b = _flat(w1a[0:2] + w1a[4:13] + w1a[22:31]), _flat(w1b[2:4] + w1b[13:22] + w1b[31:])
        kw = 9 * 4
        w4[kw - 16].name = "w4m"
        seq += _flat(w3e + w2[4:21] + w4[:kw]) + w1a + run(shift(1, 0, ((T - 32, 32),), gs))
        seq += _flat(w4[kw:] + w2[21:]) + w1b
        assert _phase(seq) == 0
        kvs, macs = kv(0, 0), mac(1, 0, 0, part=True)
        for t in range(NT):
            grp.append(Group("kv%d" % t, kvs[t], 50 + 2 * KS, ["start"], ["U%d" % t], 260))
            grp.append(Group("mac%d" % t, macs[t], 24 + 2 * KS, ["U%d" % t], ["I%d" % t], 350, 150))
        iall = ["I%d" % t for t in range(NT)]
        ln = ln2(0, 0)
        grp.append(Group("ln2a", ln2_late(), 40, ["w2a", "w2"], ["end"], 100))
        xn = lsums2(3, n2_w, as_w[2], 0)[0]
        grp.append(Group("ln2b", ln[4:8] + ln[12:16], 78 + 20 * KS, ["start"], ["w3h"], 450))
        grp.append(Group("xna", [f for i, f in enumerate(xn) if i % 4 < 2], 26 + 5 * KS, ["start"], ["w3_0"], 150))
        grp.append(Group("xnb", [f for i, f in enumerate(xn) if i % 4 >= 2], 26 + 5 * KS, ["w4c"], ["w3_0"], 150, 0))
        grp.append(Group("resid", resid(1, 0, True), 9.5 + 5 * KS, ["w4c"], ["w2f"], 100))
        for p, ts in enumerate(lsums2(4, a_w, as_w[3], 0)):
            grp.append(Group("xa%d" % p, ts, 26 + 5 * KS, ["w3_%d" % p], ["w4q"], 150, 100))
        fr = front(0, 0, ss=n1s)
        grp.append(Group("fronta", fr[0], 50 + 8 * KS, ["w2f"], ["w1a"], 240, 0))
        grp.append(Group("frontb", fr[1], 46 + 7 * KS, ["w4m"], ["w1b"], 240, 80))
        def refill(buf, cs):
            def fn(a):
                for t in range(NT):
                    buf[t, 0:8, :] = zero if a is None else a
                for c in cs:
                    c.start()
            return fn
        fr[3].append(refill(q_n[0], next_q(nxt)))
        nk = next_kv(nxt)
        grp.append(Group("refill", [refill(k_n[0], nk[:NT]), refill(v_n[0], nk[NT:])], 10, ["U4"], ["w2f"], 0, 0))
        grp.append(Group("fq", fr[2], 33 + 7 * KS, ["w4c"], ["w2f"], 100))
        grp.append(Group("spread", spread(), 30 + 8 * KS, iall, ["end"], 60))
        grp.append(Group("shift", shift_early(), 22 + 7 * KS, ["start"], ["w2f"], 200))
        _emit(seq, grp, zero, wait)
        out_b(s - 3).wait()
        out_a(s - 2).wait()
        return carry

    lax.fori_loop(NC, NB, step, 0)

    seq, grp = [], []
    w47 = mm4("w4_7", NB - 1, 1, 2, 0, 1)
    seq += _flat(mm4("w4_5", NB - 3, 0)[0] + mm2("w2_7", 0, 0, 1, True) + mm3("w3_6", 0)
                 + cat(mm4("w4_6", NB - 2, 0, 1, 1, 0)) + mm3("w3_7", 1) + w47[0][:3] + w47[1] + w47[0][3:])
    grp.append(Group("shift7", shift(2, 0, [(r, 32) for r in range(0, T, 32)], gs), 24, ["start"], ["w2_7"], 200))
    ln = ln2(0, 0)
    grp.append(Group("ln2_6", ln[4:8] + ln[12:16], 75, ["start"], ["w3_6"], 1200))
    grp.append(Group("xn6", cat(lsums2(3, n2_w, as_w[2], 0)), 26 + 5 * KS, ["w4_5"], ["w3_6_0"], 200, 800))
    grp.append(Group("ln2_7", ln2(1, 1), 75, ["w4_6"], ["w3_7"], 1500))
    grp.append(Group("xn7", cat(lsums2(3, n2_w, as_w[2], 1)), 26 + 5 * KS, ["w4_6"], ["w3_7_0"], 200, 2100))
    for j in (6, 7):
        for p, ts in enumerate(lsums2(4, a_w, as_w[3], j - 6)):
            grp.append(Group("xa%d_%d" % (j, p), ts, 26 + 5 * KS, ["w3_%d_%d" % (j, p)], ["w4_%dq" % j], 200, 150))
    _emit(seq, grp, zero, wait)
    for c in next_kv(NB - 1) + next_q(NB - 1) + [out_b(NB - 3)] + last:
        c.wait()


@jax.jit
def pallas_adaLN_cond__ssm_conv_h3__mixer_s_mlp__prompt_kernel(
        A_q, A_k, A_v, A_shift_k, A_ssm_k, A_ssm_D, B_x, B_w1, B_w2, B_w3, B_w4, c, w_mod):
    any_ = pl.BlockSpec(memory_space=pl.ANY)
    V = pltpu.VMEM
    out = pl.pallas_call(
        kernel,
        in_specs=[any_] * 12,
        out_specs=any_,
        out_shape=jax.ShapeDtypeStruct((S, D), BF16),
        scratch_shapes=[
            [V((NT, H + 8, 128), U32)] * NC, [V((NT, H + 8, 128), U32)] * NC, [V((NT, H + 8, 128), U32)] * NC,
            [V((64, S), U32)] * NT,
            V((D // 2, D), U32), V((D // 2, D), U32), V((F // 2, D), U32), V((FT * 64, D), U32),
            [V((D // 2, 3 * D), U32), V((D // 2, 2 * D), U32), V((D // 2, D), U32)], V((4 * T, D), BF16),
            V((4, D), BF16), V((D,), BF16), V((1, D), BF16), V((8, 128), I32), pltpu.SMEM((8, 128), I32),
            V((5, 8, D), F32), V((6, 8, D), F32), V((T // 2, 4 * H), U32), V((GR // 2, 2 * T), U32),
            V((NB, 3 * T + 8, D), F32), V((NC, 3 * T + 8, D), F32), V((NB - NC, 2 * T + 8, D), F32), V((4 * T, 128), F32),
            V((T, D), U32), V((NC * T, D), U32), V((NT, NC * (T + 8) + 16, 128), F32),
            V((3 * T, D), F32), V((3 * T, D), F32), V((2 * T, D), F32), V((T, D), F32),
            V((3 * T // 2, D), U32), V((T, D), U32), V((T, D), U32), V((NT, NC * T + 24, 128), F32),
            V((T, (FT + 1) * 128), U32),
            [V((128, 11 * 128), U32)] * 2 + [V((128, 31 * 128), U32), V((448, 11 * 128), U32)],
            [V((64, 11 * 128), U32)] * 2 + [V((128, 11 * 128), U32), V((128, 35 * 128), U32)],
            V((D // 2, 13 * 128), U32), V((H, D), F32), V((T, 9 * 128), F32),
            [V((64, 105 * 128), U32), V((192, 35 * 128), U32), V((32, 35 * 128), U32), V((32, 105 * 128), U32)],
            pltpu.SemaphoreType.DMA((11,)), pltpu.SemaphoreType.DMA((1,)), pltpu.SemaphoreType.DMA((3,)),
        ],
        compiler_params=pltpu.CompilerParams(vmem_limit_bytes=110 << 20, disable_semaphore_checks=True,
                                             disable_bounds_checks=True),
        name="fused",
    )(A_q[0], A_k[0], A_v[0], A_shift_k.T, A_ssm_k, A_ssm_D, B_w1, B_w2, B_w3.T, B_w4, c, w_mod)
    return out[None]
```

```python
import heapq
import numpy as np
import jax
import jax.numpy as jnp
from jax import lax
from jax.experimental import pallas as pl
from jax.experimental.pallas import tpu as pltpu

S, D, F = 2048, 640, 1728
T = 256
H = T // 2
NB = S // T
NT = D // 128
FT = (F + 127) // 128
EPS = 1e-5
F32, BF16, U32, I32 = jnp.float32, jnp.bfloat16, jnp.uint32, jnp.int32
G_C1 = 0.044715 * float(np.sqrt(2.0 / np.pi))
G_C2 = float(np.sqrt(2.0 / np.pi))
G_A = G_C1 ** (1.0 / 3.0)
G_B = G_C2 / G_A
G_POST = 0.5 / G_A
RG = 16
GR = 80
NC = 3
DL = 450
KS = 1.9
SLOT = 32


def _dft(shape, f_axis, tau, scale=1.0):
    r = lax.broadcasted_iota(I32, shape, f_axis)
    l = lax.broadcasted_iota(I32, shape, 1 - f_axis)
    f = r & 127
    odd = ((f & 63) << 2) | ((f >> 6) << 1) | 1
    p = odd * tau(l) + ((r >> 7) << 8)
    a = ((p + 512) & 1023) - 512
    u = (256 - jnp.abs(a)).astype(F32) * (np.pi / 512.0)
    u2 = u * u
    c = [scale, -scale / 6.0, scale / 120.0, -scale / 5040.0, scale / 362880.0, -scale / 39916800.0]
    poly = c[5]
    for ci in c[4::-1]:
        poly = poly * u2 + ci
    return (u * poly).astype(BF16)


def _rstd(xc, mlp):
    s2, eps = (1.0 / (G_A * G_A), EPS / (G_POST * G_POST)) if mlp else (1.0, EPS)
    v = jnp.sum(xc * xc, axis=-1, keepdims=True) * (s2 / D) + eps * s2
    return jnp.exp2(jnp.log(v) * float(-0.5 / np.log(2.0)))


def _ln(x, mlp=False):
    xc = x - jnp.sum(x, axis=-1, keepdims=True) * (1.0 / D)
    return xc * _rstd(xc, mlp)


def _gelu2(x):
    u = x * (x * x + G_B)
    return x * (1.0 + jnp.tanh(u))


def _lo(w):
    return pltpu.bitcast(w << 16, F32)


def _hi(w):
    return pltpu.bitcast(w & jnp.uint32(0xFFFF0000), F32)


def _tie(x, a):
    if a is None:
        return x
    w = pltpu.bitcast(x[:, :128], U32)
    k = w.shape[0] // 8
    w = w | (a if k == 1 else jnp.concatenate([a] * k, axis=0))
    w = pltpu.bitcast(w, x.dtype)
    return w if x.shape[1] == 128 else jnp.concatenate([w, x[:, 128:]], axis=1)


def _top(x, i):
    return jnp.concatenate([x[r:r + 16] for r in range(16 * i, x.shape[0], 32)], axis=0)


def _zip(t, b):
    return jnp.concatenate([x[r:r + 16] for r in range(0, t.shape[0], 16) for x in (t, b)], axis=0)


def _lhs_sums(x1, x2):
    a11, a21, a12, a22 = _top(x1, 0), _top(x1, 1), _top(x2, 0), _top(x2, 1)
    return [a11 + a22, a21 + a22, a11 + a12, a21 - a11, a12 - a22]


def C(i):
    return slice(i * 128, (i + 1) * 128)


class Unit:
    def __init__(self, name, tiles, epi, rows, cost, nt=False, full=True, acc=False, tail=0):
        self.tail = tail
        self.acc, self.res = acc, []
        self.name, self.tiles, self.epi, self.rows, self.cost, self.nt, self.full = name, tiles, epi, rows, cost, nt, full


class Due:
    def __init__(self, val, delay):
        self.val, self.delay = val, delay


class Group:
    def __init__(self, name, fns, cost, rel, dead, lat, rlat=200):
        self.name, self.fns, self.cost, self.rel, self.dead, self.lat, self.rlat = name, fns, cost, rel, dead, lat, rlat


def _plan(seq, groups):
    busy, n = [0] * 4, 0
    start, end, tiles, bars = {}, {}, [], []
    for it in seq:
        if isinstance(it[0], Unit):
            u = it[0]
            m = n % 4
            n += 1
            t0, t1 = busy[m], busy[m] + max(u.rows, 32)
            busy[m] = t1
            tiles.append((t0, t1, u.cost / len(u.tiles) + (u.tail if it[1] == len(u.tiles) - 1 else 0)))
            start.setdefault(u.name, t0)
            end[u.name] = max(end.get(u.name, 0), t1)
        elif it[0] == "wait":
            t = max(busy)
            busy, n = [t] * 4, 0
            start[it[1]] = end[it[1]] = t
            bars.append(t)
    total = max(busy)
    start["end"] = end["end"] = total
    start["start"] = end["start"] = 0
    ns = total // SLOT + 2
    load = np.zeros(ns)
    for t0, t1, c in tiles:
        a, b = t0 // SLOT, max(t1 // SLOT, t0 // SLOT + 1)
        load[a:b] += c / (b - a)
    win = []
    for g in groups:
        r = max(end[x] + (0 if start[x] == end[x] else g.rlat) for x in g.rel)
        d = min(start[x] for x in g.dead) - g.lat
        ok = np.zeros(ns, bool)
        ok[r // SLOT:max(d // SLOT, r // SLOT + 1)] = True
        for b in bars:
            if r < b <= d:
                ok[max((b - g.lat) // SLOT, 0):b // SLOT] = False
        win.append(np.nonzero(ok)[0])
    alloc = [np.zeros(len(w)) for w in win]
    for _ in range(60):
        for i, g in enumerate(groups):
            w = win[i]
            load[w] -= alloc[i]
            base = load[w]
            vol = g.cost * len(g.fns)
            lo, hi = base.min(), base.max() + vol
            for _ in range(50):
                mid = 0.5 * (lo + hi)
                if np.maximum(mid - base, 0).sum() > vol:
                    hi = mid
                else:
                    lo = mid
            alloc[i] = np.maximum(hi - base, 0)
            load[w] += alloc[i]
    times = []
    for i, g in enumerate(groups):
        cum = np.cumsum(alloc[i])
        ts = []
        for k in range(len(g.fns)):
            x = (k + 0.5) * cum[-1] / len(g.fns)
            j = int(np.searchsorted(cum, x))
            prev = cum[j - 1] if j else 0.0
            ts.append(win[i][j] * SLOT + SLOT * (x - prev) / max(alloc[i][j], 1e-9))
        times.append(ts)
    return times


def _emit(seq, groups, zero, wait):
    times = _plan(seq, groups)
    left = {"start": 0}
    for it in seq:
        nm = it[0].name if isinstance(it[0], Unit) else it[1]
        left[nm] = left.get(nm, 0) + 1
    heap, pend, todo, cnt = [], {}, list(range(len(groups))), 0
    busy, n, due = [0] * 4, 0, []

    def release():
        nonlocal cnt
        for i in list(todo):
            g = groups[i]
            if all(left[x] == 0 for x in g.rel):
                todo.remove(i)
                pend[i] = len(g.fns)
                for t, fn in zip(times[i], g.fns):
                    heapq.heappush(heap, (t, cnt, i, fn))
                    cnt += 1

    def force(name):
        nonlocal heap
        for i, g in enumerate(groups):
            if name in g.dead:
                assert i not in todo, (g.name, name)
                if pend[i]:
                    for it in sorted(x for x in heap if x[2] == i):
                        it[3](None)
                    heap = [x for x in heap if x[2] != i]
                    heapq.heapify(heap)
                    pend[i] = 0

    release()
    for it in seq:
        if isinstance(it[0], Unit):
            u, k = it
            force(u.name)
            lhs, rhs = u.tiles[k]()
            t0 = busy[n % 4]
            while u.full and due and due[0][0] < t0 + u.rows:
                t, x = due.pop(0)
                r = min(max(int(t - t0), 0), u.rows - 1) // 16 * 8
                w = pltpu.bitcast(lhs, U32)
                x = pltpu.bitcast(x[:, :128], U32)
                parts = [w[:r], w[r:r + 8] | ((x[0:8] | x[8:16]) & zero), w[r + 8:]]
                lhs = pltpu.bitcast(jnp.concatenate([y for y in parts if y.shape[0]], axis=0), BF16)
            dn = (((1,), (1 if u.nt else 0,)), ((), ()))
            p = lax.dot_general(lhs, rhs, dn, preferred_element_type=F32)
            u.res = [p + u.res[0]] if (u.acc and u.res) else u.res + [p]
            m = n % 4
            n += 1
            t0 = busy[m]
            busy[m] = t0 + max(u.rows, 32)
            used = -8
            while u.full and heap and heap[0][0] < t0 + u.rows:
                r = min(max(int(heap[0][0] - t0), 0), u.rows - 1) // 8 * 8
                r = max(r, used + 8)
                if r >= u.rows or r > max(heap[0][0] - t0, 8) + 16:
                    break
                used = r
                t, _, i, fn = heapq.heappop(heap)
                pend[i] -= 1
                x = fn(pltpu.bitcast(p[r:r + 8], U32) & zero)
                if isinstance(x, Due):
                    due.append((t + x.delay, x.val))
                    due.sort(key=lambda e: e[0])
            if k == len(u.tiles) - 1:
                u.epi(u.res)
            left[u.name] -= 1
        elif it[0] == "wait":
            force(it[1])
            wait(it[1])
            busy, n, due = [max(busy)] * 4, 0, []
            left[it[1]] -= 1
        else:
            it[2]()
            left[it[1]] -= 1
        release()
    force("end")
    assert not heap and not todo


def _sum(ps):
    acc = ps[0]
    for p in ps[1:]:
        acc = acc + p
    return acc


def _flat(us):
    return [(u, i) for u in us for i in range(len(u.tiles))]


def _weave(a, b):
    out = []
    for i, u in enumerate(a):
        out += [u] + b[i * len(b) // len(a):(i + 1) * len(b) // len(a)]
    return out


def _phase(seq):
    n = 0
    for it in seq:
        n = n + 1 if isinstance(it[0], Unit) else (0 if it[0] in ("wait", "sync") else n)
    return n % 4


def _mix(seq, a, b, lo=0.0, hi=1.0):
    n, k = _phase(seq), 0
    for i, t in enumerate(a):
        if k < len(b) and n % 4 == 0 and t[1] != 1 and i >= len(a) * (lo + (hi - lo) * k / len(b)):
            seq.extend(b[k])
            k += 1
        seq.append(t)
        n += 1
    assert k == len(b)


def _wait(seq, name, head=(), back=0):
    r = _phase(seq) + 4 * back
    assert all(isinstance(it[0], Unit) for it in seq[len(seq) - r:])
    seq[len(seq) - r:len(seq) - r] = [("wait", name)] + list(head)


def kernel(q_hbm, k_hbm, v_hbm, sh_hbm, ssm_hbm, sd_hbm, w1_hbm, w2_hbm, w3_hbm, w4_hbm, c_hbm, wm_hbm,
           o_hbm,
           q_n, k_n, v_n, ssm_w, w1_w, w2_w, w3_w, w4_w, wm_w, o_v,
           sh_v, sd_v, c_v, zsrc, z_s, taps, mod_v, tf_w, tg_w,
           kf, uf, acc, zraw, kv_w, zz_w, y_v, x_v, hb_v, x1_v, r_v, n1_w, n2_w, g_w, h1_v, a_w,
           ws_w, as_w, w3n_w, top_v, st_v, l2_w, cb_v,
           sem, sem_b, sem_o):
    bf = lambda r: r.bitcast(BF16)
    w1_v, w2_v, w3_v, w4_v = bf(w1_w), bf(w2_w), bf(w3_w), bf(w4_w)
    wm_v = {0: bf(wm_w[0]), 3: bf(wm_w[1]), 5: bf(wm_w[2])}
    tf_v, tg_v, n1_v, n2_v, g_v = bf(tf_w), bf(tg_w), bf(n1_w), bf(n2_w), bf(g_w)
    a_v, kv_v, zz_v = bf(a_w), bf(kv_w), bf(zz_w)
    w1s, w2s, w3s, w4s = [bf(r) for r in ws_w]
    n1s, gs, n2s, a_s = [bf(r) for r in as_w]
    w3n = bf(w3n_w)
    w3t, w4t, n2t, a_t = [bf(r) for r in l2_w]
    cp = pltpu.make_async_copy
    cat = lambda ls: [x for l in ls for x in l]

    def base(j, n):
        return j * n if isinstance(j, int) else pl.multiple_of(j * n, n)

    def rows(j, n=1, size=T):
        return pl.ds(base(j, size), n * size)

    def view(ref, j, size=T):
        return ref.at[rows(j, 1, size)]

    dmas = {}

    def group(name, *mks):
        sm = sem.at[len(dmas)]
        dmas[name] = [c for mk in mks for c in mk(sm)]

    def ssm_in(t):
        return lambda sm: [cp(ssm_hbm.at[C(t)], bf(ssm_w[t]), sm)]

    def cols(src, start, n, dst, row=0):
        return lambda sm: [cp(src.at[pl.ds(start, n), C(t)], bf(dst).at[t, pl.ds(row, n)], sm) for t in range(NT)]

    def kv_in(s, sl):
        if isinstance(s, int):
            kk = cols(k_hbm, s * T - 16, T + 16, k_n[sl]) if s else cols(k_hbm, 0, T, k_n[sl], 16)
        else:
            kk = cols(k_hbm, pl.multiple_of(s * T - 16, 16), T + 16, k_n[sl])
        return lambda sm: kk(sm) + cols(v_hbm, base(s, T), T, v_n[sl])(sm)

    def q_in(s, sl):
        return cols(q_hbm, base(s, T), T, q_n[sl])

    def wm_in(a, b):
        return lambda sm: [cp(wm_hbm.at[:, a * D:b * D], wm_v[a], sm)]

    def whole(src, dst):
        return lambda sm: [cp(src, dst, sm)]

    next_kv = lambda s: kv_in(s, 0)(sem_b.at[0])
    next_q = lambda s: q_in(s, 0)(sem_b.at[0])

    zsrc[...] = jnp.zeros((8, 128), I32)
    k_n[0][:, 0:8, :] = jnp.zeros((NT, 8, 128), U32)
    w4_w[F // 2:FT * 64, :] = jnp.zeros((FT * 64 - F // 2, D), U32)
    group("small", lambda sm: [cp(zsrc, z_s, sm), cp(sh_hbm, sh_v, sm), cp(sd_hbm, sd_v, sm), cp(c_hbm, c_v, sm)])
    for s in range(NC):
        group("c%d" % s, ssm_in(s), kv_in(s, s))
    group("c3", ssm_in(3), ssm_in(4))
    group("wma", wm_in(0, 3), q_in(0, 0), q_in(1, 1))
    group("wmb", wm_in(3, 5))
    group("w1", whole(w1_hbm, w1_v))
    group("w2", q_in(2, 2), whole(w2_hbm, w2_v))
    group("w3", whole(w3_hbm, w3_v))
    group("w4", whole(w4_hbm, w4_v.at[0:F]), wm_in(5, 6))
    for g in dmas.values():
        for c in g:
            c.start()

    def wait(name):
        for c in dmas[name]:
            c.wait()

    tau_b = lambda l: H + ((l + (H - 1)) & (H - 1))
    tf_v[:, C(0)] = _dft((T, H), 0, lambda l: jnp.where((l & 1) == 0, l, tau_b(l)), 1.0 / T)
    tf_v[:, C(1)] = _dft((T, H), 0, lambda l: jnp.where((l & 1) == 1, l, tau_b(l)), 1.0 / T)
    tf_v[:, C(2)] = _dft((T, H), 0, lambda l: 2 * l - H)
    tf_v[:, C(3)] = _dft((T, H), 0, lambda l: 2 * l + 1 - H)
    sin0 = lax.broadcasted_iota(I32, (GR, T), 1) >= H
    tg_v[:, 0:T] = _dft((GR, T), 1, lambda l: jnp.where(sin0 & (l == 0), H, 2 * l))
    tg_v[:, T:2 * T] = _dft((GR, T), 1, lambda l: 2 * l + 1)
    h1_v[:, 0:8, :] = jnp.zeros((NT, 8, 128), F32)
    h1_v[:, 8 + NC * T:16 + NC * T, :] = jnp.zeros((NT, 8, 128), F32)

    wait("small")
    z = jnp.clip(z_s[0, 0], 0, 1)
    zero = jnp.full((8, 128), z, I32).astype(U32)
    z8 = pl.multiple_of(z * 8, 8)
    for r in (x_v, hb_v, x1_v, r_v, zraw, n1_w, n2_w, g_w, a_w, kv_w, zz_w, *ws_w, *as_w, w3n_w, top_v, st_v, *l2_w, cb_v):
        r[pl.ds(z8, 8), 0:128] = jnp.zeros((8, 128), r.dtype)
    for r in (kf, uf, acc, taps, mod_v):
        r[z, 0:8, 0:128] = jnp.zeros((8, 128), r.dtype)
    for r in (tf_w, tg_w):
        r[pl.ds(z8, 8), 0:128] = r[0:8, 0:128]
    sh = sh_v[...].astype(F32)
    for i in range(4):
        taps[i] = jnp.broadcast_to(sh[i:i + 1], (8, D))
    taps[4] = jnp.broadcast_to(sd_v[...].astype(F32).reshape(1, D) * (1.0 / T), (8, D))
    cf = c_v[...].astype(F32)
    silu_c = jnp.broadcast_to((cf / (1.0 + jnp.exp(-cf))).astype(BF16), (16, D))

    def mmK(n):
        def unit(m):
            st = []

            def rhs(i):
                if not st:
                    ev = (lax.broadcasted_iota(I32, (64, 128), 1) & 1) == 0
                    a = ssm_w[n][:, m * T:m * T + H]
                    b = pltpu.roll(ssm_w[n][:, m * T + H:(m + 1) * T], 1, 1)
                    st.extend([pltpu.bitcast(jnp.where(ev, a, b), BF16), pltpu.bitcast(jnp.where(ev, b, a), BF16)])
                return st[i]

            def epi(p):
                er, ei, or_, oi = p
                cur = [er, ei, or_, oi]
                if m:
                    pv = [zraw[C(4 * ((m - 1) % 2) + (q ^ 1)), :] for q in range(4)]
                    pm = lambda x, y, up: jnp.concatenate([x[:64] + y[:64], x[64:] - y[64:]] if up else
                                                          [x[:64] - y[:64], x[64:] + y[64:]], axis=0)
                    er, ei, or_, oi = [pm(cur[q], pv[q], q & 1) for q in range(4)]
                else:
                    er = er + taps[4, 0:1, C(n)]
                if m + 1 < NB:
                    for q in range(4):
                        zraw[C(4 * (m % 2) + q), :] = cur[q]
                for h, (cr, ci) in enumerate(((er + or_, ei + oi), (er - or_, ei - oi))):
                    B = h * 3 * H
                    kf[m, B:B + H, C(n)] = cr
                    kf[m, B + H:B + 2 * H, C(n)] = ci - cr
                    kf[m, B + 2 * H:B + 3 * H, C(n)] = ci + cr
            return Unit("K%d" % n, [(lambda i=i, r=r: (tf_v[r:r + H, C(i)], rhs(i))) for i in range(2) for r in (0, H)],
                        epi, H, 260, nt=True)
        return [unit(m) for m in range(NB)]

    def kv(s, sl):
        def mk(t, w):
            def fn(a):
                ld = lambda o, n: k_n[s][t, pl.ds(8 + w + o, n), :]
                c0 = jnp.concatenate([_tie(ld(0, 8), a), ld(8, 8)], axis=0).reshape(2, 8, 128)
                c1, c2 = ld(-1, 16).reshape(2, 8, 128), ld(-2, 16).reshape(2, 8, 128)
                s0, s1, s2, s3 = (taps[i, :, C(t)] for i in range(4))
                ke, ko, ke1, ko1, ko2 = _lo(c0), _hi(c0), _lo(c1), _hi(c1), _hi(c2)
                wv = v_n[s][t, w:w + 16, :].reshape(2, 8, 128)
                kve = ((s0 * ke + s1 * ko1) + (s2 * ke1 + s3 * ko2)) * _lo(wv)
                kvo = ((s0 * ko + s1 * ke) + (s2 * ko1 + s3 * ke1)) * _hi(wv)
                kv_v[pl.ds(sl * T + w, 16), C(t)] = kve.reshape(16, 128).astype(BF16)
                kv_v[pl.ds(sl * T + H + w, 16), C(t)] = kvo.reshape(16, 128).astype(BF16)
            return fn
        return [[mk(t, w) for w in range(0, H, 16)] for t in range(NT)]

    def mmU(name, sl, us):
        def unit(n):
            def epi(p):
                er, ei, or_, oi = p
                for h, (cr, ci) in enumerate(((er + or_, ei + oi), (er - or_, ei - oi))):
                    B = h * 3 * H
                    uf[us, B:B + H, C(n)] = cr + ci
                    uf[us, B + H:B + 2 * H, C(n)] = cr
                    uf[us, B + 2 * H:B + 3 * H, C(n)] = ci
            return Unit(name(n), [(lambda i=i, r=r: (tf_v[r:r + H, C(2 + i)], kv_v[pl.ds(sl * T + i * H, H), C(n)]))
                                  for i in range(2) for r in (0, H)], epi, H, 96 + 96 * KS)
        return [unit(n) for n in range(NT)]

    def cmul(m0, u0, n, h, row, L, a):
        t = []
        for i in range(3):
            Rw = slice((3 * h + i) * H + row, (3 * h + i) * H + row + 8)
            kk = kf[m0:m0 + n, Rw, L]
            if i == 0 and a is not None:
                k0 = _tie(kk[0], a)[None]
                kk = k0 if n == 1 else jnp.concatenate([k0, kk[1:]], axis=0)
            t.append(jnp.sum(kk * uf[u0:u0 + n, Rw, L], axis=0))
        return t[0] - t[2], t[0] + t[1]

    def AR(h, q, row):
        return slice((2 * h + q) * H + row, (2 * h + q) * H + row + 8)

    def mac(n, u0, sl, part=False):
        def mk(t, rc):
            st, fin = [], []

            def piece(i):
                def fn(a):
                    h, row = i & 1, rc + (i >> 1) * 8
                    zr, zi = cmul(0, u0, n, h, row, C(t), a)
                    if part:
                        zr, zi = zr + acc[0, AR(h, 0, row), C(t)], zi + acc[0, AR(h, 1, row), C(t)]
                    st.append((zr, zi))
                    if h:
                        (pr, pi), (mr, mi) = st[-2:]
                        fin.append([pr + mr, pi + mi, pr - mr, pi - mi])
                    if i == 3:
                        for q in range(4):
                            zz_v[pl.ds(sl * 2 * T + q * H + rc, 16), C(t)] = jnp.concatenate(
                                [fin[0][q], fin[1][q]], axis=0).astype(BF16)
                return fn
            if not part:
                return [piece(i) for i in range(4)]
            both = lambda f, g: (lambda a: (f(a), g(None)))
            return [both(piece(0), piece(1)), both(piece(2), piece(3))]
        return [[fn for rc in range(0, H, 16) for fn in mk(t, rc)] for t in range(NT)]

    def pos():
        return [(t, h, row) for t in range(NT) for row in range(0, H, 8) for h in range(2)]

    def ahead(i):
        def mk(t, h, row):
            def fn(a):
                zr, zi = cmul(i + 1, 0, NC, h, row, C(t), a)
                acc[i, AR(h, 0, row), C(t)] = zr
                acc[i, AR(h, 1, row), C(t)] = zi
            return fn
        return [mk(*p) for p in pos()]

    def spread():
        n = NB - NC - 1

        def mk(t, h, row):
            def fn(a):
                p = []
                for i in range(3):
                    Rw = slice((3 * h + i) * H + row, (3 * h + i) * H + row + 8)
                    u = uf[0, Rw, C(t)]
                    p.append(kf[1:1 + n, Rw, C(t)] * (_tie(u, a) if i == 0 else u)[None])
                acc[0:n, AR(h, 0, row), C(t)] = acc[1:1 + n, AR(h, 0, row), C(t)] + (p[0] - p[2])
                acc[0:n, AR(h, 1, row), C(t)] = acc[1:1 + n, AR(h, 1, row), C(t)] + (p[0] + p[1])
            return fn
        return [mk(*p) for p in pos()]

    def mmI(name, sl, ys):
        def unit(n):
            def epi(p):
                ce, se, co, so = p
                sub = lax.broadcasted_iota(I32, (8, 128), 0)
                b0 = ys * (T + 8) + 8
                y_v[n, b0 + H - 1:b0 + H, :] = (ce[64:72] - se[0:8])[0:1]
                se = jnp.concatenate([jnp.where(sub == 0, 0.0, se[0:8]), se[8:]], axis=0)
                for d, cc, ss in ((0, ce[0:64], se), (1, co, so)):
                    y_v[n, pl.ds(b0 + H + d, 64, stride=2), :] = cc + ss
                    y_v[n, pl.ds(b0 + d - 1, 64, stride=2), :] = cc - ss
            return Unit(name(n), [(lambda i=i: (tg_v[0:(GR if i == 0 else 64), C(i)], zz_v[pl.ds(sl * 2 * T + i * H, H), C(n)]))
                                  for i in range(4)], epi, 64, 36 + 33 * KS)
        return [unit(n) for n in range(NT)]

    def mod(name, a, b):
        def unit(n):
            def epi(p):
                v = [_sum(p[i * NT:(i + 1) * NT])[0:8] for i in range(b - a)]
                if a == 0:
                    mod_v[0, :, C(n)] = v[0] * v[2]
                    mod_v[1, :, C(n)] = (v[1] + 1.0) * v[2]
                elif a == 3:
                    mod_v[3, :, C(n)] = v[0] * (1.0 / G_POST)
                    mod_v[4, :, C(n)] = (v[1] + 1.0) * (1.0 / G_POST)
                else:
                    mod_v[2, :, C(n)] = v[0] * G_POST
            return Unit(name, [(lambda i=i, k=k: (silu_c[:, C(k)], wm_v[a][C(k), pl.ds(i * D + n * 128, 128)]))
                               for i in range(b - a) for k in range(NT)], epi, 16, 10, full=False, acc=b - a == 1)
        return [unit(n) for n in range(NT)]

    HS = (slice(0, 128), slice(128, 256))
    QS = tuple(slice(r, r + 64) for r in range(0, T, 64))

    def tasks(f, due=None, tie=True, n=RG):
        def mk(R):
            def fn(a):
                x = f(R, a if tie else None)
                return Due(x, due) if due else None
            return fn
        return [mk(slice(r, r + n)) for r in range(0, T, n)]

    def load_y(sl, R):
        b0, back = sl * (T + 8) + 8, 7 - lax.broadcasted_iota(I32, (8, 128), 0)

        def ld(t, r):
            if r >= H:
                return y_v[t, b0 + r:b0 + r + 8, :]
            return jnp.take_along_axis(y_v[t, b0 + H - 8 - r:b0 + H - r, :], back, axis=0)
        return jnp.stack([jnp.concatenate([ld(t, r) for t in range(NT)], axis=1) for r in (R.start, R.start + 8)])

    def put(nn, ss, R, x):
        nn[R, :] = x.astype(BF16)
        tok = x
        if ss is not None:
            S2 = pl.ds(R.start // 32 * 16, 16)
            if R.stop % 32:
                top_v[S2, 0:2 * T] = x[:, 0:2 * T]
            else:
                if R.start % 32:
                    x = jnp.concatenate([top_v[S2, 0:2 * T], x[:, 0:2 * T]], axis=0)
                ss[S2, 0:5 * T] = jnp.concatenate(_lhs_sums(x[:, 0:T], x[:, T:2 * T]), axis=1).astype(BF16)
        return tok

    wide = lambda v: jnp.concatenate([v] * NT, axis=1)

    def mean(i, R, x):
        st_v[R, C(i)] = jnp.broadcast_to(jnp.sum(x, axis=-1, keepdims=True) * (1.0 / D), (x.shape[0], 128))

    def centred(src, i, R, a):
        return src[R, :] - wide(_tie(st_v[R, C(i)], a))

    def scale(src, i, g):
        def f(R, a):
            st_v[R, C(i + 1)] = jnp.broadcast_to(_rstd(centred(src, i, R, a), g), (RG, 128))
        return f

    def normed(src, i, R, a):
        return centred(src, i, R, a) * wide(st_v[R, C(i + 1)])

    def front(sl, xs, early=False, ss=None):
        xx, hh, nn = view(x_v, xs), view(hb_v, xs), view(n1_v, sl)

        def fa(R, a):
            q = [q_n[sl][t, R.start // 2:R.stop // 2, :] for t in range(NT)]
            q = jnp.concatenate([_tie(q[0], a)] + q[1:], axis=1)
            q = pltpu.bitcast(q, BF16).astype(F32).reshape(2, 8, D)
            x = (q + (_ln(q) * mod_v[1] + mod_v[0]) * load_y(sl, R)).reshape(RG, D)
            xx[R, :] = x
            if early:
                hh[R, :] = _ln(x)

        def fb(R, a):
            hh[R, :] = (_ln(_tie(xx[R, :], a).reshape(2, 8, D)) * mod_v[4] + mod_v[3]).reshape(RG, D)

        def fc(R, a):
            hb = _tie(hh[R, :], a)
            if early:
                hb = (hb.reshape(2, 8, D) * mod_v[4] + mod_v[3]).reshape(RG, D)
                hh[R, :] = hb
            nn[R, :] = _ln(hb, True).astype(BF16)
        if early:
            return tasks(fa), tasks(fc)
        if ss is None:
            return tasks(fa) + tasks(fb) + tasks(fc)
        qf = view(x_v, 2)

        def s1(R, a):
            q = [q_n[sl][t, R.start // 2:R.stop // 2, :] for t in range(NT)]
            q = pltpu.bitcast(jnp.concatenate([_tie(v, a) for v in q], axis=1), BF16).astype(F32)
            qf[R, :] = q
            mean(0, R, q)

        def s3(R, a):
            h = normed(qf, 0, R, a).reshape(2, 8, D) * mod_v[1] + mod_v[0]
            x = qf[R, :] + (h * load_y(sl, R)).reshape(RG, D)
            xx[R, :] = x
            mean(2, R, x)

        def s5(R, a):
            hb = (normed(xx, 2, R, a).reshape(2, 8, D) * mod_v[4] + mod_v[3]).reshape(RG, D)
            hh[R, :] = hb
            mean(4, R, hb)
        s7 = [f for g in tasks(lambda R, a: put(nn, ss, R, normed(hh, 4, R, a)), n=32) for f in (g, lambda a: None)]
        st = [tasks(s3), tasks(scale(xx, 2, False)), tasks(s5), tasks(scale(hh, 4, True)), s7]
        p = [tasks(s1), tasks(scale(qf, 0, False))]
        sk = 4.091

        def wave(ls):
            body = sorted((i * sk + g, i, g) for i in range(len(ls) - 1) for g in range(8))
            return [ls[i][g] for _, i, g in body] + ls[-1]
        qb = []
        done = lambda a: qb[0](a)
        full = wave([x[8:] for x in p + st])
        k = full.index(p[0][15]) + 1
        return wave([x[:8] for x in st]), full[:k] + [done] + full[k:], cat(x[:8] for x in p), qb

    def shift(hs, sl, pieces=((0, 64), (64, 64), (128, 64), (192, 64)), ss=None):
        gg = view(g_v, sl)

        def one_tile(t, r, n, a):
            lane = lax.broadcasted_iota(I32, (n, 128), 1)
            ld = lambda d: h1_v[t, pl.ds(hs * T + 8 + r + d, n), :]
            if t == 0:
                g = ld(-1)
            elif t == 1:
                g = jnp.where(lane < 32, ld(-1), ld(1))
            elif t == 2:
                g = jnp.where(lane < 64, ld(1), ld(-2))
            elif t == 3:
                g = jnp.where(lane < 96, ld(-2), ld(2))
            else:
                g = ld(2)
            if a is not None:
                g = jnp.concatenate([_tie(g[i:i + 8], a) if i % 16 == 0 else g[i:i + 8]
                                     for i in range(0, n, 8)], axis=0)
            gg[r:r + n, C(t)] = g.astype(BF16)
            return g

        def mk(ts, r, n):
            def fn(a):
                g = [one_tile(t, r, n, a) for t in ts]
                if len(ts) == 2:
                    for i, x in enumerate(_lhs_sums(*g)):
                        ss[r // 2:(r + n) // 2, C(2 * i + ts[0])] = x.astype(BF16)
            return fn
        sets = [(t,) for t in range(NT)] if ss is None else [(0, 2), (1, 3), (4,)]
        return [mk(ts, r, n) for ts in sets for r, n in pieces]

    def shift_early():
        def keep(a):
            h1_v[:, 2 * T - 32:2 * T + 8, :] = h1_v[:, 3 * T - 32:3 * T + 8, :]
        return shift(2, 0, [(r, 32) for r in range(0, T - 32, 32)], gs) + [keep]

    def ln2(xs, sl, fast=True):
        xx, nn, ss = view(x1_v, xs), view(n2_v, sl), view(n2s, sl, H) if fast else None
        f = lambda R, a: put(nn, ss, R, _ln(_tie(xx[R, :], a), True))
        ts = tasks(f, 900) if sl else tasks(f, DL, False)
        return ts[0::2] + ts[1::2] if fast else tasks(f)

    def ln2_late():
        xx, nn, ss = view(x1_v, 0), view(n2_v, 0), view(n2s, 0, H)
        a_, b_ = tasks(lambda R, a: mean(6, R, _tie(xx[R, :], a))), tasks(scale(xx, 6, True))
        c_ = [f for g in tasks(lambda R, a: put(nn, ss, R, normed(xx, 6, R, a)), n=32)[:4] for f in (g, lambda a: None)]
        return a_[:8] + b_[:8] + c_

    def resid(xs, x1s, rotate=False):
        xx, x1 = view(x_v, xs), view(x1_v, x1s)
        tie = lambda v, a: v if a is None else pltpu.bitcast(pltpu.bitcast(v, U32) | wide(a), F32)

        def f(R, a):
            r_v[R, :] = xx[R, :] + tie(x1[R, :], a) * mod_v[2]

        def move(dst, src):
            def g(R, a):
                dst[R, :] = tie(src[R, :], a)
            return tasks(g, n=8)
        if not rotate:
            return tasks(f, n=8)
        return cat(zip(tasks(f, n=8), move(view(hb_v, 1), hb_v), move(xx, x_v)))

    KD, KF, ND = [(0, 2), (1, 3)], [(2 * i, 2 * i + 1) for i in range(7)], [(1, 2), (3, 4)]
    Wt = {1: (lambda k, n: w1_v[C(k), C(n)], lambda i, kp, j: w1s[C(kp), C(2 * i + j)], False, KD, [4]),
          2: (lambda k, n: w2_v[C(k), C(n)], lambda i, kp, j: w2s[C(kp), C(2 * i + j)], False, KD, [4]),
          0: (lambda k, n: w3_v[C(n), C(k)], None, True, KD, [4]),
          3: (lambda k, n: w3n[C(k), C(n)], lambda i, kp, j: w3s[C(kp), C(6 * i + j)], False, KD, [4]),
          4: (lambda k, n: w4_v[C(k), C(n)], lambda i, kp, j: w4s[C(kp), C(2 * i + j)], False, KF, [])}

    def sums_task(load, store, left):
        def fn(a):
            b = [[load(u, v) for v in range(2)] for u in range(2)]
            b[0][0], b[1][1] = _tie(b[0][0], a), _tie(b[1][1], a)
            (x11, x12), (x21, x22) = [[pltpu.bitcast(x, BF16).astype(F32) for x in row] for row in b]
            r = ((x11 + x22, x21 + x22, x11 + x12, x21 - x11, x12 - x22) if left else
                 (x11 + x22, x12 - x22, x21 - x11, x11 + x12, x21 + x22))
            for m, x in enumerate(r):
                store(m, x.astype(BF16))
        return fn

    def wsums(w_w, ws, rp, cp_):
        def mk(i, j, r):
            def store(m, x):
                ws[pl.ds(128 * i + r, 16), C(len(cp_) * m + j)] = x
            return sums_task(lambda u, v: w_w[pl.ds(64 * rp[i][u] + r // 2, 8), C(cp_[j][v])], store, False)
        return [mk(i, j, r) for j in range(len(cp_)) for i in range(len(rp)) for r in range(0, 128, 16)]

    def w3_turn():
        def mk(n, k):
            def fn(a):
                x = jnp.concatenate([_tie(w3_w[64 * n:64 * n + 8, C(k)], a), w3_w[64 * n + 8:64 * n + 64, C(k)]], axis=0)
                w3n[C(k), C(n)] = pltpu.bitcast(x, BF16).T
            return fn
        return [mk(n, k) for n in range(FT - 1) for k in range(NT)]

    def plain(name, w, lhs, n, R, epi, cost):
        tile, _, nt, kp, kl = Wt[w]
        ks = sorted([k for p in kp for k in p] + kl)
        rows_ = R.stop - R.start
        return Unit(name, [(lambda k=k: (lhs[R, C(k)], tile(k, n))) for k in ks], lambda p: epi(n, R, p[0]),
                    rows_, rows_ // 8 * (len(ks) - 1), nt=nt, acc=True, tail=rows_ // 8 * cost(n))

    def quad(name, w, lhs, sums, j, cols_, R, epi, cost):
        tile, wsum, nt, kp, kl = Wt[w] if isinstance(w, int) else w
        h, S2, c = len(kp), slice(R.start // 2, R.stop // 2), {}
        a_ = lambda i, k: _top(lhs(k) if callable(lhs) else lhs[R, C(k)], i)
        s_ = sums if callable(sums) else (lambda i, p: sums[S2, C(h * i + p)])
        prod = lambda fa_, fb_: [(lambda p=p: (fa_(p), fb_(p))) for p in range(h)]
        left = lambda i, n: [(lambda k=k: (a_(i, k), tile(k, n))) for k in kl]
        mk = lambda tiles, f, x=0: Unit(name, tiles, lambda p: f(p[0]), 64, 8 * len(tiles), nt=nt, acc=True, tail=x)

        def e1(m):
            u7.res, u6.res = [m], [m]

        def e4(m):
            c[11], c[21] = c[11] + m, m

        def e2(m):
            c[21], c[22] = c[21] + m, c[22] - m
            l21.res = [c[21]]

        def e5(m):
            c[12] = m
            epi(cols_[0], R, _zip(c[11] - m, c[21]))

        def e3(m):
            l12.res, c[22] = [c[12] + m], c[22] + m
            if not kl:
                l12.epi(l12.res)
        u1 = mk(prod(lambda p: s_(0, p), lambda p: wsum(0, p, j)), e1)
        u7 = mk(prod(lambda p: s_(4, p), lambda p: wsum(4, p, j)) + left(0, cols_[0]), lambda m: c.update({11: m}))
        u6 = mk(prod(lambda p: s_(3, p), lambda p: wsum(3, p, j)) + left(1, cols_[1]), lambda m: c.update({22: m}))
        u4 = mk(prod(lambda p: a_(1, kp[p][1]), lambda p: wsum(2, p, j)), e4)
        u2 = mk(prod(lambda p: s_(1, p), lambda p: tile(kp[p][0], cols_[0])), e2, 8)
        l21 = mk(left(1, cols_[0]), lambda m: c.update({21: m}))
        u5 = mk(prod(lambda p: s_(2, p), lambda p: tile(kp[p][1], cols_[1])), e5, 16 * cost(cols_[0]))
        u3 = mk(prod(lambda p: a_(0, kp[p][0]), lambda p: wsum(1, p, j)), e3, 8 if kl else 8 + 16 * cost(cols_[1]))
        l12 = mk(left(0, cols_[1]), lambda m: epi(cols_[1], R, _zip(m, c[22])), 16 * cost(cols_[1]))
        return [u1, u7, u6, u4, u2, l21, u5, u3, l12]

    LH, RH = [0, 4, 3, (1, 1), 1, 2, (0, 0)], [0, 4, 3, 2, (0, 0), (1, 1), 1]
    L2 = {3: (w3n_w, ws_w[2], w3t, KF[:6], n2t), 4: (w4_w, ws_w[3], w4t, ND, a_t)}

    def wsums2(w):
        w_w, s_w, ws2, cp_, _ = L2[w]
        kp, nj = Wt[w][3], len(cp_)

        def mk(o, p2, j2, r):
            def load(u, v):
                p, j, y = 2 * p2 + u, 2 * j2 + v, RH[o]
                if isinstance(y, int):
                    return s_w[pl.ds(64 * p + r // 2, 8), C(nj * y + j)]
                return w_w[pl.ds(64 * kp[p][y[0]] + r // 2, 8), C(cp_[j][y[1]])]

            def store(m, x):
                ws2[pl.ds(128 * p2 + r, 16), C((5 * o + m) * (nj // 2) + j2)] = x
            return sums_task(load, store, False)
        return [mk(o, p2, j2, r) for j2 in range(nj // 2) for o in range(7) for p2 in range(len(kp) // 2)
                for r in range(0, 128, 16)]

    def wsums4():
        form = [((0, 0), (1, 1), 1), ((0, 1), (1, 1), -1), ((1, 0), (0, 0), -1), ((0, 0), (0, 1), 1), ((1, 0), (1, 1), 1)]

        def mk(o, p2, r):
            def fn(a):
                def blk(p, j, uv, t):
                    x = w4_w[pl.ds(64 * KF[p][uv[0]] + r // 2, 8), C(ND[j][uv[1]])]
                    return pltpu.bitcast(_tie(x, t), BF16).astype(F32)
                y = {}
                for u in range(2):
                    for j in range(2):
                        p = 2 * p2 + u
                        if isinstance(RH[o], int):
                            f = form[RH[o]]
                            x1, x2 = blk(p, j, f[0], a), blk(p, j, f[1], None)
                            y[u, j] = x1 + x2 if f[2] > 0 else x1 - x2
                            w4s[pl.ds(128 * p + r, 16), C(2 * RH[o] + j)] = y[u, j].astype(BF16)
                        else:
                            y[u, j] = blk(p, j, RH[o], a if u == j else None)
                for m, f in enumerate(form):
                    x = y[f[0]] + y[f[1]] if f[2] > 0 else y[f[0]] - y[f[1]]
                    w4t[pl.ds(128 * p2 + r, 16), C(5 * o + m)] = x.astype(BF16)
            return fn
        last = wsums(w4_w, w4s, KF, ND)
        return (last[48:56] + last[104:112]
                + [mk(o, p2, r) for o in range(7) for p2 in range(3) for r in range(0, 128, 16)])

    def lsums2(w, lhs_w, sums_w, sl):
        kp, xs2 = Wt[w][3], L2[w][4]
        h2 = len(kp) // 2

        def mk(o, p2, g):
            def load(u, v):
                p, ch, x = 2 * p2 + v, 2 * g + u, LH[o]
                if isinstance(x, int):
                    return sums_w[pl.ds(64 * sl + 8 * ch, 8), C(len(kp) * x + p)]
                return lhs_w[pl.ds(H * sl + 16 * ch + 8 * x[0], 8), C(kp[p][x[1]])]

            def store(m, x):
                xs2[pl.ds(16 * g, 16), C((5 * o + m) * h2 + p2)] = x
            return sums_task(load, store, True)
        return [[mk(o, p2, g) for o in range(7) for g in range(4)] for p2 in range(h2)]

    def quad2(name, w, lhs, sums, j2, epi, cost):
        tile, wsum, nt, kp, kl = Wt[w]
        ws2, cp_, xs2 = L2[w][2:]
        h, h2, nj2, c, R = len(kp), len(kp) // 2, len(cp_) // 2, {}, slice(0, T)

        b0 = 8 * (j2 if kl else 3)
        slot = lambda j, i, v: C(b0 + 4 * (j % 2) + 2 * (i - 1) + v)

        def upd(o, j, m):
            val = {}
            for i, v, sg in (((1, 0, 1), (2, 1, 1)), ((1, 0, 1),), ((2, 1, 1),), ((1, 0, 1), (2, 0, 1)),
                             ((2, 0, 1), (2, 1, -1)), ((1, 0, -1), (1, 1, 1)), ((1, 1, 1), (2, 1, 1)))[o]:
                k = (j, i, v)
                if o == 0 and i == 1:
                    c[k] = slot(j, 2, 1)
                    continue
                val[i, v] = m if k not in c else (cb_v[:, c[k]] + m if sg > 0 else cb_v[:, c[k]] - m)
                c[k] = slot(*k)
                if kl or o < 5 or v != o - 5:
                    cb_v[:, c[k]] = val[i, v]
            if o >= 5 and not kl:
                v = o - 5
                epi(cp_[j][v], R, _zip(*[val[i, v] if (i, v) in val else cb_v[:, c[j, i, v]] for i in (1, 2)]))

        def inner(o):
            x, y = LH[o], RH[o]
            xo = ((lambda p: sums[:, C(h * x + p)]) if isinstance(x, int)
                  else (lambda p: _top(lhs[:, C(kp[p][x[1]])], x[0])))
            yo = ((lambda p, j: wsum(y, p, j)) if isinstance(y, int)
                  else (lambda p, j: tile(kp[p][y[0]], cp_[j][y[1]])))
            w_ = (yo, lambda m, p2, _: ws2[C(p2), C((5 * o + m) * nj2 + j2)], nt,
                  [(2 * i, 2 * i + 1) for i in range(h2)], list(range(2 * h2, h)))
            return quad(name, w_, xo, lambda m, p2: xs2[:, C((5 * o + m) * h2 + p2)], 0, (2 * j2, 2 * j2 + 1),
                        HS[0], lambda j, _, m: upd(o, j, m), lambda j: 1.5 + KS + (2 * cost(0) if o >= 5 and not kl else 0))

        def rest(j, v, Q):
            return [Unit(name, [lambda: (lhs[Q, C(k)], tile(k, cp_[j][v]))],
                         lambda p: epi(cp_[j][v], Q, p[0] + _zip(*[cb_v[Q.start // 2:Q.stop // 2, c[j, i, v]] for i in (1, 2)])), 64, 8 * (cost(cp_[j][v]) + 1)) for k in kl]
        return cat(inner(o) for o in range(7)), [u for Q in QS for j in (2 * j2, 2 * j2 + 1) for v in range(2)
                                                 for u in rest(j, v, Q)]

    def mm(name, w, lhs, sums, epi, cost):
        if sums is None:
            return [[plain(name, w, lhs, n, R, epi, cost) for R in HS] for n in range(NT)]
        return [[plain(name, w, lhs, 0, R, epi, cost) for R in QS]] + [
            [u for R in HS for u in quad(name, w, lhs, sums, j, ND[j], R, epi, cost)] for j in range(2)]

    def mm1(name, hs, sl, fast=False):
        def epi(n, R, p):
            h1_v[n, pl.ds(hs * T + 8 + R.start, R.stop - R.start), :] = _gelu2(p)
        return cat(mm(name, 1, view(n1_v, sl), n1s if fast else None, epi, lambda n: 5 + KS))

    def mm2(name, sl, xs, x1s, fast=False):
        def epi(n, R, p):
            view(x1_v, x1s)[R, C(n)] = view(hb_v, xs)[R, C(n)] + p
        return cat(mm(name, 2, view(g_v, sl), gs if fast else None, epi, lambda n: 1 + KS))

    def mm3(name, sl, fast=True, host=None):
        nn, aa, ss, keep, tail = view(n2_v, sl), view(a_v, sl), view(a_s, sl, H), {}, []

        def epi(n, R, p):
            g = _gelu2(p)
            aa[R, C(n)] = g.astype(BF16)
            if not fast:
                return
            if n % 2 == 0 and n < 12:
                keep[n] = g
                return
            pair = (keep.pop(n - 1), g) if n % 2 else (g, tail[R.start // 128][R.start % 128:R.start % 128 + 64])
            for i, x in enumerate(_lhs_sums(*pair)):
                ss[R.start // 2:R.stop // 2, C(7 * i + n // 2)] = x.astype(BF16)

        c3 = lambda n: 5.5 + 0.5 * KS + (3.75 + 1.25 * KS if fast and (n % 2 or n == 12) else 0)

        def rem(R):
            def f(p):
                tail.append(jnp.concatenate([_gelu2(p[0]), jnp.zeros((64, 128), F32)], axis=0).T)
                aa[R, C(13)] = tail[-1].astype(BF16)
            return Unit(name, [(lambda k=k: (w3_v[13 * 128:F, C(k)], nn[R, C(k)])) for k in range(NT)], f, 64, 84,
                        nt=True, acc=True)
        odd = [rem(R) for R in HS] + [plain(name, 3 if fast else 0, nn, 12, R, epi, c3) for R in QS]
        if not fast:
            return odd + [plain(name, 0, nn, n, R, epi, c3) for p in KF[:6] for R in HS for n in p]
        qd = [quad2(name + "_%d" % j, 3, nn, view(n2s, sl, H), j, epi, c3) for j in range(3)]
        mid = qd[0][0] + _weave(qd[1][0], qd[0][1]) + _weave(qd[2][0], qd[1][1])
        if host is None:
            return odd[:2] + mid + _weave(odd[2:], qd[2][1])
        for u in (odd[0], odd[2], odd[3]):
            u.name = name + "h"
        return [odd[0], odd[2], odd[3], odd[1]] + mid, _weave(odd[4:] + host, qd[2][1])

    def cp_out(j, osl, L, sm, R=slice(0, T)):
        return cp(o_v.at[pl.ds(osl * T + R.start, R.stop - R.start), L],
                  o_hbm.at[pl.ds(base(j, T) + R.start, R.stop - R.start), L], sem_o.at[sm])

    out_a = lambda j: cp_out(j, 0, slice(128, D), 0)
    out_b = lambda j: cp_out(j, 0, C(0), 1)
    last = []

    def mm4(name, j, sl, osl=0, xs=None, x1s=None, fast=True):
        oo = view(o_v, osl)

        def epi(n, R, p):
            if xs is None:
                oo[R, C(n)] = (r_v[R, C(n)] + mod_v[2, 0:1, C(n)] * p).astype(BF16)
            else:
                oo[R, C(n)] = (view(x_v, xs)[R, C(n)] + mod_v[2, 0:1, C(n)]
                               * (view(x1_v, x1s)[R, C(n)] + p)).astype(BF16)
            if osl == 2:
                last.append(cp_out(j, osl, C(n), 2, R))
                last[-1].start()
            elif R.stop == T and osl and n == NT - 1:
                last.append(cp_out(j, osl, slice(128 if osl == 3 else 0, D), 2))
                last[-1].start()
            elif R.stop == T and osl == 0 and n in (0, NT - 1):
                (out_a if n else out_b)(j).start()
        c4 = lambda n: (3 if xs is None else 4) + KS
        if fast:
            return ([plain(name, 4, view(a_v, sl), 0, R, epi, c4) for R in QS],
                    quad2(name + "q", 4, view(a_v, sl), view(a_s, sl, H), 0, epi, c4)[0])
        return mm(name, 4, view(a_v, sl), None, epi, c4)

    def split(us):
        n = 4 // len(us)
        m, mks, st = us[0].rows // n, [u.tiles.pop(0) for u in us], {}

        def piece(i, k):
            if i not in st:
                st[i] = mks[i]()
            return st[i][0][m * k:m * (k + 1)], st[i][1]

        def epi(p):
            for i, u in enumerate(us):
                u.res = [jnp.concatenate(p[n * i:n * (i + 1)], axis=0)]
        return _flat([Unit(us[0].name, [(lambda i=i, k=k: piece(i, k)) for i in range(len(us)) for k in range(n)],
                           epi, m, 0, nt=us[0].nt)])

    W = lambda nm: [("wait", nm)]
    run = lambda fns: [("run", "run", lambda: [fn(None) for fn in fns])]
    one = lambda us: [_flat([u]) for u in us]
    nm = lambda x: (lambda n: x)

    seq, grp = [], []
    for s in range(NC):
        seq += W("c%d" % s) + _flat(mmK(s) + mmU(nm("U%d" % s), s % 2, NC - 1 - s))
        grp.append(Group("kv%d" % s, cat(kv(s, s % 2)), 50, ["c%d" % s], ["U%d" % s], 100))
    inv = [mmI(lambda n: "I%d" % n, s, s) for s in range(NC)]
    seq += W("c3") + _flat(mmK(3) + mmK(4) + [inv[s][t] for t in range(NT) for s in range(NC)])
    macs = [mac(s + 1, NC - 1 - s, s) for s in range(NC)]
    grp.append(Group("mac00", macs[0][0], 12, ["c1"], ["c2"], 0))
    grp.append(Group("mac01", macs[1][0] + macs[0][1] + macs[1][1], 16, ["c2"], ["c3"], 0))
    for t in range(NT):
        grp.append(Group("mac%d" % t, cat(macs[s][t] for s in range(2 if t < 2 else 0, NC)), 24 if t < 2 else 18,
                         ["c3", "K%d" % t], ["I%d" % t], 100, 150))
    start = lambda cs: [("run", "run", lambda: [c.start() for c in cs])]
    f0, f1 = front(0, 2, True), front(1, 1, True)
    seq += run(ahead(0))
    seq += W("wma") + _flat(mod("moda", 0, 3)) + run(f0[0] + f1[0] + ahead(1))
    seq += W("wmb") + start(next_kv(NC) + next_q(NC)) + _flat(mod("modb", 3, 5)) + run(f0[1])
    w1 = _flat(mm1("w1_0", 0, 0) + mm1("w1_1", 1, 1))
    seq += W("w1") + w1[:72] + W("w2") + w1[72:] + run(shift(0, 0))
    seq += _flat(mm2("w2_0", 0, 2, 1) + mm1("w1_2", 2, 2)) + run(shift(1, 1)) + _flat(mm2("w2_1", 1, 1, 0))
    grp.append(Group("f1", f1[1], 80, ["w1"], ["w1_1"], 450))
    grp.append(Group("f2", front(2, 0), 80, ["w2"], ["w1_2"], 450))
    grp.append(Group("ln2_0", ln2(1, 0, False), 60, ["w2_0"], ["w3"], 450))
    grp.append(Group("ahead", cat(ahead(i) for i in range(2, NB - NC)), 19 + 2 * KS, ["w1"], ["end"], 100))
    grp.append(Group("ws1", wsums(w1_w, w1s, KD, ND), 26 + 5 * KS, ["w1"], ["end"], 100))
    grp.append(Group("ws2", wsums(w2_w, w2s, KD, ND), 26 + 5 * KS, ["w2"], ["end"], 100))
    grp.append(Group("ws3", w3_turn() + wsums(w3n_w, w3s, KD, KF[:6]) + wsums2(3), 22 + 5.5 * KS, ["w3"], ["end"], 100))
    grp.append(Group("ws4", wsums4(), 40 + 8 * KS, ["w4"], ["end"], 60))
    _wait(seq, "w3", back=1)
    w3 = mm3("w3_0", 0, False)
    _mix(seq, _flat(w3[6:]), [split(w3[4:6]) + _flat(w3[:6])], 0.1)
    mc = mod("modc", 5, 6)
    mc = _flat(mc[1:] + mc[:1])
    _wait(seq, "w4", mc[:5] + [("sync", "run", lambda: None)])
    w4 = cat(mm4("w4_0", 0, 0, 3, 2, 1, False)[1:])
    qs = [split([w4[-1 - i]]) for i in range(_phase(seq))]
    _mix(seq, _flat(w4), [mc[i:i + 4] for i in range(5, 25, 4)] + qs, 0.01, 0.4)
    assert _phase(seq) == 0
    grp.append(Group("resid", resid(2, 1), 16 + 5 * KS, ["modc"], ["end"], 100))
    grp.append(Group("ln2a", ln2_late(), 40, ["w3_0"], ["end"], 100))
    _emit(seq, grp, zero, wait)

    def step(s, carry):
        for c in next_kv(s) + next_q(s):
            c.wait()
        nxt = jnp.minimum(s + 1, NB - 1)
        seq, grp = [], []
        us, it = one(mmU(lambda n: "U%d" % n, 0, 0)), one(mmI(lambda n: "I%d" % n, 0, 0))
        w4, w4c = mm4("w4", s - 2, 0)[1], mm4("w4c", s - 3, 0)[0]
        w2 = mm2("w2", 0, 1, 0, True)
        w2 = w2[0:3] + w2[4:13] + w2[22:31] + w2[3:4] + w2[13:22] + w2[31:]
        for u in w2[:21]:
            u.name = "w2a"
        w2[0].name = "w2f"
        w3, w3e = mm3("w3", 0, host=w2[:4])
        _mix(seq, _flat(w4c + w3),
             [us[0], us[1], us[2], it[0] + us[3], it[1] + us[4], it[2], it[3], it[4]],
             0.159, 0.7)
        w1a, w1b = mm1("w1a", 2, 0, True), mm1("w1b", 2, 0, True)
        w1a, w1b = _flat(w1a[0:2] + w1a[4:13] + w1a[22:31]), _flat(w1b[2:4] + w1b[13:22] + w1b[31:])
        kw = 9 * 4
        w4[kw - 16].name = "w4m"
        seq += _flat(w3e + w2[4:21] + w4[:kw]) + w1a + run(shift(1, 0, ((T - 32, 32),), gs))
        seq += _flat(w4[kw:] + w2[21:]) + w1b
        assert _phase(seq) == 0
        kvs, macs = kv(0, 0), mac(1, 0, 0, part=True)
        for t in range(NT):
            grp.append(Group("kv%d" % t, kvs[t], 50 + 2 * KS, ["start"], ["U%d" % t], 260))
            grp.append(Group("mac%d" % t, macs[t], 24 + 2 * KS, ["U%d" % t], ["I%d" % t], 350, 150))
        iall = ["I%d" % t for t in range(NT)]
        ln = ln2(0, 0)
        grp.append(Group("ln2a", ln2_late(), 40, ["w2a", "w2"], ["end"], 100))
        xn = lsums2(3, n2_w, as_w[2], 0)[0]
        grp.append(Group("ln2b", ln[4:8] + ln[12:16], 78 + 20 * KS, ["start"], ["w3h"], 450))
        grp.append(Group("xna", [f for i, f in enumerate(xn) if i % 4 < 2], 26 + 5 * KS, ["start"], ["w3_0"], 150))
        grp.append(Group("xnb", [f for i, f in enumerate(xn) if i % 4 >= 2], 26 + 5 * KS, ["w4c"], ["w3_0"], 150, 0))
        grp.append(Group("resid", resid(1, 0, True), 9.5 + 5 * KS, ["w4c"], ["w2f"], 100))
        for p, ts in enumerate(lsums2(4, a_w, as_w[3], 0)):
            grp.append(Group("xa%d" % p, ts, 26 + 5 * KS, ["w3_%d" % p], ["w4q"], 150, 100))
        fr = front(0, 0, ss=n1s)
        grp.append(Group("fronta", fr[0], 50 + 8 * KS, ["w2f"], ["w1a"], 240, 0))
        grp.append(Group("frontb", fr[1], 46 + 7 * KS, ["w4m"], ["w1b"], 240, 80))
        def refill(buf, cs):
            def fn(a):
                for t in range(NT):
                    buf[t, 0:8, :] = zero if a is None else a
                for c in cs:
                    c.start()
            return fn
        fr[3].append(refill(q_n[0], next_q(nxt)))
        nk = next_kv(nxt)
        grp.append(Group("refill", [refill(k_n[0], nk[:NT]), refill(v_n[0], nk[NT:])], 10, ["U4"], ["w2f"], 0, 0))
        grp.append(Group("fq", fr[2], 33 + 7 * KS, ["w4c"], ["w2f"], 100))
        grp.append(Group("spread", spread(), 30 + 8 * KS, iall, ["end"], 60))
        grp.append(Group("shift", shift_early(), 22 + 7 * KS, ["start"], ["w2f"], 200))
        _emit(seq, grp, zero, wait)
        out_b(s - 3).wait()
        out_a(s - 2).wait()
        return carry

    lax.fori_loop(NC, NB, step, 0)

    seq, grp = [], []
    w47 = mm4("w4_7", NB - 1, 1, 2, 0, 1)
    seq += _flat(mm4("w4_5", NB - 3, 0)[0] + mm2("w2_7", 0, 0, 1, True) + mm3("w3_6", 0)
                 + cat(mm4("w4_6", NB - 2, 0, 1, 1, 0)) + mm3("w3_7", 1) + w47[0][:3] + w47[1] + w47[0][3:])
    grp.append(Group("shift7", shift(2, 0, [(r, 32) for r in range(0, T, 32)], gs), 24, ["start"], ["w2_7"], 200))
    ln = ln2(0, 0)
    grp.append(Group("ln2_6", ln[4:8] + ln[12:16], 75, ["start"], ["w3_6"], 1200))
    grp.append(Group("xn6", cat(lsums2(3, n2_w, as_w[2], 0)), 26 + 5 * KS, ["w4_5"], ["w3_6_0"], 200, 800))
    grp.append(Group("ln2_7", ln2(1, 1), 75, ["w4_6"], ["w3_7"], 1500))
    grp.append(Group("xn7", cat(lsums2(3, n2_w, as_w[2], 1)), 26 + 5 * KS, ["w4_6"], ["w3_7_0"], 200, 2100))
    for j in (6, 7):
        for p, ts in enumerate(lsums2(4, a_w, as_w[3], j - 6)):
            grp.append(Group("xa%d_%d" % (j, p), ts, 26 + 5 * KS, ["w3_%d_%d" % (j, p)], ["w4_%dq" % j], 200, 150))
    _emit(seq, grp, zero, wait)
    for c in next_kv(NB - 1) + next_q(NB - 1) + [out_b(NB - 3)] + last:
        c.wait()


@jax.jit
def pallas_adaLN_cond__ssm_conv_h3__mixer_s_mlp__prompt_kernel(
        A_q, A_k, A_v, A_shift_k, A_ssm_k, A_ssm_D, B_x, B_w1, B_w2, B_w3, B_w4, c, w_mod):
    any_ = pl.BlockSpec(memory_space=pl.ANY)
    V = pltpu.VMEM
    out = pl.pallas_call(
        kernel,
        in_specs=[any_] * 12,
        out_specs=any_,
        out_shape=jax.ShapeDtypeStruct((S, D), BF16),
        scratch_shapes=[
            [V((NT, H + 8, 128), U32)] * NC, [V((NT, H + 8, 128), U32)] * NC, [V((NT, H + 8, 128), U32)] * NC,
            [V((64, S), U32)] * NT,
            V((D // 2, D), U32), V((D // 2, D), U32), V((F // 2, D), U32), V((FT * 64, D), U32),
            [V((D // 2, 3 * D), U32), V((D // 2, 2 * D), U32), V((D // 2, D), U32)], V((4 * T, D), BF16),
            V((4, D), BF16), V((D,), BF16), V((1, D), BF16), V((8, 128), I32), pltpu.SMEM((8, 128), I32),
            V((5, 8, D), F32), V((6, 8, D), F32), V((T // 2, 4 * H), U32), V((GR // 2, 2 * T), U32),
            V((NB, 3 * T + 8, D), F32), V((NC, 3 * T + 8, D), F32), V((NB - NC, 2 * T + 8, D), F32), V((4 * T, 128), F32),
            V((T, D), U32), V((NC * T, D), U32), V((NT, NC * (T + 8) + 16, 128), F32),
            V((3 * T, D), F32), V((3 * T, D), F32), V((2 * T, D), F32), V((T, D), F32),
            V((3 * T // 2, D), U32), V((T, D), U32), V((T, D), U32), V((NT, NC * T + 24, 128), F32),
            V((T, (FT + 1) * 128), U32),
            [V((128, 11 * 128), U32)] * 2 + [V((128, 31 * 128), U32), V((448, 11 * 128), U32)],
            [V((64, 11 * 128), U32)] * 2 + [V((128, 11 * 128), U32), V((128, 35 * 128), U32)],
            V((D // 2, 13 * 128), U32), V((H, D), F32), V((T, 9 * 128), F32),
            [V((64, 105 * 128), U32), V((192, 35 * 128), U32), V((32, 35 * 128), U32), V((32, 105 * 128), U32)], V((H, 33 * 128), F32),
            pltpu.SemaphoreType.DMA((11,)), pltpu.SemaphoreType.DMA((1,)), pltpu.SemaphoreType.DMA((3,)),
        ],
        compiler_params=pltpu.CompilerParams(vmem_limit_bytes=110 << 20, disable_semaphore_checks=True,
                                             disable_bounds_checks=True),
        name="fused",
    )(A_q[0], A_k[0], A_v[0], A_shift_k.T, A_ssm_k, A_ssm_D, B_w1, B_w2, B_w3.T, B_w4, c, w_mod)
    return out[None]
```

```python
import heapq
import numpy as np
import jax
import jax.numpy as jnp
from jax import lax
from jax.experimental import pallas as pl
from jax.experimental.pallas import tpu as pltpu

S, D, F = 2048, 640, 1728
T = 256
H = T // 2
NB = S // T
NT = D // 128
FT = (F + 127) // 128
EPS = 1e-5
F32, BF16, U32, I32 = jnp.float32, jnp.bfloat16, jnp.uint32, jnp.int32
G_C1 = 0.044715 * float(np.sqrt(2.0 / np.pi))
G_C2 = float(np.sqrt(2.0 / np.pi))
G_A = G_C1 ** (1.0 / 3.0)
G_B = G_C2 / G_A
G_POST = 0.5 / G_A
RG = 16
GR = 80
NC = 3
DL = 450
KS = 1.66
SLOT = 32


def _dft(shape, f_axis, tau, scale=1.0):
    r = lax.broadcasted_iota(I32, shape, f_axis)
    l = lax.broadcasted_iota(I32, shape, 1 - f_axis)
    f = r & 127
    odd = ((f & 63) << 2) | ((f >> 6) << 1) | 1
    p = odd * tau(l) + ((r >> 7) << 8)
    a = ((p + 512) & 1023) - 512
    u = (256 - jnp.abs(a)).astype(F32) * (np.pi / 512.0)
    u2 = u * u
    c = [scale, -scale / 6.0, scale / 120.0, -scale / 5040.0, scale / 362880.0, -scale / 39916800.0]
    poly = c[5]
    for ci in c[4::-1]:
        poly = poly * u2 + ci
    return (u * poly).astype(BF16)


def _rstd(xc, mlp):
    s2, eps = (1.0 / (G_A * G_A), EPS / (G_POST * G_POST)) if mlp else (1.0, EPS)
    v = jnp.sum(xc * xc, axis=-1, keepdims=True) * (s2 / D) + eps * s2
    return jnp.exp2(jnp.log(v) * float(-0.5 / np.log(2.0)))


def _ln(x, mlp=False):
    xc = x - jnp.sum(x, axis=-1, keepdims=True) * (1.0 / D)
    return xc * _rstd(xc, mlp)


def _gelu2(x):
    u = x * (x * x + G_B)
    return x * (1.0 + jnp.tanh(u))


def _lo(w):
    return pltpu.bitcast(w << 16, F32)


def _hi(w):
    return pltpu.bitcast(w & jnp.uint32(0xFFFF0000), F32)


def _tie(x, a):
    if a is None:
        return x
    w = pltpu.bitcast(x[:, :128], U32)
    k = w.shape[0] // 8
    w = w | (a if k == 1 else jnp.concatenate([a] * k, axis=0))
    w = pltpu.bitcast(w, x.dtype)
    return w if x.shape[1] == 128 else jnp.concatenate([w, x[:, 128:]], axis=1)


def _top(x, i):
    return jnp.concatenate([x[r:r + 16] for r in range(16 * i, x.shape[0], 32)], axis=0)


def _zip(t, b):
    return jnp.concatenate([x[r:r + 16] for r in range(0, t.shape[0], 16) for x in (t, b)], axis=0)


def _lhs_sums(x1, x2):
    a11, a21, a12, a22 = _top(x1, 0), _top(x1, 1), _top(x2, 0), _top(x2, 1)
    return [a11 + a22, a21 + a22, a11 + a12, a21 - a11, a12 - a22]


def C(i):
    return slice(i * 128, (i + 1) * 128)


class Unit:
    def __init__(self, name, tiles, epi, rows, cost, nt=False, full=True, acc=False, tail=0):
        self.tail = tail
        self.acc, self.res = acc, []
        self.name, self.tiles, self.epi, self.rows, self.cost, self.nt, self.full = name, tiles, epi, rows, cost, nt, full


class Due:
    def __init__(self, val, delay):
        self.val, self.delay = val, delay


class Group:
    def __init__(self, name, fns, cost, rel, dead, lat, rlat=200):
        self.name, self.fns, self.cost, self.rel, self.dead, self.lat, self.rlat = name, fns, cost, rel, dead, lat, rlat


def _plan(seq, groups):
    busy, n = [0] * 4, 0
    start, end, tiles, bars = {}, {}, [], []
    for it in seq:
        if isinstance(it[0], Unit):
            u = it[0]
            m = n % 4
            n += 1
            t0, t1 = busy[m], busy[m] + max(u.rows, 32)
            busy[m] = t1
            tiles.append((t0, t1, u.cost / len(u.tiles) + (u.tail if it[1] == len(u.tiles) - 1 else 0)))
            start.setdefault(u.name, t0)
            end[u.name] = max(end.get(u.name, 0), t1)
        elif it[0] == "wait":
            t = max(busy)
            busy, n = [t] * 4, 0
            start[it[1]] = end[it[1]] = t
            bars.append(t)
    total = max(busy)
    start["end"] = end["end"] = total
    start["start"] = end["start"] = 0
    ns = total // SLOT + 2
    load = np.zeros(ns)
    for t0, t1, c in tiles:
        a, b = t0 // SLOT, max(t1 // SLOT, t0 // SLOT + 1)
        load[a:b] += c / (b - a)
    win = []
    for g in groups:
        r = max(end[x] + (0 if start[x] == end[x] else g.rlat) for x in g.rel)
        d = min(start[x] for x in g.dead) - g.lat
        ok = np.zeros(ns, bool)
        ok[r // SLOT:max(d // SLOT, r // SLOT + 1)] = True
        for b in bars:
            if r < b <= d:
                ok[max((b - g.lat) // SLOT, 0):b // SLOT] = False
        win.append(np.nonzero(ok)[0])
    alloc = [np.zeros(len(w)) for w in win]
    for _ in range(60):
        for i, g in enumerate(groups):
            w = win[i]
            load[w] -= alloc[i]
            base = load[w]
            vol = g.cost * len(g.fns)
            lo, hi = base.min(), base.max() + vol
            for _ in range(50):
                mid = 0.5 * (lo + hi)
                if np.maximum(mid - base, 0).sum() > vol:
                    hi = mid
                else:
                    lo = mid
            alloc[i] = np.maximum(hi - base, 0)
            load[w] += alloc[i]
    times = []
    for i, g in enumerate(groups):
        cum = np.cumsum(alloc[i])
        ts = []
        for k in range(len(g.fns)):
            x = (k + 0.5) * cum[-1] / len(g.fns)
            j = int(np.searchsorted(cum, x))
            prev = cum[j - 1] if j else 0.0
            ts.append(win[i][j] * SLOT + SLOT * (x - prev) / max(alloc[i][j], 1e-9))
        times.append(ts)
    return times


def _emit(seq, groups, zero, wait):
    times = _plan(seq, groups)
    left = {"start": 0}
    for it in seq:
        nm = it[0].name if isinstance(it[0], Unit) else it[1]
        left[nm] = left.get(nm, 0) + 1
    heap, pend, todo, cnt = [], {}, list(range(len(groups))), 0
    busy, n, due = [0] * 4, 0, []

    def release():
        nonlocal cnt
        for i in list(todo):
            g = groups[i]
            if all(left[x] == 0 for x in g.rel):
                todo.remove(i)
                pend[i] = len(g.fns)
                for t, fn in zip(times[i], g.fns):
                    heapq.heappush(heap, (t, cnt, i, fn))
                    cnt += 1

    def force(name):
        nonlocal heap
        for i, g in enumerate(groups):
            if name in g.dead:
                assert i not in todo, (g.name, name)
                if pend[i]:
                    for it in sorted(x for x in heap if x[2] == i):
                        it[3](None)
                    heap = [x for x in heap if x[2] != i]
                    heapq.heapify(heap)
                    pend[i] = 0

    release()
    for it in seq:
        if isinstance(it[0], Unit):
            u, k = it
            force(u.name)
            lhs, rhs = u.tiles[k]()
            t0 = busy[n % 4]
            while u.full and due and due[0][0] < t0 + u.rows:
                t, x = due.pop(0)
                r = min(max(int(t - t0), 0), u.rows - 1) // 16 * 8
                w = pltpu.bitcast(lhs, U32)
                x = pltpu.bitcast(x[:, :128], U32)
                parts = [w[:r], w[r:r + 8] | ((x[0:8] | x[8:16]) & zero), w[r + 8:]]
                lhs = pltpu.bitcast(jnp.concatenate([y for y in parts if y.shape[0]], axis=0), BF16)
            dn = (((1,), (1 if u.nt else 0,)), ((), ()))
            p = lax.dot_general(lhs, rhs, dn, preferred_element_type=F32)
            u.res = [p + u.res[0]] if (u.acc and u.res) else u.res + [p]
            m = n % 4
            n += 1
            t0 = busy[m]
            busy[m] = t0 + max(u.rows, 32)
            used = -8
            while u.full and heap and heap[0][0] < t0 + u.rows:
                r = min(max(int(heap[0][0] - t0), 0), u.rows - 1) // 8 * 8
                r = max(r, used + 8)
                if r >= u.rows or r > max(heap[0][0] - t0, 8) + 8:
                    break
                used = r
                t, _, i, fn = heapq.heappop(heap)
                pend[i] -= 1
                x = fn(pltpu.bitcast(p[r:r + 8], U32) & zero)
                if isinstance(x, Due):
                    due.append((t + x.delay, x.val))
                    due.sort(key=lambda e: e[0])
            if k == len(u.tiles) - 1:
                u.epi(u.res)
            left[u.name] -= 1
        elif it[0] == "wait":
            force(it[1])
            wait(it[1])
            busy, n, due = [max(busy)] * 4, 0, []
            left[it[1]] -= 1
        else:
            it[2]()
            left[it[1]] -= 1
        release()
    force("end")
    assert not heap and not todo


def _sum(ps):
    acc = ps[0]
    for p in ps[1:]:
        acc = acc + p
    return acc


def _flat(us):
    return [(u, i) for u in us for i in range(len(u.tiles))]


def _weave(a, b):
    out = []
    for i, u in enumerate(a):
        out += [u] + b[i * len(b) // len(a):(i + 1) * len(b) // len(a)]
    return out


def _phase(seq):
    n = 0
    for it in seq:
        n = n + 1 if isinstance(it[0], Unit) else (0 if it[0] in ("wait", "sync") else n)
    return n % 4


def _mix(seq, a, b, lo=0.0, hi=1.0):
    n, k = _phase(seq), 0
    for i, t in enumerate(a):
        if k < len(b) and n % 4 == 0 and t[1] != 1 and i >= len(a) * (lo + (hi - lo) * k / len(b)):
            seq.extend(b[k])
            k += 1
        seq.append(t)
        n += 1
    assert k == len(b)


def _wait(seq, name, head=(), back=0):
    r = _phase(seq) + 4 * back
    assert all(isinstance(it[0], Unit) for it in seq[len(seq) - r:])
    seq[len(seq) - r:len(seq) - r] = [("wait", name)] + list(head)


def kernel(q_hbm, k_hbm, v_hbm, sh_hbm, ssm_hbm, sd_hbm, w1_hbm, w2_hbm, w3_hbm, w4_hbm, c_hbm, wm_hbm,
           o_hbm,
           q_n, k_n, v_n, ssm_w, w1_w, w2_w, w3_w, w4_w, wm_w, o_v,
           sh_v, sd_v, c_v, zsrc, z_s, taps, mod_v, tf_w, tg_w,
           kf, uf, acc, zraw, kv_w, zz_w, y_v, x_v, hb_v, x1_v, r_v, n1_w, n2_w, g_w, h1_v, a_w,
           ws_w, as_w, w3n_w, top_v, st_v, l2_w, cb_v,
           sem, sem_b, sem_o):
    bf = lambda r: r.bitcast(BF16)
    w1_v, w2_v, w3_v, w4_v = bf(w1_w), bf(w2_w), bf(w3_w), bf(w4_w)
    wm_v = {0: bf(wm_w[0]), 3: bf(wm_w[1]), 5: bf(wm_w[2])}
    tf_v, tg_v, n1_v, n2_v, g_v = bf(tf_w), bf(tg_w), bf(n1_w), bf(n2_w), bf(g_w)
    a_v, kv_v, zz_v = bf(a_w), bf(kv_w), bf(zz_w)
    w1s, w2s, w3s, w4s = [bf(r) for r in ws_w]
    n1s, gs, n2s, a_s = [bf(r) for r in as_w]
    w3n = bf(w3n_w)
    w3t, w4t, n2t, a_t = [bf(r) for r in l2_w]
    cp = pltpu.make_async_copy
    cat = lambda ls: [x for l in ls for x in l]

    def base(j, n):
        return j * n if isinstance(j, int) else pl.multiple_of(j * n, n)

    def rows(j, n=1, size=T):
        return pl.ds(base(j, size), n * size)

    def view(ref, j, size=T):
        return ref.at[rows(j, 1, size)]

    dmas = {}

    def group(name, *mks):
        sm = sem.at[len(dmas)]
        dmas[name] = [c for mk in mks for c in mk(sm)]

    def ssm_in(t):
        return lambda sm: [cp(ssm_hbm.at[C(t)], bf(ssm_w[t]), sm)]

    def cols(src, start, n, dst, row=0):
        return lambda sm: [cp(src.at[pl.ds(start, n), C(t)], bf(dst).at[t, pl.ds(row, n)], sm) for t in range(NT)]

    def kv_in(s, sl):
        if isinstance(s, int):
            kk = cols(k_hbm, s * T - 16, T + 16, k_n[sl]) if s else cols(k_hbm, 0, T, k_n[sl], 16)
        else:
            kk = cols(k_hbm, pl.multiple_of(s * T - 16, 16), T + 16, k_n[sl])
        return lambda sm: kk(sm) + cols(v_hbm, base(s, T), T, v_n[sl])(sm)

    def q_in(s, sl):
        return cols(q_hbm, base(s, T), T, q_n[sl])

    def wm_in(a, b):
        return lambda sm: [cp(wm_hbm.at[:, a * D:b * D], wm_v[a], sm)]

    def whole(src, dst):
        return lambda sm: [cp(src, dst, sm)]

    next_kv = lambda s: kv_in(s, 0)(sem_b.at[0])
    next_q = lambda s: q_in(s, 0)(sem_b.at[0])

    zsrc[...] = jnp.zeros((8, 128), I32)
    k_n[0][:, 0:8, :] = jnp.zeros((NT, 8, 128), U32)
    w4_w[F // 2:FT * 64, :] = jnp.zeros((FT * 64 - F // 2, D), U32)
    group("small", lambda sm: [cp(zsrc, z_s, sm), cp(sh_hbm, sh_v, sm), cp(sd_hbm, sd_v, sm), cp(c_hbm, c_v, sm)])
    for s in range(NC):
        group("c%d" % s, ssm_in(s), kv_in(s, s))
    group("c3", ssm_in(3), ssm_in(4))
    group("wma", wm_in(0, 3), q_in(0, 0), q_in(1, 1))
    group("wmb", wm_in(3, 5))
    group("w1", whole(w1_hbm, w1_v))
    group("w2", q_in(2, 2), whole(w2_hbm, w2_v))
    group("w3", whole(w3_hbm, w3_v))
    group("w4", whole(w4_hbm, w4_v.at[0:F]), wm_in(5, 6))
    for g in dmas.values():
        for c in g:
            c.start()

    def wait(name):
        for c in dmas[name]:
            c.wait()

    tau_b = lambda l: H + ((l + (H - 1)) & (H - 1))
    tf_v[:, C(0)] = _dft((T, H), 0, lambda l: jnp.where((l & 1) == 0, l, tau_b(l)), 1.0 / T)
    tf_v[:, C(1)] = _dft((T, H), 0, lambda l: jnp.where((l & 1) == 1, l, tau_b(l)), 1.0 / T)
    tf_v[:, C(2)] = _dft((T, H), 0, lambda l: 2 * l - H)
    tf_v[:, C(3)] = _dft((T, H), 0, lambda l: 2 * l + 1 - H)
    sin0 = lax.broadcasted_iota(I32, (GR, T), 1) >= H
    tg_v[:, 0:T] = _dft((GR, T), 1, lambda l: jnp.where(sin0 & (l == 0), H, 2 * l))
    tg_v[:, T:2 * T] = _dft((GR, T), 1, lambda l: 2 * l + 1)
    h1_v[:, 0:8, :] = jnp.zeros((NT, 8, 128), F32)
    h1_v[:, 8 + NC * T:16 + NC * T, :] = jnp.zeros((NT, 8, 128), F32)

    wait("small")
    z = jnp.clip(z_s[0, 0], 0, 1)
    zero = jnp.full((8, 128), z, I32).astype(U32)
    z8 = pl.multiple_of(z * 8, 8)
    for r in (x_v, hb_v, x1_v, r_v, zraw, n1_w, n2_w, g_w, a_w, kv_w, zz_w, *ws_w, *as_w, w3n_w, top_v, st_v, *l2_w, cb_v):
        r[pl.ds(z8, 8), 0:128] = jnp.zeros((8, 128), r.dtype)
    for r in (kf, uf, acc, taps, mod_v):
        r[z, 0:8, 0:128] = jnp.zeros((8, 128), r.dtype)
    for r in (tf_w, tg_w):
        r[pl.ds(z8, 8), 0:128] = r[0:8, 0:128]
    sh = sh_v[...].astype(F32)
    for i in range(4):
        taps[i] = jnp.broadcast_to(sh[i:i + 1], (8, D))
    taps[4] = jnp.broadcast_to(sd_v[...].astype(F32).reshape(1, D) * (1.0 / T), (8, D))
    cf = c_v[...].astype(F32)
    silu_c = jnp.broadcast_to((cf / (1.0 + jnp.exp(-cf))).astype(BF16), (16, D))

    def mmK(n):
        def unit(m):
            st = []

            def rhs(i):
                if not st:
                    ev = (lax.broadcasted_iota(I32, (64, 128), 1) & 1) == 0
                    a = ssm_w[n][:, m * T:m * T + H]
                    b = pltpu.roll(ssm_w[n][:, m * T + H:(m + 1) * T], 1, 1)
                    st.extend([pltpu.bitcast(jnp.where(ev, a, b), BF16), pltpu.bitcast(jnp.where(ev, b, a), BF16)])
                return st[i]

            def epi(p):
                er, ei, or_, oi = p
                cur = [er, ei, or_, oi]
                if m:
                    pv = [zraw[C(4 * ((m - 1) % 2) + (q ^ 1)), :] for q in range(4)]
                    pm = lambda x, y, up: jnp.concatenate([x[:64] + y[:64], x[64:] - y[64:]] if up else
                                                          [x[:64] - y[:64], x[64:] + y[64:]], axis=0)
                    er, ei, or_, oi = [pm(cur[q], pv[q], q & 1) for q in range(4)]
                else:
                    er = er + taps[4, 0:1, C(n)]
                if m + 1 < NB:
                    for q in range(4):
                        zraw[C(4 * (m % 2) + q), :] = cur[q]
                for h, (cr, ci) in enumerate(((er + or_, ei + oi), (er - or_, ei - oi))):
                    B = h * 3 * H
                    kf[m, B:B + H, C(n)] = cr
                    kf[m, B + H:B + 2 * H, C(n)] = ci - cr
                    kf[m, B + 2 * H:B + 3 * H, C(n)] = ci + cr
            return Unit("K%d" % n, [(lambda i=i, r=r: (tf_v[r:r + H, C(i)], rhs(i))) for i in range(2) for r in (0, H)],
                        epi, H, 260, nt=True)
        return [unit(m) for m in range(NB)]

    def kv(s, sl):
        def mk(t, w):
            def fn(a):
                ld = lambda o, n: k_n[s][t, pl.ds(8 + w + o, n), :]
                c0 = jnp.concatenate([_tie(ld(0, 8), a), ld(8, 8)], axis=0).reshape(2, 8, 128)
                c1, c2 = ld(-1, 16).reshape(2, 8, 128), ld(-2, 16).reshape(2, 8, 128)
                s0, s1, s2, s3 = (taps[i, :, C(t)] for i in range(4))
                ke, ko, ke1, ko1, ko2 = _lo(c0), _hi(c0), _lo(c1), _hi(c1), _hi(c2)
                wv = v_n[s][t, w:w + 16, :].reshape(2, 8, 128)
                kve = ((s0 * ke + s1 * ko1) + (s2 * ke1 + s3 * ko2)) * _lo(wv)
                kvo = ((s0 * ko + s1 * ke) + (s2 * ko1 + s3 * ke1)) * _hi(wv)
                kv_v[pl.ds(sl * T + w, 16), C(t)] = kve.reshape(16, 128).astype(BF16)
                kv_v[pl.ds(sl * T + H + w, 16), C(t)] = kvo.reshape(16, 128).astype(BF16)
            return fn
        return [[mk(t, w) for w in range(0, H, 16)] for t in range(NT)]

    def mmU(name, sl, us):
        def unit(n):
            def epi(p):
                er, ei, or_, oi = p
                for h, (cr, ci) in enumerate(((er + or_, ei + oi), (er - or_, ei - oi))):
                    B = h * 3 * H
                    uf[us, B:B + H, C(n)] = cr + ci
                    uf[us, B + H:B + 2 * H, C(n)] = cr
                    uf[us, B + 2 * H:B + 3 * H, C(n)] = ci
            return Unit(name(n), [(lambda i=i, r=r: (tf_v[r:r + H, C(2 + i)], kv_v[pl.ds(sl * T + i * H, H), C(n)]))
                                  for i in range(2) for r in (0, H)], epi, H, 96 + 96 * KS)
        return [unit(n) for n in range(NT)]

    def cmul(m0, u0, n, h, row, L, a):
        t = []
        for i in range(3):
            Rw = slice((3 * h + i) * H + row, (3 * h + i) * H + row + 8)
            kk = kf[m0:m0 + n, Rw, L]
            if i == 0 and a is not None:
                k0 = _tie(kk[0], a)[None]
                kk = k0 if n == 1 else jnp.concatenate([k0, kk[1:]], axis=0)
            t.append(jnp.sum(kk * uf[u0:u0 + n, Rw, L], axis=0))
        return t[0] - t[2], t[0] + t[1]

    def AR(h, q, row):
        return slice((2 * h + q) * H + row, (2 * h + q) * H + row + 8)

    def mac(n, u0, sl, part=False):
        def mk(t, rc):
            st, fin = [], []

            def piece(i):
                def fn(a):
                    h, row = i & 1, rc + (i >> 1) * 8
                    zr, zi = cmul(0, u0, n, h, row, C(t), a)
                    if part:
                        zr, zi = zr + acc[0, AR(h, 0, row), C(t)], zi + acc[0, AR(h, 1, row), C(t)]
                    st.append((zr, zi))
                    if h:
                        (pr, pi), (mr, mi) = st[-2:]
                        fin.append([pr + mr, pi + mi, pr - mr, pi - mi])
                    if i == 3:
                        for q in range(4):
                            zz_v[pl.ds(sl * 2 * T + q * H + rc, 16), C(t)] = jnp.concatenate(
                                [fin[0][q], fin[1][q]], axis=0).astype(BF16)
                return fn
            if not part:
                return [piece(i) for i in range(4)]
            both = lambda f, g: (lambda a: (f(a), g(None)))
            return [both(piece(0), piece(1)), both(piece(2), piece(3))]
        return [[fn for rc in range(0, H, 16) for fn in mk(t, rc)] for t in range(NT)]

    def pos():
        return [(t, h, row) for t in range(NT) for row in range(0, H, 8) for h in range(2)]

    def ahead(i):
        def mk(t, h, row):
            def fn(a):
                zr, zi = cmul(i + 1, 0, NC, h, row, C(t), a)
                acc[i, AR(h, 0, row), C(t)] = zr
                acc[i, AR(h, 1, row), C(t)] = zi
            return fn
        return [mk(*p) for p in pos()]

    def spread():
        n = NB - NC - 1

        def mk(t, h, row):
            def fn(a):
                p = []
                for i in range(3):
                    Rw = slice((3 * h + i) * H + row, (3 * h + i) * H + row + 8)
                    u = uf[0, Rw, C(t)]
                    p.append(kf[1:1 + n, Rw, C(t)] * (_tie(u, a) if i == 0 else u)[None])
                acc[0:n, AR(h, 0, row), C(t)] = acc[1:1 + n, AR(h, 0, row), C(t)] + (p[0] - p[2])
                acc[0:n, AR(h, 1, row), C(t)] = acc[1:1 + n, AR(h, 1, row), C(t)] + (p[0] + p[1])
            return fn
        return [mk(*p) for p in pos()]

    def mmI(name, sl, ys):
        def unit(n):
            def epi(p):
                ce, se, co, so = p
                sub = lax.broadcasted_iota(I32, (8, 128), 0)
                b0 = ys * (T + 8) + 8
                y_v[n, b0 + H - 1:b0 + H, :] = (ce[64:72] - se[0:8])[0:1]
                se = jnp.concatenate([jnp.where(sub == 0, 0.0, se[0:8]), se[8:]], axis=0)
                for d, cc, ss in ((0, ce[0:64], se), (1, co, so)):
                    y_v[n, pl.ds(b0 + H + d, 64, stride=2), :] = cc + ss
                    y_v[n, pl.ds(b0 + d - 1, 64, stride=2), :] = cc - ss
            return Unit(name(n), [(lambda i=i: (tg_v[0:(GR if i == 0 else 64), C(i)], zz_v[pl.ds(sl * 2 * T + i * H, H), C(n)]))
                                  for i in range(4)], epi, 64, 36 + 33 * KS)
        return [unit(n) for n in range(NT)]

    def mod(name, a, b):
        def unit(n):
            def epi(p):
                v = [_sum(p[i * NT:(i + 1) * NT])[0:8] for i in range(b - a)]
                if a == 0:
                    mod_v[0, :, C(n)] = v[0] * v[2]
                    mod_v[1, :, C(n)] = (v[1] + 1.0) * v[2]
                elif a == 3:
                    mod_v[3, :, C(n)] = v[0] * (1.0 / G_POST)
                    mod_v[4, :, C(n)] = (v[1] + 1.0) * (1.0 / G_POST)
                else:
                    mod_v[2, :, C(n)] = v[0] * G_POST
            return Unit(name, [(lambda i=i, k=k: (silu_c[:, C(k)], wm_v[a][C(k), pl.ds(i * D + n * 128, 128)]))
                               for i in range(b - a) for k in range(NT)], epi, 16, 10, full=False, acc=b - a == 1)
        return [unit(n) for n in range(NT)]

    HS = (slice(0, 128), slice(128, 256))
    QS = tuple(slice(r, r + 64) for r in range(0, T, 64))

    def tasks(f, due=None, tie=True, n=RG):
        def mk(R):
            def fn(a):
                x = f(R, a if tie else None)
                return Due(x, due) if due else None
            return fn
        return [mk(slice(r, r + n)) for r in range(0, T, n)]

    def load_y(sl, R):
        b0, back = sl * (T + 8) + 8, 7 - lax.broadcasted_iota(I32, (8, 128), 0)

        def ld(t, r):
            if r >= H:
                return y_v[t, b0 + r:b0 + r + 8, :]
            return jnp.take_along_axis(y_v[t, b0 + H - 8 - r:b0 + H - r, :], back, axis=0)
        return jnp.stack([jnp.concatenate([ld(t, r) for t in range(NT)], axis=1) for r in range(R.start, R.stop, 8)])

    def put(nn, ss, R, x):
        nn[R, :] = x.astype(BF16)
        tok = x
        if ss is not None:
            S2 = pl.ds(R.start // 32 * 16, 16)
            if R.stop % 32:
                top_v[S2, 0:2 * T] = x[:, 0:2 * T]
            else:
                if R.start % 32:
                    x = jnp.concatenate([top_v[S2, 0:2 * T], x[:, 0:2 * T]], axis=0)
                ss[S2, 0:5 * T] = jnp.concatenate(_lhs_sums(x[:, 0:T], x[:, T:2 * T]), axis=1).astype(BF16)
        return tok

    wide = lambda v: jnp.concatenate([v] * NT, axis=1)

    def mean(i, R, x):
        st_v[R, C(i)] = jnp.broadcast_to(jnp.sum(x, axis=-1, keepdims=True) * (1.0 / D), (x.shape[0], 128))

    def centred(src, i, R, a):
        return src[R, :] - wide(_tie(st_v[R, C(i)], a))

    def scale(src, i, g):
        def f(R, a):
            st_v[R, C(i + 1)] = jnp.broadcast_to(_rstd(centred(src, i, R, a), g), (RG, 128))
        return f

    def normed(src, i, R, a):
        return centred(src, i, R, a) * wide(st_v[R, C(i + 1)])

    def finish(src, i, nn, ss):
        def mk(r, ts):
            def fn(a):
                R = slice(r, r + 32)
                m, g = _tie(st_v[R, C(i)], a), st_v[R, C(i + 1)]
                x = [(src[R, C(t)] - m) * g for t in ts]
                for t, v in zip(ts, x):
                    nn[R, C(t)] = v.astype(BF16)
                for k, v in enumerate(_lhs_sums(*x[:2])):
                    ss[pl.ds(r // 2, 16), C(2 * k + ts[0])] = v.astype(BF16)
            return fn
        return [mk(r, ts) for r in range(0, T, 32) for ts in ((0, 2, 4), (1, 3))]

    def front(sl, xs, early=False, ss=None):
        xx, hh, nn = view(x_v, xs), view(hb_v, xs), view(n1_v, sl)

        def fa(R, a):
            q = [q_n[sl][t, R.start // 2:R.stop // 2, :] for t in range(NT)]
            q = jnp.concatenate([_tie(q[0], a)] + q[1:], axis=1)
            q = pltpu.bitcast(q, BF16).astype(F32).reshape(2, 8, D)
            x = (q + (_ln(q) * mod_v[1] + mod_v[0]) * load_y(sl, R)).reshape(RG, D)
            xx[R, :] = x
            if early:
                hh[R, :] = _ln(x)

        def fb(R, a):
            hh[R, :] = (_ln(_tie(xx[R, :], a).reshape(2, 8, D)) * mod_v[4] + mod_v[3]).reshape(RG, D)

        def fc(R, a):
            hb = _tie(hh[R, :], a)
            if early:
                hb = (hb.reshape(2, 8, D) * mod_v[4] + mod_v[3]).reshape(RG, D)
                hh[R, :] = hb
            nn[R, :] = _ln(hb, True).astype(BF16)
        if early:
            return tasks(fa), tasks(fc)
        if ss is None:
            return tasks(fa) + tasks(fb) + tasks(fc)
        qf = view(x_v, 2)

        def s1(R, a):
            q = [q_n[sl][t, R.start // 2:R.stop // 2, :] for t in range(NT)]
            q = pltpu.bitcast(jnp.concatenate([_tie(v, a) for v in q], axis=1), BF16).astype(F32)
            qf[R, :] = q
            mean(0, R, q)

        def s3(R, a):
            h = normed(qf, 0, R, a).reshape(-1, 8, D) * mod_v[1] + mod_v[0]
            x = qf[R, :] + (h * load_y(sl, R)).reshape(-1, D)
            xx[R, :] = x
            mean(2, R, x)

        def s5(R, a):
            hb = (normed(xx, 2, R, a).reshape(-1, 8, D) * mod_v[4] + mod_v[3]).reshape(-1, D)
            hh[R, :] = hb
            mean(4, R, hb)
        s7 = finish(hh, 4, nn, ss)
        one_ = lambda ts: [(t,) for t in ts]
        st = [list(zip(*[iter(tasks(s3, n=8))] * 2)), one_(tasks(scale(xx, 2, False))), one_(tasks(s5)),
              one_(tasks(scale(hh, 4, True))), one_(s7)]
        p = [one_(tasks(s1)), one_(tasks(scale(qf, 0, False)))]
        sk = 4.24

        def wave(ls):
            body = sorted((i * sk + g, i, g) for i in range(len(ls) - 1) for g in range(8))
            return cat([ls[i][g] for _, i, g in body] + ls[-1])
        qb = []
        done = lambda a: qb[0](a)
        full = wave([x[8:] for x in p + st])
        k = full.index(p[0][15][0]) + 1
        return wave([x[:8] for x in st]), full[:k] + [done] + full[k:], cat(cat(x[:8] for x in p)), qb

    def shift(hs, sl, pieces=((0, 64), (64, 64), (128, 64), (192, 64)), ss=None):
        gg = view(g_v, sl)

        def one_tile(t, r, n, a):
            lane = lax.broadcasted_iota(I32, (n, 128), 1)
            ld = lambda d: h1_v[t, pl.ds(hs * T + 8 + r + d, n), :]
            if t == 0:
                g = ld(-1)
            elif t == 1:
                g = jnp.where(lane < 32, ld(-1), ld(1))
            elif t == 2:
                g = jnp.where(lane < 64, ld(1), ld(-2))
            elif t == 3:
                g = jnp.where(lane < 96, ld(-2), ld(2))
            else:
                g = ld(2)
            if a is not None:
                g = jnp.concatenate([_tie(g[i:i + 8], a) if i % 16 == 0 else g[i:i + 8]
                                     for i in range(0, n, 8)], axis=0)
            gg[r:r + n, C(t)] = g.astype(BF16)
            return g

        def mk(ts, r, n):
            def fn(a):
                g = [one_tile(t, r, n, a) for t in ts]
                if len(ts) == 2:
                    for i, x in enumerate(_lhs_sums(*g)):
                        ss[r // 2:(r + n) // 2, C(2 * i + ts[0])] = x.astype(BF16)
            return fn
        sets = [(t,) for t in range(NT)] if ss is None else [(0, 2), (1, 3), (4,)]
        return [mk(ts, r, n) for ts in sets for r, n in pieces]

    def shift_early():
        def keep(a):
            h1_v[:, 2 * T - 32:2 * T + 8, :] = h1_v[:, 3 * T - 32:3 * T + 8, :]
        return shift(2, 0, [(r, 32) for r in range(0, T - 32, 32)], gs) + [keep]

    def ln2(xs, sl, fast=True):
        xx, nn, ss = view(x1_v, xs), view(n2_v, sl), view(n2s, sl, H) if fast else None
        f = lambda R, a: put(nn, ss, R, _ln(_tie(xx[R, :], a), True))
        ts = tasks(f, 900) if sl else tasks(f, DL, False)
        return ts[0::2] + ts[1::2] if fast else tasks(f)

    def ln2_late(h=0):
        xx, nn, ss = view(x1_v, 0), view(n2_v, 0), view(n2s, 0, H)
        a_, b_ = tasks(lambda R, a: mean(6, R, _tie(xx[R, :], a))), tasks(scale(xx, 6, True))
        c_ = finish(xx, 6, nn, ss)
        return cat(x[8 * h:8 * h + 8] for x in (a_, b_, c_))

    def resid(xs, x1s, rotate=False):
        xx, x1 = view(x_v, xs), view(x1_v, x1s)
        tie = lambda v, a: v if a is None else pltpu.bitcast(pltpu.bitcast(v, U32) | wide(a), F32)

        def f(R, a):
            r_v[R, :] = xx[R, :] + tie(x1[R, :], a) * mod_v[2]

        def move(dst, src):
            def g(R, a):
                dst[R, :] = tie(src[R, :], a)
            return tasks(g, n=8)
        if not rotate:
            return tasks(f, n=8)
        return cat(zip(tasks(f, n=8), move(view(hb_v, 1), hb_v), move(xx, x_v)))

    KD, KF, ND = [(0, 2), (1, 3)], [(2 * i, 2 * i + 1) for i in range(7)], [(1, 2), (3, 4)]
    Wt = {1: (lambda k, n: w1_v[C(k), C(n)], lambda i, kp, j: w1s[C(kp), C(2 * i + j)], False, KD, [4]),
          2: (lambda k, n: w2_v[C(k), C(n)], lambda i, kp, j: w2s[C(kp), C(2 * i + j)], False, KD, [4]),
          0: (lambda k, n: w3_v[C(n), C(k)], None, True, KD, [4]),
          3: (lambda k, n: w3n[C(k), C(n)], lambda i, kp, j: w3s[C(kp), C(6 * i + j)], False, KD, [4]),
          4: (lambda k, n: w4_v[C(k), C(n)], lambda i, kp, j: w4s[C(kp), C(2 * i + j)], False, KF, [])}

    def sums_task(load, store, left):
        def fn(a):
            b = [[load(u, v) for v in range(2)] for u in range(2)]
            b[0][0], b[1][1] = _tie(b[0][0], a), _tie(b[1][1], a)
            (x11, x12), (x21, x22) = [[pltpu.bitcast(x, BF16).astype(F32) for x in row] for row in b]
            r = ((x11 + x22, x21 + x22, x11 + x12, x21 - x11, x12 - x22) if left else
                 (x11 + x22, x12 - x22, x21 - x11, x11 + x12, x21 + x22))
            for m, x in enumerate(r):
                store(m, x.astype(BF16))
        return fn

    def wsums(w_w, ws, rp, cp_):
        def mk(i, j, r):
            def store(m, x):
                ws[pl.ds(128 * i + r, 16), C(len(cp_) * m + j)] = x
            return sums_task(lambda u, v: w_w[pl.ds(64 * rp[i][u] + r // 2, 8), C(cp_[j][v])], store, False)
        return [mk(i, j, r) for j in range(len(cp_)) for i in range(len(rp)) for r in range(0, 128, 16)]

    def w3_turn():
        def mk(n, k):
            def fn(a):
                x = jnp.concatenate([_tie(w3_w[64 * n:64 * n + 8, C(k)], a), w3_w[64 * n + 8:64 * n + 64, C(k)]], axis=0)
                w3n[C(k), C(n)] = pltpu.bitcast(x, BF16).T
            return fn
        return [mk(n, k) for n in range(FT - 1) for k in range(NT)]

    def plain(name, w, lhs, n, R, epi, cost):
        tile, _, nt, kp, kl = Wt[w]
        ks = sorted([k for p in kp for k in p] + kl)
        rows_ = R.stop - R.start
        return Unit(name, [(lambda k=k: (lhs[R, C(k)], tile(k, n))) for k in ks], lambda p: epi(n, R, p[0]),
                    rows_, rows_ // 8 * (len(ks) - 1), nt=nt, acc=True, tail=rows_ // 8 * cost(n))

    def quad(name, w, lhs, sums, j, cols_, R, epi, cost):
        tile, wsum, nt, kp, kl = Wt[w] if isinstance(w, int) else w
        h, S2, c = len(kp), slice(R.start // 2, R.stop // 2), {}
        a_ = lambda i, k: _top(lhs(k) if callable(lhs) else lhs[R, C(k)], i)
        s_ = sums if callable(sums) else (lambda i, p: sums[S2, C(h * i + p)])
        prod = lambda fa_, fb_: [(lambda p=p: (fa_(p), fb_(p))) for p in range(h)]
        left = lambda i, n: [(lambda k=k: (a_(i, k), tile(k, n))) for k in kl]
        mk = lambda tiles, f, x=0: Unit(name, tiles, lambda p: f(p[0]), 64, 8 * len(tiles), nt=nt, acc=True, tail=x)

        def e1(m):
            u7.res, u6.res = [m], [m]

        def e4(m):
            c[11], c[21] = c[11] + m, m

        def e2(m):
            c[21], c[22] = c[21] + m, c[22] - m
            l21.res = [c[21]]

        def e5(m):
            c[12] = m
            epi(cols_[0], R, _zip(c[11] - m, c[21]))

        def e3(m):
            l12.res, c[22] = [c[12] + m], c[22] + m
            if not kl:
                l12.epi(l12.res)
        u1 = mk(prod(lambda p: s_(0, p), lambda p: wsum(0, p, j)), e1)
        u7 = mk(prod(lambda p: s_(4, p), lambda p: wsum(4, p, j)) + left(0, cols_[0]), lambda m: c.update({11: m}))
        u6 = mk(prod(lambda p: s_(3, p), lambda p: wsum(3, p, j)) + left(1, cols_[1]), lambda m: c.update({22: m}))
        u4 = mk(prod(lambda p: a_(1, kp[p][1]), lambda p: wsum(2, p, j)), e4)
        u2 = mk(prod(lambda p: s_(1, p), lambda p: tile(kp[p][0], cols_[0])), e2, 8)
        l21 = mk(left(1, cols_[0]), lambda m: c.update({21: m}))
        u5 = mk(prod(lambda p: s_(2, p), lambda p: tile(kp[p][1], cols_[1])), e5, 16 * cost(cols_[0]))
        u3 = mk(prod(lambda p: a_(0, kp[p][0]), lambda p: wsum(1, p, j)), e3, 8 if kl else 8 + 16 * cost(cols_[1]))
        l12 = mk(left(0, cols_[1]), lambda m: epi(cols_[1], R, _zip(m, c[22])), 16 * cost(cols_[1]))
        return [u1, u7, u6, u4, u2, l21, u5, u3, l12]

    LH, RH = [0, 4, 3, (1, 1), 1, 2, (0, 0)], [0, 4, 3, 2, (0, 0), (1, 1), 1]
    L2 = {3: (w3n_w, ws_w[2], w3t, KF[:6], n2t), 4: (w4_w, ws_w[3], w4t, ND, a_t)}

    def wsums2(w):
        w_w, s_w, ws2, cp_, _ = L2[w]
        kp, nj = Wt[w][3], len(cp_)

        def mk(o, p2, j2, r):
            def load(u, v):
                p, j, y = 2 * p2 + u, 2 * j2 + v, RH[o]
                if isinstance(y, int):
                    return s_w[pl.ds(64 * p + r // 2, 8), C(nj * y + j)]
                return w_w[pl.ds(64 * kp[p][y[0]] + r // 2, 8), C(cp_[j][y[1]])]

            def store(m, x):
                ws2[pl.ds(128 * p2 + r, 16), C((5 * o + m) * (nj // 2) + j2)] = x
            return sums_task(load, store, False)
        return [mk(o, p2, j2, r) for j2 in range(nj // 2) for o in range(7) for p2 in range(len(kp) // 2)
                for r in range(0, 128, 16)]

    def wsums4():
        form = [((0, 0), (1, 1), 1), ((0, 1), (1, 1), -1), ((1, 0), (0, 0), -1), ((0, 0), (0, 1), 1), ((1, 0), (1, 1), 1)]

        def mk(o, p2, r):
            def fn(a):
                def blk(p, j, uv, t):
                    x = w4_w[pl.ds(64 * KF[p][uv[0]] + r // 2, 8), C(ND[j][uv[1]])]
                    return pltpu.bitcast(_tie(x, t), BF16).astype(F32)
                y = {}
                for u in range(2):
                    for j in range(2):
                        p = 2 * p2 + u
                        if isinstance(RH[o], int):
                            f = form[RH[o]]
                            x1, x2 = blk(p, j, f[0], a), blk(p, j, f[1], None)
                            y[u, j] = x1 + x2 if f[2] > 0 else x1 - x2
                            w4s[pl.ds(128 * p + r, 16), C(2 * RH[o] + j)] = y[u, j].astype(BF16)
                        else:
                            y[u, j] = blk(p, j, RH[o], a if u == j else None)
                for m, f in enumerate(form):
                    x = y[f[0]] + y[f[1]] if f[2] > 0 else y[f[0]] - y[f[1]]
                    w4t[pl.ds(128 * p2 + r, 16), C(5 * o + m)] = x.astype(BF16)
            return fn
        last = wsums(w4_w, w4s, KF, ND)
        return (last[48:56] + last[104:112]
                + [mk(o, p2, r) for o in range(7) for p2 in range(3) for r in range(0, 128, 16)])

    def lsums2(w, lhs_w, sums_w, sl):
        kp, xs2 = Wt[w][3], L2[w][4]
        h2 = len(kp) // 2

        def mk(o, p2, g):
            def load(u, v):
                p, ch, x = 2 * p2 + v, 2 * g + u, LH[o]
                if isinstance(x, int):
                    return sums_w[pl.ds(64 * sl + 8 * ch, 8), C(len(kp) * x + p)]
                return lhs_w[pl.ds(H * sl + 16 * ch + 8 * x[0], 8), C(kp[p][x[1]])]

            def store(m, x):
                xs2[pl.ds(16 * g, 16), C((5 * o + m) * h2 + p2)] = x
            return sums_task(load, store, True)
        return [[mk(o, p2, g) for o in range(7) for g in range(4)] for p2 in range(h2)]

    def quad2(name, w, lhs, sums, j2, epi, cost):
        tile, wsum, nt, kp, kl = Wt[w]
        ws2, cp_, xs2 = L2[w][2:]
        h, h2, nj2, c, R = len(kp), len(kp) // 2, len(cp_) // 2, {}, slice(0, T)

        b0 = 8 * (j2 if kl else 3)
        slot = lambda j, i, v: C(b0 + 4 * (j % 2) + 2 * (i - 1) + v)

        def upd(o, j, m):
            val = {}
            for i, v, sg in (((1, 0, 1), (2, 1, 1)), ((1, 0, 1),), ((2, 1, 1),), ((1, 0, 1), (2, 0, 1)),
                             ((2, 0, 1), (2, 1, -1)), ((1, 0, -1), (1, 1, 1)), ((1, 1, 1), (2, 1, 1)))[o]:
                k = (j, i, v)
                if o == 0 and i == 1:
                    c[k] = slot(j, 2, 1)
                    continue
                val[i, v] = m if k not in c else (cb_v[:, c[k]] + m if sg > 0 else cb_v[:, c[k]] - m)
                c[k] = slot(*k)
                if kl or (o, v) not in ((4, 0), (5, 0), (6, 1)):
                    cb_v[:, c[k]] = val[i, v]
                else:
                    for r in range(0, H, 16):
                        epi(cp_[j][v], slice(2 * r + 16 * i - 16, 2 * r + 16 * i), val[i, v][r:r + 16],
                            r == H - 16 and (o, i) in ((5, 1), (6, 2)))

        def inner(o):
            x, y = LH[o], RH[o]
            xo = ((lambda p: sums[:, C(h * x + p)]) if isinstance(x, int)
                  else (lambda p: _top(lhs[:, C(kp[p][x[1]])], x[0])))
            yo = ((lambda p, j: wsum(y, p, j)) if isinstance(y, int)
                  else (lambda p, j: tile(kp[p][y[0]], cp_[j][y[1]])))
            w_ = (yo, lambda m, p2, _: ws2[C(p2), C((5 * o + m) * nj2 + j2)], nt,
                  [(2 * i, 2 * i + 1) for i in range(h2)], list(range(2 * h2, h)))
            return quad(name, w_, xo, lambda m, p2: xs2[:, C((5 * o + m) * h2 + p2)], 0, (2 * j2, 2 * j2 + 1),
                        HS[0], lambda j, _, m: upd(o, j, m), lambda j: 1.5 + KS + ((o // 6 + 1) * cost(0) if o >= 4 and not kl else 0))

        def rest(j, v, Q):
            return [Unit(name, [lambda: (lhs[Q, C(k)], tile(k, cp_[j][v]))],
                         lambda p: epi(cp_[j][v], Q, p[0] + _zip(*[cb_v[Q.start // 2:Q.stop // 2, c[j, i, v]] for i in (1, 2)])), 64, 8 * (cost(cp_[j][v]) + 1)) for k in kl]
        return cat(inner(o) for o in range(7)), [u for Q in QS for j in (2 * j2, 2 * j2 + 1) for v in range(2)
                                                 for u in rest(j, v, Q)]

    def mm(name, w, lhs, sums, epi, cost):
        if sums is None:
            return [[plain(name, w, lhs, n, R, epi, cost) for R in HS] for n in range(NT)]
        return [[plain(name, w, lhs, 0, R, epi, cost) for R in QS]] + [
            [u for R in HS for u in quad(name, w, lhs, sums, j, ND[j], R, epi, cost)] for j in range(2)]

    def mm1(name, hs, sl, fast=False):
        def epi(n, R, p):
            h1_v[n, pl.ds(hs * T + 8 + R.start, R.stop - R.start), :] = _gelu2(p)
        return cat(mm(name, 1, view(n1_v, sl), n1s if fast else None, epi, lambda n: 5 + KS))

    def mm2(name, sl, xs, x1s, fast=False):
        def epi(n, R, p):
            view(x1_v, x1s)[R, C(n)] = view(hb_v, xs)[R, C(n)] + p
        return cat(mm(name, 2, view(g_v, sl), gs if fast else None, epi, lambda n: 1 + KS))

    def mm3(name, sl, fast=True, host=None):
        nn, aa, ss, keep = view(n2_v, sl), view(a_v, sl), view(a_s, sl, H), {}

        def epi(n, R, p):
            g = _gelu2(p)
            aa[R, C(n)] = g.astype(BF16)
            if not fast:
                return
            if n % 2 == 0 and n < 12:
                keep[n] = g
                return
            pair = (keep.pop(n - 1), g) if n % 2 else (g, st_v[R, C(8)])
            for i, x in enumerate(_lhs_sums(*pair)):
                ss[R.start // 2:R.stop // 2, C(7 * i + n // 2)] = x.astype(BF16)

        c3 = lambda n: 5.5 + 0.5 * KS + (3.75 + 1.25 * KS if fast and (n % 2 or n == 12) else 0)

        def rem(R):
            def f(p):
                g = jnp.concatenate([_gelu2(p[0]), jnp.zeros((64, 128), F32)], axis=0).T
                aa[R, C(13)] = g.astype(BF16)
                if fast:
                    st_v[R, C(8)] = g
            return Unit(name, [(lambda k=k: (w3_v[13 * 128:F, C(k)], nn[R, C(k)])) for k in range(NT)], f, 64, 84,
                        nt=True, acc=True)
        odd = [rem(R) for R in HS] + [plain(name, 3 if fast else 0, nn, 12, R, epi, c3) for R in QS]
        if not fast:
            return odd + [plain(name, 0, nn, n, R, epi, c3) for p in KF[:6] for R in HS for n in p]
        qd = [quad2(name + "_%d" % j, 3, nn, view(n2s, sl, H), j, epi, c3) for j in range(3)]
        mid = qd[0][0] + _weave(qd[1][0], qd[0][1]) + _weave(qd[2][0], qd[1][1])
        if host is None:
            return odd[:2] + mid + _weave(odd[2:], qd[2][1])
        for u in (odd[0], odd[2], odd[3]):
            u.name = name + "h"
        return [odd[0], odd[2], odd[3], odd[1]] + mid, _weave(odd[4:] + host, qd[2][1])

    def cp_out(j, osl, L, sm, R=slice(0, T)):
        return cp(o_v.at[pl.ds(osl * T + R.start, R.stop - R.start), L],
                  o_hbm.at[pl.ds(base(j, T) + R.start, R.stop - R.start), L], sem_o.at[sm])

    out_a = lambda j: cp_out(j, 0, slice(128, D), 0)
    out_b = lambda j: cp_out(j, 0, C(0), 1)
    last = []

    def mm4(name, j, sl, osl=0, xs=None, x1s=None, fast=True):
        oo = view(o_v, osl)

        def epi(n, R, p, full=None):
            if xs is None:
                oo[R, C(n)] = (r_v[R, C(n)] + mod_v[2, 0:1, C(n)] * p).astype(BF16)
            else:
                oo[R, C(n)] = (view(x_v, xs)[R, C(n)] + mod_v[2, 0:1, C(n)]
                               * (view(x1_v, x1s)[R, C(n)] + p)).astype(BF16)
            if full is not None:
                if not full:
                    return
                R = slice(0, T)
            if osl == 2:
                last.append(cp_out(j, osl, C(n), 2, R))
                last[-1].start()
            elif R.stop == T and osl and n == NT - 1:
                last.append(cp_out(j, osl, slice(128 if osl == 3 else 0, D), 2))
                last[-1].start()
            elif R.stop == T and osl == 0 and n in (0, NT - 1):
                (out_a if n else out_b)(j).start()
        c4 = lambda n: (3 if xs is None else 4) + KS
        if fast:
            return ([plain(name, 4, view(a_v, sl), 0, R, epi, c4) for R in QS],
                    quad2(name + "q", 4, view(a_v, sl), view(a_s, sl, H), 0, epi, c4)[0])
        return mm(name, 4, view(a_v, sl), None, epi, c4)

    def split(us):
        n = 4 // len(us)
        m, mks, st = us[0].rows // n, [u.tiles.pop(0) for u in us], {}

        def piece(i, k):
            if i not in st:
                st[i] = mks[i]()
            return st[i][0][m * k:m * (k + 1)], st[i][1]

        def epi(p):
            for i, u in enumerate(us):
                u.res = [jnp.concatenate(p[n * i:n * (i + 1)], axis=0)]
        return _flat([Unit(us[0].name, [(lambda i=i, k=k: piece(i, k)) for i in range(len(us)) for k in range(n)],
                           epi, m, 0, nt=us[0].nt)])

    W = lambda nm: [("wait", nm)]
    run = lambda fns: [("run", "run", lambda: [fn(None) for fn in fns])]
    one = lambda us: [_flat([u]) for u in us]
    nm = lambda x: (lambda n: x)

    seq, grp = [], []
    for s in range(NC):
        seq += W("c%d" % s) + _flat(mmK(s) + mmU(nm("U%d" % s), s % 2, NC - 1 - s))
        grp.append(Group("kv%d" % s, cat(kv(s, s % 2)), 50, ["c%d" % s], ["U%d" % s], 100))
    inv = [mmI(lambda n: "I%d" % n, s, s) for s in range(NC)]
    seq += W("c3") + _flat(mmK(3) + mmK(4) + [inv[s][t] for t in range(NT) for s in range(NC)])
    macs = [mac(s + 1, NC - 1 - s, s) for s in range(NC)]
    grp.append(Group("mac00", macs[0][0], 12, ["c1"], ["c2"], 0))
    grp.append(Group("mac01", macs[1][0] + macs[0][1] + macs[1][1], 16, ["c2"], ["c3"], 0))
    for t in range(NT):
        grp.append(Group("mac%d" % t, cat(macs[s][t] for s in range(2 if t < 2 else 0, NC)), 24 if t < 2 else 18,
                         ["c3", "K%d" % t], ["I%d" % t], 100, 150))
    start = lambda cs: [("run", "run", lambda: [c.start() for c in cs])]
    f0, f1 = front(0, 2, True), front(1, 1, True)
    seq += run(ahead(0))
    seq += W("wma") + _flat(mod("moda", 0, 3)) + run(f0[0] + f1[0] + ahead(1))
    seq += W("wmb") + start(next_kv(NC) + next_q(NC)) + _flat(mod("modb", 3, 5)) + run(f0[1])
    w1 = _flat(mm1("w1_0", 0, 0) + mm1("w1_1", 1, 1))
    seq += W("w1") + w1[:72] + W("w2") + w1[72:] + run(shift(0, 0))
    seq += _flat(mm2("w2_0", 0, 2, 1) + mm1("w1_2", 2, 2)) + run(shift(1, 1)) + _flat(mm2("w2_1", 1, 1, 0))
    grp.append(Group("f1", f1[1], 80, ["w1"], ["w1_1"], 450))
    grp.append(Group("f2", front(2, 0), 80, ["w2"], ["w1_2"], 450))
    grp.append(Group("ln2_0", ln2(1, 0, False), 60, ["w2_0"], ["w3"], 450))
    grp.append(Group("ahead", cat(ahead(i) for i in range(2, NB - NC)), 19 + 2 * KS, ["w1"], ["end"], 100))
    grp.append(Group("ws1", wsums(w1_w, w1s, KD, ND), 26 + 5 * KS, ["w1"], ["end"], 100))
    grp.append(Group("ws2", wsums(w2_w, w2s, KD, ND), 26 + 5 * KS, ["w2"], ["end"], 100))
    grp.append(Group("ws3", w3_turn() + wsums(w3n_w, w3s, KD, KF[:6]) + wsums2(3), 22 + 5.5 * KS, ["w3"], ["end"], 100))
    grp.append(Group("ws4", wsums4(), 40 + 8 * KS, ["w4"], ["end"], 60))
    _wait(seq, "w3", back=1)
    w3 = mm3("w3_0", 0, False)
    _mix(seq, _flat(w3[6:]), [split(w3[4:6]) + _flat(w3[:6])], 0.1)
    mc = mod("modc", 5, 6)
    mc = _flat(mc[1:] + mc[:1])
    _wait(seq, "w4", mc[:5] + [("sync", "run", lambda: None)])
    w4 = cat(mm4("w4_0", 0, 0, 3, 2, 1, False)[1:])
    qs = [split([w4[-1 - i]]) for i in range(_phase(seq))]
    _mix(seq, _flat(w4), [mc[i:i + 4] for i in range(5, 25, 4)] + qs, 0.01, 0.4)
    assert _phase(seq) == 0
    grp.append(Group("resid", resid(2, 1), 16 + 5 * KS, ["modc"], ["end"], 100))
    grp.append(Group("ln2a", ln2_late(), 40, ["w3_0"], ["end"], 100))
    _emit(seq, grp, zero, wait)

    def step(s, carry):
        for c in next_kv(s) + next_q(s):
            c.wait()
        nxt = jnp.minimum(s + 1, NB - 1)
        seq, grp = [], []
        us, it = one(mmU(lambda n: "U%d" % n, 0, 0)), one(mmI(lambda n: "I%d" % n, 0, 0))
        w4, w4c = mm4("w4", s - 2, 0)[1], mm4("w4c", s - 3, 0)[0]
        w2 = mm2("w2", 0, 1, 0, True)
        w2 = w2[0:3] + w2[4:13] + w2[22:31] + w2[3:4] + w2[13:22] + w2[31:]
        for u in w2[:21]:
            u.name = "w2a"
        w2[0].name = "w2f"
        w3, w3e = mm3("w3", 0, host=w2[:4])
        _mix(seq, _flat(w4c + w3),
             [us[0], us[1], us[2], it[0] + us[3], it[1] + us[4], it[2], it[3], it[4]],
             0.181, 0.618)
        w1a, w1b = mm1("w1a", 2, 0, True), mm1("w1b", 2, 0, True)
        w1a, w1b = _flat(w1a[0:2] + w1a[4:13] + w1a[22:31]), _flat(w1b[2:4] + w1b[13:22] + w1b[31:])
        kw = 9 * 4
        w4[kw - 11].name = "w4m"
        seq += _flat(w3e + w2[4:21] + w4[:kw]) + w1a + run(shift(1, 0, ((T - 32, 32),), gs))
        seq += _flat(w4[kw:] + w2[21:]) + w1b
        assert _phase(seq) == 0
        kvs, macs = kv(0, 0), mac(1, 0, 0, part=True)
        for t in range(NT):
            grp.append(Group("kv%d" % t, kvs[t], 50 + 2 * KS, ["start"], ["U%d" % t], 220))
            grp.append(Group("mac%d" % t, macs[t], 24 + 2 * KS, ["U%d" % t], ["I%d" % t], 230, 150))
        iall = ["I%d" % t for t in range(NT)]
        ln = ln2(0, 0)
        grp.append(Group("ln2a", ln2_late(), 40, ["w2a", "w4q"], ["end"], 100, 300))
        xn = lsums2(3, n2_w, as_w[2], 0)[0]
        grp.append(Group("ln2b", ln[4:8] + ln[12:16], 78 + 20 * KS, ["start"], ["w3h"], 450))
        grp.append(Group("xna", [f for i, f in enumerate(xn) if i % 4 < 2], 26 + 5 * KS, ["start"], ["w3_0"], 150))
        grp.append(Group("xnb", [f for i, f in enumerate(xn) if i % 4 >= 2], 26 + 5 * KS, ["w4c"], ["w3_0"], 150, 0))
        grp.append(Group("resid", resid(1, 0, True), 9.5 + 5 * KS, ["w4c"], ["w2f"], 100))
        for p, ts in enumerate(lsums2(4, a_w, as_w[3], 0)):
            grp.append(Group("xa%d" % p, ts, 26 + 5 * KS, ["w3_%d" % p], ["w4q"], 150, 100))
        fr = front(0, 0, ss=n1s)
        grp.append(Group("fronta", fr[0], (50 + 8 * KS) * 40 / len(fr[0]), ["w2f"], ["w1a"], 250, 0))
        grp.append(Group("frontb", fr[1], (46 + 7 * KS) * 57 / len(fr[1]), ["w4m"], ["w1b"], 250, 110))
        def refill(buf, cs):
            def fn(a):
                for t in range(NT):
                    buf[t, 0:8, :] = zero if a is None else a
                for c in cs:
                    c.start()
            return fn
        fr[3].append(refill(q_n[0], next_q(nxt)))
        nk = next_kv(nxt)
        grp.append(Group("refill", [refill(k_n[0], nk[:NT]), refill(v_n[0], nk[NT:])], 10, ["U4"], ["w2f"], 0, 0))
        grp.append(Group("fq", fr[2], 33 + 7 * KS, ["w4c"], ["w2f"], 100))
        grp.append(Group("spread", spread(), 30 + 8 * KS, iall, ["end"], 60))
        grp.append(Group("shift", shift_early(), 22 + 7 * KS, ["start"], ["w2f"], 200))
        _emit(seq, grp, zero, wait)
        out_b(s - 3).wait()
        out_a(s - 2).wait()
        return carry

    lax.fori_loop(NC, NB, step, 0)

    seq, grp = [], []
    w47 = mm4("w4_7", NB - 1, 1, 2, 0, 1)
    seq += _flat(mm4("w4_5", NB - 3, 0)[0] + mm2("w2_7", 0, 0, 1, True) + mm3("w3_6", 0)
                 + cat(mm4("w4_6", NB - 2, 0, 1, 1, 0)) + mm3("w3_7", 1) + w47[0][:3] + w47[1] + w47[0][3:])
    grp.append(Group("shift7", shift(2, 0, [(r, 32) for r in range(0, T, 32)], gs), 24, ["start"], ["w2_7"], 200))
    ln = ln2(0, 0)
    grp.append(Group("ln2_6", ln[4:8] + ln[12:16], 75, ["start"], ["w3_6"], 1200))
    grp.append(Group("xn6", cat(lsums2(3, n2_w, as_w[2], 0)), 26 + 5 * KS, ["w4_5"], ["w3_6_0"], 200, 800))
    grp.append(Group("ln2_7", ln2(1, 1), 75, ["w4_6"], ["w3_7"], 1500))
    grp.append(Group("xn7", cat(lsums2(3, n2_w, as_w[2], 1)), 26 + 5 * KS, ["w4_6"], ["w3_7_0"], 200, 2100))
    for j in (6, 7):
        for p, ts in enumerate(lsums2(4, a_w, as_w[3], j - 6)):
            grp.append(Group("xa%d_%d" % (j, p), ts, 26 + 5 * KS, ["w3_%d_%d" % (j, p)], ["w4_%dq" % j], 200, 150))
    _emit(seq, grp, zero, wait)
    for c in next_kv(NB - 1) + next_q(NB - 1) + [out_b(NB - 3)] + last:
        c.wait()


@jax.jit
def pallas_adaLN_cond__ssm_conv_h3__mixer_s_mlp__prompt_kernel(
        A_q, A_k, A_v, A_shift_k, A_ssm_k, A_ssm_D, B_x, B_w1, B_w2, B_w3, B_w4, c, w_mod):
    any_ = pl.BlockSpec(memory_space=pl.ANY)
    V = pltpu.VMEM
    out = pl.pallas_call(
        kernel,
        in_specs=[any_] * 12,
        out_specs=any_,
        out_shape=jax.ShapeDtypeStruct((S, D), BF16),
        scratch_shapes=[
            [V((NT, H + 8, 128), U32)] * NC, [V((NT, H + 8, 128), U32)] * NC, [V((NT, H + 8, 128), U32)] * NC,
            [V((64, S), U32)] * NT,
            V((D // 2, D), U32), V((D // 2, D), U32), V((F // 2, D), U32), V((FT * 64, D), U32),
            [V((D // 2, 3 * D), U32), V((D // 2, 2 * D), U32), V((D // 2, D), U32)], V((4 * T, D), BF16),
            V((4, D), BF16), V((D,), BF16), V((1, D), BF16), V((8, 128), I32), pltpu.SMEM((8, 128), I32),
            V((5, 8, D), F32), V((6, 8, D), F32), V((T // 2, 4 * H), U32), V((GR // 2, 2 * T), U32),
            V((NB, 3 * T + 8, D), F32), V((NC, 3 * T + 8, D), F32), V((NB - NC, 2 * T + 8, D), F32), V((4 * T, 128), F32),
            V((T, D), U32), V((NC * T, D), U32), V((NT, NC * (T + 8) + 16, 128), F32),
            V((3 * T, D), F32), V((3 * T, D), F32), V((2 * T, D), F32), V((T, D), F32),
            V((3 * T // 2, D), U32), V((T, D), U32), V((T, D), U32), V((NT, NC * T + 24, 128), F32),
            V((T, (FT + 1) * 128), U32),
            [V((128, 11 * 128), U32)] * 2 + [V((128, 31 * 128), U32), V((448, 11 * 128), U32)],
            [V((64, 11 * 128), U32)] * 2 + [V((128, 11 * 128), U32), V((128, 35 * 128), U32)],
            V((D // 2, 13 * 128), U32), V((H, D), F32), V((T, 9 * 128), F32),
            [V((64, 105 * 128), U32), V((192, 35 * 128), U32), V((32, 35 * 128), U32), V((32, 105 * 128), U32)], V((H, 33 * 128), F32),
            pltpu.SemaphoreType.DMA((11,)), pltpu.SemaphoreType.DMA((1,)), pltpu.SemaphoreType.DMA((3,)),
        ],
        compiler_params=pltpu.CompilerParams(vmem_limit_bytes=110 << 20, disable_semaphore_checks=True,
                                             disable_bounds_checks=True),
        name="fused",
    )(A_q[0], A_k[0], A_v[0], A_shift_k.T, A_ssm_k, A_ssm_D, B_w1, B_w2, B_w3.T, B_w4, c, w_mod)
    return out[None]
```

```python
import heapq
import numpy as np
import jax
import jax.numpy as jnp
from jax import lax
from jax.experimental import pallas as pl
from jax.experimental.pallas import tpu as pltpu

S, D, F = 2048, 640, 1728
T = 256
H = T // 2
NB = S // T
NT = D // 128
FT = (F + 127) // 128
EPS = 1e-5
F32, BF16, U32, I32 = jnp.float32, jnp.bfloat16, jnp.uint32, jnp.int32
G_C1 = 0.044715 * float(np.sqrt(2.0 / np.pi))
G_C2 = float(np.sqrt(2.0 / np.pi))
G_A = G_C1 ** (1.0 / 3.0)
G_B = G_C2 / G_A
G_POST = 0.5 / G_A
RG = 16
GR = 80
NC = 3
DL = 450
KS = 1.95
SLOT = 32


def _dft(shape, f_axis, tau, scale=1.0):
    r = lax.broadcasted_iota(I32, shape, f_axis)
    l = lax.broadcasted_iota(I32, shape, 1 - f_axis)
    f = r & 127
    odd = ((f & 63) << 2) | ((f >> 6) << 1) | 1
    p = odd * tau(l) + ((r >> 7) << 8)
    a = ((p + 512) & 1023) - 512
    u = (256 - jnp.abs(a)).astype(F32) * (np.pi / 512.0)
    u2 = u * u
    c = [scale, -scale / 6.0, scale / 120.0, -scale / 5040.0, scale / 362880.0, -scale / 39916800.0]
    poly = c[5]
    for ci in c[4::-1]:
        poly = poly * u2 + ci
    return (u * poly).astype(BF16)


def _rstd(xc, mlp):
    s2, eps = (1.0 / (G_A * G_A), EPS / (G_POST * G_POST)) if mlp else (1.0, EPS)
    v = jnp.sum(xc * xc, axis=-1, keepdims=True) * (s2 / D) + eps * s2
    return jnp.exp2(jnp.log(v) * float(-0.5 / np.log(2.0)))


def _ln(x, mlp=False):
    xc = x - jnp.sum(x, axis=-1, keepdims=True) * (1.0 / D)
    return xc * _rstd(xc, mlp)


def _gelu2(x):
    u = x * (x * x + G_B)
    return x * (1.0 + jnp.tanh(u))


def _lo(w):
    return pltpu.bitcast(w << 16, F32)


def _hi(w):
    return pltpu.bitcast(w & jnp.uint32(0xFFFF0000), F32)


def _tie(x, a):
    if a is None:
        return x
    w = pltpu.bitcast(x[:, :128], U32)
    k = w.shape[0] // 8
    w = w | (a if k == 1 else jnp.concatenate([a] * k, axis=0))
    w = pltpu.bitcast(w, x.dtype)
    return w if x.shape[1] == 128 else jnp.concatenate([w, x[:, 128:]], axis=1)


def _top(x, i):
    return jnp.concatenate([x[r:r + 16] for r in range(16 * i, x.shape[0], 32)], axis=0)


def _zip(t, b):
    return jnp.concatenate([x[r:r + 16] for r in range(0, t.shape[0], 16) for x in (t, b)], axis=0)


def _lhs_sums(x1, x2):
    a11, a21, a12, a22 = _top(x1, 0), _top(x1, 1), _top(x2, 0), _top(x2, 1)
    return [a11 + a22, a21 + a22, a11 + a12, a21 - a11, a12 - a22]


def C(i):
    return slice(i * 128, (i + 1) * 128)


class Unit:
    def __init__(self, name, tiles, epi, rows, cost, nt=False, full=True, acc=False, tail=0):
        self.tail = tail
        self.acc, self.res = acc, []
        self.name, self.tiles, self.epi, self.rows, self.cost, self.nt, self.full = name, tiles, epi, rows, cost, nt, full


class Due:
    def __init__(self, val, delay):
        self.val, self.delay = val, delay


class Group:
    def __init__(self, name, fns, cost, rel, dead, lat, rlat=200):
        self.name, self.fns, self.cost, self.rel, self.dead, self.lat, self.rlat = name, fns, cost, rel, dead, lat, rlat


def _plan(seq, groups):
    busy, n = [0] * 4, 0
    start, end, tiles, bars = {}, {}, [], []
    for it in seq:
        if isinstance(it[0], Unit):
            u = it[0]
            m = n % 4
            n += 1
            t0, t1 = busy[m], busy[m] + max(u.rows, 32)
            busy[m] = t1
            tiles.append((t0, t1, u.cost / len(u.tiles) + (u.tail if it[1] == len(u.tiles) - 1 else 0)))
            start.setdefault(u.name, t0)
            end[u.name] = max(end.get(u.name, 0), t1)
        elif it[0] == "wait":
            t = max(busy)
            busy, n = [t] * 4, 0
            start[it[1]] = end[it[1]] = t
            bars.append(t)
    total = max(busy)
    start["end"] = end["end"] = total
    start["start"] = end["start"] = 0
    ns = total // SLOT + 2
    load = np.zeros(ns)
    for t0, t1, c in tiles:
        a, b = t0 // SLOT, max(t1 // SLOT, t0 // SLOT + 1)
        load[a:b] += c / (b - a)
    win = []
    for g in groups:
        r = max(end[x] + (0 if start[x] == end[x] else g.rlat) for x in g.rel)
        d = min(start[x] for x in g.dead) - g.lat
        ok = np.zeros(ns, bool)
        ok[r // SLOT:max(d // SLOT, r // SLOT + 1)] = True
        for b in bars:
            if r < b <= d:
                ok[max((b - g.lat) // SLOT, 0):b // SLOT] = False
        win.append(np.nonzero(ok)[0])
    alloc = [np.zeros(len(w)) for w in win]
    for _ in range(60):
        for i, g in enumerate(groups):
            w = win[i]
            load[w] -= alloc[i]
            base = load[w]
            vol = g.cost * len(g.fns)
            lo, hi = base.min(), base.max() + vol
            for _ in range(50):
                mid = 0.5 * (lo + hi)
                if np.maximum(mid - base, 0).sum() > vol:
                    hi = mid
                else:
                    lo = mid
            alloc[i] = np.maximum(hi - base, 0)
            load[w] += alloc[i]
    times = []
    for i, g in enumerate(groups):
        cum = np.cumsum(alloc[i])
        ts = []
        for k in range(len(g.fns)):
            x = (k + 0.5) * cum[-1] / len(g.fns)
            j = int(np.searchsorted(cum, x))
            prev = cum[j - 1] if j else 0.0
            ts.append(win[i][j] * SLOT + SLOT * (x - prev) / max(alloc[i][j], 1e-9))
        times.append(ts)
    return times


def _emit(seq, groups, zero, wait):
    times = _plan(seq, groups)
    left = {"start": 0}
    for it in seq:
        nm = it[0].name if isinstance(it[0], Unit) else it[1]
        left[nm] = left.get(nm, 0) + 1
    heap, pend, todo, cnt = [], {}, list(range(len(groups))), 0
    busy, n, due = [0] * 4, 0, []

    def release():
        nonlocal cnt
        for i in list(todo):
            g = groups[i]
            if all(left[x] == 0 for x in g.rel):
                todo.remove(i)
                pend[i] = len(g.fns)
                for t, fn in zip(times[i], g.fns):
                    heapq.heappush(heap, (t, cnt, i, fn))
                    cnt += 1

    def force(name):
        nonlocal heap
        for i, g in enumerate(groups):
            if name in g.dead:
                assert i not in todo, (g.name, name)
                if pend[i]:
                    for it in sorted(x for x in heap if x[2] == i):
                        it[3](None)
                    heap = [x for x in heap if x[2] != i]
                    heapq.heapify(heap)
                    pend[i] = 0

    release()
    for it in seq:
        if isinstance(it[0], Unit):
            u, k = it
            force(u.name)
            lhs, rhs = u.tiles[k]()
            t0 = busy[n % 4]
            while u.full and due and due[0][0] < t0 + u.rows:
                t, x = due.pop(0)
                r = min(max(int(t - t0), 0), u.rows - 1) // 16 * 8
                w = pltpu.bitcast(lhs, U32)
                x = pltpu.bitcast(x[:, :128], U32)
                parts = [w[:r], w[r:r + 8] | ((x[0:8] | x[8:16]) & zero), w[r + 8:]]
                lhs = pltpu.bitcast(jnp.concatenate([y for y in parts if y.shape[0]], axis=0), BF16)
            dn = (((1,), (1 if u.nt else 0,)), ((), ()))
            p = lax.dot_general(lhs, rhs, dn, preferred_element_type=F32)
            u.res = [p + u.res[0]] if (u.acc and u.res) else u.res + [p]
            m = n % 4
            n += 1
            t0 = busy[m]
            busy[m] = t0 + max(u.rows, 32)
            used = -8
            while u.full and heap and heap[0][0] < t0 + u.rows:
                r = min(max(int(heap[0][0] - t0), 0), u.rows - 1) // 8 * 8
                r = max(r, used + 8)
                if r >= u.rows or r > max(heap[0][0] - t0, 8) + 8:
                    break
                used = r
                t, _, i, fn = heapq.heappop(heap)
                pend[i] -= 1
                x = fn(pltpu.bitcast(p[r:r + 8], U32) & zero)
                if isinstance(x, Due):
                    due.append((t + x.delay, x.val))
                    due.sort(key=lambda e: e[0])
            if k == len(u.tiles) - 1:
                u.epi(u.res)
            left[u.name] -= 1
        elif it[0] == "wait":
            force(it[1])
            wait(it[1])
            busy, n, due = [max(busy)] * 4, 0, []
            left[it[1]] -= 1
        else:
            it[2]()
            left[it[1]] -= 1
        release()
    force("end")
    assert not heap and not todo


def _sum(ps):
    acc = ps[0]
    for p in ps[1:]:
        acc = acc + p
    return acc


def _flat(us):
    return [(u, i) for u in us for i in range(len(u.tiles))]


def _weave(a, b):
    out = []
    for i, u in enumerate(a):
        out += [u] + b[i * len(b) // len(a):(i + 1) * len(b) // len(a)]
    return out


def _phase(seq):
    n = 0
    for it in seq:
        n = n + 1 if isinstance(it[0], Unit) else (0 if it[0] in ("wait", "sync") else n)
    return n % 4


def _mix(seq, a, b, lo=0.0, hi=1.0):
    n, k = _phase(seq), 0
    for i, t in enumerate(a):
        if k < len(b) and n % 4 == 0 and t[1] != 1 and i >= len(a) * (lo + (hi - lo) * k / len(b)):
            seq.extend(b[k])
            k += 1
        seq.append(t)
        n += 1
    assert k == len(b)


def _wait(seq, name, head=(), back=0):
    r = _phase(seq) + 4 * back
    assert all(isinstance(it[0], Unit) for it in seq[len(seq) - r:])
    seq[len(seq) - r:len(seq) - r] = [("wait", name)] + list(head)


def kernel(q_hbm, k_hbm, v_hbm, sh_hbm, ssm_hbm, sd_hbm, w1_hbm, w2_hbm, w3_hbm, w4_hbm, c_hbm, wm_hbm,
           o_hbm,
           q_n, k_n, v_n, ssm_w, w1_w, w2_w, w3_w, w4_w, wm_w, o_v,
           sh_v, sd_v, c_v, zsrc, z_s, taps, mod_v, tf_w, tg_w,
           kf, uf, acc, zraw, kv_w, zz_w, y_v, x_v, hb_v, x1_v, r_v, n1_w, n2_w, g_w, h1_v, a_w,
           ws_w, as_w, w3n_w, top_v, st_v, l2_w, cb_v,
           sem, sem_b, sem_o):
    bf = lambda r: r.bitcast(BF16)
    w1_v, w2_v, w3_v, w4_v = bf(w1_w), bf(w2_w), bf(w3_w), bf(w4_w)
    wm_v = {0: bf(wm_w[0]), 3: bf(wm_w[1]), 5: bf(wm_w[2])}
    tf_v, tg_v, n1_v, n2_v, g_v = bf(tf_w), bf(tg_w), bf(n1_w), bf(n2_w), bf(g_w)
    a_v, kv_v, zz_v = bf(a_w), bf(kv_w), bf(zz_w)
    w1s, w2s, w3s, w4s = [bf(r) for r in ws_w]
    n1s, gs, n2s, a_s = [bf(r) for r in as_w]
    w3n = bf(w3n_w)
    w3t, w4t, n2t, a_t = [bf(r) for r in l2_w]
    cp = pltpu.make_async_copy
    cat = lambda ls: [x for l in ls for x in l]

    def base(j, n):
        return j * n if isinstance(j, int) else pl.multiple_of(j * n, n)

    def rows(j, n=1, size=T):
        return pl.ds(base(j, size), n * size)

    def view(ref, j, size=T):
        return ref.at[rows(j, 1, size)]

    dmas = {}

    def group(name, *mks):
        sm = sem.at[len(dmas)]
        dmas[name] = [c for mk in mks for c in mk(sm)]

    def ssm_in(t):
        return lambda sm: [cp(ssm_hbm.at[C(t)], bf(ssm_w[t]), sm)]

    def cols(src, start, n, dst, row=0):
        return lambda sm: [cp(src.at[pl.ds(start, n), C(t)], bf(dst).at[t, pl.ds(row, n)], sm) for t in range(NT)]

    def kv_in(s, sl):
        if isinstance(s, int):
            kk = cols(k_hbm, s * T - 16, T + 16, k_n[sl]) if s else cols(k_hbm, 0, T, k_n[sl], 16)
        else:
            kk = cols(k_hbm, pl.multiple_of(s * T - 16, 16), T + 16, k_n[sl])
        return lambda sm: kk(sm) + cols(v_hbm, base(s, T), T, v_n[sl])(sm)

    def q_in(s, sl):
        return cols(q_hbm, base(s, T), T, q_n[sl])

    def wm_in(a, b):
        return lambda sm: [cp(wm_hbm.at[:, a * D:b * D], wm_v[a], sm)]

    def whole(src, dst):
        return lambda sm: [cp(src, dst, sm)]

    next_kv = lambda s: kv_in(s, 0)(sem_b.at[0])
    next_q = lambda s: q_in(s, 0)(sem_b.at[0])

    zsrc[...] = jnp.zeros((8, 128), I32)
    k_n[0][:, 0:8, :] = jnp.zeros((NT, 8, 128), U32)
    w4_w[F // 2:FT * 64, :] = jnp.zeros((FT * 64 - F // 2, D), U32)
    group("small", lambda sm: [cp(zsrc, z_s, sm), cp(sh_hbm, sh_v, sm), cp(sd_hbm, sd_v, sm), cp(c_hbm, c_v, sm)])
    for s in range(NC):
        group("c%d" % s, ssm_in(s), kv_in(s, s))
    group("c3", ssm_in(3), ssm_in(4))
    group("wma", wm_in(0, 3), q_in(0, 0), q_in(1, 1))
    group("wmb", wm_in(3, 5))
    group("w1", whole(w1_hbm, w1_v))
    group("w2", q_in(2, 2), whole(w2_hbm, w2_v))
    group("w3", whole(w3_hbm, w3_v))
    group("w4", whole(w4_hbm, w4_v.at[0:F]), wm_in(5, 6))
    for g in dmas.values():
        for c in g:
            c.start()

    def wait(name):
        for c in dmas[name]:
            c.wait()

    tau_b = lambda l: H + ((l + (H - 1)) & (H - 1))
    tf_v[:, C(0)] = _dft((T, H), 0, lambda l: jnp.where((l & 1) == 0, l, tau_b(l)), 1.0 / T)
    tf_v[:, C(1)] = _dft((T, H), 0, lambda l: jnp.where((l & 1) == 1, l, tau_b(l)), 1.0 / T)
    tf_v[:, C(2)] = _dft((T, H), 0, lambda l: 2 * l - H)
    tf_v[:, C(3)] = _dft((T, H), 0, lambda l: 2 * l + 1 - H)
    sin0 = lax.broadcasted_iota(I32, (GR, T), 1) >= H
    tg_v[:, 0:T] = _dft((GR, T), 1, lambda l: jnp.where(sin0 & (l == 0), H, 2 * l))
    tg_v[:, T:2 * T] = _dft((GR, T), 1, lambda l: 2 * l + 1)
    h1_v[:, 0:8, :] = jnp.zeros((NT, 8, 128), F32)
    h1_v[:, 8 + NC * T:16 + NC * T, :] = jnp.zeros((NT, 8, 128), F32)

    wait("small")
    z = jnp.clip(z_s[0, 0], 0, 1)
    zero = jnp.full((8, 128), z, I32).astype(U32)
    z8 = pl.multiple_of(z * 8, 8)
    for r in (x_v, hb_v, x1_v, r_v, zraw, n1_w, n2_w, g_w, a_w, kv_w, zz_w, *ws_w, *as_w, w3n_w, top_v, st_v, *l2_w, cb_v):
        r[pl.ds(z8, 8), 0:128] = jnp.zeros((8, 128), r.dtype)
    for r in (kf, uf, acc, taps, mod_v):
        r[z, 0:8, 0:128] = jnp.zeros((8, 128), r.dtype)
    for r in (tf_w, tg_w):
        r[pl.ds(z8, 8), 0:128] = r[0:8, 0:128]
    sh = sh_v[...].astype(F32)
    for i in range(4):
        taps[i] = jnp.broadcast_to(sh[i:i + 1], (8, D))
    taps[4] = jnp.broadcast_to(sd_v[...].astype(F32).reshape(1, D) * (1.0 / T), (8, D))
    cf = c_v[...].astype(F32)
    silu_c = jnp.broadcast_to((cf / (1.0 + jnp.exp(-cf))).astype(BF16), (16, D))

    def mmK(n):
        def unit(m):
            st = []

            def rhs(i):
                if not st:
                    ev = (lax.broadcasted_iota(I32, (64, 128), 1) & 1) == 0
                    a = ssm_w[n][:, m * T:m * T + H]
                    b = pltpu.roll(ssm_w[n][:, m * T + H:(m + 1) * T], 1, 1)
                    st.extend([pltpu.bitcast(jnp.where(ev, a, b), BF16), pltpu.bitcast(jnp.where(ev, b, a), BF16)])
                return st[i]

            def epi(p):
                er, ei, or_, oi = p
                cur = [er, ei, or_, oi]
                if m:
                    pv = [zraw[C(4 * ((m - 1) % 2) + (q ^ 1)), :] for q in range(4)]
                    pm = lambda x, y, up: jnp.concatenate([x[:64] + y[:64], x[64:] - y[64:]] if up else
                                                          [x[:64] - y[:64], x[64:] + y[64:]], axis=0)
                    er, ei, or_, oi = [pm(cur[q], pv[q], q & 1) for q in range(4)]
                else:
                    er = er + taps[4, 0:1, C(n)]
                if m + 1 < NB:
                    for q in range(4):
                        zraw[C(4 * (m % 2) + q), :] = cur[q]
                for h, (cr, ci) in enumerate(((er + or_, ei + oi), (er - or_, ei - oi))):
                    B = h * 3 * H
                    kf[m, B:B + H, C(n)] = cr
                    kf[m, B + H:B + 2 * H, C(n)] = ci - cr
                    kf[m, B + 2 * H:B + 3 * H, C(n)] = ci + cr
            return Unit("K%d" % n, [(lambda i=i, r=r: (tf_v[r:r + H, C(i)], rhs(i))) for i in range(2) for r in (0, H)],
                        epi, H, 260, nt=True)
        return [unit(m) for m in range(NB)]

    def kv(s, sl):
        def mk(t, w):
            def fn(a):
                ld = lambda o, n: k_n[s][t, pl.ds(8 + w + o, n), :]
                c0 = jnp.concatenate([_tie(ld(0, 8), a), ld(8, 8)], axis=0).reshape(2, 8, 128)
                c1, c2 = ld(-1, 16).reshape(2, 8, 128), ld(-2, 16).reshape(2, 8, 128)
                s0, s1, s2, s3 = (taps[i, :, C(t)] for i in range(4))
                ke, ko, ke1, ko1, ko2 = _lo(c0), _hi(c0), _lo(c1), _hi(c1), _hi(c2)
                wv = v_n[s][t, w:w + 16, :].reshape(2, 8, 128)
                kve = ((s0 * ke + s1 * ko1) + (s2 * ke1 + s3 * ko2)) * _lo(wv)
                kvo = ((s0 * ko + s1 * ke) + (s2 * ko1 + s3 * ke1)) * _hi(wv)
                kv_v[pl.ds(sl * T + w, 16), C(t)] = kve.reshape(16, 128).astype(BF16)
                kv_v[pl.ds(sl * T + H + w, 16), C(t)] = kvo.reshape(16, 128).astype(BF16)
            return fn
        return [[mk(t, w) for w in range(0, H, 16)] for t in range(NT)]

    def mmU(name, sl, us):
        def unit(n):
            def epi(p):
                er, ei, or_, oi = p
                for h, (cr, ci) in enumerate(((er + or_, ei + oi), (er - or_, ei - oi))):
                    B = h * 3 * H
                    uf[us, B:B + H, C(n)] = cr + ci
                    uf[us, B + H:B + 2 * H, C(n)] = cr
                    uf[us, B + 2 * H:B + 3 * H, C(n)] = ci
            return Unit(name(n), [(lambda i=i, r=r: (tf_v[r:r + H, C(2 + i)], kv_v[pl.ds(sl * T + i * H, H), C(n)]))
                                  for i in range(2) for r in (0, H)], epi, H, 96 + 96 * KS)
        return [unit(n) for n in range(NT)]

    def cmul(m0, u0, n, h, row, L, a):
        t = []
        for i in range(3):
            Rw = slice((3 * h + i) * H + row, (3 * h + i) * H + row + 8)
            kk = kf[m0:m0 + n, Rw, L]
            if i == 0 and a is not None:
                k0 = _tie(kk[0], a)[None]
                kk = k0 if n == 1 else jnp.concatenate([k0, kk[1:]], axis=0)
            t.append(jnp.sum(kk * uf[u0:u0 + n, Rw, L], axis=0))
        return t[0] - t[2], t[0] + t[1]

    def AR(h, q, row):
        return slice((2 * h + q) * H + row, (2 * h + q) * H + row + 8)

    def mac(n, u0, sl, part=False):
        def mk(t, rc):
            st, fin = [], []

            def piece(i):
                def fn(a):
                    h, row = i & 1, rc + (i >> 1) * 8
                    zr, zi = cmul(0, u0, n, h, row, C(t), a)
                    if part:
                        zr, zi = zr + acc[0, AR(h, 0, row), C(t)], zi + acc[0, AR(h, 1, row), C(t)]
                    st.append((zr, zi))
                    if h:
                        (pr, pi), (mr, mi) = st[-2:]
                        fin.append([pr + mr, pi + mi, pr - mr, pi - mi])
                    if i == 3:
                        for q in range(4):
                            zz_v[pl.ds(sl * 2 * T + q * H + rc, 16), C(t)] = jnp.concatenate(
                                [fin[0][q], fin[1][q]], axis=0).astype(BF16)
                return fn
            if not part:
                return [piece(i) for i in range(4)]
            both = lambda f, g: (lambda a: (f(a), g(None)))
            return [both(piece(0), piece(1)), both(piece(2), piece(3))]
        return [[fn for rc in range(0, H, 16) for fn in mk(t, rc)] for t in range(NT)]

    def pos():
        return [(t, h, row) for t in range(NT) for row in range(0, H, 8) for h in range(2)]

    def ahead(i):
        def mk(t, h, row):
            def fn(a):
                zr, zi = cmul(i + 1, 0, NC, h, row, C(t), a)
                acc[i, AR(h, 0, row), C(t)] = zr
                acc[i, AR(h, 1, row), C(t)] = zi
            return fn
        return [mk(*p) for p in pos()]

    def spread():
        n = NB - NC - 1

        def mk(t, h, row):
            def fn(a):
                p = []
                for i in range(3):
                    Rw = slice((3 * h + i) * H + row, (3 * h + i) * H + row + 8)
                    u = uf[0, Rw, C(t)]
                    p.append(kf[1:1 + n, Rw, C(t)] * (_tie(u, a) if i == 0 else u)[None])
                acc[0:n, AR(h, 0, row), C(t)] = acc[1:1 + n, AR(h, 0, row), C(t)] + (p[0] - p[2])
                acc[0:n, AR(h, 1, row), C(t)] = acc[1:1 + n, AR(h, 1, row), C(t)] + (p[0] + p[1])
            return fn
        return [mk(*p) for p in pos()]

    def mmI(name, sl, ys):
        def unit(n):
            def epi(p):
                ce, se, co, so = p
                sub = lax.broadcasted_iota(I32, (8, 128), 0)
                b0 = ys * (T + 8) + 8
                y_v[n, b0 + H - 1:b0 + H, :] = (ce[64:72] - se[0:8])[0:1]
                se = jnp.concatenate([jnp.where(sub == 0, 0.0, se[0:8]), se[8:]], axis=0)
                for d, cc, ss in ((0, ce[0:64], se), (1, co, so)):
                    y_v[n, pl.ds(b0 + H + d, 64, stride=2), :] = cc + ss
                    y_v[n, pl.ds(b0 + d - 1, 64, stride=2), :] = cc - ss
            return Unit(name(n), [(lambda i=i: (tg_v[0:(GR if i == 0 else 64), C(i)], zz_v[pl.ds(sl * 2 * T + i * H, H), C(n)]))
                                  for i in range(4)], epi, 64, 36 + 33 * KS)
        return [unit(n) for n in range(NT)]

    def mod(name, a, b):
        def unit(n):
            def epi(p):
                v = [_sum(p[i * NT:(i + 1) * NT])[0:8] for i in range(b - a)]
                if a == 0:
                    mod_v[0, :, C(n)] = v[0] * v[2]
                    mod_v[1, :, C(n)] = (v[1] + 1.0) * v[2]
                elif a == 3:
                    mod_v[3, :, C(n)] = v[0] * (1.0 / G_POST)
                    mod_v[4, :, C(n)] = (v[1] + 1.0) * (1.0 / G_POST)
                else:
                    mod_v[2, :, C(n)] = v[0] * G_POST
            return Unit(name, [(lambda i=i, k=k: (silu_c[:, C(k)], wm_v[a][C(k), pl.ds(i * D + n * 128, 128)]))
                               for i in range(b - a) for k in range(NT)], epi, 16, 10, full=False, acc=b - a == 1)
        return [unit(n) for n in range(NT)]

    HS = (slice(0, 128), slice(128, 256))
    QS = tuple(slice(r, r + 64) for r in range(0, T, 64))

    def tasks(f, due=None, tie=True, n=RG):
        def mk(R):
            def fn(a):
                x = f(R, a if tie else None)
                return Due(x, due) if due else None
            return fn
        return [mk(slice(r, r + n)) for r in range(0, T, n)]

    def load_y(sl, R):
        b0, back = sl * (T + 8) + 8, 7 - lax.broadcasted_iota(I32, (8, 128), 0)

        def ld(t, r):
            if r >= H:
                return y_v[t, b0 + r:b0 + r + 8, :]
            return jnp.take_along_axis(y_v[t, b0 + H - 8 - r:b0 + H - r, :], back, axis=0)
        return jnp.stack([jnp.concatenate([ld(t, r) for t in range(NT)], axis=1) for r in range(R.start, R.stop, 8)])

    def put(nn, ss, R, x):
        nn[R, :] = x.astype(BF16)
        tok = x
        if ss is not None:
            S2 = pl.ds(R.start // 32 * 16, 16)
            if R.stop % 32:
                top_v[S2, 0:2 * T] = x[:, 0:2 * T]
            else:
                x = jnp.concatenate([top_v[S2, 0:2 * T], x[:, 0:2 * T]], axis=0)
                ss[S2, 0:5 * T] = jnp.concatenate(_lhs_sums(x[:, 0:T], x[:, T:2 * T]), axis=1).astype(BF16)
        return tok

    wide = lambda v: jnp.concatenate([v] * NT, axis=1)

    def mean(i, R, x):
        st_v[R, C(i)] = jnp.broadcast_to(jnp.sum(x, axis=-1, keepdims=True) * (1.0 / D), (x.shape[0], 128))

    def centred(src, i, R, a):
        return src[R, :] - wide(_tie(st_v[R, C(i)], a))

    def scale(src, i, g):
        def f(R, a):
            st_v[R, C(i + 1)] = jnp.broadcast_to(_rstd(centred(src, i, R, a), g), (RG, 128))
        return f

    def normed(src, i, R, a):
        return centred(src, i, R, a) * wide(st_v[R, C(i + 1)])

    def finish(src, i, nn, ss):
        def mk(r, ts):
            def fn(a):
                R = slice(r, r + 32)
                m, g = _tie(st_v[R, C(i)], a), st_v[R, C(i + 1)]
                x = [(src[R, C(t)] - m) * g for t in ts]
                for t, v in zip(ts, x):
                    nn[R, C(t)] = v.astype(BF16)
                for k, v in enumerate(_lhs_sums(*x[:2])):
                    ss[pl.ds(r // 2, 16), C(2 * k + ts[0])] = v.astype(BF16)
            return fn
        return [mk(r, ts) for r in range(0, T, 32) for ts in ((0, 2, 4), (1, 3))]

    def front(sl, xs, early=False, halves=False):
        xx, hh, nn = view(x_v, xs), view(hb_v, xs), view(n1_v, sl)

        def fa(R, a):
            q = [q_n[sl][t, R.start // 2:R.stop // 2, :] for t in range(NT)]
            q = jnp.concatenate([_tie(q[0], a)] + q[1:], axis=1)
            q = pltpu.bitcast(q, BF16).astype(F32).reshape(2, 8, D)
            x = (q + (_ln(q) * mod_v[1] + mod_v[0]) * load_y(sl, R)).reshape(RG, D)
            xx[R, :] = x
            hh[R, :] = _ln(x)

        def fc(R, a):
            hb = (_tie(hh[R, :], a).reshape(2, 8, D) * mod_v[4] + mod_v[3]).reshape(RG, D)
            hh[R, :] = hb
            nn[R, :] = _ln(hb, True).astype(BF16)
        if early:
            return tasks(fa), tasks(fc)
        qf = view(x_v, 2) if halves else r_v

        def s1(R, a):
            q = [q_n[sl][t, R.start // 2:R.stop // 2, :] for t in range(NT)]
            q = pltpu.bitcast(jnp.concatenate([_tie(v, a) for v in q], axis=1), BF16).astype(F32)
            qf[R, :] = q
            mean(0, R, q)

        def s3(R, a):
            h = normed(qf, 0, R, a).reshape(-1, 8, D) * mod_v[1] + mod_v[0]
            x = qf[R, :] + (h * load_y(sl, R)).reshape(-1, D)
            xx[R, :] = x
            mean(2, R, x)

        def s5(R, a):
            hb = (normed(xx, 2, R, a).reshape(-1, 8, D) * mod_v[4] + mod_v[3]).reshape(-1, D)
            hh[R, :] = hb
            mean(4, R, hb)
        s7 = finish(hh, 4, nn, n1s)
        one_ = lambda ts: [(t,) for t in ts]
        st = [list(zip(*[iter(tasks(s3, n=8))] * 2)), one_(tasks(scale(xx, 2, False))), one_(tasks(s5)),
              one_(tasks(scale(hh, 4, True))), one_(s7)]
        p = [one_(tasks(s1)), one_(tasks(scale(qf, 0, False)))]
        sk = 4.244

        def wave(ls):
            body = sorted((i * sk + g, i, g) for i in range(len(ls) - 1) for g in range(8))
            return cat([ls[i][g] for _, i, g in body] + ls[-1])
        if not halves:
            body = sorted((i * 7.5 + g + (i == 6), i, g) for i in range(7) for g in range(16))
            return cat((p + st)[i][g] for _, i, g in body)
        qb = []
        done = lambda a: qb[0](a)
        full = wave([x[8:] for x in p + st])
        k = full.index(p[0][15][0]) + 1
        return wave([x[:8] for x in st]), full[:k] + [done] + full[k:], cat(cat(x[:8] for x in p)), qb

    def shift(hs, sl, pieces=((0, 64), (64, 64), (128, 64), (192, 64)), ss=None):
        gg = view(g_v, sl)

        def one_tile(t, r, n, a):
            lane = lax.broadcasted_iota(I32, (n, 128), 1)
            ld = lambda d: h1_v[t, pl.ds(hs * T + 8 + r + d, n), :]
            if t == 0:
                g = ld(-1)
            elif t == 1:
                g = jnp.where(lane < 32, ld(-1), ld(1))
            elif t == 2:
                g = jnp.where(lane < 64, ld(1), ld(-2))
            elif t == 3:
                g = jnp.where(lane < 96, ld(-2), ld(2))
            else:
                g = ld(2)
            if a is not None:
                g = jnp.concatenate([_tie(g[i:i + 8], a) if i % 16 == 0 else g[i:i + 8]
                                     for i in range(0, n, 8)], axis=0)
            gg[r:r + n, C(t)] = g.astype(BF16)
            return g

        def mk(ts, r, n):
            def fn(a):
                g = [one_tile(t, r, n, a) for t in ts]
                if len(ts) == 2:
                    for i, x in enumerate(_lhs_sums(*g)):
                        ss[r // 2:(r + n) // 2, C(2 * i + ts[0])] = x.astype(BF16)
            return fn
        sets = [(t,) for t in range(NT)] if ss is None else [(0, 2), (1, 3), (4,)]
        return [mk(ts, r, n) for ts in sets for r, n in pieces]

    def shift_early():
        def keep(a):
            h1_v[:, 2 * T - 32:2 * T + 8, :] = h1_v[:, 3 * T - 32:3 * T + 8, :]
        return shift(2, 0, [(r, 32) for r in range(0, T - 32, 32)], gs) + [keep]

    def ln2(xs, sl, fast=True):
        xx, nn, ss = view(x1_v, xs), view(n2_v, sl), view(n2s, sl, H) if fast else None
        f = lambda R, a: put(nn, ss, R, _ln(_tie(xx[R, :], a), True))
        ts = tasks(f, 900) if sl else tasks(f, DL, False)
        if not fast:
            return (tasks(lambda R, a: mean(6, R, _tie(xx[R, :], a))) + tasks(scale(xx, 6, True))
                    + tasks(lambda R, a: put(nn, None, R, normed(xx, 6, R, a))))
        return ts[0::2] + ts[1::2]

    def ln2_late():
        xx, nn, ss = view(x1_v, 0), view(n2_v, 0), view(n2s, 0, H)
        a_, b_ = tasks(lambda R, a: mean(6, R, _tie(xx[R, :], a))), tasks(scale(xx, 6, True))
        c_ = finish(xx, 6, nn, ss)
        return a_[:8] + b_[:8] + c_[:8]

    def resid(xs, x1s, rotate=False):
        xx, x1 = view(x_v, xs), view(x1_v, x1s)
        tie = lambda v, a: v if a is None else pltpu.bitcast(pltpu.bitcast(v, U32) | wide(a), F32)

        def f(R, a):
            r_v[R, :] = xx[R, :] + tie(x1[R, :], a) * mod_v[2]

        def move(dst, src):
            def g(R, a):
                dst[R, :] = tie(src[R, :], a)
            return tasks(g, n=8)
        if not rotate:
            return tasks(f, n=8)
        return cat(zip(tasks(f, n=8), move(view(hb_v, 1), hb_v), move(xx, x_v)))

    KD, KF, ND = [(0, 2), (1, 3)], [(2 * i, 2 * i + 1) for i in range(7)], [(1, 2), (3, 4)]
    Wt = {1: (lambda k, n: w1_v[C(k), C(n)], lambda i, kp, j: w1s[C(kp), C(2 * i + j)], False, KD, [4]),
          2: (lambda k, n: w2_v[C(k), C(n)], lambda i, kp, j: w2s[C(kp), C(2 * i + j)], False, KD, [4]),
          0: (lambda k, n: w3_v[C(n), C(k)], None, True, KD, [4]),
          3: (lambda k, n: w3n[C(k), C(n)], lambda i, kp, j: w3s[C(kp), C(6 * i + j)], False, KD, [4]),
          4: (lambda k, n: w4_v[C(k), C(n)], lambda i, kp, j: w4s[C(kp), C(2 * i + j)], False, KF, [])}

    def sums_task(load, store, left):
        def fn(a):
            b = [[load(u, v) for v in range(2)] for u in range(2)]
            b[0][0], b[1][1] = _tie(b[0][0], a), _tie(b[1][1], a)
            (x11, x12), (x21, x22) = [[pltpu.bitcast(x, BF16).astype(F32) for x in row] for row in b]
            r = ((x11 + x22, x21 + x22, x11 + x12, x21 - x11, x12 - x22) if left else
                 (x11 + x22, x12 - x22, x21 - x11, x11 + x12, x21 + x22))
            for m, x in enumerate(r):
                store(m, x.astype(BF16))
        return fn

    def wsums(w_w, ws, rp, cp_):
        def mk(i, j, r):
            def store(m, x):
                ws[pl.ds(128 * i + r, 16), C(len(cp_) * m + j)] = x
            return sums_task(lambda u, v: w_w[pl.ds(64 * rp[i][u] + r // 2, 8), C(cp_[j][v])], store, False)
        return [mk(i, j, r) for j in range(len(cp_)) for i in range(len(rp)) for r in range(0, 128, 16)]

    def w3_turn():
        def mk(n, k):
            def fn(a):
                x = jnp.concatenate([_tie(w3_w[64 * n:64 * n + 8, C(k)], a), w3_w[64 * n + 8:64 * n + 64, C(k)]], axis=0)
                w3n[C(k), C(n)] = pltpu.bitcast(x, BF16).T
            return fn
        return [mk(n, k) for n in range(FT - 1) for k in range(NT)]

    def plain(name, w, lhs, n, R, epi, cost):
        tile, _, nt, kp, kl = Wt[w]
        ks = sorted([k for p in kp for k in p] + kl)
        rows_ = R.stop - R.start
        return Unit(name, [(lambda k=k: (lhs[R, C(k)], tile(k, n))) for k in ks], lambda p: epi(n, R, p[0]),
                    rows_, rows_ // 8 * (len(ks) - 1), nt=nt, acc=True, tail=rows_ // 8 * cost(n))

    def quad(name, w, lhs, sums, j, cols_, R, epi, cost):
        tile, wsum, nt, kp, kl = Wt[w] if isinstance(w, int) else w
        h, S2, c = len(kp), slice(R.start // 2, R.stop // 2), {}
        a_ = lambda i, k: _top(lhs(k) if callable(lhs) else lhs[R, C(k)], i)
        s_ = sums if callable(sums) else (lambda i, p: sums[S2, C(h * i + p)])
        prod = lambda fa_, fb_: [(lambda p=p: (fa_(p), fb_(p))) for p in range(h)]
        left = lambda i, n: [(lambda k=k: (a_(i, k), tile(k, n))) for k in kl]
        mk = lambda tiles, f, x=0: Unit(name, tiles, lambda p: f(p[0]), 64, 8 * len(tiles), nt=nt, acc=True, tail=x)

        def e1(m):
            u7.res, u6.res = [m], [m]

        def e4(m):
            c[11], c[21] = c[11] + m, m

        def e2(m):
            c[21], c[22] = c[21] + m, c[22] - m
            l21.res = [c[21]]

        def e5(m):
            c[12] = m
            epi(cols_[0], R, _zip(c[11] - m, c[21]))

        def e3(m):
            l12.res, c[22] = [c[12] + m], c[22] + m
            if not kl:
                l12.epi(l12.res)
        u1 = mk(prod(lambda p: s_(0, p), lambda p: wsum(0, p, j)), e1)
        u7 = mk(prod(lambda p: s_(4, p), lambda p: wsum(4, p, j)) + left(0, cols_[0]), lambda m: c.update({11: m}))
        u6 = mk(prod(lambda p: s_(3, p), lambda p: wsum(3, p, j)) + left(1, cols_[1]), lambda m: c.update({22: m}))
        u4 = mk(prod(lambda p: a_(1, kp[p][1]), lambda p: wsum(2, p, j)), e4)
        u2 = mk(prod(lambda p: s_(1, p), lambda p: tile(kp[p][0], cols_[0])), e2, 8)
        l21 = mk(left(1, cols_[0]), lambda m: c.update({21: m}))
        u5 = mk(prod(lambda p: s_(2, p), lambda p: tile(kp[p][1], cols_[1])), e5, 16 * cost(cols_[0]))
        u3 = mk(prod(lambda p: a_(0, kp[p][0]), lambda p: wsum(1, p, j)), e3, 8 if kl else 8 + 16 * cost(cols_[1]))
        l12 = mk(left(0, cols_[1]), lambda m: epi(cols_[1], R, _zip(m, c[22])), 16 * cost(cols_[1]))
        return [u1, u7, u6, u4, u2, l21, u5, u3, l12]

    LH, RH = [0, 4, 3, (1, 1), 1, 2, (0, 0)], [0, 4, 3, 2, (0, 0), (1, 1), 1]
    L2 = {3: (w3n_w, ws_w[2], w3t, KF[:6], n2t), 4: (w4_w, ws_w[3], w4t, ND, a_t)}

    def wsums2(w):
        w_w, s_w, ws2, cp_, _ = L2[w]
        kp, nj = Wt[w][3], len(cp_)

        def mk(o, p2, j2, r):
            def load(u, v):
                p, j, y = 2 * p2 + u, 2 * j2 + v, RH[o]
                if isinstance(y, int):
                    return s_w[pl.ds(64 * p + r // 2, 8), C(nj * y + j)]
                return w_w[pl.ds(64 * kp[p][y[0]] + r // 2, 8), C(cp_[j][y[1]])]

            def store(m, x):
                ws2[pl.ds(128 * p2 + r, 16), C((5 * o + m) * (nj // 2) + j2)] = x
            return sums_task(load, store, False)
        return [mk(o, p2, j2, r) for j2 in range(nj // 2) for o in range(7) for p2 in range(len(kp) // 2)
                for r in range(0, 128, 16)]

    def wsums4():
        form = [((0, 0), (1, 1), 1), ((0, 1), (1, 1), -1), ((1, 0), (0, 0), -1), ((0, 0), (0, 1), 1), ((1, 0), (1, 1), 1)]

        def mk(o, p2, r):
            def fn(a):
                def blk(p, j, uv, t):
                    x = w4_w[pl.ds(64 * KF[p][uv[0]] + r // 2, 8), C(ND[j][uv[1]])]
                    return pltpu.bitcast(_tie(x, t), BF16).astype(F32)
                y = {}
                for u in range(2):
                    for j in range(2):
                        p = 2 * p2 + u
                        if isinstance(RH[o], int):
                            f = form[RH[o]]
                            x1, x2 = blk(p, j, f[0], a), blk(p, j, f[1], None)
                            y[u, j] = x1 + x2 if f[2] > 0 else x1 - x2
                            w4s[pl.ds(128 * p + r, 16), C(2 * RH[o] + j)] = y[u, j].astype(BF16)
                        else:
                            y[u, j] = blk(p, j, RH[o], a if u == j else None)
                for m, f in enumerate(form):
                    x = y[f[0]] + y[f[1]] if f[2] > 0 else y[f[0]] - y[f[1]]
                    w4t[pl.ds(128 * p2 + r, 16), C(5 * o + m)] = x.astype(BF16)
            return fn
        last = wsums(w4_w, w4s, KF, ND)
        return (last[48:56] + last[104:112]
                + [mk(o, p2, r) for o in range(7) for p2 in range(3) for r in range(0, 128, 16)])

    def lsums2(w, lhs_w, sums_w, sl):
        kp, xs2 = Wt[w][3], L2[w][4]
        h2 = len(kp) // 2

        def mk(o, p2, g):
            def load(u, v):
                p, ch, x = 2 * p2 + v, 2 * g + u, LH[o]
                if isinstance(x, int):
                    return sums_w[pl.ds(64 * sl + 8 * ch, 8), C(len(kp) * x + p)]
                return lhs_w[pl.ds(H * sl + 16 * ch + 8 * x[0], 8), C(kp[p][x[1]])]

            def store(m, x):
                xs2[pl.ds(16 * g, 16), C((5 * o + m) * h2 + p2)] = x
            return sums_task(load, store, True)
        return [[mk(o, p2, g) for o in range(7) for g in range(4)] for p2 in range(h2)]

    def quad2(name, w, lhs, sums, j2, epi, cost):
        tile, wsum, nt, kp, kl = Wt[w]
        ws2, cp_, xs2 = L2[w][2:]
        h, h2, nj2, c, R = len(kp), len(kp) // 2, len(cp_) // 2, {}, slice(0, T)

        b0 = 8 * (j2 if kl else 3)
        slot = lambda j, i, v: C(b0 + 4 * (j % 2) + 2 * (i - 1) + v)

        def upd(o, j, m):
            val = {}
            for i, v, sg in (((1, 0, 1), (2, 1, 1)), ((1, 0, 1),), ((2, 1, 1),), ((1, 0, 1), (2, 0, 1)),
                             ((2, 0, 1), (2, 1, -1)), ((1, 0, -1), (1, 1, 1)), ((1, 1, 1), (2, 1, 1)))[o]:
                k = (j, i, v)
                if o == 0 and i == 1:
                    c[k] = slot(j, 2, 1)
                    continue
                val[i, v] = m if k not in c else (cb_v[:, c[k]] + m if sg > 0 else cb_v[:, c[k]] - m)
                c[k] = slot(*k)
                if kl or (o, v) not in ((4, 0), (5, 0), (6, 1)):
                    cb_v[:, c[k]] = val[i, v]
                else:
                    for r in range(0, H, 16):
                        epi(cp_[j][v], slice(2 * r + 16 * i - 16, 2 * r + 16 * i), val[i, v][r:r + 16],
                            r == H - 16 and (o, i) in ((5, 1), (6, 2)))

        def inner(o):
            x, y = LH[o], RH[o]
            xo = ((lambda p: sums[:, C(h * x + p)]) if isinstance(x, int)
                  else (lambda p: _top(lhs[:, C(kp[p][x[1]])], x[0])))
            yo = ((lambda p, j: wsum(y, p, j)) if isinstance(y, int)
                  else (lambda p, j: tile(kp[p][y[0]], cp_[j][y[1]])))
            w_ = (yo, lambda m, p2, _: ws2[C(p2), C((5 * o + m) * nj2 + j2)], nt,
                  [(2 * i, 2 * i + 1) for i in range(h2)], list(range(2 * h2, h)))
            return quad(name, w_, xo, lambda m, p2: xs2[:, C((5 * o + m) * h2 + p2)], 0, (2 * j2, 2 * j2 + 1),
                        HS[0], lambda j, _, m: upd(o, j, m), lambda j: 1.5 + KS + ((o // 6 + 1) * cost(0) if o >= 4 and not kl else 0))

        def rest(j, v, Q):
            return [Unit(name, [lambda: (lhs[Q, C(k)], tile(k, cp_[j][v]))],
                         lambda p: epi(cp_[j][v], Q, p[0] + _zip(*[cb_v[Q.start // 2:Q.stop // 2, c[j, i, v]] for i in (1, 2)])), 64, 8 * (cost(cp_[j][v]) + 1)) for k in kl]
        return cat(inner(o) for o in range(7)), [u for Q in QS for j in (2 * j2, 2 * j2 + 1) for v in range(2)
                                                 for u in rest(j, v, Q)]

    def mm(name, w, lhs, sums, epi, cost):
        if sums is None:
            return [[plain(name, w, lhs, n, R, epi, cost) for R in HS] for n in range(NT)]
        return [[plain(name, w, lhs, 0, R, epi, cost) for R in QS]] + [
            [u for R in HS for u in quad(name, w, lhs, sums, j, ND[j], R, epi, cost)] for j in range(2)]

    def mm1(name, hs, sl, fast=False):
        def epi(n, R, p):
            h1_v[n, pl.ds(hs * T + 8 + R.start, R.stop - R.start), :] = _gelu2(p)
        return cat(mm(name, 1, view(n1_v, sl), n1s if fast else None, epi, lambda n: 5 + KS))

    def mm2(name, sl, xs, x1s, fast=False):
        def epi(n, R, p):
            view(x1_v, x1s)[R, C(n)] = view(hb_v, xs)[R, C(n)] + p
        return cat(mm(name, 2, view(g_v, sl), gs if fast else None, epi, lambda n: 1 + KS))

    def mm3(name, sl, fast=True, host=None):
        nn, aa, ss, keep = view(n2_v, sl), view(a_v, sl), view(a_s, sl, H), {}

        def epi(n, R, p):
            g = _gelu2(p)
            aa[R, C(n)] = g.astype(BF16)
            if not fast:
                return
            if n % 2 == 0 and n < 12:
                keep[n] = g
                return
            pair = (keep.pop(n - 1), g) if n % 2 else (g, st_v[R, C(8)])
            for i, x in enumerate(_lhs_sums(*pair)):
                ss[R.start // 2:R.stop // 2, C(7 * i + n // 2)] = x.astype(BF16)

        c3 = lambda n: 5.5 + 0.5 * KS + (3.75 + 1.25 * KS if fast and (n % 2 or n == 12) else 0)

        def rem(R):
            def f(p):
                g = jnp.concatenate([_gelu2(p[0]), jnp.zeros((64, 128), F32)], axis=0).T
                aa[R, C(13)] = g.astype(BF16)
                if fast:
                    st_v[R, C(8)] = g
            return Unit(name, [(lambda k=k: (w3_v[13 * 128:F, C(k)], nn[R, C(k)])) for k in range(NT)], f, 64, 84,
                        nt=True, acc=True)
        odd = [rem(R) for R in HS] + [plain(name, 3 if fast else 0, nn, 12, R, epi, c3) for R in QS]
        if not fast:
            return odd + [plain(name, 0, nn, n, R, epi, c3) for p in KF[:6] for R in HS for n in p]
        qd = [quad2(name + "_%d" % j, 3, nn, view(n2s, sl, H), j, epi, c3) for j in range(3)]
        mid = qd[0][0] + _weave(qd[1][0], qd[0][1]) + _weave(qd[2][0], qd[1][1])
        if host is None:
            return odd[:2] + mid + _weave(odd[2:], qd[2][1])
        for u in (odd[0], odd[2], odd[3]):
            u.name = name + "h"
        return [odd[0], odd[2], odd[3], odd[1]] + mid, _weave(odd[4:] + host, qd[2][1])

    def cp_out(j, osl, L, sm, R=slice(0, T)):
        return cp(o_v.at[pl.ds(osl * T + R.start, R.stop - R.start), L],
                  o_hbm.at[pl.ds(base(j, T) + R.start, R.stop - R.start), L], sem_o.at[sm])

    out_a = lambda j: cp_out(j, 0, slice(128, D), 0)
    out_b = lambda j: cp_out(j, 0, C(0), 1)
    last = []

    def mm4(name, j, sl, osl=0, xs=None, x1s=None, fast=True):
        oo = view(o_v, osl)

        def epi(n, R, p, full=None):
            if xs is None:
                oo[R, C(n)] = (r_v[R, C(n)] + mod_v[2, 0:1, C(n)] * p).astype(BF16)
            else:
                oo[R, C(n)] = (view(x_v, xs)[R, C(n)] + mod_v[2, 0:1, C(n)]
                               * (view(x1_v, x1s)[R, C(n)] + p)).astype(BF16)
            if full is not None:
                if not full:
                    return
                R = slice(0, T)
            if osl == 2:
                last.append(cp_out(j, osl, C(n), 2, R))
                last[-1].start()
            elif R.stop == T and osl and n == NT - 1:
                last.append(cp_out(j, osl, slice(128 if osl == 3 else 0, D), 2))
                last[-1].start()
            elif R.stop == T and osl == 0 and n in (0, NT - 1):
                (out_a if n else out_b)(j).start()
        c4 = lambda n: (3 if xs is None else 4) + KS
        if fast:
            return ([plain(name, 4, view(a_v, sl), 0, R, epi, c4) for R in QS],
                    quad2(name + "q", 4, view(a_v, sl), view(a_s, sl, H), 0, epi, c4)[0])
        return mm(name, 4, view(a_v, sl), None, epi, c4)

    def split(us):
        n = 4 // len(us)
        m, mks, st = us[0].rows // n, [u.tiles.pop(0) for u in us], {}

        def piece(i, k):
            if i not in st:
                st[i] = mks[i]()
            return st[i][0][m * k:m * (k + 1)], st[i][1]

        def epi(p):
            for i, u in enumerate(us):
                u.res = [jnp.concatenate(p[n * i:n * (i + 1)], axis=0)]
        return _flat([Unit(us[0].name, [(lambda i=i, k=k: piece(i, k)) for i in range(len(us)) for k in range(n)],
                           epi, m, 0, nt=us[0].nt)])

    W = lambda nm: [("wait", nm)]
    run = lambda fns: [("run", "run", lambda: [fn(None) for fn in fns])]
    one = lambda us: [_flat([u]) for u in us]
    nm = lambda x: (lambda n: x)

    seq, grp = [], []
    for s in range(NC):
        seq += W("c%d" % s) + _flat(mmK(s) + mmU(nm("U%d" % s), s % 2, NC - 1 - s))
        grp.append(Group("kv%d" % s, cat(kv(s, s % 2)), 50, ["c%d" % s], ["U%d" % s], 100))
    inv = [mmI(lambda n: "I%d" % n, s, s) for s in range(NC)]
    seq += W("c3") + _flat(mmK(3) + mmK(4) + [inv[s][t] for t in range(NT) for s in range(NC)])
    macs = [mac(s + 1, NC - 1 - s, s) for s in range(NC)]
    grp.append(Group("mac00", macs[0][0], 12, ["c1"], ["c2"], 0))
    grp.append(Group("mac01", macs[1][0] + macs[0][1] + macs[1][1], 16, ["c2"], ["c3"], 0))
    for t in range(NT):
        grp.append(Group("mac%d" % t, cat(macs[s][t] for s in range(2 if t < 2 else 0, NC)), 24 if t < 2 else 18,
                         ["c3", "K%d" % t], ["I%d" % t], 100, 150))
    start = lambda cs: [("run", "run", lambda: [c.start() for c in cs])]
    f0, f1 = front(0, 2, True), front(1, 1, True)
    seq += run(ahead(0))
    seq += W("wma") + _flat(mod("moda", 0, 3)) + run(f0[0] + f1[0] + ahead(1))
    seq += W("wmb") + start(next_kv(NC) + next_q(NC)) + _flat(mod("modb", 3, 5)) + run(f0[1])
    w1 = _flat(mm1("w1_0", 0, 0) + mm1("w1_1", 1, 1))
    seq += W("w1") + w1[:72] + W("w2") + w1[72:] + run(shift(0, 0))
    w20 = mm2("w2_0", 0, 2, 1)
    q = split(w20[-2:])
    _mix(seq, _flat(w20), [q], 0.3)
    late = lambda w: w[0:3] + w[4:13] + w[22:31] + w[3:4] + w[13:22] + w[31:]
    seq += _flat(mm1("w1_2", 2, 2, True)) + run(shift(1, 1, ((T - 32, 32),), gs)) + _flat(late(mm2("w2_1", 1, 1, 0, True)))
    grp.append(Group("sh1", shift(1, 1, [(r, 32) for r in range(0, T - 32, 32)], gs), 22 + 7 * KS, ["w1_1"], ["w2_1"], 200))
    grp.append(Group("f1", f1[1], 80, ["w1"], ["w1_1"], 450))
    grp.append(Group("f2", front(2, 0), 52, ["w2"], ["w1_2"], 200))
    grp.append(Group("ln2_0", ln2(1, 0, False), 33, ["w2_0"], ["w3"], 100))
    grp.append(Group("ahead", cat(ahead(i) for i in range(2, NB - NC)), 19 + 2 * KS, ["w1"], ["end"], 100))
    grp.append(Group("ws1", wsums(w1_w, w1s, KD, ND), 26 + 5 * KS, ["w1"], ["w1_2"], 200))
    grp.append(Group("ws2", wsums(w2_w, w2s, KD, ND), 26 + 5 * KS, ["w2"], ["w2_1"], 200))
    grp.append(Group("ws3", w3_turn() + wsums(w3n_w, w3s, KD, KF[:6]) + wsums2(3), 22 + 5.5 * KS, ["w3"], ["end"], 100))
    grp.append(Group("ws4", wsums4(), 40 + 8 * KS, ["w4"], ["end"], 60))
    _wait(seq, "w3", back=1)
    w3 = mm3("w3_0", 0, False)
    _mix(seq, _flat(w3[6:]), [split(w3[4:6]) + _flat(w3[:6])], 0.1)
    mc = mod("modc", 5, 6)
    mc = _flat(mc[1:] + mc[:1])
    _wait(seq, "w4", mc[:5] + [("sync", "run", lambda: None)])
    w4 = cat(mm4("w4_0", 0, 0, 3, 2, 1, False)[1:])
    qs = [split([w4[-1 - i]]) for i in range(_phase(seq))]
    _mix(seq, _flat(w4), [mc[i:i + 4] for i in range(5, 25, 4)] + qs, 0.01, 0.4)
    assert _phase(seq) == 0
    grp.append(Group("resid", resid(2, 1), 16 + 5 * KS, ["modc"], ["end"], 100))
    grp.append(Group("ln2a", ln2_late(), 40, ["w3_0"], ["end"], 100))
    _emit(seq, grp, zero, wait)

    def step(s, carry):
        for c in next_kv(s) + next_q(s):
            c.wait()
        nxt = jnp.minimum(s + 1, NB - 1)
        seq, grp = [], []
        us, it = one(mmU(lambda n: "U%d" % n, 0, 0)), one(mmI(lambda n: "I%d" % n, 0, 0))
        w4, w4c = mm4("w4", s - 2, 0)[1], mm4("w4c", s - 3, 0)[0]
        w2 = late(mm2("w2", 0, 1, 0, True))
        for u in w2[:21]:
            u.name = "w2a"
        w2[0].name = "w2f"
        w3, w3e = mm3("w3", 0, host=w2[:4])
        _mix(seq, _flat(w4c + w3),
             [us[0], us[1], us[2], it[0] + us[3], it[1] + us[4], it[2], it[3], it[4]],
             0.19, 0.531)
        w1a, w1b = mm1("w1a", 2, 0, True), mm1("w1b", 2, 0, True)
        w1a, w1b = _flat(w1a[0:2] + w1a[4:13] + w1a[22:31]), _flat(w1b[2:4] + w1b[13:22] + w1b[31:])
        kw = 9 * 4
        w4[kw - 9].name = "w4m"
        seq += _flat(w3e + w2[4:21] + w4[:kw]) + w1a + run(shift(1, 0, ((T - 32, 32),), gs))
        seq += _flat(w4[kw:] + w2[21:]) + w1b
        assert _phase(seq) == 0
        kvs, macs = kv(0, 0), mac(1, 0, 0, part=True)
        for t in range(NT):
            grp.append(Group("kv%d" % t, kvs[t], 50 + 2 * KS, ["start"], ["U%d" % t], 290))
            grp.append(Group("mac%d" % t, macs[t], 24 + 2 * KS, ["U%d" % t], ["I%d" % t], 270, 150))
        iall = ["I%d" % t for t in range(NT)]
        ln = ln2(0, 0)
        grp.append(Group("ln2a", ln2_late(), 35, ["w2a", "w4q"], ["end"], 60, 450))
        xn = lsums2(3, n2_w, as_w[2], 0)[0]
        grp.append(Group("ln2b", ln[4:8] + ln[12:16], 78 + 20 * KS, ["start"], ["w3h"], 450))
        grp.append(Group("xna", [f for i, f in enumerate(xn) if i % 4 < 2], 26 + 5 * KS, ["start"], ["w3_0"], 150))
        grp.append(Group("xnb", [f for i, f in enumerate(xn) if i % 4 >= 2], 26 + 5 * KS, ["w4c"], ["w3_0"], 150, 0))
        grp.append(Group("resid", resid(1, 0, True), 9.5 + 5 * KS, ["w4c"], ["w2f"], 100))
        for p, ts in enumerate(lsums2(4, a_w, as_w[3], 0)):
            grp.append(Group("xa%d" % p, ts, 26 + 5 * KS, ["w3_%d" % p], ["w4q"], 150, 100))
        fr = front(0, 0, halves=True)
        grp.append(Group("fronta", fr[0], (50 + 8 * KS) * 40 / len(fr[0]), ["w2f"], ["w1a"], 290, 0))
        grp.append(Group("frontb", fr[1], (46 + 7 * KS) * 57 / len(fr[1]), ["w4m"], ["w1b"], 290, 170))
        def refill(buf, cs):
            def fn(a):
                for t in range(NT):
                    buf[t, 0:8, :] = zero if a is None else a
                for c in cs:
                    c.start()
            return fn
        fr[3].append(refill(q_n[0], next_q(nxt)))
        nk = next_kv(nxt)
        grp.append(Group("refill", [refill(k_n[0], nk[:NT]), refill(v_n[0], nk[NT:])], 10, ["U4"], ["w2f"], 0, 0))
        grp.append(Group("fq", fr[2], 33 + 7 * KS, ["w4c"], ["w2f"], 100))
        grp.append(Group("spread", spread(), 30 + 8 * KS, iall, ["end"], 60))
        grp.append(Group("shift", shift_early(), 22 + 7 * KS, ["start"], ["w2f"], 200))
        _emit(seq, grp, zero, wait)
        out_b(s - 3).wait()
        out_a(s - 2).wait()
        return carry

    lax.fori_loop(NC, NB, step, 0)

    seq, grp = [], []
    w47 = mm4("w4_7", NB - 1, 1, 2, 0, 1)
    seq += _flat(mm4("w4_5", NB - 3, 0)[0] + mm2("w2_7", 0, 0, 1, True) + mm3("w3_6", 0)
                 + cat(mm4("w4_6", NB - 2, 0, 1, 1, 0)) + mm3("w3_7", 1) + w47[0][:3] + w47[1] + w47[0][3:])
    grp.append(Group("shift7", shift(2, 0, [(r, 32) for r in range(0, T, 32)], gs), 24, ["start"], ["w2_7"], 200))
    ln = ln2(0, 0)
    grp.append(Group("ln2_6", ln[4:8] + ln[12:16], 75, ["start"], ["w3_6"], 1200))
    grp.append(Group("xn6", cat(lsums2(3, n2_w, as_w[2], 0)), 26 + 5 * KS, ["w4_5"], ["w3_6_0"], 200, 800))
    grp.append(Group("ln2_7", ln2(1, 1), 75, ["w4_6"], ["w3_7"], 1500))
    grp.append(Group("xn7", cat(lsums2(3, n2_w, as_w[2], 1)), 26 + 5 * KS, ["w4_6"], ["w3_7_0"], 200, 2100))
    for j in (6, 7):
        for p, ts in enumerate(lsums2(4, a_w, as_w[3], j - 6)):
            grp.append(Group("xa%d_%d" % (j, p), ts, 26 + 5 * KS, ["w3_%d_%d" % (j, p)], ["w4_%dq" % j], 200, 150))
    _emit(seq, grp, zero, wait)
    for c in next_kv(NB - 1) + next_q(NB - 1) + [out_b(NB - 3)] + last:
        c.wait()


@jax.jit
def pallas_adaLN_cond__ssm_conv_h3__mixer_s_mlp__prompt_kernel(
        A_q, A_k, A_v, A_shift_k, A_ssm_k, A_ssm_D, B_x, B_w1, B_w2, B_w3, B_w4, c, w_mod):
    any_ = pl.BlockSpec(memory_space=pl.ANY)
    V = pltpu.VMEM
    out = pl.pallas_call(
        kernel,
        in_specs=[any_] * 12,
        out_specs=any_,
        out_shape=jax.ShapeDtypeStruct((S, D), BF16),
        scratch_shapes=[
            [V((NT, H + 8, 128), U32)] * NC, [V((NT, H + 8, 128), U32)] * NC, [V((NT, H + 8, 128), U32)] * NC,
            [V((64, S), U32)] * NT,
            V((D // 2, D), U32), V((D // 2, D), U32), V((F // 2, D), U32), V((FT * 64, D), U32),
            [V((D // 2, 3 * D), U32), V((D // 2, 2 * D), U32), V((D // 2, D), U32)], V((4 * T, D), BF16),
            V((4, D), BF16), V((D,), BF16), V((1, D), BF16), V((8, 128), I32), pltpu.SMEM((8, 128), I32),
            V((5, 8, D), F32), V((6, 8, D), F32), V((T // 2, 4 * H), U32), V((GR // 2, 2 * T), U32),
            V((NB, 3 * T + 8, D), F32), V((NC, 3 * T + 8, D), F32), V((NB - NC, 2 * T + 8, D), F32), V((4 * T, 128), F32),
            V((T, D), U32), V((NC * T, D), U32), V((NT, NC * (T + 8) + 16, 128), F32),
            V((3 * T, D), F32), V((3 * T, D), F32), V((2 * T, D), F32), V((T, D), F32),
            V((3 * T // 2, D), U32), V((T, D), U32), V((T, D), U32), V((NT, NC * T + 24, 128), F32),
            V((T, (FT + 1) * 128), U32),
            [V((128, 11 * 128), U32)] * 2 + [V((128, 31 * 128), U32), V((448, 11 * 128), U32)],
            [V((64, 11 * 128), U32)] * 2 + [V((128, 11 * 128), U32), V((128, 35 * 128), U32)],
            V((D // 2, 13 * 128), U32), V((H, D), F32), V((T, 9 * 128), F32),
            [V((64, 105 * 128), U32), V((192, 35 * 128), U32), V((32, 35 * 128), U32), V((32, 105 * 128), U32)], V((H, 33 * 128), F32),
            pltpu.SemaphoreType.DMA((11,)), pltpu.SemaphoreType.DMA((1,)), pltpu.SemaphoreType.DMA((3,)),
        ],
        compiler_params=pltpu.CompilerParams(vmem_limit_bytes=110 << 20, disable_semaphore_checks=True,
                                             disable_bounds_checks=True),
        name="fused",
    )(A_q[0], A_k[0], A_v[0], A_shift_k.T, A_ssm_k, A_ssm_D, B_w1, B_w2, B_w3.T, B_w4, c, w_mod)
    return out[None]
```
